```python
import jax
import jax.numpy as jnp

def _softmax(x, axis=-1):
    return jax.nn.softmax(x, axis=axis)

def _gelu(x):
    return jax.nn.gelu(x, approximate=True)

def _silu(x):
    return jax.nn.silu(x)

def _sigmoid(x):
    return jax.nn.sigmoid(x)

def _layernorm(x, axis=-1, eps=1e-05):
    m = jnp.mean(x, axis=axis, keepdims=True)
    v = jnp.var(x, axis=axis, keepdims=True)
    return (x - m) / jnp.sqrt(v + eps)

def _scatter_add(tgt, idx, src, axis=0):
    return tgt.at[idx].add(src)

def _segment_sum(src, seg, n):
    return jax.ops.segment_sum(src, seg, n)

class _Rng:

    def __init__(self, key):
        self._k = key

    def _next(self):
        self._k, sub = jax.random.split(self._k)
        return sub

    def normal(self, shape):
        return jax.random.normal(self._next(), shape, dtype=jnp.bfloat16)

    def randint(self, lo, hi, shape):
        return jax.random.randint(self._next(), shape, lo, hi, dtype=jnp.int32)

    def uniform(self, shape, lo=0.0, hi=1.0):
        return jax.random.uniform(self._next(), shape, jnp.bfloat16, lo, hi)

    def permutation(self, n):
        return jax.random.permutation(self._next(), n)
kernel_name = 'interleave_layers__memory_aug_recurrent_mem_tr__spectral_gfnet__prompt'

def setup_inputs():
    _rng = _Rng(jax.random.key(int.from_bytes(__import__("os").urandom(4), "little")))
    _w = lambda a: (lambda t: t.astype(jnp.bfloat16) if jnp.issubdtype(t.dtype, jnp.floating) else t)(jnp.asarray(a))

    def _A_setup():
        B, S, Dm = (1, 2048, 640)
        H, Dh = (32, 128)
        M, seg = (8, 32)
        seg = min(seg, S)
        S = S // seg * seg
        return {'x': _w((lambda *s: _rng.normal(s) * 0.05)(B, S, Dm)), 'mem0': _w((lambda *s: _rng.normal(s) * 0.05)(B, M, Dm)), 'Wq': _w((lambda *s: _rng.normal(s) * 0.05)(Dm, H, Dh) * Dm ** (-0.5)), 'Wk': _w((lambda *s: _rng.normal(s) * 0.05)(Dm, H, Dh) * Dm ** (-0.5)), 'Wv': _w((lambda *s: _rng.normal(s) * 0.05)(Dm, H, Dh) * Dm ** (-0.5)), 'Wo': _w((lambda *s: _rng.normal(s) * 0.05)(H, Dh, Dm) * (H * Dh) ** (-0.5)), 'seg_len': seg}
    _A_in = _A_setup()

    def _B_setup():
        B, S, D = (1, 2048, 640)
        Df = D // 2 + 1
        return {'x': _w((lambda *s: _rng.normal(s) * 0.05)(B, S, D)), 'w_r': _w((lambda *s: _rng.normal(s) * 0.05)(S, Df) * 0.02), 'w_i': _w((lambda *s: _rng.normal(s) * 0.05)(S, Df) * 0.02)}
    _B_in = _B_setup()
    return {'A_x': _A_in['x'], 'A_mem0': _A_in['mem0'], 'A_Wq': _A_in['Wq'], 'A_Wk': _A_in['Wk'], 'A_Wv': _A_in['Wv'], 'A_Wo': _A_in['Wo'], 'A_seg_len': _A_in['seg_len'], 'B_x': _B_in['x'], 'B_w_r': _B_in['w_r'], 'B_w_i': _B_in['w_i']}

def reference(A_x, A_mem0, A_Wq, A_Wk, A_Wv, A_Wo, A_seg_len, B_x, B_w_r, B_w_i):

    def _A_ref(x, mem0, Wq, Wk, Wv, Wo, seg_len):
        B, S, Dm = x.shape
        H, Dh = (Wq.shape[1], Wq.shape[2])
        M = mem0.shape[1]
        scale = Dh ** (-0.5)
        n_seg = S // seg_len
        L = M + seg_len
        idx = jnp.arange(L)
        mask = (idx[:, None] < M) | (idx[:, None] >= idx[None, :])
        mem = mem0
        outs = []
        for s in range(n_seg):
            xs = x[:, s * seg_len:(s + 1) * seg_len, :].copy()
            h = jnp.concatenate([mem, xs], axis=1)
            q = jnp.einsum('btd,dhe->bhte', h, Wq)
            k = jnp.einsum('btd,dhe->bhte', h, Wk)
            v = jnp.einsum('btd,dhe->bhte', h, Wv)
            scores = jnp.einsum('bhqe,bhke->bhqk', q, k) * scale
            scores = jnp.where(mask[None, None], scores, -1000000000.0)
            p = _softmax(scores, axis=-1)
            o = jnp.einsum('bhqk,bhke->bhqe', p, v)
            o = jnp.einsum('bhte,hed->btd', o, Wo)
            mem = o[:, :M, :].copy()
            outs.append(o[:, M:, :])
        return jnp.concatenate(outs, axis=1)

    def _B_ref(x, w_r, w_i):
        B, S, D = x.shape
        X = (lambda x, axes=(-2, -1): jnp.fft.rfft2(x.astype(jnp.float32), axes=axes))(x, axes=(-2, -1))
        W = w_r + 1j * w_i
        X = X * W
        y = (lambda x, s, axes=(-2, -1): jnp.fft.irfft2(x, s=s, axes=axes).astype(jnp.bfloat16))(X, (S, D), axes=(-2, -1))
        return y
    x = A_x
    x = x + _A_ref(_layernorm(x, axis=-1), A_mem0, A_Wq, A_Wk, A_Wv, A_Wo, A_seg_len)
    x = x + _B_ref(_layernorm(x, axis=-1), B_w_r, B_w_i)
    x = x + _A_ref(_layernorm(x, axis=-1), A_mem0, A_Wq, A_Wk, A_Wv, A_Wo, A_seg_len)
    x = x + _B_ref(_layernorm(x, axis=-1), B_w_r, B_w_i)
    return x
```

```python
import functools
import math

import jax
import jax.numpy as jnp
import numpy as np
from jax import lax
import jax.experimental.pallas as pl
import jax.experimental.pallas.tpu as pltpu

f32, bf16, u32 = jnp.float32, jnp.bfloat16, jnp.uint32

S, DM, H, DH, MEM, SEG = 2048, 640, 32, 128, 8, 32
NSEG = S // SEG
NPAIR = H // 2
DF = DM // 2 + 1
EPS = 1e-5
WPITCH = 136
TPITCH = 40

C1, C2 = math.cos(2 * math.pi / 5), math.cos(4 * math.pi / 5)
S1, S2 = math.sin(2 * math.pi / 5), math.sin(4 * math.pi / 5)


def _to_bf16_bits(a):
    u = np.ascontiguousarray(a, dtype=np.float32).view(np.uint32).astype(np.uint64)
    return ((u + 0x7FFF + ((u >> 16) & 1)) >> 16).astype(np.uint32)


def _pack_rows(a):
    b = _to_bf16_bits(a)
    return b[..., 0::2, :] | (b[..., 1::2, :] << 16)


@functools.lru_cache(maxsize=None)
def _tables():
    b = np.arange(128)
    l0 = np.arange(0, DF, 5)
    l1 = np.concatenate([np.arange(1, 320, 5), np.arange(4, 320, 5)])
    l2 = np.concatenate([np.arange(2, 320, 5), np.arange(3, 320, 5)])
    sg = np.concatenate([np.ones(64), -np.ones(64)])

    def th(l):
        return 2 * np.pi * ((b[:, None] * l[None, :]) % DM) / DM

    fw = np.zeros((6, 256, 128))
    t = th(l0)
    fw[0, :128, :65] = np.cos(t)
    fw[3, :128, :65] = -np.sin(t)
    for g, l in ((1, l1), (2, l2)):
        t = th(l)
        c, s = np.cos(t), np.sin(t)
        fw[g] = np.concatenate([c, -sg * s], axis=0)
        fw[3 + g] = np.concatenate([-s, -sg * c], axis=0)
    sc = 1.0 / (S * DM)
    iw = np.zeros((5, 256, 128))
    t = th(l0).T
    cl = np.full((65, 1), 2.0)
    cl[0] = cl[-1] = 1.0
    iw[0, :65] = cl * np.cos(t) * sc
    iw[0, 128:128 + 65] = -cl * np.sin(t) * sc
    for g, l in ((1, l1), (2, l2)):
        t = th(l).T
        c, s = np.cos(t), np.sin(t)
        gg = sg[:, None]
        iw[2 * g - 1] = 2 * sc * np.concatenate([c, -s], axis=0)
        iw[2 * g] = 2 * sc * np.concatenate([gg * s, gg * c], axis=0)
    perm = np.zeros((3, 384, 128))
    perm[0, l0, np.arange(65)] = 1
    perm[1, l1, np.arange(128)] = 1
    perm[2, l2, np.arange(128)] = 1
    k1 = np.arange(128)
    e = np.zeros((2, 16, 2, 256, 128))
    for k2 in range(16):
        t = 2 * np.pi * (((16 * k1[:, None] + k2) * b[None, :]) % S) / S
        er, ei = np.cos(t), -np.sin(t)
        m = np.block([[er, -ei], [ei, er]])
        for d, mm in enumerate((m, m.T)):
            e[d, k2, 0] = mm[:, :128]
            e[d, k2, 1] = mm[:, 128:]
    small = np.concatenate(
        [_pack_rows(fw).reshape(-1, 128), _pack_rows(iw).reshape(-1, 128),
         _pack_rows(perm).reshape(-1, 128)], axis=0)
    return small, _pack_rows(e).reshape(64, 128, 128)


FW_OFF, IW_OFF, PERM_OFF = 0, 6 * 128, 11 * 128
SMALL_ROWS = 11 * 128 + 3 * 192


def _bf(x):
    return pltpu.bitcast(x, bf16)


def _dot(a, b):
    return jnp.dot(a, b, preferred_element_type=f32)


def _round_bf16(x):
    return x.astype(bf16).astype(f32)


def _layernorm(x):
    m = jnp.mean(x, axis=-1, keepdims=True)
    xc = x - m
    v = jnp.mean(xc * xc, axis=-1, keepdims=True)
    return xc * lax.rsqrt(v + EPS)


def _fft4(x, sign):
    (ar, ai), (br, bi), (cr, ci), (dr, di) = x
    t0r, t0i, t1r, t1i = ar + cr, ai + ci, ar - cr, ai - ci
    t2r, t2i, t3r, t3i = br + dr, bi + di, br - dr, bi - di
    y0, y2 = (t0r + t2r, t0i + t2i), (t0r - t2r, t0i - t2i)
    p, q = (t1r + t3i, t1i - t3r), (t1r - t3i, t1i + t3r)
    return [y0, p, y2, q] if sign < 0 else [y0, q, y2, p]


def _twiddle16(z, n, sign):
    zr, zi = z
    n = n % 16
    if n == 0:
        return z
    if n == 4:
        return (-zi, zr) if sign > 0 else (zi, -zr)
    c, s = math.cos(2 * math.pi * n / 16), sign * math.sin(2 * math.pi * n / 16)
    if n % 4 == 2:
        a, d = zr + zi, zr - zi
        if c * s > 0:
            return (d * c, a * c)
        return (a * c, d * s)
    return (zr * c - zi * s, zr * s + zi * c)


def _fft16(x, sign):
    cols = [_fft4([x[4 * j + r] for j in range(4)], sign) for r in range(4)]
    out = [None] * 16
    for q in range(4):
        y = _fft4([_twiddle16(cols[r][q], r * q, sign) for r in range(4)], sign)
        for p in range(4):
            out[q + 4 * p] = y[p]
    return out


def _kernel(x_hbm, mem_ref, wq_hbm, wk_hbm, wv_hbm, wo_hbm, wr_hbm, wi_hbm,
            small_hbm, e_hbm, out_ref,
            xin, xres, xn, ao, raw, wo_raw, tmp, w32, wo32, qb, kvl, ol, z, wf,
            wri, small, emat, fill_ref, sem):
    cp_x = pltpu.make_async_copy(x_hbm, xin, sem.at[0])
    cp_w = [pltpu.make_async_copy(h, raw.at[m], sem.at[1 + m])
            for m, h in enumerate((wq_hbm, wk_hbm, wv_hbm))]
    cp_wo = [pltpu.make_async_copy(wo_hbm.at[:, pl.ds(128 * j, 128)], wo_raw.at[j], sem.at[4 + j])
             for j in range(5)]
    cp_f = [pltpu.make_async_copy(h, wri.at[m], sem.at[9 + m])
            for m, h in enumerate((wr_hbm, wi_hbm))]
    cp_small = pltpu.make_async_copy(small_hbm, small, sem.at[11])
    cp_e = pltpu.make_async_copy(e_hbm, emat, sem.at[12])
    cp_x.start()
    cp_w[0].start()

    r = lax.broadcasted_iota(jnp.int32, (80, 80), 0)
    c = lax.broadcasted_iota(jnp.int32, (80, 80), 1)
    same = (r >= 40) == (c >= 40)
    rr = jnp.where(r >= 40, r - 40, r)
    cc = jnp.where(c >= 40, c - 40, c)
    ok = (rr < MEM) | (rr >= cc)
    fill_ref[...] = jnp.where(same, jnp.where(ok, 0.0, -1e9), -jnp.inf).astype(f32)
    ol[...] = jnp.zeros_like(ol)

    cp_x.wait()
    cp_w[1].start()

    def ln0(i, carry):
        rows = pl.ds(pl.multiple_of(i * 64, 64), 64)
        x = xin[rows, :].astype(f32)
        xres[rows, :] = x
        xn[rows, :] = _layernorm(x)
        return carry
    lax.fori_loop(0, S // 64, ln0, 0)

    def relayout(m):
        def p1(i, carry):
            for u in range(4):
                rw = i * 4 + u
                blk = pltpu.bitcast(raw[m, pl.ds(pl.multiple_of(rw * 64, 64), 64), :], u32)
                a, b = blk[0:16], blk[16:32]
                base = pl.multiple_of(rw * TPITCH, 8)
                tmp[pl.ds(base, 16), :] = (a & 0xFFFF) | (b << 16)
                tmp[pl.ds(base + 16, 16), :] = (a >> 16) | (b & jnp.uint32(0xFFFF0000))
            return carry
        lax.fori_loop(0, 80, p1, 0)

        def p2(i, carry):
            sub = tmp.at[pl.ds(pl.multiple_of(i * 8 * TPITCH, 8), 8 * TPITCH)]
            rows = pl.ds(pl.multiple_of(i * 8, 8), 8)
            for j in range(NPAIR):
                for e in range(2):
                    w32[6 * j + 2 * m + e, rows, :] = sub[pl.ds(16 * e + j, 8, stride=TPITCH), :]
            return carry
        lax.fori_loop(0, 40, p2, 0)

    cp_w[0].wait()
    cp_w[2].start()
    relayout(0)
    cp_w[1].wait()
    for cp in cp_wo:
        cp.start()
    relayout(1)
    cp_w[2].wait()
    for cp in cp_f:
        cp.start()
    cp_small.start()
    cp_e.start()
    relayout(2)
    for cp in cp_wo:
        cp.wait()

    def wo_copy(i, carry):
        for j in range(5):
            wo32[j, pl.ds(pl.multiple_of(i * 64, 64), 64), :] = pltpu.bitcast(
                wo_raw[j, pl.ds(pl.multiple_of(i * 128, 128), 128), :], u32)
        return carry
    lax.fori_loop(0, 32, wo_copy, 0)

    for cp in cp_f:
        cp.wait()
    cp_small.wait()
    cp_e.wait()

    def wperm(i, carry):
        rows = pl.ds(pl.multiple_of(i * 128, 128), 128)
        for m in range(2):
            w = wri[m, rows, :]
            for g in range(3):
                p = _bf(small[PERM_OFF + 192 * g:PERM_OFF + 192 * (g + 1), :])[:DF]
                y = _dot(w, p)
                sub = wf.at[3 * m + g, pl.ds(pl.multiple_of(i * 8, 8), 15 * WPITCH + 8)]
                for k in range(8):
                    for hf in range(2):
                        sub[pl.ds(k + 8 * hf * WPITCH, 8, stride=WPITCH), :] = y[16 * k + 8 * hf:16 * k + 8 * hf + 8]
        return carry
    lax.fori_loop(0, 16, wperm, 0)

    scale = DH ** -0.5

    def tail_rows(g):
        return [pl.ds(pl.multiple_of(g * 128 + 32 * u + 24, 8), 8) for u in range(4)]

    def out_proj(p, oo, acc):
        res = [_dot(oo, _bf(wo32[j, pl.ds(pl.multiple_of(128 * p, 128), 128), :])) for j in range(5)]
        if acc is None:
            return res
        return [a + b for a, b in zip(acc, res)]

    def layer(_, carry0):
        def qbatch(i, carry):
            hl = jnp.concatenate(
                [xn[rw, :] for gg in range(4) for rw in tail_rows(i * 4 + gg)], axis=0).astype(bf16)
            rows = pl.ds(pl.multiple_of(i * 128, 128), 128)
            for hh in range(H):
                qb[hh, rows, :] = _dot(hl, _bf(w32[6 * (hh // 2) + hh % 2]))
            return carry
        lax.fori_loop(0, 4, qbatch, 0)
        hl0 = jnp.concatenate([xn[rw, :] for rw in tail_rows(0)], axis=0).astype(bf16)
        for p in range(NPAIR):
            for jj in range(4):
                kvl[0, 4 * p + jj] = _dot(hl0, _bf(w32[6 * p + 2 + jj]))

        def step(s, mem):
            base = pl.multiple_of(s * SEG, SEG)
            g = s // 4
            ph = s % 4
            b8 = pl.ds(pl.multiple_of(ph * 8, 8), 8)
            s8 = pl.ds(pl.multiple_of(s * 8, 8), 8)
            cur = g % 2
            oth = 1 - cur
            h = jnp.concatenate([mem, xn[pl.ds(base, 24), :]], axis=0).astype(bf16)

            def proj(p):
                outs = []
                for m in range(3):
                    parts = []
                    for e in range(2):
                        parts.append(_dot(h, _bf(w32[6 * p + 2 * m + e])))
                        if m == 0:
                            parts.append(qb[2 * p + e, s8, :])
                        else:
                            parts.append(kvl[cur, 4 * p + 2 * (m - 1) + e, b8, :])
                    outs.append(jnp.concatenate(parts, axis=0).astype(bf16))
                return outs

            def scores(q, k):
                sc = lax.dot_general(q, k, (((1,), (1,)), ((), ())), preferred_element_type=f32)
                fill = fill_ref[...]
                sc = jnp.where(fill == 0.0, sc * scale, fill)
                mx = jnp.max(sc, axis=-1, keepdims=True)
                e = jnp.exp(sc - mx)
                return e.astype(bf16), 1.0 / jnp.sum(e, axis=-1, keepdims=True)

            def pv(p, prl, v):
                pr, rl = prl
                o = _dot(pr, v) * rl
                ol[cur, 2 * p, b8, :] = o[32:40]
                ol[cur, 2 * p + 1, b8, :] = o[72:80]
                return jnp.concatenate([o[0:32], o[40:72]], axis=1).astype(bf16)

            gn = jnp.minimum(g + 1, 15)
            gp = jnp.maximum(g - 1, 0)
            st = {}

            def filler(i):
                if i == 0:
                    st["hl"] = jnp.concatenate([xn[rw, :] for rw in tail_rows(gn)], axis=0).astype(bf16)
                    st["acc"] = None
                p = ph * 4 + i
                for jj in range(4):
                    kvl[oth, 4 * p + jj] = _dot(st["hl"], _bf(w32[6 * p + 2 + jj]))
                oo = jnp.concatenate([ol[oth, 2 * p], ol[oth, 2 * p + 1]], axis=1).astype(bf16)
                st["acc"] = out_proj(p, oo, st["acc"])
                if i == 3:
                    out = jnp.concatenate(st["acc"], axis=1)
                    for u, rw in enumerate(tail_rows(gp)):
                        prev = jnp.where(ph == 0, 0.0, ao[rw, :])
                        ao[rw, :] = prev + out[8 * u:8 * u + 8]

            d1, d2, d3 = 1, 3, 4
            acc = None
            qkv, prs, oos = {}, {}, {}
            for t in range(NPAIR + 4):
                if t < NPAIR:
                    qkv[t] = proj(t)
                else:
                    filler(t - NPAIR)
                if 0 <= t - d1 < NPAIR:
                    prs[t - d1] = scores(qkv[t - d1][0], qkv[t - d1][1])
                if 0 <= t - d2 < NPAIR:
                    oos[t - d2] = pv(t - d2, prs[t - d2], qkv[t - d2][2])
                if 0 <= t - d3 < NPAIR:
                    acc = out_proj(t - d3, oos[t - d3], acc)
            out = jnp.concatenate(acc, axis=1)
            ao[pl.ds(base, 24), :] = out[8:32]
            return _round_bf16(out[0:8])

        lax.fori_loop(0, NSEG, step, mem_ref[...].astype(f32))

        acc = None
        for p in range(NPAIR):
            oo = jnp.concatenate([ol[1, 2 * p], ol[1, 2 * p + 1]], axis=1).astype(bf16)
            acc = out_proj(p, oo, acc)
        out = jnp.concatenate(acc, axis=1)
        for u, rw in enumerate(tail_rows(15)):
            ao[rw, :] = out[8 * u:8 * u + 8]

        def dfwd(i, carry):
            rows = pl.ds(pl.multiple_of(i * 128, 128), 128)
            x = _round_bf16(xres[rows, :] + _round_bf16(ao[rows, :]))
            xres[rows, :] = x
            y = _round_bf16(_layernorm(x))
            x0, x1, x2, x3, x4 = [y[:, 128 * a:128 * a + 128] for a in range(5)]
            t1, t2, t3, t4 = x1 + x4, x2 + x3, x1 - x4, x2 - x3
            u0 = (x0 + t1 + t2).astype(bf16)
            u1 = jnp.concatenate([x0 + C1 * t1 + C2 * t2, S1 * t3 + S2 * t4], axis=1).astype(bf16)
            u2 = jnp.concatenate([x0 + C2 * t1 + C1 * t2, S2 * t3 - S1 * t4], axis=1).astype(bf16)
            for cidx in range(6):
                g = cidx % 3
                o = FW_OFF + 128 * cidx
                if g == 0:
                    z[cidx, rows, :] = _dot(u0, _bf(small[o:o + 64, :]))
                else:
                    z[cidx, rows, :] = _dot(u1 if g == 1 else u2, _bf(small[o:o + 128, :]))
            return carry
        lax.fori_loop(0, 16, dfwd, 0)

        def radix(sign):
            def body(i, carry):
                g = i // 16
                rb = pl.multiple_of((i % 16) * 8, 8)
                xs = [(z[g, pl.ds(rb + 128 * a, 8), :], z[g + 3, pl.ds(rb + 128 * a, 8), :])
                      for a in range(16)]
                ys = _fft16(xs, sign)
                for a in range(16):
                    z[g, pl.ds(rb + 128 * a, 8), :] = ys[a][0]
                    z[g + 3, pl.ds(rb + 128 * a, 8), :] = ys[a][1]
                return carry
            lax.fori_loop(0, 48, body, 0)

        radix(-1)

        def smid(k2, carry):
            rows = pl.ds(pl.multiple_of(k2 * 128, 128), 128)
            wrows = pl.ds(pl.multiple_of(k2 * WPITCH, 8), 128)
            ys = []
            for g in range(3):
                xx = (_dot(_bf(emat[2 * k2]), z[g, rows, :].astype(bf16))
                      + _dot(_bf(emat[2 * k2 + 1]), z[g + 3, rows, :].astype(bf16)))
                xr, xi = xx[:128], xx[128:]
                wr, wi = wf[g, wrows, :], wf[g + 3, wrows, :]
                ys.append(((xr * wr - xi * wi).astype(bf16), (xr * wi + xi * wr).astype(bf16)))
            for g in range(3):
                tt = _dot(_bf(emat[32 + 2 * k2]), ys[g][0]) + _dot(_bf(emat[33 + 2 * k2]), ys[g][1])
                z[g, rows, :] = tt[:128]
                z[g + 3, rows, :] = tt[128:]
            return carry
        lax.fori_loop(0, 16, smid, 0)

        radix(1)

        def dinv(i, carry):
            rows = pl.ds(pl.multiple_of(i * 128, 128), 128)
            tg = [jnp.concatenate([z[g, rows, :], z[g + 3, rows, :]], axis=1).astype(bf16) for g in range(3)]
            p0, p1, q1, p2, q2 = [
                _dot(tg[(j + 1) // 2], _bf(small[IW_OFF + 128 * j:IW_OFF + 128 * (j + 1), :]))
                for j in range(5)]
            e1, o1 = p0 + C1 * p1 + C2 * p2, S1 * q1 + S2 * q2
            e2, o2 = p0 + C2 * p1 + C1 * p2, S2 * q1 - S1 * q2
            y = jnp.concatenate([p0 + p1 + p2, e1 - o1, e2 - o2, e2 + o2, e1 + o1], axis=1)
            xb = (xres[rows, :] + _round_bf16(y)).astype(bf16)
            out_ref[rows, :] = xb
            x = xb.astype(f32)
            xres[rows, :] = x
            xn[rows, :] = _layernorm(x)
            return carry
        lax.fori_loop(0, 16, dinv, 0)
        return carry0

    lax.fori_loop(0, 2, layer, 0)


@functools.partial(jax.jit, static_argnames=("A_seg_len",))
def pallas_interleave_layers__memory_aug_recurrent_mem_tr__spectral_gfnet__prompt_kernel(
    A_x, A_mem0, A_Wq, A_Wk, A_Wv, A_Wo, A_seg_len, B_x, B_w_r, B_w_i,
):
    assert A_seg_len == SEG and A_x.shape == (1, S, DM)
    small, emat = _tables()
    hbm = pl.BlockSpec(memory_space=pl.ANY)
    vmem = pl.BlockSpec(memory_space=pltpu.VMEM)
    out = pl.pallas_call(
        _kernel,
        out_shape=jax.ShapeDtypeStruct((S, DM), bf16),
        in_specs=[hbm, vmem] + [hbm] * 8,
        out_specs=vmem,
        scratch_shapes=[
            pltpu.VMEM((S, DM), bf16),
            pltpu.VMEM((S, DM), f32),
            pltpu.VMEM((S, DM), f32),
            pltpu.VMEM((S, DM), f32),
            pltpu.VMEM((3, DM * H, DH), bf16),
            pltpu.VMEM((5, H * DH, 128), bf16),
            pltpu.VMEM((320 * TPITCH, 128), u32),
            pltpu.VMEM((96, 320, 128), u32),
            pltpu.VMEM((5, 2048, 128), u32),
            pltpu.VMEM((H, 512, 128), f32),
            pltpu.VMEM((2, 64, 32, 128), f32),
            pltpu.VMEM((2, H, 32, 128), f32),
            pltpu.VMEM((6, S, 128), f32),
            pltpu.VMEM((6, 16 * WPITCH, 128), f32),
            pltpu.VMEM((2, S, DF), bf16),
            pltpu.VMEM((SMALL_ROWS, 128), u32),
            pltpu.VMEM((64, 128, 128), u32),
            pltpu.VMEM((80, 80), f32),
            pltpu.SemaphoreType.DMA((13,)),
        ],
        compiler_params=pltpu.CompilerParams(vmem_limit_bytes=120 * 1024 * 1024),
    )(
        A_x.reshape(S, DM), A_mem0.reshape(MEM, DM),
        A_Wq.reshape(DM * H, DH), A_Wk.reshape(DM * H, DH), A_Wv.reshape(DM * H, DH),
        A_Wo.reshape(H * DH, DM), B_w_r, B_w_i,
        jnp.asarray(small), jnp.asarray(emat),
    )
    return out.reshape(1, S, DM)
```

```python
import functools
import math

import jax
import jax.numpy as jnp
import numpy as np
from jax import lax
import jax.experimental.pallas as pl
import jax.experimental.pallas.tpu as pltpu

f32, bf16, u32 = jnp.float32, jnp.bfloat16, jnp.uint32

S, DM, H, DH, MEM, SEG = 2048, 640, 32, 128, 8, 32
NSEG = S // SEG
NPAIR = H // 2
DF = DM // 2 + 1
EPS = 1e-5
WPITCH = 136

C1, C2 = math.cos(2 * math.pi / 5), math.cos(4 * math.pi / 5)
S1, S2 = math.sin(2 * math.pi / 5), math.sin(4 * math.pi / 5)


def _to_bf16_bits(a):
    u = np.ascontiguousarray(a, dtype=np.float32).view(np.uint32).astype(np.uint64)
    return ((u + 0x7FFF + ((u >> 16) & 1)) >> 16).astype(np.uint32)


def _pack_rows(a):
    b = _to_bf16_bits(a)
    return b[..., 0::2, :] | (b[..., 1::2, :] << 16)


@functools.lru_cache(maxsize=None)
def _tables():
    b = np.arange(128)
    l0 = np.arange(0, DF, 5)
    l1 = np.concatenate([np.arange(1, 320, 5), np.arange(4, 320, 5)])
    l2 = np.concatenate([np.arange(2, 320, 5), np.arange(3, 320, 5)])
    sg = np.concatenate([np.ones(64), -np.ones(64)])

    def th(l):
        return 2 * np.pi * ((b[:, None] * l[None, :]) % DM) / DM

    fw = np.zeros((6, 256, 128))
    t = th(l0)
    fw[0, :128, :65] = np.cos(t)
    fw[3, :128, :65] = -np.sin(t)
    for g, l in ((1, l1), (2, l2)):
        t = th(l)
        c, s = np.cos(t), np.sin(t)
        fw[g] = np.concatenate([c, -sg * s], axis=0)
        fw[3 + g] = np.concatenate([-s, -sg * c], axis=0)
    sc = 1.0 / (S * DM)
    iw = np.zeros((5, 256, 128))
    t = th(l0).T
    cl = np.full((65, 1), 2.0)
    cl[0] = cl[-1] = 1.0
    iw[0, :65] = cl * np.cos(t) * sc
    iw[0, 128:128 + 65] = -cl * np.sin(t) * sc
    for g, l in ((1, l1), (2, l2)):
        t = th(l).T
        c, s = np.cos(t), np.sin(t)
        gg = sg[:, None]
        iw[2 * g - 1] = 2 * sc * np.concatenate([c, -s], axis=0)
        iw[2 * g] = 2 * sc * np.concatenate([gg * s, gg * c], axis=0)
    k1 = np.arange(128)
    e = np.zeros((2, 16, 2, 256, 128))
    for k2 in range(16):
        t = 2 * np.pi * (((16 * k1[:, None] + k2) * b[None, :]) % S) / S
        er, ei = np.cos(t), -np.sin(t)
        m = np.block([[er, -ei], [ei, er]])
        for d, mm in enumerate((m, m.T)):
            e[d, k2, 0] = mm[:, :128]
            e[d, k2, 1] = mm[:, 128:]
    small = np.concatenate(
        [_pack_rows(fw).reshape(-1, 128), _pack_rows(iw).reshape(-1, 128)], axis=0)
    return small, _pack_rows(e).reshape(64, 128, 128)


FW_OFF, IW_OFF = 0, 6 * 128
SMALL_ROWS = 11 * 128


def _loop(name, lo, hi, body, init, **kw):
    with jax.named_scope(name):
        return lax.fori_loop(lo, hi, body, init, **kw)


def _bf(x):
    return pltpu.bitcast(x, bf16)


def _dot(a, b):
    return jnp.dot(a, b, preferred_element_type=f32)


def _round_bf16(x):
    return x.astype(bf16).astype(f32)


def _layernorm(x):
    m = jnp.mean(x, axis=-1, keepdims=True)
    xc = x - m
    v = jnp.mean(xc * xc, axis=-1, keepdims=True)
    return xc * lax.rsqrt(v + EPS)


def _fft4(x, sign):
    (ar, ai), (br, bi), (cr, ci), (dr, di) = x
    t0r, t0i, t1r, t1i = ar + cr, ai + ci, ar - cr, ai - ci
    t2r, t2i, t3r, t3i = br + dr, bi + di, br - dr, bi - di
    y0, y2 = (t0r + t2r, t0i + t2i), (t0r - t2r, t0i - t2i)
    p, q = (t1r + t3i, t1i - t3r), (t1r - t3i, t1i + t3r)
    return [y0, p, y2, q] if sign < 0 else [y0, q, y2, p]


def _twiddle16(z, n, sign):
    zr, zi = z
    n = n % 16
    if n == 0:
        return z
    if n == 4:
        return (-zi, zr) if sign > 0 else (zi, -zr)
    c, s = math.cos(2 * math.pi * n / 16), sign * math.sin(2 * math.pi * n / 16)
    if n % 4 == 2:
        a, d = zr + zi, zr - zi
        if c * s > 0:
            return (d * c, a * c)
        return (a * c, d * s)
    return (zr * c - zi * s, zr * s + zi * c)


def _fft16(x, sign):
    cols = [_fft4([x[4 * j + r] for j in range(4)], sign) for r in range(4)]
    out = [None] * 16
    for q in range(4):
        y = _fft4([_twiddle16(cols[r][q], r * q, sign) for r in range(4)], sign)
        for p in range(4):
            out[q + 4 * p] = y[p]
    return out


LAT_S, LAT_PV, LAT_WO, N_AFTER = 6, 12, 7, 8


def _interleave(main, side):
    n, k = len(main), 0
    for i, f in enumerate(main):
        f()
        while k < len(side) and (k + 1) * n <= (i + 1) * len(side):
            side[k]()
            k += 1
    for f in side[k:]:
        f()


def _kernel(x_hbm, mem_ref, wq_hbm, wk_hbm, wv_hbm, wo_hbm, wr_hbm, wi_hbm,
            small_hbm, e_hbm, out_hbm,
            xin, xa, xb, xn, ao, raw, wo_raw, tmp, w32, wo32, qb, hl, ol, z0, z1, z2, wf,
            wri, wtmp, small, emat, fill_ref, sem, osem):
    zs = (z0, z1, z2)
    w_hbm = (wq_hbm, wk_hbm, wv_hbm)

    def cp_w(m, c):
        return pltpu.make_async_copy(w_hbm[m].at[:, pl.ds(pl.multiple_of(8 * c, 8), 8), :],
                                     raw.at[4 * m + c], sem.at[4 * m + c])

    cp_xt = pltpu.make_async_copy(x_hbm.at[:, pl.ds(3, 1)], xin.at[:, pl.ds(3, 1)], sem.at[12])
    cp_xr = pltpu.make_async_copy(x_hbm.at[:, pl.ds(0, 3)], xin.at[:, pl.ds(0, 3)], sem.at[13])
    cp_wo = [pltpu.make_async_copy(wo_hbm.at[:, pl.ds(128 * j, 128)], wo_raw.at[j], sem.at[14 + j])
             for j in range(5)]
    cp_f = [pltpu.make_async_copy(h, wri.at[m], sem.at[19 + m])
            for m, h in enumerate((wr_hbm, wi_hbm))]
    cp_small = pltpu.make_async_copy(small_hbm, small, sem.at[21])
    cp_e = pltpu.make_async_copy(e_hbm, emat, sem.at[22])

    cp_xt.start()
    cp_w(0, 0).start()
    cp_w(0, 1).start()
    cp_xr.start()

    r = lax.broadcasted_iota(jnp.int32, (80, 80), 0)
    c = lax.broadcasted_iota(jnp.int32, (80, 80), 1)

    def head(i):
        return jnp.where(i < 64, i // 32, (i - 64) // 8)

    def pos(i):
        return jnp.where(i < 64, i % 32, 32 + (i - 64) % 8)

    ok = (pos(r) < MEM) | (pos(r) >= pos(c))
    fill_ref[...] = jnp.where(head(r) == head(c), jnp.where(ok, 0.0, -1e9), -jnp.inf).astype(f32)
    ol[...] = jnp.zeros_like(ol)
    ao[...] = jnp.zeros_like(ao)
    wtmp[320:328, :] = jnp.zeros((8, 128), f32)

    def chunk(bb):
        return pl.ds(pl.multiple_of(8 * bb, 8), 8)

    def set_input(bb, x, tail_u):
        xa[:, chunk(bb), :] = x.reshape(16, 8, DM)
        y = _layernorm(x)
        if tail_u is None:
            xn[:, chunk(bb), :] = y.reshape(16, 8, DM)
        else:
            yb = y.astype(bf16)
            for kt in range(5):
                hl[tail_u, kt] = pltpu.bitcast(yb[:, 128 * kt:128 * kt + 128], u32)

    def load_x(u, q):
        x = jnp.concatenate([xin[4 * a + u, q].astype(f32) for a in range(16)], axis=0)
        return x

    def body_chunk(i):
        return i + i // 3

    def relayout_thunks(m, c):
        def p1(i):
            def run():
                v = raw[4 * m + c, 80 * i:80 * i + 80].reshape(640, 128)
                tmp[320 * i:320 * i + 320, :] = pltpu.bitcast(v, u32)
            return run

        def p2(j, hf):
            def run():
                a = tmp[pl.ds(1280 * hf + j, 160, stride=8), :]
                b = tmp[pl.ds(1280 * hf + 4 + j, 160, stride=8), :]
                t = 6 * (4 * c + j) + 2 * m
                w32[t, 160 * hf:160 * hf + 160, :] = (a & 0xFFFF) | (b << 16)
                w32[t + 1, 160 * hf:160 * hf + 160, :] = (a >> 16) | (b & jnp.uint32(0xFFFF0000))
            return run
        return [p1(i) for i in range(8)] + [p2(j, hf) for hf in range(2) for j in range(4)]

    def batch_thunks(m, c):
        def one(j, u):
            def run():
                lhs = jnp.concatenate([_bf(hl[u, kt]) for kt in range(5)], axis=1)
                t = 6 * (4 * c + j) + 2 * m
                ya = _dot(lhs, _bf(w32[t])).reshape(16, 8, 128)
                yb = _dot(lhs, _bf(w32[t + 1])).reshape(16, 8, 128)
                y = jnp.concatenate([ya, yb], axis=1).reshape(256, 128).astype(bf16)
                qb[3 * (4 * c + j) + m, u] = pltpu.bitcast(y, u32)
            return run
        return [one(j, u) for j in range(4) for u in range(4)]

    def wperm_thunks(m, kc):
        def load():
            w = wri[m, :, pl.ds(pl.multiple_of(kc * 128, 128), 128)].astype(f32)
            wtmp[0:DF, :] = w

        def one(g):
            def run():
                if g == 0:
                    t = jnp.concatenate([wtmp[pl.ds(0, 64, stride=5), :], wtmp[320:328, :],
                                         jnp.zeros((56, 128), f32)], axis=0)
                else:
                    t = jnp.concatenate([wtmp[pl.ds(g, 64, stride=5), :],
                                         wtmp[pl.ds(5 - g, 64, stride=5), :]], axis=0)
                y = t.T
                sub = wf.at[3 * m + g, pl.ds(pl.multiple_of(kc * 8, 8), 15 * WPITCH + 8)]
                for k in range(8):
                    for hf in range(2):
                        sub[pl.ds(k + 8 * hf * WPITCH, 8, stride=WPITCH), :] = (
                            y[16 * k + 8 * hf:16 * k + 8 * hf + 8])
            return run
        return [load] + [one(g) for g in range(3)]

    def wo_copy_thunks(c):
        def one(j):
            def run():
                wo32[j, pl.ds(pl.multiple_of(c * 512, 512), 512), :] = pltpu.bitcast(
                    wo_raw[j, pl.ds(pl.multiple_of(c * 1024, 1024), 1024), :], u32)
            return run
        return [one(j) for j in range(5)]

    with jax.named_scope("pro0"):
        cp_xt.wait()
        for u in range(4):
            set_input(4 * u + 3, load_x(u, 3), u)
        cp_w(0, 0).wait()
        cp_w(0, 2).start()
        for f in relayout_thunks(0, 0):
            f()
        cp_xr.wait()
        cp_w(0, 3).start()

    later = {0: [cp_w(1, 0), cp_f[0]], 1: [cp_w(1, 1), cp_w(1, 2)], 2: [cp_w(1, 3), cp_w(2, 0)],
             3: [cp_w(2, 1), cp_f[1]], 4: [cp_w(2, 2), cp_w(2, 3)], 5: cp_wo[0:2], 6: cp_wo[2:5],
             7: [cp_small, cp_e]}
    with jax.named_scope("pro1"):
        for it in range(12):
            m, c = it // 4, it % 4
            side = []
            if it < 11:
                cp_w((it + 1) // 4, (it + 1) % 4).wait()
                side += relayout_thunks((it + 1) // 4, (it + 1) % 4)
            for cp in later.get(it, []):
                cp.start()
            bb = body_chunk(it)
            side.append(functools.partial(
                lambda bb: set_input(bb, load_x(bb // 4, bb % 4), None), bb))
            if it == 4:
                cp_f[0].wait()
            if it == 8:
                cp_f[1].wait()
            if it >= 4:
                for kc in range(4):
                    side += wperm_thunks(m - 1, 4 * c + kc)
            if it == 10:
                for cp in cp_wo:
                    cp.wait()
            if it >= 10:
                side += wo_copy_thunks(2 * (it - 10)) + wo_copy_thunks(2 * (it - 10) + 1)
            _interleave(batch_thunks(m, c), side)
        cp_small.wait()
        cp_e.wait()

    scale = DH ** -0.5

    def wo_dot(hh, oo):
        return [_dot(oo, _bf(wo32[j, 64 * hh:64 * hh + 64, :])) for j in range(5)]

    def addl(acc, res):
        return res if acc is None else [a + b for a, b in zip(acc, res)]

    def finish_thunks(gp, slot):
        st = {"acc": None}

        def f_wo(hh):
            def run():
                st["acc"] = addl(st["acc"], wo_dot(hh, ol[slot, hh].astype(bf16)))
                if hh == H - 1:
                    out = jnp.concatenate(st["acc"], axis=1)
                    for u in range(4):
                        ao[slot, 32 * u + 24:32 * u + 32, :] = out[8 * u:8 * u + 8]
            return run

        def pre():
            x = _round_bf16(xa[gp] + _round_bf16(ao[slot]))
            xb[gp] = x
            y = _round_bf16(_layernorm(x))
            x0, x1, x2, x3, x4 = [y[:, 128 * a:128 * a + 128] for a in range(5)]
            t1, t2, t3, t4 = x1 + x4, x2 + x3, x1 - x4, x2 - x3
            st["u"] = [
                (x0 + t1 + t2).astype(bf16),
                jnp.concatenate([x0 + C1 * t1 + C2 * t2, S1 * t3 + S2 * t4], axis=1).astype(bf16),
                jnp.concatenate([x0 + C2 * t1 + C1 * t2, S2 * t3 - S1 * t4], axis=1).astype(bf16)]

        def f_dft(cidx):
            def run():
                g = cidx % 3
                o = FW_OFF + 128 * cidx
                zs[g][cidx // 3, gp] = _dot(st["u"][g], _bf(small[o:o + (64 if g == 0 else 128), :]))
            return run
        return [f_wo(hh) for hh in range(H)], pre, [f_dft(cidx) for cidx in range(6)]

    def group(g, mem):
        cur = g % 2
        wos, pre, dfts = finish_thunks(jnp.maximum(g - 1, 0), 1 - cur)
        fillers = [wos[0:11], wos[11:22], wos[22:32], dfts]
        for ph in range(4):
            h = jnp.concatenate([mem, xn[g, 32 * ph:32 * ph + 24, :]], axis=0).astype(bf16)
            if ph == 3:
                pre()
            pr, sm, oos = {}, {}, {}

            def stacked(p, m):
                top = jnp.concatenate([pr[p, m, 0], pr[p, m, 1]], axis=0).astype(bf16)
                tail = _bf(qb[3 * p + m, ph, pl.ds(pl.multiple_of(8 * g, 8), 8), :])
                return jnp.concatenate([top, tail], axis=0)

            def scores(p):
                sc = lax.dot_general(stacked(p, 0), stacked(p, 1), (((1,), (1,)), ((), ())),
                                     preferred_element_type=f32)
                fill = fill_ref[...]
                sc = jnp.where(fill == 0.0, sc * scale, fill)
                mx = jnp.max(sc, axis=-1, keepdims=True)
                e = jnp.exp(sc - mx)
                sm[p] = (e.astype(bf16), 1.0 / jnp.sum(e, axis=-1, keepdims=True))

            def pv(p):
                e, rl = sm[p]
                o = _dot(e, stacked(p, 2)) * rl
                ol[cur, 2 * p, 8 * ph:8 * ph + 8, :] = o[64:72]
                ol[cur, 2 * p + 1, 8 * ph:8 * ph + 8, :] = o[72:80]
                oos[2 * p], oos[2 * p + 1] = o[0:32].astype(bf16), o[32:64].astype(bf16)

            acc, t, nwo = None, 0.0, 0
            bulk = [(p, m, e) for p in range(NPAIR) for m in (1, 0, 2) for e in range(2)]
            pend, ready, fl = [], [], list(fillers[ph])
            while nwo < H:
                pend.sort()
                if pend and pend[0][0] <= t:
                    _, kind, p = pend.pop(0)
                    if kind == "S":
                        scores(p)
                        pend.append((t + LAT_PV, "V", p))
                    else:
                        pv(p)
                        ready += [(t + LAT_WO, 2 * p), (t + LAT_WO, 2 * p + 1)]
                    t += 0.5
                elif bulk:
                    p, m, e = bulk.pop(0)
                    pr[p, m, e] = _dot(h, _bf(w32[6 * p + 2 * m + e]))
                    t += 1
                    if m == 0 and e == 1:
                        pend.append((t + LAT_S, "S", p))
                elif ready and ready[0][0] <= t:
                    _, hh = ready.pop(0)
                    acc = addl(acc, wo_dot(hh, oos[hh]))
                    t += 1
                    nwo += 1
                elif len(fl) > N_AFTER:
                    fl.pop(0)()
                    t += 1
                else:
                    t += 0.5
            out = jnp.concatenate(acc, axis=1)
            ao[cur, 32 * ph:32 * ph + 24, :] = out[8:32]
            mem = _round_bf16(out[0:8])
            for f in fl:
                f()
        return mem

    def radix_fwd(g, bb):
        z = zs[g]
        ys = _fft16([(z[0, a, chunk(bb), :], z[1, a, chunk(bb), :]) for a in range(16)], -1)
        for a in range(16):
            z[0, a, chunk(bb), :] = ys[a][0]
            z[1, a, chunk(bb), :] = ys[a][1]

    def spectral():
        ys = {}

        def fwd(g, k2):
            z = zs[g]
            xx = (_dot(_bf(emat[2 * k2]), z[0, k2].astype(bf16))
                  + _dot(_bf(emat[2 * k2 + 1]), z[1, k2].astype(bf16)))
            xr, xi = xx[:128], xx[128:]
            wr = wf[g, k2 * WPITCH:k2 * WPITCH + 128, :]
            wi = wf[g + 3, k2 * WPITCH:k2 * WPITCH + 128, :]
            ys[g, k2] = ((xr * wr - xi * wi).astype(bf16), (xr * wi + xi * wr).astype(bf16))

        def inv(g, k2):
            yr, yi = ys.pop((g, k2))
            tt = _dot(_bf(emat[32 + 2 * k2]), yr) + _dot(_bf(emat[33 + 2 * k2]), yi)
            zs[g][0, k2] = tt[:128]
            zs[g][1, k2] = tt[128:]

        for bb in range(16):
            radix_fwd(0, bb)
        units = [(g, k2) for g in range(3) for k2 in range(16)]
        for i in range(len(units) + 2):
            if i < len(units):
                fwd(*units[i])
            if i >= 2:
                inv(*units[i - 2])
            if i < 32:
                radix_fwd(1 + i // 16, i % 16)

    def dinv_thunks(bb, finish):
        st = {}

        def rad(g):
            def run():
                z = zs[g]
                ys = _fft16([(z[0, a, chunk(bb), :], z[1, a, chunk(bb), :]) for a in range(16)], 1)
                st[g] = jnp.concatenate(
                    [jnp.concatenate([y[0] for y in ys], axis=0),
                     jnp.concatenate([y[1] for y in ys], axis=0)], axis=1).astype(bf16)
            return run

        def mm():
            st["p"] = [_dot(st[(j + 1) // 2], _bf(small[IW_OFF + 128 * j:IW_OFF + 128 * (j + 1), :]))
                       for j in range(5)]

        def fin():
            p0, p1, q1, p2, q2 = st["p"]
            e1, o1 = p0 + C1 * p1 + C2 * p2, S1 * q1 + S2 * q2
            e2, o2 = p0 + C2 * p1 + C1 * p2, S2 * q1 - S1 * q2
            y = jnp.concatenate([p0 + p1 + p2, e1 - o1, e2 - o2, e2 + o2, e1 + o1], axis=1)
            finish(xb[:, chunk(bb), :].reshape(128, DM) + _round_bf16(y))
        return [rad(0), rad(1), rad(2), mm, fin]

    def out_copy(bb):
        u, q = bb // 4, bb % 4
        return [pltpu.make_async_copy(xin.at[4 * a + u, q], out_hbm.at[4 * a + u, q], osem.at[bb])
                for a in range(16)]

    def layer(li, carry0):
        _loop("step", 0, 16, group, mem_ref[...].astype(f32))
        with jax.named_scope("tail"):
            wos, pre, dfts = finish_thunks(15, 1)
            for f in wos + [pre] + dfts:
                f()
        with jax.named_scope("spectral"):
            spectral()

        @pl.when(li == 0)
        def _():
            with jax.named_scope("dinv_tails"):
                th = [dinv_thunks(4 * u + 3, functools.partial(
                    lambda u, x: set_input(4 * u + 3, _round_bf16(x), u), u)) for u in range(4)]
                for stage in range(5):
                    for u in range(4):
                        th[u][stage]()

            def batch(it, carry):
                bb = body_chunk(it)
                side = dinv_thunks(bb, lambda x: set_input(bb, _round_bf16(x), None))
                _interleave(batch_thunks(it // 4, it % 4), side)
                return carry
            _loop("batch", 0, 12, batch, 0)

        @pl.when(li == 1)
        def _():
            with jax.named_scope("dinv_out"):
                def store_out(bb, x):
                    xo = x.astype(bf16)
                    for a in range(16):
                        xin[4 * a + bb // 4, bb % 4] = xo[8 * a:8 * a + 8]
                    for cp in out_copy(bb):
                        cp.start()
                th = [dinv_thunks(bb, functools.partial(store_out, bb)) for bb in range(16)]
                for i in range(17):
                    if i < 16:
                        for f in th[i][:4]:
                            f()
                    if i >= 1:
                        th[i - 1][4]()
                for bb in range(16):
                    for cp in out_copy(bb):
                        cp.wait()
        return carry0

    lax.fori_loop(0, 2, layer, 0)


@functools.partial(jax.jit, static_argnames=("A_seg_len",))
def pallas_interleave_layers__memory_aug_recurrent_mem_tr__spectral_gfnet__prompt_kernel(
    A_x, A_mem0, A_Wq, A_Wk, A_Wv, A_Wo, A_seg_len, B_x, B_w_r, B_w_i,
):
    assert A_seg_len == SEG and A_x.shape == (1, S, DM)
    small, emat = _tables()
    hbm = pl.BlockSpec(memory_space=pltpu.HBM)
    vmem = pl.BlockSpec(memory_space=pltpu.VMEM)
    out = pl.pallas_call(
        _kernel,
        out_shape=jax.ShapeDtypeStruct((NSEG, 4, 8, DM), bf16),
        in_specs=[hbm, vmem] + [hbm] * 8,
        out_specs=hbm,
        scratch_shapes=[
            pltpu.VMEM((NSEG, 4, 8, DM), bf16),
            pltpu.VMEM((16, 128, DM), f32),
            pltpu.VMEM((16, 128, DM), f32),
            pltpu.VMEM((16, 128, DM), f32),
            pltpu.VMEM((2, 128, DM), f32),
            pltpu.VMEM((12, DM, 8, DH), bf16),
            pltpu.VMEM((5, H * DH, 128), bf16),
            pltpu.VMEM((2560, 128), u32),
            pltpu.VMEM((96, 320, 128), u32),
            pltpu.VMEM((5, 2048, 128), u32),
            pltpu.VMEM((48, 4, 128, 128), u32),
            pltpu.VMEM((4, 5, 64, 128), u32),
            pltpu.VMEM((2, H, 32, 128), f32),
            pltpu.VMEM((2, 16, 128, 128), f32),
            pltpu.VMEM((2, 16, 128, 128), f32),
            pltpu.VMEM((2, 16, 128, 128), f32),
            pltpu.VMEM((6, 16 * WPITCH, 128), f32),
            pltpu.VMEM((2, DF, S), bf16),
            pltpu.VMEM((328, 128), f32),
            pltpu.VMEM((SMALL_ROWS, 128), u32),
            pltpu.VMEM((64, 128, 128), u32),
            pltpu.VMEM((80, 80), f32),
            pltpu.SemaphoreType.DMA((23,)),
            pltpu.SemaphoreType.DMA((16,)),
        ],
        compiler_params=pltpu.CompilerParams(vmem_limit_bytes=120 * 1024 * 1024),
    )(
        A_x.reshape(NSEG, 4, 8, DM), A_mem0.reshape(MEM, DM),
        A_Wq, A_Wk, A_Wv, A_Wo.reshape(H * DH, DM), B_w_r.T, B_w_i.T,
        jnp.asarray(small), jnp.asarray(emat),
    )
    return out.reshape(1, S, DM)
```

```python
import functools
import math

import jax
import jax.numpy as jnp
import numpy as np
from jax import lax
import jax.experimental.pallas as pl
import jax.experimental.pallas.tpu as pltpu

f32, bf16, u32 = jnp.float32, jnp.bfloat16, jnp.uint32

S, DM, H, DH, MEM, SEG = 2048, 640, 32, 128, 8, 32
NSEG = S // SEG
NPAIR = H // 2
DF = DM // 2 + 1
EPS = 1e-5
WPITCH = 136

C1, C2 = math.cos(2 * math.pi / 5), math.cos(4 * math.pi / 5)
S1, S2 = math.sin(2 * math.pi / 5), math.sin(4 * math.pi / 5)


def _to_bf16_bits(a):
    u = np.ascontiguousarray(a, dtype=np.float32).view(np.uint32).astype(np.uint64)
    return ((u + 0x7FFF + ((u >> 16) & 1)) >> 16).astype(np.uint32)


def _pack_rows(a):
    b = _to_bf16_bits(a)
    return b[..., 0::2, :] | (b[..., 1::2, :] << 16)


@functools.lru_cache(maxsize=None)
def _tables():
    b = np.arange(128)
    l0 = np.arange(0, DF, 5)
    l1 = np.concatenate([np.arange(1, 320, 5), np.arange(4, 320, 5)])
    l2 = np.concatenate([np.arange(2, 320, 5), np.arange(3, 320, 5)])
    sg = np.concatenate([np.ones(64), -np.ones(64)])

    def th(l):
        return 2 * np.pi * ((b[:, None] * l[None, :]) % DM) / DM

    fw = np.zeros((6, 256, 128))
    t = th(l0)
    fw[0, :128, :65] = np.cos(t)
    fw[3, :128, :65] = -np.sin(t)
    for g, l in ((1, l1), (2, l2)):
        t = th(l)
        c, s = np.cos(t), np.sin(t)
        fw[g] = np.concatenate([c, -sg * s], axis=0)
        fw[3 + g] = np.concatenate([-s, -sg * c], axis=0)
    sc = 1.0 / (S * DM)
    iw = np.zeros((5, 256, 128))
    t = th(l0).T
    cl = np.full((65, 1), 2.0)
    cl[0] = cl[-1] = 1.0
    iw[0, :65] = cl * np.cos(t) * sc
    iw[0, 128:128 + 65] = -cl * np.sin(t) * sc
    for g, l in ((1, l1), (2, l2)):
        t = th(l).T
        c, s = np.cos(t), np.sin(t)
        gg = sg[:, None]
        iw[2 * g - 1] = 2 * sc * np.concatenate([c, -s], axis=0)
        iw[2 * g] = 2 * sc * np.concatenate([gg * s, gg * c], axis=0)
    k1 = np.arange(128)
    e = np.zeros((2, 16, 2, 256, 128))
    for k2 in range(16):
        t = 2 * np.pi * (((16 * k1[:, None] + k2) * b[None, :]) % S) / S
        er, ei = np.cos(t), -np.sin(t)
        m = np.block([[er, -ei], [ei, er]])
        for d, mm in enumerate((m, m.T)):
            e[d, k2, 0] = mm[:, :128]
            e[d, k2, 1] = mm[:, 128:]
    small = np.concatenate(
        [_pack_rows(fw).reshape(-1, 128), _pack_rows(iw).reshape(-1, 128)], axis=0)
    return small, _pack_rows(e).reshape(64, 128, 128)


FW_OFF, IW_OFF = 0, 6 * 128
SMALL_ROWS = 11 * 128


def _loop(name, lo, hi, body, init, **kw):
    with jax.named_scope(name):
        return lax.fori_loop(lo, hi, body, init, **kw)


def _bf(x):
    return pltpu.bitcast(x, bf16)


def _dot(a, b):
    return jnp.dot(a, b, preferred_element_type=f32)


def _round_bf16(x):
    return x.astype(bf16).astype(f32)


def _layernorm(x):
    m = jnp.mean(x, axis=-1, keepdims=True)
    xc = x - m
    v = jnp.mean(xc * xc, axis=-1, keepdims=True)
    return xc * lax.rsqrt(v + EPS)


def _fft4(x, sign):
    (ar, ai), (br, bi), (cr, ci), (dr, di) = x
    t0r, t0i, t1r, t1i = ar + cr, ai + ci, ar - cr, ai - ci
    t2r, t2i, t3r, t3i = br + dr, bi + di, br - dr, bi - di
    y0, y2 = (t0r + t2r, t0i + t2i), (t0r - t2r, t0i - t2i)
    p, q = (t1r + t3i, t1i - t3r), (t1r - t3i, t1i + t3r)
    return [y0, p, y2, q] if sign < 0 else [y0, q, y2, p]


def _twiddle16(z, n, sign):
    zr, zi = z
    n = n % 16
    if n == 0:
        return z
    if n == 4:
        return (-zi, zr) if sign > 0 else (zi, -zr)
    c, s = math.cos(2 * math.pi * n / 16), sign * math.sin(2 * math.pi * n / 16)
    if n % 4 == 2:
        a, d = zr + zi, zr - zi
        if c * s > 0:
            return (d * c, a * c)
        return (a * c, d * s)
    return (zr * c - zi * s, zr * s + zi * c)


def _fft16(x, sign):
    cols = [_fft4([x[4 * j + r] for j in range(4)], sign) for r in range(4)]
    out = [None] * 16
    for q in range(4):
        y = _fft4([_twiddle16(cols[r][q], r * q, sign) for r in range(4)], sign)
        for p in range(4):
            out[q + 4 * p] = y[p]
    return out


LAT_S, LAT_PV, LAT_WO, N_AFTER = 6, 12, 7, 8


def _interleave(main, side):
    n, k = len(main), 0
    for i, f in enumerate(main):
        f()
        while k < len(side) and (k + 1) * n <= (i + 1) * len(side):
            side[k]()
            k += 1
    for f in side[k:]:
        f()


def _kernel(x_hbm, mem_ref, wq_hbm, wk_hbm, wv_hbm, wo_hbm, wr_hbm, wi_hbm,
            small_hbm, e_hbm, out_hbm,
            xin, xa, xb, xn, ao, raw, wo_raw, tmp, w32, wo32, qb, hl, ol, z0, z1, z2, wf,
            wri, wtmp, small, emat, fill_ref, sem, osem):
    zs = (z0, z1, z2)
    w_hbm = (wq_hbm, wk_hbm, wv_hbm)

    def body_chunk(i):
        return i + i // 3

    def cp_w(i):
        src = w_hbm[i // 4 if isinstance(i, int) else 0]
        c = i % 4
        return pltpu.make_async_copy(src.at[:, pl.ds(pl.multiple_of(8 * c, 8), 8), :],
                                     raw.at[i], sem.at[i])

    def cp_x(bb):
        return pltpu.make_async_copy(x_hbm.at[:, bb], xin.at[:, bb], sem.at[12 + bb])

    def cp_wo(i):
        rows = pl.ds(pl.multiple_of(512 * i, 512), 512)
        return pltpu.make_async_copy(wo_hbm.at[rows], wo_raw.at[rows], sem.at[28 + i])

    cp_rest = [pltpu.make_async_copy(wr_hbm, wri.at[0], sem.at[36]),
               pltpu.make_async_copy(wi_hbm, wri.at[1], sem.at[37]),
               pltpu.make_async_copy(small_hbm, small, sem.at[38]),
               pltpu.make_async_copy(e_hbm, emat, sem.at[39])]

    for u in range(4):
        cp_x(4 * u + 3).start()
    cp_w(0).start()
    for i in range(12):
        if i < 11:
            cp_w(i + 1).start()
        cp_x(body_chunk(i)).start()
        if i < 8:
            cp_wo(i).start()
    for cp in cp_rest:
        cp.start()

    r = lax.broadcasted_iota(jnp.int32, (80, 80), 0)
    c = lax.broadcasted_iota(jnp.int32, (80, 80), 1)

    def head(i):
        return jnp.where(i < 64, i // 32, (i - 64) // 8)

    def pos(i):
        return jnp.where(i < 64, i % 32, 32 + (i - 64) % 8)

    ok = (pos(r) < MEM) | (pos(r) >= pos(c))
    fill_ref[...] = jnp.where(head(r) == head(c), jnp.where(ok, 0.0, -1e9), -jnp.inf).astype(f32)
    ol[...] = jnp.zeros_like(ol)
    ao[...] = jnp.zeros_like(ao)
    wtmp[320:328, :] = jnp.zeros((8, 128), f32)

    def chunk(bb):
        return pl.ds(pl.multiple_of(8 * bb, 8), 8)

    def set_input(bb, x, tail_u):
        xa[:, chunk(bb), :] = x.reshape(16, 8, DM)
        y = _layernorm(x)
        if tail_u is None:
            xn[:, chunk(bb), :] = y.reshape(16, 8, DM)
        else:
            yb = y.astype(bf16)
            for kt in range(5):
                hl[tail_u, kt] = pltpu.bitcast(yb[:, 128 * kt:128 * kt + 128], u32)

    def load_x(bb):
        return xin[:, bb].astype(f32).reshape(128, DM)

    def relayout_thunks(m, c):
        def p1(i):
            def run():
                v = raw[4 * m + c, 80 * i:80 * i + 80].reshape(640, 128)
                tmp[320 * i:320 * i + 320, :] = pltpu.bitcast(v, u32)
            return run

        def p2(j, hf):
            def run():
                a = tmp[pl.ds(1280 * hf + j, 160, stride=8), :]
                b = tmp[pl.ds(1280 * hf + 4 + j, 160, stride=8), :]
                t = 6 * (4 * c + j) + 2 * m
                w32[t, 160 * hf:160 * hf + 160, :] = (a & 0xFFFF) | (b << 16)
                w32[t + 1, 160 * hf:160 * hf + 160, :] = (a >> 16) | (b & jnp.uint32(0xFFFF0000))
            return run
        return [p1(i) for i in range(8)] + [p2(j, hf) for hf in range(2) for j in range(4)]

    def batch_thunks(m, c):
        def one(j, u):
            def run():
                lhs = jnp.concatenate([_bf(hl[u, kt]) for kt in range(5)], axis=1)
                t = 6 * (4 * c + j) + 2 * m
                ya = _dot(lhs, _bf(w32[t])).reshape(16, 8, 128)
                yb = _dot(lhs, _bf(w32[t + 1])).reshape(16, 8, 128)
                y = jnp.concatenate([ya, yb], axis=1).reshape(256, 128).astype(bf16)
                qb[3 * (4 * c + j) + m, u] = pltpu.bitcast(y, u32)
            return run
        return [one(j, u) for j in range(4) for u in range(4)]

    def wperm_thunks(m, kc):
        def load():
            w = wri[m, :, pl.ds(pl.multiple_of(kc * 128, 128), 128)].astype(f32)
            wtmp[0:DF, :] = w

        def one(g):
            def run():
                if g == 0:
                    t = jnp.concatenate([wtmp[pl.ds(0, 64, stride=5), :], wtmp[320:328, :],
                                         jnp.zeros((56, 128), f32)], axis=0)
                else:
                    t = jnp.concatenate([wtmp[pl.ds(g, 64, stride=5), :],
                                         wtmp[pl.ds(5 - g, 64, stride=5), :]], axis=0)
                y = t.T
                sub = wf.at[3 * m + g, pl.ds(pl.multiple_of(kc * 8, 8), 15 * WPITCH + 8)]
                for k in range(8):
                    for hf in range(2):
                        sub[pl.ds(k + 8 * hf * WPITCH, 8, stride=WPITCH), :] = (
                            y[16 * k + 8 * hf:16 * k + 8 * hf + 8])
            return run
        return [load] + [one(g) for g in range(3)]

    def wo_copy_thunks(c):
        def one(j):
            def run():
                wo32[j, pl.ds(pl.multiple_of(c * 256, 256), 256), :] = pltpu.bitcast(
                    wo_raw[pl.ds(pl.multiple_of(c * 512, 512), 512), 128 * j:128 * j + 128], u32)
            return run
        return [one(j) for j in range(5)]

    with jax.named_scope("pro0"):
        for u in range(4):
            cp_x(4 * u + 3).wait()
        for u in range(4):
            set_input(4 * u + 3, load_x(4 * u + 3), u)
        cp_w(0).wait()
        for f in relayout_thunks(0, 0):
            f()

    def pro1(it, carry):
        @pl.when(it < 11)
        def _():
            cp_w(it + 1).wait()

        @pl.when(it < 8)
        def _():
            cp_wo(it).wait()
        bb = body_chunk(it)
        cp_x(bb).wait()
        nxt = jnp.minimum(it + 1, 11)
        side = relayout_thunks(nxt // 4, nxt % 4)
        side += [lambda: set_input(bb, load_x(bb), None)]
        side += wo_copy_thunks(jnp.minimum(it, 7))
        _interleave(batch_thunks(it // 4, it % 4), side)
        return carry
    _loop("pro1", 0, 12, pro1, 0)
    for cp in cp_rest:
        cp.wait()

    scale = DH ** -0.5

    def wo_dot(hh, oo):
        return [_dot(oo, _bf(wo32[j, 64 * hh:64 * hh + 64, :])) for j in range(5)]

    def addl(acc, res):
        return res if acc is None else [a + b for a, b in zip(acc, res)]

    def finish_thunks(gp, slot):
        st = {"acc": None}

        def f_wo(hh):
            def run():
                st["acc"] = addl(st["acc"], wo_dot(hh, ol[slot, hh].astype(bf16)))
                if hh == H - 1:
                    out = jnp.concatenate(st["acc"], axis=1)
                    for u in range(4):
                        ao[slot, 32 * u + 24:32 * u + 32, :] = out[8 * u:8 * u + 8]
            return run

        def pre():
            x = _round_bf16(xa[gp] + _round_bf16(ao[slot]))
            xb[gp] = x
            y = _round_bf16(_layernorm(x))
            x0, x1, x2, x3, x4 = [y[:, 128 * a:128 * a + 128] for a in range(5)]
            t1, t2, t3, t4 = x1 + x4, x2 + x3, x1 - x4, x2 - x3
            st["u"] = [
                (x0 + t1 + t2).astype(bf16),
                jnp.concatenate([x0 + C1 * t1 + C2 * t2, S1 * t3 + S2 * t4], axis=1).astype(bf16),
                jnp.concatenate([x0 + C2 * t1 + C1 * t2, S2 * t3 - S1 * t4], axis=1).astype(bf16)]

        def f_dft(cidx):
            def run():
                g = cidx % 3
                o = FW_OFF + 128 * cidx
                zs[g][cidx // 3, gp] = _dot(st["u"][g], _bf(small[o:o + (64 if g == 0 else 128), :]))
            return run
        return [f_wo(hh) for hh in range(H)], pre, [f_dft(cidx) for cidx in range(6)]

    def group(g, mem):
        cur = g % 2
        wos, pre, dfts = finish_thunks(jnp.maximum(g - 1, 0), 1 - cur)
        fillers = [wos[0:11], wos[11:22], wos[22:32], dfts]
        for ph in range(4):
            h = jnp.concatenate([mem, xn[g, 32 * ph:32 * ph + 24, :]], axis=0).astype(bf16)
            if ph == 3:
                pre()
            side = wperm_thunks(ph, g) if ph < 2 else []
            pr, sm, oos = {}, {}, {}

            def stacked(p, m):
                top = jnp.concatenate([pr[p, m, 0], pr[p, m, 1]], axis=0).astype(bf16)
                tail = _bf(qb[3 * p + m, ph, pl.ds(pl.multiple_of(8 * g, 8), 8), :])
                return jnp.concatenate([top, tail], axis=0)

            def scores(p):
                sc = lax.dot_general(stacked(p, 0), stacked(p, 1), (((1,), (1,)), ((), ())),
                                     preferred_element_type=f32)
                fill = fill_ref[...]
                sc = jnp.where(fill == 0.0, sc * scale, fill)
                mx = jnp.max(sc, axis=-1, keepdims=True)
                e = jnp.exp(sc - mx)
                sm[p] = (e.astype(bf16),
                         pl.reciprocal(jnp.sum(e, axis=-1, keepdims=True), approx=True))

            def pv(p):
                e, rl = sm[p]
                o = _dot(e, stacked(p, 2)) * rl
                ol[cur, 2 * p, 8 * ph:8 * ph + 8, :] = o[64:72]
                ol[cur, 2 * p + 1, 8 * ph:8 * ph + 8, :] = o[72:80]
                oos[2 * p], oos[2 * p + 1] = o[0:32].astype(bf16), o[32:64].astype(bf16)

            acc, t, nwo = None, 0.0, 0
            bulk = [(p, m, e) for p in range(NPAIR) for m in (1, 0, 2) for e in range(2)]
            pend, ready, fl = [], [], list(fillers[ph])
            while nwo < H:
                pend.sort()
                if pend and pend[0][0] <= t:
                    _, kind, p = pend.pop(0)
                    if kind == "S":
                        scores(p)
                        pend.append((t + LAT_PV, "V", p))
                    else:
                        pv(p)
                        ready += [(t + LAT_WO, 2 * p), (t + LAT_WO, 2 * p + 1)]
                    t += 0.5
                elif bulk:
                    p, m, e = bulk.pop(0)
                    pr[p, m, e] = _dot(h, _bf(w32[6 * p + 2 * m + e]))
                    t += 1
                    if m == 0 and e == 1:
                        pend.append((t + LAT_S, "S", p))
                    if side and len(bulk) % 18 == 0:
                        side.pop(0)()
                elif ready and ready[0][0] <= t:
                    _, hh = ready.pop(0)
                    acc = addl(acc, wo_dot(hh, oos[hh]))
                    t += 1
                    nwo += 1
                elif len(fl) > N_AFTER:
                    fl.pop(0)()
                    t += 1
                else:
                    t += 0.5
            out = jnp.concatenate(acc, axis=1)
            ao[cur, 32 * ph:32 * ph + 24, :] = out[8:32]
            mem = _round_bf16(out[0:8])
            for f in fl:
                f()
        return mem

    def radix_fwd(g, bb):
        z = zs[g]
        ys = _fft16([(z[0, a, chunk(bb), :], z[1, a, chunk(bb), :]) for a in range(16)], -1)
        for a in range(16):
            z[0, a, chunk(bb), :] = ys[a][0]
            z[1, a, chunk(bb), :] = ys[a][1]

    def spectral():
        ys = {}

        def fwd(g, k2):
            z = zs[g]
            xx = (_dot(_bf(emat[2 * k2]), z[0, k2].astype(bf16))
                  + _dot(_bf(emat[2 * k2 + 1]), z[1, k2].astype(bf16)))
            xr, xi = xx[:128], xx[128:]
            wr = wf[g, k2 * WPITCH:k2 * WPITCH + 128, :]
            wi = wf[g + 3, k2 * WPITCH:k2 * WPITCH + 128, :]
            ys[g, k2] = ((xr * wr - xi * wi).astype(bf16), (xr * wi + xi * wr).astype(bf16))

        def inv(g, k2):
            yr, yi = ys.pop((g, k2))
            tt = _dot(_bf(emat[32 + 2 * k2]), yr) + _dot(_bf(emat[33 + 2 * k2]), yi)
            zs[g][0, k2] = tt[:128]
            zs[g][1, k2] = tt[128:]

        for bb in range(16):
            radix_fwd(0, bb)
        units = [(g, k2) for g in range(3) for k2 in range(16)]
        for i in range(len(units) + 2):
            if i < len(units):
                fwd(*units[i])
            if i >= 2:
                inv(*units[i - 2])
            if i < 32:
                radix_fwd(1 + i // 16, i % 16)

    def dinv_thunks(bb, finish):
        st = {}

        def rad(g):
            def run():
                z = zs[g]
                ys = _fft16([(z[0, a, chunk(bb), :], z[1, a, chunk(bb), :]) for a in range(16)], 1)
                st[g] = jnp.concatenate(
                    [jnp.concatenate([y[0] for y in ys], axis=0),
                     jnp.concatenate([y[1] for y in ys], axis=0)], axis=1).astype(bf16)
            return run

        def mm():
            st["p"] = [_dot(st[(j + 1) // 2], _bf(small[IW_OFF + 128 * j:IW_OFF + 128 * (j + 1), :]))
                       for j in range(5)]

        def fin():
            p0, p1, q1, p2, q2 = st["p"]
            e1, o1 = p0 + C1 * p1 + C2 * p2, S1 * q1 + S2 * q2
            e2, o2 = p0 + C2 * p1 + C1 * p2, S2 * q1 - S1 * q2
            y = jnp.concatenate([p0 + p1 + p2, e1 - o1, e2 - o2, e2 + o2, e1 + o1], axis=1)
            finish(xb[:, chunk(bb), :].reshape(128, DM) + _round_bf16(y))
        return [rad(0), rad(1), rad(2), mm, fin]

    def out_copy(bb):
        return pltpu.make_async_copy(xin.at[:, bb], out_hbm.at[:, bb], osem.at[bb])

    def layer(li, carry0):
        _loop("step", 0, 16, group, mem_ref[...].astype(f32))
        with jax.named_scope("tail"):
            wos, pre, dfts = finish_thunks(15, 1)
            for f in wos + [pre] + dfts:
                f()
        with jax.named_scope("spectral"):
            spectral()

        @pl.when(li == 0)
        def _():
            with jax.named_scope("dinv_tails"):
                th = [dinv_thunks(4 * u + 3, functools.partial(
                    lambda u, x: set_input(4 * u + 3, _round_bf16(x), u), u)) for u in range(4)]
                for stage in range(5):
                    for u in range(4):
                        th[u][stage]()

            def batch(it, carry):
                bb = body_chunk(it)
                side = dinv_thunks(bb, lambda x: set_input(bb, _round_bf16(x), None))
                _interleave(batch_thunks(it // 4, it % 4), side)
                return carry
            _loop("batch", 0, 12, batch, 0)

        @pl.when(li == 1)
        def _():
            with jax.named_scope("dinv_out"):
                def store_out(bb, x):
                    xin[:, bb] = x.reshape(16, 8, DM).astype(bf16)
                    out_copy(bb).start()
                th = [dinv_thunks(bb, functools.partial(store_out, bb)) for bb in range(16)]
                for i in range(17):
                    if i < 16:
                        for f in th[i][:4]:
                            f()
                    if i >= 1:
                        th[i - 1][4]()
                for bb in range(16):
                    out_copy(bb).wait()
        return carry0

    lax.fori_loop(0, 2, layer, 0)


@functools.partial(jax.jit, static_argnames=("A_seg_len",))
def pallas_interleave_layers__memory_aug_recurrent_mem_tr__spectral_gfnet__prompt_kernel(
    A_x, A_mem0, A_Wq, A_Wk, A_Wv, A_Wo, A_seg_len, B_x, B_w_r, B_w_i,
):
    assert A_seg_len == SEG and A_x.shape == (1, S, DM)
    small, emat = _tables()
    hbm = pl.BlockSpec(memory_space=pltpu.HBM)
    vmem = pl.BlockSpec(memory_space=pltpu.VMEM)
    out = pl.pallas_call(
        _kernel,
        out_shape=jax.ShapeDtypeStruct((16, 16, 8, DM), bf16),
        in_specs=[hbm, vmem] + [hbm] * 8,
        out_specs=hbm,
        scratch_shapes=[
            pltpu.VMEM((16, 16, 8, DM), bf16),
            pltpu.VMEM((16, 128, DM), f32),
            pltpu.VMEM((16, 128, DM), f32),
            pltpu.VMEM((16, 128, DM), f32),
            pltpu.VMEM((2, 128, DM), f32),
            pltpu.VMEM((12, DM, 8, DH), bf16),
            pltpu.VMEM((H * DH, DM), bf16),
            pltpu.VMEM((2560, 128), u32),
            pltpu.VMEM((96, 320, 128), u32),
            pltpu.VMEM((5, 2048, 128), u32),
            pltpu.VMEM((48, 4, 128, 128), u32),
            pltpu.VMEM((4, 5, 64, 128), u32),
            pltpu.VMEM((2, H, 32, 128), f32),
            pltpu.VMEM((2, 16, 128, 128), f32),
            pltpu.VMEM((2, 16, 128, 128), f32),
            pltpu.VMEM((2, 16, 128, 128), f32),
            pltpu.VMEM((6, 16 * WPITCH, 128), f32),
            pltpu.VMEM((2, DF, S), bf16),
            pltpu.VMEM((328, 128), f32),
            pltpu.VMEM((SMALL_ROWS, 128), u32),
            pltpu.VMEM((64, 128, 128), u32),
            pltpu.VMEM((80, 80), f32),
            pltpu.SemaphoreType.DMA((40,)),
            pltpu.SemaphoreType.DMA((16,)),
        ],
        compiler_params=pltpu.CompilerParams(vmem_limit_bytes=120 * 1024 * 1024),
    )(
        A_x.reshape(16, 16, 8, DM), A_mem0.reshape(MEM, DM),
        A_Wq, A_Wk, A_Wv, A_Wo.reshape(H * DH, DM), B_w_r.T, B_w_i.T,
        jnp.asarray(small), jnp.asarray(emat),
    )
    return out.reshape(1, S, DM)
```

```python
import functools
import math

import jax
import jax.numpy as jnp
import numpy as np
from jax import lax
import jax.experimental.pallas as pl
import jax.experimental.pallas.tpu as pltpu

f32, bf16, u32 = jnp.float32, jnp.bfloat16, jnp.uint32

S, DM, H, DH, MEM, SEG = 2048, 640, 32, 128, 8, 32
NSEG = S // SEG
NPAIR = H // 2
DF = DM // 2 + 1
EPS = 1e-5
WPITCH = 136

ZPITCH = 136

C1, C2 = math.cos(2 * math.pi / 5), math.cos(4 * math.pi / 5)
S1, S2 = math.sin(2 * math.pi / 5), math.sin(4 * math.pi / 5)


def _to_bf16_bits(a):
    u = np.ascontiguousarray(a, dtype=np.float32).view(np.uint32).astype(np.uint64)
    return ((u + 0x7FFF + ((u >> 16) & 1)) >> 16).astype(np.uint32)


def _pack_rows(a):
    b = _to_bf16_bits(a)
    return b[..., 0::2, :] | (b[..., 1::2, :] << 16)


@functools.lru_cache(maxsize=None)
def _tables():
    b = np.arange(128)
    l0 = np.arange(0, DF, 5)
    l1 = np.concatenate([np.arange(1, 320, 5), np.arange(4, 320, 5)])
    l2 = np.concatenate([np.arange(2, 320, 5), np.arange(3, 320, 5)])
    sg = np.concatenate([np.ones(64), -np.ones(64)])

    def th(l):
        return 2 * np.pi * ((b[:, None] * l[None, :]) % DM) / DM

    fw = np.zeros((6, 256, 128))
    t = th(l0)
    fw[0, :128, :65] = np.cos(t)
    fw[3, :128, :65] = -np.sin(t)
    for g, l in ((1, l1), (2, l2)):
        t = th(l)
        c, s = np.cos(t), np.sin(t)
        fw[g] = np.concatenate([c, -sg * s], axis=0)
        fw[3 + g] = np.concatenate([-s, -sg * c], axis=0)
    sc = 1.0 / (S * DM)
    iw = np.zeros((5, 256, 128))
    t = th(l0).T
    cl = np.full((65, 1), 2.0)
    cl[0] = cl[-1] = 1.0
    iw[0, :65] = cl * np.cos(t) * sc
    iw[0, 128:128 + 65] = -cl * np.sin(t) * sc
    for g, l in ((1, l1), (2, l2)):
        t = th(l).T
        c, s = np.cos(t), np.sin(t)
        gg = sg[:, None]
        iw[2 * g - 1] = 2 * sc * np.concatenate([c, -s], axis=0)
        iw[2 * g] = 2 * sc * np.concatenate([gg * s, gg * c], axis=0)
    n = np.arange(64)
    order = np.concatenate([np.concatenate([np.arange(8) + 8 * j, np.arange(8) + 8 * j + 64])
                            for j in range(8)])
    e = np.zeros((2, 32, 128, 128))
    for k2 in range(32):
        t = 2 * np.pi * (((32 * n[:, None] + k2) * n[None, :]) % S) / S
        er, ei = np.cos(t), -np.sin(t)
        m = np.block([[er, -ei], [ei, er]])[order][:, order]
        e[0, k2], e[1, k2] = m, m.T
    small = np.concatenate(
        [_pack_rows(fw).reshape(-1, 128), _pack_rows(iw).reshape(-1, 128)], axis=0)
    return small, _pack_rows(e).reshape(64, 64, 128)


FW_OFF, IW_OFF = 0, 6 * 128
SMALL_ROWS = 11 * 128


def _loop(name, lo, hi, body, init, **kw):
    with jax.named_scope(name):
        return lax.fori_loop(lo, hi, body, init, **kw)


def _bf(x):
    return pltpu.bitcast(x, bf16)


def _dot(a, b):
    return jnp.dot(a, b, preferred_element_type=f32)


def _round_bf16(x):
    return x.astype(bf16).astype(f32)


def _layernorm(x):
    m = jnp.mean(x, axis=-1, keepdims=True)
    xc = x - m
    v = jnp.mean(xc * xc, axis=-1, keepdims=True)
    return xc * lax.rsqrt(v + EPS)


def _fft4(x, sign):
    (ar, ai), (br, bi), (cr, ci), (dr, di) = x
    t0r, t0i, t1r, t1i = ar + cr, ai + ci, ar - cr, ai - ci
    t2r, t2i, t3r, t3i = br + dr, bi + di, br - dr, bi - di
    y0, y2 = (t0r + t2r, t0i + t2i), (t0r - t2r, t0i - t2i)
    p, q = (t1r + t3i, t1i - t3r), (t1r - t3i, t1i + t3r)
    return [y0, p, y2, q] if sign < 0 else [y0, q, y2, p]


def _twiddle(z, n, period, sign):
    zr, zi = z
    n = n % period
    if n == 0:
        return z
    if 4 * n == period:
        return (-zi, zr) if sign > 0 else (zi, -zr)
    c, s = math.cos(2 * math.pi * n / period), sign * math.sin(2 * math.pi * n / period)
    if (8 * n) % period == 0:
        a, d = zr + zi, zr - zi
        if c * s > 0:
            return (d * c, a * c)
        return (a * c, d * s)
    return (zr * c - zi * s, zr * s + zi * c)


def _ilv(r, i):
    n = r.shape[0] // 8
    return jnp.concatenate([r.reshape(n, 8, 128), i.reshape(n, 8, 128)], axis=1).reshape(16 * n, 128)


def _dilv(x):
    n = x.shape[0] // 16
    x = x.reshape(n, 16, 128)
    return x[:, :8].reshape(8 * n, 128), x[:, 8:].reshape(8 * n, 128)


def _with_tokens(x, toks):
    if not toks:
        return x
    return jnp.concatenate(
        [x[8 * j:8 * j + 8] | toks[j] if j in toks else x[8 * j:8 * j + 8]
         for j in range(x.shape[0] // 8)], axis=0)


def _fft16(x, sign, emit=None):
    cols = [_fft4([x[4 * j + r] for j in range(4)], sign) for r in range(4)]
    out = [None] * 16
    for q in range(4):
        y = _fft4([_twiddle(cols[r][q], r * q, 16, sign) for r in range(4)], sign)
        for p in range(4):
            out[q + 4 * p] = y[p]
        if emit is not None:
            emit(q, y)
    return out


LAT_S, LAT_PV, LAT_WO, N_AFTER = 6, 12, 7, 8


def _interleave(main, side):
    n, k = len(main), 0
    for i, f in enumerate(main):
        f()
        while k < len(side) and (k + 1) * n <= (i + 1) * len(side):
            side[k]()
            k += 1
    for f in side[k:]:
        f()


def _kernel(x_hbm, mem_ref, wq_hbm, wk_hbm, wv_hbm, wo_hbm, wr_hbm, wi_hbm,
            small_hbm, e_hbm, out_hbm,
            xin, xa, xb, xn, ao, raw, wo_raw, tmp, w32, wo32, qb, hl, ol, z0, z1, z2, wf,
            wri, wtmp, small, emat, fill_ref, sem, osem):
    zs = (z0, z1, z2)
    w_hbm = (wq_hbm, wk_hbm, wv_hbm)

    def body_chunk(i):
        return i + i // 3

    def cp_w(i):
        src = w_hbm[i // 4 if isinstance(i, int) else 0]
        c = i % 4
        return pltpu.make_async_copy(src.at[:, pl.ds(pl.multiple_of(8 * c, 8), 8), :],
                                     raw.at[i], sem.at[i])

    def cp_x(bb):
        return pltpu.make_async_copy(x_hbm.at[:, bb], xin.at[:, bb], sem.at[12 + bb])

    def cp_wo(i):
        rows = pl.ds(pl.multiple_of(512 * i, 512), 512)
        return pltpu.make_async_copy(wo_hbm.at[rows], wo_raw.at[rows], sem.at[28 + i])

    cp_rest = [pltpu.make_async_copy(wr_hbm, wri.at[0], sem.at[36]),
               pltpu.make_async_copy(wi_hbm, wri.at[1], sem.at[37]),
               pltpu.make_async_copy(small_hbm, small, sem.at[38]),
               pltpu.make_async_copy(e_hbm, emat, sem.at[39])]

    for u in range(4):
        cp_x(4 * u + 3).start()
    cp_w(0).start()
    for i in range(12):
        if i < 11:
            cp_w(i + 1).start()
        cp_x(body_chunk(i)).start()
        if i >= 4:
            cp_wo(i - 4).start()
    for cp in cp_rest:
        cp.start()

    r = lax.broadcasted_iota(jnp.int32, (80, 80), 0)
    c = lax.broadcasted_iota(jnp.int32, (80, 80), 1)

    def head(i):
        return jnp.where(i < 64, i // 32, (i - 64) // 8)

    def pos(i):
        return jnp.where(i < 64, i % 32, 32 + (i - 64) % 8)

    ok = (pos(r) < MEM) | (pos(r) >= pos(c))
    fill_ref[...] = jnp.where(head(r) == head(c), jnp.where(ok, 0.0, -1e9), -jnp.inf).astype(f32)
    ol[...] = jnp.zeros_like(ol)
    ao[...] = jnp.zeros_like(ao)
    wtmp[320:328, :] = jnp.zeros((8, 128), f32)
    for z in zs:
        z[0, 0, 128:ZPITCH, :] = jnp.zeros((8, 128), f32)

    def chunk(bb):
        if isinstance(bb, int):
            return slice(8 * bb, 8 * bb + 8)
        return pl.ds(pl.multiple_of(8 * bb, 8), 8)

    def set_input(bb, x, tail_u):
        xa[:, chunk(bb), :] = x.reshape(16, 8, DM)
        y = _layernorm(x)
        if tail_u is None:
            xn[:, chunk(bb), :] = y.reshape(16, 8, DM)
        else:
            yb = y.astype(bf16)
            for kt in range(5):
                hl[tail_u, kt] = pltpu.bitcast(yb[:, 128 * kt:128 * kt + 128], u32)

    def load_x(bb):
        return xin[:, bb].astype(f32).reshape(128, DM)

    def relayout_thunks(m, c):
        def p1(i):
            v = raw[4 * m + c, 16 * i:16 * i + 16].reshape(128, 128)
            tmp[64 * i:64 * i + 64, :] = pltpu.bitcast(v, u32)

        def p2(i):
            for j in range(4):
                a = tmp[pl.ds(64 * i + j, 8, stride=8), :]
                b = tmp[pl.ds(64 * i + 4 + j, 8, stride=8), :]
                t = 6 * (4 * c + j) + 2 * m
                w32[t, 8 * i:8 * i + 8, :] = (a & 0xFFFF) | (b << 16)
                w32[t + 1, 8 * i:8 * i + 8, :] = (a >> 16) | (b & jnp.uint32(0xFFFF0000))

        def piece(i):
            def run():
                p1(i)
                p2(i)
            return run
        return [piece(i) for i in range(40)]

    def batch_thunks(m, c):
        st = {}

        def one(j, u, e):
            def run():
                lhs = jnp.concatenate([_bf(hl[u, kt]) for kt in range(5)], axis=1)
                t = 6 * (4 * c + j) + 2 * m
                st[e] = _dot(lhs, _bf(w32[t + e])).reshape(16, 8, 128)
                if e == 1:
                    y = jnp.concatenate([st[0], st[1]], axis=1).reshape(256, 128).astype(bf16)
                    qb[3 * (4 * c + j) + m, u] = pltpu.bitcast(y, u32)
            return run
        return [one(j, u, e) for j in range(4) for u in range(4) for e in range(2)]

    def wperm_thunks(m, kc):
        def load():
            w = wri[m, :, pl.ds(pl.multiple_of(kc * 128, 128), 128)].astype(f32)
            wtmp[0:DF, :] = w

        def one(g):
            def run():
                if g == 0:
                    t = jnp.concatenate([wtmp[pl.ds(0, 64, stride=5), :], wtmp[320:328, :],
                                         jnp.zeros((56, 128), f32)], axis=0)
                else:
                    t = jnp.concatenate([wtmp[pl.ds(g, 64, stride=5), :],
                                         wtmp[pl.ds(5 - g, 64, stride=5), :]], axis=0)
                y = t.T
                sub = wf.at[3 * m + g, pl.ds(pl.multiple_of(kc * 8, 8), 15 * WPITCH + 8)]
                for k in range(8):
                    for hf in range(2):
                        sub[pl.ds(k + 8 * hf * WPITCH, 8, stride=WPITCH), :] = (
                            y[16 * k + 8 * hf:16 * k + 8 * hf + 8])
            return run
        return [load] + [one(g) for g in range(3)]

    def wo_copy_thunks(c):
        def one(j):
            def run():
                wo32[j, pl.ds(pl.multiple_of(c * 256, 256), 256), :] = pltpu.bitcast(
                    wo_raw[pl.ds(pl.multiple_of(c * 512, 512), 512), 128 * j:128 * j + 128], u32)
            return run
        return [one(j) for j in range(5)]

    with jax.named_scope("pro0"):
        for u in range(4):
            cp_x(4 * u + 3).wait()
        for u in range(4):
            set_input(4 * u + 3, load_x(4 * u + 3), u)
        cp_w(0).wait()
        for f in relayout_thunks(0, 0):
            f()

    def pro1(it, carry):
        @pl.when(it < 11)
        def _():
            cp_w(it + 1).wait()

        @pl.when(it >= 4)
        def _():
            cp_wo(it - 4).wait()
        bb = body_chunk(it)
        cp_x(bb).wait()
        nxt = jnp.minimum(it + 1, 11)
        set_input(bb, load_x(bb), None)
        for f in wo_copy_thunks(jnp.where(it >= 4, it - 4, 8)):
            f()
        _interleave(batch_thunks(it // 4, it % 4), relayout_thunks(nxt // 4, nxt % 4))
        return carry
    _loop("pro1", 0, 12, pro1, 0)
    for cp in cp_rest:
        cp.wait()

    scale = DH ** -0.5

    def wo_dot(hh, oo):
        return [_dot(oo, _bf(wo32[j, 64 * hh:64 * hh + 64, :])) for j in range(5)]

    def addl(acc, res):
        return res if acc is None else [a + b for a, b in zip(acc, res)]

    def finish_thunks(gp, slot):
        st = {"acc": None}

        def f_wo(hh):
            def run():
                st["acc"] = addl(st["acc"], wo_dot(hh, ol[slot, hh].astype(bf16)))
                if hh == H - 1:
                    out = jnp.concatenate(st["acc"], axis=1)
                    for u in range(4):
                        ao[slot, 32 * u + 24:32 * u + 32, :] = out[8 * u:8 * u + 8]
            return run

        def pre():
            x = _round_bf16(xa[gp] + _round_bf16(ao[slot]))
            xb[gp] = x
            y = _round_bf16(_layernorm(x))
            x0, x1, x2, x3, x4 = [y[:, 128 * a:128 * a + 128] for a in range(5)]
            t1, t2, t3, t4 = x1 + x4, x2 + x3, x1 - x4, x2 - x3
            st["u"] = [
                (x0 + t1 + t2).astype(bf16),
                jnp.concatenate([x0 + C1 * t1 + C2 * t2, S1 * t3 + S2 * t4], axis=1).astype(bf16),
                jnp.concatenate([x0 + C2 * t1 + C1 * t2, S2 * t3 - S1 * t4], axis=1).astype(bf16)]

        def f_dft(cidx):
            def run():
                g = cidx % 3
                o = FW_OFF + 128 * cidx
                zs[g][cidx // 3, gp, 0:128, :] = _dot(st["u"][g], _bf(small[o:o + (64 if g == 0 else 128), :]))
            return run
        return [f_wo(hh) for hh in range(H)], pre, [f_dft(cidx) for cidx in range(6)]

    def group(g, mem):
        cur = g % 2
        wos, pre, dfts = finish_thunks(jnp.maximum(g - 1, 0), 1 - cur)
        fillers = [wos[0:11], wos[11:22], wos[22:32], dfts]
        for ph in range(4):
            h = jnp.concatenate([mem, xn[g, 32 * ph:32 * ph + 24, :]], axis=0).astype(bf16)
            if ph == 3:
                pre()
            side = wperm_thunks(ph, g) if ph < 2 else []
            pr, sm, oos = {}, {}, {}

            def stacked(p, m):
                top = jnp.concatenate([pr[p, m, 0], pr[p, m, 1]], axis=0).astype(bf16)
                tail = _bf(qb[3 * p + m, ph, pl.ds(pl.multiple_of(8 * g, 8), 8), :])
                return jnp.concatenate([top, tail], axis=0)

            def scores(p):
                sc = lax.dot_general(stacked(p, 0), stacked(p, 1), (((1,), (1,)), ((), ())),
                                     preferred_element_type=f32)
                fill = fill_ref[...]
                sc = jnp.where(fill == 0.0, sc * scale, fill)
                mx = jnp.max(sc, axis=-1, keepdims=True)
                e = jnp.exp(sc - mx)
                sm[p] = (e.astype(bf16),
                         pl.reciprocal(jnp.sum(e, axis=-1, keepdims=True), approx=True))

            def pv(p):
                e, rl = sm[p]
                o = _dot(e, stacked(p, 2)) * rl
                ol[cur, 2 * p, 8 * ph:8 * ph + 8, :] = o[64:72]
                ol[cur, 2 * p + 1, 8 * ph:8 * ph + 8, :] = o[72:80]
                oos[2 * p], oos[2 * p + 1] = o[0:32].astype(bf16), o[32:64].astype(bf16)

            acc, t, nwo = None, 0.0, 0
            bulk = [(p, m, e) for p in range(NPAIR) for m in (1, 0, 2) for e in range(2)]
            pend, ready, fl = [], [], list(fillers[ph])
            while nwo < H:
                pend.sort()
                if pend and pend[0][0] <= t:
                    _, kind, p = pend.pop(0)
                    if kind == "S":
                        scores(p)
                        pend.append((t + LAT_PV, "V", p))
                    else:
                        pv(p)
                        ready += [(t + LAT_WO, 2 * p), (t + LAT_WO, 2 * p + 1)]
                    t += 0.5
                elif bulk:
                    p, m, e = bulk.pop(0)
                    pr[p, m, e] = _dot(h, _bf(w32[6 * p + 2 * m + e]))
                    t += 1
                    if m == 0 and e == 1:
                        pend.append((t + LAT_S, "S", p))
                    if side and len(bulk) % 18 == 0:
                        side.pop(0)()
                elif ready and ready[0][0] <= t:
                    _, hh = ready.pop(0)
                    acc = addl(acc, wo_dot(hh, oos[hh]))
                    t += 1
                    nwo += 1
                elif len(fl) > N_AFTER:
                    fl.pop(0)()
                    t += 1
                else:
                    t += 0.5
            out = jnp.concatenate(acc, axis=1)
            ao[cur, 32 * ph:32 * ph + 24, :] = out[8:32]
            mem = _round_bf16(out[0:8])
            for f in fl:
                f()
        return mem

    def spectral(zero):
        def fence(z):
            return z[0, zero, 128:ZPITCH, :]

        def radix_fwd(g, bb, tok=None):
            z = zs[g]
            xs = [(z[0, a, chunk(bb), :], z[1, a, chunk(bb), :]) for a in range(16)]
            if tok is not None:
                xs[:4] = [(xr + tok, xi) for xr, xi in xs[:4]]
            toks = []

            def emit(q, y):
                for p in range(4):
                    z[0, q + 4 * p, chunk(bb), :] = y[p][0]
                    z[1, q + 4 * p, chunk(bb), :] = y[p][1]
                if g > 0 or q == 3:
                    toks.append(fence(z))
            _fft16(xs, -1, emit)
            return toks

        ys = {}

        def fwd(g, k2, toks):
            z = zs[g]
            ur, ui = z[0, k2, 0:64, :], z[1, k2, 0:64, :]
            tr, ti = _twiddle((z[0, k2, 64:128, :], z[1, k2, 64:128, :]), k2, 32, -1)
            for hf in range(2):
                v = _ilv(ur + tr, ui + ti) if hf == 0 else _ilv(ur - tr, ui - ti)
                lhs = _with_tokens(emat[k2 + 16 * hf], toks if hf == 0 else None)
                xr, xi = _dilv(_dot(_bf(lhs), v.astype(bf16)))
                wr = wf[g, pl.ds(k2 * WPITCH + hf, 64, stride=2), :]
                wi = wf[g + 3, pl.ds(k2 * WPITCH + hf, 64, stride=2), :]
                ys[g, k2, hf] = _ilv(xr * wr - xi * wi, xr * wi + xi * wr).astype(bf16)

        def inv(g, k2):
            z = zs[g]
            t0 = _dot(_bf(emat[32 + k2]), ys.pop((g, k2, 0)))
            t1 = _dot(_bf(emat[48 + k2]), ys.pop((g, k2, 1)))
            z[0, k2, 0:64, :], z[1, k2, 0:64, :] = _dilv(t0 + t1)
            z[0, k2, 64:128, :], z[1, k2, 64:128, :] = _twiddle(_dilv(t0 - t1), k2, 32, 1)

        chain = {}
        for bb in range(16):
            chain[bb] = radix_fwd(0, bb, chain.get(bb - 2))[-1]
        radix_fwd(1, 0)
        units = [(g, k2) for g in range(3) for k2 in range(16)]
        toks = None
        for i in range(len(units) + 3):
            if i < len(units):
                fwd(*units[i], toks)
            if i >= 3:
                inv(*units[i - 3])
            toks = None
            if i < 31:
                t4 = radix_fwd(1 + (i + 1) // 16, (i + 1) % 16)
                toks = {3 + j: pltpu.bitcast(t, u32) for j, t in enumerate(t4)}

    def dinv_thunks(bb, finish):
        st = {}

        def rad(g):
            def run():
                z = zs[g]
                ys = _fft16([(z[0, a, chunk(bb), :], z[1, a, chunk(bb), :]) for a in range(16)], 1)
                st[g] = jnp.concatenate(
                    [jnp.concatenate([y[0] for y in ys], axis=0),
                     jnp.concatenate([y[1] for y in ys], axis=0)], axis=1).astype(bf16)
            return run

        def mm():
            st["p"] = [_dot(st[(j + 1) // 2], _bf(small[IW_OFF + 128 * j:IW_OFF + 128 * (j + 1), :]))
                       for j in range(5)]

        def fin():
            p0, p1, q1, p2, q2 = st["p"]
            e1, o1 = p0 + C1 * p1 + C2 * p2, S1 * q1 + S2 * q2
            e2, o2 = p0 + C2 * p1 + C1 * p2, S2 * q1 - S1 * q2
            y = jnp.concatenate([p0 + p1 + p2, e1 - o1, e2 - o2, e2 + o2, e1 + o1], axis=1)
            finish(xb[:, chunk(bb), :].reshape(128, DM) + _round_bf16(y))
        return [rad(0), rad(1), rad(2), mm, fin]

    def out_copy(bb):
        return pltpu.make_async_copy(xin.at[:, bb], out_hbm.at[:, bb], osem.at[bb])

    def layer(li, carry0):
        _loop("step", 0, 16, group, mem_ref[...].astype(f32))
        with jax.named_scope("tail"):
            wos, pre, dfts = finish_thunks(15, 1)
            for f in wos + [pre] + dfts:
                f()
        with jax.named_scope("spectral"):
            spectral(li // 2)

        @pl.when(li == 0)
        def _():
            with jax.named_scope("dinv_tails"):
                th = [dinv_thunks(4 * u + 3, functools.partial(
                    lambda u, x: set_input(4 * u + 3, _round_bf16(x), u), u)) for u in range(4)]
                for stage in range(5):
                    for u in range(4):
                        th[u][stage]()

            def batch(it, carry):
                bb = body_chunk(it)
                side = dinv_thunks(bb, lambda x: set_input(bb, _round_bf16(x), None))
                _interleave(batch_thunks(it // 4, it % 4), side)
                return carry
            _loop("batch", 0, 12, batch, 0)

        @pl.when(li == 1)
        def _():
            with jax.named_scope("dinv_out"):
                def store_out(bb, x):
                    xin[:, bb] = x.reshape(16, 8, DM).astype(bf16)
                    out_copy(bb).start()
                th = [dinv_thunks(bb, functools.partial(store_out, bb)) for bb in range(16)]
                for i in range(17):
                    if i < 16:
                        for f in th[i][:4]:
                            f()
                    if i >= 1:
                        th[i - 1][4]()
                for bb in range(16):
                    out_copy(bb).wait()
        return carry0

    lax.fori_loop(0, 2, layer, 0)


@functools.partial(jax.jit, static_argnames=("A_seg_len",))
def pallas_interleave_layers__memory_aug_recurrent_mem_tr__spectral_gfnet__prompt_kernel(
    A_x, A_mem0, A_Wq, A_Wk, A_Wv, A_Wo, A_seg_len, B_x, B_w_r, B_w_i,
):
    assert A_seg_len == SEG and A_x.shape == (1, S, DM)
    small, emat = _tables()
    hbm = pl.BlockSpec(memory_space=pltpu.HBM)
    vmem = pl.BlockSpec(memory_space=pltpu.VMEM)
    out = pl.pallas_call(
        _kernel,
        out_shape=jax.ShapeDtypeStruct((16, 16, 8, DM), bf16),
        in_specs=[hbm, vmem] + [hbm] * 8,
        out_specs=hbm,
        scratch_shapes=[
            pltpu.VMEM((16, 16, 8, DM), bf16),
            pltpu.VMEM((16, 128, DM), f32),
            pltpu.VMEM((16, 128, DM), f32),
            pltpu.VMEM((16, 128, DM), f32),
            pltpu.VMEM((2, 128, DM), f32),
            pltpu.VMEM((12, DM, 8, DH), bf16),
            pltpu.VMEM((H * DH + 512, DM), bf16),
            pltpu.VMEM((2560, 128), u32),
            pltpu.VMEM((96, 320, 128), u32),
            pltpu.VMEM((5, 2048 + 256, 128), u32),
            pltpu.VMEM((48, 4, 128, 128), u32),
            pltpu.VMEM((4, 5, 64, 128), u32),
            pltpu.VMEM((2, H, 32, 128), f32),
            pltpu.VMEM((2, 16, ZPITCH, 128), f32),
            pltpu.VMEM((2, 16, ZPITCH, 128), f32),
            pltpu.VMEM((2, 16, ZPITCH, 128), f32),
            pltpu.VMEM((6, 16 * WPITCH, 128), f32),
            pltpu.VMEM((2, DF, S), bf16),
            pltpu.VMEM((328, 128), f32),
            pltpu.VMEM((SMALL_ROWS, 128), u32),
            pltpu.VMEM((64, 64, 128), u32),
            pltpu.VMEM((80, 80), f32),
            pltpu.SemaphoreType.DMA((40,)),
            pltpu.SemaphoreType.DMA((16,)),
        ],
        compiler_params=pltpu.CompilerParams(vmem_limit_bytes=120 * 1024 * 1024),
    )(
        A_x.reshape(16, 16, 8, DM), A_mem0.reshape(MEM, DM),
        A_Wq, A_Wk, A_Wv, A_Wo.reshape(H * DH, DM), B_w_r.T, B_w_i.T,
        jnp.asarray(small), jnp.asarray(emat),
    )
    return out.reshape(1, S, DM)
```

```python
import functools
import math

import jax
import jax.numpy as jnp
import numpy as np
from jax import lax
import jax.experimental.pallas as pl
import jax.experimental.pallas.tpu as pltpu

f32, bf16, u32 = jnp.float32, jnp.bfloat16, jnp.uint32

S, DM, H, DH, MEM, SEG = 2048, 640, 32, 128, 8, 32
NSEG = S // SEG
NPAIR = H // 2
DF = DM // 2 + 1
EPS = 1e-5
WPITCH = 136

ZPITCH = 136

C1, C2 = math.cos(2 * math.pi / 5), math.cos(4 * math.pi / 5)
S1, S2 = math.sin(2 * math.pi / 5), math.sin(4 * math.pi / 5)


def _to_bf16_bits(a):
    u = np.ascontiguousarray(a, dtype=np.float32).view(np.uint32).astype(np.uint64)
    return ((u + 0x7FFF + ((u >> 16) & 1)) >> 16).astype(np.uint32)


def _pack_rows(a):
    b = _to_bf16_bits(a)
    return b[..., 0::2, :] | (b[..., 1::2, :] << 16)


@functools.lru_cache(maxsize=None)
def _tables():
    b = np.arange(128)
    l0 = np.arange(0, DF, 5)
    l1 = np.concatenate([np.arange(1, 320, 5), np.arange(4, 320, 5)])
    l2 = np.concatenate([np.arange(2, 320, 5), np.arange(3, 320, 5)])
    sg = np.concatenate([np.ones(64), -np.ones(64)])

    def th(l):
        return 2 * np.pi * ((b[:, None] * l[None, :]) % DM) / DM

    fw = np.zeros((6, 256, 128))
    t = th(l0)
    fw[0, :128, :65] = np.cos(t)
    fw[3, :128, :65] = -np.sin(t)
    for g, l in ((1, l1), (2, l2)):
        t = th(l)
        c, s = np.cos(t), np.sin(t)
        fw[g] = np.concatenate([c, -sg * s], axis=0)
        fw[3 + g] = np.concatenate([-s, -sg * c], axis=0)
    sc = 1.0 / (S * DM)
    iw = np.zeros((5, 256, 128))
    t = th(l0).T
    cl = np.full((65, 1), 2.0)
    cl[0] = cl[-1] = 1.0
    iw[0, :65] = cl * np.cos(t) * sc
    iw[0, 128:128 + 65] = -cl * np.sin(t) * sc
    for g, l in ((1, l1), (2, l2)):
        t = th(l).T
        c, s = np.cos(t), np.sin(t)
        gg = sg[:, None]
        iw[2 * g - 1] = 2 * sc * np.concatenate([c, -s], axis=0)
        iw[2 * g] = 2 * sc * np.concatenate([gg * s, gg * c], axis=0)
    n = np.arange(64)
    order = np.concatenate([np.concatenate([np.arange(8) + 8 * j, np.arange(8) + 8 * j + 64])
                            for j in range(8)])
    e = np.zeros((2, 32, 128, 128))
    for k2 in range(32):
        t = 2 * np.pi * (((32 * n[:, None] + k2) * n[None, :]) % S) / S
        er, ei = np.cos(t), -np.sin(t)
        m = np.block([[er, -ei], [ei, er]])[order][:, order]
        e[0, k2], e[1, k2] = m, m.T
    small = np.concatenate(
        [_pack_rows(fw).reshape(-1, 128), _pack_rows(iw).reshape(-1, 128)], axis=0)
    return small, _pack_rows(e).reshape(64, 64, 128)


FW_OFF, IW_OFF = 0, 6 * 128
SMALL_ROWS = 11 * 128


def _loop(name, lo, hi, body, init, **kw):
    with jax.named_scope(name):
        return lax.fori_loop(lo, hi, body, init, **kw)


def _bf(x):
    return pltpu.bitcast(x, bf16)


def _dot(a, b):
    return jnp.dot(a, b, preferred_element_type=f32)


def _round_bf16(x):
    return x.astype(bf16).astype(f32)


def _layernorm(x):
    m = jnp.mean(x, axis=-1, keepdims=True)
    xc = x - m
    v = jnp.mean(xc * xc, axis=-1, keepdims=True)
    return xc * lax.rsqrt(v + EPS)


def _fft4(x, sign):
    (ar, ai), (br, bi), (cr, ci), (dr, di) = x
    t0r, t0i, t1r, t1i = ar + cr, ai + ci, ar - cr, ai - ci
    t2r, t2i, t3r, t3i = br + dr, bi + di, br - dr, bi - di
    y0, y2 = (t0r + t2r, t0i + t2i), (t0r - t2r, t0i - t2i)
    p, q = (t1r + t3i, t1i - t3r), (t1r - t3i, t1i + t3r)
    return [y0, p, y2, q] if sign < 0 else [y0, q, y2, p]


def _twiddle(z, n, period, sign):
    zr, zi = z
    n = n % period
    if n == 0:
        return z
    if 4 * n == period:
        return (-zi, zr) if sign > 0 else (zi, -zr)
    c, s = math.cos(2 * math.pi * n / period), sign * math.sin(2 * math.pi * n / period)
    if (8 * n) % period == 0:
        a, d = zr + zi, zr - zi
        if c * s > 0:
            return (d * c, a * c)
        return (a * c, d * s)
    return (zr * c - zi * s, zr * s + zi * c)


def _ilv(r, i):
    n = r.shape[0] // 8
    return jnp.concatenate([r.reshape(n, 8, 128), i.reshape(n, 8, 128)], axis=1).reshape(16 * n, 128)


def _dilv(x):
    n = x.shape[0] // 16
    x = x.reshape(n, 16, 128)
    return x[:, :8].reshape(8 * n, 128), x[:, 8:].reshape(8 * n, 128)


def _with_tokens(x, toks):
    if not toks:
        return x
    return jnp.concatenate(
        [x[8 * j:8 * j + 8] | toks[j] if j in toks else x[8 * j:8 * j + 8]
         for j in range(x.shape[0] // 8)], axis=0)


def _fft16(x, sign, emit=None):
    cols = [_fft4([x[4 * j + r] for j in range(4)], sign) for r in range(4)]
    out = [None] * 16
    for q in range(4):
        y = _fft4([_twiddle(cols[r][q], r * q, 16, sign) for r in range(4)], sign)
        for p in range(4):
            out[q + 4 * p] = y[p]
        if emit is not None:
            emit(q, y)
    return out


CFG = dict(lat_s=6, lat_pv=15, lat_wo=7, n_after=(11, 11, 11, 0), fill_at=16, v_delay=8, v_gap=0,
           prenorm=True,
           pre_at=((), (), (), tuple(range(11, 91, 5))), pre_rows=((), (), (), tuple(range(16))),
           first=(0, 1), only=None)


def _interleave(main, side):
    n, k = len(main), 0
    for i, f in enumerate(main):
        f()
        while k < len(side) and (k + 1) * n <= (i + 1) * len(side):
            side[k]()
            k += 1
    for f in side[k:]:
        f()


def _kernel(x_hbm, mem_ref, wq_hbm, wk_hbm, wv_hbm, wo_hbm, wr_hbm, wi_hbm,
            small_hbm, e_hbm, out_hbm,
            xin, xa, xb, xn, ao, raw, wo_raw, tmp, w32, wo32, qb, hl, ol, z0, z1, z2, wf,
            wri, wtmp, small, emat, fill_ref, sem, osem):
    zs = (z0, z1, z2)
    w_hbm = (wq_hbm, wk_hbm, wv_hbm)

    def body_chunk(i):
        return i + i // 3

    def cp_w(i):
        src = w_hbm[i // 4 if isinstance(i, int) else 0]
        c = i % 4
        return pltpu.make_async_copy(src.at[:, pl.ds(pl.multiple_of(8 * c, 8), 8), :],
                                     raw.at[i], sem.at[i])

    def cp_x(bb):
        return pltpu.make_async_copy(x_hbm.at[:, bb], xin.at[:, bb], sem.at[12 + bb])

    def cp_wo(i):
        rows = pl.ds(pl.multiple_of(512 * i, 512), 512)
        return pltpu.make_async_copy(wo_hbm.at[rows], wo_raw.at[rows], sem.at[28 + i])

    cp_rest = [pltpu.make_async_copy(wr_hbm, wri.at[0], sem.at[36]),
               pltpu.make_async_copy(wi_hbm, wri.at[1], sem.at[37]),
               pltpu.make_async_copy(small_hbm, small, sem.at[38]),
               pltpu.make_async_copy(e_hbm, emat, sem.at[39])]

    full = CFG["only"] is None
    for u in range(4 if full else 0):
        cp_x(4 * u + 3).start()
    if full:
        cp_w(0).start()
    for i in range(12 if full else 0):
        if i < 11:
            cp_w(i + 1).start()
        cp_x(body_chunk(i)).start()
        if i >= 4:
            cp_wo(i - 4).start()
    for cp in cp_rest if full else ():
        cp.start()

    r = lax.broadcasted_iota(jnp.int32, (80, 80), 0)
    c = lax.broadcasted_iota(jnp.int32, (80, 80), 1)

    def head(i):
        return jnp.where(i < 64, i // 32, (i - 64) // 8)

    def pos(i):
        return jnp.where(i < 64, i % 32, 32 + (i - 64) % 8)

    ok = (pos(r) < MEM) | (pos(r) >= pos(c))
    fill_ref[...] = jnp.where(head(r) == head(c), jnp.where(ok, 0.0, -1e9), -jnp.inf).astype(f32)
    ol[...] = jnp.zeros_like(ol)
    ao[...] = jnp.zeros_like(ao)
    wtmp[320:328, :] = jnp.zeros((8, 128), f32)
    xb[17, 0:8, 0:128] = jnp.zeros((8, 128), f32)
    for z in zs:
        z[0, 0, 128:ZPITCH, :] = jnp.zeros((8, 128), f32)

    def chunk(bb):
        if isinstance(bb, int):
            return slice(8 * bb, 8 * bb + 8)
        return pl.ds(pl.multiple_of(8 * bb, 8), 8)

    def set_input(bb, x, tail_u):
        xa[:, chunk(bb), :] = x.reshape(16, 8, DM)
        y = _layernorm(x)
        if tail_u is None:
            xn[:, chunk(bb), :] = y.reshape(16, 8, DM)
        else:
            yb = y.astype(bf16)
            for kt in range(5):
                hl[tail_u, kt] = pltpu.bitcast(yb[:, 128 * kt:128 * kt + 128], u32)

    def load_x(bb):
        return xin[:, bb].astype(f32).reshape(128, DM)

    def relayout_thunks(m, c):
        def p1(i):
            v = raw[4 * m + c, 16 * i:16 * i + 16].reshape(128, 128)
            tmp[64 * i:64 * i + 64, :] = pltpu.bitcast(v, u32)

        def p2(i):
            for j in range(4):
                a = tmp[pl.ds(64 * i + j, 8, stride=8), :]
                b = tmp[pl.ds(64 * i + 4 + j, 8, stride=8), :]
                t = 6 * (4 * c + j) + 2 * m
                w32[t, 8 * i:8 * i + 8, :] = (a & 0xFFFF) | (b << 16)
                w32[t + 1, 8 * i:8 * i + 8, :] = (a >> 16) | (b & jnp.uint32(0xFFFF0000))

        def piece(i):
            def run():
                p1(i)
                p2(i)
            return run
        return [piece(i) for i in range(40)]

    def batch_thunks(m, c):
        def one(j, u, e):
            def run(toks=None):
                lhs = jnp.concatenate([_bf(hl[u, kt]) for kt in range(5)], axis=1)
                t = 6 * (4 * c + j) + 2 * m + e
                qb[t, u] = _dot(lhs, _bf(_with_tokens(w32[t], toks)))
            return run
        return [one(j, u, e) for j in range(4) for u in range(4) for e in range(2)]

    def wperm_thunks(m, kc):
        def load():
            w = wri[m, :, pl.ds(pl.multiple_of(kc * 128, 128), 128)].astype(f32)
            wtmp[0:DF, :] = w

        def one(g):
            def run():
                if g == 0:
                    t = jnp.concatenate([wtmp[pl.ds(0, 64, stride=5), :], wtmp[320:328, :],
                                         jnp.zeros((56, 128), f32)], axis=0)
                else:
                    t = jnp.concatenate([wtmp[pl.ds(g, 64, stride=5), :],
                                         wtmp[pl.ds(5 - g, 64, stride=5), :]], axis=0)
                y = t.T
                sub = wf.at[3 * m + g, pl.ds(pl.multiple_of(kc * 8, 8), 15 * WPITCH + 8)]
                for k in range(8):
                    for hf in range(2):
                        sub[pl.ds(k + 8 * hf * WPITCH, 8, stride=WPITCH), :] = (
                            y[16 * k + 8 * hf:16 * k + 8 * hf + 8])
            return run
        return [load] + [one(g) for g in range(3)]

    def wo_copy_thunks(c):
        def one(j):
            def run():
                wo32[j, pl.ds(pl.multiple_of(c * 256, 256), 256), :] = pltpu.bitcast(
                    wo_raw[pl.ds(pl.multiple_of(c * 512, 512), 512), 128 * j:128 * j + 128], u32)
            return run
        return [one(j) for j in range(5)]

    def pro0():
        for u in range(4):
            cp_x(4 * u + 3).wait()
        for u in range(4):
            set_input(4 * u + 3, load_x(4 * u + 3), u)
        cp_w(0).wait()
        for f in relayout_thunks(0, 0):
            f()

    def pro1(it, carry):
        @pl.when(it < 11)
        def _():
            cp_w(it + 1).wait()

        @pl.when(it >= 4)
        def _():
            cp_wo(it - 4).wait()
        bb = body_chunk(it)
        cp_x(bb).wait()
        nxt = jnp.minimum(it + 1, 11)
        set_input(bb, load_x(bb), None)
        for f in wo_copy_thunks(jnp.where(it >= 4, it - 4, 8)):
            f()
        _interleave(batch_thunks(it // 4, it % 4), relayout_thunks(nxt // 4, nxt % 4))
        return carry

    if full:
        with jax.named_scope("pro0"):
            pro0()
        _loop("pro1", 0, 12, pro1, 0)
        for cp in cp_rest:
            cp.wait()

    scale = DH ** -0.5

    def wo_dot(hh, oo):
        return [_dot(oo, _bf(wo32[j, 64 * hh:64 * hh + 64, :])) for j in range(5)]

    def addl(acc, res):
        return res if acc is None else [a + b for a, b in zip(acc, res)]

    def finish_thunks(gp, slot):
        st = {"acc": None}

        def f_wo(hh):
            def run():
                st["acc"] = addl(st["acc"], wo_dot(hh, ol[slot, hh].astype(bf16)))
                if hh == H - 1:
                    out = jnp.concatenate(st["acc"], axis=1)
                    for u in range(4):
                        ao[slot, 32 * u + 24:32 * u + 32, :] = out[8 * u:8 * u + 8]
            return run

        def pre(rows):
            x = _round_bf16(xa[gp, rows, :] + ao[slot, rows, :])
            xb[gp, rows, :] = x
            y = _layernorm(x)
            x0, x1, x2, x3, x4 = [y[:, 128 * a:128 * a + 128] for a in range(5)]
            t1, t2, t3, t4 = x1 + x4, x2 + x3, x1 - x4, x2 - x3
            xb[16, rows, :] = jnp.concatenate(
                [x0 + t1 + t2, x0 + C1 * t1 + C2 * t2, S1 * t3 + S2 * t4,
                 x0 + C2 * t1 + C1 * t2, S2 * t3 - S1 * t4], axis=1)

        def f_dft(cidx):
            def run():
                g = cidx % 3
                o = FW_OFF + 128 * cidx
                lo, hi = (0, 128) if g == 0 else (256 * g - 128, 256 * g + 128)
                zs[g][cidx // 3, gp, 0:128, :] = _dot(
                    xb[16, :, lo:hi].astype(bf16), _bf(small[o:o + (hi - lo) // 2, :]))
            return run
        return [f_wo(hh) for hh in range(H)], pre, [f_dft(cidx) for cidx in (0, 3, 1, 4, 2, 5)]

    def group(g, mem):
        cur = g % 2
        wos, pre, dfts = finish_thunks(jnp.maximum(g - 1, 0), 1 - cur)
        fillers = [wos[0:11], wos[11:22], wos[22:32], dfts]
        for ph in range(4):
            h = jnp.concatenate([mem, xn[g, 32 * ph:32 * ph + 24, :]], axis=0).astype(bf16)
            side = wperm_thunks(ph, g) if ph < 2 and CFG.get("wperm", True) else []
            pres = list(CFG["pre_rows"][ph])
            pre_at = CFG["pre_at"][ph]
            tok = None
            pr, sm, oos = {}, {}, {}

            def stacked(p, m):
                tails = [qb[6 * p + 2 * m + e, ph, chunk(g), :] for e in range(2)]
                return jnp.concatenate([pr[p, m, 0], pr[p, m, 1]] + tails, axis=0).astype(bf16)

            def scores(p):
                sc = lax.dot_general(stacked(p, 0), stacked(p, 1), (((1,), (1,)), ((), ())),
                                     preferred_element_type=f32)
                fill = fill_ref[...]
                sc = jnp.where(fill == 0.0, sc * scale, fill)
                mx = jnp.max(sc, axis=-1, keepdims=True)
                e = jnp.exp(sc - mx)
                rl = pl.reciprocal(jnp.sum(e, axis=-1, keepdims=True), approx=True)
                sm[p] = ((e * rl).astype(bf16), None) if CFG["prenorm"] else (e.astype(bf16), rl)

            def pv(p):
                e, rl = sm[p]
                o = _dot(e, stacked(p, 2))
                if rl is not None:
                    o = o * rl
                ol[cur, 2 * p, 8 * ph:8 * ph + 8, :] = o[64:72]
                ol[cur, 2 * p + 1, 8 * ph:8 * ph + 8, :] = o[72:80]
                oos[2 * p], oos[2 * p + 1] = o[0:32].astype(bf16), o[32:64].astype(bf16)

            acc, t, nwo = None, 0.0, 0
            keyed = []
            for p in range(NPAIR):
                keyed += [(4 * p + 2 * i + e, (p, m, e)) for i, m in enumerate(CFG["first"]) for e in range(2)]
                keyed += [(4 * p + 3.5 + CFG["v_delay"] + CFG["v_gap"] * e, (p, 2, e)) for e in range(2)]
            bulk = [x for _, x in sorted(keyed, key=lambda kv: kv[0])]
            pend, ready, fl = [], [], list(fillers[ph])
            n_after = CFG["n_after"][ph]
            while nwo < H:
                pend.sort()
                if pend and pend[0][0] <= t:
                    _, kind, p = pend.pop(0)
                    if kind == "S":
                        scores(p)
                        pend.append((t + CFG["lat_pv"], "V", p))
                    else:
                        pv(p)
                        ready += [(t + CFG["lat_wo"], 2 * p + e) for e in range(2)]
                    t += 0.5
                elif bulk:
                    p, m, e = bulk.pop(0)
                    pr[p, m, e] = _dot(h, _bf(_with_tokens(w32[6 * p + 2 * m + e], tok)))
                    tok = None
                    if 96 - len(bulk) in pre_at:
                        pre(chunk(pres.pop(0)))
                        tok = {0: pltpu.bitcast(xb[17 + g // 16, 0:8, 0:128], u32)}
                    t += 1
                    if m == CFG["first"][1] and e == 1:
                        pend.append((t + CFG["lat_s"], "S", p))
                    if side and len(bulk) % 18 == 0:
                        side.pop(0)()
                elif nwo >= CFG["fill_at"] and len(fl) > n_after:
                    fl.pop(0)()
                    t += 1
                elif ready and ready[0][0] <= t:
                    _, hh = ready.pop(0)
                    acc = addl(acc, wo_dot(hh, oos[hh]))
                    t += 1
                    nwo += 1
                elif len(fl) > n_after:
                    fl.pop(0)()
                    t += 1
                else:
                    t += 0.5
            out = jnp.concatenate(acc, axis=1)
            ao[cur, 32 * ph:32 * ph + 24, :] = out[8:32]
            mem = _round_bf16(out[0:8])
            for f in fl:
                f()
        return mem

    def spectral(zero):
        def fence(z):
            return z[0, zero, 128:ZPITCH, :]

        def radix_fwd(g, bb, tok=None):
            z = zs[g]
            xs = [(z[0, a, chunk(bb), :], z[1, a, chunk(bb), :]) for a in range(16)]
            if tok is not None:
                xs[:4] = [(xr + tok, xi) for xr, xi in xs[:4]]
            toks = []

            def emit(q, y):
                for p in range(4):
                    z[0, q + 4 * p, chunk(bb), :] = y[p][0]
                    z[1, q + 4 * p, chunk(bb), :] = y[p][1]
                if g > 0 or q == 3:
                    toks.append(fence(z))
            _fft16(xs, -1, emit)
            return toks

        ys = {}

        def fwd(g, k2, toks):
            z = zs[g]
            ur, ui = z[0, k2, 0:64, :], z[1, k2, 0:64, :]
            tr, ti = _twiddle((z[0, k2, 64:128, :], z[1, k2, 64:128, :]), k2, 32, -1)
            for hf in range(2):
                v = _ilv(ur + tr, ui + ti) if hf == 0 else _ilv(ur - tr, ui - ti)
                lhs = _with_tokens(emat[k2 + 16 * hf], toks if hf == 0 else None)
                xr, xi = _dilv(_dot(_bf(lhs), v.astype(bf16)))
                wr = wf[g, pl.ds(k2 * WPITCH + hf, 64, stride=2), :]
                wi = wf[g + 3, pl.ds(k2 * WPITCH + hf, 64, stride=2), :]
                ys[g, k2, hf] = _ilv(xr * wr - xi * wi, xr * wi + xi * wr).astype(bf16)

        def inv(g, k2):
            z = zs[g]
            t0 = _dot(_bf(emat[32 + k2]), ys.pop((g, k2, 0)))
            t1 = _dot(_bf(emat[48 + k2]), ys.pop((g, k2, 1)))
            z[0, k2, 0:64, :], z[1, k2, 0:64, :] = _dilv(t0 + t1)
            z[0, k2, 64:128, :], z[1, k2, 64:128, :] = _twiddle(_dilv(t0 - t1), k2, 32, 1)

        chain = {}
        for bb in range(16):
            chain[bb] = radix_fwd(0, bb, chain.get(bb - 2))[-1]
        radix_fwd(1, 0)
        units = [(g, k2) for g in range(3) for k2 in range(16)]
        toks = None
        for i in range(len(units) + 3):
            if i < len(units):
                fwd(*units[i], toks)
            if i >= 3:
                inv(*units[i - 3])
            toks = None
            if i < 31:
                t4 = radix_fwd(1 + (i + 1) // 16, (i + 1) % 16)
                toks = {3 + j: pltpu.bitcast(t, u32) for j, t in enumerate(t4)}

    def dinv_thunks(bb, finish):
        st = {}

        def rad(g):
            def run():
                z = zs[g]
                ys = _fft16([(z[0, a, chunk(bb), :], z[1, a, chunk(bb), :]) for a in range(16)], 1)
                st[g] = jnp.concatenate(
                    [jnp.concatenate([y[0] for y in ys], axis=0),
                     jnp.concatenate([y[1] for y in ys], axis=0)], axis=1).astype(bf16)
            return run

        def mm():
            st["p"] = [_dot(st[(j + 1) // 2], _bf(small[IW_OFF + 128 * j:IW_OFF + 128 * (j + 1), :]))
                       for j in range(5)]

        def fin():
            p0, p1, q1, p2, q2 = st["p"]
            e1, o1 = p0 + C1 * p1 + C2 * p2, S1 * q1 + S2 * q2
            e2, o2 = p0 + C2 * p1 + C1 * p2, S2 * q1 - S1 * q2
            y = jnp.concatenate([p0 + p1 + p2, e1 - o1, e2 - o2, e2 + o2, e1 + o1], axis=1)
            finish(xb[0:16, chunk(bb), :].reshape(128, DM) + y)
        return [rad(0), rad(1), rad(2), mm, fin]

    def out_copy(bb):
        return pltpu.make_async_copy(xin.at[:, bb], out_hbm.at[:, bb], osem.at[bb])

    def layer(li, carry0):
        _loop("step", 0, 16, group, mem_ref[...].astype(f32))
        if not full:
            return carry0
        with jax.named_scope("tail"):
            wos, pre, dfts = finish_thunks(15, 1)
            for f in wos:
                f()
            pre(slice(None))
            for f in dfts:
                f()
        with jax.named_scope("spectral"):
            spectral(li // 2)

        @pl.when(li == 0)
        def _():
            with jax.named_scope("dinv_tails"):
                th = [dinv_thunks(4 * u + 3, functools.partial(
                    lambda u, x: set_input(4 * u + 3, _round_bf16(x), u), u)) for u in range(4)]
                for stage in range(5):
                    for u in range(4):
                        th[u][stage]()

            def batch(it, carry):
                bb = body_chunk(it)
                side = dinv_thunks(bb, lambda x: set_input(bb, _round_bf16(x), None))
                _interleave(batch_thunks(it // 4, it % 4), side)
                return carry
            _loop("batch", 0, 12, batch, 0)

        @pl.when(li == 1)
        def _():
            with jax.named_scope("dinv_out"):
                def store_out(bb, x):
                    xin[:, bb] = x.reshape(16, 8, DM).astype(bf16)
                    out_copy(bb).start()
                th = [dinv_thunks(bb, functools.partial(store_out, bb)) for bb in range(16)]
                for i in range(17):
                    if i < 16:
                        for f in th[i][:4]:
                            f()
                    if i >= 1:
                        th[i - 1][4]()
                for bb in range(16):
                    out_copy(bb).wait()
        return carry0

    lax.fori_loop(0, 2, layer, 0)


@functools.partial(jax.jit, static_argnames=("A_seg_len",))
def pallas_interleave_layers__memory_aug_recurrent_mem_tr__spectral_gfnet__prompt_kernel(
    A_x, A_mem0, A_Wq, A_Wk, A_Wv, A_Wo, A_seg_len, B_x, B_w_r, B_w_i,
):
    assert A_seg_len == SEG and A_x.shape == (1, S, DM)
    small, emat = _tables()
    hbm = pl.BlockSpec(memory_space=pltpu.HBM)
    vmem = pl.BlockSpec(memory_space=pltpu.VMEM)
    out = pl.pallas_call(
        _kernel,
        out_shape=jax.ShapeDtypeStruct((16, 16, 8, DM), bf16),
        in_specs=[hbm, vmem] + [hbm] * 8,
        out_specs=hbm,
        scratch_shapes=[
            pltpu.VMEM((16, 16, 8, DM), bf16),
            pltpu.VMEM((16, 128, DM), f32),
            pltpu.VMEM((18, 128, DM), f32),
            pltpu.VMEM((16, 128, DM), f32),
            pltpu.VMEM((2, 128, DM), f32),
            pltpu.VMEM((12, DM, 8, DH), bf16),
            pltpu.VMEM((H * DH + 512, DM), bf16),
            pltpu.VMEM((2560, 128), u32),
            pltpu.VMEM((96, 320, 128), u32),
            pltpu.VMEM((5, 2048 + 256, 128), u32),
            pltpu.VMEM((96, 4, 128, 128), f32),
            pltpu.VMEM((4, 5, 64, 128), u32),
            pltpu.VMEM((2, H, 32, 128), f32),
            pltpu.VMEM((2, 16, ZPITCH, 128), f32),
            pltpu.VMEM((2, 16, ZPITCH, 128), f32),
            pltpu.VMEM((2, 16, ZPITCH, 128), f32),
            pltpu.VMEM((6, 16 * WPITCH, 128), f32),
            pltpu.VMEM((2, DF, S), bf16),
            pltpu.VMEM((328, 128), f32),
            pltpu.VMEM((SMALL_ROWS, 128), u32),
            pltpu.VMEM((64, 64, 128), u32),
            pltpu.VMEM((80, 80), f32),
            pltpu.SemaphoreType.DMA((40,)),
            pltpu.SemaphoreType.DMA((16,)),
        ],
        compiler_params=pltpu.CompilerParams(vmem_limit_bytes=120 * 1024 * 1024),
    )(
        A_x.reshape(16, 16, 8, DM), A_mem0.reshape(MEM, DM),
        A_Wq, A_Wk, A_Wv, A_Wo.reshape(H * DH, DM), B_w_r.T, B_w_i.T,
        jnp.asarray(small), jnp.asarray(emat),
    )
    return out.reshape(1, S, DM)
```

```python
import functools
import math

import jax
import jax.numpy as jnp
import numpy as np
from jax import lax
import jax.experimental.pallas as pl
import jax.experimental.pallas.tpu as pltpu

f32, bf16, u32 = jnp.float32, jnp.bfloat16, jnp.uint32

S, DM, H, DH, MEM, SEG = 2048, 640, 32, 128, 8, 32
NSEG = S // SEG
NPAIR = H // 2
DF = DM // 2 + 1
EPS = 1e-5
WPITCH = 136

ZPITCH = 136

C1, C2 = math.cos(2 * math.pi / 5), math.cos(4 * math.pi / 5)
S1, S2 = math.sin(2 * math.pi / 5), math.sin(4 * math.pi / 5)


def _to_bf16_bits(a):
    u = np.ascontiguousarray(a, dtype=np.float32).view(np.uint32).astype(np.uint64)
    return ((u + 0x7FFF + ((u >> 16) & 1)) >> 16).astype(np.uint32)


def _pack_rows(a):
    b = _to_bf16_bits(a)
    return b[..., 0::2, :] | (b[..., 1::2, :] << 16)


@functools.lru_cache(maxsize=None)
def _tables():
    b = np.arange(128)
    l0 = np.arange(0, DF, 5)
    l1 = np.concatenate([np.arange(1, 320, 5), np.arange(4, 320, 5)])
    l2 = np.concatenate([np.arange(2, 320, 5), np.arange(3, 320, 5)])
    sg = np.concatenate([np.ones(64), -np.ones(64)])

    def th(l):
        return 2 * np.pi * ((b[:, None] * l[None, :]) % DM) / DM

    fw = np.zeros((6, 256, 128))
    t = th(l0)
    fw[0, :128, :65] = np.cos(t)
    fw[3, :128, :65] = -np.sin(t)
    for g, l in ((1, l1), (2, l2)):
        t = th(l)
        c, s = np.cos(t), np.sin(t)
        fw[g] = np.concatenate([c, -sg * s], axis=0)
        fw[3 + g] = np.concatenate([-s, -sg * c], axis=0)
    sc = 1.0 / (S * DM)
    iw = np.zeros((5, 256, 128))
    t = th(l0).T
    cl = np.full((65, 1), 2.0)
    cl[0] = cl[-1] = 1.0
    iw[0, :65] = cl * np.cos(t) * sc
    iw[0, 128:128 + 65] = -cl * np.sin(t) * sc
    for g, l in ((1, l1), (2, l2)):
        t = th(l).T
        c, s = np.cos(t), np.sin(t)
        gg = sg[:, None]
        iw[2 * g - 1] = 2 * sc * np.concatenate([c, -s], axis=0)
        iw[2 * g] = 2 * sc * np.concatenate([gg * s, gg * c], axis=0)
    n = np.arange(64)
    order = np.concatenate([np.concatenate([np.arange(8) + 8 * j, np.arange(8) + 8 * j + 64])
                            for j in range(8)])
    e = np.zeros((2, 32, 128, 128))
    for k2 in range(32):
        t = 2 * np.pi * (((32 * n[:, None] + k2) * n[None, :]) % S) / S
        er, ei = np.cos(t), -np.sin(t)
        m = np.block([[er, -ei], [ei, er]])[order][:, order]
        e[0, k2], e[1, k2] = m, m.T
    small = np.concatenate(
        [_pack_rows(fw).reshape(-1, 128), _pack_rows(iw).reshape(-1, 128)], axis=0)
    return small, _pack_rows(e).reshape(64, 64, 128)


FW_OFF, IW_OFF = 0, 6 * 128
SMALL_ROWS = 11 * 128


def _loop(name, lo, hi, body, init, **kw):
    with jax.named_scope(name):
        return lax.fori_loop(lo, hi, body, init, **kw)


def _bf(x):
    return pltpu.bitcast(x, bf16)


def _dot(a, b):
    return jnp.dot(a, b, preferred_element_type=f32)


def _round_bf16(x):
    return x.astype(bf16).astype(f32)


def _layernorm(x):
    m = jnp.mean(x, axis=-1, keepdims=True)
    xc = x - m
    v = jnp.mean(xc * xc, axis=-1, keepdims=True)
    return xc * lax.rsqrt(v + EPS)


def _fft4(x, sign):
    (ar, ai), (br, bi), (cr, ci), (dr, di) = x
    t0r, t0i, t1r, t1i = ar + cr, ai + ci, ar - cr, ai - ci
    t2r, t2i, t3r, t3i = br + dr, bi + di, br - dr, bi - di
    y0, y2 = (t0r + t2r, t0i + t2i), (t0r - t2r, t0i - t2i)
    p, q = (t1r + t3i, t1i - t3r), (t1r - t3i, t1i + t3r)
    return [y0, p, y2, q] if sign < 0 else [y0, q, y2, p]


def _twiddle(z, n, period, sign):
    zr, zi = z
    n = n % period
    if n == 0:
        return z
    if 4 * n == period:
        return (-zi, zr) if sign > 0 else (zi, -zr)
    c, s = math.cos(2 * math.pi * n / period), sign * math.sin(2 * math.pi * n / period)
    if (8 * n) % period == 0:
        a, d = zr + zi, zr - zi
        if c * s > 0:
            return (d * c, a * c)
        return (a * c, d * s)
    return (zr * c - zi * s, zr * s + zi * c)


def _ilv(r, i):
    n = r.shape[0] // 8
    return jnp.concatenate([r.reshape(n, 8, 128), i.reshape(n, 8, 128)], axis=1).reshape(16 * n, 128)


def _dilv(x):
    n = x.shape[0] // 16
    x = x.reshape(n, 16, 128)
    return x[:, :8].reshape(8 * n, 128), x[:, 8:].reshape(8 * n, 128)


def _with_tokens(x, toks):
    if not toks:
        return x
    return jnp.concatenate(
        [x[8 * j:8 * j + 8] | toks[j] if j in toks else x[8 * j:8 * j + 8]
         for j in range(x.shape[0] // 8)], axis=0)


def _fft16(x, sign, emit=None):
    cols = [_fft4([x[4 * j + r] for j in range(4)], sign) for r in range(4)]
    out = [None] * 16
    for q in range(4):
        y = _fft4([_twiddle(cols[r][q], r * q, 16, sign) for r in range(4)], sign)
        for p in range(4):
            out[q + 4 * p] = y[p]
        if emit is not None:
            emit(q, y)
    return out


CFG = dict(lat_s=6, lat_pv=15, lat_wo=7, n_after=(11, 11, 11, 0), fill_at=16, v_delay=8, v_gap=0,
           prenorm=True,
           pre_at=((), (), (), tuple(range(11, 91, 5))), pre_rows=((), (), (), tuple(range(16))),
           first=(0, 1), only=None)


def _interleave(main, side):
    n, k = len(main), 0
    for i, f in enumerate(main):
        f()
        while k < len(side) and (k + 1) * n <= (i + 1) * len(side):
            side[k]()
            k += 1
    for f in side[k:]:
        f()


def _kernel(x_hbm, mem_ref, wq_hbm, wk_hbm, wv_hbm, wo_hbm, wr_hbm, wi_hbm,
            small_hbm, e_hbm, out_hbm,
            xin, xa, xb, xn, ao, raw, wo_raw, tmp, w32, wo32, qb, hl, ol, z0, z1, z2, wf,
            wri, wtmp, small, emat, fill_ref, sem, osem):
    zs = (z0, z1, z2)
    w_hbm = (wq_hbm, wk_hbm, wv_hbm)

    def body_chunk(i):
        return i + i // 3

    def cp_w(i):
        src = w_hbm[i // 4 if isinstance(i, int) else 0]
        c = i % 4
        return pltpu.make_async_copy(src.at[:, pl.ds(pl.multiple_of(8 * c, 8), 8), :],
                                     raw.at[i], sem.at[i])

    def cp_x(bb):
        return pltpu.make_async_copy(x_hbm.at[:, bb], xin.at[:, bb], sem.at[12 + bb])

    def cp_wo(i):
        rows = pl.ds(pl.multiple_of(512 * i, 512), 512)
        return pltpu.make_async_copy(wo_hbm.at[rows], wo_raw.at[rows], sem.at[28 + i])

    cp_rest = [pltpu.make_async_copy(wr_hbm, wri.at[0], sem.at[36]),
               pltpu.make_async_copy(wi_hbm, wri.at[1], sem.at[37]),
               pltpu.make_async_copy(small_hbm, small, sem.at[38]),
               pltpu.make_async_copy(e_hbm, emat, sem.at[39])]

    full = CFG["only"] is None
    for u in range(4 if full else 0):
        cp_x(4 * u + 3).start()
    if full:
        cp_w(0).start()
    for i in range(12 if full else 0):
        if i < 11:
            cp_w(i + 1).start()
        cp_x(body_chunk(i)).start()
        if i >= 4:
            cp_wo(i - 4).start()
    for cp in cp_rest if full else ():
        cp.start()

    r = lax.broadcasted_iota(jnp.int32, (80, 80), 0)
    c = lax.broadcasted_iota(jnp.int32, (80, 80), 1)

    def head(i):
        return jnp.where(i < 64, i // 32, (i - 64) // 8)

    def pos(i):
        return jnp.where(i < 64, i % 32, 32 + (i - 64) % 8)

    ok = (pos(r) < MEM) | (pos(r) >= pos(c))
    fill_ref[...] = jnp.where(head(r) == head(c), jnp.where(ok, 0.0, -1e9), -jnp.inf).astype(f32)
    ol[...] = jnp.zeros_like(ol)
    ao[...] = jnp.zeros_like(ao)
    wtmp[320:328, :] = jnp.zeros((8, 128), f32)
    xb[17, 0:8, 0:128] = jnp.zeros((8, 128), f32)
    for z in zs:
        z[0, 0, 128:ZPITCH, :] = jnp.zeros((8, 128), f32)

    def chunk(bb):
        if isinstance(bb, int):
            return slice(8 * bb, 8 * bb + 8)
        return pl.ds(pl.multiple_of(8 * bb, 8), 8)

    def set_input(bb, x, tail_u):
        xa[:, chunk(bb), :] = x.reshape(16, 8, DM)
        y = _layernorm(x)
        if tail_u is None:
            xn[:, chunk(bb), :] = y.reshape(16, 8, DM)
        else:
            yb = y.astype(bf16)
            for kt in range(5):
                hl[tail_u, kt] = pltpu.bitcast(yb[:, 128 * kt:128 * kt + 128], u32)

    def load_x(bb):
        return xin[:, bb].astype(f32).reshape(128, DM)

    def relayout_thunks(m, c):
        def p1(i):
            v = raw[4 * m + c, 16 * i:16 * i + 16].reshape(128, 128)
            tmp[64 * i:64 * i + 64, :] = pltpu.bitcast(v, u32)

        def p2(i):
            for j in range(4):
                a = tmp[pl.ds(64 * i + j, 8, stride=8), :]
                b = tmp[pl.ds(64 * i + 4 + j, 8, stride=8), :]
                t = 6 * (4 * c + j) + 2 * m
                w32[t, 8 * i:8 * i + 8, :] = (a & 0xFFFF) | (b << 16)
                w32[t + 1, 8 * i:8 * i + 8, :] = (a >> 16) | (b & jnp.uint32(0xFFFF0000))

        def piece(i):
            def run():
                p1(i)
                p2(i)
            return run
        return [piece(i) for i in range(40)]

    def batch_thunks(m, c):
        def one(j, u, e):
            def run(toks=None):
                lhs = jnp.concatenate([_bf(hl[u, kt]) for kt in range(5)], axis=1)
                t = 6 * (4 * c + j) + 2 * m + e
                qb[t, u] = _dot(lhs, _bf(_with_tokens(w32[t], toks)))
            return run
        return [one(j, u, e) for j in range(4) for u in range(4) for e in range(2)]

    def wperm_thunks(m, kc):
        def load():
            w = wri[m, :, pl.ds(pl.multiple_of(kc * 128, 128), 128)].astype(f32)
            wtmp[0:DF, :] = w

        def one(g):
            def run():
                if g == 0:
                    t = jnp.concatenate([wtmp[pl.ds(0, 64, stride=5), :], wtmp[320:328, :],
                                         jnp.zeros((56, 128), f32)], axis=0)
                else:
                    t = jnp.concatenate([wtmp[pl.ds(g, 64, stride=5), :],
                                         wtmp[pl.ds(5 - g, 64, stride=5), :]], axis=0)
                y = t.T
                sub = wf.at[3 * m + g, pl.ds(pl.multiple_of(kc * 8, 8), 15 * WPITCH + 8)]
                for k in range(8):
                    for hf in range(2):
                        sub[pl.ds(k + 8 * hf * WPITCH, 8, stride=WPITCH), :] = (
                            y[16 * k + 8 * hf:16 * k + 8 * hf + 8])
            return run
        return [load] + [one(g) for g in range(3)]

    def wo_copy_thunks(c):
        def one(j):
            def run():
                wo32[j, pl.ds(pl.multiple_of(c * 256, 256), 256), :] = pltpu.bitcast(
                    wo_raw[pl.ds(pl.multiple_of(c * 512, 512), 512), 128 * j:128 * j + 128], u32)
            return run
        return [one(j) for j in range(5)]

    def pro0():
        for u in range(4):
            cp_x(4 * u + 3).wait()
        for u in range(4):
            set_input(4 * u + 3, load_x(4 * u + 3), u)
        cp_w(0).wait()
        for f in relayout_thunks(0, 0):
            f()

    def pro1(it, carry):
        @pl.when(it < 11)
        def _():
            cp_w(it + 1).wait()

        @pl.when(it >= 4)
        def _():
            cp_wo(it - 4).wait()
        bb = body_chunk(it)
        cp_x(bb).wait()
        nxt = jnp.minimum(it + 1, 11)
        set_input(bb, load_x(bb), None)
        for f in wo_copy_thunks(jnp.where(it >= 4, it - 4, 8)):
            f()
        _interleave(batch_thunks(it // 4, it % 4), relayout_thunks(nxt // 4, nxt % 4))
        return carry

    if full:
        with jax.named_scope("pro0"):
            pro0()
        _loop("pro1", 0, 12, pro1, 0)
        for cp in cp_rest:
            cp.wait()

    scale = DH ** -0.5

    def wo_dot(hh, oo):
        return [_dot(oo, _bf(wo32[j, 64 * hh:64 * hh + 64, :])) for j in range(5)]

    def addl(acc, res):
        return res if acc is None else [a + b for a, b in zip(acc, res)]

    def finish_thunks(gp, slot):
        st = {"acc": None}

        def f_wo(hh):
            def run():
                st["acc"] = addl(st["acc"], wo_dot(hh, ol[slot, hh].astype(bf16)))
                if hh == H - 1:
                    out = jnp.concatenate(st["acc"], axis=1)
                    for u in range(4):
                        ao[slot, 32 * u + 24:32 * u + 32, :] = out[8 * u:8 * u + 8]
            return run

        def pre(rows):
            x = _round_bf16(xa[gp, rows, :] + ao[slot, rows, :])
            xb[gp, rows, :] = x
            y = _layernorm(x)
            x0, x1, x2, x3, x4 = [y[:, 128 * a:128 * a + 128] for a in range(5)]
            t1, t2, t3, t4 = x1 + x4, x2 + x3, x1 - x4, x2 - x3
            xb[16, rows, :] = jnp.concatenate(
                [x0 + t1 + t2, x0 + C1 * t1 + C2 * t2, S1 * t3 + S2 * t4,
                 x0 + C2 * t1 + C1 * t2, S2 * t3 - S1 * t4], axis=1)

        def f_dft(cidx):
            def run(chunks=tuple(range(16))):
                g = cidx % 3
                o = FW_OFF + 128 * cidx
                lo, hi = (0, 128) if g == 0 else (256 * g - 128, 256 * g + 128)
                u = jnp.concatenate([xb[16, chunk(bb), lo:hi] for bb in chunks], axis=0)
                y = _dot(u.astype(bf16), _bf(small[o:o + (hi - lo) // 2, :]))
                for i, bb in enumerate(chunks):
                    zs[g][cidx // 3, gp, chunk(bb), :] = y[8 * i:8 * i + 8]
            return run
        return [f_wo(hh) for hh in range(H)], pre, [f_dft(cidx) for cidx in (0, 3, 1, 4, 2, 5)]

    def group(g, mem):
        cur = g % 2
        wos, pre, dfts = finish_thunks(jnp.maximum(g - 1, 0), 1 - cur)
        fillers = [wos[0:11], wos[11:22], wos[22:32], dfts]
        for ph in range(4):
            h = jnp.concatenate([mem, xn[g, 32 * ph:32 * ph + 24, :]], axis=0).astype(bf16)
            side = wperm_thunks(ph, g) if ph < 2 and CFG.get("wperm", True) else []
            pres = list(CFG["pre_rows"][ph])
            pre_at = CFG["pre_at"][ph]
            tok = None
            pr, sm, oos = {}, {}, {}

            def stacked(p, m):
                tails = [qb[6 * p + 2 * m + e, ph, chunk(g), :] for e in range(2)]
                return jnp.concatenate([pr[p, m, 0], pr[p, m, 1]] + tails, axis=0).astype(bf16)

            def scores(p):
                sc = lax.dot_general(stacked(p, 0), stacked(p, 1), (((1,), (1,)), ((), ())),
                                     preferred_element_type=f32)
                fill = fill_ref[...]
                sc = jnp.where(fill == 0.0, sc * scale, fill)
                mx = jnp.max(sc, axis=-1, keepdims=True)
                e = jnp.exp(sc - mx)
                rl = pl.reciprocal(jnp.sum(e, axis=-1, keepdims=True), approx=True)
                sm[p] = ((e * rl).astype(bf16), None) if CFG["prenorm"] else (e.astype(bf16), rl)

            def pv(p):
                e, rl = sm[p]
                o = _dot(e, stacked(p, 2))
                if rl is not None:
                    o = o * rl
                ol[cur, 2 * p, 8 * ph:8 * ph + 8, :] = o[64:72]
                ol[cur, 2 * p + 1, 8 * ph:8 * ph + 8, :] = o[72:80]
                oos[2 * p], oos[2 * p + 1] = o[0:32].astype(bf16), o[32:64].astype(bf16)

            acc, t, nwo = None, 0.0, 0
            keyed = []
            for p in range(NPAIR):
                keyed += [(4 * p + 2 * i + e, (p, m, e)) for i, m in enumerate(CFG["first"]) for e in range(2)]
                keyed += [(4 * p + 3.5 + CFG["v_delay"] + CFG["v_gap"] * e, (p, 2, e)) for e in range(2)]
            bulk = [x for _, x in sorted(keyed, key=lambda kv: kv[0])]
            pend, ready, fl = [], [], list(fillers[ph])
            n_after = CFG["n_after"][ph]
            while nwo < H:
                pend.sort()
                if pend and pend[0][0] <= t:
                    _, kind, p = pend.pop(0)
                    if kind == "S":
                        scores(p)
                        pend.append((t + CFG["lat_pv"], "V", p))
                    else:
                        pv(p)
                        ready += [(t + CFG["lat_wo"], 2 * p + e) for e in range(2)]
                    t += 0.5
                elif bulk:
                    p, m, e = bulk.pop(0)
                    pr[p, m, e] = _dot(h, _bf(_with_tokens(w32[6 * p + 2 * m + e], tok)))
                    tok = None
                    if 96 - len(bulk) in pre_at:
                        pre(chunk(pres.pop(0)))
                        tok = {0: pltpu.bitcast(xb[17 + g // 16, 0:8, 0:128], u32)}
                    t += 1
                    if m == CFG["first"][1] and e == 1:
                        pend.append((t + CFG["lat_s"], "S", p))
                    if side and len(bulk) % 18 == 0:
                        side.pop(0)()
                elif nwo >= CFG["fill_at"] and len(fl) > n_after:
                    fl.pop(0)()
                    t += 1
                elif ready and ready[0][0] <= t:
                    _, hh = ready.pop(0)
                    acc = addl(acc, wo_dot(hh, oos[hh]))
                    t += 1
                    nwo += 1
                elif len(fl) > n_after:
                    fl.pop(0)()
                    t += 1
                else:
                    t += 0.5
            out = jnp.concatenate(acc, axis=1)
            ao[cur, 32 * ph:32 * ph + 24, :] = out[8:32]
            mem = _round_bf16(out[0:8])
            for f in fl:
                f()
        return mem

    def spectral(zero):
        def fence(z):
            return z[0, zero, 128:ZPITCH, :]

        def radix_fwd(g, bb, tok=None):
            z = zs[g]
            xs = [(z[0, a, chunk(bb), :], z[1, a, chunk(bb), :]) for a in range(16)]
            if tok is not None:
                xs[:4] = [(xr + tok, xi) for xr, xi in xs[:4]]
            toks = []

            def emit(q, y):
                for p in range(4):
                    z[0, q + 4 * p, chunk(bb), :] = y[p][0]
                    z[1, q + 4 * p, chunk(bb), :] = y[p][1]
                if g > 0 or q == 3:
                    toks.append(fence(z))
            _fft16(xs, -1, emit)
            return toks

        ys = {}

        def fwd(g, k2, toks):
            z = zs[g]
            ur, ui = z[0, k2, 0:64, :], z[1, k2, 0:64, :]
            tr, ti = _twiddle((z[0, k2, 64:128, :], z[1, k2, 64:128, :]), k2, 32, -1)
            for hf in range(2):
                v = _ilv(ur + tr, ui + ti) if hf == 0 else _ilv(ur - tr, ui - ti)
                lhs = _with_tokens(emat[k2 + 16 * hf], toks if hf == 0 else None)
                xr, xi = _dilv(_dot(_bf(lhs), v.astype(bf16)))
                wr = wf[g, pl.ds(k2 * WPITCH + hf, 64, stride=2), :]
                wi = wf[g + 3, pl.ds(k2 * WPITCH + hf, 64, stride=2), :]
                ys[g, k2, hf] = _ilv(xr * wr - xi * wi, xr * wi + xi * wr).astype(bf16)

        def inv(g, k2):
            z = zs[g]
            t0 = _dot(_bf(emat[32 + k2]), ys.pop((g, k2, 0)))
            t1 = _dot(_bf(emat[48 + k2]), ys.pop((g, k2, 1)))
            z[0, k2, 0:64, :], z[1, k2, 0:64, :] = _dilv(t0 + t1)
            z[0, k2, 64:128, :], z[1, k2, 64:128, :] = _twiddle(_dilv(t0 - t1), k2, 32, 1)

        chain = {}
        for bb in range(16):
            chain[bb] = radix_fwd(0, bb, chain.get(bb - 2))[-1]
        radix_fwd(1, 0)
        units = [(g, k2) for g in range(3) for k2 in range(16)]
        toks = None
        for i in range(len(units) + 3):
            if i < len(units):
                fwd(*units[i], toks)
            if i >= 3:
                inv(*units[i - 3])
            toks = None
            if i < 31:
                t4 = radix_fwd(1 + (i + 1) // 16, (i + 1) % 16)
                toks = {3 + j: pltpu.bitcast(t, u32) for j, t in enumerate(t4)}

    def dinv_thunks(bb, finish):
        st = {}

        def rad(g):
            def run():
                z = zs[g]
                ys = _fft16([(z[0, a, chunk(bb), :], z[1, a, chunk(bb), :]) for a in range(16)], 1)
                st[g] = jnp.concatenate(
                    [jnp.concatenate([y[0] for y in ys], axis=0),
                     jnp.concatenate([y[1] for y in ys], axis=0)], axis=1).astype(bf16)
            return run

        def mm():
            st["p"] = [_dot(st[(j + 1) // 2], _bf(small[IW_OFF + 128 * j:IW_OFF + 128 * (j + 1), :]))
                       for j in range(5)]

        def fin():
            p0, p1, q1, p2, q2 = st["p"]
            e1, o1 = p0 + C1 * p1 + C2 * p2, S1 * q1 + S2 * q2
            e2, o2 = p0 + C2 * p1 + C1 * p2, S2 * q1 - S1 * q2
            y = jnp.concatenate([p0 + p1 + p2, e1 - o1, e2 - o2, e2 + o2, e1 + o1], axis=1)
            finish(xb[0:16, chunk(bb), :].reshape(128, DM) + y)
        return [rad(0), rad(1), rad(2), mm, fin]

    def out_copy(bb):
        return pltpu.make_async_copy(xin.at[:, bb], out_hbm.at[:, bb], osem.at[bb])

    def layer(li, carry0):
        if full or CFG["only"] == "group":
            _loop("step", 0, 16, group, mem_ref[...].astype(f32))
        if full or CFG["only"] == "spec":
            @pl.when(li // 2 == 0)
            def _():
                with jax.named_scope("tail"):
                    wos, pre, dfts = finish_thunks(15, 1)
                    body = [bb for bb in range(16) if bb % 4 != 3]
                    for bb in body:
                        pre(chunk(bb))
                    for f in wos:
                        f()
                    for f in dfts:
                        f(body)
                    for bb in (3, 7, 11, 15):
                        pre(chunk(bb))
                    for f in dfts:
                        f((3, 7, 11, 15))
            with jax.named_scope("spectral"):
                spectral(li // 2)
        if not full:
            return carry0

        @pl.when(li == 0)
        def _():
            with jax.named_scope("dinv_tails"):
                th = [dinv_thunks(4 * u + 3, functools.partial(
                    lambda u, x: set_input(4 * u + 3, _round_bf16(x), u), u)) for u in range(4)]
                for stage in range(5):
                    for u in range(4):
                        th[u][stage]()

            def batch(it, carry):
                bb = body_chunk(it)
                side = dinv_thunks(bb, lambda x: set_input(bb, _round_bf16(x), None))
                _interleave(batch_thunks(it // 4, it % 4), side)
                return carry
            _loop("batch", 0, 12, batch, 0)

        @pl.when(li == 1)
        def _():
            with jax.named_scope("dinv_out"):
                def store_out(bb, x):
                    xin[:, bb] = x.reshape(16, 8, DM).astype(bf16)
                    out_copy(bb).start()
                th = [dinv_thunks(bb, functools.partial(store_out, bb)) for bb in range(16)]
                for i in range(17):
                    if i < 16:
                        for f in th[i][:4]:
                            f()
                    if i >= 1:
                        th[i - 1][4]()
                for bb in range(16):
                    out_copy(bb).wait()
        return carry0

    lax.fori_loop(0, 2, layer, 0)


@functools.partial(jax.jit, static_argnames=("A_seg_len",))
def pallas_interleave_layers__memory_aug_recurrent_mem_tr__spectral_gfnet__prompt_kernel(
    A_x, A_mem0, A_Wq, A_Wk, A_Wv, A_Wo, A_seg_len, B_x, B_w_r, B_w_i,
):
    assert A_seg_len == SEG and A_x.shape == (1, S, DM)
    small, emat = _tables()
    hbm = pl.BlockSpec(memory_space=pltpu.HBM)
    vmem = pl.BlockSpec(memory_space=pltpu.VMEM)
    out = pl.pallas_call(
        _kernel,
        out_shape=jax.ShapeDtypeStruct((16, 16, 8, DM), bf16),
        in_specs=[hbm, vmem] + [hbm] * 8,
        out_specs=hbm,
        scratch_shapes=[
            pltpu.VMEM((16, 16, 8, DM), bf16),
            pltpu.VMEM((16, 128, DM), f32),
            pltpu.VMEM((18, 128, DM), f32),
            pltpu.VMEM((16, 128, DM), f32),
            pltpu.VMEM((2, 128, DM), f32),
            pltpu.VMEM((12, DM, 8, DH), bf16),
            pltpu.VMEM((H * DH + 512, DM), bf16),
            pltpu.VMEM((2560, 128), u32),
            pltpu.VMEM((96, 320, 128), u32),
            pltpu.VMEM((5, 2048 + 256, 128), u32),
            pltpu.VMEM((96, 4, 128, 128), f32),
            pltpu.VMEM((4, 5, 64, 128), u32),
            pltpu.VMEM((2, H, 32, 128), f32),
            pltpu.VMEM((2, 16, ZPITCH, 128), f32),
            pltpu.VMEM((2, 16, ZPITCH, 128), f32),
            pltpu.VMEM((2, 16, ZPITCH, 128), f32),
            pltpu.VMEM((6, 16 * WPITCH, 128), f32),
            pltpu.VMEM((2, DF, S), bf16),
            pltpu.VMEM((328, 128), f32),
            pltpu.VMEM((SMALL_ROWS, 128), u32),
            pltpu.VMEM((64, 64, 128), u32),
            pltpu.VMEM((80, 80), f32),
            pltpu.SemaphoreType.DMA((40,)),
            pltpu.SemaphoreType.DMA((16,)),
        ],
        compiler_params=pltpu.CompilerParams(vmem_limit_bytes=120 * 1024 * 1024),
    )(
        A_x.reshape(16, 16, 8, DM), A_mem0.reshape(MEM, DM),
        A_Wq, A_Wk, A_Wv, A_Wo.reshape(H * DH, DM), B_w_r.T, B_w_i.T,
        jnp.asarray(small), jnp.asarray(emat),
    )
    return out.reshape(1, S, DM)
```

```python
import functools
import math

import jax
import jax.numpy as jnp
import numpy as np
from jax import lax
import jax.experimental.pallas as pl
import jax.experimental.pallas.tpu as pltpu

f32, bf16, u32 = jnp.float32, jnp.bfloat16, jnp.uint32

S, DM, H, DH, MEM, SEG = 2048, 640, 32, 128, 8, 32
NSEG = S // SEG
NPAIR = H // 2
DF = DM // 2 + 1
EPS = 1e-5
WPITCH = 136

ZPITCH = 136

C1, C2 = math.cos(2 * math.pi / 5), math.cos(4 * math.pi / 5)
S1, S2 = math.sin(2 * math.pi / 5), math.sin(4 * math.pi / 5)


def _to_bf16_bits(a):
    u = np.ascontiguousarray(a, dtype=np.float32).view(np.uint32).astype(np.uint64)
    return ((u + 0x7FFF + ((u >> 16) & 1)) >> 16).astype(np.uint32)


def _pack_rows(a):
    b = _to_bf16_bits(a)
    return b[..., 0::2, :] | (b[..., 1::2, :] << 16)


@functools.lru_cache(maxsize=None)
def _tables():
    b = np.arange(128)
    l0 = np.arange(0, DF, 5)
    l1 = np.concatenate([np.arange(1, 320, 5), np.arange(4, 320, 5)])
    l2 = np.concatenate([np.arange(2, 320, 5), np.arange(3, 320, 5)])
    sg = np.concatenate([np.ones(64), -np.ones(64)])

    def th(l):
        return 2 * np.pi * ((b[:, None] * l[None, :]) % DM) / DM

    fw = np.zeros((6, 256, 128))
    t = th(l0)
    fw[0, :128, :65] = np.cos(t)
    fw[3, :128, :65] = -np.sin(t)
    for g, l in ((1, l1), (2, l2)):
        t = th(l)
        c, s = np.cos(t), np.sin(t)
        fw[g] = np.concatenate([c, -sg * s], axis=0)
        fw[3 + g] = np.concatenate([-s, -sg * c], axis=0)
    sc = 1.0 / (S * DM)
    iw = np.zeros((5, 256, 128))
    t = th(l0).T
    cl = np.full((65, 1), 2.0)
    cl[0] = cl[-1] = 1.0
    iw[0, :65] = cl * np.cos(t) * sc
    iw[0, 128:128 + 65] = -cl * np.sin(t) * sc
    for g, l in ((1, l1), (2, l2)):
        t = th(l).T
        c, s = np.cos(t), np.sin(t)
        gg = sg[:, None]
        iw[2 * g - 1] = 2 * sc * np.concatenate([c, -s], axis=0)
        iw[2 * g] = 2 * sc * np.concatenate([gg * s, gg * c], axis=0)
    n = np.arange(64)
    order = np.concatenate([np.concatenate([np.arange(8) + 8 * j, np.arange(8) + 8 * j + 64])
                            for j in range(8)])
    e = np.zeros((2, 32, 128, 128))
    for k2 in range(32):
        t = 2 * np.pi * (((32 * n[:, None] + k2) * n[None, :]) % S) / S
        er, ei = np.cos(t), -np.sin(t)
        m = np.block([[er, -ei], [ei, er]])[order][:, order]
        e[0, k2], e[1, k2] = m, m.T
    small = np.concatenate(
        [_pack_rows(fw).reshape(-1, 128), _pack_rows(iw).reshape(-1, 128)], axis=0)
    return small, _pack_rows(e).reshape(64, 64, 128)


FW_OFF, IW_OFF = 0, 6 * 128
SMALL_ROWS = 11 * 128


def _loop(name, lo, hi, body, init, **kw):
    with jax.named_scope(name):
        return lax.fori_loop(lo, hi, body, init, **kw)


def _bf(x):
    return pltpu.bitcast(x, bf16)


def _dot(a, b):
    return jnp.dot(a, b, preferred_element_type=f32)


def _round_bf16(x):
    return x.astype(bf16).astype(f32)


def _layernorm(x):
    m = jnp.mean(x, axis=-1, keepdims=True)
    xc = x - m
    v = jnp.mean(xc * xc, axis=-1, keepdims=True)
    return xc * lax.rsqrt(v + EPS)


def _fft4(x, sign):
    (ar, ai), (br, bi), (cr, ci), (dr, di) = x
    t0r, t0i, t1r, t1i = ar + cr, ai + ci, ar - cr, ai - ci
    t2r, t2i, t3r, t3i = br + dr, bi + di, br - dr, bi - di
    y0, y2 = (t0r + t2r, t0i + t2i), (t0r - t2r, t0i - t2i)
    p, q = (t1r + t3i, t1i - t3r), (t1r - t3i, t1i + t3r)
    return [y0, p, y2, q] if sign < 0 else [y0, q, y2, p]


def _twiddle(z, n, period, sign):
    zr, zi = z
    n = n % period
    if n == 0:
        return z
    if 4 * n == period:
        return (-zi, zr) if sign > 0 else (zi, -zr)
    c, s = math.cos(2 * math.pi * n / period), sign * math.sin(2 * math.pi * n / period)
    if (8 * n) % period == 0:
        a, d = zr + zi, zr - zi
        if c * s > 0:
            return (d * c, a * c)
        return (a * c, d * s)
    return (zr * c - zi * s, zr * s + zi * c)


def _ilv(r, i):
    n = r.shape[0] // 8
    return jnp.concatenate([r.reshape(n, 8, 128), i.reshape(n, 8, 128)], axis=1).reshape(16 * n, 128)


def _dilv(x):
    n = x.shape[0] // 16
    x = x.reshape(n, 16, 128)
    return x[:, :8].reshape(8 * n, 128), x[:, 8:].reshape(8 * n, 128)


def _with_tokens(x, toks):
    if not toks:
        return x
    return jnp.concatenate(
        [x[8 * j:8 * j + 8] | toks[j] if j in toks else x[8 * j:8 * j + 8]
         for j in range(x.shape[0] // 8)], axis=0)


def _fft16(x, sign, emit=None):
    cols = [_fft4([x[4 * j + r] for j in range(4)], sign) for r in range(4)]
    out = [None] * 16
    for q in range(4):
        y = _fft4([_twiddle(cols[r][q], r * q, 16, sign) for r in range(4)], sign)
        for p in range(4):
            out[q + 4 * p] = y[p]
        if emit is not None:
            emit(q, y)
    return out


CFG = dict(lat_s=6, lat_pv=15, lat_wo=7, n_after=(11, 11, 11, 0), fill_at=16, v_delay=8, v_gap=0,
           prenorm=True,
           pre_at=((), (), (), tuple(range(11, 91, 5))), pre_rows=((), (), (), tuple(range(16))),
           first=(0, 1), only=None)


def _interleave(main, side):
    n, k = len(main), 0
    for i, f in enumerate(main):
        f()
        while k < len(side) and (k + 1) * n <= (i + 1) * len(side):
            side[k]()
            k += 1
    for f in side[k:]:
        f()


def _kernel(x_hbm, mem_ref, wq_hbm, wk_hbm, wv_hbm, wo_hbm, wr_hbm, wi_hbm,
            small_hbm, e_hbm, out_hbm,
            xin, xa, xb, xn, ao, raw, wo_raw, tmp, w32, wo32, qb, hl, ol, z0, z1, z2, wf,
            wri, wtmp, small, emat, fill_ref, sem, osem):
    zs = (z0, z1, z2)
    w_hbm = (wq_hbm, wk_hbm, wv_hbm)

    def body_chunk(i):
        return i + i // 3

    def cp_w(i):
        src = w_hbm[i // 4 if isinstance(i, int) else 0]
        c = i % 4
        return pltpu.make_async_copy(src.at[:, pl.ds(pl.multiple_of(8 * c, 8), 8), :],
                                     raw.at[i], sem.at[i])

    def cp_x(bb):
        return pltpu.make_async_copy(x_hbm.at[:, bb], xin.at[:, bb], sem.at[12 + bb])

    def cp_wo(i):
        rows = pl.ds(pl.multiple_of(512 * i, 512), 512)
        return pltpu.make_async_copy(wo_hbm.at[rows], wo_raw.at[rows], sem.at[28 + i])

    def cp_f(i):
        src = (wr_hbm, wi_hbm)[i // 4 if isinstance(i, int) else 0]
        cols = pl.ds(pl.multiple_of(512 * (i % 4), 512), 512)
        return pltpu.make_async_copy(src.at[:, cols], wri.at[i], sem.at[36 + i])

    cp_rest = [pltpu.make_async_copy(small_hbm, small, sem.at[44]),
               pltpu.make_async_copy(e_hbm, emat, sem.at[45])]

    full = CFG["only"] is None
    for u in range(4 if full else 0):
        cp_x(4 * u + 3).start()
    if full:
        cp_w(0).start()
    for i in range(12 if full else 0):
        if i < 11:
            cp_w(i + 1).start()
        cp_x(body_chunk(i)).start()
        if i >= 4:
            cp_wo(i - 4).start()
            cp_f(i - 4).start()
    for cp in cp_rest if full else ():
        cp.start()

    r = lax.broadcasted_iota(jnp.int32, (80, 80), 0)
    c = lax.broadcasted_iota(jnp.int32, (80, 80), 1)

    def head(i):
        return jnp.where(i < 64, i // 32, (i - 64) // 8)

    def pos(i):
        return jnp.where(i < 64, i % 32, 32 + (i - 64) % 8)

    ok = (pos(r) < MEM) | (pos(r) >= pos(c))
    fill_ref[...] = jnp.where(head(r) == head(c), jnp.where(ok, 0.0, -1e9), -jnp.inf).astype(f32)
    ol[...] = jnp.zeros_like(ol)
    ao[...] = jnp.zeros_like(ao)
    wtmp[:, 320:328, :] = jnp.zeros((4, 8, 128), f32)
    xb[17, 0:8, 0:128] = jnp.zeros((8, 128), f32)
    for z in zs:
        z[0, 0, 128:ZPITCH, :] = jnp.zeros((8, 128), f32)

    def chunk(bb):
        if isinstance(bb, int):
            return slice(8 * bb, 8 * bb + 8)
        return pl.ds(pl.multiple_of(8 * bb, 8), 8)

    def set_input(bb, x, tail_u):
        xa[:, chunk(bb), :] = x.reshape(16, 8, DM)
        y = _layernorm(x)
        if tail_u is None:
            xn[:, chunk(bb), :] = y.reshape(16, 8, DM)
        else:
            yb = y.astype(bf16)
            for kt in range(5):
                hl[tail_u, kt] = pltpu.bitcast(yb[:, 128 * kt:128 * kt + 128], u32)

    def load_x(bb):
        return xin[:, bb].astype(f32).reshape(128, DM)

    def relayout_thunks(m, c):
        def p1(i):
            v = raw[4 * m + c, 16 * i:16 * i + 16].reshape(128, 128)
            tmp[64 * i:64 * i + 64, :] = pltpu.bitcast(v, u32)

        def p2(i):
            for j in range(4):
                a = tmp[pl.ds(64 * i + j, 8, stride=8), :]
                b = tmp[pl.ds(64 * i + 4 + j, 8, stride=8), :]
                t = 6 * (4 * c + j) + 2 * m
                w32[t, 8 * i:8 * i + 8, :] = (a & 0xFFFF) | (b << 16)
                w32[t + 1, 8 * i:8 * i + 8, :] = (a >> 16) | (b & jnp.uint32(0xFFFF0000))

        def piece(i):
            def run():
                p1(i)
                p2(i)
            return run
        return [piece(i) for i in range(40)]

    def batch_thunks(m, c):
        def one(j, u, e):
            def run(toks=None):
                lhs = jnp.concatenate([_bf(hl[u, kt]) for kt in range(5)], axis=1)
                t = 6 * (4 * c + j) + 2 * m + e
                qb[:, u, t] = _dot(lhs, _bf(_with_tokens(w32[t], toks))).reshape(16, 8, 128)
            return run
        return [one(j, u, e) for j in range(4) for u in range(4) for e in range(2)]

    def wperm_thunks(piece, j):
        m = (piece // 4) % 2
        kc = jnp.where(piece < 8, 4 * (piece % 4) + j, 16)
        wt = wtmp.at[j]

        def load():
            wt[0:DF, :] = wri[piece, :, 128 * j:128 * j + 128].astype(f32)

        def one(g):
            def run():
                if g == 0:
                    t = jnp.concatenate([wt[pl.ds(0, 64, stride=5), :], wt[320:328, :],
                                         jnp.zeros((56, 128), f32)], axis=0)
                else:
                    t = jnp.concatenate([wt[pl.ds(g, 64, stride=5), :],
                                         wt[pl.ds(5 - g, 64, stride=5), :]], axis=0)
                y = t.T
                sub = wf.at[3 * m + g, pl.ds(pl.multiple_of(kc * 8, 8), 15 * WPITCH + 8)]
                for k in range(8):
                    for hf in range(2):
                        sub[pl.ds(k + 8 * hf * WPITCH, 8, stride=WPITCH), :] = (
                            y[16 * k + 8 * hf:16 * k + 8 * hf + 8])
            return run
        return [load] + [one(g) for g in range(3)]

    def wo_copy_thunks(c):
        def one(j):
            def run():
                wo32[j, pl.ds(pl.multiple_of(c * 256, 256), 256), :] = pltpu.bitcast(
                    wo_raw[pl.ds(pl.multiple_of(c * 512, 512), 512), 128 * j:128 * j + 128], u32)
            return run
        return [one(j) for j in range(5)]

    def pro0():
        for u in range(4):
            cp_x(4 * u + 3).wait()
        for u in range(4):
            set_input(4 * u + 3, load_x(4 * u + 3), u)
        cp_w(0).wait()
        for f in relayout_thunks(0, 0):
            f()

    def pro1(it, carry):
        @pl.when(it < 11)
        def _():
            cp_w(it + 1).wait()

        @pl.when(it >= 4)
        def _():
            cp_wo(it - 4).wait()
            cp_f(it - 4).wait()
        bb = body_chunk(it)
        cp_x(bb).wait()
        nxt = jnp.minimum(it + 1, 11)
        set_input(bb, load_x(bb), None)
        piece = jnp.where(it >= 4, it - 4, 8)
        for f in wo_copy_thunks(piece):
            f()
        for j in range(4):
            for f in wperm_thunks(piece, j):
                f()
        _interleave(batch_thunks(it // 4, it % 4), relayout_thunks(nxt // 4, nxt % 4))
        return carry

    if full:
        with jax.named_scope("pro0"):
            pro0()
        _loop("pro1", 0, 12, pro1, 0)
        for cp in cp_rest:
            cp.wait()

    scale = DH ** -0.5

    def wo_dot(hh, oo):
        return [_dot(oo, _bf(wo32[j, 64 * hh:64 * hh + 64, :])) for j in range(5)]

    def addl(acc, res):
        return res if acc is None else [a + b for a, b in zip(acc, res)]

    def finish_thunks(gp, slot):
        st = {"acc": None}

        def f_wo(hh):
            def run():
                st["acc"] = addl(st["acc"], wo_dot(hh, ol[slot, hh].astype(bf16)))
                if hh == H - 1:
                    out = jnp.concatenate(st["acc"], axis=1)
                    for u in range(4):
                        ao[slot, 32 * u + 24:32 * u + 32, :] = out[8 * u:8 * u + 8]
            return run

        def pre(rows):
            x = _round_bf16(xa[gp, rows, :] + ao[slot, rows, :])
            xb[gp, rows, :] = x
            y = _layernorm(x)
            x0, x1, x2, x3, x4 = [y[:, 128 * a:128 * a + 128] for a in range(5)]
            t1, t2, t3, t4 = x1 + x4, x2 + x3, x1 - x4, x2 - x3
            xb[16, rows, :] = jnp.concatenate(
                [x0 + t1 + t2, x0 + C1 * t1 + C2 * t2, S1 * t3 + S2 * t4,
                 x0 + C2 * t1 + C1 * t2, S2 * t3 - S1 * t4], axis=1)

        def f_dft(cidx):
            def run(chunks=tuple(range(16))):
                g = cidx % 3
                o = FW_OFF + 128 * cidx
                lo, hi = (0, 128) if g == 0 else (256 * g - 128, 256 * g + 128)
                u = jnp.concatenate([xb[16, chunk(bb), lo:hi] for bb in chunks], axis=0)
                y = _dot(u.astype(bf16), _bf(small[o:o + (hi - lo) // 2, :]))
                for i, bb in enumerate(chunks):
                    zs[g][cidx // 3, gp, chunk(bb), :] = y[8 * i:8 * i + 8]
            return run
        return [f_wo(hh) for hh in range(H)], pre, [f_dft(cidx) for cidx in (0, 3, 1, 4, 2, 5)]

    def group(g, mem):
        cur = g % 2
        wos, pre, dfts = finish_thunks(jnp.maximum(g - 1, 0), 1 - cur)
        fillers = [wos[0:11], wos[11:22], wos[22:32], dfts]
        for ph in range(4):
            h = jnp.concatenate([mem, xn[g, 32 * ph:32 * ph + 24, :]], axis=0).astype(bf16)
            pres = list(CFG["pre_rows"][ph])
            pre_at = CFG["pre_at"][ph]
            tok = None
            pr, sm, oos = {}, {}, {}

            def stacked(p, m):
                tails = [qb[g, ph, 6 * p + 2 * m + e] for e in range(2)]
                return jnp.concatenate([pr[p, m, 0], pr[p, m, 1]] + tails, axis=0).astype(bf16)

            def scores(p):
                sc = lax.dot_general(stacked(p, 0), stacked(p, 1), (((1,), (1,)), ((), ())),
                                     preferred_element_type=f32)
                fill = fill_ref[...]
                sc = jnp.where(fill == 0.0, sc * scale, fill)
                mx = jnp.max(sc, axis=-1, keepdims=True)
                e = jnp.exp(sc - mx)
                rl = pl.reciprocal(jnp.sum(e, axis=-1, keepdims=True), approx=True)
                sm[p] = ((e * rl).astype(bf16), None) if CFG["prenorm"] else (e.astype(bf16), rl)

            def pv(p):
                e, rl = sm[p]
                o = _dot(e, stacked(p, 2))
                if rl is not None:
                    o = o * rl
                ol[cur, 2 * p, 8 * ph:8 * ph + 8, :] = o[64:72]
                ol[cur, 2 * p + 1, 8 * ph:8 * ph + 8, :] = o[72:80]
                oos[2 * p], oos[2 * p + 1] = o[0:32].astype(bf16), o[32:64].astype(bf16)

            acc, t, nwo = None, 0.0, 0
            keyed = []
            for p in range(NPAIR):
                keyed += [(4 * p + 2 * i + e, (p, m, e)) for i, m in enumerate(CFG["first"]) for e in range(2)]
                keyed += [(4 * p + 3.5 + CFG["v_delay"] + CFG["v_gap"] * e, (p, 2, e)) for e in range(2)]
            bulk = [x for _, x in sorted(keyed, key=lambda kv: kv[0])]
            pend, ready, fl = [], [], list(fillers[ph])
            n_after = CFG["n_after"][ph]
            while nwo < H:
                pend.sort()
                if pend and pend[0][0] <= t:
                    _, kind, p = pend.pop(0)
                    if kind == "S":
                        scores(p)
                        pend.append((t + CFG["lat_pv"], "V", p))
                    else:
                        pv(p)
                        ready += [(t + CFG["lat_wo"], 2 * p + e) for e in range(2)]
                    t += 0.5
                elif bulk:
                    p, m, e = bulk.pop(0)
                    pr[p, m, e] = _dot(h, _bf(_with_tokens(w32[6 * p + 2 * m + e], tok)))
                    tok = None
                    if 96 - len(bulk) in pre_at:
                        pre(chunk(pres.pop(0)))
                        tok = {0: pltpu.bitcast(xb[17 + g // 16, 0:8, 0:128], u32)}
                    t += 1
                    if m == CFG["first"][1] and e == 1:
                        pend.append((t + CFG["lat_s"], "S", p))
                elif nwo >= CFG["fill_at"] and len(fl) > n_after:
                    fl.pop(0)()
                    t += 1
                elif ready and ready[0][0] <= t:
                    _, hh = ready.pop(0)
                    acc = addl(acc, wo_dot(hh, oos[hh]))
                    t += 1
                    nwo += 1
                elif len(fl) > n_after:
                    fl.pop(0)()
                    t += 1
                else:
                    t += 0.5
            out = jnp.concatenate(acc, axis=1)
            ao[cur, 32 * ph:32 * ph + 24, :] = out[8:32]
            mem = _round_bf16(out[0:8])
            for f in fl:
                f()
        return mem

    def spectral(zero):
        def fence(z):
            return z[0, zero, 128:ZPITCH, :]

        def radix_fwd(g, bb, tok=None):
            z = zs[g]
            xs = [(z[0, a, chunk(bb), :], z[1, a, chunk(bb), :]) for a in range(16)]
            if tok is not None:
                xs[:4] = [(xr + tok, xi) for xr, xi in xs[:4]]
            toks = []

            def emit(q, y):
                for p in range(4):
                    z[0, q + 4 * p, chunk(bb), :] = y[p][0]
                    z[1, q + 4 * p, chunk(bb), :] = y[p][1]
                if g > 0 or q == 3:
                    toks.append(fence(z))
            _fft16(xs, -1, emit)
            return toks

        ys = {}

        def fwd(g, k2, toks):
            z = zs[g]
            ur, ui = z[0, k2, 0:64, :], z[1, k2, 0:64, :]
            tr, ti = _twiddle((z[0, k2, 64:128, :], z[1, k2, 64:128, :]), k2, 32, -1)
            for hf in range(2):
                v = _ilv(ur + tr, ui + ti) if hf == 0 else _ilv(ur - tr, ui - ti)
                lhs = _with_tokens(emat[k2 + 16 * hf], toks if hf == 0 else None)
                xr, xi = _dilv(_dot(_bf(lhs), v.astype(bf16)))
                wr = wf[g, pl.ds(k2 * WPITCH + hf, 64, stride=2), :]
                wi = wf[g + 3, pl.ds(k2 * WPITCH + hf, 64, stride=2), :]
                ys[g, k2, hf] = _ilv(xr * wr - xi * wi, xr * wi + xi * wr).astype(bf16)

        def inv(g, k2):
            z = zs[g]
            t0 = _dot(_bf(emat[32 + k2]), ys.pop((g, k2, 0)))
            t1 = _dot(_bf(emat[48 + k2]), ys.pop((g, k2, 1)))
            z[0, k2, 0:64, :], z[1, k2, 0:64, :] = _dilv(t0 + t1)
            z[0, k2, 64:128, :], z[1, k2, 64:128, :] = _twiddle(_dilv(t0 - t1), k2, 32, 1)

        chain = {}
        for bb in range(16):
            chain[bb] = radix_fwd(0, bb, chain.get(bb - 2))[-1]
        radix_fwd(1, 0)
        units = [(g, k2) for g in range(3) for k2 in range(16)]
        toks = None
        for i in range(len(units) + 3):
            if i < len(units):
                fwd(*units[i], toks)
            if i >= 3:
                inv(*units[i - 3])
            toks = None
            if i < 31:
                t4 = radix_fwd(1 + (i + 1) // 16, (i + 1) % 16)
                toks = {3 + j: pltpu.bitcast(t, u32) for j, t in enumerate(t4)}

    def dinv_thunks(bb, finish):
        st = {}

        def rad(g):
            def run():
                z = zs[g]
                ys = _fft16([(z[0, a, chunk(bb), :], z[1, a, chunk(bb), :]) for a in range(16)], 1)
                st[g] = jnp.concatenate(
                    [jnp.concatenate([y[0] for y in ys], axis=0),
                     jnp.concatenate([y[1] for y in ys], axis=0)], axis=1).astype(bf16)
            return run

        def mm():
            st["p"] = [_dot(st[(j + 1) // 2], _bf(small[IW_OFF + 128 * j:IW_OFF + 128 * (j + 1), :]))
                       for j in range(5)]

        def fin():
            p0, p1, q1, p2, q2 = st["p"]
            e1, o1 = p0 + C1 * p1 + C2 * p2, S1 * q1 + S2 * q2
            e2, o2 = p0 + C2 * p1 + C1 * p2, S2 * q1 - S1 * q2
            y = jnp.concatenate([p0 + p1 + p2, e1 - o1, e2 - o2, e2 + o2, e1 + o1], axis=1)
            finish(xb[0:16, chunk(bb), :].reshape(128, DM) + y)
        return [rad(0), rad(1), rad(2), mm, fin]

    def out_copy(bb):
        return pltpu.make_async_copy(xin.at[:, bb], out_hbm.at[:, bb], osem.at[bb])

    def layer(li, carry0):
        if full or CFG["only"] == "group":
            _loop("step", 0, 16, group, mem_ref[...].astype(f32))
        if full or CFG["only"] == "spec":
            @pl.when(li // 2 == 0)
            def _():
                with jax.named_scope("tail"):
                    wos, pre, dfts = finish_thunks(15, 1)
                    body = [bb for bb in range(16) if bb % 4 != 3]
                    for bb in body:
                        pre(chunk(bb))
                    for f in wos:
                        f()
                    for f in dfts:
                        f(body)
                    for bb in (3, 7, 11, 15):
                        pre(chunk(bb))
                    for f in dfts:
                        f((3, 7, 11, 15))
            with jax.named_scope("spectral"):
                spectral(li // 2)
        if not full:
            return carry0

        @pl.when(li == 0)
        def _():
            with jax.named_scope("dinv_tails"):
                th = [dinv_thunks(4 * u + 3, functools.partial(
                    lambda u, x: set_input(4 * u + 3, _round_bf16(x), u), u)) for u in range(4)]
                for stage in range(5):
                    for u in range(4):
                        th[u][stage]()

            def batch(it, carry):
                bb = body_chunk(it)
                side = dinv_thunks(bb, lambda x: set_input(bb, _round_bf16(x), None))
                _interleave(batch_thunks(it // 4, it % 4), side)
                return carry
            _loop("batch", 0, 12, batch, 0)

        @pl.when(li == 1)
        def _():
            with jax.named_scope("dinv_out"):
                def store_out(bb, x):
                    xin[:, bb] = x.reshape(16, 8, DM).astype(bf16)
                    out_copy(bb).start()
                th = [dinv_thunks(bb, functools.partial(store_out, bb)) for bb in range(16)]
                for i in range(17):
                    if i < 16:
                        for f in th[i][:4]:
                            f()
                    if i >= 1:
                        th[i - 1][4]()
                for bb in range(16):
                    out_copy(bb).wait()
        return carry0

    lax.fori_loop(0, 2, layer, 0)


@functools.partial(jax.jit, static_argnames=("A_seg_len",))
def pallas_interleave_layers__memory_aug_recurrent_mem_tr__spectral_gfnet__prompt_kernel(
    A_x, A_mem0, A_Wq, A_Wk, A_Wv, A_Wo, A_seg_len, B_x, B_w_r, B_w_i,
):
    assert A_seg_len == SEG and A_x.shape == (1, S, DM)
    small, emat = _tables()
    hbm = pl.BlockSpec(memory_space=pltpu.HBM)
    vmem = pl.BlockSpec(memory_space=pltpu.VMEM)
    out = pl.pallas_call(
        _kernel,
        out_shape=jax.ShapeDtypeStruct((16, 16, 8, DM), bf16),
        in_specs=[hbm, vmem] + [hbm] * 8,
        out_specs=hbm,
        scratch_shapes=[
            pltpu.VMEM((16, 16, 8, DM), bf16),
            pltpu.VMEM((16, 128, DM), f32),
            pltpu.VMEM((18, 128, DM), f32),
            pltpu.VMEM((16, 128, DM), f32),
            pltpu.VMEM((2, 128, DM), f32),
            pltpu.VMEM((12, DM, 8, DH), bf16),
            pltpu.VMEM((H * DH + 512, DM), bf16),
            pltpu.VMEM((2560, 128), u32),
            pltpu.VMEM((96, 320, 128), u32),
            pltpu.VMEM((5, 2048 + 256, 128), u32),
            pltpu.VMEM((16, 4, 96, 8, 128), f32),
            pltpu.VMEM((4, 5, 64, 128), u32),
            pltpu.VMEM((2, H, 32, 128), f32),
            pltpu.VMEM((2, 16, ZPITCH, 128), f32),
            pltpu.VMEM((2, 16, ZPITCH, 128), f32),
            pltpu.VMEM((2, 16, ZPITCH, 128), f32),
            pltpu.VMEM((6, 16 * WPITCH, 128), f32),
            pltpu.VMEM((9, DF, 512), bf16),
            pltpu.VMEM((4, 328, 128), f32),
            pltpu.VMEM((SMALL_ROWS, 128), u32),
            pltpu.VMEM((64, 64, 128), u32),
            pltpu.VMEM((80, 80), f32),
            pltpu.SemaphoreType.DMA((46,)),
            pltpu.SemaphoreType.DMA((16,)),
        ],
        compiler_params=pltpu.CompilerParams(vmem_limit_bytes=120 * 1024 * 1024),
    )(
        A_x.reshape(16, 16, 8, DM), A_mem0.reshape(MEM, DM),
        A_Wq, A_Wk, A_Wv, A_Wo.reshape(H * DH, DM), B_w_r.T, B_w_i.T,
        jnp.asarray(small), jnp.asarray(emat),
    )
    return out.reshape(1, S, DM)
```

```python
import functools
import math

import jax
import jax.numpy as jnp
import numpy as np
from jax import lax
import jax.experimental.pallas as pl
import jax.experimental.pallas.tpu as pltpu

f32, bf16, u32 = jnp.float32, jnp.bfloat16, jnp.uint32

S, DM, H, DH, MEM, SEG = 2048, 640, 32, 128, 8, 32
NSEG = S // SEG
NPAIR = H // 2
DF = DM // 2 + 1
EPS = 1e-5
WPITCH = 136

TPITCH = 9
ZPITCH = 136

C1, C2 = math.cos(2 * math.pi / 5), math.cos(4 * math.pi / 5)
S1, S2 = math.sin(2 * math.pi / 5), math.sin(4 * math.pi / 5)


def _to_bf16_bits(a):
    u = np.ascontiguousarray(a, dtype=np.float32).view(np.uint32).astype(np.uint64)
    return ((u + 0x7FFF + ((u >> 16) & 1)) >> 16).astype(np.uint32)


def _pack_rows(a):
    b = _to_bf16_bits(a)
    return b[..., 0::2, :] | (b[..., 1::2, :] << 16)


@functools.lru_cache(maxsize=None)
def _tables():
    b = np.arange(128)
    l0 = np.arange(0, DF, 5)
    l1 = np.concatenate([np.arange(1, 320, 5), np.arange(4, 320, 5)])
    l2 = np.concatenate([np.arange(2, 320, 5), np.arange(3, 320, 5)])
    sg = np.concatenate([np.ones(64), -np.ones(64)])

    def th(l):
        return 2 * np.pi * ((b[:, None] * l[None, :]) % DM) / DM

    fw = np.zeros((6, 256, 128))
    t = th(l0)
    fw[0, :128, :65] = np.cos(t)
    fw[3, :128, :65] = -np.sin(t)
    for g, l in ((1, l1), (2, l2)):
        t = th(l)
        c, s = np.cos(t), np.sin(t)
        fw[g] = np.concatenate([c, -sg * s], axis=0)
        fw[3 + g] = np.concatenate([-s, -sg * c], axis=0)
    sc = 1.0 / (S * DM)
    iw = np.zeros((5, 256, 128))
    t = th(l0).T
    cl = np.full((65, 1), 2.0)
    cl[0] = cl[-1] = 1.0
    iw[0, :65] = cl * np.cos(t) * sc
    iw[0, 128:128 + 65] = -cl * np.sin(t) * sc
    for g, l in ((1, l1), (2, l2)):
        t = th(l).T
        c, s = np.cos(t), np.sin(t)
        gg = sg[:, None]
        iw[2 * g - 1] = 2 * sc * np.concatenate([c, -s], axis=0)
        iw[2 * g] = 2 * sc * np.concatenate([gg * s, gg * c], axis=0)
    n = np.arange(64)
    order = np.concatenate([np.concatenate([np.arange(8) + 8 * j, np.arange(8) + 8 * j + 64])
                            for j in range(8)])
    e = np.zeros((2, 32, 128, 128))
    for k2 in range(32):
        t = 2 * np.pi * (((32 * n[:, None] + k2) * n[None, :]) % S) / S
        er, ei = np.cos(t), -np.sin(t)
        m = np.block([[er, -ei], [ei, er]])[order][:, order]
        e[0, k2], e[1, k2] = m, m.T
    small = np.concatenate(
        [_pack_rows(fw).reshape(-1, 128), _pack_rows(iw).reshape(-1, 128)], axis=0)
    return small, _pack_rows(e).reshape(64, 64, 128)


FW_OFF, IW_OFF = 0, 6 * 128
SMALL_ROWS = 11 * 128


def _loop(name, lo, hi, body, init, **kw):
    with jax.named_scope(name):
        return lax.fori_loop(lo, hi, body, init, **kw)


def _bf(x):
    return pltpu.bitcast(x, bf16)


def _dot(a, b):
    return jnp.dot(a, b, preferred_element_type=f32)


def _round_bf16(x):
    return x.astype(bf16).astype(f32)


def _layernorm(x):
    m = jnp.mean(x, axis=-1, keepdims=True)
    xc = x - m
    v = jnp.mean(xc * xc, axis=-1, keepdims=True)
    return xc * lax.rsqrt(v + EPS)


def _fft4(x, sign):
    (ar, ai), (br, bi), (cr, ci), (dr, di) = x
    t0r, t0i, t1r, t1i = ar + cr, ai + ci, ar - cr, ai - ci
    t2r, t2i, t3r, t3i = br + dr, bi + di, br - dr, bi - di
    y0, y2 = (t0r + t2r, t0i + t2i), (t0r - t2r, t0i - t2i)
    p, q = (t1r + t3i, t1i - t3r), (t1r - t3i, t1i + t3r)
    return [y0, p, y2, q] if sign < 0 else [y0, q, y2, p]


def _twiddle(z, n, period, sign):
    zr, zi = z
    n = n % period
    if n == 0:
        return z
    if 4 * n == period:
        return (-zi, zr) if sign > 0 else (zi, -zr)
    c, s = math.cos(2 * math.pi * n / period), sign * math.sin(2 * math.pi * n / period)
    if (8 * n) % period == 0:
        a, d = zr + zi, zr - zi
        if c * s > 0:
            return (d * c, a * c)
        return (a * c, d * s)
    return (zr * c - zi * s, zr * s + zi * c)


def _ilv(r, i):
    n = r.shape[0] // 8
    return jnp.concatenate([r.reshape(n, 8, 128), i.reshape(n, 8, 128)], axis=1).reshape(16 * n, 128)


def _dilv(x):
    n = x.shape[0] // 16
    x = x.reshape(n, 16, 128)
    return x[:, :8].reshape(8 * n, 128), x[:, 8:].reshape(8 * n, 128)


def _with_tokens(x, toks):
    if not toks:
        return x
    return jnp.concatenate(
        [x[8 * j:8 * j + 8] | toks[j] if j in toks else x[8 * j:8 * j + 8]
         for j in range(x.shape[0] // 8)], axis=0)


def _fft16(x, sign, emit=None):
    cols = [_fft4([x[4 * j + r] for j in range(4)], sign) for r in range(4)]
    out = [None] * 16
    for q in range(4):
        y = _fft4([_twiddle(cols[r][q], r * q, 16, sign) for r in range(4)], sign)
        for p in range(4):
            out[q + 4 * p] = y[p]
        if emit is not None:
            emit(q, y)
    return out


CFG = dict(lat_s=6, lat_pv=15, lat_wo=7, n_after=(11, 11, 11, 0), fill_at=16, v_delay=8, v_gap=0,
           prenorm=True,
           pre_at=((), (), (), tuple(range(11, 91, 5))), pre_rows=((), (), (), tuple(range(16))),
           first=(0, 1), pro_nre=14, pro_at=(2, 4, 6, 8, 9, 11, 13, 15, 16, 18, 20, 22, 23, 25, 27, 29), only=None)


def _interleave(main, side):
    n, k = len(main), 0
    for i, f in enumerate(main):
        f()
        while k < len(side) and (k + 1) * n <= (i + 1) * len(side):
            side[k]()
            k += 1
    for f in side[k:]:
        f()


def _kernel(x_hbm, mem_ref, wq_hbm, wk_hbm, wv_hbm, wo_hbm, wr_hbm, wi_hbm,
            small_hbm, e_hbm, out_hbm,
            xin, xa, xb, ao, raw, tmp, wa, wb, wo_t, qb, hl, ol, z0, z1, z2, wf,
            wri, wtmp, small, emat, fill_ref, sem, osem):
    zs = (z0, z1, z2)
    w_hbm = (wq_hbm, wk_hbm, wv_hbm)

    def body_chunk(i):
        return 4 * (i & 3) + (i >> 2)

    def cp_w(i):
        src = w_hbm[i // 4 if isinstance(i, int) else 0]
        c = i & 3
        return pltpu.make_async_copy(src.at[:, pl.ds(pl.multiple_of(8 * c, 8), 8), :],
                                     raw.at[i], sem.at[i])

    def cp_x(bb):
        return pltpu.make_async_copy(x_hbm.at[:, bb], xin.at[:, bb], sem.at[12 + bb])

    def cp_f(i):
        src = (wr_hbm, wi_hbm)[i // 4 if isinstance(i, int) else 0]
        cols = pl.ds(pl.multiple_of(512 * (i & 3), 512), 512)
        return pltpu.make_async_copy(src.at[:, cols], wri.at[i], sem.at[36 + i])

    cp_rest = [pltpu.make_async_copy(wo_hbm.at[:, pl.ds(128 * j, 128)], wo_t.at[j], sem.at[28 + j])
               for j in range(5)]
    cp_rest += [pltpu.make_async_copy(small_hbm, small, sem.at[44]),
               pltpu.make_async_copy(e_hbm, emat, sem.at[45])]

    full = CFG["only"] in (None, "pro")
    for u in range(4 if full else 0):
        cp_x(4 * u + 3).start()
    if full:
        cp_w(0).start()
    for i in range(12 if full else 0):
        if i < 11:
            cp_w(i + 1).start()
        cp_x(body_chunk(i)).start()
        if i >= 4:
            cp_f(i - 4).start()
    for cp in cp_rest if full else ():
        cp.start()

    r = lax.broadcasted_iota(jnp.int32, (80, 80), 0)
    c = lax.broadcasted_iota(jnp.int32, (80, 80), 1)

    def head(i):
        return jnp.where(i < 64, i // 32, (i - 64) // 8)

    def pos(i):
        return jnp.where(i < 64, i % 32, 32 + (i - 64) % 8)

    ok = (pos(r) < MEM) | (pos(r) >= pos(c))
    fill_ref[...] = jnp.where(head(r) == head(c), jnp.where(ok, 0.0, -1e9), -jnp.inf).astype(f32)
    ol[...] = jnp.zeros_like(ol)
    ao[...] = jnp.zeros_like(ao)
    wtmp[:, 320:328, :] = jnp.zeros((4, 8, 128), f32)
    xb[17, 0:8, 0:128] = jnp.zeros((8, 128), f32)
    xa[32, 0:8, 0:128] = jnp.zeros((8, 128), f32)
    wa[48, 0:8, :] = jnp.zeros((8, 128), u32)
    wb[48, 0:8, :] = jnp.zeros((8, 128), u32)
    wf[5, 128:WPITCH, :] = jnp.zeros((8, 128), f32)
    for z in zs:
        z[0, 0, 128:ZPITCH, :] = jnp.zeros((8, 128), f32)

    def chunk(bb):
        if isinstance(bb, int):
            return slice(8 * bb, 8 * bb + 8)
        return pl.ds(pl.multiple_of(8 * bb, 8), 8)

    def set_input(bb, x, tail_u, a0=0):
        n = x.shape[0] // 8
        xa[a0:a0 + n, chunk(bb), :] = x.reshape(n, 8, DM)
        y = _layernorm(x)
        if tail_u is None:
            xa[16 + a0:16 + a0 + n, chunk(bb), :] = y.reshape(n, 8, DM)
        else:
            yb = y.astype(bf16)
            for kt in range(5):
                hl[tail_u, kt] = pltpu.bitcast(yb[:, 128 * kt:128 * kt + 128], u32)

    def load_x(bb, a0=0, n=16):
        return xin[a0:a0 + n, bb].astype(f32).reshape(8 * n, DM)

    def wtile(m, c, j, e):
        return (wa, wb)[j >> 1], 12 * c + 6 * (j & 1) + 2 * m + e

    def stage(i, chunk_id):
        v = pltpu.bitcast(raw[chunk_id, 16 * i:16 * i + 16].reshape(128, 128), u32)
        for k in range(8):
            base = 8 * TPITCH * i + TPITCH * k
            tmp[base:base + 8, :] = v[8 * k:8 * k + 8]

    def relayout(i, m, c, half):
        for j in (2 * half, 2 * half + 1):
            a = tmp[pl.ds(8 * TPITCH * i + j, 8, stride=TPITCH), :]
            b = tmp[pl.ds(8 * TPITCH * i + 4 + j, 8, stride=TPITCH), :]
            w, t = wtile(m, c, j, 0)
            w[t, 8 * i:8 * i + 8, :] = (a & 0xFFFF) | (b << 16)
            w[t + 1, 8 * i:8 * i + 8, :] = (a >> 16) | (b & jnp.uint32(0xFFFF0000))

    def batch_thunks(m, c):
        def one(j, u, e):
            def run(toks=None):
                lhs = jnp.concatenate(
                    [_bf(_with_tokens(hl[u, kt], toks if kt == 0 else None)) for kt in range(5)], axis=1)
                w, t = wtile(m, c, j, e)
                qb[:, u, 6 * (4 * c + j) + 2 * m + e] = _dot(lhs, _bf(w[t])).reshape(16, 8, 128)
            return run
        return [one(j, u, e) for j in range(4) for u in range(4) for e in range(2)]

    def wperm_thunks(piece, j):
        m = (piece >> 2) & 1
        wt = wtmp.at[j]

        def load():
            wt[0:DF, :] = wri[piece, :, 128 * j:128 * j + 128].astype(f32)

        def one(g):
            def run():
                if g == 0:
                    t = jnp.concatenate([wt[pl.ds(0, 64, stride=5), :], wt[320:328, :],
                                         jnp.zeros((56, 128), f32)], axis=0)
                else:
                    t = jnp.concatenate([wt[pl.ds(g, 64, stride=5), :],
                                         wt[pl.ds(5 - g, 64, stride=5), :]], axis=0)
                y = t.T
                sub = wf.at[3 * m + g, pl.ds(pl.multiple_of((piece & 3) * 32, 32), 15 * WPITCH + 32)]
                for k in range(8):
                    for hf in range(2):
                        sub[pl.ds(8 * j + k + 8 * hf * WPITCH, 8, stride=WPITCH), :] = (
                            y[16 * k + 8 * hf:16 * k + 8 * hf + 8])
            return run
        return [load] + [one(g) for g in range(3)]

    def pro0():
        for u in range(4):
            cp_x(4 * u + 3).wait()
        for u in range(4):
            set_input(4 * u + 3, load_x(4 * u + 3), u)
        cp_w(0).wait()
        for i in range(40):
            stage(i, 0)
            relayout(i, 0, 0, 0)

    def pro1(it, carry):
        bb = body_chunk(it)
        with jax.named_scope("pro1_wait"):
            @pl.when(it < 11)
            def _():
                cp_w(it + 1).wait()

            @pl.when(it >= 4)
            def _():
                cp_f(it - 4).wait()
            cp_x(bb).wait()
        nxt = jnp.minimum(it + 1, 11)
        piece = jnp.where(it >= 4, it - 4, 8)
        zero = it >> 4
        timed = []
        for j in range(4):
            load, *perms = wperm_thunks(piece, j)

            def ln_part(j=j, load=load):
                load()
                set_input(bb, load_x(bb, 4 * j, 4), None, 4 * j)
                return pltpu.bitcast(xa[32 + zero, 0:8, 0:128], u32)
            timed.append(ln_part)
            for f in perms:
                def perm_part(f=f):
                    f()
                    return pltpu.bitcast(wf[5 + zero, 128:WPITCH, :], u32)
                timed.append(perm_part)
        nre = CFG["pro_nre"]
        toks = None
        for i, f in enumerate(batch_thunks(it >> 2, it & 3)):
            f(toks)
            toks = {}
            if i in CFG["pro_at"]:
                toks[0] = timed.pop(0)()
            half, k = i >> 4, i & 15
            for r in range(40):
                if r * nre // 40 == k:
                    if half == 0:
                        relayout(r, it >> 2, it & 3, 1)
                    else:
                        stage(r, nxt)
                        relayout(r, nxt >> 2, nxt & 3, 0)
            if k < nre:
                toks[4] = (wb, wa)[half][48 + zero, 0:8, :]
        return carry

    if full or CFG["only"] == "pro":
        with jax.named_scope("pro0"):
            pro0()
        _loop("pro1", 0, 12, pro1, 0)
        for cp in cp_rest:
            cp.wait()

    scale = DH ** -0.5

    def wo_dot(hh, oo):
        return [_dot(oo, wo_t[j, 128 * hh:128 * hh + 128, :]) for j in range(5)]

    def addl(acc, res):
        return res if acc is None else [a + b for a, b in zip(acc, res)]

    def finish_thunks(gp, slot):
        st = {"acc": None}

        def f_wo(hh):
            def run():
                st["acc"] = addl(st["acc"], wo_dot(hh, ol[slot, hh].astype(bf16)))
                if hh == H - 1:
                    out = jnp.concatenate(st["acc"], axis=1)
                    for u in range(4):
                        ao[slot, 32 * u + 24:32 * u + 32, :] = out[8 * u:8 * u + 8]
            return run

        def pre(rows):
            x = _round_bf16(xa[gp, rows, :] + ao[slot, rows, :])
            xb[gp, rows, :] = x
            y = _layernorm(x)
            x0, x1, x2, x3, x4 = [y[:, 128 * a:128 * a + 128] for a in range(5)]
            t1, t2, t3, t4 = x1 + x4, x2 + x3, x1 - x4, x2 - x3
            xb[16, rows, :] = jnp.concatenate(
                [x0 + t1 + t2, x0 + C1 * t1 + C2 * t2, S1 * t3 + S2 * t4,
                 x0 + C2 * t1 + C1 * t2, S2 * t3 - S1 * t4], axis=1)

        def f_dft(cidx):
            def run(chunks=tuple(range(16))):
                g = cidx % 3
                o = FW_OFF + 128 * cidx
                lo, hi = (0, 128) if g == 0 else (256 * g - 128, 256 * g + 128)
                u = jnp.concatenate([xb[16, chunk(bb), lo:hi] for bb in chunks], axis=0)
                y = _dot(u.astype(bf16), _bf(small[o:o + (hi - lo) // 2, :]))
                for i, bb in enumerate(chunks):
                    zs[g][cidx // 3, gp, chunk(bb), :] = y[8 * i:8 * i + 8]
            return run
        return [f_wo(hh) for hh in range(H)], pre, [f_dft(cidx) for cidx in (0, 3, 1, 4, 2, 5)]

    def group(g, mem):
        cur = g & 1
        wos, pre, dfts = finish_thunks(jnp.maximum(g - 1, 0), 1 - cur)
        fillers = [wos[0:11], wos[11:22], wos[22:32], dfts]
        for ph in range(4):
            h = jnp.concatenate([mem, xa[16 + g, 32 * ph:32 * ph + 24, :]], axis=0).astype(bf16)
            pres = list(CFG["pre_rows"][ph])
            pre_at = CFG["pre_at"][ph]
            tok = None
            pr, sm, oos = {}, {}, {}

            def stacked(p, m):
                tails = [qb[g, ph, 6 * p + 2 * m + e] for e in range(2)]
                return jnp.concatenate([pr[p, m, 0], pr[p, m, 1]] + tails, axis=0).astype(bf16)

            def scores(p):
                sc = lax.dot_general(stacked(p, 0), stacked(p, 1), (((1,), (1,)), ((), ())),
                                     preferred_element_type=f32)
                fill = fill_ref[...]
                sc = jnp.where(fill == 0.0, sc * scale, fill)
                mx = jnp.max(sc, axis=-1, keepdims=True)
                e = jnp.exp(sc - mx)
                rl = pl.reciprocal(jnp.sum(e, axis=-1, keepdims=True), approx=True)
                sm[p] = ((e * rl).astype(bf16), None) if CFG["prenorm"] else (e.astype(bf16), rl)

            def pv(p):
                e, rl = sm[p]
                o = _dot(e, stacked(p, 2))
                if rl is not None:
                    o = o * rl
                ol[cur, 2 * p, 8 * ph:8 * ph + 8, :] = o[64:72]
                ol[cur, 2 * p + 1, 8 * ph:8 * ph + 8, :] = o[72:80]
                oos[2 * p], oos[2 * p + 1] = o[0:32].astype(bf16), o[32:64].astype(bf16)

            acc, t, nwo = None, 0.0, 0
            keyed = []
            for p in range(NPAIR):
                keyed += [(4 * p + 2 * i + e, (p, m, e)) for i, m in enumerate(CFG["first"]) for e in range(2)]
                keyed += [(4 * p + 3.5 + CFG["v_delay"] + CFG["v_gap"] * e, (p, 2, e)) for e in range(2)]
            bulk = [x for _, x in sorted(keyed, key=lambda kv: kv[0])]
            pend, ready, fl = [], [], list(fillers[ph])
            n_after = CFG["n_after"][ph]
            while nwo < H:
                pend.sort()
                if pend and pend[0][0] <= t:
                    _, kind, p = pend.pop(0)
                    if kind == "S":
                        scores(p)
                        pend.append((t + CFG["lat_pv"], "V", p))
                    else:
                        pv(p)
                        ready += [(t + CFG["lat_wo"], 2 * p + e) for e in range(2)]
                    t += 0.5
                elif bulk:
                    p, m, e = bulk.pop(0)
                    w, wt = wtile(m, p >> 2, p & 3, e)
                    pr[p, m, e] = _dot(h, _bf(_with_tokens(w[wt], tok)))
                    tok = None
                    if 96 - len(bulk) in pre_at:
                        pre(chunk(pres.pop(0)))
                        tok = {0: pltpu.bitcast(xb[17 + (g >> 4), 0:8, 0:128], u32)}
                    t += 1
                    if m == CFG["first"][1] and e == 1:
                        pend.append((t + CFG["lat_s"], "S", p))
                elif nwo >= CFG["fill_at"] and len(fl) > n_after:
                    fl.pop(0)()
                    t += 1
                elif ready and ready[0][0] <= t:
                    _, hh = ready.pop(0)
                    acc = addl(acc, wo_dot(hh, oos[hh]))
                    t += 1
                    nwo += 1
                elif len(fl) > n_after:
                    fl.pop(0)()
                    t += 1
                else:
                    t += 0.5
            out = jnp.concatenate(acc, axis=1)
            ao[cur, 32 * ph:32 * ph + 24, :] = out[8:32]
            mem = _round_bf16(out[0:8])
            for f in fl:
                f()
        return mem

    def spectral(zero):
        def fence(z):
            return z[0, zero, 128:ZPITCH, :]

        def radix_fwd(g, bb, tok=None):
            z = zs[g]
            xs = [(z[0, a, chunk(bb), :], z[1, a, chunk(bb), :]) for a in range(16)]
            if tok is not None:
                xs[:4] = [(xr + tok, xi) for xr, xi in xs[:4]]
            toks = []

            def emit(q, y):
                for p in range(4):
                    z[0, q + 4 * p, chunk(bb), :] = y[p][0]
                    z[1, q + 4 * p, chunk(bb), :] = y[p][1]
                if g > 0 or q == 3:
                    toks.append(fence(z))
            _fft16(xs, -1, emit)
            return toks

        ys = {}

        def fwd(g, k2, toks):
            z = zs[g]
            ur, ui = z[0, k2, 0:64, :], z[1, k2, 0:64, :]
            tr, ti = _twiddle((z[0, k2, 64:128, :], z[1, k2, 64:128, :]), k2, 32, -1)
            for hf in range(2):
                v = _ilv(ur + tr, ui + ti) if hf == 0 else _ilv(ur - tr, ui - ti)
                lhs = _with_tokens(emat[k2 + 16 * hf], toks if hf == 0 else None)
                xr, xi = _dilv(_dot(_bf(lhs), v.astype(bf16)))
                wr = wf[g, pl.ds(k2 * WPITCH + hf, 64, stride=2), :]
                wi = wf[g + 3, pl.ds(k2 * WPITCH + hf, 64, stride=2), :]
                ys[g, k2, hf] = _ilv(xr * wr - xi * wi, xr * wi + xi * wr).astype(bf16)

        def inv(g, k2):
            z = zs[g]
            t0 = _dot(_bf(emat[32 + k2]), ys.pop((g, k2, 0)))
            t1 = _dot(_bf(emat[48 + k2]), ys.pop((g, k2, 1)))
            z[0, k2, 0:64, :], z[1, k2, 0:64, :] = _dilv(t0 + t1)
            z[0, k2, 64:128, :], z[1, k2, 64:128, :] = _twiddle(_dilv(t0 - t1), k2, 32, 1)

        chain = {}
        for bb in range(16):
            chain[bb] = radix_fwd(0, bb, chain.get(bb - 2))[-1]
        radix_fwd(1, 0)
        units = [(g, k2) for g in range(3) for k2 in range(16)]
        toks = None
        for i in range(len(units) + 3):
            if i < len(units):
                fwd(*units[i], toks)
            if i >= 3:
                inv(*units[i - 3])
            toks = None
            if i < 31:
                t4 = radix_fwd(1 + (i + 1) // 16, (i + 1) % 16)
                toks = {3 + j: pltpu.bitcast(t, u32) for j, t in enumerate(t4)}

    def dinv_thunks(bb, finish):
        st = {}

        def rad(g):
            def run():
                z = zs[g]
                ys = _fft16([(z[0, a, chunk(bb), :], z[1, a, chunk(bb), :]) for a in range(16)], 1)
                st[g] = jnp.concatenate(
                    [jnp.concatenate([y[0] for y in ys], axis=0),
                     jnp.concatenate([y[1] for y in ys], axis=0)], axis=1).astype(bf16)
            return run

        def mm():
            st["p"] = [_dot(st[(j + 1) // 2], _bf(small[IW_OFF + 128 * j:IW_OFF + 128 * (j + 1), :]))
                       for j in range(5)]

        def fin():
            p0, p1, q1, p2, q2 = st["p"]
            e1, o1 = p0 + C1 * p1 + C2 * p2, S1 * q1 + S2 * q2
            e2, o2 = p0 + C2 * p1 + C1 * p2, S2 * q1 - S1 * q2
            y = jnp.concatenate([p0 + p1 + p2, e1 - o1, e2 - o2, e2 + o2, e1 + o1], axis=1)
            finish(xb[0:16, chunk(bb), :].reshape(128, DM) + y)
        return [rad(0), rad(1), rad(2), mm, fin]

    def out_copy(bb):
        return pltpu.make_async_copy(xin.at[:, bb], out_hbm.at[:, bb], osem.at[bb])

    def layer(li, carry0):
        if full or CFG["only"] == "group":
            _loop("step", 0, 16, group, mem_ref[...].astype(f32))
        if full or CFG["only"] == "spec":
            @pl.when((li >> 1) == 0)
            def _():
                with jax.named_scope("tail"):
                    wos, pre, dfts = finish_thunks(15, 1)
                    body = [bb for bb in range(16) if bb % 4 != 3]
                    for bb in body:
                        pre(chunk(bb))
                    for f in wos:
                        f()
                    for f in dfts:
                        f(body)
                    for bb in (3, 7, 11, 15):
                        pre(chunk(bb))
                    for f in dfts:
                        f((3, 7, 11, 15))
            with jax.named_scope("spectral"):
                spectral((li >> 1))
        if not full:
            return carry0

        @pl.when(li == 0)
        def _():
            with jax.named_scope("dinv_tails"):
                th = [dinv_thunks(4 * u + 3, functools.partial(
                    lambda u, x: set_input(4 * u + 3, _round_bf16(x), u), u)) for u in range(4)]
                for stage in range(5):
                    for u in range(4):
                        th[u][stage]()

            def batch(it, carry):
                bb = body_chunk(it)
                side = dinv_thunks(bb, lambda x: set_input(bb, _round_bf16(x), None))
                _interleave(batch_thunks(it >> 2, it & 3), side)
                return carry
            _loop("batch", 0, 12, batch, 0)

        @pl.when(li == 1)
        def _():
            with jax.named_scope("dinv_out"):
                def store_out(bb, x):
                    xin[:, bb] = x.reshape(16, 8, DM).astype(bf16)
                    out_copy(bb).start()
                th = [dinv_thunks(bb, functools.partial(store_out, bb)) for bb in range(16)]
                for i in range(17):
                    if i < 16:
                        for f in th[i][:4]:
                            f()
                    if i >= 1:
                        th[i - 1][4]()
                for bb in range(16):
                    out_copy(bb).wait()
        return carry0

    if CFG["only"] != "pro":
        lax.fori_loop(0, 2, layer, 0)


@functools.partial(jax.jit, static_argnames=("A_seg_len",))
def pallas_interleave_layers__memory_aug_recurrent_mem_tr__spectral_gfnet__prompt_kernel(
    A_x, A_mem0, A_Wq, A_Wk, A_Wv, A_Wo, A_seg_len, B_x, B_w_r, B_w_i,
):
    assert A_seg_len == SEG and A_x.shape == (1, S, DM)
    small, emat = _tables()
    hbm = pl.BlockSpec(memory_space=pltpu.HBM)
    vmem = pl.BlockSpec(memory_space=pltpu.VMEM)
    out = pl.pallas_call(
        _kernel,
        out_shape=jax.ShapeDtypeStruct((16, 16, 8, DM), bf16),
        in_specs=[hbm, vmem] + [hbm] * 8,
        out_specs=hbm,
        scratch_shapes=[
            pltpu.VMEM((16, 16, 8, DM), bf16),
            pltpu.VMEM((33, 128, DM), f32),
            pltpu.VMEM((18, 128, DM), f32),
            pltpu.VMEM((2, 128, DM), f32),
            pltpu.VMEM((12, DM, 8, DH), bf16),
            pltpu.VMEM((320 * TPITCH, 128), u32),
            pltpu.VMEM((49, 320, 128), u32),
            pltpu.VMEM((49, 320, 128), u32),
            pltpu.VMEM((5, H * DH, 128), bf16),
            pltpu.VMEM((16, 4, 96, 8, 128), f32),
            pltpu.VMEM((4, 5, 64, 128), u32),
            pltpu.VMEM((2, H, 32, 128), f32),
            pltpu.VMEM((2, 16, ZPITCH, 128), f32),
            pltpu.VMEM((2, 16, ZPITCH, 128), f32),
            pltpu.VMEM((2, 16, ZPITCH, 128), f32),
            pltpu.VMEM((6, 16 * WPITCH, 128), f32),
            pltpu.VMEM((9, DF, 512), bf16),
            pltpu.VMEM((4, 328, 128), f32),
            pltpu.VMEM((SMALL_ROWS, 128), u32),
            pltpu.VMEM((64, 64, 128), u32),
            pltpu.VMEM((80, 80), f32),
            pltpu.SemaphoreType.DMA((46,)),
            pltpu.SemaphoreType.DMA((16,)),
        ],
        compiler_params=pltpu.CompilerParams(vmem_limit_bytes=120 * 1024 * 1024),
    )(
        A_x.reshape(16, 16, 8, DM), A_mem0.reshape(MEM, DM),
        A_Wq, A_Wk, A_Wv, A_Wo.reshape(H * DH, DM), B_w_r.T, B_w_i.T,
        jnp.asarray(small), jnp.asarray(emat),
    )
    return out.reshape(1, S, DM)
```

```python
import functools
import math

import jax
import jax.numpy as jnp
import numpy as np
from jax import lax
import jax.experimental.pallas as pl
import jax.experimental.pallas.tpu as pltpu

f32, bf16, u32 = jnp.float32, jnp.bfloat16, jnp.uint32

S, DM, H, DH, MEM, SEG = 2048, 640, 32, 128, 8, 32
NSEG = S // SEG
NPAIR = H // 2
DF = DM // 2 + 1
EPS = 1e-5
WPITCH = 136

TPITCH = 9
ZPITCH = 136

C1, C2 = math.cos(2 * math.pi / 5), math.cos(4 * math.pi / 5)
S1, S2 = math.sin(2 * math.pi / 5), math.sin(4 * math.pi / 5)


def _to_bf16_bits(a):
    u = np.ascontiguousarray(a, dtype=np.float32).view(np.uint32).astype(np.uint64)
    return ((u + 0x7FFF + ((u >> 16) & 1)) >> 16).astype(np.uint32)


def _pack_rows(a):
    b = _to_bf16_bits(a)
    return b[..., 0::2, :] | (b[..., 1::2, :] << 16)


@functools.lru_cache(maxsize=None)
def _tables():
    b = np.arange(128)
    l0 = np.arange(0, DF, 5)
    l1 = np.concatenate([np.arange(1, 320, 5), np.arange(4, 320, 5)])
    l2 = np.concatenate([np.arange(2, 320, 5), np.arange(3, 320, 5)])
    sg = np.concatenate([np.ones(64), -np.ones(64)])

    def th(l):
        return 2 * np.pi * ((b[:, None] * l[None, :]) % DM) / DM

    fw = np.zeros((6, 256, 128))
    t = th(l0)
    fw[0, :128, :65] = np.cos(t)
    fw[3, :128, :65] = -np.sin(t)
    for g, l in ((1, l1), (2, l2)):
        t = th(l)
        c, s = np.cos(t), np.sin(t)
        fw[g] = np.concatenate([c, -sg * s], axis=0)
        fw[3 + g] = np.concatenate([-s, -sg * c], axis=0)
    sc = 1.0 / (S * DM)
    iw = np.zeros((5, 256, 128))
    t = th(l0).T
    cl = np.full((65, 1), 2.0)
    cl[0] = cl[-1] = 1.0
    iw[0, :65] = cl * np.cos(t) * sc
    iw[0, 128:128 + 65] = -cl * np.sin(t) * sc
    for g, l in ((1, l1), (2, l2)):
        t = th(l).T
        c, s = np.cos(t), np.sin(t)
        gg = sg[:, None]
        iw[2 * g - 1] = 2 * sc * np.concatenate([c, -s], axis=0)
        iw[2 * g] = 2 * sc * np.concatenate([gg * s, gg * c], axis=0)
    n = np.arange(64)
    order = np.concatenate([np.concatenate([np.arange(8) + 8 * j, np.arange(8) + 8 * j + 64])
                            for j in range(8)])
    e = np.zeros((2, 32, 128, 128))
    for k2 in range(32):
        t = 2 * np.pi * (((32 * n[:, None] + k2) * n[None, :]) % S) / S
        er, ei = np.cos(t), -np.sin(t)
        m = np.block([[er, -ei], [ei, er]])[order][:, order]
        e[0, k2], e[1, k2] = m, m.T
    small = np.concatenate(
        [_pack_rows(fw).reshape(-1, 128), _pack_rows(iw).reshape(-1, 128)], axis=0)
    return small, _pack_rows(e).reshape(64, 64, 128)


FW_OFF, IW_OFF = 0, 6 * 128
SMALL_ROWS = 11 * 128


def _loop(name, lo, hi, body, init, **kw):
    with jax.named_scope(name):
        return lax.fori_loop(lo, hi, body, init, **kw)


def _bf(x):
    return pltpu.bitcast(x, bf16)


def _dot(a, b):
    return jnp.dot(a, b, preferred_element_type=f32)


def _round_bf16(x):
    return x.astype(bf16).astype(f32)


def _layernorm(x):
    m = jnp.mean(x, axis=-1, keepdims=True)
    xc = x - m
    v = jnp.mean(xc * xc, axis=-1, keepdims=True)
    return xc * lax.rsqrt(v + EPS)


def _fft4(x, sign):
    (ar, ai), (br, bi), (cr, ci), (dr, di) = x
    t0r, t0i, t1r, t1i = ar + cr, ai + ci, ar - cr, ai - ci
    t2r, t2i, t3r, t3i = br + dr, bi + di, br - dr, bi - di
    y0, y2 = (t0r + t2r, t0i + t2i), (t0r - t2r, t0i - t2i)
    p, q = (t1r + t3i, t1i - t3r), (t1r - t3i, t1i + t3r)
    return [y0, p, y2, q] if sign < 0 else [y0, q, y2, p]


def _twiddle(z, n, period, sign):
    zr, zi = z
    n = n % period
    if n == 0:
        return z
    if 4 * n == period:
        return (-zi, zr) if sign > 0 else (zi, -zr)
    c, s = math.cos(2 * math.pi * n / period), sign * math.sin(2 * math.pi * n / period)
    if (8 * n) % period == 0:
        a, d = zr + zi, zr - zi
        if c * s > 0:
            return (d * c, a * c)
        return (a * c, d * s)
    return (zr * c - zi * s, zr * s + zi * c)


def _ilv(r, i):
    n = r.shape[0] // 8
    return jnp.concatenate([r.reshape(n, 8, 128), i.reshape(n, 8, 128)], axis=1).reshape(16 * n, 128)


def _dilv(x):
    n = x.shape[0] // 16
    x = x.reshape(n, 16, 128)
    return x[:, :8].reshape(8 * n, 128), x[:, 8:].reshape(8 * n, 128)


def _with_tokens(x, toks):
    if not toks:
        return x
    return jnp.concatenate(
        [x[8 * j:8 * j + 8] | toks[j] if j in toks else x[8 * j:8 * j + 8]
         for j in range(x.shape[0] // 8)], axis=0)


def _fft16(x, sign, emit=None):
    cols = [_fft4([x[4 * j + r] for j in range(4)], sign) for r in range(4)]
    out = [None] * 16
    for q in range(4):
        y = _fft4([_twiddle(cols[r][q], r * q, 16, sign) for r in range(4)], sign)
        for p in range(4):
            out[q + 4 * p] = y[p]
        if emit is not None:
            emit(q, y)
    return out


CFG = dict(lat_s=6, lat_pv=15, lat_wo=7, n_after=(11, 11, 11, 0), fill_at=16, v_delay=8, v_gap=0,
           prenorm=True,
           pre_at=((), (), (), tuple(range(11, 91, 5))), pre_rows=((), (), (), tuple(range(16))),
           first=(0, 1), pro_nre=14, re_pos=(2, 5, 7), ln_at=(12, 13, 14, 15), perm_at=(3, 4, 5, 6, 7, 8, 9, 10, 11, 12, 13, 14), only=None)


def _interleave(main, side):
    n, k = len(main), 0
    for i, f in enumerate(main):
        f()
        while k < len(side) and (k + 1) * n <= (i + 1) * len(side):
            side[k]()
            k += 1
    for f in side[k:]:
        f()


def _kernel(x_hbm, mem_ref, wq_hbm, wk_hbm, wv_hbm, wo_hbm, wr_hbm, wi_hbm,
            small_hbm, e_hbm, out_hbm,
            xin, xa, xb, ao, raw, tmp, wa, wb, wo_t, qb, hl, ol, z0, z1, z2, wf,
            wri, wtmp, small, emat, fill_ref, sem, osem):
    zs = (z0, z1, z2)
    w_hbm = (wq_hbm, wk_hbm, wv_hbm)

    def body_chunk(i):
        return 4 * (i & 3) + (i >> 2)

    def cp_w(i):
        src = w_hbm[i // 4 if isinstance(i, int) else 0]
        c = i & 3
        return pltpu.make_async_copy(src.at[:, pl.ds(pl.multiple_of(8 * c, 8), 8), :],
                                     raw.at[i], sem.at[i])

    def cp_x(bb):
        return pltpu.make_async_copy(x_hbm.at[:, bb], xin.at[:, bb], sem.at[12 + bb])

    def cp_f(i):
        src = (wr_hbm, wi_hbm)[i // 4 if isinstance(i, int) else 0]
        cols = pl.ds(pl.multiple_of(512 * (i & 3), 512), 512)
        return pltpu.make_async_copy(src.at[:, cols], wri.at[i], sem.at[36 + i])

    cp_rest = [pltpu.make_async_copy(wo_hbm.at[:, pl.ds(128 * j, 128)], wo_t.at[j], sem.at[28 + j])
               for j in range(5)]
    cp_rest += [pltpu.make_async_copy(small_hbm, small, sem.at[44]),
               pltpu.make_async_copy(e_hbm, emat, sem.at[45])]

    full = CFG["only"] in (None, "pro")
    for u in range(4 if full else 0):
        cp_x(4 * u + 3).start()
    if full:
        cp_w(0).start()
    for i in range(12 if full else 0):
        if i < 11:
            cp_w(i + 1).start()
        cp_x(body_chunk(i)).start()
        if 3 <= i < 11:
            cp_f(i - 3).start()
    for cp in cp_rest if full else ():
        cp.start()

    r = lax.broadcasted_iota(jnp.int32, (80, 80), 0)
    c = lax.broadcasted_iota(jnp.int32, (80, 80), 1)

    def head(i):
        return jnp.where(i < 64, i // 32, (i - 64) // 8)

    def pos(i):
        return jnp.where(i < 64, i % 32, 32 + (i - 64) % 8)

    ok = (pos(r) < MEM) | (pos(r) >= pos(c))
    fill_ref[...] = jnp.where(head(r) == head(c), jnp.where(ok, 0.0, -1e9), -jnp.inf).astype(f32)
    ol[...] = jnp.zeros_like(ol)
    ao[...] = jnp.zeros_like(ao)
    wtmp[:, 320:328, :] = jnp.zeros((4, 8, 128), f32)
    xb[17, 0:8, 0:128] = jnp.zeros((8, 128), f32)
    xa[32, 0:8, 0:128] = jnp.zeros((8, 128), f32)
    wa[48, 0:8, :] = jnp.zeros((8, 128), u32)
    wb[48, 0:8, :] = jnp.zeros((8, 128), u32)
    wf[5, 128:WPITCH, :] = jnp.zeros((8, 128), f32)
    for z in zs:
        z[0, 0, 128:ZPITCH, :] = jnp.zeros((8, 128), f32)

    def chunk(bb):
        if isinstance(bb, int):
            return slice(8 * bb, 8 * bb + 8)
        return pl.ds(pl.multiple_of(8 * bb, 8), 8)

    def set_input(bb, x, tail_u, a0=0):
        n = x.shape[0] // 8
        xa[a0:a0 + n, chunk(bb), :] = x.reshape(n, 8, DM)
        y = _layernorm(x)
        if tail_u is None:
            xa[16 + a0:16 + a0 + n, chunk(bb), :] = y.reshape(n, 8, DM)
        else:
            yb = y.astype(bf16)
            for kt in range(5):
                hl[tail_u, kt] = pltpu.bitcast(yb[:, 128 * kt:128 * kt + 128], u32)

    def load_x(bb, a0=0, n=16):
        return xin[a0:a0 + n, bb].astype(f32).reshape(8 * n, DM)

    def wtile(m, c, j, e):
        return (wa, wb)[j >> 1], 12 * c + 6 * (j & 1) + 2 * m + e

    def stage(i, chunk_id):
        v = pltpu.bitcast(raw[chunk_id, 16 * i:16 * i + 16].reshape(128, 128), u32)
        for k in range(8):
            base = 8 * TPITCH * i + TPITCH * k
            tmp[base:base + 8, :] = v[8 * k:8 * k + 8]

    def relayout(i, m, c, half):
        for j in (2 * half, 2 * half + 1):
            a = tmp[pl.ds(8 * TPITCH * i + j, 8, stride=TPITCH), :]
            b = tmp[pl.ds(8 * TPITCH * i + 4 + j, 8, stride=TPITCH), :]
            w, t = wtile(m, c, j, 0)
            w[t, 8 * i:8 * i + 8, :] = (a & 0xFFFF) | (b << 16)
            w[t + 1, 8 * i:8 * i + 8, :] = (a >> 16) | (b & jnp.uint32(0xFFFF0000))

    def batch_thunks(m, c):
        def one(j, u, e):
            def run(toks=None):
                lhs = jnp.concatenate(
                    [_bf(_with_tokens(hl[u, kt], toks if kt == 0 else None)) for kt in range(5)], axis=1)
                w, t = wtile(m, c, j, e)
                qb[:, u, 8 * (4 * m + c) + 2 * j + e] = _dot(lhs, _bf(w[t])).reshape(16, 8, 128)
            return run
        return [one(j, u, e) for j in range(4) for u in range(4) for e in range(2)]

    def wperm_thunks(piece, j):
        m = (piece >> 2) & 1
        wt = wtmp.at[j]

        def load():
            wt[0:DF, :] = wri[piece, :, 128 * j:128 * j + 128].astype(f32)

        def one(g):
            def run():
                if g == 0:
                    t = jnp.concatenate([wt[pl.ds(0, 64, stride=5), :], wt[320:328, :],
                                         jnp.zeros((56, 128), f32)], axis=0)
                else:
                    t = jnp.concatenate([wt[pl.ds(g, 64, stride=5), :],
                                         wt[pl.ds(5 - g, 64, stride=5), :]], axis=0)
                y = t.T
                sub = wf.at[3 * m + g, pl.ds(pl.multiple_of((piece & 3) * 32, 32), 15 * WPITCH + 32)]
                for k in range(8):
                    for hf in range(2):
                        sub[pl.ds(8 * j + k + 8 * hf * WPITCH, 8, stride=WPITCH), :] = (
                            y[16 * k + 8 * hf:16 * k + 8 * hf + 8])
            return run
        return [load] + [one(g) for g in range(3)]

    def half_pass(cid, half, fill, zero, timed=(), at=()):
        timed = list(timed)
        nre = CFG["pro_nre"]
        toks = None
        for k, f in enumerate(batch_thunks(cid >> 2, cid & 3)[16 * half:16 * half + 16]):
            f(toks)
            toks = {}
            if k in at and timed:
                toks[0] = timed.pop(0)()
            if fill is not None:
                for n, r in enumerate(r for r in range(40) if r * nre // 40 == k):
                    if half == 1:
                        stage(r, fill)
                    relayout(r, fill >> 2, fill & 3, 1 - half)
                    toks[CFG["re_pos"][n]] = (wb, wa)[half][48 + zero, 0:8, :]

    def ln_parts(bb, zero):
        def part(j):
            set_input(bb, load_x(bb, 4 * j, 4), None, 4 * j)
            return pltpu.bitcast(xa[32 + zero, 0:8, 0:128], u32)
        return [functools.partial(part, j) for j in range(4)]

    def perm_parts(piece, zero):
        def part(fs):
            for f in fs:
                f()
            return pltpu.bitcast(wf[5 + zero, 128:WPITCH, :], u32)
        out = []
        for j in range(4):
            th = wperm_thunks(piece, j)
            out += [functools.partial(part, th[0:2]), functools.partial(part, th[2:3]),
                    functools.partial(part, th[3:4])]
        return out

    def pro0(zero, carry):
        for u in range(4):
            cp_x(4 * u + 3).wait()
        for u in range(4):
            set_input(4 * u + 3, load_x(4 * u + 3), u)
        cp_w(0).wait()
        for i in range(40):
            stage(i, 0)
            relayout(i, 0, 0, 0)
        half_pass(0, 0, 0, zero)
        return carry

    def pro1(it, carry):
        bb = body_chunk(it)
        with jax.named_scope("pro1_wait"):
            cp_w(it + 1).wait()

            @pl.when(it >= 3)
            def _():
                cp_f(it - 3).wait()
            cp_x(bb).wait()
        piece = jnp.where(it >= 3, it - 3, 8)
        zero = it >> 4
        half_pass(it, 1, it + 1, zero, ln_parts(bb, zero) if 'l' not in CFG.get('skip', '') else (), CFG["ln_at"])
        half_pass(it + 1, 0, it + 1, zero, perm_parts(piece, zero) if 'w' not in CFG.get('skip', '') else (), CFG["perm_at"])
        return carry

    def pro2(zero, carry):
        cp_x(body_chunk(11)).wait()
        for cp in cp_rest:
            cp.wait()
        half_pass(11, 1, None, zero, ln_parts(body_chunk(11), zero), CFG["ln_at"])
        return carry

    if full:
        _loop("pro0", 0, 1, pro0, 0)
        _loop("pro1", 0, 11, pro1, 0)
        _loop("pro2", 0, 1, pro2, 0)

    scale = DH ** -0.5

    def wo_dot(hh, oo):
        return [_dot(oo, wo_t[j, 128 * hh:128 * hh + 128, :]) for j in range(5)]

    def addl(acc, res):
        return res if acc is None else [a + b for a, b in zip(acc, res)]

    def finish_thunks(gp, slot):
        st = {"acc": None}

        def f_wo(hh):
            def run():
                st["acc"] = addl(st["acc"], wo_dot(hh, ol[slot, hh].astype(bf16)))
                if hh == H - 1:
                    out = jnp.concatenate(st["acc"], axis=1)
                    for u in range(4):
                        ao[slot, 32 * u + 24:32 * u + 32, :] = out[8 * u:8 * u + 8]
            return run

        def pre(rows):
            x = _round_bf16(xa[gp, rows, :] + ao[slot, rows, :])
            xb[gp, rows, :] = x
            y = _layernorm(x)
            x0, x1, x2, x3, x4 = [y[:, 128 * a:128 * a + 128] for a in range(5)]
            t1, t2, t3, t4 = x1 + x4, x2 + x3, x1 - x4, x2 - x3
            xb[16, rows, :] = jnp.concatenate(
                [x0 + t1 + t2, x0 + C1 * t1 + C2 * t2, S1 * t3 + S2 * t4,
                 x0 + C2 * t1 + C1 * t2, S2 * t3 - S1 * t4], axis=1)

        def f_dft(cidx):
            def run(chunks=tuple(range(16))):
                g = cidx % 3
                o = FW_OFF + 128 * cidx
                lo, hi = (0, 128) if g == 0 else (256 * g - 128, 256 * g + 128)
                u = jnp.concatenate([xb[16, chunk(bb), lo:hi] for bb in chunks], axis=0)
                y = _dot(u.astype(bf16), _bf(small[o:o + (hi - lo) // 2, :]))
                for i, bb in enumerate(chunks):
                    zs[g][cidx // 3, gp, chunk(bb), :] = y[8 * i:8 * i + 8]
            return run
        return [f_wo(hh) for hh in range(H)], pre, [f_dft(cidx) for cidx in (0, 3, 1, 4, 2, 5)]

    def group(g, mem):
        cur = g & 1
        wos, pre, dfts = finish_thunks(jnp.maximum(g - 1, 0), 1 - cur)
        fillers = [wos[0:11], wos[11:22], wos[22:32], dfts]
        for ph in range(4):
            h = jnp.concatenate([mem, xa[16 + g, 32 * ph:32 * ph + 24, :]], axis=0).astype(bf16)
            pres = list(CFG["pre_rows"][ph])
            pre_at = CFG["pre_at"][ph]
            tok = None
            pr, sm, oos = {}, {}, {}

            def stacked(p, m):
                tails = [qb[g, ph, 32 * m + 2 * p + e] for e in range(2)]
                return jnp.concatenate([pr[p, m, 0], pr[p, m, 1]] + tails, axis=0).astype(bf16)

            def scores(p):
                sc = lax.dot_general(stacked(p, 0), stacked(p, 1), (((1,), (1,)), ((), ())),
                                     preferred_element_type=f32)
                fill = fill_ref[...]
                sc = jnp.where(fill == 0.0, sc * scale, fill)
                mx = jnp.max(sc, axis=-1, keepdims=True)
                e = jnp.exp(sc - mx)
                rl = pl.reciprocal(jnp.sum(e, axis=-1, keepdims=True), approx=True)
                sm[p] = ((e * rl).astype(bf16), None) if CFG["prenorm"] else (e.astype(bf16), rl)

            def pv(p):
                e, rl = sm[p]
                o = _dot(e, stacked(p, 2))
                if rl is not None:
                    o = o * rl
                ol[cur, 2 * p, 8 * ph:8 * ph + 8, :] = o[64:72]
                ol[cur, 2 * p + 1, 8 * ph:8 * ph + 8, :] = o[72:80]
                oos[2 * p], oos[2 * p + 1] = o[0:32].astype(bf16), o[32:64].astype(bf16)

            acc, t, nwo = None, 0.0, 0
            keyed = []
            for p in range(NPAIR):
                keyed += [(4 * p + 2 * i + e, (p, m, e)) for i, m in enumerate(CFG["first"]) for e in range(2)]
                keyed += [(4 * p + 3.5 + CFG["v_delay"] + CFG["v_gap"] * e, (p, 2, e)) for e in range(2)]
            bulk = [x for _, x in sorted(keyed, key=lambda kv: kv[0])]
            pend, ready, fl = [], [], list(fillers[ph])
            n_after = CFG["n_after"][ph]
            while nwo < H:
                pend.sort()
                if pend and pend[0][0] <= t:
                    _, kind, p = pend.pop(0)
                    if kind == "S":
                        scores(p)
                        pend.append((t + CFG["lat_pv"], "V", p))
                    else:
                        pv(p)
                        ready += [(t + CFG["lat_wo"], 2 * p + e) for e in range(2)]
                    t += 0.5
                elif bulk:
                    p, m, e = bulk.pop(0)
                    w, wt = wtile(m, p >> 2, p & 3, e)
                    pr[p, m, e] = _dot(h, _bf(_with_tokens(w[wt], tok)))
                    tok = None
                    if 96 - len(bulk) in pre_at:
                        pre(chunk(pres.pop(0)))
                        tok = {0: pltpu.bitcast(xb[17 + (g >> 4), 0:8, 0:128], u32)}
                    t += 1
                    if m == CFG["first"][1] and e == 1:
                        pend.append((t + CFG["lat_s"], "S", p))
                elif nwo >= CFG["fill_at"] and len(fl) > n_after:
                    fl.pop(0)()
                    t += 1
                elif ready and ready[0][0] <= t:
                    _, hh = ready.pop(0)
                    acc = addl(acc, wo_dot(hh, oos[hh]))
                    t += 1
                    nwo += 1
                elif len(fl) > n_after:
                    fl.pop(0)()
                    t += 1
                else:
                    t += 0.5
            out = jnp.concatenate(acc, axis=1)
            ao[cur, 32 * ph:32 * ph + 24, :] = out[8:32]
            mem = _round_bf16(out[0:8])
            for f in fl:
                f()
        return mem

    def spectral(zero):
        def fence(z):
            return z[0, zero, 128:ZPITCH, :]

        def radix_fwd(g, bb, tok=None):
            z = zs[g]
            xs = [(z[0, a, chunk(bb), :], z[1, a, chunk(bb), :]) for a in range(16)]
            if tok is not None:
                xs[:4] = [(xr + tok, xi) for xr, xi in xs[:4]]
            toks = []

            def emit(q, y):
                for p in range(4):
                    z[0, q + 4 * p, chunk(bb), :] = y[p][0]
                    z[1, q + 4 * p, chunk(bb), :] = y[p][1]
                if g > 0 or q == 3:
                    toks.append(fence(z))
            _fft16(xs, -1, emit)
            return toks

        ys = {}

        def fwd(g, k2, toks):
            z = zs[g]
            ur, ui = z[0, k2, 0:64, :], z[1, k2, 0:64, :]
            tr, ti = _twiddle((z[0, k2, 64:128, :], z[1, k2, 64:128, :]), k2, 32, -1)
            for hf in range(2):
                v = _ilv(ur + tr, ui + ti) if hf == 0 else _ilv(ur - tr, ui - ti)
                lhs = _with_tokens(emat[k2 + 16 * hf], toks if hf == 0 else None)
                xr, xi = _dilv(_dot(_bf(lhs), v.astype(bf16)))
                wr = wf[g, pl.ds(k2 * WPITCH + hf, 64, stride=2), :]
                wi = wf[g + 3, pl.ds(k2 * WPITCH + hf, 64, stride=2), :]
                ys[g, k2, hf] = _ilv(xr * wr - xi * wi, xr * wi + xi * wr).astype(bf16)

        def inv(g, k2):
            z = zs[g]
            t0 = _dot(_bf(emat[32 + k2]), ys.pop((g, k2, 0)))
            t1 = _dot(_bf(emat[48 + k2]), ys.pop((g, k2, 1)))
            z[0, k2, 0:64, :], z[1, k2, 0:64, :] = _dilv(t0 + t1)
            z[0, k2, 64:128, :], z[1, k2, 64:128, :] = _twiddle(_dilv(t0 - t1), k2, 32, 1)

        chain = {}
        for bb in range(16):
            chain[bb] = radix_fwd(0, bb, chain.get(bb - 2))[-1]
        radix_fwd(1, 0)
        units = [(g, k2) for g in range(3) for k2 in range(16)]
        toks = None
        for i in range(len(units) + 3):
            if i < len(units):
                fwd(*units[i], toks)
            if i >= 3:
                inv(*units[i - 3])
            toks = None
            if i < 31:
                t4 = radix_fwd(1 + (i + 1) // 16, (i + 1) % 16)
                toks = {3 + j: pltpu.bitcast(t, u32) for j, t in enumerate(t4)}

    def dinv_thunks(bb, finish):
        st = {}

        def rad(g):
            def run():
                z = zs[g]
                ys = _fft16([(z[0, a, chunk(bb), :], z[1, a, chunk(bb), :]) for a in range(16)], 1)
                st[g] = jnp.concatenate(
                    [jnp.concatenate([y[0] for y in ys], axis=0),
                     jnp.concatenate([y[1] for y in ys], axis=0)], axis=1).astype(bf16)
            return run

        def mm():
            st["p"] = [_dot(st[(j + 1) // 2], _bf(small[IW_OFF + 128 * j:IW_OFF + 128 * (j + 1), :]))
                       for j in range(5)]

        def fin():
            p0, p1, q1, p2, q2 = st["p"]
            e1, o1 = p0 + C1 * p1 + C2 * p2, S1 * q1 + S2 * q2
            e2, o2 = p0 + C2 * p1 + C1 * p2, S2 * q1 - S1 * q2
            y = jnp.concatenate([p0 + p1 + p2, e1 - o1, e2 - o2, e2 + o2, e1 + o1], axis=1)
            finish(xb[0:16, chunk(bb), :].reshape(128, DM) + y)
        return [rad(0), rad(1), rad(2), mm, fin]

    def out_copy(bb):
        return pltpu.make_async_copy(xin.at[:, bb], out_hbm.at[:, bb], osem.at[bb])

    def layer(li, carry0):
        if full or CFG["only"] == "group":
            _loop("step", 0, 16, group, mem_ref[...].astype(f32))
        if full or CFG["only"] == "spec":
            @pl.when((li >> 1) == 0)
            def _():
                with jax.named_scope("tail"):
                    wos, pre, dfts = finish_thunks(15, 1)
                    body = [bb for bb in range(16) if bb % 4 != 3]
                    for bb in body:
                        pre(chunk(bb))
                    for f in wos:
                        f()
                    for f in dfts:
                        f(body)
                    for bb in (3, 7, 11, 15):
                        pre(chunk(bb))
                    for f in dfts:
                        f((3, 7, 11, 15))
            with jax.named_scope("spectral"):
                spectral((li >> 1))
        if not full:
            return carry0

        @pl.when(li == 0)
        def _():
            with jax.named_scope("dinv_tails"):
                th = [dinv_thunks(4 * u + 3, functools.partial(
                    lambda u, x: set_input(4 * u + 3, _round_bf16(x), u), u)) for u in range(4)]
                for stage in range(5):
                    for u in range(4):
                        th[u][stage]()

            def batch(it, carry):
                bb = body_chunk(it)
                side = dinv_thunks(bb, lambda x: set_input(bb, _round_bf16(x), None))
                _interleave(batch_thunks(it >> 2, it & 3), side)
                return carry
            _loop("batch", 0, 12, batch, 0)

        @pl.when(li == 1)
        def _():
            with jax.named_scope("dinv_out"):
                def store_out(bb, x):
                    xin[:, bb] = x.reshape(16, 8, DM).astype(bf16)
                    out_copy(bb).start()
                th = [dinv_thunks(bb, functools.partial(store_out, bb)) for bb in range(16)]
                for i in range(17):
                    if i < 16:
                        for f in th[i][:4]:
                            f()
                    if i >= 1:
                        th[i - 1][4]()
                for bb in range(16):
                    out_copy(bb).wait()
        return carry0

    if CFG["only"] != "pro":
        lax.fori_loop(0, 2, layer, 0)


@functools.partial(jax.jit, static_argnames=("A_seg_len",))
def pallas_interleave_layers__memory_aug_recurrent_mem_tr__spectral_gfnet__prompt_kernel(
    A_x, A_mem0, A_Wq, A_Wk, A_Wv, A_Wo, A_seg_len, B_x, B_w_r, B_w_i,
):
    assert A_seg_len == SEG and A_x.shape == (1, S, DM)
    small, emat = _tables()
    hbm = pl.BlockSpec(memory_space=pltpu.HBM)
    vmem = pl.BlockSpec(memory_space=pltpu.VMEM)
    out = pl.pallas_call(
        _kernel,
        out_shape=jax.ShapeDtypeStruct((16, 16, 8, DM), bf16),
        in_specs=[hbm, vmem] + [hbm] * 8,
        out_specs=hbm,
        scratch_shapes=[
            pltpu.VMEM((16, 16, 8, DM), bf16),
            pltpu.VMEM((33, 128, DM), f32),
            pltpu.VMEM((18, 128, DM), f32),
            pltpu.VMEM((2, 128, DM), f32),
            pltpu.VMEM((12, DM, 8, DH), bf16),
            pltpu.VMEM((320 * TPITCH, 128), u32),
            pltpu.VMEM((49, 320, 128), u32),
            pltpu.VMEM((49, 320, 128), u32),
            pltpu.VMEM((5, H * DH, 128), bf16),
            pltpu.VMEM((16, 4, 96, 8, 128), f32),
            pltpu.VMEM((4, 5, 64, 128), u32),
            pltpu.VMEM((2, H, 32, 128), f32),
            pltpu.VMEM((2, 16, ZPITCH, 128), f32),
            pltpu.VMEM((2, 16, ZPITCH, 128), f32),
            pltpu.VMEM((2, 16, ZPITCH, 128), f32),
            pltpu.VMEM((6, 16 * WPITCH, 128), f32),
            pltpu.VMEM((9, DF, 512), bf16),
            pltpu.VMEM((4, 328, 128), f32),
            pltpu.VMEM((SMALL_ROWS, 128), u32),
            pltpu.VMEM((64, 64, 128), u32),
            pltpu.VMEM((80, 80), f32),
            pltpu.SemaphoreType.DMA((46,)),
            pltpu.SemaphoreType.DMA((16,)),
        ],
        compiler_params=pltpu.CompilerParams(vmem_limit_bytes=120 * 1024 * 1024),
    )(
        A_x.reshape(16, 16, 8, DM), A_mem0.reshape(MEM, DM),
        A_Wq, A_Wk, A_Wv, A_Wo.reshape(H * DH, DM), B_w_r.T, B_w_i.T,
        jnp.asarray(small), jnp.asarray(emat),
    )
    return out.reshape(1, S, DM)
```

```python
import functools
import math

import jax
import jax.numpy as jnp
import numpy as np
from jax import lax
import jax.experimental.pallas as pl
import jax.experimental.pallas.tpu as pltpu

f32, bf16, u32 = jnp.float32, jnp.bfloat16, jnp.uint32

S, DM, H, DH, MEM, SEG = 2048, 640, 32, 128, 8, 32
NSEG = S // SEG
NPAIR = H // 2
DF = DM // 2 + 1
EPS = 1e-5
WPITCH = 136

TPITCH = 9
ZPITCH = 136

S1 = math.sin(2 * math.pi / 5)
R5_D = (math.cos(2 * math.pi / 5) - math.cos(4 * math.pi / 5)) / 2
R5_R = math.sin(4 * math.pi / 5) / S1


def _to_bf16_bits(a):
    u = np.ascontiguousarray(a, dtype=np.float32).view(np.uint32).astype(np.uint64)
    return ((u + 0x7FFF + ((u >> 16) & 1)) >> 16).astype(np.uint32)


def _pack_rows(a):
    b = _to_bf16_bits(a)
    return b[..., 0::2, :] | (b[..., 1::2, :] << 16)


@functools.lru_cache(maxsize=None)
def _tables():
    b = np.arange(128)
    l0 = np.arange(0, DF, 5)
    l1 = np.concatenate([np.arange(1, 320, 5), np.arange(4, 320, 5)])
    l2 = np.concatenate([np.arange(2, 320, 5), np.arange(3, 320, 5)])
    sg = np.concatenate([np.ones(64), -np.ones(64)])

    def th(l):
        return 2 * np.pi * ((b[:, None] * l[None, :]) % DM) / DM

    fw = np.zeros((6, 256, 128))
    t = th(l0)
    fw[0, :128, :65] = np.cos(t)
    fw[3, :128, :65] = -np.sin(t)
    for g, l in ((1, l1), (2, l2)):
        t = th(l)
        c, s = np.cos(t), np.sin(t)
        fw[g] = np.concatenate([c, -S1 * sg * s], axis=0)
        fw[3 + g] = np.concatenate([-s, -S1 * sg * c], axis=0)
    sc = 1.0 / (S * DM)
    iw = np.zeros((5, 256, 128))
    t = th(l0).T
    cl = np.full((65, 1), 2.0)
    cl[0] = cl[-1] = 1.0
    iw[0, :65] = cl * np.cos(t) * sc
    iw[0, 128:128 + 65] = -cl * np.sin(t) * sc
    for g, l in ((1, l1), (2, l2)):
        t = th(l).T
        c, s = np.cos(t), np.sin(t)
        gg = sg[:, None]
        iw[2 * g - 1] = 2 * sc * np.concatenate([c, -s], axis=0)
        iw[2 * g] = 2 * sc * S1 * np.concatenate([gg * s, gg * c], axis=0)
    n = np.arange(64)
    order = np.concatenate([np.concatenate([np.arange(8) + 8 * j, np.arange(8) + 8 * j + 64])
                            for j in range(8)])
    e = np.zeros((2, 32, 128, 128))
    for k2 in range(32):
        t = 2 * np.pi * (((32 * n[:, None] + k2) * n[None, :]) % S) / S
        er, ei = np.cos(t), -np.sin(t)
        m = np.block([[er, -ei], [ei, er]])[order][:, order]
        e[0, k2], e[1, k2] = m, m.T
    small = np.concatenate(
        [_pack_rows(fw).reshape(-1, 128), _pack_rows(iw).reshape(-1, 128)], axis=0)
    return small, _pack_rows(e).reshape(64, 64, 128)


FW_OFF, IW_OFF = 0, 6 * 128
SMALL_ROWS = 11 * 128


def _loop(name, lo, hi, body, init, **kw):
    with jax.named_scope(name):
        return lax.fori_loop(lo, hi, body, init, **kw)


def _bf(x):
    return pltpu.bitcast(x, bf16)


def _dot(a, b):
    return jnp.dot(a, b, preferred_element_type=f32)


def _round_bf16(x):
    return x.astype(bf16).astype(f32)


def _layernorm(x):
    m = jnp.mean(x, axis=-1, keepdims=True)
    xc = x - m
    v = jnp.mean(xc * xc, axis=-1, keepdims=True)
    return xc * lax.rsqrt(v + EPS)


def _fft4(x, sign):
    (ar, ai), (br, bi), (cr, ci), (dr, di) = x
    t0r, t0i, t1r, t1i = ar + cr, ai + ci, ar - cr, ai - ci
    t2r, t2i, t3r, t3i = br + dr, bi + di, br - dr, bi - di
    y0, y2 = (t0r + t2r, t0i + t2i), (t0r - t2r, t0i - t2i)
    p, q = (t1r + t3i, t1i - t3r), (t1r - t3i, t1i + t3r)
    return [y0, p, y2, q] if sign < 0 else [y0, q, y2, p]


def _twiddle(z, n, period, sign):
    zr, zi = z
    n = n % period
    if n == 0:
        return z
    if 4 * n == period:
        return (-zi, zr) if sign > 0 else (zi, -zr)
    c, s = math.cos(2 * math.pi * n / period), sign * math.sin(2 * math.pi * n / period)
    if (8 * n) % period == 0:
        a, d = zr + zi, zr - zi
        if c * s > 0:
            return (d * c, a * c)
        return (a * c, d * s)
    return (zr * c - zi * s, zr * s + zi * c)


def _ilv(r, i):
    n = r.shape[0] // 8
    return jnp.concatenate([r.reshape(n, 8, 128), i.reshape(n, 8, 128)], axis=1).reshape(16 * n, 128)


def _dilv(x):
    n = x.shape[0] // 16
    x = x.reshape(n, 16, 128)
    return x[:, :8].reshape(8 * n, 128), x[:, 8:].reshape(8 * n, 128)


def _with_tokens(x, toks):
    if not toks:
        return x
    return jnp.concatenate(
        [x[8 * j:8 * j + 8] | toks[j] if j in toks else x[8 * j:8 * j + 8]
         for j in range(x.shape[0] // 8)], axis=0)


def _fft16(x, sign, emit=None):
    cols = [_fft4([x[4 * j + r] for j in range(4)], sign) for r in range(4)]
    out = [None] * 16
    for q in range(4):
        y = _fft4([_twiddle(cols[r][q], r * q, 16, sign) for r in range(4)], sign)
        for p in range(4):
            out[q + 4 * p] = y[p]
        if emit is not None:
            emit(q, y)
    return out


CFG = dict(lat_s=6, lat_pv=15, lat_wo=7, n_after=(11, 11, 11, 0), fill_at=16, v_delay=8, v_gap=0,
           prenorm=True,
           pre_at=((), (), (), tuple(range(11, 91, 5))), pre_rows=((), (), (), tuple(range(16))),
           first=(0, 1), dinv_at=(8, 9, 10, 11), rel=(1, 4), pro_nre=14, re_pos=(2, 5, 7), ln_at=(12, 13, 14, 15), perm_at=(3, 4, 5, 6, 7, 8, 9, 10, 11, 12, 13, 14), only=None)


def _interleave(main, side):
    n, k = len(main), 0
    for i, f in enumerate(main):
        f()
        while k < len(side) and (k + 1) * n <= (i + 1) * len(side):
            side[k]()
            k += 1
    for f in side[k:]:
        f()


def _kernel(x_hbm, mem_hbm, wq_hbm, wk_hbm, wv_hbm, wo_hbm, wr_hbm, wi_hbm,
            small_hbm, e_hbm, out_hbm,
            xin, xa, xb, ao, raw, tmp, wa, wb, wo_t, qb, hl, ol, z0, z1, z2, wf,
            wri, wtmp, small, emat, fill_ref, mem_ref, sem, osem):
    zs = (z0, z1, z2)
    w_hbm = (wq_hbm, wk_hbm, wv_hbm)

    def body_chunk(i):
        return 4 * (i & 3) + (i >> 2)

    def cp_w(i):
        src = w_hbm[i // 4 if isinstance(i, int) else 0]
        c = i & 3
        return pltpu.make_async_copy(src.at[:, pl.ds(pl.multiple_of(8 * c, 8), 8), :],
                                     raw.at[i], sem.at[i])

    def cp_x(bb):
        return pltpu.make_async_copy(x_hbm.at[:, bb], xin.at[:, bb], sem.at[12 + bb])

    def cp_f(i):
        src = (wr_hbm, wi_hbm)[i // 4 if isinstance(i, int) else 0]
        cols = pl.ds(pl.multiple_of(512 * (i & 3), 512), 512)
        return pltpu.make_async_copy(src.at[:, cols], wri.at[i], sem.at[36 + i])

    cp_rest = [pltpu.make_async_copy(wo_hbm.at[:, pl.ds(128 * j, 128)], wo_t.at[j], sem.at[28 + j])
               for j in range(5)]
    cp_rest += [pltpu.make_async_copy(mem_hbm, mem_ref, sem.at[33]),
                pltpu.make_async_copy(small_hbm, small, sem.at[44]),
               pltpu.make_async_copy(e_hbm, emat, sem.at[45])]

    full = CFG["only"] in (None, "pro")
    for u in range(4 if full else 0):
        cp_x(4 * u + 3).start()
    if full:
        cp_w(0).start()
    for i in range(12 if full else 0):
        if i < 11:
            cp_w(i + 1).start()
        cp_x(body_chunk(i)).start()
        if 3 <= i < 11:
            cp_f(i - 3).start()
    for cp in cp_rest if full else ():
        cp.start()

    r = lax.broadcasted_iota(jnp.int32, (80, 80), 0)
    c = lax.broadcasted_iota(jnp.int32, (80, 80), 1)

    def head(i):
        return jnp.where(i < 64, i // 32, (i - 64) // 8)

    def pos(i):
        return jnp.where(i < 64, i % 32, 32 + (i - 64) % 8)

    ok = (pos(r) < MEM) | (pos(r) >= pos(c))
    fill_ref[...] = jnp.where(head(r) == head(c), jnp.where(ok, 0.0, -1e9), -jnp.inf).astype(f32)
    ol[...] = jnp.zeros_like(ol)
    ao[...] = jnp.zeros_like(ao)
    wtmp[:, 320:328, :] = jnp.zeros((4, 8, 128), f32)
    xb[17, 0:8, 0:128] = jnp.zeros((8, 128), f32)
    xa[32, 0:8, 0:128] = jnp.zeros((8, 128), f32)
    wa[48, 0:8, :] = jnp.zeros((8, 128), u32)
    wb[48, 0:8, :] = jnp.zeros((8, 128), u32)
    wf[5, 128:WPITCH, :] = jnp.zeros((8, 128), f32)
    for z in zs:
        z[0, 0, 128:ZPITCH, :] = jnp.zeros((8, 128), f32)

    def chunk(bb):
        if isinstance(bb, int):
            return slice(8 * bb, 8 * bb + 8)
        return pl.ds(pl.multiple_of(8 * bb, 8), 8)

    def set_input(bb, x, tail_u, a0=0):
        n = x.shape[0] // 8
        xa[a0:a0 + n, chunk(bb), :] = x.reshape(n, 8, DM)
        y = _layernorm(x)
        if tail_u is None:
            xa[16 + a0:16 + a0 + n, chunk(bb), :] = y.reshape(n, 8, DM)
        else:
            yb = y.astype(bf16)
            for kt in range(5):
                hl[tail_u, kt] = pltpu.bitcast(yb[:, 128 * kt:128 * kt + 128], u32)

    def load_x(bb, a0=0, n=16):
        return xin[a0:a0 + n, bb].astype(f32).reshape(8 * n, DM)

    def wtile(m, c, j, e):
        return (wa, wb)[j >> 1], 12 * c + 6 * (j & 1) + 2 * m + e

    def stage(i, chunk_id):
        v = pltpu.bitcast(raw[chunk_id, 16 * i:16 * i + 16].reshape(128, 128), u32)
        for k in range(8):
            base = 8 * TPITCH * i + TPITCH * k
            tmp[base:base + 8, :] = v[8 * k:8 * k + 8]

    def relayout(i, m, c, half):
        for j in (2 * half, 2 * half + 1):
            a = tmp[pl.ds(8 * TPITCH * i + j, 8, stride=TPITCH), :]
            b = tmp[pl.ds(8 * TPITCH * i + 4 + j, 8, stride=TPITCH), :]
            w, t = wtile(m, c, j, 0)
            w[t, 8 * i:8 * i + 8, :] = (a & 0xFFFF) | (b << 16)
            w[t + 1, 8 * i:8 * i + 8, :] = (a >> 16) | (b & jnp.uint32(0xFFFF0000))

    def batch_thunks(m, c):
        def one(j, u, e):
            def run(toks=None):
                lhs = jnp.concatenate(
                    [_bf(_with_tokens(hl[u, kt], toks if kt == 0 else None)) for kt in range(5)], axis=1)
                w, t = wtile(m, c, j, e)
                qb[:, u, 8 * (4 * m + c) + 2 * j + e] = _dot(lhs, _bf(w[t])).reshape(16, 8, 128)
            return run
        return [one(j, u, e) for j in range(4) for u in range(4) for e in range(2)]

    def wperm_thunks(piece, j):
        m = (piece >> 2) & 1
        wt = wtmp.at[j]

        def load():
            wt[0:DF, :] = wri[piece, :, 128 * j:128 * j + 128].astype(f32)

        def one(g):
            def run():
                if g == 0:
                    t = jnp.concatenate([wt[pl.ds(0, 64, stride=5), :], wt[320:328, :],
                                         jnp.zeros((56, 128), f32)], axis=0)
                else:
                    t = jnp.concatenate([wt[pl.ds(g, 64, stride=5), :],
                                         wt[pl.ds(5 - g, 64, stride=5), :]], axis=0)
                y = t.T
                sub = wf.at[3 * m + g, pl.ds(pl.multiple_of((piece & 3) * 32, 32), 15 * WPITCH + 32)]
                for k in range(8):
                    for hf in range(2):
                        sub[pl.ds(8 * j + k + 8 * hf * WPITCH, 8, stride=WPITCH), :] = (
                            y[16 * k + 8 * hf:16 * k + 8 * hf + 8])
            return run
        return [load] + [one(g) for g in range(3)]

    def half_pass(cid, half, fill, zero, timed=(), at=()):
        timed = list(timed)
        nre = CFG["pro_nre"]
        toks = None
        for k, f in enumerate(batch_thunks(cid >> 2, cid & 3)[16 * half:16 * half + 16]):
            f(toks)
            toks = {}
            if k in at and timed:
                toks[0] = timed.pop(0)()
            if fill is not None:
                for n, r in enumerate(r for r in range(40) if r * nre // 40 == k):
                    if half == 1:
                        stage(r, fill)
                    relayout(r, fill >> 2, fill & 3, 1 - half)
                    toks[CFG["re_pos"][n]] = (wb, wa)[half][48 + zero, 0:8, :]

    def ln_parts(bb, zero):
        def part(j):
            set_input(bb, load_x(bb, 4 * j, 4), None, 4 * j)
            return pltpu.bitcast(xa[32 + zero, 0:8, 0:128], u32)
        return [functools.partial(part, j) for j in range(4)]

    def perm_parts(piece, zero):
        def part(fs):
            for f in fs:
                f()
            return pltpu.bitcast(wf[5 + zero, 128:WPITCH, :], u32)
        out = []
        for j in range(4):
            th = wperm_thunks(piece, j)
            out += [functools.partial(part, th[0:2]), functools.partial(part, th[2:3]),
                    functools.partial(part, th[3:4])]
        return out

    def pro0(zero, carry):
        for u in range(4):
            cp_x(4 * u + 3).wait()
        for u in range(4):
            set_input(4 * u + 3, load_x(4 * u + 3), u)
        cp_w(0).wait()
        for i in range(40):
            stage(i, 0)
            relayout(i, 0, 0, 0)
        half_pass(0, 0, 0, zero)
        return carry

    def pro1(it, carry):
        bb = body_chunk(it)
        with jax.named_scope("pro1_wait"):
            cp_w(it + 1).wait()

            @pl.when(it >= 3)
            def _():
                cp_f(it - 3).wait()
            cp_x(bb).wait()
        piece = jnp.where(it >= 3, it - 3, 8)
        zero = it >> 4
        half_pass(it, 1, it + 1, zero, ln_parts(bb, zero) if 'l' not in CFG.get('skip', '') else (), CFG["ln_at"])
        half_pass(it + 1, 0, it + 1, zero, perm_parts(piece, zero) if 'w' not in CFG.get('skip', '') else (), CFG["perm_at"])
        return carry

    def pro2(zero, carry):
        cp_x(body_chunk(11)).wait()
        for cp in cp_rest:
            cp.wait()
        half_pass(11, 1, None, zero, ln_parts(body_chunk(11), zero), CFG["ln_at"])
        return carry

    if full:
        _loop("pro0", 0, 1, pro0, 0)
        _loop("pro1", 0, 11, pro1, 0)
        _loop("pro2", 0, 1, pro2, 0)

    scale = DH ** -0.5

    def wo_dot(hh, oo):
        return [_dot(oo, wo_t[j, 128 * hh:128 * hh + 128, :]) for j in range(5)]

    def addl(acc, res):
        return res if acc is None else [a + b for a, b in zip(acc, res)]

    def finish_thunks(gp, slot):
        st = {"acc": None}

        def f_wo(hh):
            def run():
                st["acc"] = addl(st["acc"], wo_dot(hh, ol[slot, hh].astype(bf16)))
                if hh == H - 1:
                    out = jnp.concatenate(st["acc"], axis=1)
                    for u in range(4):
                        ao[slot, 32 * u + 24:32 * u + 32, :] = out[8 * u:8 * u + 8]
            return run

        def pre(rows):
            x = _round_bf16(xa[gp, rows, :] + ao[slot, rows, :])
            xb[gp, rows, :] = x
            y = _layernorm(x)
            x0, x1, x2, x3, x4 = [y[:, 128 * a:128 * a + 128] for a in range(5)]
            t1, t2, t3, t4 = x1 + x4, x2 + x3, x1 - x4, x2 - x3
            t = t1 + t2
            m, n = x0 - 0.25 * t, R5_D * (t1 - t2)
            xb[16, rows, :] = jnp.concatenate(
                [x0 + t, m + n, t3 + R5_R * t4, m - n, R5_R * t3 - t4], axis=1)

        def f_dft(cidx):
            def run(chunks=tuple(range(16))):
                g = cidx % 3
                o = FW_OFF + 128 * cidx
                lo, hi = (0, 128) if g == 0 else (256 * g - 128, 256 * g + 128)
                u = jnp.concatenate([xb[16, chunk(bb), lo:hi] for bb in chunks], axis=0)
                y = _dot(u.astype(bf16), _bf(small[o:o + (hi - lo) // 2, :]))
                for i, bb in enumerate(chunks):
                    zs[g][cidx // 3, gp, chunk(bb), :] = y[8 * i:8 * i + 8]
            return run
        return [f_wo(hh) for hh in range(H)], pre, [f_dft(cidx) for cidx in (0, 3, 1, 4, 2, 5)]

    def group(g, mem):
        cur = g & 1
        wos, pre, dfts = finish_thunks(jnp.maximum(g - 1, 0), 1 - cur)
        fillers = [wos[0:11], wos[11:22], wos[22:32], dfts]
        for ph in range(4):
            h = jnp.concatenate([mem, xa[16 + g, 32 * ph:32 * ph + 24, :]], axis=0).astype(bf16)
            pres = list(CFG["pre_rows"][ph])
            pre_at = CFG["pre_at"][ph]
            tok = None
            pr, sm, oos = {}, {}, {}

            def stacked(p, m):
                tails = [qb[g, ph, 32 * m + 2 * p + e] for e in range(2)]
                return jnp.concatenate([pr[p, m, 0], pr[p, m, 1]] + tails, axis=0).astype(bf16)

            def scores(p):
                sc = lax.dot_general(stacked(p, 0), stacked(p, 1), (((1,), (1,)), ((), ())),
                                     preferred_element_type=f32)
                fill = fill_ref[...]
                sc = jnp.where(fill == 0.0, sc * scale, fill)
                mx = jnp.max(sc, axis=-1, keepdims=True)
                e = jnp.exp(sc - mx)
                rl = pl.reciprocal(jnp.sum(e, axis=-1, keepdims=True), approx=True)
                sm[p] = ((e * rl).astype(bf16), None) if CFG["prenorm"] else (e.astype(bf16), rl)

            def pv(p):
                e, rl = sm[p]
                o = _dot(e, stacked(p, 2))
                if rl is not None:
                    o = o * rl
                ol[cur, 2 * p, 8 * ph:8 * ph + 8, :] = o[64:72]
                ol[cur, 2 * p + 1, 8 * ph:8 * ph + 8, :] = o[72:80]
                oos[2 * p], oos[2 * p + 1] = o[0:32].astype(bf16), o[32:64].astype(bf16)

            acc, t, nwo = None, 0.0, 0
            keyed = []
            for p in range(NPAIR):
                keyed += [(4 * p + 2 * i + e, (p, m, e)) for i, m in enumerate(CFG["first"]) for e in range(2)]
                keyed += [(4 * p + 3.5 + CFG["v_delay"] + CFG["v_gap"] * e, (p, 2, e)) for e in range(2)]
            bulk = [x for _, x in sorted(keyed, key=lambda kv: kv[0])]
            pend, ready, fl = [], [], list(fillers[ph])
            n_after = CFG["n_after"][ph]
            while nwo < H:
                pend.sort()
                if pend and pend[0][0] <= t:
                    _, kind, p = pend.pop(0)
                    if kind == "S":
                        scores(p)
                        pend.append((t + CFG["lat_pv"], "V", p))
                    else:
                        pv(p)
                        ready += [(t + CFG["lat_wo"], 2 * p + e) for e in range(2)]
                    t += 0.5
                elif bulk:
                    p, m, e = bulk.pop(0)
                    w, wt = wtile(m, p >> 2, p & 3, e)
                    pr[p, m, e] = _dot(h, _bf(_with_tokens(w[wt], tok)))
                    tok = None
                    if 96 - len(bulk) in pre_at:
                        pre(chunk(pres.pop(0)))
                        tok = {0: pltpu.bitcast(xb[17 + (g >> 4), 0:8, 0:128], u32)}
                    t += 1
                    if m == CFG["first"][1] and e == 1:
                        pend.append((t + CFG["lat_s"], "S", p))
                elif nwo >= CFG["fill_at"] and len(fl) > n_after:
                    fl.pop(0)()
                    t += 1
                elif ready and ready[0][0] <= t:
                    _, hh = ready.pop(0)
                    acc = addl(acc, wo_dot(hh, oos[hh]))
                    t += 1
                    nwo += 1
                elif len(fl) > n_after:
                    fl.pop(0)()
                    t += 1
                else:
                    t += 0.5
            out = jnp.concatenate(acc, axis=1)
            ao[cur, 32 * ph:32 * ph + 24, :] = out[8:32]
            mem = _round_bf16(out[0:8])
            for f in fl:
                f()
        return mem

    def spectral(zero):
        def fence(z):
            return z[0, zero, 128:ZPITCH, :]

        def radix_fwd(g, bb, tok=None, sign=-1):
            z = zs[g]
            xs = [(z[0, a, chunk(bb), :], z[1, a, chunk(bb), :]) for a in range(16)]
            if tok is not None:
                xs[:4] = [(xr + tok, xi) for xr, xi in xs[:4]]
            toks = []

            def emit(q, y):
                for p in range(4):
                    z[0, q + 4 * p, chunk(bb), :] = y[p][0]
                    z[1, q + 4 * p, chunk(bb), :] = y[p][1]
                if g > 0 or sign > 0 or q == 3:
                    toks.append(fence(z))
            _fft16(xs, sign, emit)
            return toks

        ys = {}

        def fwd(g, k2, toks):
            z = zs[g]
            ur, ui = z[0, k2, 0:64, :], z[1, k2, 0:64, :]
            tr, ti = _twiddle((z[0, k2, 64:128, :], z[1, k2, 64:128, :]), k2, 32, -1)
            for hf in range(2):
                v = _ilv(ur + tr, ui + ti) if hf == 0 else _ilv(ur - tr, ui - ti)
                lhs = _with_tokens(emat[k2 + 16 * hf], toks if hf == 0 else None)
                xr, xi = _dilv(_dot(_bf(lhs), v.astype(bf16)))
                ys["x", 16 * g + k2] = xr
                wr = wf[g, pl.ds(k2 * WPITCH + hf, 64, stride=2), :]
                wi = wf[g + 3, pl.ds(k2 * WPITCH + hf, 64, stride=2), :]
                ys[g, k2, hf] = _ilv(xr * wr - xi * wi, xr * wi + xi * wr).astype(bf16)

        def inv(g, k2):
            z = zs[g]
            t0 = _dot(_bf(emat[32 + k2]), ys.pop((g, k2, 0)))
            t1 = _dot(_bf(emat[48 + k2]), ys.pop((g, k2, 1)))
            z[0, k2, 0:64, :], z[1, k2, 0:64, :] = _dilv(t0 + t1)
            z[0, k2, 64:128, :], z[1, k2, 64:128, :] = _twiddle(_dilv(t0 - t1), k2, 32, 1)

        chain = {}
        for bb in range(16):
            chain[bb] = radix_fwd(0, bb, chain.get(bb - 2))[-1]
        radix_fwd(1, 0)
        units = [(g, k2) for g in range(3) for k2 in range(16)]
        toks = None
        for i in range(len(units) + 3):
            if i < len(units):
                fwd(*units[i], toks)
            if i >= 3:
                inv(*units[i - 3])
            toks = None
            if i < 47:
                if i < 31:
                    t4 = radix_fwd(1 + (i + 1) // 16, (i + 1) % 16)
                else:
                    back, r = CFG["rel"]
                    z0[1, zero, 128:ZPITCH, :] = ys["x", i - back][8 * r:8 * r + 8]
                    t4 = radix_fwd(0, i - 31, sign=1)
                toks = {3 + j: pltpu.bitcast(t, u32) for j, t in enumerate(t4)}

    def dinv_thunks(bb, finish):
        st = {}

        def part(g):
            def run():
                z = zs[g]
                ys = [(z[0, a, chunk(bb), :], z[1, a, chunk(bb), :]) for a in range(16)]
                if g > 0:
                    ys = _fft16(ys, 1)
                lhs = jnp.concatenate(
                    [jnp.concatenate([y[0] for y in ys], axis=0),
                     jnp.concatenate([y[1] for y in ys], axis=0)], axis=1).astype(bf16)
                for j in ((0,), (1, 2), (3, 4))[g]:
                    st[j] = _dot(lhs, _bf(small[IW_OFF + 128 * j:IW_OFF + 128 * (j + 1), :]))
            return run

        def fin():
            p0, p1, q1, p2, q2 = [st[j] for j in range(5)]
            t = p1 + p2
            m, n = p0 - 0.25 * t, R5_D * (p1 - p2)
            e1, e2 = m + n, m - n
            o1, o2 = q1 + R5_R * q2, R5_R * q1 - q2
            y = jnp.concatenate([p0 + t, e1 - o1, e2 - o2, e2 + o2, e1 + o1], axis=1)
            finish(xb[0:16, chunk(bb), :].reshape(128, DM) + y)
        return [part(0), part(1), part(2), fin]

    def out_copy(bb):
        return pltpu.make_async_copy(xin.at[:, bb], out_hbm.at[:, bb], osem.at[bb])

    def layer(li, carry0):
        if full or CFG["only"] == "group":
            _loop("step", 0, 16, group, mem_ref[...].astype(f32))
        if full or CFG["only"] == "spec":
            @pl.when((li >> 1) == 0)
            def _():
                with jax.named_scope("tail"):
                    wos, pre, dfts = finish_thunks(15, 1)
                    body = [bb for bb in range(16) if bb % 4 != 3]
                    for bb in body:
                        pre(chunk(bb))
                    for f in wos:
                        f()
                    for f in dfts:
                        f(body)
                    for bb in (3, 7, 11, 15):
                        pre(chunk(bb))
                    for f in dfts:
                        f((3, 7, 11, 15))
            with jax.named_scope("spectral"):
                spectral((li >> 1))
        if not full:
            return carry0

        @pl.when(li == 0)
        def _():
            with jax.named_scope("dinv_tails"):
                th = [dinv_thunks(4 * u + 3, functools.partial(
                    lambda u, x: set_input(4 * u + 3, _round_bf16(x), u), u)) for u in range(4)]
                for i in range(5):
                    if i < 4:
                        for f in th[i][:3]:
                            f()
                    if i >= 1:
                        th[i - 1][3]()

            def batch(it, carry):
                bb = body_chunk(it)
                side = dinv_thunks(bb, lambda x: set_input(bb, _round_bf16(x), None))
                for k, f in enumerate(batch_thunks(it >> 2, it & 3)):
                    f()
                    if k in CFG["dinv_at"]:
                        side.pop(0)()
                return carry
            _loop("batch", 0, 12, batch, 0)

        @pl.when(li == 1)
        def _():
            with jax.named_scope("dinv_out"):
                def store_out(bb, x):
                    xin[:, bb] = x.reshape(16, 8, DM).astype(bf16)
                    out_copy(bb).start()
                th = [dinv_thunks(bb, functools.partial(store_out, bb)) for bb in range(16)]
                for i in range(17):
                    if i < 16:
                        for f in th[i][:3]:
                            f()
                    if i >= 1:
                        th[i - 1][3]()
                for bb in range(16):
                    out_copy(bb).wait()
        return carry0

    if CFG["only"] != "pro":
        lax.fori_loop(0, 2, layer, 0)


@functools.partial(jax.jit, static_argnames=("A_seg_len",))
def pallas_interleave_layers__memory_aug_recurrent_mem_tr__spectral_gfnet__prompt_kernel(
    A_x, A_mem0, A_Wq, A_Wk, A_Wv, A_Wo, A_seg_len, B_x, B_w_r, B_w_i,
):
    assert A_seg_len == SEG and A_x.shape == (1, S, DM)
    small, emat = _tables()
    hbm = pl.BlockSpec(memory_space=pltpu.HBM)
    out = pl.pallas_call(
        _kernel,
        out_shape=jax.ShapeDtypeStruct((16, 16, 8, DM), bf16),
        in_specs=[hbm] * 10,
        out_specs=hbm,
        scratch_shapes=[
            pltpu.VMEM((16, 16, 8, DM), bf16),
            pltpu.VMEM((33, 128, DM), f32),
            pltpu.VMEM((18, 128, DM), f32),
            pltpu.VMEM((2, 128, DM), f32),
            pltpu.VMEM((12, DM, 8, DH), bf16),
            pltpu.VMEM((320 * TPITCH, 128), u32),
            pltpu.VMEM((49, 320, 128), u32),
            pltpu.VMEM((49, 320, 128), u32),
            pltpu.VMEM((5, H * DH, 128), bf16),
            pltpu.VMEM((16, 4, 96, 8, 128), f32),
            pltpu.VMEM((4, 5, 64, 128), u32),
            pltpu.VMEM((2, H, 32, 128), f32),
            pltpu.VMEM((2, 16, ZPITCH, 128), f32),
            pltpu.VMEM((2, 16, ZPITCH, 128), f32),
            pltpu.VMEM((2, 16, ZPITCH, 128), f32),
            pltpu.VMEM((6, 16 * WPITCH, 128), f32),
            pltpu.VMEM((9, DF, 512), bf16),
            pltpu.VMEM((4, 328, 128), f32),
            pltpu.VMEM((SMALL_ROWS, 128), u32),
            pltpu.VMEM((64, 64, 128), u32),
            pltpu.VMEM((80, 80), f32),
            pltpu.VMEM((MEM, DM), bf16),
            pltpu.SemaphoreType.DMA((46,)),
            pltpu.SemaphoreType.DMA((16,)),
        ],
        compiler_params=pltpu.CompilerParams(vmem_limit_bytes=120 * 1024 * 1024),
    )(
        A_x.reshape(16, 16, 8, DM), A_mem0.reshape(MEM, DM),
        A_Wq, A_Wk, A_Wv, A_Wo.reshape(H * DH, DM), B_w_r.T, B_w_i.T,
        jnp.asarray(small), jnp.asarray(emat),
    )
    return out.reshape(1, S, DM)
```

```python
import functools
import math

import jax
import jax.numpy as jnp
import numpy as np
from jax import lax
import jax.experimental.pallas as pl
import jax.experimental.pallas.tpu as pltpu

f32, bf16, u32 = jnp.float32, jnp.bfloat16, jnp.uint32

S, DM, H, DH, MEM, SEG = 2048, 640, 32, 128, 8, 32
NSEG = S // SEG
NPAIR = H // 2
DF = DM // 2 + 1
EPS = 1e-5
WPITCH = 136

TPITCH = 9
ZPITCH = 136

S1 = math.sin(2 * math.pi / 5)
R5_D = (math.cos(2 * math.pi / 5) - math.cos(4 * math.pi / 5)) / 2
R5_R = math.sin(4 * math.pi / 5) / S1


def _to_bf16_bits(a):
    u = np.ascontiguousarray(a, dtype=np.float32).view(np.uint32).astype(np.uint64)
    return ((u + 0x7FFF + ((u >> 16) & 1)) >> 16).astype(np.uint32)


def _pack_rows(a):
    b = _to_bf16_bits(a)
    return b[..., 0::2, :] | (b[..., 1::2, :] << 16)


@functools.lru_cache(maxsize=None)
def _tables():
    b = np.arange(128)
    l0 = np.arange(0, DF, 5)
    l1 = np.concatenate([np.arange(1, 320, 5), np.arange(4, 320, 5)])
    l2 = np.concatenate([np.arange(2, 320, 5), np.arange(3, 320, 5)])
    sg = np.concatenate([np.ones(64), -np.ones(64)])

    def th(l):
        return 2 * np.pi * ((b[:, None] * l[None, :]) % DM) / DM

    fw = np.zeros((6, 256, 128))
    t = th(l0)
    fw[0, :128, :65] = np.cos(t)
    fw[3, :128, :65] = -np.sin(t)
    for g, l in ((1, l1), (2, l2)):
        t = th(l)
        c, s = np.cos(t), np.sin(t)
        fw[g] = np.concatenate([c, -S1 * sg * s], axis=0)
        fw[3 + g] = np.concatenate([-s, -S1 * sg * c], axis=0)
    sc = 1.0 / (S * DM)
    iw = np.zeros((5, 256, 128))
    t = th(l0).T
    cl = np.full((65, 1), 2.0)
    cl[0] = cl[-1] = 1.0
    iw[0, :65] = cl * np.cos(t) * sc
    iw[0, 128:128 + 65] = -cl * np.sin(t) * sc
    for g, l in ((1, l1), (2, l2)):
        t = th(l).T
        c, s = np.cos(t), np.sin(t)
        gg = sg[:, None]
        iw[2 * g - 1] = 2 * sc * np.concatenate([c, -s], axis=0)
        iw[2 * g] = 2 * sc * S1 * np.concatenate([gg * s, gg * c], axis=0)
    n = np.arange(64)
    order = np.concatenate([np.concatenate([np.arange(8) + 8 * j, np.arange(8) + 8 * j + 64])
                            for j in range(8)])
    e = np.zeros((2, 32, 128, 128))
    for k2 in range(32):
        t = 2 * np.pi * (((32 * n[:, None] + k2) * n[None, :]) % S) / S
        er, ei = np.cos(t), -np.sin(t)
        m = np.block([[er, -ei], [ei, er]])[order][:, order]
        e[0, k2], e[1, k2] = m, m.T
    small = np.concatenate(
        [_pack_rows(fw).reshape(-1, 128), _pack_rows(iw).reshape(-1, 128)], axis=0)
    return small, _pack_rows(e).reshape(64, 64, 128)


FW_OFF, IW_OFF = 0, 6 * 128
SMALL_ROWS = 11 * 128


def _loop(name, lo, hi, body, init, **kw):
    with jax.named_scope(name):
        return lax.fori_loop(lo, hi, body, init, **kw)


def _bf(x):
    return pltpu.bitcast(x, bf16)


def _dot(a, b):
    return jnp.dot(a, b, preferred_element_type=f32)


def _round_bf16(x):
    return x.astype(bf16).astype(f32)


def _layernorm(x):
    m = jnp.mean(x, axis=-1, keepdims=True)
    xc = x - m
    v = jnp.mean(xc * xc, axis=-1, keepdims=True)
    return xc * lax.rsqrt(v + EPS)


def _fft4(x, sign):
    (ar, ai), (br, bi), (cr, ci), (dr, di) = x
    t0r, t0i, t1r, t1i = ar + cr, ai + ci, ar - cr, ai - ci
    t2r, t2i, t3r, t3i = br + dr, bi + di, br - dr, bi - di
    y0, y2 = (t0r + t2r, t0i + t2i), (t0r - t2r, t0i - t2i)
    p, q = (t1r + t3i, t1i - t3r), (t1r - t3i, t1i + t3r)
    return [y0, p, y2, q] if sign < 0 else [y0, q, y2, p]


def _twiddle(z, n, period, sign):
    zr, zi = z
    n = n % period
    if n == 0:
        return z
    if 4 * n == period:
        return (-zi, zr) if sign > 0 else (zi, -zr)
    c, s = math.cos(2 * math.pi * n / period), sign * math.sin(2 * math.pi * n / period)
    if (8 * n) % period == 0:
        a, d = zr + zi, zr - zi
        if c * s > 0:
            return (d * c, a * c)
        return (a * c, d * s)
    return (zr * c - zi * s, zr * s + zi * c)


def _ilv(r, i):
    n = r.shape[0] // 8
    return jnp.concatenate([r.reshape(n, 8, 128), i.reshape(n, 8, 128)], axis=1).reshape(16 * n, 128)


def _dilv(x):
    n = x.shape[0] // 16
    x = x.reshape(n, 16, 128)
    return x[:, :8].reshape(8 * n, 128), x[:, 8:].reshape(8 * n, 128)


def _with_tokens(x, toks):
    if not toks:
        return x
    return jnp.concatenate(
        [x[8 * j:8 * j + 8] | toks[j] if j in toks else x[8 * j:8 * j + 8]
         for j in range(x.shape[0] // 8)], axis=0)


def _fft16(x, sign, emit=None):
    cols = [_fft4([x[4 * j + r] for j in range(4)], sign) for r in range(4)]
    out = [None] * 16
    for q in range(4):
        y = _fft4([_twiddle(cols[r][q], r * q, 16, sign) for r in range(4)], sign)
        for p in range(4):
            out[q + 4 * p] = y[p]
        if emit is not None:
            emit(q, y)
    return out


CFG = dict(lat_s=6, lat_pv=15, lat_wo=7, n_after=(11, 11, 11, 0), fill_at=16, v_delay=8, v_gap=0,
           prenorm=True,
           pre_at=((), (), (), tuple(range(11, 91, 5))), pre_rows=((), (), (), tuple(range(16))),
           first=(0, 1), dinv_at=(8, 9, 10, 11), rel=(1, 4), batch_unroll=2, pro_nre=14, re_pos=(2, 5, 7), ln_at=(12, 13, 14, 15), perm_at=(3, 4, 5, 6, 7, 8, 9, 10, 11, 12, 13, 14), only=None)


def _interleave(main, side):
    n, k = len(main), 0
    for i, f in enumerate(main):
        f()
        while k < len(side) and (k + 1) * n <= (i + 1) * len(side):
            side[k]()
            k += 1
    for f in side[k:]:
        f()


def _kernel(x_hbm, mem_hbm, wq_hbm, wk_hbm, wv_hbm, wo_hbm, wr_hbm, wi_hbm,
            small_hbm, e_hbm, out_hbm,
            xin, xa, xb, ao, raw, tmp, wa, wb, wo_t, qb, hl, ol, z0, z1, z2, wf,
            wri, wtmp, small, emat, fill_ref, mem_ref, sem, osem):
    zs = (z0, z1, z2)
    w_hbm = (wq_hbm, wk_hbm, wv_hbm)

    def body_chunk(i):
        return 4 * (i & 3) + (i >> 2)

    def cp_w(i):
        src = w_hbm[i >> 2].at[:, pl.ds(8 * (i & 3), 8), :] if isinstance(i, int) else raw.at[i]
        return pltpu.make_async_copy(src, raw.at[i], sem.at[i])

    def cp_x(bb):
        return pltpu.make_async_copy(x_hbm.at[:, bb], xin.at[:, bb], sem.at[12 + bb])

    def cp_f(i):
        src = ((wr_hbm, wi_hbm)[i >> 2].at[:, pl.ds(512 * (i & 3), 512)]
               if isinstance(i, int) else wri.at[i])
        return pltpu.make_async_copy(src, wri.at[i], sem.at[36 + i])

    cp_rest = [pltpu.make_async_copy(wo_hbm.at[:, pl.ds(128 * j, 128)], wo_t.at[j], sem.at[28 + j])
               for j in range(5)]
    cp_rest += [pltpu.make_async_copy(mem_hbm, mem_ref, sem.at[33]),
                pltpu.make_async_copy(small_hbm, small, sem.at[44]),
               pltpu.make_async_copy(e_hbm, emat, sem.at[45])]

    full = CFG["only"] in (None, "pro")
    for u in range(4 if full else 0):
        cp_x(4 * u + 3).start()
    if full:
        cp_w(0).start()
    for i in range(12 if full else 0):
        if i < 11:
            cp_w(i + 1).start()
        cp_x(body_chunk(i)).start()
        if 3 <= i < 11:
            cp_f(i - 3).start()
    for cp in cp_rest if full else ():
        cp.start()

    r = lax.broadcasted_iota(jnp.int32, (80, 80), 0)
    c = lax.broadcasted_iota(jnp.int32, (80, 80), 1)

    def head(i):
        return jnp.where(i < 64, i // 32, (i - 64) // 8)

    def pos(i):
        return jnp.where(i < 64, i % 32, 32 + (i - 64) % 8)

    ok = (pos(r) < MEM) | (pos(r) >= pos(c))
    fill_ref[...] = jnp.where(head(r) == head(c), jnp.where(ok, 0.0, -1e9), -jnp.inf).astype(f32)
    ol[...] = jnp.zeros_like(ol)
    ao[...] = jnp.zeros_like(ao)
    wtmp[:, 320:328, :] = jnp.zeros((4, 8, 128), f32)
    xb[17, 0:8, 0:128] = jnp.zeros((8, 128), f32)
    xa[32, 0:8, 0:128] = jnp.zeros((8, 128), f32)
    wa[48, 0:8, :] = jnp.zeros((8, 128), u32)
    wb[48, 0:8, :] = jnp.zeros((8, 128), u32)
    wf[5, 128:WPITCH, :] = jnp.zeros((8, 128), f32)
    for z in zs:
        z[0, 0, 128:ZPITCH, :] = jnp.zeros((8, 128), f32)

    def chunk(bb):
        if isinstance(bb, int):
            return slice(8 * bb, 8 * bb + 8)
        return pl.ds(pl.multiple_of(8 * bb, 8), 8)

    def set_input(bb, x, tail_u, a0=0):
        n = x.shape[0] // 8
        xa[a0:a0 + n, chunk(bb), :] = x.reshape(n, 8, DM)
        y = _layernorm(x)
        if tail_u is None:
            xa[16 + a0:16 + a0 + n, chunk(bb), :] = y.reshape(n, 8, DM)
        else:
            yb = y.astype(bf16)
            for kt in range(5):
                hl[tail_u, kt] = pltpu.bitcast(yb[:, 128 * kt:128 * kt + 128], u32)

    def load_x(bb, a0=0, n=16):
        return xin[a0:a0 + n, bb].astype(f32).reshape(8 * n, DM)

    def wtile(m, c, j, e):
        return (wa, wb)[j >> 1], 12 * c + 6 * (j & 1) + 2 * m + e

    def stage(i, chunk_id):
        v = pltpu.bitcast(raw[chunk_id, 16 * i:16 * i + 16].reshape(128, 128), u32)
        for k in range(8):
            base = 8 * TPITCH * i + TPITCH * k
            tmp[base:base + 8, :] = v[8 * k:8 * k + 8]

    def relayout(i, m, c, half):
        for j in (2 * half, 2 * half + 1):
            a = tmp[pl.ds(8 * TPITCH * i + j, 8, stride=TPITCH), :]
            b = tmp[pl.ds(8 * TPITCH * i + 4 + j, 8, stride=TPITCH), :]
            w, t = wtile(m, c, j, 0)
            w[t, 8 * i:8 * i + 8, :] = (a & 0xFFFF) | (b << 16)
            w[t + 1, 8 * i:8 * i + 8, :] = (a >> 16) | (b & jnp.uint32(0xFFFF0000))

    def batch_thunks(m, c):
        def one(j, u, e):
            def run(toks=None):
                lhs = jnp.concatenate(
                    [_bf(_with_tokens(hl[u, kt], toks if kt == 0 else None)) for kt in range(5)], axis=1)
                w, t = wtile(m, c, j, e)
                qb[:, u, 8 * (4 * m + c) + 2 * j + e] = _dot(lhs, _bf(w[t])).reshape(16, 8, 128)
            return run
        return [one(j, u, e) for j in range(4) for u in range(4) for e in range(2)]

    def wperm_thunks(piece, j):
        m = (piece >> 2) & 1
        wt = wtmp.at[j]

        def load():
            wt[0:DF, :] = wri[piece, :, 128 * j:128 * j + 128].astype(f32)

        def one(g):
            def run():
                if g == 0:
                    t = jnp.concatenate([wt[pl.ds(0, 64, stride=5), :], wt[320:328, :],
                                         jnp.zeros((56, 128), f32)], axis=0)
                else:
                    t = jnp.concatenate([wt[pl.ds(g, 64, stride=5), :],
                                         wt[pl.ds(5 - g, 64, stride=5), :]], axis=0)
                y = t.T
                sub = wf.at[3 * m + g, pl.ds(pl.multiple_of((piece & 3) * 32, 32), 15 * WPITCH + 32)]
                for k in range(8):
                    for hf in range(2):
                        sub[pl.ds(8 * j + k + 8 * hf * WPITCH, 8, stride=WPITCH), :] = (
                            y[16 * k + 8 * hf:16 * k + 8 * hf + 8])
            return run
        return [load] + [one(g) for g in range(3)]

    def half_pass(cid, half, fill, zero, timed=(), at=()):
        timed = list(timed)
        nre = CFG["pro_nre"]
        toks = None
        for k, f in enumerate(batch_thunks(cid >> 2, cid & 3)[16 * half:16 * half + 16]):
            f(toks)
            toks = {}
            if k in at and timed:
                toks[0] = timed.pop(0)()
            if fill is not None:
                for n, r in enumerate(r for r in range(40) if r * nre // 40 == k):
                    if half == 1:
                        stage(r, fill)
                    relayout(r, fill >> 2, fill & 3, 1 - half)
                    toks[CFG["re_pos"][n]] = (wb, wa)[half][48 + zero, 0:8, :]

    def ln_parts(bb, zero):
        def part(j):
            set_input(bb, load_x(bb, 4 * j, 4), None, 4 * j)
            return pltpu.bitcast(xa[32 + zero, 0:8, 0:128], u32)
        return [functools.partial(part, j) for j in range(4)]

    def perm_parts(piece, zero):
        def part(fs):
            for f in fs:
                f()
            return pltpu.bitcast(wf[5 + zero, 128:WPITCH, :], u32)
        out = []
        for j in range(4):
            th = wperm_thunks(piece, j)
            out += [functools.partial(part, th[0:2]), functools.partial(part, th[2:3]),
                    functools.partial(part, th[3:4])]
        return out

    def pro0(zero, carry):
        for u in range(4):
            cp_x(4 * u + 3).wait()
        for u in range(4):
            set_input(4 * u + 3, load_x(4 * u + 3), u)
        cp_w(0).wait()
        for i in range(40):
            stage(i, 0)
            relayout(i, 0, 0, 0)
        half_pass(0, 0, 0, zero)
        return carry

    def pro1(it, carry):
        bb = body_chunk(it)
        with jax.named_scope("pro1_wait"):
            cp_w(it + 1).wait()

            @pl.when(it >= 3)
            def _():
                cp_f(it - 3).wait()
            cp_x(bb).wait()
        piece = jnp.where(it >= 3, it - 3, 8)
        zero = it >> 4
        half_pass(it, 1, it + 1, zero, ln_parts(bb, zero) if 'l' not in CFG.get('skip', '') else (), CFG["ln_at"])
        half_pass(it + 1, 0, it + 1, zero, perm_parts(piece, zero) if 'w' not in CFG.get('skip', '') else (), CFG["perm_at"])
        return carry

    def pro2(zero, carry):
        cp_x(body_chunk(11)).wait()
        for cp in cp_rest:
            cp.wait()
        half_pass(11, 1, None, zero, ln_parts(body_chunk(11), zero), CFG["ln_at"])
        return carry

    if full:
        _loop("pro0", 0, 1, pro0, 0)
        _loop("pro1", 0, 11, pro1, 0)
        _loop("pro2", 0, 1, pro2, 0)

    scale = DH ** -0.5

    def wo_dot(hh, oo):
        return [_dot(oo, wo_t[j, 128 * hh:128 * hh + 128, :]) for j in range(5)]

    def addl(acc, res):
        return res if acc is None else [a + b for a, b in zip(acc, res)]

    def finish_thunks(gp, slot):
        st = {"acc": None}

        def f_wo(hh):
            def run():
                st["acc"] = addl(st["acc"], wo_dot(hh, ol[slot, hh].astype(bf16)))
                if hh == H - 1:
                    out = jnp.concatenate(st["acc"], axis=1)
                    for u in range(4):
                        ao[slot, 32 * u + 24:32 * u + 32, :] = out[8 * u:8 * u + 8]
            return run

        def pre(rows):
            x = _round_bf16(xa[gp, rows, :] + ao[slot, rows, :])
            xb[gp, rows, :] = x
            y = _layernorm(x)
            x0, x1, x2, x3, x4 = [y[:, 128 * a:128 * a + 128] for a in range(5)]
            t1, t2, t3, t4 = x1 + x4, x2 + x3, x1 - x4, x2 - x3
            t = t1 + t2
            m, n = x0 - 0.25 * t, R5_D * (t1 - t2)
            xb[16, rows, :] = jnp.concatenate(
                [x0 + t, m + n, t3 + R5_R * t4, m - n, R5_R * t3 - t4], axis=1)

        def f_dft(cidx):
            def run(chunks=tuple(range(16))):
                g = cidx % 3
                o = FW_OFF + 128 * cidx
                lo, hi = (0, 128) if g == 0 else (256 * g - 128, 256 * g + 128)
                u = jnp.concatenate([xb[16, chunk(bb), lo:hi] for bb in chunks], axis=0)
                y = _dot(u.astype(bf16), _bf(small[o:o + (hi - lo) // 2, :]))
                for i, bb in enumerate(chunks):
                    zs[g][cidx // 3, gp, chunk(bb), :] = y[8 * i:8 * i + 8]
            return run
        return [f_wo(hh) for hh in range(H)], pre, [f_dft(cidx) for cidx in (0, 3, 1, 4, 2, 5)]

    def group(g, mem):
        cur = g & 1
        wos, pre, dfts = finish_thunks(jnp.maximum(g - 1, 0), 1 - cur)
        fillers = [wos[0:11], wos[11:22], wos[22:32], dfts]
        for ph in range(4):
            h = jnp.concatenate([mem, xa[16 + g, 32 * ph:32 * ph + 24, :]], axis=0).astype(bf16)
            pres = list(CFG["pre_rows"][ph])
            pre_at = CFG["pre_at"][ph]
            tok = None
            pr, sm, oos = {}, {}, {}

            def stacked(p, m):
                tails = [qb[g, ph, 32 * m + 2 * p + e] for e in range(2)]
                return jnp.concatenate([pr[p, m, 0], pr[p, m, 1]] + tails, axis=0).astype(bf16)

            def scores(p):
                sc = lax.dot_general(stacked(p, 0), stacked(p, 1), (((1,), (1,)), ((), ())),
                                     preferred_element_type=f32)
                fill = fill_ref[...]
                sc = jnp.where(fill == 0.0, sc * scale, fill)
                mx = jnp.max(sc, axis=-1, keepdims=True)
                e = jnp.exp(sc - mx)
                rl = pl.reciprocal(jnp.sum(e, axis=-1, keepdims=True), approx=True)
                sm[p] = ((e * rl).astype(bf16), None) if CFG["prenorm"] else (e.astype(bf16), rl)

            def pv(p):
                e, rl = sm[p]
                o = _dot(e, stacked(p, 2))
                if rl is not None:
                    o = o * rl
                ol[cur, 2 * p, 8 * ph:8 * ph + 8, :] = o[64:72]
                ol[cur, 2 * p + 1, 8 * ph:8 * ph + 8, :] = o[72:80]
                oos[2 * p], oos[2 * p + 1] = o[0:32].astype(bf16), o[32:64].astype(bf16)

            acc, t, nwo = None, 0.0, 0
            keyed = []
            for p in range(NPAIR):
                keyed += [(4 * p + 2 * i + e, (p, m, e)) for i, m in enumerate(CFG["first"]) for e in range(2)]
                keyed += [(4 * p + 3.5 + CFG["v_delay"] + CFG["v_gap"] * e, (p, 2, e)) for e in range(2)]
            bulk = [x for _, x in sorted(keyed, key=lambda kv: kv[0])]
            pend, ready, fl = [], [], list(fillers[ph])
            n_after = CFG["n_after"][ph]
            while nwo < H:
                pend.sort()
                if pend and pend[0][0] <= t:
                    _, kind, p = pend.pop(0)
                    if kind == "S":
                        scores(p)
                        pend.append((t + CFG["lat_pv"], "V", p))
                    else:
                        pv(p)
                        ready += [(t + CFG["lat_wo"], 2 * p + e) for e in range(2)]
                    t += 0.5
                elif bulk:
                    p, m, e = bulk.pop(0)
                    w, wt = wtile(m, p >> 2, p & 3, e)
                    pr[p, m, e] = _dot(h, _bf(_with_tokens(w[wt], tok)))
                    tok = None
                    if 96 - len(bulk) in pre_at:
                        pre(chunk(pres.pop(0)))
                        tok = {0: pltpu.bitcast(xb[17 + (g >> 4), 0:8, 0:128], u32)}
                    t += 1
                    if m == CFG["first"][1] and e == 1:
                        pend.append((t + CFG["lat_s"], "S", p))
                elif nwo >= CFG["fill_at"] and len(fl) > n_after:
                    fl.pop(0)()
                    t += 1
                elif ready and ready[0][0] <= t:
                    _, hh = ready.pop(0)
                    acc = addl(acc, wo_dot(hh, oos[hh]))
                    t += 1
                    nwo += 1
                elif len(fl) > n_after:
                    fl.pop(0)()
                    t += 1
                else:
                    t += 0.5
            out = jnp.concatenate(acc, axis=1)
            ao[cur, 32 * ph:32 * ph + 24, :] = out[8:32]
            mem = _round_bf16(out[0:8])
            for f in fl:
                f()
        return mem

    def spectral(zero):
        def fence(z):
            return z[0, zero, 128:ZPITCH, :]

        def radix_fwd(g, bb, tok=None, sign=-1):
            z = zs[g]
            xs = [(z[0, a, chunk(bb), :], z[1, a, chunk(bb), :]) for a in range(16)]
            if tok is not None:
                xs[:4] = [(xr + tok, xi) for xr, xi in xs[:4]]
            toks = []

            def emit(q, y):
                for p in range(4):
                    z[0, q + 4 * p, chunk(bb), :] = y[p][0]
                    z[1, q + 4 * p, chunk(bb), :] = y[p][1]
                if g > 0 or sign > 0 or q == 3:
                    toks.append(fence(z))
            _fft16(xs, sign, emit)
            return toks

        ys = {}

        def fwd(g, k2, toks):
            z = zs[g]
            ur, ui = z[0, k2, 0:64, :], z[1, k2, 0:64, :]
            tr, ti = _twiddle((z[0, k2, 64:128, :], z[1, k2, 64:128, :]), k2, 32, -1)
            for hf in range(2):
                v = _ilv(ur + tr, ui + ti) if hf == 0 else _ilv(ur - tr, ui - ti)
                lhs = _with_tokens(emat[k2 + 16 * hf], toks if hf == 0 else None)
                xr, xi = _dilv(_dot(_bf(lhs), v.astype(bf16)))
                ys["x", 16 * g + k2] = xr
                wr = wf[g, pl.ds(k2 * WPITCH + hf, 64, stride=2), :]
                wi = wf[g + 3, pl.ds(k2 * WPITCH + hf, 64, stride=2), :]
                ys[g, k2, hf] = _ilv(xr * wr - xi * wi, xr * wi + xi * wr).astype(bf16)

        def inv(g, k2):
            z = zs[g]
            t0 = _dot(_bf(emat[32 + k2]), ys.pop((g, k2, 0)))
            t1 = _dot(_bf(emat[48 + k2]), ys.pop((g, k2, 1)))
            z[0, k2, 0:64, :], z[1, k2, 0:64, :] = _dilv(t0 + t1)
            z[0, k2, 64:128, :], z[1, k2, 64:128, :] = _twiddle(_dilv(t0 - t1), k2, 32, 1)

        chain = {}
        for bb in range(16):
            chain[bb] = radix_fwd(0, bb, chain.get(bb - 2))[-1]
        radix_fwd(1, 0)
        units = [(g, k2) for g in range(3) for k2 in range(16)]
        toks = None
        for i in range(len(units) + 3):
            if i < len(units):
                fwd(*units[i], toks)
            if i >= 3:
                inv(*units[i - 3])
            toks = None
            if i < 47:
                if i < 31:
                    t4 = radix_fwd(1 + (i + 1) // 16, (i + 1) % 16)
                else:
                    back, r = CFG["rel"]
                    z0[1, zero, 128:ZPITCH, :] = ys["x", i - back][8 * r:8 * r + 8]
                    t4 = radix_fwd(0, i - 31, sign=1)
                toks = {3 + j: pltpu.bitcast(t, u32) for j, t in enumerate(t4)}

    def dinv_thunks(bb, finish):
        st = {}

        def part(g):
            def run():
                z = zs[g]
                ys = [(z[0, a, chunk(bb), :], z[1, a, chunk(bb), :]) for a in range(16)]
                if g > 0:
                    ys = _fft16(ys, 1)
                lhs = jnp.concatenate(
                    [jnp.concatenate([y[0] for y in ys], axis=0),
                     jnp.concatenate([y[1] for y in ys], axis=0)], axis=1).astype(bf16)
                for j in ((0,), (1, 2), (3, 4))[g]:
                    st[j] = _dot(lhs, _bf(small[IW_OFF + 128 * j:IW_OFF + 128 * (j + 1), :]))
            return run

        def fin():
            p0, p1, q1, p2, q2 = [st[j] for j in range(5)]
            t = p1 + p2
            m, n = p0 - 0.25 * t, R5_D * (p1 - p2)
            e1, e2 = m + n, m - n
            o1, o2 = q1 + R5_R * q2, R5_R * q1 - q2
            y = jnp.concatenate([p0 + t, e1 - o1, e2 - o2, e2 + o2, e1 + o1], axis=1)
            finish(xb[0:16, chunk(bb), :].reshape(128, DM) + y)
        return [part(0), part(1), part(2), fin]

    def out_copy(bb):
        return pltpu.make_async_copy(xin.at[:, bb], out_hbm.at[:, bb], osem.at[bb])

    def layer(li, carry0):
        if full or CFG["only"] == "group":
            _loop("step", 0, 16, group, mem_ref[...].astype(f32))
        if full or CFG["only"] == "spec":
            @pl.when((li >> 1) == 0)
            def _():
                with jax.named_scope("tail"):
                    wos, pre, dfts = finish_thunks(15, 1)
                    body = [bb for bb in range(16) if bb % 4 != 3]
                    for bb in body:
                        pre(chunk(bb))
                    for f in wos:
                        f()
                    for f in dfts:
                        f(body)
                    for bb in (3, 7, 11, 15):
                        pre(chunk(bb))
                    for f in dfts:
                        f((3, 7, 11, 15))
            with jax.named_scope("spectral"):
                spectral((li >> 1))
        if not full:
            return carry0

        @pl.when(li == 0)
        def _():
            with jax.named_scope("dinv_tails"):
                th = [dinv_thunks(4 * u + 3, functools.partial(
                    lambda u, x: set_input(4 * u + 3, _round_bf16(x), u), u)) for u in range(4)]
                for i in range(5):
                    if i < 4:
                        for f in th[i][:3]:
                            f()
                    if i >= 1:
                        th[i - 1][3]()

            def batch(it, carry):
                bb = body_chunk(it)
                side = dinv_thunks(bb, lambda x: set_input(bb, _round_bf16(x), None))
                for k, f in enumerate(batch_thunks(it >> 2, it & 3)):
                    f()
                    if k in CFG["dinv_at"]:
                        side.pop(0)()
                return carry
            _loop("batch", 0, 12, batch, 0, unroll=CFG["batch_unroll"])

        @pl.when(li == 1)
        def _():
            with jax.named_scope("dinv_out"):
                def store_out(bb, x):
                    xin[:, bb] = x.reshape(16, 8, DM).astype(bf16)
                    out_copy(bb).start()
                th = [dinv_thunks(bb, functools.partial(store_out, bb)) for bb in range(16)]
                for i in range(17):
                    if i < 16:
                        for f in th[i][:3]:
                            f()
                    if i >= 1:
                        th[i - 1][3]()
                for bb in range(16):
                    out_copy(bb).wait()
        return carry0

    if CFG["only"] != "pro":
        lax.fori_loop(0, 2, layer, 0)


@functools.partial(jax.jit, static_argnames=("A_seg_len",))
def pallas_interleave_layers__memory_aug_recurrent_mem_tr__spectral_gfnet__prompt_kernel(
    A_x, A_mem0, A_Wq, A_Wk, A_Wv, A_Wo, A_seg_len, B_x, B_w_r, B_w_i,
):
    assert A_seg_len == SEG and A_x.shape == (1, S, DM)
    small, emat = _tables()
    hbm = pl.BlockSpec(memory_space=pltpu.HBM)
    out = pl.pallas_call(
        _kernel,
        out_shape=jax.ShapeDtypeStruct((16, 16, 8, DM), bf16),
        in_specs=[hbm] * 10,
        out_specs=hbm,
        scratch_shapes=[
            pltpu.VMEM((16, 16, 8, DM), bf16),
            pltpu.VMEM((33, 128, DM), f32),
            pltpu.VMEM((18, 128, DM), f32),
            pltpu.VMEM((2, 128, DM), f32),
            pltpu.VMEM((12, DM, 8, DH), bf16),
            pltpu.VMEM((320 * TPITCH, 128), u32),
            pltpu.VMEM((49, 320, 128), u32),
            pltpu.VMEM((49, 320, 128), u32),
            pltpu.VMEM((5, H * DH, 128), bf16),
            pltpu.VMEM((16, 4, 96, 8, 128), f32),
            pltpu.VMEM((4, 5, 64, 128), u32),
            pltpu.VMEM((2, H, 32, 128), f32),
            pltpu.VMEM((2, 16, ZPITCH, 128), f32),
            pltpu.VMEM((2, 16, ZPITCH, 128), f32),
            pltpu.VMEM((2, 16, ZPITCH, 128), f32),
            pltpu.VMEM((6, 16 * WPITCH, 128), f32),
            pltpu.VMEM((9, DF, 512), bf16),
            pltpu.VMEM((4, 328, 128), f32),
            pltpu.VMEM((SMALL_ROWS, 128), u32),
            pltpu.VMEM((64, 64, 128), u32),
            pltpu.VMEM((80, 80), f32),
            pltpu.VMEM((MEM, DM), bf16),
            pltpu.SemaphoreType.DMA((46,)),
            pltpu.SemaphoreType.DMA((16,)),
        ],
        compiler_params=pltpu.CompilerParams(vmem_limit_bytes=120 * 1024 * 1024,
                                             disable_semaphore_checks=True),
    )(
        A_x.reshape(16, 16, 8, DM), A_mem0.reshape(MEM, DM),
        A_Wq, A_Wk, A_Wv, A_Wo.reshape(H * DH, DM), B_w_r.T, B_w_i.T,
        jnp.asarray(small), jnp.asarray(emat),
    )
    return out.reshape(1, S, DM)
```

```python
import functools
import math

import jax
import jax.numpy as jnp
import numpy as np
from jax import lax
import jax.experimental.pallas as pl
import jax.experimental.pallas.tpu as pltpu

f32, bf16, u32 = jnp.float32, jnp.bfloat16, jnp.uint32

S, DM, H, DH, MEM, SEG = 2048, 640, 32, 128, 8, 32
NSEG = S // SEG
NPAIR = H // 2
DF = DM // 2 + 1
EPS = 1e-5
WPITCH = 136

HPITCH = 168
ZPITCH = 136

S1 = math.sin(2 * math.pi / 5)
R5_D = (math.cos(2 * math.pi / 5) - math.cos(4 * math.pi / 5)) / 2
R5_R = math.sin(4 * math.pi / 5) / S1


def _to_bf16_bits(a):
    u = np.ascontiguousarray(a, dtype=np.float32).view(np.uint32).astype(np.uint64)
    return ((u + 0x7FFF + ((u >> 16) & 1)) >> 16).astype(np.uint32)


def _pack_rows(a):
    b = _to_bf16_bits(a)
    return b[..., 0::2, :] | (b[..., 1::2, :] << 16)


@functools.lru_cache(maxsize=None)
def _tables():
    b = np.arange(128)
    l0 = np.arange(0, DF, 5)
    l1 = np.concatenate([np.arange(1, 320, 5), np.arange(4, 320, 5)])
    l2 = np.concatenate([np.arange(2, 320, 5), np.arange(3, 320, 5)])
    sg = np.concatenate([np.ones(64), -np.ones(64)])

    def th(l):
        return 2 * np.pi * ((b[:, None] * l[None, :]) % DM) / DM

    fw = np.zeros((6, 256, 128))
    t = th(l0)
    fw[0, :128, :65] = np.cos(t)
    fw[3, :128, :65] = -np.sin(t)
    for g, l in ((1, l1), (2, l2)):
        t = th(l)
        c, s = np.cos(t), np.sin(t)
        fw[g] = np.concatenate([c, -S1 * sg * s], axis=0)
        fw[3 + g] = np.concatenate([-s, -S1 * sg * c], axis=0)
    sc = 1.0 / (S * DM)
    iw = np.zeros((5, 256, 128))
    t = th(l0).T
    cl = np.full((65, 1), 2.0)
    cl[0] = cl[-1] = 1.0
    iw[0, :65] = cl * np.cos(t) * sc
    iw[0, 128:128 + 65] = -cl * np.sin(t) * sc
    for g, l in ((1, l1), (2, l2)):
        t = th(l).T
        c, s = np.cos(t), np.sin(t)
        gg = sg[:, None]
        iw[2 * g - 1] = 2 * sc * np.concatenate([c, -s], axis=0)
        iw[2 * g] = 2 * sc * S1 * np.concatenate([gg * s, gg * c], axis=0)
    n = np.arange(64)
    order = np.concatenate([np.concatenate([np.arange(8) + 8 * j, np.arange(8) + 8 * j + 64])
                            for j in range(8)])
    e = np.zeros((2, 32, 128, 128))
    for k2 in range(32):
        t = 2 * np.pi * (((32 * n[:, None] + k2) * n[None, :]) % S) / S
        er, ei = np.cos(t), -np.sin(t)
        m = np.block([[er, -ei], [ei, er]])[order][:, order]
        e[0, k2], e[1, k2] = m, m.T
    small = np.concatenate(
        [_pack_rows(fw).reshape(-1, 128), _pack_rows(iw).reshape(-1, 128)], axis=0)
    return small, _pack_rows(e).reshape(64, 64, 128)


FW_OFF, IW_OFF = 0, 6 * 128
SMALL_ROWS = 11 * 128


def _loop(name, lo, hi, body, init, **kw):
    with jax.named_scope(name):
        return lax.fori_loop(lo, hi, body, init, **kw)


def _bf(x):
    return pltpu.bitcast(x, bf16)


def _dot(a, b):
    return jnp.dot(a, b, preferred_element_type=f32)


def _round_bf16(x):
    return x.astype(bf16).astype(f32)


def _layernorm(x):
    m = jnp.mean(x, axis=-1, keepdims=True)
    xc = x - m
    v = jnp.mean(xc * xc, axis=-1, keepdims=True)
    return xc * lax.rsqrt(v + EPS)


def _fft4(x, sign):
    (ar, ai), (br, bi), (cr, ci), (dr, di) = x
    t0r, t0i, t1r, t1i = ar + cr, ai + ci, ar - cr, ai - ci
    t2r, t2i, t3r, t3i = br + dr, bi + di, br - dr, bi - di
    y0, y2 = (t0r + t2r, t0i + t2i), (t0r - t2r, t0i - t2i)
    p, q = (t1r + t3i, t1i - t3r), (t1r - t3i, t1i + t3r)
    return [y0, p, y2, q] if sign < 0 else [y0, q, y2, p]


def _twiddle(z, n, period, sign):
    zr, zi = z
    n = n % period
    if n == 0:
        return z
    if 4 * n == period:
        return (-zi, zr) if sign > 0 else (zi, -zr)
    c, s = math.cos(2 * math.pi * n / period), sign * math.sin(2 * math.pi * n / period)
    if (8 * n) % period == 0:
        a, d = zr + zi, zr - zi
        if c * s > 0:
            return (d * c, a * c)
        return (a * c, d * s)
    return (zr * c - zi * s, zr * s + zi * c)


def _ilv(r, i):
    n = r.shape[0] // 8
    return jnp.concatenate([r.reshape(n, 8, 128), i.reshape(n, 8, 128)], axis=1).reshape(16 * n, 128)


def _dilv(x):
    n = x.shape[0] // 16
    x = x.reshape(n, 16, 128)
    return x[:, :8].reshape(8 * n, 128), x[:, 8:].reshape(8 * n, 128)


def _with_tokens(x, toks):
    if not toks:
        return x
    return jnp.concatenate(
        [x[8 * j:8 * j + 8] | toks[j] if j in toks else x[8 * j:8 * j + 8]
         for j in range(x.shape[0] // 8)], axis=0)


def _fft16(x, sign, emit=None):
    cols = [_fft4([x[4 * j + r] for j in range(4)], sign) for r in range(4)]
    out = [None] * 16
    for q in range(4):
        y = _fft4([_twiddle(cols[r][q], r * q, 16, sign) for r in range(4)], sign)
        for p in range(4):
            out[q + 4 * p] = y[p]
        if emit is not None:
            emit(q, y)
    return out


CFG = dict(lat_s=6, lat_pv=15, lat_wo=7, n_after=(11, 11, 11, 0), fill_at=16, v_delay=8, v_gap=0,
           prenorm=True,
           pre_at=((), (), (), tuple(range(11, 91, 5))), pre_rows=((), (), (), tuple(range(16))),
           first=(0, 1), dinv_at=(8, 9, 10, 11), rel=(1, 4), batch_unroll=2, pro_nre=14, re_pos=(2, 5, 7), ln_at=(12, 13, 14, 15), perm_at=(3, 4, 5, 6, 7, 8, 9, 10, 11, 12, 13, 14), only=None)


def _interleave(main, side):
    n, k = len(main), 0
    for i, f in enumerate(main):
        f()
        while k < len(side) and (k + 1) * n <= (i + 1) * len(side):
            side[k]()
            k += 1
    for f in side[k:]:
        f()


def _kernel(x_hbm, mem_hbm, wq_hbm, wk_hbm, wv_hbm, wo_hbm, wr_hbm, wi_hbm,
            small_hbm, e_hbm, out_hbm,
            xin, xa, xb, ao, raw, wa, wb, wo_t, qb, hl, ol, z0, z1, z2, wf,
            wri, wtmp, small, emat, fill_ref, mem_ref, sem, osem):
    zs = (z0, z1, z2)
    w_hbm = (wq_hbm, wk_hbm, wv_hbm)

    def body_chunk(i):
        return 4 * (i & 3) + (i >> 2)

    def cp_w(i):
        src = w_hbm[i >> 2].at[:, pl.ds(8 * (i & 3), 8), :] if isinstance(i, int) else raw.at[i]
        return pltpu.make_async_copy(src, raw.at[i], sem.at[i])

    def cp_x(bb):
        return pltpu.make_async_copy(x_hbm.at[:, bb], xin.at[:, bb], sem.at[12 + bb])

    def cp_f(i):
        src = ((wr_hbm, wi_hbm)[i >> 2].at[:, pl.ds(512 * (i & 3), 512)]
               if isinstance(i, int) else wri.at[i])
        return pltpu.make_async_copy(src, wri.at[i], sem.at[36 + i])

    cp_rest = [pltpu.make_async_copy(wo_hbm.at[:, pl.ds(128 * j, 128)], wo_t.at[j], sem.at[28 + j])
               for j in range(5)]
    cp_rest += [pltpu.make_async_copy(mem_hbm, mem_ref, sem.at[33]),
                pltpu.make_async_copy(small_hbm, small, sem.at[44]),
               pltpu.make_async_copy(e_hbm, emat, sem.at[45])]

    full = CFG["only"] in (None, "pro")
    for u in range(4 if full else 0):
        cp_x(4 * u + 3).start()
    if full:
        cp_w(0).start()
    for i in range(12 if full else 0):
        if i < 11:
            cp_w(i + 1).start()
        cp_x(body_chunk(i)).start()
        if 3 <= i < 11:
            cp_f(i - 3).start()
    for cp in cp_rest if full else ():
        cp.start()

    r = lax.broadcasted_iota(jnp.int32, (80, 80), 0)
    c = lax.broadcasted_iota(jnp.int32, (80, 80), 1)

    def head(i):
        return jnp.where(i < 64, i // 32, (i - 64) // 8)

    def pos(i):
        return jnp.where(i < 64, i % 32, 32 + (i - 64) % 8)

    ok = (pos(r) < MEM) | (pos(r) >= pos(c))
    fill_ref[...] = jnp.where(head(r) == head(c), jnp.where(ok, 0.0, -1e9), -jnp.inf).astype(f32)
    ol[...] = jnp.zeros_like(ol)
    ao[...] = jnp.zeros_like(ao)
    wtmp[:, 320:328, :] = jnp.zeros((4, 8, 128), f32)
    xb[17, 0:8, 0:128] = jnp.zeros((8, 128), f32)
    xa[32, 0:8, 0:128] = jnp.zeros((8, 128), f32)
    wa[12, 0:8, :] = jnp.zeros((8, 128), u32)
    wb[12, 0:8, :] = jnp.zeros((8, 128), u32)
    wf[5, 128:WPITCH, :] = jnp.zeros((8, 128), f32)
    for z in zs:
        z[0, 0, 128:ZPITCH, :] = jnp.zeros((8, 128), f32)

    def chunk(bb):
        if isinstance(bb, int):
            return slice(8 * bb, 8 * bb + 8)
        return pl.ds(pl.multiple_of(8 * bb, 8), 8)

    def set_input(bb, x, tail_u, a0=0):
        n = x.shape[0] // 8
        xa[a0:a0 + n, chunk(bb), :] = x.reshape(n, 8, DM)
        y = _layernorm(x)
        if tail_u is None:
            xa[16 + a0:16 + a0 + n, chunk(bb), :] = y.reshape(n, 8, DM)
        else:
            yb = y.astype(bf16)
            for kt in range(5):
                hl[tail_u, kt] = pltpu.bitcast(yb[:, 128 * kt:128 * kt + 128], u32)

    def load_x(bb, a0=0, n=16):
        return xin[a0:a0 + n, bb].astype(f32).reshape(8 * n, DM)

    def wtile(cid, j, e):
        w = (wa, wb)[e]
        return jnp.concatenate([w[cid, (4 * hf + j) * HPITCH:(4 * hf + j) * HPITCH + 160, :]
                                for hf in range(2)], axis=0)

    def relayout(i, cid, e):
        for r in range(4 * i, 4 * i + 4):
            a, b = [pltpu.bitcast(jnp.concatenate([raw[cid, d], raw[cid, d + 320]], axis=0), u32)
                    for d in (2 * r, 2 * r + 1)]
            v = (a & 0xFFFF) | (b << 16) if e == 0 else (a >> 16) | (b & jnp.uint32(0xFFFF0000))
            (wa, wb)[e][cid, pl.ds(r, 8, stride=HPITCH), :] = v

    def batch_thunks(cid):
        def one(j, u, e):
            def run(toks=None):
                lhs = jnp.concatenate(
                    [_bf(_with_tokens(hl[u, kt], toks if kt == 0 else None)) for kt in range(5)], axis=1)
                qb[:, u, 8 * cid + 2 * j + e] = _dot(lhs, _bf(wtile(cid, j, e))).reshape(16, 8, 128)
            return run
        return [one(j, u, e) for e in range(2) for j in range(4) for u in range(4)]

    def wperm_thunks(piece, j):
        m = (piece >> 2) & 1
        wt = wtmp.at[j]

        def load():
            wt[0:DF, :] = wri[piece, :, 128 * j:128 * j + 128].astype(f32)

        def one(g):
            def run():
                if g == 0:
                    t = jnp.concatenate([wt[pl.ds(0, 64, stride=5), :], wt[320:328, :],
                                         jnp.zeros((56, 128), f32)], axis=0)
                else:
                    t = jnp.concatenate([wt[pl.ds(g, 64, stride=5), :],
                                         wt[pl.ds(5 - g, 64, stride=5), :]], axis=0)
                y = t.T
                sub = wf.at[3 * m + g, pl.ds(pl.multiple_of((piece & 3) * 32, 32), 15 * WPITCH + 32)]
                for k in range(8):
                    for hf in range(2):
                        sub[pl.ds(8 * j + k + 8 * hf * WPITCH, 8, stride=WPITCH), :] = (
                            y[16 * k + 8 * hf:16 * k + 8 * hf + 8])
            return run
        return [load] + [one(g) for g in range(3)]

    def half_pass(cid, half, fill, zero, timed=(), at=()):
        timed = list(timed)
        nre = CFG["pro_nre"]
        toks = None
        for k, f in enumerate(batch_thunks(cid)[16 * half:16 * half + 16]):
            f(toks)
            toks = {}
            if k in at and timed:
                toks[0] = timed.pop(0)()
            if fill is not None:
                for n, r in enumerate(r for r in range(40) if r * nre // 40 == k):
                    relayout(r, fill, 1 - half)
                    toks[CFG["re_pos"][n]] = (wb, wa)[half][12 + zero, 0:8, :]

    def ln_parts(bb, zero):
        def part(j):
            set_input(bb, load_x(bb, 4 * j, 4), None, 4 * j)
            return pltpu.bitcast(xa[32 + zero, 0:8, 0:128], u32)
        return [functools.partial(part, j) for j in range(4)]

    def perm_parts(piece, zero):
        def part(fs):
            for f in fs:
                f()
            return pltpu.bitcast(wf[5 + zero, 128:WPITCH, :], u32)
        out = []
        for j in range(4):
            th = wperm_thunks(piece, j)
            out += [functools.partial(part, th[0:2]), functools.partial(part, th[2:3]),
                    functools.partial(part, th[3:4])]
        return out

    def pro0(zero, carry):
        for u in range(4):
            cp_x(4 * u + 3).wait()
        for u in range(4):
            set_input(4 * u + 3, load_x(4 * u + 3), u)
        cp_w(0).wait()
        for i in range(40):
            relayout(i, 0, 0)
        half_pass(0, 0, 0, zero)
        return carry

    def pro1(it, carry):
        bb = body_chunk(it)
        with jax.named_scope("pro1_wait"):
            cp_w(it + 1).wait()

            @pl.when(it >= 3)
            def _():
                cp_f(it - 3).wait()
            cp_x(bb).wait()
        piece = jnp.where(it >= 3, it - 3, 8)
        zero = it >> 4
        half_pass(it, 1, it + 1, zero, ln_parts(bb, zero) if 'l' not in CFG.get('skip', '') else (), CFG["ln_at"])
        half_pass(it + 1, 0, it + 1, zero, perm_parts(piece, zero) if 'w' not in CFG.get('skip', '') else (), CFG["perm_at"])
        return carry

    def pro2(zero, carry):
        cp_x(body_chunk(11)).wait()
        for cp in cp_rest:
            cp.wait()
        half_pass(11, 1, None, zero, ln_parts(body_chunk(11), zero), CFG["ln_at"])
        return carry

    if full:
        _loop("pro0", 0, 1, pro0, 0)
        _loop("pro1", 0, 11, pro1, 0)
        _loop("pro2", 0, 1, pro2, 0)

    scale = DH ** -0.5

    def wo_dot(hh, oo):
        return [_dot(oo, wo_t[j, 128 * hh:128 * hh + 128, :]) for j in range(5)]

    def addl(acc, res):
        return res if acc is None else [a + b for a, b in zip(acc, res)]

    def finish_thunks(gp, slot):
        st = {"acc": None}

        def f_wo(hh):
            def run():
                st["acc"] = addl(st["acc"], wo_dot(hh, ol[slot, hh].astype(bf16)))
                if hh == H - 1:
                    out = jnp.concatenate(st["acc"], axis=1)
                    for u in range(4):
                        ao[slot, 32 * u + 24:32 * u + 32, :] = out[8 * u:8 * u + 8]
            return run

        def pre(rows):
            x = _round_bf16(xa[gp, rows, :] + ao[slot, rows, :])
            xb[gp, rows, :] = x
            y = _layernorm(x)
            x0, x1, x2, x3, x4 = [y[:, 128 * a:128 * a + 128] for a in range(5)]
            t1, t2, t3, t4 = x1 + x4, x2 + x3, x1 - x4, x2 - x3
            t = t1 + t2
            m, n = x0 - 0.25 * t, R5_D * (t1 - t2)
            xb[16, rows, :] = jnp.concatenate(
                [x0 + t, m + n, t3 + R5_R * t4, m - n, R5_R * t3 - t4], axis=1)

        def f_dft(cidx):
            def run(chunks=tuple(range(16))):
                g = cidx % 3
                o = FW_OFF + 128 * cidx
                lo, hi = (0, 128) if g == 0 else (256 * g - 128, 256 * g + 128)
                u = jnp.concatenate([xb[16, chunk(bb), lo:hi] for bb in chunks], axis=0)
                y = _dot(u.astype(bf16), _bf(small[o:o + (hi - lo) // 2, :]))
                for i, bb in enumerate(chunks):
                    zs[g][cidx // 3, gp, chunk(bb), :] = y[8 * i:8 * i + 8]
            return run
        return [f_wo(hh) for hh in range(H)], pre, [f_dft(cidx) for cidx in (0, 3, 1, 4, 2, 5)]

    def group(g, mem):
        cur = g & 1
        wos, pre, dfts = finish_thunks(jnp.maximum(g - 1, 0), 1 - cur)
        fillers = [wos[0:11], wos[11:22], wos[22:32], dfts]
        for ph in range(4):
            h = jnp.concatenate([mem, xa[16 + g, 32 * ph:32 * ph + 24, :]], axis=0).astype(bf16)
            pres = list(CFG["pre_rows"][ph])
            pre_at = CFG["pre_at"][ph]
            tok = None
            pr, sm, oos = {}, {}, {}

            def stacked(p, m):
                tails = [qb[g, ph, 32 * m + 2 * p + e] for e in range(2)]
                return jnp.concatenate([pr[p, m, 0], pr[p, m, 1]] + tails, axis=0).astype(bf16)

            def scores(p):
                sc = lax.dot_general(stacked(p, 0), stacked(p, 1), (((1,), (1,)), ((), ())),
                                     preferred_element_type=f32)
                fill = fill_ref[...]
                sc = jnp.where(fill == 0.0, sc * scale, fill)
                mx = jnp.max(sc, axis=-1, keepdims=True)
                e = jnp.exp(sc - mx)
                rl = pl.reciprocal(jnp.sum(e, axis=-1, keepdims=True), approx=True)
                sm[p] = ((e * rl).astype(bf16), None) if CFG["prenorm"] else (e.astype(bf16), rl)

            def pv(p):
                e, rl = sm[p]
                o = _dot(e, stacked(p, 2))
                if rl is not None:
                    o = o * rl
                ol[cur, 2 * p, 8 * ph:8 * ph + 8, :] = o[64:72]
                ol[cur, 2 * p + 1, 8 * ph:8 * ph + 8, :] = o[72:80]
                oos[2 * p], oos[2 * p + 1] = o[0:32].astype(bf16), o[32:64].astype(bf16)

            acc, t, nwo = None, 0.0, 0
            keyed = []
            for p in range(NPAIR):
                keyed += [(4 * p + 2 * i + e, (p, m, e)) for i, m in enumerate(CFG["first"]) for e in range(2)]
                keyed += [(4 * p + 3.5 + CFG["v_delay"] + CFG["v_gap"] * e, (p, 2, e)) for e in range(2)]
            bulk = [x for _, x in sorted(keyed, key=lambda kv: kv[0])]
            pend, ready, fl = [], [], list(fillers[ph])
            n_after = CFG["n_after"][ph]
            while nwo < H:
                pend.sort()
                if pend and pend[0][0] <= t:
                    _, kind, p = pend.pop(0)
                    if kind == "S":
                        scores(p)
                        pend.append((t + CFG["lat_pv"], "V", p))
                    else:
                        pv(p)
                        ready += [(t + CFG["lat_wo"], 2 * p + e) for e in range(2)]
                    t += 0.5
                elif bulk:
                    p, m, e = bulk.pop(0)
                    pr[p, m, e] = _dot(h, _bf(_with_tokens(wtile(4 * m + (p >> 2), p & 3, e), tok)))
                    tok = None
                    if 96 - len(bulk) in pre_at:
                        pre(chunk(pres.pop(0)))
                        tok = {0: pltpu.bitcast(xb[17 + (g >> 4), 0:8, 0:128], u32)}
                    t += 1
                    if m == CFG["first"][1] and e == 1:
                        pend.append((t + CFG["lat_s"], "S", p))
                elif nwo >= CFG["fill_at"] and len(fl) > n_after:
                    fl.pop(0)()
                    t += 1
                elif ready and ready[0][0] <= t:
                    _, hh = ready.pop(0)
                    acc = addl(acc, wo_dot(hh, oos[hh]))
                    t += 1
                    nwo += 1
                elif len(fl) > n_after:
                    fl.pop(0)()
                    t += 1
                else:
                    t += 0.5
            out = jnp.concatenate(acc, axis=1)
            ao[cur, 32 * ph:32 * ph + 24, :] = out[8:32]
            mem = _round_bf16(out[0:8])
            for f in fl:
                f()
        return mem

    def spectral(zero):
        def fence(z):
            return z[0, zero, 128:ZPITCH, :]

        def radix_fwd(g, bb, tok=None, sign=-1):
            z = zs[g]
            xs = [(z[0, a, chunk(bb), :], z[1, a, chunk(bb), :]) for a in range(16)]
            if tok is not None:
                xs[:4] = [(xr + tok, xi) for xr, xi in xs[:4]]
            toks = []

            def emit(q, y):
                for p in range(4):
                    z[0, q + 4 * p, chunk(bb), :] = y[p][0]
                    z[1, q + 4 * p, chunk(bb), :] = y[p][1]
                if g > 0 or sign > 0 or q == 3:
                    toks.append(fence(z))
            _fft16(xs, sign, emit)
            return toks

        ys = {}

        def fwd(g, k2, toks):
            z = zs[g]
            ur, ui = z[0, k2, 0:64, :], z[1, k2, 0:64, :]
            tr, ti = _twiddle((z[0, k2, 64:128, :], z[1, k2, 64:128, :]), k2, 32, -1)
            for hf in range(2):
                v = _ilv(ur + tr, ui + ti) if hf == 0 else _ilv(ur - tr, ui - ti)
                lhs = _with_tokens(emat[k2 + 16 * hf], toks if hf == 0 else None)
                xr, xi = _dilv(_dot(_bf(lhs), v.astype(bf16)))
                ys["x", 16 * g + k2] = xr
                wr = wf[g, pl.ds(k2 * WPITCH + hf, 64, stride=2), :]
                wi = wf[g + 3, pl.ds(k2 * WPITCH + hf, 64, stride=2), :]
                ys[g, k2, hf] = _ilv(xr * wr - xi * wi, xr * wi + xi * wr).astype(bf16)

        def inv(g, k2):
            z = zs[g]
            t0 = _dot(_bf(emat[32 + k2]), ys.pop((g, k2, 0)))
            t1 = _dot(_bf(emat[48 + k2]), ys.pop((g, k2, 1)))
            z[0, k2, 0:64, :], z[1, k2, 0:64, :] = _dilv(t0 + t1)
            z[0, k2, 64:128, :], z[1, k2, 64:128, :] = _twiddle(_dilv(t0 - t1), k2, 32, 1)

        chain = {}
        for bb in range(16):
            chain[bb] = radix_fwd(0, bb, chain.get(bb - 2))[-1]
        radix_fwd(1, 0)
        units = [(g, k2) for g in range(3) for k2 in range(16)]
        toks = None
        for i in range(len(units) + 3):
            if i < len(units):
                fwd(*units[i], toks)
            if i >= 3:
                inv(*units[i - 3])
            toks = None
            if i < 47:
                if i < 31:
                    t4 = radix_fwd(1 + (i + 1) // 16, (i + 1) % 16)
                else:
                    back, r = CFG["rel"]
                    z0[1, zero, 128:ZPITCH, :] = ys["x", i - back][8 * r:8 * r + 8]
                    t4 = radix_fwd(0, i - 31, sign=1)
                toks = {3 + j: pltpu.bitcast(t, u32) for j, t in enumerate(t4)}

    def dinv_thunks(bb, finish):
        st = {}

        def part(g):
            def run():
                z = zs[g]
                ys = [(z[0, a, chunk(bb), :], z[1, a, chunk(bb), :]) for a in range(16)]
                if g > 0:
                    ys = _fft16(ys, 1)
                lhs = jnp.concatenate(
                    [jnp.concatenate([y[0] for y in ys], axis=0),
                     jnp.concatenate([y[1] for y in ys], axis=0)], axis=1).astype(bf16)
                for j in ((0,), (1, 2), (3, 4))[g]:
                    st[j] = _dot(lhs, _bf(small[IW_OFF + 128 * j:IW_OFF + 128 * (j + 1), :]))
            return run

        def fin():
            p0, p1, q1, p2, q2 = [st[j] for j in range(5)]
            t = p1 + p2
            m, n = p0 - 0.25 * t, R5_D * (p1 - p2)
            e1, e2 = m + n, m - n
            o1, o2 = q1 + R5_R * q2, R5_R * q1 - q2
            y = jnp.concatenate([p0 + t, e1 - o1, e2 - o2, e2 + o2, e1 + o1], axis=1)
            finish(xb[0:16, chunk(bb), :].reshape(128, DM) + y)
        return [part(0), part(1), part(2), fin]

    def out_copy(bb):
        return pltpu.make_async_copy(xin.at[:, bb], out_hbm.at[:, bb], osem.at[bb])

    def layer(li, carry0):
        if full or CFG["only"] == "group":
            _loop("step", 0, 16, group, mem_ref[...].astype(f32))
        if full or CFG["only"] == "spec":
            @pl.when((li >> 1) == 0)
            def _():
                with jax.named_scope("tail"):
                    wos, pre, dfts = finish_thunks(15, 1)
                    body = [bb for bb in range(16) if bb % 4 != 3]
                    for bb in body:
                        pre(chunk(bb))
                    for f in wos:
                        f()
                    for f in dfts:
                        f(body)
                    for bb in (3, 7, 11, 15):
                        pre(chunk(bb))
                    for f in dfts:
                        f((3, 7, 11, 15))
            with jax.named_scope("spectral"):
                spectral((li >> 1))
        if not full:
            return carry0

        @pl.when(li == 0)
        def _():
            with jax.named_scope("dinv_tails"):
                th = [dinv_thunks(4 * u + 3, functools.partial(
                    lambda u, x: set_input(4 * u + 3, _round_bf16(x), u), u)) for u in range(4)]
                for i in range(5):
                    if i < 4:
                        for f in th[i][:3]:
                            f()
                    if i >= 1:
                        th[i - 1][3]()

            def batch(it, carry):
                bb = body_chunk(it)
                side = dinv_thunks(bb, lambda x: set_input(bb, _round_bf16(x), None))
                for k, f in enumerate(batch_thunks(it)):
                    f()
                    if k in CFG["dinv_at"]:
                        side.pop(0)()
                return carry
            _loop("batch", 0, 12, batch, 0, unroll=CFG["batch_unroll"])

        @pl.when(li == 1)
        def _():
            with jax.named_scope("dinv_out"):
                def store_out(bb, x):
                    xin[:, bb] = x.reshape(16, 8, DM).astype(bf16)
                    out_copy(bb).start()
                th = [dinv_thunks(bb, functools.partial(store_out, bb)) for bb in range(16)]
                for i in range(17):
                    if i < 16:
                        for f in th[i][:3]:
                            f()
                    if i >= 1:
                        th[i - 1][3]()
                for bb in range(16):
                    out_copy(bb).wait()
        return carry0

    if CFG["only"] != "pro":
        lax.fori_loop(0, 2, layer, 0)


@functools.partial(jax.jit, static_argnames=("A_seg_len",))
def pallas_interleave_layers__memory_aug_recurrent_mem_tr__spectral_gfnet__prompt_kernel(
    A_x, A_mem0, A_Wq, A_Wk, A_Wv, A_Wo, A_seg_len, B_x, B_w_r, B_w_i,
):
    assert A_seg_len == SEG and A_x.shape == (1, S, DM)
    small, emat = _tables()
    hbm = pl.BlockSpec(memory_space=pltpu.HBM)
    out = pl.pallas_call(
        _kernel,
        out_shape=jax.ShapeDtypeStruct((16, 16, 8, DM), bf16),
        in_specs=[hbm] * 10,
        out_specs=hbm,
        scratch_shapes=[
            pltpu.VMEM((16, 16, 8, DM), bf16),
            pltpu.VMEM((33, 128, DM), f32),
            pltpu.VMEM((18, 128, DM), f32),
            pltpu.VMEM((2, 128, DM), f32),
            pltpu.VMEM((12, DM, 8, DH), bf16),
            pltpu.VMEM((13, 8 * HPITCH, 128), u32),
            pltpu.VMEM((13, 8 * HPITCH, 128), u32),
            pltpu.VMEM((5, H * DH, 128), bf16),
            pltpu.VMEM((16, 4, 96, 8, 128), f32),
            pltpu.VMEM((4, 5, 64, 128), u32),
            pltpu.VMEM((2, H, 32, 128), f32),
            pltpu.VMEM((2, 16, ZPITCH, 128), f32),
            pltpu.VMEM((2, 16, ZPITCH, 128), f32),
            pltpu.VMEM((2, 16, ZPITCH, 128), f32),
            pltpu.VMEM((6, 16 * WPITCH, 128), f32),
            pltpu.VMEM((9, DF, 512), bf16),
            pltpu.VMEM((4, 328, 128), f32),
            pltpu.VMEM((SMALL_ROWS, 128), u32),
            pltpu.VMEM((64, 64, 128), u32),
            pltpu.VMEM((80, 80), f32),
            pltpu.VMEM((MEM, DM), bf16),
            pltpu.SemaphoreType.DMA((46,)),
            pltpu.SemaphoreType.DMA((16,)),
        ],
        compiler_params=pltpu.CompilerParams(vmem_limit_bytes=120 * 1024 * 1024,
                                             disable_semaphore_checks=True),
    )(
        A_x.reshape(16, 16, 8, DM), A_mem0.reshape(MEM, DM),
        A_Wq, A_Wk, A_Wv, A_Wo.reshape(H * DH, DM), B_w_r.T, B_w_i.T,
        jnp.asarray(small), jnp.asarray(emat),
    )
    return out.reshape(1, S, DM)
```

```python
import functools
import math

import jax
import jax.numpy as jnp
import numpy as np
from jax import lax
import jax.experimental.pallas as pl
import jax.experimental.pallas.tpu as pltpu

f32, bf16, u32 = jnp.float32, jnp.bfloat16, jnp.uint32

S, DM, H, DH, MEM, SEG = 2048, 640, 32, 128, 8, 32
NSEG = S // SEG
NPAIR = H // 2
DF = DM // 2 + 1
EPS = 1e-5
WPITCH = 132

HPITCH = 164
ZPITCH = 136

S1 = math.sin(2 * math.pi / 5)
R5_D = (math.cos(2 * math.pi / 5) - math.cos(4 * math.pi / 5)) / 2
R5_R = math.sin(4 * math.pi / 5) / S1


def _to_bf16_bits(a):
    u = np.ascontiguousarray(a, dtype=np.float32).view(np.uint32).astype(np.uint64)
    return ((u + 0x7FFF + ((u >> 16) & 1)) >> 16).astype(np.uint32)


def _pack_rows(a):
    b = _to_bf16_bits(a)
    return b[..., 0::2, :] | (b[..., 1::2, :] << 16)


@functools.lru_cache(maxsize=None)
def _tables():
    b = np.arange(128)
    l0 = np.arange(0, DF, 5)
    l1 = np.concatenate([np.arange(1, 320, 5), np.arange(4, 320, 5)])
    l2 = np.concatenate([np.arange(2, 320, 5), np.arange(3, 320, 5)])
    sg = np.concatenate([np.ones(64), -np.ones(64)])

    def th(l):
        return 2 * np.pi * ((b[:, None] * l[None, :]) % DM) / DM

    fw = np.zeros((6, 256, 128))
    t = th(l0)
    fw[0, :128, :65] = np.cos(t)
    fw[3, :128, :65] = -np.sin(t)
    for g, l in ((1, l1), (2, l2)):
        t = th(l)
        c, s = np.cos(t), np.sin(t)
        fw[g] = np.concatenate([c, -S1 * sg * s], axis=0)
        fw[3 + g] = np.concatenate([-s, -S1 * sg * c], axis=0)
    sc = 1.0 / (S * DM)
    iw = np.zeros((5, 256, 128))
    t = th(l0).T
    cl = np.full((65, 1), 2.0)
    cl[0] = cl[-1] = 1.0
    iw[0, :65] = cl * np.cos(t) * sc
    iw[0, 128:128 + 65] = -cl * np.sin(t) * sc
    for g, l in ((1, l1), (2, l2)):
        t = th(l).T
        c, s = np.cos(t), np.sin(t)
        gg = sg[:, None]
        iw[2 * g - 1] = 2 * sc * np.concatenate([c, -s], axis=0)
        iw[2 * g] = 2 * sc * S1 * np.concatenate([gg * s, gg * c], axis=0)
    n = np.arange(64)
    order = np.concatenate([np.concatenate([np.arange(8) + 8 * j, np.arange(8) + 8 * j + 64])
                            for j in range(8)])
    e = np.zeros((2, 32, 128, 128))
    for k2 in range(32):
        t = 2 * np.pi * (((32 * n[:, None] + k2) * n[None, :]) % S) / S
        er, ei = np.cos(t), -np.sin(t)
        m = np.block([[er, -ei], [ei, er]])[order][:, order]
        e[0, k2], e[1, k2] = m, m.T
    small = np.concatenate(
        [_pack_rows(fw).reshape(-1, 128), _pack_rows(iw).reshape(-1, 128)], axis=0)
    return small, _pack_rows(e).reshape(64, 64, 128)


FW_OFF, IW_OFF = 0, 6 * 128
SMALL_ROWS = 11 * 128


def _loop(name, lo, hi, body, init, **kw):
    with jax.named_scope(name):
        return lax.fori_loop(lo, hi, body, init, **kw)


def _bf(x):
    return pltpu.bitcast(x, bf16)


def _dot(a, b):
    return jnp.dot(a, b, preferred_element_type=f32)


def _round_bf16(x):
    return x.astype(bf16).astype(f32)


def _layernorm(x):
    m = jnp.mean(x, axis=-1, keepdims=True)
    xc = x - m
    v = jnp.mean(xc * xc, axis=-1, keepdims=True)
    return xc * lax.rsqrt(v + EPS)


def _fft4(x, sign):
    (ar, ai), (br, bi), (cr, ci), (dr, di) = x
    t0r, t0i, t1r, t1i = ar + cr, ai + ci, ar - cr, ai - ci
    t2r, t2i, t3r, t3i = br + dr, bi + di, br - dr, bi - di
    y0, y2 = (t0r + t2r, t0i + t2i), (t0r - t2r, t0i - t2i)
    p, q = (t1r + t3i, t1i - t3r), (t1r - t3i, t1i + t3r)
    return [y0, p, y2, q] if sign < 0 else [y0, q, y2, p]


def _twiddle(z, n, period, sign):
    zr, zi = z
    n = n % period
    if n == 0:
        return z
    if 4 * n == period:
        return (-zi, zr) if sign > 0 else (zi, -zr)
    c, s = math.cos(2 * math.pi * n / period), sign * math.sin(2 * math.pi * n / period)
    if (8 * n) % period == 0:
        a, d = zr + zi, zr - zi
        if c * s > 0:
            return (d * c, a * c)
        return (a * c, d * s)
    return (zr * c - zi * s, zr * s + zi * c)


def _ilv(r, i):
    n = r.shape[0] // 8
    return jnp.concatenate([r.reshape(n, 8, 128), i.reshape(n, 8, 128)], axis=1).reshape(16 * n, 128)


def _dilv(x):
    n = x.shape[0] // 16
    x = x.reshape(n, 16, 128)
    return x[:, :8].reshape(8 * n, 128), x[:, 8:].reshape(8 * n, 128)


def _with_tokens(x, toks):
    if not toks:
        return x
    return jnp.concatenate(
        [x[8 * j:8 * j + 8] | toks[j] if j in toks else x[8 * j:8 * j + 8]
         for j in range(x.shape[0] // 8)], axis=0)


def _fft16(x, sign, emit=None):
    cols = [_fft4([x[4 * j + r] for j in range(4)], sign) for r in range(4)]
    out = [None] * 16
    for q in range(4):
        y = _fft4([_twiddle(cols[r][q], r * q, 16, sign) for r in range(4)], sign)
        for p in range(4):
            out[q + 4 * p] = y[p]
        if emit is not None:
            emit(q, y)
    return out


CFG = dict(lat_s=6, lat_pv=15, lat_wo=7, n_after=(11, 11, 11, 0), fill_at=16, v_delay=8, v_gap=0,
           prenorm=True,
           pre_at=((), (), (), tuple(range(11, 91, 5))), pre_rows=((), (), (), tuple(range(16))),
           first=(0, 1), dinv_at=(8, 9, 10, 11), rel=(1, 4), batch_unroll=2, pro_nre=14, re_pos=(2, 5, 7), ln_at=(12, 13, 14, 15), ln_at2=(4, 7, 10, 13), perm_at=(3, 4, 5, 6, 7, 8, 9, 10, 11, 12, 13, 14), only=None)


def _interleave(main, side):
    n, k = len(main), 0
    for i, f in enumerate(main):
        f()
        while k < len(side) and (k + 1) * n <= (i + 1) * len(side):
            side[k]()
            k += 1
    for f in side[k:]:
        f()


def _kernel(x_hbm, mem_hbm, wq_hbm, wk_hbm, wv_hbm, wo_hbm, wr_hbm, wi_hbm,
            small_hbm, e_hbm, out_hbm,
            xin, xa, xb, ao, raw, wa, wb, wo_t, qb, hl, ol, z0, z1, z2, wf,
            wri, wtmp, small, emat, fill_ref, mem_ref, zero_ref, sem, osem):
    zs = (z0, z1, z2)
    w_hbm = (wq_hbm, wk_hbm, wv_hbm)

    def body_chunk(i):
        return 4 * (i & 3) + (i >> 2)

    def cp_w(i):
        src = w_hbm[i >> 2].at[:, :, pl.ds(8 * (i & 3), 8), :] if isinstance(i, int) else raw.at[i]
        return pltpu.make_async_copy(src, raw.at[i], sem.at[i])

    def cp_x(bb):
        return pltpu.make_async_copy(x_hbm.at[:, bb], xin.at[:, bb], sem.at[12 + bb])

    def cp_f(i):
        src = ((wr_hbm, wi_hbm)[i >> 2].at[:, pl.ds(512 * (i & 3), 512)]
               if isinstance(i, int) else wri.at[i])
        return pltpu.make_async_copy(src, wri.at[i], sem.at[36 + i])

    cp_rest = [pltpu.make_async_copy(wo_hbm.at[:, pl.ds(128 * j, 128)], wo_t.at[j], sem.at[28 + j])
               for j in range(5)]
    cp_rest += [pltpu.make_async_copy(mem_hbm, mem_ref, sem.at[33]),
                pltpu.make_async_copy(small_hbm, small, sem.at[44]),
               pltpu.make_async_copy(e_hbm, emat, sem.at[45])]

    full = CFG["only"] in (None, "pro")
    for u in range(4 if full else 0):
        cp_x(4 * u + 3).start()
    if full:
        cp_w(0).start()
    for i in range(12 if full else 0):
        if i < 11:
            cp_w(i + 1).start()
        cp_x(body_chunk(i)).start()
        if 3 <= i < 11:
            cp_f(i - 3).start()
    for cp in cp_rest if full else ():
        cp.start()

    zero_ref[0] = 0

    r = lax.broadcasted_iota(jnp.int32, (80, 80), 0)
    c = lax.broadcasted_iota(jnp.int32, (80, 80), 1)

    def head(i):
        return jnp.where(i < 64, i // 32, (i - 64) // 8)

    def pos(i):
        return jnp.where(i < 64, i % 32, 32 + (i - 64) % 8)

    ok = (pos(r) < MEM) | (pos(r) >= pos(c))
    fill_ref[...] = jnp.where(head(r) == head(c), jnp.where(ok, 0.0, -1e9), -jnp.inf).astype(f32)
    ol[...] = jnp.zeros_like(ol)
    ao[...] = jnp.zeros_like(ao)
    wtmp[:, 320:328, :] = jnp.zeros((4, 8, 128), f32)
    xb[17, 0:8, 0:128] = jnp.zeros((8, 128), f32)
    xa[32, 0:8, 0:128] = jnp.zeros((8, 128), f32)
    wa[12, 0:8, :] = jnp.zeros((8, 128), u32)
    wb[12, 0:8, :] = jnp.zeros((8, 128), u32)
    wf[5, 16 * WPITCH:16 * WPITCH + 8, :] = jnp.zeros((8, 128), f32)
    for z in zs:
        z[0, 0, 128:ZPITCH, :] = jnp.zeros((8, 128), f32)

    def chunk(bb):
        if isinstance(bb, int):
            return slice(8 * bb, 8 * bb + 8)
        return pl.ds(pl.multiple_of(8 * bb, 8), 8)

    def set_input(bb, x, tail_u, a0=0):
        n = x.shape[0] // 8
        xa[a0:a0 + n, chunk(bb), :] = x.reshape(n, 8, DM)
        y = _layernorm(x)
        if tail_u is None:
            xa[16 + a0:16 + a0 + n, chunk(bb), :] = y.reshape(n, 8, DM)
        else:
            yb = y.astype(bf16)
            for kt in range(5):
                hl[tail_u, kt] = pltpu.bitcast(yb[:, 128 * kt:128 * kt + 128], u32)

    def load_x(bb, a0=0, n=16):
        return xin[a0:a0 + n, bb].astype(f32).reshape(8 * n, DM)

    def wtile(cid, j, e):
        w = (wa, wb)[e]
        return jnp.concatenate([w[cid, (4 * hf + j) * HPITCH:(4 * hf + j) * HPITCH + 160, :]
                                for hf in range(2)], axis=0)

    def relayout(i, cid, e):
        for r in range(4 * i, 4 * i + 4):
            a, b = [pltpu.bitcast(raw[cid, :, d].reshape(16, 128), u32) for d in (2 * r, 2 * r + 1)]
            v = (a & 0xFFFF) | (b << 16) if e == 0 else (a >> 16) | (b & jnp.uint32(0xFFFF0000))
            (wa, wb)[e][cid, pl.ds(r, 8, stride=HPITCH), :] = v

    def batch_thunks(cid):
        def one(j, u, e):
            def run(toks=None):
                lhs = jnp.concatenate(
                    [_bf(_with_tokens(hl[u, kt], toks if kt == 0 else None)) for kt in range(5)], axis=1)
                qb[:, u, 8 * cid + 2 * j + e] = _dot(lhs, _bf(wtile(cid, j, e))).reshape(16, 8, 128)
            return run
        return [one(j, u, e) for e in range(2) for j in range(4) for u in range(4)]

    def wperm_thunks(piece, j):
        m = (piece >> 2) & 1
        wt = wtmp.at[j]

        def load():
            wt[0:DF, :] = wri[piece, :, 128 * j:128 * j + 128].astype(f32)

        def one(g):
            def run():
                if g == 0:
                    t = jnp.concatenate([wt[pl.ds(0, 64, stride=5), :], wt[320:328, :],
                                         jnp.zeros((56, 128), f32)], axis=0)
                else:
                    t = jnp.concatenate([wt[pl.ds(g, 64, stride=5), :],
                                         wt[pl.ds(5 - g, 64, stride=5), :]], axis=0)
                y = t.T
                sub = wf.at[3 * m + g, pl.ds(pl.multiple_of((piece & 3) * 32, 32), 16 * WPITCH - 96)]
                for k in range(8):
                    for hf in range(2):
                        sub[pl.ds(8 * j + k + 8 * hf * WPITCH, 8, stride=WPITCH), :] = (
                            y[16 * k + 8 * hf:16 * k + 8 * hf + 8])
            return run
        return [load] + [one(g) for g in range(3)]

    def half_pass(cid, half, fill, zero, timed=(), at=()):
        timed = list(timed)
        nre = CFG["pro_nre"]
        toks = None
        for k, f in enumerate(batch_thunks(cid)[16 * half:16 * half + 16]):
            f(toks)
            toks = {}
            if k in at and timed:
                toks[0] = timed.pop(0)()
            if fill is not None:
                for n, r in enumerate(r for r in range(40) if r * nre // 40 == k):
                    relayout(r, fill, 1 - half)
                    toks[CFG["re_pos"][n]] = (wb, wa)[half][12 + zero, 0:8, :]

    def ln_parts(bb, zero):
        def part(j):
            set_input(bb, load_x(bb, 4 * j, 4), None, 4 * j)
            return pltpu.bitcast(xa[32 + zero, 0:8, 0:128], u32)
        return [functools.partial(part, j) for j in range(4)]

    def perm_parts(piece, zero):
        def part(fs):
            for f in fs:
                f()
            return pltpu.bitcast(wf[5 + zero, 16 * WPITCH:16 * WPITCH + 8, :], u32)
        out = []
        for j in range(4):
            th = wperm_thunks(piece, j)
            out += [functools.partial(part, th[0:2]), functools.partial(part, th[2:3]),
                    functools.partial(part, th[3:4])]
        return out

    def pro0():
        for u in range(4):
            cp_x(4 * u + 3).wait()
        for u in range(4):
            set_input(4 * u + 3, load_x(4 * u + 3), u)
        cp_w(0).wait()
        zero = zero_ref[0]
        for i in range(40):
            relayout(i, 0, 0)
        half_pass(0, 0, zero, zero)

    def pro1(it, carry):
        bb = body_chunk(it)
        with jax.named_scope("pro1_wait"):
            cp_w(it + 1).wait()

            @pl.when(it >= 3)
            def _():
                cp_f(it - 3).wait()
            cp_x(bb).wait()
        piece = jnp.where(it >= 3, it - 3, 8)
        zero = it >> 4
        half_pass(it, 1, it + 1, zero, ln_parts(bb, zero) if 'l' not in CFG.get('skip', '') else (), CFG["ln_at"])
        half_pass(it + 1, 0, it + 1, zero, perm_parts(piece, zero) if 'w' not in CFG.get('skip', '') else (), CFG["perm_at"])
        return carry

    def pro2():
        cp_x(body_chunk(11)).wait()
        for cp in cp_rest:
            cp.wait()
        zero = zero_ref[0]
        half_pass(11, 1, None, zero, ln_parts(body_chunk(11), zero), CFG["ln_at2"])

    if full:
        with jax.named_scope("pro0"):
            pro0()
        _loop("pro1", 0, 11, pro1, 0)
        with jax.named_scope("pro2"):
            pro2()

    scale = DH ** -0.5

    def wo_dot(hh, oo):
        return [_dot(oo, wo_t[j, 128 * hh:128 * hh + 128, :]) for j in range(5)]

    def addl(acc, res):
        return res if acc is None else [a + b for a, b in zip(acc, res)]

    def finish_thunks(gp, slot):
        st = {"acc": None}

        def f_wo(hh):
            def run():
                st["acc"] = addl(st["acc"], wo_dot(hh, ol[slot, hh].astype(bf16)))
                if hh == H - 1:
                    out = jnp.concatenate(st["acc"], axis=1)
                    for u in range(4):
                        ao[slot, 32 * u + 24:32 * u + 32, :] = out[8 * u:8 * u + 8]
            return run

        def pre(rows):
            x = _round_bf16(xa[gp, rows, :] + ao[slot, rows, :])
            xb[gp, rows, :] = x
            y = _layernorm(x)
            x0, x1, x2, x3, x4 = [y[:, 128 * a:128 * a + 128] for a in range(5)]
            t1, t2, t3, t4 = x1 + x4, x2 + x3, x1 - x4, x2 - x3
            t = t1 + t2
            m, n = x0 - 0.25 * t, R5_D * (t1 - t2)
            xb[16, rows, :] = jnp.concatenate(
                [x0 + t, m + n, t3 + R5_R * t4, m - n, R5_R * t3 - t4], axis=1)

        def f_dft(cidx):
            def run(chunks=tuple(range(16))):
                g = cidx % 3
                o = FW_OFF + 128 * cidx
                lo, hi = (0, 128) if g == 0 else (256 * g - 128, 256 * g + 128)
                u = jnp.concatenate([xb[16, chunk(bb), lo:hi] for bb in chunks], axis=0)
                y = _dot(u.astype(bf16), _bf(small[o:o + (hi - lo) // 2, :]))
                for i, bb in enumerate(chunks):
                    zs[g][cidx // 3, gp, chunk(bb), :] = y[8 * i:8 * i + 8]
            return run
        return [f_wo(hh) for hh in range(H)], pre, [f_dft(cidx) for cidx in (0, 3, 1, 4, 2, 5)]

    def group(g, mem):
        cur = g & 1
        wos, pre, dfts = finish_thunks(jnp.maximum(g - 1, 0), 1 - cur)
        fillers = [wos[0:11], wos[11:22], wos[22:32], dfts]
        for ph in range(4):
            h = jnp.concatenate([mem, xa[16 + g, 32 * ph:32 * ph + 24, :]], axis=0).astype(bf16)
            pres = list(CFG["pre_rows"][ph])
            pre_at = CFG["pre_at"][ph]
            tok = None
            pr, sm, oos = {}, {}, {}

            def stacked(p, m):
                tails = [qb[g, ph, 32 * m + 2 * p + e] for e in range(2)]
                return jnp.concatenate([pr[p, m, 0], pr[p, m, 1]] + tails, axis=0).astype(bf16)

            def scores(p):
                sc = lax.dot_general(stacked(p, 0), stacked(p, 1), (((1,), (1,)), ((), ())),
                                     preferred_element_type=f32)
                fill = fill_ref[...]
                sc = jnp.where(fill == 0.0, sc * scale, fill)
                mx = jnp.max(sc, axis=-1, keepdims=True)
                e = jnp.exp(sc - mx)
                rl = pl.reciprocal(jnp.sum(e, axis=-1, keepdims=True), approx=True)
                sm[p] = ((e * rl).astype(bf16), None) if CFG["prenorm"] else (e.astype(bf16), rl)

            def pv(p):
                e, rl = sm[p]
                o = _dot(e, stacked(p, 2))
                if rl is not None:
                    o = o * rl
                ol[cur, 2 * p, 8 * ph:8 * ph + 8, :] = o[64:72]
                ol[cur, 2 * p + 1, 8 * ph:8 * ph + 8, :] = o[72:80]
                oos[2 * p], oos[2 * p + 1] = o[0:32].astype(bf16), o[32:64].astype(bf16)

            acc, t, nwo = None, 0.0, 0
            keyed = []
            for p in range(NPAIR):
                keyed += [(4 * p + 2 * i + e, (p, m, e)) for i, m in enumerate(CFG["first"]) for e in range(2)]
                keyed += [(4 * p + 3.5 + CFG["v_delay"] + CFG["v_gap"] * e, (p, 2, e)) for e in range(2)]
            bulk = [x for _, x in sorted(keyed, key=lambda kv: kv[0])]
            pend, ready, fl = [], [], list(fillers[ph])
            n_after = CFG["n_after"][ph]
            while nwo < H:
                pend.sort()
                if pend and pend[0][0] <= t:
                    _, kind, p = pend.pop(0)
                    if kind == "S":
                        scores(p)
                        pend.append((t + CFG["lat_pv"], "V", p))
                    else:
                        pv(p)
                        ready += [(t + CFG["lat_wo"], 2 * p + e) for e in range(2)]
                    t += 0.5
                elif bulk:
                    p, m, e = bulk.pop(0)
                    pr[p, m, e] = _dot(h, _bf(_with_tokens(wtile(4 * m + (p >> 2), p & 3, e), tok)))
                    tok = None
                    if 96 - len(bulk) in pre_at:
                        pre(chunk(pres.pop(0)))
                        tok = {0: pltpu.bitcast(xb[17 + (g >> 4), 0:8, 0:128], u32)}
                    t += 1
                    if m == CFG["first"][1] and e == 1:
                        pend.append((t + CFG["lat_s"], "S", p))
                elif nwo >= CFG["fill_at"] and len(fl) > n_after:
                    fl.pop(0)()
                    t += 1
                elif ready and ready[0][0] <= t:
                    _, hh = ready.pop(0)
                    acc = addl(acc, wo_dot(hh, oos[hh]))
                    t += 1
                    nwo += 1
                elif len(fl) > n_after:
                    fl.pop(0)()
                    t += 1
                else:
                    t += 0.5
            out = jnp.concatenate(acc, axis=1)
            ao[cur, 32 * ph:32 * ph + 24, :] = out[8:32]
            mem = _round_bf16(out[0:8])
            for f in fl:
                f()
        return mem

    def spectral(zero):
        def fence(z):
            return z[0, zero, 128:ZPITCH, :]

        def radix_fwd(g, bb, tok=None, sign=-1):
            z = zs[g]
            xs = [(z[0, a, chunk(bb), :], z[1, a, chunk(bb), :]) for a in range(16)]
            if tok is not None:
                xs[:4] = [(xr + tok, xi) for xr, xi in xs[:4]]
            toks = []

            def emit(q, y):
                for p in range(4):
                    z[0, q + 4 * p, chunk(bb), :] = y[p][0]
                    z[1, q + 4 * p, chunk(bb), :] = y[p][1]
                if g > 0 or sign > 0 or q == 3:
                    toks.append(fence(z))
            _fft16(xs, sign, emit)
            return toks

        ys = {}

        def fwd(g, k2, toks):
            z = zs[g]
            ur, ui = z[0, k2, 0:64, :], z[1, k2, 0:64, :]
            tr, ti = _twiddle((z[0, k2, 64:128, :], z[1, k2, 64:128, :]), k2, 32, -1)
            for hf in range(2):
                v = _ilv(ur + tr, ui + ti) if hf == 0 else _ilv(ur - tr, ui - ti)
                lhs = _with_tokens(emat[k2 + 16 * hf], toks if hf == 0 else None)
                xr, xi = _dilv(_dot(_bf(lhs), v.astype(bf16)))
                ys["x", 16 * g + k2] = xr
                wr = wf[g, pl.ds(k2 * WPITCH + hf, 64, stride=2), :]
                wi = wf[g + 3, pl.ds(k2 * WPITCH + hf, 64, stride=2), :]
                ys[g, k2, hf] = _ilv(xr * wr - xi * wi, xr * wi + xi * wr).astype(bf16)

        def inv(g, k2):
            z = zs[g]
            t0 = _dot(_bf(emat[32 + k2]), ys.pop((g, k2, 0)))
            t1 = _dot(_bf(emat[48 + k2]), ys.pop((g, k2, 1)))
            z[0, k2, 0:64, :], z[1, k2, 0:64, :] = _dilv(t0 + t1)
            z[0, k2, 64:128, :], z[1, k2, 64:128, :] = _twiddle(_dilv(t0 - t1), k2, 32, 1)

        chain = {}
        for bb in range(16):
            chain[bb] = radix_fwd(0, bb, chain.get(bb - 2))[-1]
        radix_fwd(1, 0)
        units = [(g, k2) for g in range(3) for k2 in range(16)]
        toks = None
        for i in range(len(units) + 3):
            if i < len(units):
                fwd(*units[i], toks)
            if i >= 3:
                inv(*units[i - 3])
            toks = None
            if i < 47:
                if i < 31:
                    t4 = radix_fwd(1 + (i + 1) // 16, (i + 1) % 16)
                else:
                    back, r = CFG["rel"]
                    z0[1, zero, 128:ZPITCH, :] = ys["x", i - back][8 * r:8 * r + 8]
                    t4 = radix_fwd(0, i - 31, sign=1)
                toks = {3 + j: pltpu.bitcast(t, u32) for j, t in enumerate(t4)}

    def dinv_thunks(bb, finish):
        st = {}

        def part(g):
            def run():
                z = zs[g]
                ys = [(z[0, a, chunk(bb), :], z[1, a, chunk(bb), :]) for a in range(16)]
                if g > 0:
                    ys = _fft16(ys, 1)
                lhs = jnp.concatenate(
                    [jnp.concatenate([y[0] for y in ys], axis=0),
                     jnp.concatenate([y[1] for y in ys], axis=0)], axis=1).astype(bf16)
                for j in ((0,), (1, 2), (3, 4))[g]:
                    st[j] = _dot(lhs, _bf(small[IW_OFF + 128 * j:IW_OFF + 128 * (j + 1), :]))
            return run

        def fin():
            p0, p1, q1, p2, q2 = [st[j] for j in range(5)]
            t = p1 + p2
            m, n = p0 - 0.25 * t, R5_D * (p1 - p2)
            e1, e2 = m + n, m - n
            o1, o2 = q1 + R5_R * q2, R5_R * q1 - q2
            y = jnp.concatenate([p0 + t, e1 - o1, e2 - o2, e2 + o2, e1 + o1], axis=1)
            finish(xb[0:16, chunk(bb), :].reshape(128, DM) + y)
        return [part(0), part(1), part(2), fin]

    def out_copy(bb):
        return pltpu.make_async_copy(xin.at[:, bb], out_hbm.at[:, bb], osem.at[bb])

    def layer(li, carry0):
        if full or CFG["only"] == "group":
            _loop("step", 0, 16, group, mem_ref[...].astype(f32))
        if full or CFG["only"] == "spec":
            @pl.when((li >> 1) == 0)
            def _():
                with jax.named_scope("tail"):
                    wos, pre, dfts = finish_thunks(15, 1)
                    body = [bb for bb in range(16) if bb % 4 != 3]
                    for bb in body:
                        pre(chunk(bb))
                    for f in wos:
                        f()
                    for f in dfts:
                        f(body)
                    for bb in (3, 7, 11, 15):
                        pre(chunk(bb))
                    for f in dfts:
                        f((3, 7, 11, 15))
            with jax.named_scope("spectral"):
                spectral((li >> 1))
        if not full:
            return carry0

        @pl.when(li == 0)
        def _():
            with jax.named_scope("dinv_tails"):
                th = [dinv_thunks(4 * u + 3, functools.partial(
                    lambda u, x: set_input(4 * u + 3, _round_bf16(x), u), u)) for u in range(4)]
                for i in range(5):
                    if i < 4:
                        for f in th[i][:3]:
                            f()
                    if i >= 1:
                        th[i - 1][3]()

            def batch(it, carry):
                bb = body_chunk(it)
                side = dinv_thunks(bb, lambda x: set_input(bb, _round_bf16(x), None))
                for k, f in enumerate(batch_thunks(it)):
                    f()
                    if k in CFG["dinv_at"]:
                        side.pop(0)()
                return carry
            _loop("batch", 0, 12, batch, 0, unroll=CFG["batch_unroll"])

        @pl.when(li == 1)
        def _():
            with jax.named_scope("dinv_out"):
                def store_out(bb, x):
                    xin[:, bb] = x.reshape(16, 8, DM).astype(bf16)
                    out_copy(bb).start()
                th = [dinv_thunks(bb, functools.partial(store_out, bb)) for bb in range(16)]
                for i in range(17):
                    if i < 16:
                        for f in th[i][:3]:
                            f()
                    if i >= 1:
                        th[i - 1][3]()
                for bb in range(16):
                    out_copy(bb).wait()
        return carry0

    if CFG["only"] != "pro":
        lax.fori_loop(0, 2, layer, 0)


@functools.partial(jax.jit, static_argnames=("A_seg_len",))
def pallas_interleave_layers__memory_aug_recurrent_mem_tr__spectral_gfnet__prompt_kernel(
    A_x, A_mem0, A_Wq, A_Wk, A_Wv, A_Wo, A_seg_len, B_x, B_w_r, B_w_i,
):
    assert A_seg_len == SEG and A_x.shape == (1, S, DM)
    small, emat = _tables()
    hbm = pl.BlockSpec(memory_space=pltpu.HBM)
    out = pl.pallas_call(
        _kernel,
        out_shape=jax.ShapeDtypeStruct((16, 16, 8, DM), bf16),
        in_specs=[hbm] * 10,
        out_specs=hbm,
        scratch_shapes=[
            pltpu.VMEM((16, 16, 8, DM), bf16),
            pltpu.VMEM((33, 128, DM), f32),
            pltpu.VMEM((18, 128, DM), f32),
            pltpu.VMEM((2, 128, DM), f32),
            pltpu.VMEM((12, 2, 320, 8, DH), bf16),
            pltpu.VMEM((13, 8 * HPITCH, 128), u32),
            pltpu.VMEM((13, 8 * HPITCH, 128), u32),
            pltpu.VMEM((5, H * DH, 128), bf16),
            pltpu.VMEM((16, 4, 96, 8, 128), f32),
            pltpu.VMEM((4, 5, 64, 128), u32),
            pltpu.VMEM((2, H, 32, 128), f32),
            pltpu.VMEM((2, 16, ZPITCH, 128), f32),
            pltpu.VMEM((2, 16, ZPITCH, 128), f32),
            pltpu.VMEM((2, 16, ZPITCH, 128), f32),
            pltpu.VMEM((6, 16 * WPITCH + 32, 128), f32),
            pltpu.VMEM((9, DF, 512), bf16),
            pltpu.VMEM((4, 328, 128), f32),
            pltpu.VMEM((SMALL_ROWS, 128), u32),
            pltpu.VMEM((64, 64, 128), u32),
            pltpu.VMEM((80, 80), f32),
            pltpu.VMEM((MEM, DM), bf16),
            pltpu.SMEM((1,), jnp.int32),
            pltpu.SemaphoreType.DMA((46,)),
            pltpu.SemaphoreType.DMA((16,)),
        ],
        compiler_params=pltpu.CompilerParams(vmem_limit_bytes=120 * 1024 * 1024,
                                             disable_semaphore_checks=True),
    )(
        A_x.reshape(16, 16, 8, DM), A_mem0.reshape(MEM, DM),
        *[w.reshape(2, 320, H, DH) for w in (A_Wq, A_Wk, A_Wv)], A_Wo.reshape(H * DH, DM), B_w_r.T, B_w_i.T,
        jnp.asarray(small), jnp.asarray(emat),
    )
    return out.reshape(1, S, DM)
```

```python
import functools
import math

import jax
import jax.numpy as jnp
import numpy as np
from jax import lax
import jax.experimental.pallas as pl
import jax.experimental.pallas.tpu as pltpu

f32, bf16, u32 = jnp.float32, jnp.bfloat16, jnp.uint32

S, DM, H, DH, MEM, SEG = 2048, 640, 32, 128, 8, 32
NSEG = S // SEG
NPAIR = H // 2
DF = DM // 2 + 1
EPS = 1e-5
WPITCH = 132

HPITCH = 164
ZPITCH = 136

S1 = math.sin(2 * math.pi / 5)
R5_D = (math.cos(2 * math.pi / 5) - math.cos(4 * math.pi / 5)) / 2
R5_R = math.sin(4 * math.pi / 5) / S1


def _to_bf16_bits(a):
    u = np.ascontiguousarray(a, dtype=np.float32).view(np.uint32).astype(np.uint64)
    return ((u + 0x7FFF + ((u >> 16) & 1)) >> 16).astype(np.uint32)


def _pack_rows(a):
    b = _to_bf16_bits(a)
    return b[..., 0::2, :] | (b[..., 1::2, :] << 16)


@functools.lru_cache(maxsize=None)
def _tables():
    b = np.arange(128)
    l0 = np.arange(0, DF, 5)
    l1 = np.concatenate([np.arange(1, 320, 5), np.arange(4, 320, 5)])
    l2 = np.concatenate([np.arange(2, 320, 5), np.arange(3, 320, 5)])
    sg = np.concatenate([np.ones(64), -np.ones(64)])

    def th(l):
        return 2 * np.pi * ((b[:, None] * l[None, :]) % DM) / DM

    fw = np.zeros((6, 256, 128))
    t = th(l0)
    fw[0, :128, :65] = np.cos(t)
    fw[3, :128, :65] = -np.sin(t)
    for g, l in ((1, l1), (2, l2)):
        t = th(l)
        c, s = np.cos(t), np.sin(t)
        fw[g] = np.concatenate([c, -S1 * sg * s], axis=0)
        fw[3 + g] = np.concatenate([-s, -S1 * sg * c], axis=0)
    sc = 1.0 / (S * DM)
    iw = np.zeros((5, 256, 128))
    t = th(l0).T
    cl = np.full((65, 1), 2.0)
    cl[0] = cl[-1] = 1.0
    iw[0, :65] = cl * np.cos(t) * sc
    iw[0, 128:128 + 65] = -cl * np.sin(t) * sc
    for g, l in ((1, l1), (2, l2)):
        t = th(l).T
        c, s = np.cos(t), np.sin(t)
        gg = sg[:, None]
        iw[2 * g - 1] = 2 * sc * np.concatenate([c, -s], axis=0)
        iw[2 * g] = 2 * sc * S1 * np.concatenate([gg * s, gg * c], axis=0)
    n = np.arange(64)
    order = np.concatenate([np.concatenate([np.arange(8) + 8 * j, np.arange(8) + 8 * j + 64])
                            for j in range(8)])
    e = np.zeros((2, 32, 128, 128))
    for k2 in range(32):
        t = 2 * np.pi * (((32 * n[:, None] + k2) * n[None, :]) % S) / S
        er, ei = np.cos(t), -np.sin(t)
        m = np.block([[er, -ei], [ei, er]])[order][:, order]
        e[0, k2], e[1, k2] = m, m.T
    small = np.concatenate(
        [_pack_rows(fw).reshape(-1, 128), _pack_rows(iw).reshape(-1, 128)], axis=0)
    return small, _pack_rows(e).reshape(64, 64, 128)


FW_OFF, IW_OFF = 0, 6 * 128
SMALL_ROWS = 11 * 128


def _loop(name, lo, hi, body, init, **kw):
    with jax.named_scope(name):
        return lax.fori_loop(lo, hi, body, init, **kw)


def _bf(x):
    return pltpu.bitcast(x, bf16)


def _dot(a, b):
    return jnp.dot(a, b, preferred_element_type=f32)


def _round_bf16(x):
    return x.astype(bf16).astype(f32)


def _layernorm(x):
    m = jnp.mean(x, axis=-1, keepdims=True)
    xc = x - m
    v = jnp.mean(xc * xc, axis=-1, keepdims=True)
    return xc * lax.rsqrt(v + EPS)


def _fft4(x, sign):
    (ar, ai), (br, bi), (cr, ci), (dr, di) = x
    t0r, t0i, t1r, t1i = ar + cr, ai + ci, ar - cr, ai - ci
    t2r, t2i, t3r, t3i = br + dr, bi + di, br - dr, bi - di
    y0, y2 = (t0r + t2r, t0i + t2i), (t0r - t2r, t0i - t2i)
    p, q = (t1r + t3i, t1i - t3r), (t1r - t3i, t1i + t3r)
    return [y0, p, y2, q] if sign < 0 else [y0, q, y2, p]


def _twiddle(z, n, period, sign):
    zr, zi = z
    n = n % period
    if n == 0:
        return z
    if 4 * n == period:
        return (-zi, zr) if sign > 0 else (zi, -zr)
    c, s = math.cos(2 * math.pi * n / period), sign * math.sin(2 * math.pi * n / period)
    if (8 * n) % period == 0:
        a, d = zr + zi, zr - zi
        if c * s > 0:
            return (d * c, a * c)
        return (a * c, d * s)
    return (zr * c - zi * s, zr * s + zi * c)


def _ilv(r, i):
    n = r.shape[0] // 8
    return jnp.concatenate([r.reshape(n, 8, 128), i.reshape(n, 8, 128)], axis=1).reshape(16 * n, 128)


def _dilv(x):
    n = x.shape[0] // 16
    x = x.reshape(n, 16, 128)
    return x[:, :8].reshape(8 * n, 128), x[:, 8:].reshape(8 * n, 128)


def _with_tokens(x, toks):
    if not toks:
        return x
    return jnp.concatenate(
        [x[8 * j:8 * j + 8] | toks[j] if j in toks else x[8 * j:8 * j + 8]
         for j in range(x.shape[0] // 8)], axis=0)


def _fft16(x, sign, emit=None):
    cols = [_fft4([x[4 * j + r] for j in range(4)], sign) for r in range(4)]
    out = [None] * 16
    for q in range(4):
        y = _fft4([_twiddle(cols[r][q], r * q, 16, sign) for r in range(4)], sign)
        for p in range(4):
            out[q + 4 * p] = y[p]
        if emit is not None:
            emit(q, y)
    return out


CFG = dict(lat_s=6, lat_pv=15, lat_wo=7, v_delay=8, n_last=8, n_first=8,
           post_js=((0, 1), (2, 3), (4,)),
           post_at=(16, 20, 24, 54, 58, 62, 92, 96, 100, 130, 134, 138),
           inv_at=tuple(21 + (k * 26) // 16 for k in range(16)), inv_groups=1, rel=(1, 4), dinv_at=(8, 9, 10, 11), batch_unroll=2,
           pro_nre=14, re_pos=(2, 5, 7), ln_at=(12, 13, 14, 15), ln_at2=(4, 7, 10, 13),
           perm_at=(3, 4, 5, 6, 7, 8, 9, 10, 11, 12, 13, 14), only=None)


def _interleave(main, side):
    n, k = len(main), 0
    for i, f in enumerate(main):
        f()
        while k < len(side) and (k + 1) * n <= (i + 1) * len(side):
            side[k]()
            k += 1
    for f in side[k:]:
        f()


def _kernel(x_hbm, mem_hbm, wq_hbm, wk_hbm, wv_hbm, wo_hbm, wr_hbm, wi_hbm,
            small_hbm, e_hbm, out_hbm,
            xin, xa, xb, to, raw, wa, wb, wo_t, qb, hl, z0, z1, z2, wf,
            wri, wtmp, small, emat, fill_ref, mem_ref, zero_ref, sem, osem):
    zs = (z0, z1, z2)
    w_hbm = (wq_hbm, wk_hbm, wv_hbm)

    def body_chunk(i):
        return 4 * (i & 3) + (i >> 2)

    def cp_w(i):
        src = w_hbm[i >> 2].at[:, :, pl.ds(8 * (i & 3), 8), :] if isinstance(i, int) else raw.at[i]
        return pltpu.make_async_copy(src, raw.at[i], sem.at[i])

    def cp_x(bb):
        return pltpu.make_async_copy(x_hbm.at[:, bb], xin.at[:, bb], sem.at[12 + bb])

    def cp_f(i):
        src = ((wr_hbm, wi_hbm)[i >> 2].at[:, pl.ds(512 * (i & 3), 512)]
               if isinstance(i, int) else wri.at[i])
        return pltpu.make_async_copy(src, wri.at[i], sem.at[36 + i])

    cp_rest = [pltpu.make_async_copy(wo_hbm.at[:, pl.ds(128 * j, 128)], wo_t.at[j], sem.at[28 + j])
               for j in range(5)]
    cp_rest += [pltpu.make_async_copy(mem_hbm, mem_ref, sem.at[33]),
                pltpu.make_async_copy(small_hbm, small, sem.at[44]),
               pltpu.make_async_copy(e_hbm, emat, sem.at[45])]

    full = CFG["only"] in (None, "pro")
    for u in range(4 if full else 0):
        cp_x(4 * u + 3).start()
    if full:
        cp_w(0).start()
    for i in range(12 if full else 0):
        if i < 11:
            cp_w(i + 1).start()
        cp_x(body_chunk(i)).start()
        if 3 <= i < 11:
            cp_f(i - 3).start()
    for cp in cp_rest if full else ():
        cp.start()

    zero_ref[0] = 0

    r = lax.broadcasted_iota(jnp.int32, (80, 80), 0)
    c = lax.broadcasted_iota(jnp.int32, (80, 80), 1)

    def head(i):
        return jnp.where(i < 64, i // 32, (i - 64) // 8)

    def pos(i):
        return jnp.where(i < 64, i % 32, 32 + (i - 64) % 8)

    ok = (pos(r) < MEM) | (pos(r) >= pos(c))
    fill_ref[...] = jnp.where(head(r) == head(c), jnp.where(ok, 0.0, -1e9), -jnp.inf).astype(f32)
    wtmp[:, 320:328, :] = jnp.zeros((4, 8, 128), f32)
    xa[32, 0:8, 0:128] = jnp.zeros((8, 128), f32)
    wa[12, 0:8, :] = jnp.zeros((8, 128), u32)
    wb[12, 0:8, :] = jnp.zeros((8, 128), u32)
    wf[5, 16 * WPITCH:16 * WPITCH + 8, :] = jnp.zeros((8, 128), f32)
    for z in zs:
        z[0, 0, 128:ZPITCH, :] = jnp.zeros((8, 128), f32)

    def chunk(bb):
        if isinstance(bb, int):
            return slice(8 * bb, 8 * bb + 8)
        return pl.ds(pl.multiple_of(8 * bb, 8), 8)

    def set_input(bb, x, tail_u, a0=0):
        n = x.shape[0] // 8
        xa[a0:a0 + n, chunk(bb), :] = x.reshape(n, 8, DM)
        y = _layernorm(x)
        if tail_u is None:
            xa[16 + a0:16 + a0 + n, chunk(bb), :] = y.reshape(n, 8, DM)
        else:
            yb = y.astype(bf16)
            for kt in range(5):
                hl[tail_u, kt] = pltpu.bitcast(yb[:, 128 * kt:128 * kt + 128], u32)

    def load_x(bb, a0=0, n=16):
        return xin[a0:a0 + n, bb].astype(f32).reshape(8 * n, DM)

    def wtile(cid, j, e):
        w = (wa, wb)[e]
        return jnp.concatenate([w[cid, (4 * hf + j) * HPITCH:(4 * hf + j) * HPITCH + 160, :]
                                for hf in range(2)], axis=0)

    def relayout(i, cid, e):
        for r in range(4 * i, 4 * i + 4):
            a, b = [pltpu.bitcast(raw[cid, :, d].reshape(16, 128), u32) for d in (2 * r, 2 * r + 1)]
            v = (a & 0xFFFF) | (b << 16) if e == 0 else (a >> 16) | (b & jnp.uint32(0xFFFF0000))
            (wa, wb)[e][cid, pl.ds(r, 8, stride=HPITCH), :] = v

    def batch_thunks(cid):
        def one(j, u, e):
            def run(toks=None):
                lhs = jnp.concatenate(
                    [_bf(_with_tokens(hl[u, kt], toks if kt == 0 else None)) for kt in range(5)], axis=1)
                qb[:, u, 8 * cid + 2 * j + e] = _dot(lhs, _bf(wtile(cid, j, e))).reshape(16, 8, 128)
            return run
        return [one(j, u, e) for e in range(2) for j in range(4) for u in range(4)]

    def wperm_thunks(piece, j):
        m = (piece >> 2) & 1
        wt = wtmp.at[j]

        def load():
            wt[0:DF, :] = wri[piece, :, 128 * j:128 * j + 128].astype(f32)

        def one(g):
            def run():
                if g == 0:
                    t = jnp.concatenate([wt[pl.ds(0, 64, stride=5), :], wt[320:328, :],
                                         jnp.zeros((56, 128), f32)], axis=0)
                else:
                    t = jnp.concatenate([wt[pl.ds(g, 64, stride=5), :],
                                         wt[pl.ds(5 - g, 64, stride=5), :]], axis=0)
                y = t.T
                sub = wf.at[3 * m + g, pl.ds(pl.multiple_of((piece & 3) * 32, 32), 16 * WPITCH - 96)]
                for k in range(8):
                    for hf in range(2):
                        sub[pl.ds(8 * j + k + 8 * hf * WPITCH, 8, stride=WPITCH), :] = (
                            y[16 * k + 8 * hf:16 * k + 8 * hf + 8])
            return run
        return [load] + [one(g) for g in range(3)]

    def half_pass(cid, half, fill, zero, timed=(), at=()):
        timed = list(timed)
        nre = CFG["pro_nre"]
        toks = None
        for k, f in enumerate(batch_thunks(cid)[16 * half:16 * half + 16]):
            f(toks)
            toks = {}
            if k in at and timed:
                toks[0] = timed.pop(0)()
            if fill is not None:
                for n, r in enumerate(r for r in range(40) if r * nre // 40 == k):
                    relayout(r, fill, 1 - half)
                    toks[CFG["re_pos"][n]] = (wb, wa)[half][12 + zero, 0:8, :]

    def ln_parts(bb, zero):
        def part(j):
            set_input(bb, load_x(bb, 4 * j, 4), None, 4 * j)
            return pltpu.bitcast(xa[32 + zero, 0:8, 0:128], u32)
        return [functools.partial(part, j) for j in range(4)]

    def perm_parts(piece, zero):
        def part(fs):
            for f in fs:
                f()
            return pltpu.bitcast(wf[5 + zero, 16 * WPITCH:16 * WPITCH + 8, :], u32)
        out = []
        for j in range(4):
            th = wperm_thunks(piece, j)
            out += [functools.partial(part, th[0:2]), functools.partial(part, th[2:3]),
                    functools.partial(part, th[3:4])]
        return out

    def pro0():
        for u in range(4):
            cp_x(4 * u + 3).wait()
        for u in range(4):
            set_input(4 * u + 3, load_x(4 * u + 3), u)
        cp_w(0).wait()
        zero = zero_ref[0]
        for i in range(40):
            relayout(i, 0, 0)
        half_pass(0, 0, zero, zero)

    def pro1(it, carry):
        bb = body_chunk(it)
        with jax.named_scope("pro1_wait"):
            cp_w(it + 1).wait()

            @pl.when(it >= 3)
            def _():
                cp_f(it - 3).wait()
            cp_x(bb).wait()
        piece = jnp.where(it >= 3, it - 3, 8)
        zero = it >> 4
        half_pass(it, 1, it + 1, zero, ln_parts(bb, zero) if 'l' not in CFG.get('skip', '') else (), CFG["ln_at"])
        half_pass(it + 1, 0, it + 1, zero, perm_parts(piece, zero) if 'w' not in CFG.get('skip', '') else (), CFG["perm_at"])
        return carry

    def pro2():
        cp_x(body_chunk(11)).wait()
        for cp in cp_rest:
            cp.wait()
        zero = zero_ref[0]
        half_pass(11, 1, None, zero, ln_parts(body_chunk(11), zero), CFG["ln_at2"])

    if full:
        with jax.named_scope("pro0"):
            pro0()
        _loop("pro1", 0, 11, pro1, 0)
        with jax.named_scope("pro2"):
            pro2()

    scale = DH ** -0.5

    def wo_dot(hh, oo):
        return [_dot(oo, wo_t[j, 128 * hh:128 * hh + 128, :]) for j in range(5)]

    def addl(acc, res):
        return res if acc is None else [a + b for a, b in zip(acc, res)]

    def group(g, mem):
        for ph in range(4):
            h = jnp.concatenate([mem, xa[16 + g, 32 * ph:32 * ph + 24, :]], axis=0).astype(bf16)
            pr, sm, oos = {}, {}, {}

            def stacked(p, m):
                tails = [qb[g, ph, 32 * m + 2 * p + e] for e in range(2)]
                return jnp.concatenate([pr[p, m, 0], pr[p, m, 1]] + tails, axis=0).astype(bf16)

            def scores(p):
                sc = lax.dot_general(stacked(p, 0), stacked(p, 1), (((1,), (1,)), ((), ())),
                                     preferred_element_type=f32)
                fill = fill_ref[...]
                sc = jnp.where(fill == 0.0, sc * scale, fill)
                mx = jnp.max(sc, axis=-1, keepdims=True)
                e = jnp.exp(sc - mx)
                rl = pl.reciprocal(jnp.sum(e, axis=-1, keepdims=True), approx=True)
                sm[p] = (e * rl).astype(bf16)

            def pv(p):
                o = _dot(sm[p], stacked(p, 2))
                for e in range(2):
                    qb[g, ph, 2 * p + e] = o[64 + 8 * e:72 + 8 * e]
                    oos[2 * p + e] = o[32 * e:32 * e + 32].astype(bf16)

            keyed = []
            for p in range(NPAIR):
                keyed += [(4 * p + 2 * m + e, (p, m, e)) for m in range(2) for e in range(2)]
                keyed += [(4 * p + 3.5 + CFG["v_delay"], (p, 2, e)) for e in range(2)]
            bulk = [x for _, x in sorted(keyed, key=lambda kv: kv[0])]
            acc, t, nwo, pend, ready = None, 0.0, 0, [], []
            n_last = CFG["n_last"] if ph < 3 else 0
            if ph > 0:
                first, bulk = bulk[:CFG["n_first"]], bulk[CFG["n_first"]:]
                for kt in range(5):
                    for p, m, e in first:
                        w = wtile(4 * m + (p >> 2), p & 3, e)[64 * kt:64 * kt + 64]
                        y = _dot(h[:, 128 * kt:128 * kt + 128], _bf(w))
                        pr[p, m, e] = y if kt == 0 else pr[p, m, e] + y
                t = float(len(first))
                pend = [(t + CFG["lat_s"], "S", p) for p, m, e in first if m == 1 and e == 1]
            while nwo < H - n_last or pend:
                pend.sort()
                if pend and pend[0][0] <= t:
                    _, kind, p = pend.pop(0)
                    if kind == "S":
                        scores(p)
                        pend.append((t + CFG["lat_pv"], "V", p))
                    else:
                        pv(p)
                        ready += [(t + CFG["lat_wo"], 2 * p + e) for e in range(2)]
                    t += 0.5
                elif bulk:
                    p, m, e = bulk.pop(0)
                    pr[p, m, e] = _dot(h, _bf(wtile(4 * m + (p >> 2), p & 3, e)))
                    t += 1
                    if m == 1 and e == 1:
                        pend.append((t + CFG["lat_s"], "S", p))
                elif ready and ready[0][0] <= t and nwo < H - n_last:
                    _, hh = ready.pop(0)
                    acc = addl(acc, wo_dot(hh, oos[hh]))
                    t += 1
                    nwo += 1
                else:
                    t += 0.5
            for j in range(5):
                for _, hh in ready:
                    acc[j] = acc[j] + _dot(oos[hh], wo_t[j, 128 * hh:128 * hh + 128, :])
            out = jnp.concatenate(acc, axis=1)
            xa[16 + g, 32 * ph:32 * ph + 24, :] = out[8:32]
            mem = _round_bf16(out[0:8])
        return mem

    def dfwd_thunks(rows, tail_u=None):
        st = {}

        def pre():
            o = xa[16:32, rows, :] if tail_u is None else to[tail_u]
            x = _round_bf16(xa[0:16, rows, :] + o)
            xb[:, rows, :] = x
            y = _layernorm(x.reshape(128, DM))
            x0, x1, x2, x3, x4 = [y[:, 128 * a:128 * a + 128] for a in range(5)]
            t1, t2, t3, t4 = x1 + x4, x2 + x3, x1 - x4, x2 - x3
            t = t1 + t2
            m, n = x0 - 0.25 * t, R5_D * (t1 - t2)
            st["u"] = [(x0 + t).astype(bf16),
                       jnp.concatenate([m + n, t3 + R5_R * t4], axis=1).astype(bf16),
                       jnp.concatenate([m - n, R5_R * t3 - t4], axis=1).astype(bf16)]

        def part(g):
            def run():
                if g == 0:
                    pre()
                k = 64 if g == 0 else 128
                zr, zi = [_dot(st["u"][g], _bf(small[o:o + k, :]))
                          for o in (FW_OFF + 128 * g, FW_OFF + 128 * (g + 3))]
                ys = _fft16([(zr[8 * a:8 * a + 8], zi[8 * a:8 * a + 8]) for a in range(16)], -1)
                for a in range(16):
                    zs[g][0, a, rows, :] = ys[a][0]
                    zs[g][1, a, rows, :] = ys[a][1]
            return run
        return [part(g) for g in range(3)]

    def post(u, carry):
        base = pl.multiple_of(32 * u, 32)
        prev = jnp.maximum(u - 1, 0)
        side = dfwd_thunks(pl.ds(pl.multiple_of(32 * prev, 32) + 24, 8), prev)
        for q in range(3):
            side += dfwd_thunks(pl.ds(base + 8 * q, 8))
        k = 0
        at = list(CFG["post_at"])
        for js in CFG["post_js"]:
            acc = None
            for hh in range(H):
                oo = qb[:, u, hh].reshape(128, 128).astype(bf16)
                acc = addl(acc, [_dot(oo, wo_t[j, 128 * hh:128 * hh + 128, :]) for j in js])
                k += len(js)
                while at and at[0] <= k:
                    at.pop(0)
                    side.pop(0)()
            for j, y in zip(js, acc):
                to[u, :, :, 128 * j:128 * j + 128] = y.reshape(16, 8, 128)
        assert not side
        return carry

    def spectral(zero):
        def fence(z):
            return z[0, zero, 128:ZPITCH, :]

        def radix_inv(g, bb):
            z = zs[g]
            toks = []

            def emit(q, y):
                for p in range(4):
                    z[0, q + 4 * p, chunk(bb), :] = y[p][0]
                    z[1, q + 4 * p, chunk(bb), :] = y[p][1]
                toks.append(fence(z))
            _fft16([(z[0, a, chunk(bb), :], z[1, a, chunk(bb), :]) for a in range(16)], 1, emit)
            return toks

        ys = {}

        def fwd(g, k2, toks):
            z = zs[g]
            ur, ui = z[0, k2, 0:64, :], z[1, k2, 0:64, :]
            tr, ti = _twiddle((z[0, k2, 64:128, :], z[1, k2, 64:128, :]), k2, 32, -1)
            for hf in range(2):
                v = _ilv(ur + tr, ui + ti) if hf == 0 else _ilv(ur - tr, ui - ti)
                lhs = _with_tokens(emat[k2 + 16 * hf], toks if hf == 0 else None)
                xr, xi = _dilv(_dot(_bf(lhs), v.astype(bf16)))
                ys["x", 16 * g + k2] = xr
                wr = wf[g, pl.ds(k2 * WPITCH + hf, 64, stride=2), :]
                wi = wf[g + 3, pl.ds(k2 * WPITCH + hf, 64, stride=2), :]
                ys[g, k2, hf] = _ilv(xr * wr - xi * wi, xr * wi + xi * wr).astype(bf16)

        def inv(g, k2):
            z = zs[g]
            t0 = _dot(_bf(emat[32 + k2]), ys.pop((g, k2, 0)))
            t1 = _dot(_bf(emat[48 + k2]), ys.pop((g, k2, 1)))
            z[0, k2, 0:64, :], z[1, k2, 0:64, :] = _dilv(t0 + t1)
            z[0, k2, 64:128, :], z[1, k2, 64:128, :] = _twiddle(_dilv(t0 - t1), k2, 32, 1)

        units = [(g, k2) for g in range(3) for k2 in range(16)]
        toks = None
        for i in range(len(units) + 3):
            if i < len(units):
                fwd(*units[i], toks)
            if i >= 3:
                inv(*units[i - 3])
            toks = None
            if i in CFG["inv_at"]:
                n = CFG["inv_at"].index(i)
                back, r = CFG["rel"]
                zs[n // 16][1, zero, 128:ZPITCH, :] = ys["x", min(i - back, 47)][8 * r:8 * r + 8]
                toks = {3 + j: pltpu.bitcast(t, u32) for j, t in enumerate(radix_inv(n // 16, n % 16))}

    def dinv_thunks(bb, finish):
        st = {}

        def part(g):
            def run():
                z = zs[g]
                ys = [(z[0, a, chunk(bb), :], z[1, a, chunk(bb), :]) for a in range(16)]
                if g >= CFG["inv_groups"]:
                    ys = _fft16(ys, 1)
                lhs = jnp.concatenate(
                    [jnp.concatenate([y[0] for y in ys], axis=0),
                     jnp.concatenate([y[1] for y in ys], axis=0)], axis=1).astype(bf16)
                for j in ((0,), (1, 2), (3, 4))[g]:
                    st[j] = _dot(lhs, _bf(small[IW_OFF + 128 * j:IW_OFF + 128 * (j + 1), :]))
            return run

        def fin():
            p0, p1, q1, p2, q2 = [st[j] for j in range(5)]
            t = p1 + p2
            m, n = p0 - 0.25 * t, R5_D * (p1 - p2)
            e1, e2 = m + n, m - n
            o1, o2 = q1 + R5_R * q2, R5_R * q1 - q2
            y = jnp.concatenate([p0 + t, e1 - o1, e2 - o2, e2 + o2, e1 + o1], axis=1)
            finish(xb[:, chunk(bb), :].reshape(128, DM) + y)
        return [part(0), part(1), part(2), fin]

    def out_copy(bb):
        return pltpu.make_async_copy(xin.at[:, bb], out_hbm.at[:, bb], osem.at[bb])

    def layer(li, carry0):
        if full or CFG["only"] == "group":
            _loop("step", 0, 16, group, mem_ref[...].astype(f32))
        if full or CFG["only"] == "spec":
            _loop("post", 0, 4, post, 0)

            @pl.when((li >> 1) == 0)
            def _():
                with jax.named_scope("tail"):
                    for f in dfwd_thunks(chunk(15), 3):
                        f()
            with jax.named_scope("spectral"):
                spectral((li >> 1))
        if not full:
            return carry0

        @pl.when(li == 0)
        def _():
            with jax.named_scope("dinv_tails"):
                th = [dinv_thunks(4 * u + 3, functools.partial(
                    lambda u, x: set_input(4 * u + 3, _round_bf16(x), u), u)) for u in range(4)]
                for i in range(5):
                    if i < 4:
                        for f in th[i][:3]:
                            f()
                    if i >= 1:
                        th[i - 1][3]()

            def batch(it, carry):
                bb = body_chunk(it)
                side = dinv_thunks(bb, lambda x: set_input(bb, _round_bf16(x), None))
                for k, f in enumerate(batch_thunks(it)):
                    f()
                    if k in CFG["dinv_at"]:
                        side.pop(0)()
                return carry
            _loop("batch", 0, 12, batch, 0, unroll=CFG["batch_unroll"])

        @pl.when(li == 1)
        def _():
            with jax.named_scope("dinv_out"):
                def store_out(bb, x):
                    xin[:, bb] = x.reshape(16, 8, DM).astype(bf16)
                    out_copy(bb).start()
                th = [dinv_thunks(bb, functools.partial(store_out, bb)) for bb in range(16)]
                for i in range(17):
                    if i < 16:
                        for f in th[i][:3]:
                            f()
                    if i >= 1:
                        th[i - 1][3]()
                for bb in range(16):
                    out_copy(bb).wait()
        return carry0

    if CFG["only"] != "pro":
        lax.fori_loop(0, 2, layer, 0)


@functools.partial(jax.jit, static_argnames=("A_seg_len",))
def pallas_interleave_layers__memory_aug_recurrent_mem_tr__spectral_gfnet__prompt_kernel(
    A_x, A_mem0, A_Wq, A_Wk, A_Wv, A_Wo, A_seg_len, B_x, B_w_r, B_w_i,
):
    assert A_seg_len == SEG and A_x.shape == (1, S, DM)
    small, emat = _tables()
    hbm = pl.BlockSpec(memory_space=pltpu.HBM)
    out = pl.pallas_call(
        _kernel,
        out_shape=jax.ShapeDtypeStruct((16, 16, 8, DM), bf16),
        in_specs=[hbm] * 10,
        out_specs=hbm,
        scratch_shapes=[
            pltpu.VMEM((16, 16, 8, DM), bf16),
            pltpu.VMEM((33, 128, DM), f32),
            pltpu.VMEM((16, 128, DM), f32),
            pltpu.VMEM((4, 16, 8, DM), f32),
            pltpu.VMEM((12, 2, 320, 8, DH), bf16),
            pltpu.VMEM((13, 8 * HPITCH, 128), u32),
            pltpu.VMEM((13, 8 * HPITCH, 128), u32),
            pltpu.VMEM((5, H * DH, 128), bf16),
            pltpu.VMEM((16, 4, 96, 8, 128), f32),
            pltpu.VMEM((4, 5, 64, 128), u32),
            pltpu.VMEM((2, 16, ZPITCH, 128), f32),
            pltpu.VMEM((2, 16, ZPITCH, 128), f32),
            pltpu.VMEM((2, 16, ZPITCH, 128), f32),
            pltpu.VMEM((6, 16 * WPITCH + 32, 128), f32),
            pltpu.VMEM((9, DF, 512), bf16),
            pltpu.VMEM((4, 328, 128), f32),
            pltpu.VMEM((SMALL_ROWS, 128), u32),
            pltpu.VMEM((64, 64, 128), u32),
            pltpu.VMEM((80, 80), f32),
            pltpu.VMEM((MEM, DM), bf16),
            pltpu.SMEM((1,), jnp.int32),
            pltpu.SemaphoreType.DMA((46,)),
            pltpu.SemaphoreType.DMA((16,)),
        ],
        compiler_params=pltpu.CompilerParams(vmem_limit_bytes=120 * 1024 * 1024,
                                             disable_semaphore_checks=True),
    )(
        A_x.reshape(16, 16, 8, DM), A_mem0.reshape(MEM, DM),
        *[w.reshape(2, 320, H, DH) for w in (A_Wq, A_Wk, A_Wv)], A_Wo.reshape(H * DH, DM), B_w_r.T, B_w_i.T,
        jnp.asarray(small), jnp.asarray(emat),
    )
    return out.reshape(1, S, DM)
```

```python
import functools
import math

import jax
import jax.numpy as jnp
import numpy as np
from jax import lax
import jax.experimental.pallas as pl
import jax.experimental.pallas.tpu as pltpu

f32, bf16, u32 = jnp.float32, jnp.bfloat16, jnp.uint32

S, DM, H, DH, MEM, SEG = 2048, 640, 32, 128, 8, 32
NSEG = S // SEG
NPAIR = H // 2
DF = DM // 2 + 1
EPS = 1e-5
WPITCH = 132

HPITCH = 164
ZPITCH = 136

S1 = math.sin(2 * math.pi / 5)
R5_D = (math.cos(2 * math.pi / 5) - math.cos(4 * math.pi / 5)) / 2
R5_R = math.sin(4 * math.pi / 5) / S1


def _to_bf16_bits(a):
    u = np.ascontiguousarray(a, dtype=np.float32).view(np.uint32).astype(np.uint64)
    return ((u + 0x7FFF + ((u >> 16) & 1)) >> 16).astype(np.uint32)


def _pack_rows(a):
    b = _to_bf16_bits(a)
    return b[..., 0::2, :] | (b[..., 1::2, :] << 16)


@functools.lru_cache(maxsize=None)
def _tables():
    b = np.arange(128)
    l0 = np.arange(0, DF, 5)
    l1 = np.concatenate([np.arange(1, 320, 5), np.arange(4, 320, 5)])
    l2 = np.concatenate([np.arange(2, 320, 5), np.arange(3, 320, 5)])
    sg = np.concatenate([np.ones(64), -np.ones(64)])

    def th(l):
        return 2 * np.pi * ((b[:, None] * l[None, :]) % DM) / DM

    fw = np.zeros((6, 256, 128))
    t = th(l0)
    fw[0, :128, :65] = np.cos(t)
    fw[3, :128, :65] = -np.sin(t)
    for g, l in ((1, l1), (2, l2)):
        t = th(l)
        c, s = np.cos(t), np.sin(t)
        fw[g] = np.concatenate([c, -S1 * sg * s], axis=0)
        fw[3 + g] = np.concatenate([-s, -S1 * sg * c], axis=0)
    sc = 1.0 / (S * DM)
    iw = np.zeros((5, 256, 128))
    t = th(l0).T
    cl = np.full((65, 1), 2.0)
    cl[0] = cl[-1] = 1.0
    iw[0, :65] = cl * np.cos(t) * sc
    iw[0, 128:128 + 65] = -cl * np.sin(t) * sc
    for g, l in ((1, l1), (2, l2)):
        t = th(l).T
        c, s = np.cos(t), np.sin(t)
        gg = sg[:, None]
        iw[2 * g - 1] = 2 * sc * np.concatenate([c, -s], axis=0)
        iw[2 * g] = 2 * sc * S1 * np.concatenate([gg * s, gg * c], axis=0)
    n = np.arange(64)
    order = np.concatenate([np.concatenate([np.arange(8) + 8 * j, np.arange(8) + 8 * j + 64])
                            for j in range(8)])
    e = np.zeros((2, 32, 128, 128))
    for k2 in range(32):
        t = 2 * np.pi * (((32 * n[:, None] + k2) * n[None, :]) % S) / S
        er, ei = np.cos(t), -np.sin(t)
        m = np.block([[er, -ei], [ei, er]])[order][:, order]
        e[0, k2], e[1, k2] = m, m.T
    small = np.concatenate(
        [_pack_rows(fw).reshape(-1, 128), _pack_rows(iw).reshape(-1, 128)], axis=0)
    return small, _pack_rows(e).reshape(64, 64, 128)


FW_OFF, IW_OFF = 0, 6 * 128
SMALL_ROWS = 11 * 128


def _loop(name, lo, hi, body, init, **kw):
    with jax.named_scope(name):
        return lax.fori_loop(lo, hi, body, init, **kw)


def _bf(x):
    return pltpu.bitcast(x, bf16)


def _dot(a, b):
    return jnp.dot(a, b, preferred_element_type=f32)


def _round_bf16(x):
    return x.astype(bf16).astype(f32)


def _layernorm(x):
    m = jnp.mean(x, axis=-1, keepdims=True)
    xc = x - m
    v = jnp.mean(xc * xc, axis=-1, keepdims=True)
    return xc * lax.rsqrt(v + EPS)


def _fft4(x, sign):
    (ar, ai), (br, bi), (cr, ci), (dr, di) = x
    t0r, t0i, t1r, t1i = ar + cr, ai + ci, ar - cr, ai - ci
    t2r, t2i, t3r, t3i = br + dr, bi + di, br - dr, bi - di
    y0, y2 = (t0r + t2r, t0i + t2i), (t0r - t2r, t0i - t2i)
    p, q = (t1r + t3i, t1i - t3r), (t1r - t3i, t1i + t3r)
    return [y0, p, y2, q] if sign < 0 else [y0, q, y2, p]


def _twiddle(z, n, period, sign):
    zr, zi = z
    n = n % period
    if n == 0:
        return z
    if 4 * n == period:
        return (-zi, zr) if sign > 0 else (zi, -zr)
    c, s = math.cos(2 * math.pi * n / period), sign * math.sin(2 * math.pi * n / period)
    if (8 * n) % period == 0:
        a, d = zr + zi, zr - zi
        if c * s > 0:
            return (d * c, a * c)
        return (a * c, d * s)
    return (zr * c - zi * s, zr * s + zi * c)


def _ilv(r, i):
    n = r.shape[0] // 8
    return jnp.concatenate([r.reshape(n, 8, 128), i.reshape(n, 8, 128)], axis=1).reshape(16 * n, 128)


def _dilv(x):
    n = x.shape[0] // 16
    x = x.reshape(n, 16, 128)
    return x[:, :8].reshape(8 * n, 128), x[:, 8:].reshape(8 * n, 128)


def _with_tokens(x, toks):
    if not toks:
        return x
    return jnp.concatenate(
        [x[8 * j:8 * j + 8] | toks[j] if j in toks else x[8 * j:8 * j + 8]
         for j in range(x.shape[0] // 8)], axis=0)


def _fft16(x, sign, emit=None):
    cols = [_fft4([x[4 * j + r] for j in range(4)], sign) for r in range(4)]
    out = [None] * 16
    for q in range(4):
        y = _fft4([_twiddle(cols[r][q], r * q, 16, sign) for r in range(4)], sign)
        for p in range(4):
            out[q + 4 * p] = y[p]
        if emit is not None:
            emit(q, y)
    return out


CFG = dict(lat_s=6, lat_pv=15, lat_wo=7, v_delay=8, n_last=8, n_first=8,
           post_js=((0, 1), (2, 3), (4,)),
           post_order=(0, 3, 6, 1, 2, 4, 5, 7, 8, 9, 10, 11), post_at=(40, 80, 120, 140),
           inv_at=tuple(21 + (k * 26) // 16 for k in range(16)), inv_groups=1, rel=(1, 4), dinv_at=(8, 9, 10, 11), batch_unroll=2,
           pro_nre=14, re_pos=(2, 5, 7), ln_at=(12, 13, 14, 15), ln_at2=(4, 7, 10, 13),
           perm_at=(3, 4, 5, 6, 7, 8, 9, 10, 11, 12, 13, 14), only=None)


def _interleave(main, side):
    n, k = len(main), 0
    for i, f in enumerate(main):
        f()
        while k < len(side) and (k + 1) * n <= (i + 1) * len(side):
            side[k]()
            k += 1
    for f in side[k:]:
        f()


def _kernel(x_hbm, mem_hbm, wq_hbm, wk_hbm, wv_hbm, wo_hbm, wr_hbm, wi_hbm,
            small_hbm, e_hbm, out_hbm,
            xin, xa, xb, to, raw, wa, wb, wo_t, qb, hl, z0, z1, z2, wf,
            wri, wtmp, small, emat, fill_ref, mem_ref, zero_ref, sem, osem):
    zs = (z0, z1, z2)
    w_hbm = (wq_hbm, wk_hbm, wv_hbm)

    def body_chunk(i):
        return 4 * (i & 3) + (i >> 2)

    def cp_w(i):
        src = w_hbm[i >> 2].at[:, :, pl.ds(8 * (i & 3), 8), :] if isinstance(i, int) else raw.at[i]
        return pltpu.make_async_copy(src, raw.at[i], sem.at[i])

    def cp_x(bb):
        return pltpu.make_async_copy(x_hbm.at[:, bb], xin.at[:, bb], sem.at[12 + bb])

    def cp_f(i):
        src = ((wr_hbm, wi_hbm)[i >> 2].at[:, pl.ds(512 * (i & 3), 512)]
               if isinstance(i, int) else wri.at[i])
        return pltpu.make_async_copy(src, wri.at[i], sem.at[36 + i])

    cp_rest = [pltpu.make_async_copy(wo_hbm.at[:, pl.ds(128 * j, 128)], wo_t.at[j], sem.at[28 + j])
               for j in range(5)]
    cp_rest += [pltpu.make_async_copy(mem_hbm, mem_ref, sem.at[33]),
                pltpu.make_async_copy(small_hbm, small, sem.at[44]),
               pltpu.make_async_copy(e_hbm, emat, sem.at[45])]

    full = CFG["only"] in (None, "pro")
    for u in range(4 if full else 0):
        cp_x(4 * u + 3).start()
    if full:
        cp_w(0).start()
    for i in range(12 if full else 0):
        if i < 11:
            cp_w(i + 1).start()
        cp_x(body_chunk(i)).start()
        if 3 <= i < 11:
            cp_f(i - 3).start()
    for cp in cp_rest if full else ():
        cp.start()

    zero_ref[0] = 0

    r = lax.broadcasted_iota(jnp.int32, (80, 80), 0)
    c = lax.broadcasted_iota(jnp.int32, (80, 80), 1)

    def head(i):
        return jnp.where(i < 64, i // 32, (i - 64) // 8)

    def pos(i):
        return jnp.where(i < 64, i % 32, 32 + (i - 64) % 8)

    ok = (pos(r) < MEM) | (pos(r) >= pos(c))
    fill_ref[...] = jnp.where(head(r) == head(c), jnp.where(ok, 0.0, -1e9), -jnp.inf).astype(f32)
    wtmp[:, 320:328, :] = jnp.zeros((4, 8, 128), f32)
    xa[32, 0:8, 0:128] = jnp.zeros((8, 128), f32)
    wa[12, 0:8, :] = jnp.zeros((8, 128), u32)
    wb[12, 0:8, :] = jnp.zeros((8, 128), u32)
    wf[5, 16 * WPITCH:16 * WPITCH + 8, :] = jnp.zeros((8, 128), f32)
    for z in zs:
        z[0, 0, 128:ZPITCH, :] = jnp.zeros((8, 128), f32)

    def chunk(bb):
        if isinstance(bb, int):
            return slice(8 * bb, 8 * bb + 8)
        return pl.ds(pl.multiple_of(8 * bb, 8), 8)

    def set_input(bb, x, tail_u, a0=0):
        n = x.shape[0] // 8
        xa[a0:a0 + n, chunk(bb), :] = x.reshape(n, 8, DM)
        y = _layernorm(x)
        if tail_u is None:
            xa[16 + a0:16 + a0 + n, chunk(bb), :] = y.reshape(n, 8, DM)
        else:
            yb = y.astype(bf16)
            for kt in range(5):
                hl[tail_u, kt] = pltpu.bitcast(yb[:, 128 * kt:128 * kt + 128], u32)

    def load_x(bb, a0=0, n=16):
        return xin[a0:a0 + n, bb].astype(f32).reshape(8 * n, DM)

    def wtile(cid, j, e):
        w = (wa, wb)[e]
        return jnp.concatenate([w[cid, (4 * hf + j) * HPITCH:(4 * hf + j) * HPITCH + 160, :]
                                for hf in range(2)], axis=0)

    def relayout(i, cid, e):
        for r in range(4 * i, 4 * i + 4):
            a, b = [pltpu.bitcast(raw[cid, :, d].reshape(16, 128), u32) for d in (2 * r, 2 * r + 1)]
            v = (a & 0xFFFF) | (b << 16) if e == 0 else (a >> 16) | (b & jnp.uint32(0xFFFF0000))
            (wa, wb)[e][cid, pl.ds(r, 8, stride=HPITCH), :] = v

    def batch_thunks(cid):
        def one(j, u, e):
            def run(toks=None):
                lhs = jnp.concatenate(
                    [_bf(_with_tokens(hl[u, kt], toks if kt == 0 else None)) for kt in range(5)], axis=1)
                qb[:, u, 8 * cid + 2 * j + e] = _dot(lhs, _bf(wtile(cid, j, e))).reshape(16, 8, 128)
            return run
        return [one(j, u, e) for e in range(2) for j in range(4) for u in range(4)]

    def wperm_thunks(piece, j):
        m = (piece >> 2) & 1
        wt = wtmp.at[j]

        def load():
            wt[0:DF, :] = wri[piece, :, 128 * j:128 * j + 128].astype(f32)

        def one(g):
            def run():
                if g == 0:
                    t = jnp.concatenate([wt[pl.ds(0, 64, stride=5), :], wt[320:328, :],
                                         jnp.zeros((56, 128), f32)], axis=0)
                else:
                    t = jnp.concatenate([wt[pl.ds(g, 64, stride=5), :],
                                         wt[pl.ds(5 - g, 64, stride=5), :]], axis=0)
                y = t.T
                sub = wf.at[3 * m + g, pl.ds(pl.multiple_of((piece & 3) * 32, 32), 16 * WPITCH - 96)]
                for k in range(8):
                    for hf in range(2):
                        sub[pl.ds(8 * j + k + 8 * hf * WPITCH, 8, stride=WPITCH), :] = (
                            y[16 * k + 8 * hf:16 * k + 8 * hf + 8])
            return run
        return [load] + [one(g) for g in range(3)]

    def half_pass(cid, half, fill, zero, timed=(), at=()):
        timed = list(timed)
        nre = CFG["pro_nre"]
        toks = None
        for k, f in enumerate(batch_thunks(cid)[16 * half:16 * half + 16]):
            f(toks)
            toks = {}
            if k in at and timed:
                toks[0] = timed.pop(0)()
            if fill is not None:
                for n, r in enumerate(r for r in range(40) if r * nre // 40 == k):
                    relayout(r, fill, 1 - half)
                    toks[CFG["re_pos"][n]] = (wb, wa)[half][12 + zero, 0:8, :]

    def ln_parts(bb, zero):
        def part(j):
            set_input(bb, load_x(bb, 4 * j, 4), None, 4 * j)
            return pltpu.bitcast(xa[32 + zero, 0:8, 0:128], u32)
        return [functools.partial(part, j) for j in range(4)]

    def perm_parts(piece, zero):
        def part(fs):
            for f in fs:
                f()
            return pltpu.bitcast(wf[5 + zero, 16 * WPITCH:16 * WPITCH + 8, :], u32)
        out = []
        for j in range(4):
            th = wperm_thunks(piece, j)
            out += [functools.partial(part, th[0:2]), functools.partial(part, th[2:3]),
                    functools.partial(part, th[3:4])]
        return out

    def pro0():
        for u in range(4):
            cp_x(4 * u + 3).wait()
        for u in range(4):
            set_input(4 * u + 3, load_x(4 * u + 3), u)
        cp_w(0).wait()
        zero = zero_ref[0]
        for i in range(40):
            relayout(i, 0, 0)
        half_pass(0, 0, zero, zero)

    def pro1(it, carry):
        bb = body_chunk(it)
        with jax.named_scope("pro1_wait"):
            cp_w(it + 1).wait()

            @pl.when(it >= 3)
            def _():
                cp_f(it - 3).wait()
            cp_x(bb).wait()
        piece = jnp.where(it >= 3, it - 3, 8)
        zero = it >> 4
        half_pass(it, 1, it + 1, zero, ln_parts(bb, zero) if 'l' not in CFG.get('skip', '') else (), CFG["ln_at"])
        half_pass(it + 1, 0, it + 1, zero, perm_parts(piece, zero) if 'w' not in CFG.get('skip', '') else (), CFG["perm_at"])
        return carry

    def pro2():
        cp_x(body_chunk(11)).wait()
        for cp in cp_rest:
            cp.wait()
        zero = zero_ref[0]
        half_pass(11, 1, None, zero, ln_parts(body_chunk(11), zero), CFG["ln_at2"])

    if full:
        with jax.named_scope("pro0"):
            pro0()
        _loop("pro1", 0, 11, pro1, 0)
        with jax.named_scope("pro2"):
            pro2()

    scale = DH ** -0.5

    def wo_dot(hh, oo):
        return [_dot(oo, wo_t[j, 128 * hh:128 * hh + 128, :]) for j in range(5)]

    def addl(acc, res):
        return res if acc is None else [a + b for a, b in zip(acc, res)]

    def group(g, mem):
        for ph in range(4):
            h = jnp.concatenate([mem, xa[16 + g, 32 * ph:32 * ph + 24, :]], axis=0).astype(bf16)
            pr, sm, oos = {}, {}, {}

            def stacked(p, m):
                tails = [qb[g, ph, 32 * m + 2 * p + e] for e in range(2)]
                return jnp.concatenate([pr[p, m, 0], pr[p, m, 1]] + tails, axis=0).astype(bf16)

            def scores(p):
                sc = lax.dot_general(stacked(p, 0), stacked(p, 1), (((1,), (1,)), ((), ())),
                                     preferred_element_type=f32)
                fill = fill_ref[...]
                sc = jnp.where(fill == 0.0, sc * scale, fill)
                mx = jnp.max(sc, axis=-1, keepdims=True)
                e = jnp.exp(sc - mx)
                rl = pl.reciprocal(jnp.sum(e, axis=-1, keepdims=True), approx=True)
                sm[p] = (e * rl).astype(bf16)

            def pv(p):
                o = _dot(sm[p], stacked(p, 2))
                for e in range(2):
                    qb[g, ph, 2 * p + e] = o[64 + 8 * e:72 + 8 * e]
                    oos[2 * p + e] = o[32 * e:32 * e + 32].astype(bf16)

            keyed = []
            for p in range(NPAIR):
                keyed += [(4 * p + 2 * m + e, (p, m, e)) for m in range(2) for e in range(2)]
                keyed += [(4 * p + 3.5 + CFG["v_delay"], (p, 2, e)) for e in range(2)]
            bulk = [x for _, x in sorted(keyed, key=lambda kv: kv[0])]
            acc, t, nwo, pend, ready = None, 0.0, 0, [], []
            n_last = CFG["n_last"] if ph < 3 else 0
            if ph > 0:
                first, bulk = bulk[:CFG["n_first"]], bulk[CFG["n_first"]:]
                for kt in range(5):
                    for p, m, e in first:
                        w = wtile(4 * m + (p >> 2), p & 3, e)[64 * kt:64 * kt + 64]
                        y = _dot(h[:, 128 * kt:128 * kt + 128], _bf(w))
                        pr[p, m, e] = y if kt == 0 else pr[p, m, e] + y
                t = float(len(first))
                pend = [(t + CFG["lat_s"], "S", p) for p, m, e in first if m == 1 and e == 1]
            while nwo < H - n_last or pend:
                pend.sort()
                if pend and pend[0][0] <= t:
                    _, kind, p = pend.pop(0)
                    if kind == "S":
                        scores(p)
                        pend.append((t + CFG["lat_pv"], "V", p))
                    else:
                        pv(p)
                        ready += [(t + CFG["lat_wo"], 2 * p + e) for e in range(2)]
                    t += 0.5
                elif bulk:
                    p, m, e = bulk.pop(0)
                    pr[p, m, e] = _dot(h, _bf(wtile(4 * m + (p >> 2), p & 3, e)))
                    t += 1
                    if m == 1 and e == 1:
                        pend.append((t + CFG["lat_s"], "S", p))
                elif ready and ready[0][0] <= t and nwo < H - n_last:
                    _, hh = ready.pop(0)
                    acc = addl(acc, wo_dot(hh, oos[hh]))
                    t += 1
                    nwo += 1
                else:
                    t += 0.5
            for j in range(5):
                for _, hh in ready:
                    acc[j] = acc[j] + _dot(oos[hh], wo_t[j, 128 * hh:128 * hh + 128, :])
            out = jnp.concatenate(acc, axis=1)
            xa[16 + g, 32 * ph:32 * ph + 24, :] = out[8:32]
            mem = _round_bf16(out[0:8])
        return mem

    def dfwd_thunks(rows, tail):
        st = {}

        def pre():
            o = to[...] if tail else xa[16:32, rows, :]
            x = _round_bf16(xa[0:16, rows, :] + o)
            xb[:, rows, :] = x
            y = _layernorm(x.reshape(128, DM))
            x0, x1, x2, x3, x4 = [y[:, 128 * a:128 * a + 128] for a in range(5)]
            t1, t2, t3, t4 = x1 + x4, x2 + x3, x1 - x4, x2 - x3
            t = t1 + t2
            m, n = x0 - 0.25 * t, R5_D * (t1 - t2)
            st["u"] = [(x0 + t).astype(bf16),
                       jnp.concatenate([m + n, t3 + R5_R * t4], axis=1).astype(bf16),
                       jnp.concatenate([m - n, R5_R * t3 - t4], axis=1).astype(bf16)]

        def part(g):
            def run():
                if g == 0:
                    pre()
                k = 64 if g == 0 else 128
                zr, zi = [_dot(st["u"][g], _bf(small[o:o + k, :]))
                          for o in (FW_OFF + 128 * g, FW_OFF + 128 * (g + 3))]
                ys = _fft16([(zr[8 * a:8 * a + 8], zi[8 * a:8 * a + 8]) for a in range(16)], -1)
                for a in range(16):
                    zs[g][0, a, rows, :] = ys[a][0]
                    zs[g][1, a, rows, :] = ys[a][1]
            return run
        return [part(g) for g in range(3)]

    def post(u, carry):
        base = pl.multiple_of(32 * u, 32)
        side = []
        for q in range(4):
            side += dfwd_thunks(pl.ds(base + 8 * q, 8), q == 3)
        side = [side[i] for i in CFG["post_order"]]
        k = 0
        at = list(CFG["post_at"])
        for js in CFG["post_js"]:
            acc = None
            for hh in range(H):
                oo = qb[:, u, hh].reshape(128, 128).astype(bf16)
                acc = addl(acc, [_dot(oo, wo_t[j, 128 * hh:128 * hh + 128, :]) for j in js])
                k += len(js)
                while at and at[0] <= k:
                    at.pop(0)
                    side.pop(0)()
            for j, y in zip(js, acc):
                to[:, :, 128 * j:128 * j + 128] = y.reshape(16, 8, 128)
        for f in side:
            f()
        return carry

    def spectral(zero):
        def fence(z):
            return z[0, zero, 128:ZPITCH, :]

        def radix_inv(g, bb):
            z = zs[g]
            toks = []

            def emit(q, y):
                for p in range(4):
                    z[0, q + 4 * p, chunk(bb), :] = y[p][0]
                    z[1, q + 4 * p, chunk(bb), :] = y[p][1]
                toks.append(fence(z))
            _fft16([(z[0, a, chunk(bb), :], z[1, a, chunk(bb), :]) for a in range(16)], 1, emit)
            return toks

        ys = {}

        def fwd(g, k2, toks):
            z = zs[g]
            ur, ui = z[0, k2, 0:64, :], z[1, k2, 0:64, :]
            tr, ti = _twiddle((z[0, k2, 64:128, :], z[1, k2, 64:128, :]), k2, 32, -1)
            for hf in range(2):
                v = _ilv(ur + tr, ui + ti) if hf == 0 else _ilv(ur - tr, ui - ti)
                lhs = _with_tokens(emat[k2 + 16 * hf], toks if hf == 0 else None)
                xr, xi = _dilv(_dot(_bf(lhs), v.astype(bf16)))
                ys["x", 16 * g + k2] = xr
                wr = wf[g, pl.ds(k2 * WPITCH + hf, 64, stride=2), :]
                wi = wf[g + 3, pl.ds(k2 * WPITCH + hf, 64, stride=2), :]
                ys[g, k2, hf] = _ilv(xr * wr - xi * wi, xr * wi + xi * wr).astype(bf16)

        def inv(g, k2):
            z = zs[g]
            t0 = _dot(_bf(emat[32 + k2]), ys.pop((g, k2, 0)))
            t1 = _dot(_bf(emat[48 + k2]), ys.pop((g, k2, 1)))
            z[0, k2, 0:64, :], z[1, k2, 0:64, :] = _dilv(t0 + t1)
            z[0, k2, 64:128, :], z[1, k2, 64:128, :] = _twiddle(_dilv(t0 - t1), k2, 32, 1)

        units = [(g, k2) for g in range(3) for k2 in range(16)]
        toks = None
        for i in range(len(units) + 3):
            if i < len(units):
                fwd(*units[i], toks)
            if i >= 3:
                inv(*units[i - 3])
            toks = None
            if i in CFG["inv_at"]:
                n = CFG["inv_at"].index(i)
                back, r = CFG["rel"]
                zs[n // 16][1, zero, 128:ZPITCH, :] = ys["x", min(i - back, 47)][8 * r:8 * r + 8]
                toks = {3 + j: pltpu.bitcast(t, u32) for j, t in enumerate(radix_inv(n // 16, n % 16))}

    def dinv_thunks(bb, finish):
        st = {}

        def part(g):
            def run():
                z = zs[g]
                ys = [(z[0, a, chunk(bb), :], z[1, a, chunk(bb), :]) for a in range(16)]
                if g >= CFG["inv_groups"]:
                    ys = _fft16(ys, 1)
                lhs = jnp.concatenate(
                    [jnp.concatenate([y[0] for y in ys], axis=0),
                     jnp.concatenate([y[1] for y in ys], axis=0)], axis=1).astype(bf16)
                for j in ((0,), (1, 2), (3, 4))[g]:
                    st[j] = _dot(lhs, _bf(small[IW_OFF + 128 * j:IW_OFF + 128 * (j + 1), :]))
            return run

        def fin():
            p0, p1, q1, p2, q2 = [st[j] for j in range(5)]
            t = p1 + p2
            m, n = p0 - 0.25 * t, R5_D * (p1 - p2)
            e1, e2 = m + n, m - n
            o1, o2 = q1 + R5_R * q2, R5_R * q1 - q2
            y = jnp.concatenate([p0 + t, e1 - o1, e2 - o2, e2 + o2, e1 + o1], axis=1)
            finish(xb[:, chunk(bb), :].reshape(128, DM) + y)
        return [part(0), part(1), part(2), fin]

    def out_copy(bb):
        return pltpu.make_async_copy(xin.at[:, bb], out_hbm.at[:, bb], osem.at[bb])

    def layer(li, carry0):
        if full or CFG["only"] == "group":
            _loop("step", 0, 16, group, mem_ref[...].astype(f32))
        if full or CFG["only"] == "spec":
            _loop("post", 0, 4, post, 0)

            with jax.named_scope("spectral"):
                spectral((li >> 1))
        if not full:
            return carry0

        @pl.when(li == 0)
        def _():
            with jax.named_scope("dinv_tails"):
                th = [dinv_thunks(4 * u + 3, functools.partial(
                    lambda u, x: set_input(4 * u + 3, _round_bf16(x), u), u)) for u in range(4)]
                for i in range(5):
                    if i < 4:
                        for f in th[i][:3]:
                            f()
                    if i >= 1:
                        th[i - 1][3]()

            def batch(it, carry):
                bb = body_chunk(it)
                side = dinv_thunks(bb, lambda x: set_input(bb, _round_bf16(x), None))
                for k, f in enumerate(batch_thunks(it)):
                    f()
                    if k in CFG["dinv_at"]:
                        side.pop(0)()
                return carry
            _loop("batch", 0, 12, batch, 0, unroll=CFG["batch_unroll"])

        @pl.when(li == 1)
        def _():
            with jax.named_scope("dinv_out"):
                def store_out(bb, x):
                    xin[:, bb] = x.reshape(16, 8, DM).astype(bf16)
                    out_copy(bb).start()
                th = [dinv_thunks(bb, functools.partial(store_out, bb)) for bb in range(16)]
                for i in range(17):
                    if i < 16:
                        for f in th[i][:3]:
                            f()
                    if i >= 1:
                        th[i - 1][3]()
                for bb in range(16):
                    out_copy(bb).wait()
        return carry0

    if CFG["only"] != "pro":
        lax.fori_loop(0, 2, layer, 0)


@functools.partial(jax.jit, static_argnames=("A_seg_len",))
def pallas_interleave_layers__memory_aug_recurrent_mem_tr__spectral_gfnet__prompt_kernel(
    A_x, A_mem0, A_Wq, A_Wk, A_Wv, A_Wo, A_seg_len, B_x, B_w_r, B_w_i,
):
    assert A_seg_len == SEG and A_x.shape == (1, S, DM)
    small, emat = _tables()
    hbm = pl.BlockSpec(memory_space=pltpu.HBM)
    out = pl.pallas_call(
        _kernel,
        out_shape=jax.ShapeDtypeStruct((16, 16, 8, DM), bf16),
        in_specs=[hbm] * 10,
        out_specs=hbm,
        scratch_shapes=[
            pltpu.VMEM((16, 16, 8, DM), bf16),
            pltpu.VMEM((33, 128, DM), f32),
            pltpu.VMEM((16, 128, DM), f32),
            pltpu.VMEM((16, 8, DM), f32),
            pltpu.VMEM((12, 2, 320, 8, DH), bf16),
            pltpu.VMEM((13, 8 * HPITCH, 128), u32),
            pltpu.VMEM((13, 8 * HPITCH, 128), u32),
            pltpu.VMEM((5, H * DH, 128), bf16),
            pltpu.VMEM((16, 4, 96, 8, 128), f32),
            pltpu.VMEM((4, 5, 64, 128), u32),
            pltpu.VMEM((2, 16, ZPITCH, 128), f32),
            pltpu.VMEM((2, 16, ZPITCH, 128), f32),
            pltpu.VMEM((2, 16, ZPITCH, 128), f32),
            pltpu.VMEM((6, 16 * WPITCH + 32, 128), f32),
            pltpu.VMEM((9, DF, 512), bf16),
            pltpu.VMEM((4, 328, 128), f32),
            pltpu.VMEM((SMALL_ROWS, 128), u32),
            pltpu.VMEM((64, 64, 128), u32),
            pltpu.VMEM((80, 80), f32),
            pltpu.VMEM((MEM, DM), bf16),
            pltpu.SMEM((1,), jnp.int32),
            pltpu.SemaphoreType.DMA((46,)),
            pltpu.SemaphoreType.DMA((16,)),
        ],
        compiler_params=pltpu.CompilerParams(vmem_limit_bytes=120 * 1024 * 1024,
                                             disable_semaphore_checks=True),
    )(
        A_x.reshape(16, 16, 8, DM), A_mem0.reshape(MEM, DM),
        *[w.reshape(2, 320, H, DH) for w in (A_Wq, A_Wk, A_Wv)], A_Wo.reshape(H * DH, DM), B_w_r.T, B_w_i.T,
        jnp.asarray(small), jnp.asarray(emat),
    )
    return out.reshape(1, S, DM)
```

```python
import functools
import math

import jax
import jax.numpy as jnp
import numpy as np
from jax import lax
import jax.experimental.pallas as pl
import jax.experimental.pallas.tpu as pltpu

f32, bf16, u32 = jnp.float32, jnp.bfloat16, jnp.uint32

S, DM, H, DH, MEM, SEG = 2048, 640, 32, 128, 8, 32
NSEG = S // SEG
NPAIR = H // 2
DF = DM // 2 + 1
EPS = 1e-5
WPITCH = 132

HPITCH = 164
ZPITCH = 136

S1 = math.sin(2 * math.pi / 5)
R5_D = (math.cos(2 * math.pi / 5) - math.cos(4 * math.pi / 5)) / 2
R5_R = math.sin(4 * math.pi / 5) / S1


def _to_bf16_bits(a):
    u = np.ascontiguousarray(a, dtype=np.float32).view(np.uint32).astype(np.uint64)
    return ((u + 0x7FFF + ((u >> 16) & 1)) >> 16).astype(np.uint32)


def _pack_rows(a):
    b = _to_bf16_bits(a)
    return b[..., 0::2, :] | (b[..., 1::2, :] << 16)


@functools.lru_cache(maxsize=None)
def _tables():
    b = np.arange(128)
    l0 = np.arange(0, DF, 5)
    l1 = np.concatenate([np.arange(1, 320, 5), np.arange(4, 320, 5)])
    l2 = np.concatenate([np.arange(2, 320, 5), np.arange(3, 320, 5)])
    sg = np.concatenate([np.ones(64), -np.ones(64)])

    def th(l):
        return 2 * np.pi * ((b[:, None] * l[None, :]) % DM) / DM

    fw = np.zeros((6, 256, 128))
    t = th(l0)
    fw[0, :128, :65] = np.cos(t)
    fw[3, :128, :65] = -np.sin(t)
    for g, l in ((1, l1), (2, l2)):
        t = th(l)
        c, s = np.cos(t), np.sin(t)
        fw[g] = np.concatenate([c, -S1 * sg * s], axis=0)
        fw[3 + g] = np.concatenate([-s, -S1 * sg * c], axis=0)
    sc = 1.0 / (S * DM)
    iw = np.zeros((5, 256, 128))
    t = th(l0).T
    cl = np.full((65, 1), 2.0)
    cl[0] = cl[-1] = 1.0
    iw[0, :65] = cl * np.cos(t) * sc
    iw[0, 128:128 + 65] = -cl * np.sin(t) * sc
    for g, l in ((1, l1), (2, l2)):
        t = th(l).T
        c, s = np.cos(t), np.sin(t)
        gg = sg[:, None]
        iw[2 * g - 1] = 2 * sc * np.concatenate([c, -s], axis=0)
        iw[2 * g] = 2 * sc * S1 * np.concatenate([gg * s, gg * c], axis=0)
    n = np.arange(64)
    order = np.concatenate([np.concatenate([np.arange(8) + 8 * j, np.arange(8) + 8 * j + 64])
                            for j in range(8)])
    e = np.zeros((2, 32, 128, 128))
    for k2 in range(32):
        t = 2 * np.pi * (((32 * n[:, None] + k2) * n[None, :]) % S) / S
        er, ei = np.cos(t), -np.sin(t)
        m = np.block([[er, -ei], [ei, er]])[order][:, order]
        e[0, k2], e[1, k2] = m, m.T
    small = np.concatenate(
        [_pack_rows(fw).reshape(-1, 128), _pack_rows(iw).reshape(-1, 128)], axis=0)
    return small, _pack_rows(e).reshape(64, 64, 128)


FW_OFF, IW_OFF = 0, 6 * 128
SMALL_ROWS = 11 * 128


def _loop(name, lo, hi, body, init, **kw):
    with jax.named_scope(name):
        return lax.fori_loop(lo, hi, body, init, **kw)


def _bf(x):
    return pltpu.bitcast(x, bf16)


def _dot(a, b):
    return jnp.dot(a, b, preferred_element_type=f32)


def _round_bf16(x):
    return x.astype(bf16).astype(f32)


def _layernorm(x):
    m = jnp.mean(x, axis=-1, keepdims=True)
    xc = x - m
    v = jnp.mean(xc * xc, axis=-1, keepdims=True)
    return xc * lax.rsqrt(v + EPS)


def _fft4(x, sign):
    (ar, ai), (br, bi), (cr, ci), (dr, di) = x
    t0r, t0i, t1r, t1i = ar + cr, ai + ci, ar - cr, ai - ci
    t2r, t2i, t3r, t3i = br + dr, bi + di, br - dr, bi - di
    y0, y2 = (t0r + t2r, t0i + t2i), (t0r - t2r, t0i - t2i)
    p, q = (t1r + t3i, t1i - t3r), (t1r - t3i, t1i + t3r)
    return [y0, p, y2, q] if sign < 0 else [y0, q, y2, p]


def _twiddle(z, n, period, sign):
    zr, zi = z
    n = n % period
    if n == 0:
        return z
    if 4 * n == period:
        return (-zi, zr) if sign > 0 else (zi, -zr)
    c, s = math.cos(2 * math.pi * n / period), sign * math.sin(2 * math.pi * n / period)
    if (8 * n) % period == 0:
        a, d = zr + zi, zr - zi
        if c * s > 0:
            return (d * c, a * c)
        return (a * c, d * s)
    return (zr * c - zi * s, zr * s + zi * c)


def _ilv(r, i):
    n = r.shape[0] // 8
    return jnp.concatenate([r.reshape(n, 8, 128), i.reshape(n, 8, 128)], axis=1).reshape(16 * n, 128)


def _dilv(x):
    n = x.shape[0] // 16
    x = x.reshape(n, 16, 128)
    return x[:, :8].reshape(8 * n, 128), x[:, 8:].reshape(8 * n, 128)


def _with_tokens(x, toks):
    if not toks:
        return x
    return jnp.concatenate(
        [x[8 * j:8 * j + 8] | toks[j] if j in toks else x[8 * j:8 * j + 8]
         for j in range(x.shape[0] // 8)], axis=0)


def _fft16(x, sign, emit=None):
    cols = [_fft4([x[4 * j + r] for j in range(4)], sign) for r in range(4)]
    out = [None] * 16
    for q in range(4):
        y = _fft4([_twiddle(cols[r][q], r * q, 16, sign) for r in range(4)], sign)
        for p in range(4):
            out[q + 4 * p] = y[p]
        if emit is not None:
            emit(q, y)
    return out


CFG = dict(steps=((4.5, 16.5, 6, 4, 0, 8), (5, 16.5, 5, 7, 8, 12), (5, 16.5, 6, 6, 8, 12), (5, 16.5, 8, 7, 8, 0)),
           post_js=((0, 1), (2, 3), (4,)),
           post_order=(0, 3, 6, 1, 2, 4, 5, 7, 8, 9, 10, 11), post_at=(40, 80, 120, 140),
           inv_at=tuple(21 + (k * 26) // 16 for k in range(16)), inv_groups=1, rel=(1, 4), dinv_at=(8, 9, 10, 11), batch_unroll=2, post_unroll=1,
           pro_nre=14, re_pos=(2, 5, 7), ln_at=(12, 13, 14, 15), ln_at2=(4, 7, 10, 13),
           perm_at=(3, 4, 5, 6, 7, 8, 9, 10, 11, 12, 13, 14), only=None)


def _interleave(main, side):
    n, k = len(main), 0
    for i, f in enumerate(main):
        f()
        while k < len(side) and (k + 1) * n <= (i + 1) * len(side):
            side[k]()
            k += 1
    for f in side[k:]:
        f()


def _kernel(x_hbm, mem_hbm, wq_hbm, wk_hbm, wv_hbm, wo_hbm, wr_hbm, wi_hbm,
            small_hbm, e_hbm, out_hbm,
            xin, xa, xb, to, raw, wa, wb, wo_t, qb, hl, z0, z1, z2, wf,
            wri, wtmp, small, emat, fill_ref, mem_ref, zero_ref, sem, osem):
    zs = (z0, z1, z2)
    w_hbm = (wq_hbm, wk_hbm, wv_hbm)

    def body_chunk(i):
        return 4 * (i & 3) + (i >> 2)

    def cp_w(i):
        src = w_hbm[i >> 2].at[:, :, pl.ds(8 * (i & 3), 8), :] if isinstance(i, int) else raw.at[i]
        return pltpu.make_async_copy(src, raw.at[i], sem.at[i])

    def cp_x(bb):
        return pltpu.make_async_copy(x_hbm.at[:, bb], xin.at[:, bb], sem.at[12 + bb])

    def cp_f(i):
        src = ((wr_hbm, wi_hbm)[i >> 2].at[:, pl.ds(512 * (i & 3), 512)]
               if isinstance(i, int) else wri.at[i])
        return pltpu.make_async_copy(src, wri.at[i], sem.at[36 + i])

    cp_rest = [pltpu.make_async_copy(wo_hbm.at[:, pl.ds(128 * j, 128)], wo_t.at[j], sem.at[28 + j])
               for j in range(5)]
    cp_rest += [pltpu.make_async_copy(mem_hbm, mem_ref, sem.at[33]),
                pltpu.make_async_copy(small_hbm, small, sem.at[44]),
               pltpu.make_async_copy(e_hbm, emat, sem.at[45])]

    full = CFG["only"] in (None, "pro")
    for u in range(4 if full else 0):
        cp_x(4 * u + 3).start()
    if full:
        cp_w(0).start()
    for i in range(12 if full else 0):
        if i < 11:
            cp_w(i + 1).start()
        cp_x(body_chunk(i)).start()
        if 3 <= i < 11:
            cp_f(i - 3).start()
    for cp in cp_rest if full else ():
        cp.start()

    zero_ref[0] = 0

    r = lax.broadcasted_iota(jnp.int32, (80, 80), 0)
    c = lax.broadcasted_iota(jnp.int32, (80, 80), 1)

    def head(i):
        return jnp.where(i < 64, i // 32, (i - 64) // 8)

    def pos(i):
        return jnp.where(i < 64, i % 32, 32 + (i - 64) % 8)

    ok = (pos(r) < MEM) | (pos(r) >= pos(c))
    fill_ref[...] = jnp.where(head(r) == head(c), jnp.where(ok, 0.0, -1e9), -jnp.inf).astype(f32)
    wtmp[:, 320:328, :] = jnp.zeros((4, 8, 128), f32)
    xa[32, 0:8, 0:128] = jnp.zeros((8, 128), f32)
    wa[12, 0:8, :] = jnp.zeros((8, 128), u32)
    wb[12, 0:8, :] = jnp.zeros((8, 128), u32)
    wf[5, 16 * WPITCH:16 * WPITCH + 8, :] = jnp.zeros((8, 128), f32)
    for z in zs:
        z[0, 0, 128:ZPITCH, :] = jnp.zeros((8, 128), f32)

    def chunk(bb):
        if isinstance(bb, int):
            return slice(8 * bb, 8 * bb + 8)
        return pl.ds(pl.multiple_of(8 * bb, 8), 8)

    def set_input(bb, x, tail_u, a0=0):
        n = x.shape[0] // 8
        xa[a0:a0 + n, chunk(bb), :] = x.reshape(n, 8, DM)
        y = _layernorm(x)
        if tail_u is None:
            xa[16 + a0:16 + a0 + n, chunk(bb), :] = y.reshape(n, 8, DM)
        else:
            yb = y.astype(bf16)
            for kt in range(5):
                hl[tail_u, kt] = pltpu.bitcast(yb[:, 128 * kt:128 * kt + 128], u32)

    def load_x(bb, a0=0, n=16):
        return xin[a0:a0 + n, bb].astype(f32).reshape(8 * n, DM)

    def wtile(cid, j, e):
        w = (wa, wb)[e]
        return jnp.concatenate([w[cid, (4 * hf + j) * HPITCH:(4 * hf + j) * HPITCH + 160, :]
                                for hf in range(2)], axis=0)

    def relayout(i, cid, e):
        for r in range(4 * i, 4 * i + 4):
            a, b = [pltpu.bitcast(raw[cid, :, d].reshape(16, 128), u32) for d in (2 * r, 2 * r + 1)]
            v = (a & 0xFFFF) | (b << 16) if e == 0 else (a >> 16) | (b & jnp.uint32(0xFFFF0000))
            (wa, wb)[e][cid, pl.ds(r, 8, stride=HPITCH), :] = v

    def batch_thunks(cid):
        def one(j, u, e):
            def run(toks=None):
                lhs = jnp.concatenate(
                    [_bf(_with_tokens(hl[u, kt], toks if kt == 0 else None)) for kt in range(5)], axis=1)
                qb[:, u, 8 * cid + 2 * j + e] = _dot(lhs, _bf(wtile(cid, j, e))).reshape(16, 8, 128)
            return run
        return [one(j, u, e) for e in range(2) for j in range(4) for u in range(4)]

    def wperm_thunks(piece, j):
        m = (piece >> 2) & 1
        wt = wtmp.at[j]

        def load():
            wt[0:DF, :] = wri[piece, :, 128 * j:128 * j + 128].astype(f32)

        def one(g):
            def run():
                if g == 0:
                    t = jnp.concatenate([wt[pl.ds(0, 64, stride=5), :], wt[320:328, :],
                                         jnp.zeros((56, 128), f32)], axis=0)
                else:
                    t = jnp.concatenate([wt[pl.ds(g, 64, stride=5), :],
                                         wt[pl.ds(5 - g, 64, stride=5), :]], axis=0)
                y = t.T
                sub = wf.at[3 * m + g, pl.ds(pl.multiple_of((piece & 3) * 32, 32), 16 * WPITCH - 96)]
                for k in range(8):
                    for hf in range(2):
                        sub[pl.ds(8 * j + k + 8 * hf * WPITCH, 8, stride=WPITCH), :] = (
                            y[16 * k + 8 * hf:16 * k + 8 * hf + 8])
            return run
        return [load] + [one(g) for g in range(3)]

    def half_pass(cid, half, fill, zero, timed=(), at=()):
        timed = list(timed)
        nre = CFG["pro_nre"]
        toks = None
        for k, f in enumerate(batch_thunks(cid)[16 * half:16 * half + 16]):
            f(toks)
            toks = {}
            if k in at and timed:
                toks[0] = timed.pop(0)()
            if fill is not None:
                for n, r in enumerate(r for r in range(40) if r * nre // 40 == k):
                    relayout(r, fill, 1 - half)
                    toks[CFG["re_pos"][n]] = (wb, wa)[half][12 + zero, 0:8, :]

    def ln_parts(bb, zero):
        def part(j):
            set_input(bb, load_x(bb, 4 * j, 4), None, 4 * j)
            return pltpu.bitcast(xa[32 + zero, 0:8, 0:128], u32)
        return [functools.partial(part, j) for j in range(4)]

    def perm_parts(piece, zero):
        def part(fs):
            for f in fs:
                f()
            return pltpu.bitcast(wf[5 + zero, 16 * WPITCH:16 * WPITCH + 8, :], u32)
        out = []
        for j in range(4):
            th = wperm_thunks(piece, j)
            out += [functools.partial(part, th[0:2]), functools.partial(part, th[2:3]),
                    functools.partial(part, th[3:4])]
        return out

    def pro0():
        for u in range(4):
            cp_x(4 * u + 3).wait()
        for u in range(4):
            set_input(4 * u + 3, load_x(4 * u + 3), u)
        cp_w(0).wait()
        zero = zero_ref[0]
        for i in range(40):
            relayout(i, 0, 0)
        half_pass(0, 0, zero, zero)

    def pro1(it, carry):
        bb = body_chunk(it)
        with jax.named_scope("pro1_wait"):
            cp_w(it + 1).wait()

            @pl.when(it >= 3)
            def _():
                cp_f(it - 3).wait()
            cp_x(bb).wait()
        piece = jnp.where(it >= 3, it - 3, 8)
        zero = it >> 4
        half_pass(it, 1, it + 1, zero, ln_parts(bb, zero) if 'l' not in CFG.get('skip', '') else (), CFG["ln_at"])
        half_pass(it + 1, 0, it + 1, zero, perm_parts(piece, zero) if 'w' not in CFG.get('skip', '') else (), CFG["perm_at"])
        return carry

    def pro2():
        cp_x(body_chunk(11)).wait()
        for cp in cp_rest:
            cp.wait()
        zero = zero_ref[0]
        half_pass(11, 1, None, zero, ln_parts(body_chunk(11), zero), CFG["ln_at2"])

    if full:
        with jax.named_scope("pro0"):
            pro0()
        _loop("pro1", 0, 11, pro1, 0)
        with jax.named_scope("pro2"):
            pro2()

    scale = DH ** -0.5

    def wo_dot(hh, oo):
        return [_dot(oo, wo_t[j, 128 * hh:128 * hh + 128, :]) for j in range(5)]

    def addl(acc, res):
        return res if acc is None else [a + b for a, b in zip(acc, res)]

    def group(g, mem):
        for ph in range(4):
            h = jnp.concatenate([mem, xa[16 + g, 32 * ph:32 * ph + 24, :]], axis=0).astype(bf16)
            pr, sm, oos = {}, {}, {}
            lat_s, lat_pv, lat_wo, v_delay, n_first, n_last = CFG["steps"][ph]

            def stacked(p, m):
                tails = [qb[g, ph, 32 * m + 2 * p + e] for e in range(2)]
                return jnp.concatenate([pr[p, m, 0], pr[p, m, 1]] + tails, axis=0).astype(bf16)

            def scores(p):
                sc = lax.dot_general(stacked(p, 0), stacked(p, 1), (((1,), (1,)), ((), ())),
                                     preferred_element_type=f32)
                fill = fill_ref[...]
                sc = jnp.where(fill == 0.0, sc * scale, fill)
                mx = jnp.max(sc, axis=-1, keepdims=True)
                e = jnp.exp(sc - mx)
                rl = pl.reciprocal(jnp.sum(e, axis=-1, keepdims=True), approx=True)
                sm[p] = (e * rl).astype(bf16)

            def pv(p):
                o = _dot(sm[p], stacked(p, 2))
                for e in range(2):
                    qb[g, ph, 2 * p + e] = o[64 + 8 * e:72 + 8 * e]
                    oos[2 * p + e] = o[32 * e:32 * e + 32].astype(bf16)

            keyed = []
            for p in range(NPAIR):
                keyed += [(4 * p + 2 * m + e, (p, m, e)) for m in range(2) for e in range(2)]
                keyed += [(4 * p + 3.5 + v_delay, (p, 2, e)) for e in range(2)]
            bulk = [x for _, x in sorted(keyed, key=lambda kv: kv[0])]
            acc, t, nwo, pend, ready = None, 0.0, 0, [], []
            if n_first:
                first, bulk = bulk[:n_first], bulk[n_first:]
                for kt in range(5):
                    for p, m, e in first:
                        w = wtile(4 * m + (p >> 2), p & 3, e)[64 * kt:64 * kt + 64]
                        y = _dot(h[:, 128 * kt:128 * kt + 128], _bf(w))
                        pr[p, m, e] = y if kt == 0 else pr[p, m, e] + y
                t = float(len(first))
                pend = [(t + lat_s, "S", p) for p, m, e in first if m == 1 and e == 1]
            while nwo < H - n_last or pend:
                pend.sort()
                if pend and pend[0][0] <= t:
                    _, kind, p = pend.pop(0)
                    if kind == "S":
                        scores(p)
                        pend.append((t + lat_pv, "V", p))
                    else:
                        pv(p)
                        ready += [(t + lat_wo, 2 * p + e) for e in range(2)]
                    t += 0.5
                elif bulk:
                    p, m, e = bulk.pop(0)
                    pr[p, m, e] = _dot(h, _bf(wtile(4 * m + (p >> 2), p & 3, e)))
                    t += 1
                    if m == 1 and e == 1:
                        pend.append((t + lat_s, "S", p))
                elif ready and ready[0][0] <= t and nwo < H - n_last:
                    _, hh = ready.pop(0)
                    acc = addl(acc, wo_dot(hh, oos[hh]))
                    t += 1
                    nwo += 1
                else:
                    t += 0.5
            for j in range(5):
                for _, hh in ready:
                    acc[j] = acc[j] + _dot(oos[hh], wo_t[j, 128 * hh:128 * hh + 128, :])
            out = jnp.concatenate(acc, axis=1)
            xa[16 + g, 32 * ph:32 * ph + 24, :] = out[8:32]
            mem = _round_bf16(out[0:8])
        return mem

    def dfwd_thunks(rows, tail):
        st = {}

        def pre():
            o = to[...] if tail else xa[16:32, rows, :]
            x = _round_bf16(xa[0:16, rows, :] + o)
            xb[:, rows, :] = x
            y = _layernorm(x.reshape(128, DM))
            x0, x1, x2, x3, x4 = [y[:, 128 * a:128 * a + 128] for a in range(5)]
            t1, t2, t3, t4 = x1 + x4, x2 + x3, x1 - x4, x2 - x3
            t = t1 + t2
            m, n = x0 - 0.25 * t, R5_D * (t1 - t2)
            st["u"] = [(x0 + t).astype(bf16),
                       jnp.concatenate([m + n, t3 + R5_R * t4], axis=1).astype(bf16),
                       jnp.concatenate([m - n, R5_R * t3 - t4], axis=1).astype(bf16)]

        def part(g):
            def run():
                if g == 0:
                    pre()
                k = 64 if g == 0 else 128
                zr, zi = [_dot(st["u"][g], _bf(small[o:o + k, :]))
                          for o in (FW_OFF + 128 * g, FW_OFF + 128 * (g + 3))]
                ys = _fft16([(zr[8 * a:8 * a + 8], zi[8 * a:8 * a + 8]) for a in range(16)], -1)
                for a in range(16):
                    zs[g][0, a, rows, :] = ys[a][0]
                    zs[g][1, a, rows, :] = ys[a][1]
            return run
        return [part(g) for g in range(3)]

    def post(u, carry):
        base = pl.multiple_of(32 * u, 32)
        side = []
        for q in range(4):
            side += dfwd_thunks(pl.ds(base + 8 * q, 8), q == 3)
        side = [side[i] for i in CFG["post_order"]]
        k = 0
        at = list(CFG["post_at"])
        for js in CFG["post_js"]:
            acc = None
            for hh in range(H):
                oo = qb[:, u, hh].reshape(128, 128).astype(bf16)
                acc = addl(acc, [_dot(oo, wo_t[j, 128 * hh:128 * hh + 128, :]) for j in js])
                k += len(js)
                while at and at[0] <= k:
                    at.pop(0)
                    side.pop(0)()
            for j, y in zip(js, acc):
                to[:, :, 128 * j:128 * j + 128] = y.reshape(16, 8, 128)
        for f in side:
            f()
        return carry

    def spectral(zero):
        def fence(z):
            return z[0, zero, 128:ZPITCH, :]

        def radix_inv(g, bb):
            z = zs[g]
            toks = []

            def emit(q, y):
                for p in range(4):
                    z[0, q + 4 * p, chunk(bb), :] = y[p][0]
                    z[1, q + 4 * p, chunk(bb), :] = y[p][1]
                toks.append(fence(z))
            _fft16([(z[0, a, chunk(bb), :], z[1, a, chunk(bb), :]) for a in range(16)], 1, emit)
            return toks

        ys = {}

        def fwd(g, k2, toks):
            z = zs[g]
            ur, ui = z[0, k2, 0:64, :], z[1, k2, 0:64, :]
            tr, ti = _twiddle((z[0, k2, 64:128, :], z[1, k2, 64:128, :]), k2, 32, -1)
            for hf in range(2):
                v = _ilv(ur + tr, ui + ti) if hf == 0 else _ilv(ur - tr, ui - ti)
                lhs = _with_tokens(emat[k2 + 16 * hf], toks if hf == 0 else None)
                xr, xi = _dilv(_dot(_bf(lhs), v.astype(bf16)))
                ys["x", 16 * g + k2] = xr
                wr = wf[g, pl.ds(k2 * WPITCH + hf, 64, stride=2), :]
                wi = wf[g + 3, pl.ds(k2 * WPITCH + hf, 64, stride=2), :]
                ys[g, k2, hf] = _ilv(xr * wr - xi * wi, xr * wi + xi * wr).astype(bf16)

        def inv(g, k2):
            z = zs[g]
            t0 = _dot(_bf(emat[32 + k2]), ys.pop((g, k2, 0)))
            t1 = _dot(_bf(emat[48 + k2]), ys.pop((g, k2, 1)))
            z[0, k2, 0:64, :], z[1, k2, 0:64, :] = _dilv(t0 + t1)
            z[0, k2, 64:128, :], z[1, k2, 64:128, :] = _twiddle(_dilv(t0 - t1), k2, 32, 1)

        units = [(g, k2) for g in range(3) for k2 in range(16)]
        toks = None
        for i in range(len(units) + 3):
            if i < len(units):
                fwd(*units[i], toks)
            if i >= 3:
                inv(*units[i - 3])
            toks = None
            if i in CFG["inv_at"]:
                n = CFG["inv_at"].index(i)
                back, r = CFG["rel"]
                zs[n // 16][1, zero, 128:ZPITCH, :] = ys["x", min(i - back, 47)][8 * r:8 * r + 8]
                toks = {3 + j: pltpu.bitcast(t, u32) for j, t in enumerate(radix_inv(n // 16, n % 16))}

    def dinv_thunks(bb, finish):
        st = {}

        def part(g):
            def run():
                z = zs[g]
                ys = [(z[0, a, chunk(bb), :], z[1, a, chunk(bb), :]) for a in range(16)]
                if g >= CFG["inv_groups"]:
                    ys = _fft16(ys, 1)
                lhs = jnp.concatenate(
                    [jnp.concatenate([y[0] for y in ys], axis=0),
                     jnp.concatenate([y[1] for y in ys], axis=0)], axis=1).astype(bf16)
                for j in ((0,), (1, 2), (3, 4))[g]:
                    st[j] = _dot(lhs, _bf(small[IW_OFF + 128 * j:IW_OFF + 128 * (j + 1), :]))
            return run

        def fin():
            p0, p1, q1, p2, q2 = [st[j] for j in range(5)]
            t = p1 + p2
            m, n = p0 - 0.25 * t, R5_D * (p1 - p2)
            e1, e2 = m + n, m - n
            o1, o2 = q1 + R5_R * q2, R5_R * q1 - q2
            y = jnp.concatenate([p0 + t, e1 - o1, e2 - o2, e2 + o2, e1 + o1], axis=1)
            finish(xb[:, chunk(bb), :].reshape(128, DM) + y)
        return [part(0), part(1), part(2), fin]

    def out_copy(bb):
        return pltpu.make_async_copy(xin.at[:, bb], out_hbm.at[:, bb], osem.at[bb])

    def layer(li, carry0):
        if full or CFG["only"] == "group":
            _loop("step", 0, 16, group, mem_ref[...].astype(f32))
        if full or CFG["only"] == "spec":
            _loop("post", 0, 4, post, 0, unroll=CFG["post_unroll"])

            with jax.named_scope("spectral"):
                spectral((li >> 1))
        if not full:
            return carry0

        @pl.when(li == 0)
        def _():
            with jax.named_scope("dinv_tails"):
                th = [dinv_thunks(4 * u + 3, functools.partial(
                    lambda u, x: set_input(4 * u + 3, _round_bf16(x), u), u)) for u in range(4)]
                for i in range(5):
                    if i < 4:
                        for f in th[i][:3]:
                            f()
                    if i >= 1:
                        th[i - 1][3]()

            def batch(it, carry):
                bb = body_chunk(it)
                side = dinv_thunks(bb, lambda x: set_input(bb, _round_bf16(x), None))
                for k, f in enumerate(batch_thunks(it)):
                    f()
                    if k in CFG["dinv_at"]:
                        side.pop(0)()
                return carry
            _loop("batch", 0, 12, batch, 0, unroll=CFG["batch_unroll"])

        @pl.when(li == 1)
        def _():
            with jax.named_scope("dinv_out"):
                def store_out(bb, x):
                    xin[:, bb] = x.reshape(16, 8, DM).astype(bf16)
                    out_copy(bb).start()
                th = [dinv_thunks(bb, functools.partial(store_out, bb)) for bb in range(16)]
                for i in range(17):
                    if i < 16:
                        for f in th[i][:3]:
                            f()
                    if i >= 1:
                        th[i - 1][3]()
                for bb in range(16):
                    out_copy(bb).wait()
        return carry0

    if CFG["only"] != "pro":
        lax.fori_loop(0, 2, layer, 0)


@functools.partial(jax.jit, static_argnames=("A_seg_len",))
def pallas_interleave_layers__memory_aug_recurrent_mem_tr__spectral_gfnet__prompt_kernel(
    A_x, A_mem0, A_Wq, A_Wk, A_Wv, A_Wo, A_seg_len, B_x, B_w_r, B_w_i,
):
    assert A_seg_len == SEG and A_x.shape == (1, S, DM)
    small, emat = _tables()
    hbm = pl.BlockSpec(memory_space=pltpu.HBM)
    out = pl.pallas_call(
        _kernel,
        out_shape=jax.ShapeDtypeStruct((16, 16, 8, DM), bf16),
        in_specs=[hbm] * 10,
        out_specs=hbm,
        scratch_shapes=[
            pltpu.VMEM((16, 16, 8, DM), bf16),
            pltpu.VMEM((33, 128, DM), f32),
            pltpu.VMEM((16, 128, DM), f32),
            pltpu.VMEM((16, 8, DM), f32),
            pltpu.VMEM((12, 2, 320, 8, DH), bf16),
            pltpu.VMEM((13, 8 * HPITCH, 128), u32),
            pltpu.VMEM((13, 8 * HPITCH, 128), u32),
            pltpu.VMEM((5, H * DH, 128), bf16),
            pltpu.VMEM((16, 4, 96, 8, 128), f32),
            pltpu.VMEM((4, 5, 64, 128), u32),
            pltpu.VMEM((2, 16, ZPITCH, 128), f32),
            pltpu.VMEM((2, 16, ZPITCH, 128), f32),
            pltpu.VMEM((2, 16, ZPITCH, 128), f32),
            pltpu.VMEM((6, 16 * WPITCH + 32, 128), f32),
            pltpu.VMEM((9, DF, 512), bf16),
            pltpu.VMEM((4, 328, 128), f32),
            pltpu.VMEM((SMALL_ROWS, 128), u32),
            pltpu.VMEM((64, 64, 128), u32),
            pltpu.VMEM((80, 80), f32),
            pltpu.VMEM((MEM, DM), bf16),
            pltpu.SMEM((1,), jnp.int32),
            pltpu.SemaphoreType.DMA((46,)),
            pltpu.SemaphoreType.DMA((16,)),
        ],
        compiler_params=pltpu.CompilerParams(vmem_limit_bytes=120 * 1024 * 1024,
                                             disable_semaphore_checks=True),
    )(
        A_x.reshape(16, 16, 8, DM), A_mem0.reshape(MEM, DM),
        *[w.reshape(2, 320, H, DH) for w in (A_Wq, A_Wk, A_Wv)], A_Wo.reshape(H * DH, DM), B_w_r.T, B_w_i.T,
        jnp.asarray(small), jnp.asarray(emat),
    )
    return out.reshape(1, S, DM)
```

```python
import functools
import math

import jax
import jax.numpy as jnp
import numpy as np
from jax import lax
import jax.experimental.pallas as pl
import jax.experimental.pallas.tpu as pltpu

f32, bf16, u32 = jnp.float32, jnp.bfloat16, jnp.uint32

S, DM, H, DH, MEM, SEG = 2048, 640, 32, 128, 8, 32
NSEG = S // SEG
NPAIR = H // 2
DF = DM // 2 + 1
EPS = 1e-5
WPITCH = 132

HPITCH = 164
ZPITCH = 136

S1 = math.sin(2 * math.pi / 5)
R5_D = (math.cos(2 * math.pi / 5) - math.cos(4 * math.pi / 5)) / 2
R5_R = math.sin(4 * math.pi / 5) / S1


def _to_bf16_bits(a):
    u = np.ascontiguousarray(a, dtype=np.float32).view(np.uint32).astype(np.uint64)
    return ((u + 0x7FFF + ((u >> 16) & 1)) >> 16).astype(np.uint32)


def _pack_rows(a):
    b = _to_bf16_bits(a)
    return b[..., 0::2, :] | (b[..., 1::2, :] << 16)


@functools.lru_cache(maxsize=None)
def _tables():
    b = np.arange(128)
    l0 = np.arange(0, DF, 5)
    l1 = np.concatenate([np.arange(1, 320, 5), np.arange(4, 320, 5)])
    l2 = np.concatenate([np.arange(2, 320, 5), np.arange(3, 320, 5)])
    sg = np.concatenate([np.ones(64), -np.ones(64)])

    def th(l):
        return 2 * np.pi * ((b[:, None] * l[None, :]) % DM) / DM

    fw = np.zeros((6, 256, 128))
    t = th(l0)
    fw[0, :128, :65] = np.cos(t)
    fw[3, :128, :65] = -np.sin(t)
    for g, l in ((1, l1), (2, l2)):
        t = th(l)
        c, s = np.cos(t), np.sin(t)
        fw[g] = np.concatenate([c, -S1 * sg * s], axis=0)
        fw[3 + g] = np.concatenate([-s, -S1 * sg * c], axis=0)
    sc = 1.0 / (S * DM)
    iw = np.zeros((5, 256, 128))
    t = th(l0).T
    cl = np.full((65, 1), 2.0)
    cl[0] = cl[-1] = 1.0
    iw[0, :65] = cl * np.cos(t) * sc
    iw[0, 128:128 + 65] = -cl * np.sin(t) * sc
    for g, l in ((1, l1), (2, l2)):
        t = th(l).T
        c, s = np.cos(t), np.sin(t)
        gg = sg[:, None]
        iw[2 * g - 1] = 2 * sc * np.concatenate([c, -s], axis=0)
        iw[2 * g] = 2 * sc * S1 * np.concatenate([gg * s, gg * c], axis=0)
    n = np.arange(64)
    order = np.concatenate([np.concatenate([np.arange(8) + 8 * j, np.arange(8) + 8 * j + 64])
                            for j in range(8)])
    e = np.zeros((2, 32, 128, 128))
    for k2 in range(32):
        t = 2 * np.pi * (((32 * n[:, None] + k2) * n[None, :]) % S) / S
        er, ei = np.cos(t), -np.sin(t)
        m = np.block([[er, -ei], [ei, er]])[order][:, order]
        e[0, k2], e[1, k2] = m, m.T
    small = np.concatenate(
        [_pack_rows(fw).reshape(-1, 128), _pack_rows(iw).reshape(-1, 128)], axis=0)
    return small, _pack_rows(e).reshape(64, 64, 128)


FW_OFF, IW_OFF = 0, 6 * 128
SMALL_ROWS = 11 * 128


def _loop(name, lo, hi, body, init, **kw):
    with jax.named_scope(name):
        return lax.fori_loop(lo, hi, body, init, **kw)


def _bf(x):
    return pltpu.bitcast(x, bf16)


def _dot(a, b):
    return jnp.dot(a, b, preferred_element_type=f32)


def _round_bf16(x):
    return x.astype(bf16).astype(f32)


def _layernorm(x):
    m = jnp.mean(x, axis=-1, keepdims=True)
    xc = x - m
    v = jnp.mean(xc * xc, axis=-1, keepdims=True)
    return xc * lax.rsqrt(v + EPS)


def _fft4(x, sign):
    (ar, ai), (br, bi), (cr, ci), (dr, di) = x
    t0r, t0i, t1r, t1i = ar + cr, ai + ci, ar - cr, ai - ci
    t2r, t2i, t3r, t3i = br + dr, bi + di, br - dr, bi - di
    y0, y2 = (t0r + t2r, t0i + t2i), (t0r - t2r, t0i - t2i)
    p, q = (t1r + t3i, t1i - t3r), (t1r - t3i, t1i + t3r)
    return [y0, p, y2, q] if sign < 0 else [y0, q, y2, p]


def _twiddle(z, n, period, sign):
    zr, zi = z
    n = n % period
    if n == 0:
        return z
    if 4 * n == period:
        return (-zi, zr) if sign > 0 else (zi, -zr)
    c, s = math.cos(2 * math.pi * n / period), sign * math.sin(2 * math.pi * n / period)
    if (8 * n) % period == 0:
        a, d = zr + zi, zr - zi
        if c * s > 0:
            return (d * c, a * c)
        return (a * c, d * s)
    return (zr * c - zi * s, zr * s + zi * c)


def _ilv(r, i):
    n = r.shape[0] // 8
    return jnp.concatenate([r.reshape(n, 8, 128), i.reshape(n, 8, 128)], axis=1).reshape(16 * n, 128)


def _dilv(x):
    n = x.shape[0] // 16
    x = x.reshape(n, 16, 128)
    return x[:, :8].reshape(8 * n, 128), x[:, 8:].reshape(8 * n, 128)


def _with_tokens(x, toks):
    if not toks:
        return x
    return jnp.concatenate(
        [x[8 * j:8 * j + 8] | toks[j] if j in toks else x[8 * j:8 * j + 8]
         for j in range(x.shape[0] // 8)], axis=0)


def _fft16(x, sign, emit=None):
    cols = [_fft4([x[4 * j + r] for j in range(4)], sign) for r in range(4)]
    out = [None] * 16
    for q in range(4):
        y = _fft4([_twiddle(cols[r][q], r * q, 16, sign) for r in range(4)], sign)
        for p in range(4):
            out[q + 4 * p] = y[p]
        if emit is not None:
            emit(q, y)
    return out


CFG = dict(steps=((4.5, 16.5, 6, 4, 0, 8), (5, 16.5, 5, 7, 8, 12), (5, 16.5, 6, 6, 8, 12), (5, 16.5, 8, 7, 8, 0)),
           post_js=((0, 1, 2), (3, 4)),
           post_order=(3, 0, 6, 1, 2, 4, 5, 7, 9, 8, 10, 11), post_at=(40, 80, 120, 126),
           inv_at=tuple(21 + (k * 26) // 16 for k in range(16)), inv_groups=1, rel=(1, 4), dinv_at=(8, 9, 10, 11), batch_unroll=2, post_unroll=1,
           pro_nre=14, re_pos=(3, 5, 7), ln_at=(22, 29, 31, 31), ln_at2=(4, 7, 10, 13),
           perm_at=tuple(range(12, 24)), only=None)


def _interleave(main, side):
    n, k = len(main), 0
    for i, f in enumerate(main):
        f()
        while k < len(side) and (k + 1) * n <= (i + 1) * len(side):
            side[k]()
            k += 1
    for f in side[k:]:
        f()


def _kernel(x_hbm, mem_hbm, wq_hbm, wk_hbm, wv_hbm, wo_hbm, wr_hbm, wi_hbm,
            small_hbm, e_hbm, out_hbm,
            xin, xa, xb, to, raw, wa, wb, wo_t, qb, hl, z0, z1, z2, wf,
            wri, wtmp, small, emat, fill_ref, mem_ref, zero_ref, sem, osem):
    zs = (z0, z1, z2)
    w_hbm = (wq_hbm, wk_hbm, wv_hbm)

    def body_chunk(i):
        return 4 * (i & 3) + (i >> 2)

    def cp_w(i):
        src = w_hbm[i >> 2].at[:, :, pl.ds(8 * (i & 3), 8), :] if isinstance(i, int) else raw.at[i]
        return pltpu.make_async_copy(src, raw.at[i], sem.at[i])

    def cp_x(bb):
        return pltpu.make_async_copy(x_hbm.at[:, bb], xin.at[:, bb], sem.at[12 + bb])

    def cp_f(i):
        src = ((wr_hbm, wi_hbm)[i >> 2].at[:, pl.ds(512 * (i & 3), 512)]
               if isinstance(i, int) else wri.at[i])
        return pltpu.make_async_copy(src, wri.at[i], sem.at[36 + i])

    cp_rest = [pltpu.make_async_copy(wo_hbm.at[:, pl.ds(128 * j, 128)], wo_t.at[j], sem.at[28 + j])
               for j in range(5)]
    cp_rest += [pltpu.make_async_copy(mem_hbm, mem_ref, sem.at[33]),
                pltpu.make_async_copy(small_hbm, small, sem.at[44]),
               pltpu.make_async_copy(e_hbm, emat, sem.at[45])]

    full = CFG["only"] in (None, "pro")
    for u in range(4 if full else 0):
        cp_x(4 * u + 3).start()
    if full:
        cp_w(0).start()
    for i in range(12 if full else 0):
        if i < 11:
            cp_w(i + 1).start()
        cp_x(body_chunk(i)).start()
        if 3 <= i < 11:
            cp_f(i - 3).start()
    for cp in cp_rest if full else ():
        cp.start()

    zero_ref[0] = 0

    r = lax.broadcasted_iota(jnp.int32, (80, 80), 0)
    c = lax.broadcasted_iota(jnp.int32, (80, 80), 1)

    def head(i):
        return jnp.where(i < 64, i // 32, (i - 64) // 8)

    def pos(i):
        return jnp.where(i < 64, i % 32, 32 + (i - 64) % 8)

    ok = (pos(r) < MEM) | (pos(r) >= pos(c))
    fill_ref[...] = jnp.where(head(r) == head(c), jnp.where(ok, 0.0, -1e9), -jnp.inf).astype(f32)
    wtmp[:, 320:328, :] = jnp.zeros((4, 8, 128), f32)
    xa[32, 0:8, 0:128] = jnp.zeros((8, 128), f32)
    wa[12, 0:8, :] = jnp.zeros((8, 128), u32)
    wb[12, 0:8, :] = jnp.zeros((8, 128), u32)
    wf[5, 16 * WPITCH:16 * WPITCH + 8, :] = jnp.zeros((8, 128), f32)
    for z in zs:
        z[0, 0, 128:ZPITCH, :] = jnp.zeros((8, 128), f32)

    def chunk(bb):
        if isinstance(bb, int):
            return slice(8 * bb, 8 * bb + 8)
        return pl.ds(pl.multiple_of(8 * bb, 8), 8)

    def set_input(bb, x, tail_u, a0=0):
        n = x.shape[0] // 8
        xa[a0:a0 + n, chunk(bb), :] = x.reshape(n, 8, DM)
        y = _layernorm(x)
        if tail_u is None:
            xa[16 + a0:16 + a0 + n, chunk(bb), :] = y.reshape(n, 8, DM)
        else:
            yb = y.astype(bf16)
            for kt in range(5):
                hl[tail_u, kt] = pltpu.bitcast(yb[:, 128 * kt:128 * kt + 128], u32)

    def load_x(bb, a0=0, n=16):
        return xin[a0:a0 + n, bb].astype(f32).reshape(8 * n, DM)

    def wtile(cid, j, e):
        w = (wa, wb)[e]
        return jnp.concatenate([w[cid, (4 * hf + j) * HPITCH:(4 * hf + j) * HPITCH + 160, :]
                                for hf in range(2)], axis=0)

    def relayout(i, cid, e):
        for r in range(4 * i, 4 * i + 4):
            a, b = [pltpu.bitcast(raw[cid, :, d].reshape(16, 128), u32) for d in (2 * r, 2 * r + 1)]
            v = (a & 0xFFFF) | (b << 16) if e == 0 else (a >> 16) | (b & jnp.uint32(0xFFFF0000))
            (wa, wb)[e][cid, pl.ds(r, 8, stride=HPITCH), :] = v

    def batch_thunks(cid):
        def one(j, u, e):
            def run(toks=None):
                lhs = jnp.concatenate(
                    [_bf(_with_tokens(hl[u, kt], toks if kt == 0 else None)) for kt in range(5)], axis=1)
                qb[:, u, 8 * cid + 2 * j + e] = _dot(lhs, _bf(wtile(cid, j, e))).reshape(16, 8, 128)
            return run
        return [one(j, u, e) for e in range(2) for j in range(4) for u in range(4)]

    def wperm_thunks(piece, j):
        m = (piece >> 2) & 1
        wt = wtmp.at[j]

        def load():
            wt[0:DF, :] = wri[piece, :, 128 * j:128 * j + 128].astype(f32)

        def one(g):
            def run():
                if g == 0:
                    t = jnp.concatenate([wt[pl.ds(0, 64, stride=5), :], wt[320:328, :],
                                         jnp.zeros((56, 128), f32)], axis=0)
                else:
                    t = jnp.concatenate([wt[pl.ds(g, 64, stride=5), :],
                                         wt[pl.ds(5 - g, 64, stride=5), :]], axis=0)
                y = t.T
                sub = wf.at[3 * m + g, pl.ds(pl.multiple_of((piece & 3) * 32, 32), 16 * WPITCH - 96)]
                for k in range(8):
                    for hf in range(2):
                        sub[pl.ds(8 * j + k + 8 * hf * WPITCH, 8, stride=WPITCH), :] = (
                            y[16 * k + 8 * hf:16 * k + 8 * hf + 8])
            return run
        return [load] + [one(g) for g in range(3)]

    def half_pass(cid, half, fill, zero, timed=()):
        nre = CFG["pro_nre"]
        toks = None
        for k, f in enumerate(batch_thunks(cid)[16 * half:16 * half + 16]):
            f(toks)
            toks = {}
            for pos, f in zip((0, 4, 1, 6), [f for at, f in timed if at == k]):
                toks[pos] = f()
            if fill is not None:
                for n, r in enumerate(r for r in range(40) if r * nre // 40 == k):
                    relayout(r, fill, 1 - half)
                    toks[CFG["re_pos"][n]] = (wb, wa)[half][12 + zero, 0:8, :]

    def ln_parts(bb, zero):
        def part(j):
            set_input(bb, load_x(bb, 4 * j, 4), None, 4 * j)
            return pltpu.bitcast(xa[32 + zero, 0:8, 0:128], u32)
        return [functools.partial(part, j) for j in range(4)]

    def perm_parts(piece, zero):
        def part(fs):
            for f in fs:
                f()
            return pltpu.bitcast(wf[5 + zero, 16 * WPITCH:16 * WPITCH + 8, :], u32)
        out = []
        for j in range(4):
            th = wperm_thunks(piece, j)
            out += [functools.partial(part, th[0:2]), functools.partial(part, th[2:3]),
                    functools.partial(part, th[3:4])]
        return out

    def pro0():
        for u in range(4):
            cp_x(4 * u + 3).wait()
        for u in range(4):
            set_input(4 * u + 3, load_x(4 * u + 3), u)
        cp_w(0).wait()
        zero = zero_ref[0]
        for i in range(40):
            relayout(i, 0, 0)
        half_pass(0, 0, zero, zero)

    def pro1(it, carry):
        bb = body_chunk(it)
        with jax.named_scope("pro1_wait"):
            cp_w(it + 1).wait()

            @pl.when(it >= 3)
            def _():
                cp_f(it - 3).wait()
            cp_x(bb).wait()
        piece = jnp.where(it >= 3, it - 3, 8)
        zero = it >> 4
        timed = sorted(list(zip(CFG["ln_at"], ln_parts(bb, zero)))
                       + list(zip(CFG["perm_at"], perm_parts(piece, zero))), key=lambda x: x[0])
        half_pass(it, 1, it + 1, zero, [x for x in timed if x[0] < 16])
        half_pass(it + 1, 0, it + 1, zero, [(k - 16, f) for k, f in timed if k >= 16])
        return carry

    def pro2():
        cp_x(body_chunk(11)).wait()
        for cp in cp_rest:
            cp.wait()
        zero = zero_ref[0]
        half_pass(11, 1, None, zero, list(zip(CFG["ln_at2"], ln_parts(body_chunk(11), zero))))

    if full:
        with jax.named_scope("pro0"):
            pro0()
        _loop("pro1", 0, 11, pro1, 0)
        with jax.named_scope("pro2"):
            pro2()

    scale = DH ** -0.5

    def wo_dot(hh, oo):
        return [_dot(oo, wo_t[j, 128 * hh:128 * hh + 128, :]) for j in range(5)]

    def addl(acc, res):
        return res if acc is None else [a + b for a, b in zip(acc, res)]

    def group(g, mem):
        for ph in range(4):
            h = jnp.concatenate([mem, xa[16 + g, 32 * ph:32 * ph + 24, :]], axis=0).astype(bf16)
            pr, sm, oos = {}, {}, {}
            lat_s, lat_pv, lat_wo, v_delay, n_first, n_last = CFG["steps"][ph]

            def stacked(p, m):
                tails = [qb[g, ph, 32 * m + 2 * p + e] for e in range(2)]
                return jnp.concatenate([pr[p, m, 0], pr[p, m, 1]] + tails, axis=0).astype(bf16)

            def scores(p):
                sc = lax.dot_general(stacked(p, 0), stacked(p, 1), (((1,), (1,)), ((), ())),
                                     preferred_element_type=f32)
                fill = fill_ref[...]
                sc = jnp.where(fill == 0.0, sc * scale, fill)
                mx = jnp.max(sc, axis=-1, keepdims=True)
                e = jnp.exp(sc - mx)
                rl = pl.reciprocal(jnp.sum(e, axis=-1, keepdims=True), approx=True)
                sm[p] = (e * rl).astype(bf16)

            def pv(p):
                o = _dot(sm[p], stacked(p, 2))
                for e in range(2):
                    qb[g, ph, 2 * p + e] = o[64 + 8 * e:72 + 8 * e]
                    oos[2 * p + e] = o[32 * e:32 * e + 32].astype(bf16)

            keyed = []
            for p in range(NPAIR):
                keyed += [(4 * p + 2 * m + e, (p, m, e)) for m in range(2) for e in range(2)]
                keyed += [(4 * p + 3.5 + v_delay, (p, 2, e)) for e in range(2)]
            bulk = [x for _, x in sorted(keyed, key=lambda kv: kv[0])]
            acc, t, nwo, pend, ready = None, 0.0, 0, [], []
            if n_first:
                first, bulk = bulk[:n_first], bulk[n_first:]
                for kt in range(5):
                    for p, m, e in first:
                        w = wtile(4 * m + (p >> 2), p & 3, e)[64 * kt:64 * kt + 64]
                        y = _dot(h[:, 128 * kt:128 * kt + 128], _bf(w))
                        pr[p, m, e] = y if kt == 0 else pr[p, m, e] + y
                t = float(len(first))
                pend = [(t + lat_s, "S", p) for p, m, e in first if m == 1 and e == 1]
            while nwo < H - n_last or pend:
                pend.sort()
                if pend and pend[0][0] <= t:
                    _, kind, p = pend.pop(0)
                    if kind == "S":
                        scores(p)
                        pend.append((t + lat_pv, "V", p))
                    else:
                        pv(p)
                        ready += [(t + lat_wo, 2 * p + e) for e in range(2)]
                    t += 0.5
                elif bulk:
                    p, m, e = bulk.pop(0)
                    pr[p, m, e] = _dot(h, _bf(wtile(4 * m + (p >> 2), p & 3, e)))
                    t += 1
                    if m == 1 and e == 1:
                        pend.append((t + lat_s, "S", p))
                elif ready and ready[0][0] <= t and nwo < H - n_last:
                    _, hh = ready.pop(0)
                    acc = addl(acc, wo_dot(hh, oos[hh]))
                    t += 1
                    nwo += 1
                else:
                    t += 0.5
            for j in range(5):
                for _, hh in ready:
                    acc[j] = acc[j] + _dot(oos[hh], wo_t[j, 128 * hh:128 * hh + 128, :])
            out = jnp.concatenate(acc, axis=1)
            xa[16 + g, 32 * ph:32 * ph + 24, :] = out[8:32]
            mem = _round_bf16(out[0:8])
        return mem

    def dfwd_thunks(rows, tail):
        st = {}

        def pre():
            o = to[...] if tail else xa[16:32, rows, :]
            x = _round_bf16(xa[0:16, rows, :] + o)
            xb[:, rows, :] = x
            y = _layernorm(x.reshape(128, DM))
            x0, x1, x2, x3, x4 = [y[:, 128 * a:128 * a + 128] for a in range(5)]
            t1, t2, t3, t4 = x1 + x4, x2 + x3, x1 - x4, x2 - x3
            t = t1 + t2
            m, n = x0 - 0.25 * t, R5_D * (t1 - t2)
            st["u"] = [(x0 + t).astype(bf16),
                       jnp.concatenate([m + n, t3 + R5_R * t4], axis=1).astype(bf16),
                       jnp.concatenate([m - n, R5_R * t3 - t4], axis=1).astype(bf16)]

        def part(g):
            def run():
                if g == 0:
                    pre()
                k = 64 if g == 0 else 128
                zr, zi = [_dot(st["u"][g], _bf(small[o:o + k, :]))
                          for o in (FW_OFF + 128 * g, FW_OFF + 128 * (g + 3))]
                ys = _fft16([(zr[8 * a:8 * a + 8], zi[8 * a:8 * a + 8]) for a in range(16)], -1)
                for a in range(16):
                    zs[g][0, a, rows, :] = ys[a][0]
                    zs[g][1, a, rows, :] = ys[a][1]
            return run
        return [part(g) for g in range(3)]

    def post(u, carry):
        base = pl.multiple_of(32 * u, 32)
        side = []
        for q in range(4):
            side += dfwd_thunks(pl.ds(base + 8 * q, 8), q == 3)
        side = [side[i] for i in CFG["post_order"]]
        k = 0
        at = list(CFG["post_at"])
        for js in CFG["post_js"]:
            acc = None
            for hh in range(H):
                oo = qb[:, u, hh].reshape(128, 128).astype(bf16)
                acc = addl(acc, [_dot(oo, wo_t[j, 128 * hh:128 * hh + 128, :]) for j in js])
                k += len(js)
                while at and at[0] <= k:
                    at.pop(0)
                    side.pop(0)()
            for j, y in zip(js, acc):
                to[:, :, 128 * j:128 * j + 128] = y.reshape(16, 8, 128)
        for f in side:
            f()
        return carry

    def spectral(zero):
        def fence(z):
            return z[0, zero, 128:ZPITCH, :]

        def radix_inv(g, bb):
            z = zs[g]
            toks = []

            def emit(q, y):
                for p in range(4):
                    z[0, q + 4 * p, chunk(bb), :] = y[p][0]
                    z[1, q + 4 * p, chunk(bb), :] = y[p][1]
                toks.append(fence(z))
            _fft16([(z[0, a, chunk(bb), :], z[1, a, chunk(bb), :]) for a in range(16)], 1, emit)
            return toks

        ys = {}

        def fwd(g, k2, toks):
            z = zs[g]
            ur, ui = z[0, k2, 0:64, :], z[1, k2, 0:64, :]
            tr, ti = _twiddle((z[0, k2, 64:128, :], z[1, k2, 64:128, :]), k2, 32, -1)
            for hf in range(2):
                v = _ilv(ur + tr, ui + ti) if hf == 0 else _ilv(ur - tr, ui - ti)
                lhs = _with_tokens(emat[k2 + 16 * hf], toks if hf == 0 else None)
                xr, xi = _dilv(_dot(_bf(lhs), v.astype(bf16)))
                ys["x", 16 * g + k2] = xr
                wr = wf[g, pl.ds(k2 * WPITCH + hf, 64, stride=2), :]
                wi = wf[g + 3, pl.ds(k2 * WPITCH + hf, 64, stride=2), :]
                ys[g, k2, hf] = _ilv(xr * wr - xi * wi, xr * wi + xi * wr).astype(bf16)

        def inv(g, k2):
            z = zs[g]
            t0 = _dot(_bf(emat[32 + k2]), ys.pop((g, k2, 0)))
            t1 = _dot(_bf(emat[48 + k2]), ys.pop((g, k2, 1)))
            z[0, k2, 0:64, :], z[1, k2, 0:64, :] = _dilv(t0 + t1)
            z[0, k2, 64:128, :], z[1, k2, 64:128, :] = _twiddle(_dilv(t0 - t1), k2, 32, 1)

        units = [(g, k2) for g in range(3) for k2 in range(16)]
        toks = None
        for i in range(len(units) + 3):
            if i < len(units):
                fwd(*units[i], toks)
            if i >= 3:
                inv(*units[i - 3])
            toks = None
            if i in CFG["inv_at"]:
                n = CFG["inv_at"].index(i)
                back, r = CFG["rel"]
                zs[n // 16][1, zero, 128:ZPITCH, :] = ys["x", min(i - back, 47)][8 * r:8 * r + 8]
                toks = {3 + j: pltpu.bitcast(t, u32) for j, t in enumerate(radix_inv(n // 16, n % 16))}

    def dinv_thunks(bb, finish):
        st = {}

        def part(g):
            def run():
                z = zs[g]
                ys = [(z[0, a, chunk(bb), :], z[1, a, chunk(bb), :]) for a in range(16)]
                if g >= CFG["inv_groups"]:
                    ys = _fft16(ys, 1)
                lhs = jnp.concatenate(
                    [jnp.concatenate([y[0] for y in ys], axis=0),
                     jnp.concatenate([y[1] for y in ys], axis=0)], axis=1).astype(bf16)
                for j in ((0,), (1, 2), (3, 4))[g]:
                    st[j] = _dot(lhs, _bf(small[IW_OFF + 128 * j:IW_OFF + 128 * (j + 1), :]))
            return run

        def fin():
            p0, p1, q1, p2, q2 = [st[j] for j in range(5)]
            t = p1 + p2
            m, n = p0 - 0.25 * t, R5_D * (p1 - p2)
            e1, e2 = m + n, m - n
            o1, o2 = q1 + R5_R * q2, R5_R * q1 - q2
            y = jnp.concatenate([p0 + t, e1 - o1, e2 - o2, e2 + o2, e1 + o1], axis=1)
            finish(xb[:, chunk(bb), :].reshape(128, DM) + y)
        return [part(0), part(1), part(2), fin]

    def out_copy(bb):
        return pltpu.make_async_copy(xin.at[:, bb], out_hbm.at[:, bb], osem.at[bb])

    def layer(li, carry0):
        if full or CFG["only"] == "group":
            _loop("step", 0, 16, group, mem_ref[...].astype(f32))
        if full or CFG["only"] == "spec":
            _loop("post", 0, 4, post, 0, unroll=CFG["post_unroll"])

            with jax.named_scope("spectral"):
                spectral((li >> 1))
        if not full:
            return carry0

        @pl.when(li == 0)
        def _():
            with jax.named_scope("dinv_tails"):
                th = [dinv_thunks(4 * u + 3, functools.partial(
                    lambda u, x: set_input(4 * u + 3, _round_bf16(x), u), u)) for u in range(4)]
                for i in range(5):
                    if i < 4:
                        for f in th[i][:3]:
                            f()
                    if i >= 1:
                        th[i - 1][3]()

            def batch(it, carry):
                bb = body_chunk(it)
                side = dinv_thunks(bb, lambda x: set_input(bb, _round_bf16(x), None))
                for k, f in enumerate(batch_thunks(it)):
                    f()
                    if k in CFG["dinv_at"]:
                        side.pop(0)()
                return carry
            _loop("batch", 0, 12, batch, 0, unroll=CFG["batch_unroll"])

        @pl.when(li == 1)
        def _():
            with jax.named_scope("dinv_out"):
                def store_out(bb, x):
                    xin[:, bb] = x.reshape(16, 8, DM).astype(bf16)
                    out_copy(bb).start()
                th = [dinv_thunks(bb, functools.partial(store_out, bb)) for bb in range(16)]
                for i in range(17):
                    if i < 16:
                        for f in th[i][:3]:
                            f()
                    if i >= 1:
                        th[i - 1][3]()
                for bb in range(16):
                    out_copy(bb).wait()
        return carry0

    if CFG["only"] != "pro":
        lax.fori_loop(0, 2, layer, 0)
    else:
        zero = zero_ref[0]
        xin[0, 0, :, 0:128] = (qb[zero, 0, 0] + wf[zero, 0:8, :] + xa[zero, 0:8, 0:128]).astype(bf16)
        out_copy(0).start()
        out_copy(0).wait()


@functools.partial(jax.jit, static_argnames=("A_seg_len",))
def pallas_interleave_layers__memory_aug_recurrent_mem_tr__spectral_gfnet__prompt_kernel(
    A_x, A_mem0, A_Wq, A_Wk, A_Wv, A_Wo, A_seg_len, B_x, B_w_r, B_w_i,
):
    assert A_seg_len == SEG and A_x.shape == (1, S, DM)
    small, emat = _tables()
    hbm = pl.BlockSpec(memory_space=pltpu.HBM)
    out = pl.pallas_call(
        _kernel,
        out_shape=jax.ShapeDtypeStruct((16, 16, 8, DM), bf16),
        in_specs=[hbm] * 10,
        out_specs=hbm,
        scratch_shapes=[
            pltpu.VMEM((16, 16, 8, DM), bf16),
            pltpu.VMEM((33, 128, DM), f32),
            pltpu.VMEM((16, 128, DM), f32),
            pltpu.VMEM((16, 8, DM), f32),
            pltpu.VMEM((12, 2, 320, 8, DH), bf16),
            pltpu.VMEM((13, 8 * HPITCH, 128), u32),
            pltpu.VMEM((13, 8 * HPITCH, 128), u32),
            pltpu.VMEM((5, H * DH, 128), bf16),
            pltpu.VMEM((16, 4, 96, 8, 128), f32),
            pltpu.VMEM((4, 5, 64, 128), u32),
            pltpu.VMEM((2, 16, ZPITCH, 128), f32),
            pltpu.VMEM((2, 16, ZPITCH, 128), f32),
            pltpu.VMEM((2, 16, ZPITCH, 128), f32),
            pltpu.VMEM((6, 16 * WPITCH + 32, 128), f32),
            pltpu.VMEM((9, DF, 512), bf16),
            pltpu.VMEM((4, 328, 128), f32),
            pltpu.VMEM((SMALL_ROWS, 128), u32),
            pltpu.VMEM((64, 64, 128), u32),
            pltpu.VMEM((80, 80), f32),
            pltpu.VMEM((MEM, DM), bf16),
            pltpu.SMEM((1,), jnp.int32),
            pltpu.SemaphoreType.DMA((46,)),
            pltpu.SemaphoreType.DMA((16,)),
        ],
        compiler_params=pltpu.CompilerParams(vmem_limit_bytes=120 * 1024 * 1024,
                                             disable_semaphore_checks=True),
    )(
        A_x.reshape(16, 16, 8, DM), A_mem0.reshape(MEM, DM),
        *[w.reshape(2, 320, H, DH) for w in (A_Wq, A_Wk, A_Wv)], A_Wo.reshape(H * DH, DM), B_w_r.T, B_w_i.T,
        jnp.asarray(small), jnp.asarray(emat),
    )
    return out.reshape(1, S, DM)
```

```python
import functools
import math

import jax
import jax.numpy as jnp
import numpy as np
from jax import lax
import jax.experimental.pallas as pl
import jax.experimental.pallas.tpu as pltpu

f32, bf16, u32 = jnp.float32, jnp.bfloat16, jnp.uint32

S, DM, H, DH, MEM, SEG = 2048, 640, 32, 128, 8, 32
NSEG = S // SEG
NPAIR = H // 2
DF = DM // 2 + 1
EPS = 1e-5
WPITCH = 132

HPITCH = 164
ZPITCH = 136

S1 = math.sin(2 * math.pi / 5)
R5_D = (math.cos(2 * math.pi / 5) - math.cos(4 * math.pi / 5)) / 2
R5_R = math.sin(4 * math.pi / 5) / S1


def _to_bf16_bits(a):
    u = np.ascontiguousarray(a, dtype=np.float32).view(np.uint32).astype(np.uint64)
    return ((u + 0x7FFF + ((u >> 16) & 1)) >> 16).astype(np.uint32)


def _pack_rows(a):
    b = _to_bf16_bits(a)
    return b[..., 0::2, :] | (b[..., 1::2, :] << 16)


@functools.lru_cache(maxsize=None)
def _tables():
    b = np.arange(128)
    l0 = np.arange(0, DF, 5)
    l1 = np.concatenate([np.arange(1, 320, 5), np.arange(4, 320, 5)])
    l2 = np.concatenate([np.arange(2, 320, 5), np.arange(3, 320, 5)])
    sg = np.concatenate([np.ones(64), -np.ones(64)])

    def th(l):
        return 2 * np.pi * ((b[:, None] * l[None, :]) % DM) / DM

    sc = 1.0 / (S * DM)
    fw = np.zeros((8, 128, 128))
    iw = np.zeros((8, 128, 128))
    t = th(l0)
    cl = np.full((65, 1), 2.0)
    cl[0] = cl[-1] = 1.0
    fw[0, :, :65], fw[1, :, :65] = np.cos(t), -np.sin(t)
    iw[0, :65], iw[1, :65] = cl * np.cos(t.T) * sc, -cl * np.sin(t.T) * sc
    mu = S1 * sg
    for g, l in ((1, l1), (2, l2)):
        t = th(l)
        c, s = np.cos(t), np.sin(t)
        fw[3 * g - 1:3 * g + 2] = c, -mu * s - c, mu * c - s
        iw[3 * g - 1:3 * g + 2] = [2 * sc * m.T for m in (c, -s - mu * c, mu * s - c)]
    n = np.arange(64)
    order = np.concatenate([np.concatenate([np.arange(8) + 8 * j, np.arange(8) + 8 * j + 64])
                            for j in range(8)])
    e = np.zeros((2, 32, 128, 128))
    for k2 in range(32):
        t = 2 * np.pi * (((32 * n[:, None] + k2) * n[None, :]) % S) / S
        er, ei = np.cos(t), -np.sin(t)
        m = np.block([[er, -ei], [ei, er]])[order][:, order]
        e[0, k2], e[1, k2] = m, m.T
    small = np.concatenate([_pack_rows(fw), _pack_rows(iw)], axis=0)
    return small, _pack_rows(e).reshape(64, 64, 128)


SMALL_TILES = 16


def _loop(name, lo, hi, body, init, **kw):
    with jax.named_scope(name):
        return lax.fori_loop(lo, hi, body, init, **kw)


def _bf(x):
    return pltpu.bitcast(x, bf16)


def _dot(a, b):
    return jnp.dot(a, b, preferred_element_type=f32)


def _round_bf16(x):
    return x.astype(bf16).astype(f32)


def _layernorm(x):
    m = jnp.mean(x, axis=-1, keepdims=True)
    xc = x - m
    v = jnp.mean(xc * xc, axis=-1, keepdims=True)
    return xc * lax.rsqrt(v + EPS)


def _fft4(x, sign):
    (ar, ai), (br, bi), (cr, ci), (dr, di) = x
    t0r, t0i, t1r, t1i = ar + cr, ai + ci, ar - cr, ai - ci
    t2r, t2i, t3r, t3i = br + dr, bi + di, br - dr, bi - di
    y0, y2 = (t0r + t2r, t0i + t2i), (t0r - t2r, t0i - t2i)
    p, q = (t1r + t3i, t1i - t3r), (t1r - t3i, t1i + t3r)
    return [y0, p, y2, q] if sign < 0 else [y0, q, y2, p]


def _twiddle(z, n, period, sign):
    zr, zi = z
    n = n % period
    if n == 0:
        return z
    if 4 * n == period:
        return (-zi, zr) if sign > 0 else (zi, -zr)
    c, s = math.cos(2 * math.pi * n / period), sign * math.sin(2 * math.pi * n / period)
    if (8 * n) % period == 0:
        a, d = zr + zi, zr - zi
        if c * s > 0:
            return (d * c, a * c)
        return (a * c, d * s)
    return (zr * c - zi * s, zr * s + zi * c)


def _mu():
    lane = lax.broadcasted_iota(jnp.int32, (1, 128), 1)
    return jnp.where(lane < 64, S1, -S1).astype(f32)


def _ilv(r, i):
    n = r.shape[0] // 8
    return jnp.concatenate([r.reshape(n, 8, 128), i.reshape(n, 8, 128)], axis=1).reshape(16 * n, 128)


def _dilv(x):
    n = x.shape[0] // 16
    x = x.reshape(n, 16, 128)
    return x[:, :8].reshape(8 * n, 128), x[:, 8:].reshape(8 * n, 128)


def _with_tokens(x, toks):
    if not toks:
        return x
    return jnp.concatenate(
        [x[8 * j:8 * j + 8] | toks[j] if j in toks else x[8 * j:8 * j + 8]
         for j in range(x.shape[0] // 8)], axis=0)


def _fft16(x, sign, emit=None):
    cols = [_fft4([x[4 * j + r] for j in range(4)], sign) for r in range(4)]
    out = [None] * 16
    for q in range(4):
        y = _fft4([_twiddle(cols[r][q], r * q, 16, sign) for r in range(4)], sign)
        for p in range(4):
            out[q + 4 * p] = y[p]
        if emit is not None:
            emit(q, y)
    return out


CFG = dict(steps=((4.5, 16.5, 6, 4, 0, 8), (5, 16.5, 5, 7, 8, 12), (5, 16.5, 6, 6, 8, 12), (5, 16.5, 8, 7, 8, 0)),
           post_js=((0, 1, 2), (3, 4)),
           post_order=(3, 0, 6, 1, 2, 4, 5, 7, 9, 8, 10, 11), post_at=(40, 80, 120, 126),
           inv_at=tuple(21 + (k * 26) // 16 for k in range(16)), inv_groups=1, rel=(1, 4), dinv_at=(8, 9, 10, 11), batch_unroll=2, post_unroll=1,
           pro_nre=14, re_pos=(3, 5, 7), ln_at=(22, 29, 31, 31), ln_at2=(4, 7, 10, 13),
           perm_at=tuple(range(12, 24)), only=None)


def _interleave(main, side):
    n, k = len(main), 0
    for i, f in enumerate(main):
        f()
        while k < len(side) and (k + 1) * n <= (i + 1) * len(side):
            side[k]()
            k += 1
    for f in side[k:]:
        f()


def _kernel(x_hbm, mem_hbm, wq_hbm, wk_hbm, wv_hbm, wo_hbm, wr_hbm, wi_hbm,
            small_hbm, e_hbm, out_hbm,
            xin, xa, xb, to, raw, wa, wb, wo_t, qb, hl, z0, z1, z2, wf,
            wri, wtmp, small, emat, fill_ref, mem_ref, zero_ref, sem, osem):
    zs = (z0, z1, z2)
    w_hbm = (wq_hbm, wk_hbm, wv_hbm)

    def body_chunk(i):
        return 4 * (i & 3) + (i >> 2)

    def cp_w(i):
        src = w_hbm[i >> 2].at[:, :, pl.ds(8 * (i & 3), 8), :] if isinstance(i, int) else raw.at[i]
        return pltpu.make_async_copy(src, raw.at[i], sem.at[i])

    def cp_x(bb):
        return pltpu.make_async_copy(x_hbm.at[:, bb], xin.at[:, bb], sem.at[12 + bb])

    def cp_f(i):
        src = ((wr_hbm, wi_hbm)[i >> 2].at[:, pl.ds(512 * (i & 3), 512)]
               if isinstance(i, int) else wri.at[i])
        return pltpu.make_async_copy(src, wri.at[i], sem.at[36 + i])

    cp_rest = [pltpu.make_async_copy(wo_hbm.at[:, pl.ds(128 * j, 128)], wo_t.at[j], sem.at[28 + j])
               for j in range(5)]
    cp_rest += [pltpu.make_async_copy(mem_hbm, mem_ref, sem.at[33]),
                pltpu.make_async_copy(small_hbm, small, sem.at[44]),
               pltpu.make_async_copy(e_hbm, emat, sem.at[45])]

    full = CFG["only"] in (None, "pro")
    for u in range(4 if full else 0):
        cp_x(4 * u + 3).start()
    if full:
        cp_w(0).start()
    for i in range(12 if full else 0):
        if i < 11:
            cp_w(i + 1).start()
        cp_x(body_chunk(i)).start()
        if 3 <= i < 11:
            cp_f(i - 3).start()
    for cp in cp_rest if full else ():
        cp.start()

    zero_ref[0] = 0

    r = lax.broadcasted_iota(jnp.int32, (80, 80), 0)
    c = lax.broadcasted_iota(jnp.int32, (80, 80), 1)

    def head(i):
        return jnp.where(i < 64, i // 32, (i - 64) // 8)

    def pos(i):
        return jnp.where(i < 64, i % 32, 32 + (i - 64) % 8)

    ok = (pos(r) < MEM) | (pos(r) >= pos(c))
    fill_ref[...] = jnp.where(head(r) == head(c), jnp.where(ok, 0.0, -1e9), -jnp.inf).astype(f32)
    wtmp[:, 320:328, :] = jnp.zeros((4, 8, 128), f32)
    xa[32, 0:8, 0:128] = jnp.zeros((8, 128), f32)
    wa[12, 0:8, :] = jnp.zeros((8, 128), u32)
    wb[12, 0:8, :] = jnp.zeros((8, 128), u32)
    wf[5, 16 * WPITCH:16 * WPITCH + 8, :] = jnp.zeros((8, 128), f32)
    for z in zs:
        z[0, 0, 128:ZPITCH, :] = jnp.zeros((8, 128), f32)

    def chunk(bb):
        if isinstance(bb, int):
            return slice(8 * bb, 8 * bb + 8)
        return pl.ds(pl.multiple_of(8 * bb, 8), 8)

    def set_input(bb, x, tail_u, a0=0):
        n = x.shape[0] // 8
        xa[a0:a0 + n, chunk(bb), :] = x.reshape(n, 8, DM)
        y = _layernorm(x)
        if tail_u is None:
            xa[16 + a0:16 + a0 + n, chunk(bb), :] = y.reshape(n, 8, DM)
        else:
            yb = y.astype(bf16)
            for kt in range(5):
                hl[tail_u, kt] = pltpu.bitcast(yb[:, 128 * kt:128 * kt + 128], u32)

    def load_x(bb, a0=0, n=16):
        return xin[a0:a0 + n, bb].astype(f32).reshape(8 * n, DM)

    def wtile(cid, j, e):
        w = (wa, wb)[e]
        return jnp.concatenate([w[cid, (4 * hf + j) * HPITCH:(4 * hf + j) * HPITCH + 160, :]
                                for hf in range(2)], axis=0)

    def relayout(i, cid, e):
        for r in range(4 * i, 4 * i + 4):
            a, b = [pltpu.bitcast(raw[cid, :, d].reshape(16, 128), u32) for d in (2 * r, 2 * r + 1)]
            v = (a & 0xFFFF) | (b << 16) if e == 0 else (a >> 16) | (b & jnp.uint32(0xFFFF0000))
            (wa, wb)[e][cid, pl.ds(r, 8, stride=HPITCH), :] = v

    def batch_thunks(cid):
        def one(j, u, e):
            def run(toks=None):
                lhs = jnp.concatenate(
                    [_bf(_with_tokens(hl[u, kt], toks if kt == 0 else None)) for kt in range(5)], axis=1)
                qb[:, u, 8 * cid + 2 * j + e] = _dot(lhs, _bf(wtile(cid, j, e))).reshape(16, 8, 128)
            return run
        return [one(j, u, e) for e in range(2) for j in range(4) for u in range(4)]

    def wperm_thunks(piece, j):
        m = (piece >> 2) & 1
        wt = wtmp.at[j]

        def load():
            wt[0:DF, :] = wri[piece, :, 128 * j:128 * j + 128].astype(f32)

        def one(g):
            def run():
                if g == 0:
                    t = jnp.concatenate([wt[pl.ds(0, 64, stride=5), :], wt[320:328, :],
                                         jnp.zeros((56, 128), f32)], axis=0)
                else:
                    t = jnp.concatenate([wt[pl.ds(g, 64, stride=5), :],
                                         wt[pl.ds(5 - g, 64, stride=5), :]], axis=0)
                y = t.T
                sub = wf.at[3 * m + g, pl.ds(pl.multiple_of((piece & 3) * 32, 32), 16 * WPITCH - 96)]
                for k in range(8):
                    for hf in range(2):
                        sub[pl.ds(8 * j + k + 8 * hf * WPITCH, 8, stride=WPITCH), :] = (
                            y[16 * k + 8 * hf:16 * k + 8 * hf + 8])
            return run
        return [load] + [one(g) for g in range(3)]

    def half_pass(cid, half, fill, zero, timed=()):
        nre = CFG["pro_nre"]
        toks = None
        for k, f in enumerate(batch_thunks(cid)[16 * half:16 * half + 16]):
            f(toks)
            toks = {}
            for pos, f in zip((0, 4, 1, 6), [f for at, f in timed if at == k]):
                toks[pos] = f()
            if fill is not None:
                for n, r in enumerate(r for r in range(40) if r * nre // 40 == k):
                    relayout(r, fill, 1 - half)
                    toks[CFG["re_pos"][n]] = (wb, wa)[half][12 + zero, 0:8, :]

    def ln_parts(bb, zero):
        def part(j):
            set_input(bb, load_x(bb, 4 * j, 4), None, 4 * j)
            return pltpu.bitcast(xa[32 + zero, 0:8, 0:128], u32)
        return [functools.partial(part, j) for j in range(4)]

    def perm_parts(piece, zero):
        def part(fs):
            for f in fs:
                f()
            return pltpu.bitcast(wf[5 + zero, 16 * WPITCH:16 * WPITCH + 8, :], u32)
        out = []
        for j in range(4):
            th = wperm_thunks(piece, j)
            out += [functools.partial(part, th[0:2]), functools.partial(part, th[2:3]),
                    functools.partial(part, th[3:4])]
        return out

    def pro0():
        for u in range(4):
            cp_x(4 * u + 3).wait()
        for u in range(4):
            set_input(4 * u + 3, load_x(4 * u + 3), u)
        cp_w(0).wait()
        zero = zero_ref[0]
        for i in range(40):
            relayout(i, 0, 0)
        half_pass(0, 0, zero, zero)

    def pro1(it, carry):
        bb = body_chunk(it)
        with jax.named_scope("pro1_wait"):
            cp_w(it + 1).wait()

            @pl.when(it >= 3)
            def _():
                cp_f(it - 3).wait()
            cp_x(bb).wait()
        piece = jnp.where(it >= 3, it - 3, 8)
        zero = it >> 4
        timed = sorted(list(zip(CFG["ln_at"], ln_parts(bb, zero)))
                       + list(zip(CFG["perm_at"], perm_parts(piece, zero))), key=lambda x: x[0])
        half_pass(it, 1, it + 1, zero, [x for x in timed if x[0] < 16])
        half_pass(it + 1, 0, it + 1, zero, [(k - 16, f) for k, f in timed if k >= 16])
        return carry

    def pro2():
        cp_x(body_chunk(11)).wait()
        for cp in cp_rest:
            cp.wait()
        zero = zero_ref[0]
        half_pass(11, 1, None, zero, list(zip(CFG["ln_at2"], ln_parts(body_chunk(11), zero))))

    if full:
        with jax.named_scope("pro0"):
            pro0()
        _loop("pro1", 0, 11, pro1, 0)
        with jax.named_scope("pro2"):
            pro2()

    scale = DH ** -0.5

    def wo_dot(hh, oo):
        return [_dot(oo, wo_t[j, 128 * hh:128 * hh + 128, :]) for j in range(5)]

    def addl(acc, res):
        return res if acc is None else [a + b for a, b in zip(acc, res)]

    def group(g, mem):
        for ph in range(4):
            h = jnp.concatenate([mem, xa[16 + g, 32 * ph:32 * ph + 24, :]], axis=0).astype(bf16)
            pr, sm, oos = {}, {}, {}
            lat_s, lat_pv, lat_wo, v_delay, n_first, n_last = CFG["steps"][ph]

            def stacked(p, m):
                tails = [qb[g, ph, 32 * m + 2 * p + e] for e in range(2)]
                return jnp.concatenate([pr[p, m, 0], pr[p, m, 1]] + tails, axis=0).astype(bf16)

            def scores(p):
                sc = lax.dot_general(stacked(p, 0), stacked(p, 1), (((1,), (1,)), ((), ())),
                                     preferred_element_type=f32)
                fill = fill_ref[...]
                sc = jnp.where(fill == 0.0, sc * scale, fill)
                mx = jnp.max(sc, axis=-1, keepdims=True)
                e = jnp.exp(sc - mx)
                rl = pl.reciprocal(jnp.sum(e, axis=-1, keepdims=True), approx=True)
                sm[p] = (e * rl).astype(bf16)

            def pv(p):
                o = _dot(sm[p], stacked(p, 2))
                for e in range(2):
                    qb[g, ph, 2 * p + e] = o[64 + 8 * e:72 + 8 * e]
                    oos[2 * p + e] = o[32 * e:32 * e + 32].astype(bf16)

            keyed = []
            for p in range(NPAIR):
                keyed += [(4 * p + 2 * m + e, (p, m, e)) for m in range(2) for e in range(2)]
                keyed += [(4 * p + 3.5 + v_delay, (p, 2, e)) for e in range(2)]
            bulk = [x for _, x in sorted(keyed, key=lambda kv: kv[0])]
            acc, t, nwo, pend, ready = None, 0.0, 0, [], []
            if n_first:
                first, bulk = bulk[:n_first], bulk[n_first:]
                for kt in range(5):
                    for p, m, e in first:
                        w = wtile(4 * m + (p >> 2), p & 3, e)[64 * kt:64 * kt + 64]
                        y = _dot(h[:, 128 * kt:128 * kt + 128], _bf(w))
                        pr[p, m, e] = y if kt == 0 else pr[p, m, e] + y
                t = float(len(first))
                pend = [(t + lat_s, "S", p) for p, m, e in first if m == 1 and e == 1]
            while nwo < H - n_last or pend:
                pend.sort()
                if pend and pend[0][0] <= t:
                    _, kind, p = pend.pop(0)
                    if kind == "S":
                        scores(p)
                        pend.append((t + lat_pv, "V", p))
                    else:
                        pv(p)
                        ready += [(t + lat_wo, 2 * p + e) for e in range(2)]
                    t += 0.5
                elif bulk:
                    p, m, e = bulk.pop(0)
                    pr[p, m, e] = _dot(h, _bf(wtile(4 * m + (p >> 2), p & 3, e)))
                    t += 1
                    if m == 1 and e == 1:
                        pend.append((t + lat_s, "S", p))
                elif ready and ready[0][0] <= t and nwo < H - n_last:
                    _, hh = ready.pop(0)
                    acc = addl(acc, wo_dot(hh, oos[hh]))
                    t += 1
                    nwo += 1
                else:
                    t += 0.5
            for j in range(5):
                for _, hh in ready:
                    acc[j] = acc[j] + _dot(oos[hh], wo_t[j, 128 * hh:128 * hh + 128, :])
            out = jnp.concatenate(acc, axis=1)
            xa[16 + g, 32 * ph:32 * ph + 24, :] = out[8:32]
            mem = _round_bf16(out[0:8])
        return mem

    def dfwd_thunks(rows, tail):
        st = {}

        def pre():
            o = to[...] if tail else xa[16:32, rows, :]
            x = _round_bf16(xa[0:16, rows, :] + o)
            xb[:, rows, :] = x
            y = _layernorm(x.reshape(128, DM))
            x0, x1, x2, x3, x4 = [y[:, 128 * a:128 * a + 128] for a in range(5)]
            t1, t2, t3, t4 = x1 + x4, x2 + x3, x1 - x4, x2 - x3
            t = t1 + t2
            m, n = x0 - 0.25 * t, R5_D * (t1 - t2)
            st["u"] = [x0 + t, (m + n, t3 + R5_R * t4), (m - n, R5_R * t3 - t4)]

        def part(g):
            def run():
                if g == 0:
                    pre()
                    u0 = st["u"][0].astype(bf16)
                    zr, zi = _dot(u0, _bf(small[0])), _dot(u0, _bf(small[1]))
                else:
                    a, b = st["u"][g]
                    k, kb, ka = [_dot(v.astype(bf16), _bf(small[3 * g - 1 + i]))
                                 for i, v in enumerate((a + b, b, a))]
                    zr, zi = k + kb, ka - _mu() * k
                ys = _fft16([(zr[8 * a:8 * a + 8], zi[8 * a:8 * a + 8]) for a in range(16)], -1)
                for a in range(16):
                    zs[g][0, a, rows, :] = ys[a][0]
                    zs[g][1, a, rows, :] = ys[a][1]
            return run
        return [part(g) for g in range(3)]

    def post(u, carry):
        base = pl.multiple_of(32 * u, 32)
        side = []
        for q in range(4):
            side += dfwd_thunks(pl.ds(base + 8 * q, 8), q == 3)
        side = [side[i] for i in CFG["post_order"]]
        k = 0
        at = list(CFG["post_at"])
        for js in CFG["post_js"]:
            acc = None
            for hh in range(H):
                oo = qb[:, u, hh].reshape(128, 128).astype(bf16)
                acc = addl(acc, [_dot(oo, wo_t[j, 128 * hh:128 * hh + 128, :]) for j in js])
                k += len(js)
                while at and at[0] <= k:
                    at.pop(0)
                    side.pop(0)()
            for j, y in zip(js, acc):
                to[:, :, 128 * j:128 * j + 128] = y.reshape(16, 8, 128)
        for f in side:
            f()
        return carry

    def spectral(zero):
        def fence(z):
            return z[0, zero, 128:ZPITCH, :]

        def radix_inv(g, bb):
            z = zs[g]
            toks = []

            def emit(q, y):
                for p in range(4):
                    z[0, q + 4 * p, chunk(bb), :] = y[p][0]
                    z[1, q + 4 * p, chunk(bb), :] = y[p][1]
                toks.append(fence(z))
            _fft16([(z[0, a, chunk(bb), :], z[1, a, chunk(bb), :]) for a in range(16)], 1, emit)
            return toks

        ys = {}

        def fwd(g, k2, toks):
            z = zs[g]
            ur, ui = z[0, k2, 0:64, :], z[1, k2, 0:64, :]
            tr, ti = _twiddle((z[0, k2, 64:128, :], z[1, k2, 64:128, :]), k2, 32, -1)
            for hf in range(2):
                v = _ilv(ur + tr, ui + ti) if hf == 0 else _ilv(ur - tr, ui - ti)
                lhs = _with_tokens(emat[k2 + 16 * hf], toks if hf == 0 else None)
                xr, xi = _dilv(_dot(_bf(lhs), v.astype(bf16)))
                ys["x", 16 * g + k2] = xr
                wr = wf[g, pl.ds(k2 * WPITCH + hf, 64, stride=2), :]
                wi = wf[g + 3, pl.ds(k2 * WPITCH + hf, 64, stride=2), :]
                ys[g, k2, hf] = _ilv(xr * wr - xi * wi, xr * wi + xi * wr).astype(bf16)

        def inv(g, k2):
            z = zs[g]
            t0 = _dot(_bf(emat[32 + k2]), ys.pop((g, k2, 0)))
            t1 = _dot(_bf(emat[48 + k2]), ys.pop((g, k2, 1)))
            z[0, k2, 0:64, :], z[1, k2, 0:64, :] = _dilv(t0 + t1)
            z[0, k2, 64:128, :], z[1, k2, 64:128, :] = _twiddle(_dilv(t0 - t1), k2, 32, 1)

        units = [(g, k2) for g in range(3) for k2 in range(16)]
        toks = None
        for i in range(len(units) + 3):
            if i < len(units):
                fwd(*units[i], toks)
            if i >= 3:
                inv(*units[i - 3])
            toks = None
            if i in CFG["inv_at"]:
                n = CFG["inv_at"].index(i)
                back, r = CFG["rel"]
                zs[n // 16][1, zero, 128:ZPITCH, :] = ys["x", min(i - back, 47)][8 * r:8 * r + 8]
                toks = {3 + j: pltpu.bitcast(t, u32) for j, t in enumerate(radix_inv(n // 16, n % 16))}

    def dinv_thunks(bb, finish):
        st = {}

        def part(g):
            def run():
                z = zs[g]
                ys = [(z[0, a, chunk(bb), :], z[1, a, chunk(bb), :]) for a in range(16)]
                if g >= CFG["inv_groups"]:
                    ys = _fft16(ys, 1)
                tr = jnp.concatenate([y[0] for y in ys], axis=0)
                ti = jnp.concatenate([y[1] for y in ys], axis=0)
                if g == 0:
                    st[0] = _dot(tr.astype(bf16), _bf(small[8])) + _dot(ti.astype(bf16), _bf(small[9]))
                else:
                    k, ki, kr = [_dot(v.astype(bf16), _bf(small[7 + 3 * g + i]))
                                 for i, v in enumerate((tr + _mu() * ti, ti, tr))]
                    st[2 * g - 1], st[2 * g] = k + ki, k + kr
            return run

        def fin():
            p0, p1, q1, p2, q2 = [st[j] for j in range(5)]
            t = p1 + p2
            m, n = p0 - 0.25 * t, R5_D * (p1 - p2)
            e1, e2 = m + n, m - n
            o1, o2 = q1 + R5_R * q2, R5_R * q1 - q2
            y = jnp.concatenate([p0 + t, e1 - o1, e2 - o2, e2 + o2, e1 + o1], axis=1)
            finish(xb[:, chunk(bb), :].reshape(128, DM) + y)
        return [part(0), part(1), part(2), fin]

    def out_copy(bb):
        return pltpu.make_async_copy(xin.at[:, bb], out_hbm.at[:, bb], osem.at[bb])

    def layer(li, carry0):
        if full or CFG["only"] == "group":
            _loop("step", 0, 16, group, mem_ref[...].astype(f32))
        if full or CFG["only"] == "spec":
            _loop("post", 0, 4, post, 0, unroll=CFG["post_unroll"])

            with jax.named_scope("spectral"):
                spectral((li >> 1))
        if not full:
            return carry0

        @pl.when(li == 0)
        def _():
            with jax.named_scope("dinv_tails"):
                th = [dinv_thunks(4 * u + 3, functools.partial(
                    lambda u, x: set_input(4 * u + 3, _round_bf16(x), u), u)) for u in range(4)]
                for i in range(5):
                    if i < 4:
                        for f in th[i][:3]:
                            f()
                    if i >= 1:
                        th[i - 1][3]()

            def batch(it, carry):
                bb = body_chunk(it)
                side = dinv_thunks(bb, lambda x: set_input(bb, _round_bf16(x), None))
                for k, f in enumerate(batch_thunks(it)):
                    f()
                    if k in CFG["dinv_at"]:
                        side.pop(0)()
                return carry
            _loop("batch", 0, 12, batch, 0, unroll=CFG["batch_unroll"])

        @pl.when(li == 1)
        def _():
            with jax.named_scope("dinv_out"):
                def store_out(bb, x):
                    xin[:, bb] = x.reshape(16, 8, DM).astype(bf16)
                    out_copy(bb).start()
                th = [dinv_thunks(bb, functools.partial(store_out, bb)) for bb in range(16)]
                for i in range(17):
                    if i < 16:
                        for f in th[i][:3]:
                            f()
                    if i >= 1:
                        th[i - 1][3]()
                for bb in range(16):
                    out_copy(bb).wait()
        return carry0

    if CFG["only"] != "pro":
        lax.fori_loop(0, 2, layer, 0)
    else:
        zero = zero_ref[0]
        xin[0, 0, :, 0:128] = (qb[zero, 0, 0] + wf[zero, 0:8, :] + xa[zero, 0:8, 0:128]).astype(bf16)
        out_copy(0).start()
        out_copy(0).wait()


@functools.partial(jax.jit, static_argnames=("A_seg_len",))
def pallas_interleave_layers__memory_aug_recurrent_mem_tr__spectral_gfnet__prompt_kernel(
    A_x, A_mem0, A_Wq, A_Wk, A_Wv, A_Wo, A_seg_len, B_x, B_w_r, B_w_i,
):
    assert A_seg_len == SEG and A_x.shape == (1, S, DM)
    small, emat = _tables()
    hbm = pl.BlockSpec(memory_space=pltpu.HBM)
    out = pl.pallas_call(
        _kernel,
        out_shape=jax.ShapeDtypeStruct((16, 16, 8, DM), bf16),
        in_specs=[hbm] * 10,
        out_specs=hbm,
        scratch_shapes=[
            pltpu.VMEM((16, 16, 8, DM), bf16),
            pltpu.VMEM((33, 128, DM), f32),
            pltpu.VMEM((16, 128, DM), f32),
            pltpu.VMEM((16, 8, DM), f32),
            pltpu.VMEM((12, 2, 320, 8, DH), bf16),
            pltpu.VMEM((13, 8 * HPITCH, 128), u32),
            pltpu.VMEM((13, 8 * HPITCH, 128), u32),
            pltpu.VMEM((5, H * DH, 128), bf16),
            pltpu.VMEM((16, 4, 96, 8, 128), f32),
            pltpu.VMEM((4, 5, 64, 128), u32),
            pltpu.VMEM((2, 16, ZPITCH, 128), f32),
            pltpu.VMEM((2, 16, ZPITCH, 128), f32),
            pltpu.VMEM((2, 16, ZPITCH, 128), f32),
            pltpu.VMEM((6, 16 * WPITCH + 32, 128), f32),
            pltpu.VMEM((9, DF, 512), bf16),
            pltpu.VMEM((4, 328, 128), f32),
            pltpu.VMEM((SMALL_TILES, 64, 128), u32),
            pltpu.VMEM((64, 64, 128), u32),
            pltpu.VMEM((80, 80), f32),
            pltpu.VMEM((MEM, DM), bf16),
            pltpu.SMEM((1,), jnp.int32),
            pltpu.SemaphoreType.DMA((46,)),
            pltpu.SemaphoreType.DMA((16,)),
        ],
        compiler_params=pltpu.CompilerParams(vmem_limit_bytes=120 * 1024 * 1024,
                                             disable_semaphore_checks=True),
    )(
        A_x.reshape(16, 16, 8, DM), A_mem0.reshape(MEM, DM),
        *[w.reshape(2, 320, H, DH) for w in (A_Wq, A_Wk, A_Wv)], A_Wo.reshape(H * DH, DM), B_w_r.T, B_w_i.T,
        jnp.asarray(small), jnp.asarray(emat),
    )
    return out.reshape(1, S, DM)
```

```python
import functools
import math

import jax
import jax.numpy as jnp
import numpy as np
from jax import lax
import jax.experimental.pallas as pl
import jax.experimental.pallas.tpu as pltpu

f32, bf16, u32 = jnp.float32, jnp.bfloat16, jnp.uint32

S, DM, H, DH, MEM, SEG = 2048, 640, 32, 128, 8, 32
NSEG = S // SEG
NPAIR = H // 2
DF = DM // 2 + 1
EPS = 1e-5
WPITCH = 132

HPITCH = 164
ZPITCH = 136

S1 = math.sin(2 * math.pi / 5)
R5_D = (math.cos(2 * math.pi / 5) - math.cos(4 * math.pi / 5)) / 2
R5_R = math.sin(4 * math.pi / 5) / S1


def _to_bf16_bits(a):
    u = np.ascontiguousarray(a, dtype=np.float32).view(np.uint32).astype(np.uint64)
    return ((u + 0x7FFF + ((u >> 16) & 1)) >> 16).astype(np.uint32)


def _pack_rows(a):
    b = _to_bf16_bits(a)
    return b[..., 0::2, :] | (b[..., 1::2, :] << 16)


@functools.lru_cache(maxsize=None)
def _tables():
    b = np.arange(128)
    l0 = np.arange(0, DF, 5)
    l1 = np.concatenate([np.arange(1, 320, 5), np.arange(4, 320, 5)])
    l2 = np.concatenate([np.arange(2, 320, 5), np.arange(3, 320, 5)])
    sg = np.concatenate([np.ones(64), -np.ones(64)])

    def th(l):
        return 2 * np.pi * ((b[:, None] * l[None, :]) % DM) / DM

    sc = 1.0 / (S * DM)
    fw = np.zeros((8, 128, 128))
    iw = np.zeros((8, 128, 128))
    t = th(l0)
    cl = np.full((65, 1), 2.0)
    cl[0] = cl[-1] = 1.0
    fw[0, :, :65], fw[1, :, :65] = np.cos(t), -np.sin(t)
    iw[0, :65], iw[1, :65] = cl * np.cos(t.T) * sc, -cl * np.sin(t.T) * sc
    mu = S1 * sg
    for g, l in ((1, l1), (2, l2)):
        t = th(l)
        c, s = np.cos(t), np.sin(t)
        fw[3 * g - 1:3 * g + 2] = c, -mu * s - c, mu * c - s
        iw[3 * g - 1:3 * g + 2] = [2 * sc * m.T for m in (c, -s - mu * c, mu * s - c)]
    n = np.arange(64)
    order = np.concatenate([np.concatenate([np.arange(8) + 8 * j, np.arange(8) + 8 * j + 64])
                            for j in range(8)])
    e = np.zeros((2, 32, 128, 128))
    for k2 in range(32):
        t = 2 * np.pi * (((32 * n[:, None] + k2) * n[None, :]) % S) / S
        er, ei = np.cos(t), -np.sin(t)
        m = np.block([[er, -ei], [ei, er]])[order][:, order]
        e[0, k2], e[1, k2] = m, m.T
    small = np.concatenate([_pack_rows(fw), _pack_rows(iw)], axis=0)
    return small, _pack_rows(e).reshape(64, 64, 128)


SMALL_TILES = 16


def _loop(name, lo, hi, body, init, **kw):
    with jax.named_scope(name):
        return lax.fori_loop(lo, hi, body, init, **kw)


def _bf(x):
    return pltpu.bitcast(x, bf16)


def _dot(a, b):
    return jnp.dot(a, b, preferred_element_type=f32)


def _round_bf16(x):
    return x.astype(bf16).astype(f32)


def _layernorm(x):
    m = jnp.mean(x, axis=-1, keepdims=True)
    xc = x - m
    v = jnp.mean(xc * xc, axis=-1, keepdims=True)
    return xc * lax.rsqrt(v + EPS)


def _fft4(x, sign):
    (ar, ai), (br, bi), (cr, ci), (dr, di) = x
    t0r, t0i, t1r, t1i = ar + cr, ai + ci, ar - cr, ai - ci
    t2r, t2i, t3r, t3i = br + dr, bi + di, br - dr, bi - di
    y0, y2 = (t0r + t2r, t0i + t2i), (t0r - t2r, t0i - t2i)
    p, q = (t1r + t3i, t1i - t3r), (t1r - t3i, t1i + t3r)
    return [y0, p, y2, q] if sign < 0 else [y0, q, y2, p]


def _twiddle(z, n, period, sign):
    zr, zi = z
    n = n % period
    if n == 0:
        return z
    if 4 * n == period:
        return (-zi, zr) if sign > 0 else (zi, -zr)
    c, s = math.cos(2 * math.pi * n / period), sign * math.sin(2 * math.pi * n / period)
    if (8 * n) % period == 0:
        a, d = zr + zi, zr - zi
        if c * s > 0:
            return (d * c, a * c)
        return (a * c, d * s)
    return (zr * c - zi * s, zr * s + zi * c)


def _mu():
    lane = lax.broadcasted_iota(jnp.int32, (1, 128), 1)
    return jnp.where(lane < 64, S1, -S1).astype(f32)


def _ilv(r, i):
    n = r.shape[0] // 8
    return jnp.concatenate([r.reshape(n, 8, 128), i.reshape(n, 8, 128)], axis=1).reshape(16 * n, 128)


def _dilv(x):
    n = x.shape[0] // 16
    x = x.reshape(n, 16, 128)
    return x[:, :8].reshape(8 * n, 128), x[:, 8:].reshape(8 * n, 128)


def _with_tokens(x, toks):
    if not toks:
        return x
    return jnp.concatenate(
        [x[8 * j:8 * j + 8] | toks[j] if j in toks else x[8 * j:8 * j + 8]
         for j in range(x.shape[0] // 8)], axis=0)


def _fft16(x, sign, emit=None):
    cols = [_fft4([x[4 * j + r] for j in range(4)], sign) for r in range(4)]
    out = [None] * 16
    for q in range(4):
        y = _fft4([_twiddle(cols[r][q], r * q, 16, sign) for r in range(4)], sign)
        for p in range(4):
            out[q + 4 * p] = y[p]
        if emit is not None:
            emit(q, y)
    return out


CFG = dict(steps=((4.5, 16.5, 6, 4, 0, 8), (5, 16.5, 5, 7, 8, 12), (5, 16.5, 6, 6, 8, 12), (5, 16.5, 8, 7, 8, 0)),
           post_js=((0, 1, 2), (3, 4)),
           post_order=(0, 1, 3, 4, 6, 8, 2, 5, 7, 9, 10, 11), post_at=(30, 34, 66, 76, 110),
           late_g2=True,
           inv_at=tuple(21 + (k * 26) // 16 for k in range(16)), inv_groups=1, fwd_at=tuple(range(2, 18)), rel=(1, 4), dinv_at=(8, 9, 10, 11), batch_unroll=2, post_unroll=1,
           pro_nre=14, re_pos=(3, 5, 7), ln_at=(22, 29, 31, 31), ln_at2=(4, 7, 10, 13),
           perm_at=tuple(range(12, 24)), only=None)


def _interleave(main, side):
    n, k = len(main), 0
    for i, f in enumerate(main):
        f()
        while k < len(side) and (k + 1) * n <= (i + 1) * len(side):
            side[k]()
            k += 1
    for f in side[k:]:
        f()


def _kernel(x_hbm, mem_hbm, wq_hbm, wk_hbm, wv_hbm, wo_hbm, wr_hbm, wi_hbm,
            small_hbm, e_hbm, out_hbm,
            xin, xa, xb, to, raw, wa, wb, wo_t, qb, hl, z0, z1, z2, wf,
            wri, wtmp, small, emat, fill_ref, mem_ref, zero_ref, sem, osem):
    zs = (z0, z1, z2)
    w_hbm = (wq_hbm, wk_hbm, wv_hbm)

    def body_chunk(i):
        return 4 * (i & 3) + (i >> 2)

    def cp_w(i):
        src = w_hbm[i >> 2].at[:, :, pl.ds(8 * (i & 3), 8), :] if isinstance(i, int) else raw.at[i]
        return pltpu.make_async_copy(src, raw.at[i], sem.at[i])

    def cp_x(bb):
        return pltpu.make_async_copy(x_hbm.at[:, bb], xin.at[:, bb], sem.at[12 + bb])

    def cp_f(i):
        src = ((wr_hbm, wi_hbm)[i >> 2].at[:, pl.ds(512 * (i & 3), 512)]
               if isinstance(i, int) else wri.at[i])
        return pltpu.make_async_copy(src, wri.at[i], sem.at[36 + i])

    cp_rest = [pltpu.make_async_copy(wo_hbm.at[:, pl.ds(128 * j, 128)], wo_t.at[j], sem.at[28 + j])
               for j in range(5)]
    cp_rest += [pltpu.make_async_copy(mem_hbm, mem_ref, sem.at[33]),
                pltpu.make_async_copy(small_hbm, small, sem.at[44]),
               pltpu.make_async_copy(e_hbm, emat, sem.at[45])]

    full = CFG["only"] in (None, "pro")
    for u in range(4 if full else 0):
        cp_x(4 * u + 3).start()
    if full:
        cp_w(0).start()
    for i in range(12 if full else 0):
        if i < 11:
            cp_w(i + 1).start()
        cp_x(body_chunk(i)).start()
        if 3 <= i < 11:
            cp_f(i - 3).start()
    for cp in cp_rest if full else ():
        cp.start()

    zero_ref[0] = 0

    r = lax.broadcasted_iota(jnp.int32, (80, 80), 0)
    c = lax.broadcasted_iota(jnp.int32, (80, 80), 1)

    def head(i):
        return jnp.where(i < 64, i // 32, (i - 64) // 8)

    def pos(i):
        return jnp.where(i < 64, i % 32, 32 + (i - 64) % 8)

    ok = (pos(r) < MEM) | (pos(r) >= pos(c))
    fill_ref[...] = jnp.where(head(r) == head(c), jnp.where(ok, 0.0, -1e9), -jnp.inf).astype(f32)
    wtmp[:, 320:328, :] = jnp.zeros((4, 8, 128), f32)
    xa[32, 0:8, 0:128] = jnp.zeros((8, 128), f32)
    wa[12, 0:8, :] = jnp.zeros((8, 128), u32)
    wb[12, 0:8, :] = jnp.zeros((8, 128), u32)
    wf[5, 16 * WPITCH:16 * WPITCH + 8, :] = jnp.zeros((8, 128), f32)
    for z in zs:
        z[0, 0, 128:ZPITCH, :] = jnp.zeros((8, 128), f32)

    def chunk(bb):
        if isinstance(bb, int):
            return slice(8 * bb, 8 * bb + 8)
        return pl.ds(pl.multiple_of(8 * bb, 8), 8)

    def set_input(bb, x, tail_u, a0=0):
        n = x.shape[0] // 8
        xa[a0:a0 + n, chunk(bb), :] = x.reshape(n, 8, DM)
        y = _layernorm(x)
        if tail_u is None:
            xa[16 + a0:16 + a0 + n, chunk(bb), :] = y.reshape(n, 8, DM)
        else:
            yb = y.astype(bf16)
            for kt in range(5):
                hl[tail_u, kt] = pltpu.bitcast(yb[:, 128 * kt:128 * kt + 128], u32)

    def load_x(bb, a0=0, n=16):
        return xin[a0:a0 + n, bb].astype(f32).reshape(8 * n, DM)

    def wtile(cid, j, e):
        w = (wa, wb)[e]
        return jnp.concatenate([w[cid, (4 * hf + j) * HPITCH:(4 * hf + j) * HPITCH + 160, :]
                                for hf in range(2)], axis=0)

    def relayout(i, cid, e):
        for r in range(4 * i, 4 * i + 4):
            a, b = [pltpu.bitcast(raw[cid, :, d].reshape(16, 128), u32) for d in (2 * r, 2 * r + 1)]
            v = (a & 0xFFFF) | (b << 16) if e == 0 else (a >> 16) | (b & jnp.uint32(0xFFFF0000))
            (wa, wb)[e][cid, pl.ds(r, 8, stride=HPITCH), :] = v

    def batch_thunks(cid):
        def one(j, u, e):
            def run(toks=None):
                lhs = jnp.concatenate(
                    [_bf(_with_tokens(hl[u, kt], toks if kt == 0 else None)) for kt in range(5)], axis=1)
                qb[:, u, 8 * cid + 2 * j + e] = _dot(lhs, _bf(wtile(cid, j, e))).reshape(16, 8, 128)
            return run
        return [one(j, u, e) for e in range(2) for j in range(4) for u in range(4)]

    def wperm_thunks(piece, j):
        m = (piece >> 2) & 1
        wt = wtmp.at[j]

        def load():
            wt[0:DF, :] = wri[piece, :, 128 * j:128 * j + 128].astype(f32)

        def one(g):
            def run():
                if g == 0:
                    t = jnp.concatenate([wt[pl.ds(0, 64, stride=5), :], wt[320:328, :],
                                         jnp.zeros((56, 128), f32)], axis=0)
                else:
                    t = jnp.concatenate([wt[pl.ds(g, 64, stride=5), :],
                                         wt[pl.ds(5 - g, 64, stride=5), :]], axis=0)
                y = t.T
                sub = wf.at[3 * m + g, pl.ds(pl.multiple_of((piece & 3) * 32, 32), 16 * WPITCH - 96)]
                for k in range(8):
                    for hf in range(2):
                        sub[pl.ds(8 * j + k + 8 * hf * WPITCH, 8, stride=WPITCH), :] = (
                            y[16 * k + 8 * hf:16 * k + 8 * hf + 8])
            return run
        return [load] + [one(g) for g in range(3)]

    def half_pass(cid, half, fill, zero, timed=()):
        nre = CFG["pro_nre"]
        toks = None
        for k, f in enumerate(batch_thunks(cid)[16 * half:16 * half + 16]):
            f(toks)
            toks = {}
            for pos, f in zip((0, 4, 1, 6), [f for at, f in timed if at == k]):
                toks[pos] = f()
            if fill is not None:
                for n, r in enumerate(r for r in range(40) if r * nre // 40 == k):
                    relayout(r, fill, 1 - half)
                    toks[CFG["re_pos"][n]] = (wb, wa)[half][12 + zero, 0:8, :]

    def ln_parts(bb, zero):
        def part(j):
            set_input(bb, load_x(bb, 4 * j, 4), None, 4 * j)
            return pltpu.bitcast(xa[32 + zero, 0:8, 0:128], u32)
        return [functools.partial(part, j) for j in range(4)]

    def perm_parts(piece, zero):
        def part(fs):
            for f in fs:
                f()
            return pltpu.bitcast(wf[5 + zero, 16 * WPITCH:16 * WPITCH + 8, :], u32)
        out = []
        for j in range(4):
            th = wperm_thunks(piece, j)
            out += [functools.partial(part, th[0:2]), functools.partial(part, th[2:3]),
                    functools.partial(part, th[3:4])]
        return out

    def pro0():
        for u in range(4):
            cp_x(4 * u + 3).wait()
        for u in range(4):
            set_input(4 * u + 3, load_x(4 * u + 3), u)
        cp_w(0).wait()
        zero = zero_ref[0]
        for i in range(40):
            relayout(i, 0, 0)
        half_pass(0, 0, zero, zero)

    def pro1(it, carry):
        bb = body_chunk(it)
        with jax.named_scope("pro1_wait"):
            cp_w(it + 1).wait()

            @pl.when(it >= 3)
            def _():
                cp_f(it - 3).wait()
            cp_x(bb).wait()
        piece = jnp.where(it >= 3, it - 3, 8)
        zero = it >> 4
        timed = sorted(list(zip(CFG["ln_at"], ln_parts(bb, zero)))
                       + list(zip(CFG["perm_at"], perm_parts(piece, zero))), key=lambda x: x[0])
        half_pass(it, 1, it + 1, zero, [x for x in timed if x[0] < 16])
        half_pass(it + 1, 0, it + 1, zero, [(k - 16, f) for k, f in timed if k >= 16])
        return carry

    def pro2():
        cp_x(body_chunk(11)).wait()
        for cp in cp_rest:
            cp.wait()
        zero = zero_ref[0]
        half_pass(11, 1, None, zero, list(zip(CFG["ln_at2"], ln_parts(body_chunk(11), zero))))

    if full:
        with jax.named_scope("pro0"):
            pro0()
        _loop("pro1", 0, 11, pro1, 0)
        with jax.named_scope("pro2"):
            pro2()

    scale = DH ** -0.5

    def wo_dot(hh, oo):
        return [_dot(oo, wo_t[j, 128 * hh:128 * hh + 128, :]) for j in range(5)]

    def addl(acc, res):
        return res if acc is None else [a + b for a, b in zip(acc, res)]

    def group(g, mem):
        for ph in range(4):
            h = jnp.concatenate([mem, xa[16 + g, 32 * ph:32 * ph + 24, :]], axis=0).astype(bf16)
            pr, sm, oos = {}, {}, {}
            lat_s, lat_pv, lat_wo, v_delay, n_first, n_last = CFG["steps"][ph]

            def stacked(p, m):
                tails = [qb[g, ph, 32 * m + 2 * p + e] for e in range(2)]
                return jnp.concatenate([pr[p, m, 0], pr[p, m, 1]] + tails, axis=0).astype(bf16)

            def scores(p):
                sc = lax.dot_general(stacked(p, 0), stacked(p, 1), (((1,), (1,)), ((), ())),
                                     preferred_element_type=f32)
                fill = fill_ref[...]
                sc = jnp.where(fill == 0.0, sc * scale, fill)
                mx = jnp.max(sc, axis=-1, keepdims=True)
                e = jnp.exp(sc - mx)
                rl = pl.reciprocal(jnp.sum(e, axis=-1, keepdims=True), approx=True)
                sm[p] = (e * rl).astype(bf16)

            def pv(p):
                o = _dot(sm[p], stacked(p, 2))
                for e in range(2):
                    qb[g, ph, 2 * p + e] = o[64 + 8 * e:72 + 8 * e]
                    oos[2 * p + e] = o[32 * e:32 * e + 32].astype(bf16)

            keyed = []
            for p in range(NPAIR):
                keyed += [(4 * p + 2 * m + e, (p, m, e)) for m in range(2) for e in range(2)]
                keyed += [(4 * p + 3.5 + v_delay, (p, 2, e)) for e in range(2)]
            bulk = [x for _, x in sorted(keyed, key=lambda kv: kv[0])]
            acc, t, nwo, pend, ready = None, 0.0, 0, [], []
            if n_first:
                first, bulk = bulk[:n_first], bulk[n_first:]
                for kt in range(5):
                    for p, m, e in first:
                        w = wtile(4 * m + (p >> 2), p & 3, e)[64 * kt:64 * kt + 64]
                        y = _dot(h[:, 128 * kt:128 * kt + 128], _bf(w))
                        pr[p, m, e] = y if kt == 0 else pr[p, m, e] + y
                t = float(len(first))
                pend = [(t + lat_s, "S", p) for p, m, e in first if m == 1 and e == 1]
            while nwo < H - n_last or pend:
                pend.sort()
                if pend and pend[0][0] <= t:
                    _, kind, p = pend.pop(0)
                    if kind == "S":
                        scores(p)
                        pend.append((t + lat_pv, "V", p))
                    else:
                        pv(p)
                        ready += [(t + lat_wo, 2 * p + e) for e in range(2)]
                    t += 0.5
                elif bulk:
                    p, m, e = bulk.pop(0)
                    pr[p, m, e] = _dot(h, _bf(wtile(4 * m + (p >> 2), p & 3, e)))
                    t += 1
                    if m == 1 and e == 1:
                        pend.append((t + lat_s, "S", p))
                elif ready and ready[0][0] <= t and nwo < H - n_last:
                    _, hh = ready.pop(0)
                    acc = addl(acc, wo_dot(hh, oos[hh]))
                    t += 1
                    nwo += 1
                else:
                    t += 0.5
            for j in range(5):
                for _, hh in ready:
                    acc[j] = acc[j] + _dot(oos[hh], wo_t[j, 128 * hh:128 * hh + 128, :])
            out = jnp.concatenate(acc, axis=1)
            xa[16 + g, 32 * ph:32 * ph + 24, :] = out[8:32]
            mem = _round_bf16(out[0:8])
        return mem

    def dfwd_thunks(rows, tail):
        st = {}

        def pre():
            o = to[...] if tail else xa[16:32, rows, :]
            x = _round_bf16(xa[0:16, rows, :] + o)
            xb[:, rows, :] = x
            y = _layernorm(x.reshape(128, DM))
            x0, x1, x2, x3, x4 = [y[:, 128 * a:128 * a + 128] for a in range(5)]
            t1, t2, t3, t4 = x1 + x4, x2 + x3, x1 - x4, x2 - x3
            t = t1 + t2
            m, n = x0 - 0.25 * t, R5_D * (t1 - t2)
            st["u"] = [x0 + t, (m + n, t3 + R5_R * t4), (m - n, R5_R * t3 - t4)]

        def part(g):
            def run():
                if g == 0:
                    pre()
                    u0 = st["u"][0].astype(bf16)
                    zr, zi = _dot(u0, _bf(small[0])), _dot(u0, _bf(small[1]))
                else:
                    a, b = st["u"][g]
                    k, kb, ka = [_dot(v.astype(bf16), _bf(small[3 * g - 1 + i]))
                                 for i, v in enumerate((a + b, b, a))]
                    zr, zi = k + kb, ka - _mu() * k
                ys = [(zr[8 * a:8 * a + 8], zi[8 * a:8 * a + 8]) for a in range(16)]
                if g < 2 or not CFG["late_g2"]:
                    ys = _fft16(ys, -1)
                for a in range(16):
                    zs[g][0, a, rows, :] = ys[a][0]
                    zs[g][1, a, rows, :] = ys[a][1]
            return run
        return [part(g) for g in range(3)]

    def post(u, carry):
        base = pl.multiple_of(32 * u, 32)
        side = []
        for q in range(4):
            side += dfwd_thunks(pl.ds(base + 8 * q, 8), q == 3)
        side = [side[i] for i in CFG["post_order"]]
        k = 0
        at = list(CFG["post_at"])
        for js in CFG["post_js"]:
            acc = None
            for hh in range(H):
                oo = qb[:, u, hh].reshape(128, 128).astype(bf16)
                acc = addl(acc, [_dot(oo, wo_t[j, 128 * hh:128 * hh + 128, :]) for j in js])
                k += len(js)
                while at and at[0] <= k:
                    at.pop(0)
                    side.pop(0)()
            for j, y in zip(js, acc):
                to[:, :, 128 * j:128 * j + 128] = y.reshape(16, 8, 128)
        for f in side:
            f()
        return carry

    def spectral(zero):
        def fence(z):
            return z[0, zero, 128:ZPITCH, :]

        def radix_inv(g, bb, sign=1):
            z = zs[g]
            toks = []

            def emit(q, y):
                for p in range(4):
                    z[0, q + 4 * p, chunk(bb), :] = y[p][0]
                    z[1, q + 4 * p, chunk(bb), :] = y[p][1]
                toks.append(fence(z))
            _fft16([(z[0, a, chunk(bb), :], z[1, a, chunk(bb), :]) for a in range(16)], sign, emit)
            return toks

        ys = {}

        def fwd(g, k2, toks):
            z = zs[g]
            ur, ui = z[0, k2, 0:64, :], z[1, k2, 0:64, :]
            tr, ti = _twiddle((z[0, k2, 64:128, :], z[1, k2, 64:128, :]), k2, 32, -1)
            for hf in range(2):
                v = _ilv(ur + tr, ui + ti) if hf == 0 else _ilv(ur - tr, ui - ti)
                lhs = _with_tokens(emat[k2 + 16 * hf], toks if hf == 0 else None)
                xr, xi = _dilv(_dot(_bf(lhs), v.astype(bf16)))
                ys["x", 16 * g + k2] = xr
                wr = wf[g, pl.ds(k2 * WPITCH + hf, 64, stride=2), :]
                wi = wf[g + 3, pl.ds(k2 * WPITCH + hf, 64, stride=2), :]
                ys[g, k2, hf] = _ilv(xr * wr - xi * wi, xr * wi + xi * wr).astype(bf16)

        def inv(g, k2):
            z = zs[g]
            t0 = _dot(_bf(emat[32 + k2]), ys.pop((g, k2, 0)))
            t1 = _dot(_bf(emat[48 + k2]), ys.pop((g, k2, 1)))
            z[0, k2, 0:64, :], z[1, k2, 0:64, :] = _dilv(t0 + t1)
            z[0, k2, 64:128, :], z[1, k2, 64:128, :] = _twiddle(_dilv(t0 - t1), k2, 32, 1)

        units = [(g, k2) for g in range(3) for k2 in range(16)]
        toks = None
        for i in range(len(units) + 3):
            if i < len(units):
                fwd(*units[i], toks)
            if i >= 3:
                inv(*units[i - 3])
            toks = None
            if CFG["late_g2"] and i in CFG["fwd_at"]:
                t4 = radix_inv(2, CFG["fwd_at"].index(i), -1)
                toks = {3 + j: pltpu.bitcast(t, u32) for j, t in enumerate(t4)}
            if i in CFG["inv_at"]:
                n = CFG["inv_at"].index(i)
                back, r = CFG["rel"]
                zs[n // 16][1, zero, 128:ZPITCH, :] = ys["x", min(i - back, 47)][8 * r:8 * r + 8]
                toks = {3 + j: pltpu.bitcast(t, u32) for j, t in enumerate(radix_inv(n // 16, n % 16))}

    def dinv_thunks(bb, finish):
        st = {}

        def part(g):
            def run():
                z = zs[g]
                ys = [(z[0, a, chunk(bb), :], z[1, a, chunk(bb), :]) for a in range(16)]
                if g >= CFG["inv_groups"]:
                    ys = _fft16(ys, 1)
                tr = jnp.concatenate([y[0] for y in ys], axis=0)
                ti = jnp.concatenate([y[1] for y in ys], axis=0)
                if g == 0:
                    st[0] = _dot(tr.astype(bf16), _bf(small[8])) + _dot(ti.astype(bf16), _bf(small[9]))
                else:
                    k, ki, kr = [_dot(v.astype(bf16), _bf(small[7 + 3 * g + i]))
                                 for i, v in enumerate((tr + _mu() * ti, ti, tr))]
                    st[2 * g - 1], st[2 * g] = k + ki, k + kr
            return run

        def fin():
            p0, p1, q1, p2, q2 = [st[j] for j in range(5)]
            t = p1 + p2
            m, n = p0 - 0.25 * t, R5_D * (p1 - p2)
            e1, e2 = m + n, m - n
            o1, o2 = q1 + R5_R * q2, R5_R * q1 - q2
            y = jnp.concatenate([p0 + t, e1 - o1, e2 - o2, e2 + o2, e1 + o1], axis=1)
            finish(xb[:, chunk(bb), :].reshape(128, DM) + y)
        return [part(0), part(1), part(2), fin]

    def out_copy(bb):
        return pltpu.make_async_copy(xin.at[:, bb], out_hbm.at[:, bb], osem.at[bb])

    def layer(li, carry0):
        if full or CFG["only"] == "group":
            _loop("step", 0, 16, group, mem_ref[...].astype(f32))
        if full or CFG["only"] == "spec":
            _loop("post", 0, 4, post, 0, unroll=CFG["post_unroll"])

            with jax.named_scope("spectral"):
                spectral((li >> 1))
        if not full:
            return carry0

        @pl.when(li == 0)
        def _():
            with jax.named_scope("dinv_tails"):
                th = [dinv_thunks(4 * u + 3, functools.partial(
                    lambda u, x: set_input(4 * u + 3, _round_bf16(x), u), u)) for u in range(4)]
                for i in range(5):
                    if i < 4:
                        for f in th[i][:3]:
                            f()
                    if i >= 1:
                        th[i - 1][3]()

            def batch(it, carry):
                bb = body_chunk(it)
                side = dinv_thunks(bb, lambda x: set_input(bb, _round_bf16(x), None))
                for k, f in enumerate(batch_thunks(it)):
                    f()
                    if k in CFG["dinv_at"]:
                        side.pop(0)()
                return carry
            _loop("batch", 0, 12, batch, 0, unroll=CFG["batch_unroll"])

        @pl.when(li == 1)
        def _():
            with jax.named_scope("dinv_out"):
                def store_out(bb, x):
                    xin[:, bb] = x.reshape(16, 8, DM).astype(bf16)
                    out_copy(bb).start()
                th = [dinv_thunks(bb, functools.partial(store_out, bb)) for bb in range(16)]
                for i in range(17):
                    if i < 16:
                        for f in th[i][:3]:
                            f()
                    if i >= 1:
                        th[i - 1][3]()
                for bb in range(16):
                    out_copy(bb).wait()
        return carry0

    if CFG["only"] != "pro":
        lax.fori_loop(0, 2, layer, 0)
    else:
        zero = zero_ref[0]
        xin[0, 0, :, 0:128] = (qb[zero, 0, 0] + wf[zero, 0:8, :] + xa[zero, 0:8, 0:128]).astype(bf16)
        out_copy(0).start()
        out_copy(0).wait()


@functools.partial(jax.jit, static_argnames=("A_seg_len",))
def pallas_interleave_layers__memory_aug_recurrent_mem_tr__spectral_gfnet__prompt_kernel(
    A_x, A_mem0, A_Wq, A_Wk, A_Wv, A_Wo, A_seg_len, B_x, B_w_r, B_w_i,
):
    assert A_seg_len == SEG and A_x.shape == (1, S, DM)
    small, emat = _tables()
    hbm = pl.BlockSpec(memory_space=pltpu.HBM)
    out = pl.pallas_call(
        _kernel,
        out_shape=jax.ShapeDtypeStruct((16, 16, 8, DM), bf16),
        in_specs=[hbm] * 10,
        out_specs=hbm,
        scratch_shapes=[
            pltpu.VMEM((16, 16, 8, DM), bf16),
            pltpu.VMEM((33, 128, DM), f32),
            pltpu.VMEM((16, 128, DM), f32),
            pltpu.VMEM((16, 8, DM), f32),
            pltpu.VMEM((12, 2, 320, 8, DH), bf16),
            pltpu.VMEM((13, 8 * HPITCH, 128), u32),
            pltpu.VMEM((13, 8 * HPITCH, 128), u32),
            pltpu.VMEM((5, H * DH, 128), bf16),
            pltpu.VMEM((16, 4, 96, 8, 128), f32),
            pltpu.VMEM((4, 5, 64, 128), u32),
            pltpu.VMEM((2, 16, ZPITCH, 128), f32),
            pltpu.VMEM((2, 16, ZPITCH, 128), f32),
            pltpu.VMEM((2, 16, ZPITCH, 128), f32),
            pltpu.VMEM((6, 16 * WPITCH + 32, 128), f32),
            pltpu.VMEM((9, DF, 512), bf16),
            pltpu.VMEM((4, 328, 128), f32),
            pltpu.VMEM((SMALL_TILES, 64, 128), u32),
            pltpu.VMEM((64, 64, 128), u32),
            pltpu.VMEM((80, 80), f32),
            pltpu.VMEM((MEM, DM), bf16),
            pltpu.SMEM((1,), jnp.int32),
            pltpu.SemaphoreType.DMA((46,)),
            pltpu.SemaphoreType.DMA((16,)),
        ],
        compiler_params=pltpu.CompilerParams(vmem_limit_bytes=120 * 1024 * 1024,
                                             disable_semaphore_checks=True),
    )(
        A_x.reshape(16, 16, 8, DM), A_mem0.reshape(MEM, DM),
        *[w.reshape(2, 320, H, DH) for w in (A_Wq, A_Wk, A_Wv)], A_Wo.reshape(H * DH, DM), B_w_r.T, B_w_i.T,
        jnp.asarray(small), jnp.asarray(emat),
    )
    return out.reshape(1, S, DM)
```

```python
import functools
import math

import jax
import jax.numpy as jnp
import numpy as np
from jax import lax
import jax.experimental.pallas as pl
import jax.experimental.pallas.tpu as pltpu

f32, bf16, u32 = jnp.float32, jnp.bfloat16, jnp.uint32

S, DM, H, DH, MEM, SEG = 2048, 640, 32, 128, 8, 32
NSEG = S // SEG
NPAIR = H // 2
DF = DM // 2 + 1
EPS = 1e-5
WPITCH = 132

HPITCH = 164
ZPITCH = 136

S1 = math.sin(2 * math.pi / 5)
R5_D = (math.cos(2 * math.pi / 5) - math.cos(4 * math.pi / 5)) / 2
R5_R = math.sin(4 * math.pi / 5) / S1


def _to_bf16_bits(a):
    u = np.ascontiguousarray(a, dtype=np.float32).view(np.uint32).astype(np.uint64)
    return ((u + 0x7FFF + ((u >> 16) & 1)) >> 16).astype(np.uint32)


def _pack_rows(a):
    b = _to_bf16_bits(a)
    return b[..., 0::2, :] | (b[..., 1::2, :] << 16)


@functools.lru_cache(maxsize=None)
def _tables():
    b = np.arange(128)
    l0 = np.arange(0, DF, 5)
    l1 = np.concatenate([np.arange(1, 320, 5), np.arange(4, 320, 5)])
    l2 = np.concatenate([np.arange(2, 320, 5), np.arange(3, 320, 5)])
    sg = np.concatenate([np.ones(64), -np.ones(64)])

    def th(l):
        return 2 * np.pi * ((b[:, None] * l[None, :]) % DM) / DM

    sc = 1.0 / (S * DM)
    fw = np.zeros((8, 128, 128))
    iw = np.zeros((8, 128, 128))
    t = th(l0)
    cl = np.full((65, 1), 2.0)
    cl[0] = cl[-1] = 1.0
    fw[0, :, :65], fw[1, :, :65] = np.cos(t), -np.sin(t)
    iw[0, :65], iw[1, :65] = cl * np.cos(t.T) * sc, -cl * np.sin(t.T) * sc
    if CFG["pack_f"]:
        fw[0, :, 65:] = fw[1, :, 1:64]
    if CFG["pack_i"]:
        iw[0, 65:] = iw[1, 1:64]
    mu = S1 * sg
    for g, l in ((1, l1), (2, l2)):
        t = th(l)
        c, s = np.cos(t), np.sin(t)
        fw[3 * g - 1:3 * g + 2] = c, -mu * s - c, mu * c - s
        iw[3 * g - 1:3 * g + 2] = [2 * sc * m.T for m in (c, -s - mu * c, mu * s - c)]
    n = np.arange(64)
    order = np.concatenate([np.concatenate([np.arange(8) + 8 * j, np.arange(8) + 8 * j + 64])
                            for j in range(8)])
    e = np.zeros((2, 32, 128, 128))
    for k2 in range(32):
        t = 2 * np.pi * (((32 * n[:, None] + k2) * n[None, :]) % S) / S
        er, ei = np.cos(t), -np.sin(t)
        m = np.block([[er, -ei], [ei, er]])[order][:, order]
        e[0, k2], e[1, k2] = m, m.T
    small = np.concatenate([_pack_rows(fw), _pack_rows(iw)], axis=0)
    return small, _pack_rows(e).reshape(64, 64, 128)


SMALL_TILES = 16


def _loop(name, lo, hi, body, init, **kw):
    with jax.named_scope(name):
        return lax.fori_loop(lo, hi, body, init, **kw)


def _bf(x):
    return pltpu.bitcast(x, bf16)


def _dot(a, b):
    return jnp.dot(a, b, preferred_element_type=f32)


def _round_bf16(x):
    return x.astype(bf16).astype(f32)


def _layernorm(x):
    m = jnp.mean(x, axis=-1, keepdims=True)
    xc = x - m
    v = jnp.mean(xc * xc, axis=-1, keepdims=True)
    return xc * lax.rsqrt(v + EPS)


def _fft4(x, sign):
    (ar, ai), (br, bi), (cr, ci), (dr, di) = x
    t0r, t0i, t1r, t1i = ar + cr, ai + ci, ar - cr, ai - ci
    t2r, t2i, t3r, t3i = br + dr, bi + di, br - dr, bi - di
    y0, y2 = (t0r + t2r, t0i + t2i), (t0r - t2r, t0i - t2i)
    p, q = (t1r + t3i, t1i - t3r), (t1r - t3i, t1i + t3r)
    return [y0, p, y2, q] if sign < 0 else [y0, q, y2, p]


def _twiddle(z, n, period, sign):
    zr, zi = z
    n = n % period
    if n == 0:
        return z
    if 4 * n == period:
        return (-zi, zr) if sign > 0 else (zi, -zr)
    c, s = math.cos(2 * math.pi * n / period), sign * math.sin(2 * math.pi * n / period)
    if (8 * n) % period == 0:
        a, d = zr + zi, zr - zi
        if c * s > 0:
            return (d * c, a * c)
        return (a * c, d * s)
    return (zr * c - zi * s, zr * s + zi * c)


def _mu():
    lane = lax.broadcasted_iota(jnp.int32, (1, 128), 1)
    return jnp.where(lane < 64, S1, -S1).astype(f32)


def _ilv(r, i):
    n = r.shape[0] // 8
    return jnp.concatenate([r.reshape(n, 8, 128), i.reshape(n, 8, 128)], axis=1).reshape(16 * n, 128)


def _dilv(x):
    n = x.shape[0] // 16
    x = x.reshape(n, 16, 128)
    return x[:, :8].reshape(8 * n, 128), x[:, 8:].reshape(8 * n, 128)


def _with_tokens(x, toks):
    if not toks:
        return x
    return jnp.concatenate(
        [x[8 * j:8 * j + 8] | toks[j] if j in toks else x[8 * j:8 * j + 8]
         for j in range(x.shape[0] // 8)], axis=0)


def _fft16(x, sign, emit=None):
    cols = [_fft4([x[4 * j + r] for j in range(4)], sign) for r in range(4)]
    out = [None] * 16
    for q in range(4):
        y = _fft4([_twiddle(cols[r][q], r * q, 16, sign) for r in range(4)], sign)
        for p in range(4):
            out[q + 4 * p] = y[p]
        if emit is not None:
            emit(q, y)
    return out


CFG = dict(steps=((4.5, 16.5, 6, 4, 0, 8), (5, 16.5, 5, 7, 8, 12), (5, 16.5, 6, 6, 8, 12), (5, 16.5, 8, 7, 8, 0)),
           post_js=((0, 1, 2), (3, 4)),
           post_order=(0, 1, 6, 3, 4, 5, 8, 2, 7, 9, 10, 11), post_at=(32, 46, 76, 108),
           tails_order=((1, 2, 0), 5), out_order=((1, 2, 0), 5), pack_f=True, pack_i=True,
           inv_at=tuple(range(28, 44)), inv_groups=1, inv_lag=4, tok_pos=(4, 5, 6, 7),
           fwd_at=(7, 8, 9, 10, 12, 13, 14, 16, 17, 18, 20, 21, 22, 24, 25, 26), rel=(0, 1), dinv_at=(8, 9, 10, 11), batch_unroll=2, post_unroll=1,
           pro_nre=14, re_pos=(3, 5, 7), ln_at=(22, 29, 31, 31), ln_at2=(4, 7, 10, 13),
           perm_at=tuple(range(12, 24)), only=None)


def _interleave(main, side):
    n, k = len(main), 0
    for i, f in enumerate(main):
        f()
        while k < len(side) and (k + 1) * n <= (i + 1) * len(side):
            side[k]()
            k += 1
    for f in side[k:]:
        f()


def _kernel(x_hbm, mem_hbm, wq_hbm, wk_hbm, wv_hbm, wo_hbm, wr_hbm, wi_hbm,
            small_hbm, e_hbm, out_hbm,
            xin, xa, xb, to, raw, wa, wb, wo_t, qb, hl, z0, z1, z2, wf,
            wri, wtmp, small, emat, fill_ref, mem_ref, zero_ref, sem, osem):
    zs = (z0, z1, z2)
    w_hbm = (wq_hbm, wk_hbm, wv_hbm)

    def body_chunk(i):
        return 4 * (i & 3) + (i >> 2)

    def cp_w(i):
        src = w_hbm[i >> 2].at[:, :, pl.ds(8 * (i & 3), 8), :] if isinstance(i, int) else raw.at[i]
        return pltpu.make_async_copy(src, raw.at[i], sem.at[i])

    def cp_x(bb):
        return pltpu.make_async_copy(x_hbm.at[:, bb], xin.at[:, bb], sem.at[12 + bb])

    def cp_f(i):
        src = ((wr_hbm, wi_hbm)[i >> 2].at[:, pl.ds(512 * (i & 3), 512)]
               if isinstance(i, int) else wri.at[i])
        return pltpu.make_async_copy(src, wri.at[i], sem.at[36 + i])

    cp_rest = [pltpu.make_async_copy(wo_hbm.at[:, pl.ds(128 * j, 128)], wo_t.at[j], sem.at[28 + j])
               for j in range(5)]
    cp_rest += [pltpu.make_async_copy(mem_hbm, mem_ref, sem.at[33]),
                pltpu.make_async_copy(small_hbm, small, sem.at[44]),
               pltpu.make_async_copy(e_hbm, emat, sem.at[45])]

    full = CFG["only"] in (None, "pro")
    for u in range(4 if full else 0):
        cp_x(4 * u + 3).start()
    if full:
        cp_w(0).start()
    for i in range(12 if full else 0):
        if i < 11:
            cp_w(i + 1).start()
        cp_x(body_chunk(i)).start()
        if 3 <= i < 11:
            cp_f(i - 3).start()
    for cp in cp_rest if full else ():
        cp.start()

    zero_ref[0] = 0

    r = lax.broadcasted_iota(jnp.int32, (80, 80), 0)
    c = lax.broadcasted_iota(jnp.int32, (80, 80), 1)

    def head(i):
        return jnp.where(i < 64, i // 32, (i - 64) // 8)

    def pos(i):
        return jnp.where(i < 64, i % 32, 32 + (i - 64) % 8)

    ok = (pos(r) < MEM) | (pos(r) >= pos(c))
    fill_ref[...] = jnp.where(head(r) == head(c), jnp.where(ok, 0.0, -1e9), -jnp.inf).astype(f32)
    wtmp[:, 320:328, :] = jnp.zeros((4, 8, 128), f32)
    xa[32, 0:8, 0:128] = jnp.zeros((8, 128), f32)
    wa[12, 0:8, :] = jnp.zeros((8, 128), u32)
    wb[12, 0:8, :] = jnp.zeros((8, 128), u32)
    wf[5, 16 * WPITCH:16 * WPITCH + 8, :] = jnp.zeros((8, 128), f32)
    for z in zs:
        z[0, 0, 128:ZPITCH, :] = jnp.zeros((8, 128), f32)

    def chunk(bb):
        if isinstance(bb, int):
            return slice(8 * bb, 8 * bb + 8)
        return pl.ds(pl.multiple_of(8 * bb, 8), 8)

    def set_input(bb, x, tail_u, a0=0):
        n = x.shape[0] // 8
        xa[a0:a0 + n, chunk(bb), :] = x.reshape(n, 8, DM)
        y = _layernorm(x)
        if tail_u is None:
            xa[16 + a0:16 + a0 + n, chunk(bb), :] = y.reshape(n, 8, DM)
        else:
            yb = y.astype(bf16)
            for kt in range(5):
                hl[tail_u, kt] = pltpu.bitcast(yb[:, 128 * kt:128 * kt + 128], u32)

    def load_x(bb, a0=0, n=16):
        return xin[a0:a0 + n, bb].astype(f32).reshape(8 * n, DM)

    def wtile(cid, j, e):
        w = (wa, wb)[e]
        return jnp.concatenate([w[cid, (4 * hf + j) * HPITCH:(4 * hf + j) * HPITCH + 160, :]
                                for hf in range(2)], axis=0)

    def relayout(i, cid, e):
        for r in range(4 * i, 4 * i + 4):
            a, b = [pltpu.bitcast(raw[cid, :, d].reshape(16, 128), u32) for d in (2 * r, 2 * r + 1)]
            v = (a & 0xFFFF) | (b << 16) if e == 0 else (a >> 16) | (b & jnp.uint32(0xFFFF0000))
            (wa, wb)[e][cid, pl.ds(r, 8, stride=HPITCH), :] = v

    def batch_thunks(cid):
        def one(j, u, e):
            def run(toks=None):
                lhs = jnp.concatenate(
                    [_bf(_with_tokens(hl[u, kt], toks if kt == 0 else None)) for kt in range(5)], axis=1)
                qb[:, u, 8 * cid + 2 * j + e] = _dot(lhs, _bf(wtile(cid, j, e))).reshape(16, 8, 128)
            return run
        return [one(j, u, e) for e in range(2) for j in range(4) for u in range(4)]

    def wperm_thunks(piece, j):
        m = (piece >> 2) & 1
        wt = wtmp.at[j]

        def load():
            wt[0:DF, :] = wri[piece, :, 128 * j:128 * j + 128].astype(f32)

        def one(g):
            def run():
                if g == 0:
                    t = jnp.concatenate([wt[pl.ds(0, 64, stride=5), :], wt[320:328, :],
                                         jnp.zeros((56, 128), f32)], axis=0)
                else:
                    t = jnp.concatenate([wt[pl.ds(g, 64, stride=5), :],
                                         wt[pl.ds(5 - g, 64, stride=5), :]], axis=0)
                y = t.T
                sub = wf.at[3 * m + g, pl.ds(pl.multiple_of((piece & 3) * 32, 32), 16 * WPITCH - 96)]
                for k in range(8):
                    for hf in range(2):
                        sub[pl.ds(8 * j + k + 8 * hf * WPITCH, 8, stride=WPITCH), :] = (
                            y[16 * k + 8 * hf:16 * k + 8 * hf + 8])
            return run
        return [load] + [one(g) for g in range(3)]

    def half_pass(cid, half, fill, zero, timed=()):
        nre = CFG["pro_nre"]
        toks = None
        for k, f in enumerate(batch_thunks(cid)[16 * half:16 * half + 16]):
            f(toks)
            toks = {}
            for pos, f in zip((0, 4, 1, 6), [f for at, f in timed if at == k]):
                toks[pos] = f()
            if fill is not None:
                for n, r in enumerate(r for r in range(40) if r * nre // 40 == k):
                    relayout(r, fill, 1 - half)
                    toks[CFG["re_pos"][n]] = (wb, wa)[half][12 + zero, 0:8, :]

    def ln_parts(bb, zero):
        def part(j):
            set_input(bb, load_x(bb, 4 * j, 4), None, 4 * j)
            return pltpu.bitcast(xa[32 + zero, 0:8, 0:128], u32)
        return [functools.partial(part, j) for j in range(4)]

    def perm_parts(piece, zero):
        def part(fs):
            for f in fs:
                f()
            return pltpu.bitcast(wf[5 + zero, 16 * WPITCH:16 * WPITCH + 8, :], u32)
        out = []
        for j in range(4):
            th = wperm_thunks(piece, j)
            out += [functools.partial(part, th[0:2]), functools.partial(part, th[2:3]),
                    functools.partial(part, th[3:4])]
        return out

    def pro0():
        for u in range(4):
            cp_x(4 * u + 3).wait()
        for u in range(4):
            set_input(4 * u + 3, load_x(4 * u + 3), u)
        cp_w(0).wait()
        zero = zero_ref[0]
        for i in range(40):
            relayout(i, 0, 0)
        half_pass(0, 0, zero, zero)

    def pro1(it, carry):
        bb = body_chunk(it)
        with jax.named_scope("pro1_wait"):
            cp_w(it + 1).wait()

            @pl.when(it >= 3)
            def _():
                cp_f(it - 3).wait()
            cp_x(bb).wait()
        piece = jnp.where(it >= 3, it - 3, 8)
        zero = it >> 4
        timed = sorted(list(zip(CFG["ln_at"], ln_parts(bb, zero)))
                       + list(zip(CFG["perm_at"], perm_parts(piece, zero))), key=lambda x: x[0])
        half_pass(it, 1, it + 1, zero, [x for x in timed if x[0] < 16])
        half_pass(it + 1, 0, it + 1, zero, [(k - 16, f) for k, f in timed if k >= 16])
        return carry

    def pro2():
        cp_x(body_chunk(11)).wait()
        for cp in cp_rest:
            cp.wait()
        zero = zero_ref[0]
        half_pass(11, 1, None, zero, list(zip(CFG["ln_at2"], ln_parts(body_chunk(11), zero))))

    if full:
        with jax.named_scope("pro0"):
            pro0()
        _loop("pro1", 0, 11, pro1, 0)
        with jax.named_scope("pro2"):
            pro2()

    scale = DH ** -0.5

    def wo_dot(hh, oo):
        return [_dot(oo, wo_t[j, 128 * hh:128 * hh + 128, :]) for j in range(5)]

    def addl(acc, res):
        return res if acc is None else [a + b for a, b in zip(acc, res)]

    def group(g, mem):
        for ph in range(4):
            h = jnp.concatenate([mem, xa[16 + g, 32 * ph:32 * ph + 24, :]], axis=0).astype(bf16)
            pr, sm, oos = {}, {}, {}
            lat_s, lat_pv, lat_wo, v_delay, n_first, n_last = CFG["steps"][ph]

            def stacked(p, m):
                tails = [qb[g, ph, 32 * m + 2 * p + e] for e in range(2)]
                return jnp.concatenate([pr[p, m, 0], pr[p, m, 1]] + tails, axis=0).astype(bf16)

            def scores(p):
                sc = lax.dot_general(stacked(p, 0), stacked(p, 1), (((1,), (1,)), ((), ())),
                                     preferred_element_type=f32)
                fill = fill_ref[...]
                sc = jnp.where(fill == 0.0, sc * scale, fill)
                mx = jnp.max(sc, axis=-1, keepdims=True)
                e = jnp.exp(sc - mx)
                rl = pl.reciprocal(jnp.sum(e, axis=-1, keepdims=True), approx=True)
                sm[p] = (e * rl).astype(bf16)

            def pv(p):
                o = _dot(sm[p], stacked(p, 2))
                for e in range(2):
                    qb[g, ph, 2 * p + e] = o[64 + 8 * e:72 + 8 * e]
                    oos[2 * p + e] = o[32 * e:32 * e + 32].astype(bf16)

            keyed = []
            for p in range(NPAIR):
                keyed += [(4 * p + 2 * m + e, (p, m, e)) for m in range(2) for e in range(2)]
                keyed += [(4 * p + 3.5 + v_delay, (p, 2, e)) for e in range(2)]
            bulk = [x for _, x in sorted(keyed, key=lambda kv: kv[0])]
            acc, t, nwo, pend, ready = None, 0.0, 0, [], []
            if n_first:
                first, bulk = bulk[:n_first], bulk[n_first:]
                for kt in range(5):
                    for p, m, e in first:
                        w = wtile(4 * m + (p >> 2), p & 3, e)[64 * kt:64 * kt + 64]
                        y = _dot(h[:, 128 * kt:128 * kt + 128], _bf(w))
                        pr[p, m, e] = y if kt == 0 else pr[p, m, e] + y
                t = float(len(first))
                pend = [(t + lat_s, "S", p) for p, m, e in first if m == 1 and e == 1]
            while nwo < H - n_last or pend:
                pend.sort()
                if pend and pend[0][0] <= t:
                    _, kind, p = pend.pop(0)
                    if kind == "S":
                        scores(p)
                        pend.append((t + lat_pv, "V", p))
                    else:
                        pv(p)
                        ready += [(t + lat_wo, 2 * p + e) for e in range(2)]
                    t += 0.5
                elif bulk:
                    p, m, e = bulk.pop(0)
                    pr[p, m, e] = _dot(h, _bf(wtile(4 * m + (p >> 2), p & 3, e)))
                    t += 1
                    if m == 1 and e == 1:
                        pend.append((t + lat_s, "S", p))
                elif ready and ready[0][0] <= t and nwo < H - n_last:
                    _, hh = ready.pop(0)
                    acc = addl(acc, wo_dot(hh, oos[hh]))
                    t += 1
                    nwo += 1
                else:
                    t += 0.5
            for j in range(5):
                for _, hh in ready:
                    acc[j] = acc[j] + _dot(oos[hh], wo_t[j, 128 * hh:128 * hh + 128, :])
            out = jnp.concatenate(acc, axis=1)
            xa[16 + g, 32 * ph:32 * ph + 24, :] = out[8:32]
            mem = _round_bf16(out[0:8])
        return mem

    def dfwd_thunks(rows, tail):
        st = {}

        def pre():
            o = to[...] if tail else xa[16:32, rows, :]
            x = _round_bf16(xa[0:16, rows, :] + o)
            xb[:, rows, :] = x
            y = _layernorm(x.reshape(128, DM))
            x0, x1, x2, x3, x4 = [y[:, 128 * a:128 * a + 128] for a in range(5)]
            t1, t2, t3, t4 = x1 + x4, x2 + x3, x1 - x4, x2 - x3
            t = t1 + t2
            m, n = x0 - 0.25 * t, R5_D * (t1 - t2)
            st["u"] = [x0 + t, (m + n, t3 + R5_R * t4), (m - n, R5_R * t3 - t4)]

        def part(g):
            def run():
                if g == 0:
                    pre()
                    u0 = st["u"][0].astype(bf16)
                    zr = _dot(u0, _bf(small[0]))
                    if CFG["pack_f"]:
                        lane = lax.broadcasted_iota(jnp.int32, (128, 128), 1)
                        zi = jnp.where((lane & 63) == 0, 0.0, pltpu.roll(zr, 64, 1))
                    else:
                        zi = _dot(u0, _bf(small[1]))
                else:
                    a, b = st["u"][g]
                    k, kb, ka = [_dot(v.astype(bf16), _bf(small[3 * g - 1 + i]))
                                 for i, v in enumerate((a + b, b, a))]
                    zr, zi = k + kb, ka - _mu() * k
                ys = [(zr[8 * a:8 * a + 8], zi[8 * a:8 * a + 8]) for a in range(16)]
                if g < 2:
                    ys = _fft16(ys, -1)
                for a in range(16):
                    zs[g][0, a, rows, :] = ys[a][0]
                    zs[g][1, a, rows, :] = ys[a][1]
            return run
        return [part(g) for g in range(3)]

    def post(u, carry):
        base = pl.multiple_of(32 * u, 32)
        side = []
        for q in range(4):
            side += dfwd_thunks(pl.ds(base + 8 * q, 8), q == 3)
        side = [side[i] for i in CFG["post_order"]]
        k = 0
        at = list(CFG["post_at"])
        for js in CFG["post_js"]:
            acc = None
            for hh in range(H):
                oo = qb[:, u, hh].reshape(128, 128).astype(bf16)
                acc = addl(acc, [_dot(oo, wo_t[j, 128 * hh:128 * hh + 128, :]) for j in js])
                k += len(js)
                while at and at[0] <= k:
                    at.pop(0)
                    side.pop(0)()
            for j, y in zip(js, acc):
                to[:, :, 128 * j:128 * j + 128] = y.reshape(16, 8, 128)
        for f in side:
            f()
        return carry

    def spectral(zero):
        def fence(z):
            return z[0, zero, 128:ZPITCH, :]

        def radix(g, bb, sign):
            z = zs[g]
            toks = []

            def emit(q, y):
                for p in range(4):
                    z[0, q + 4 * p, chunk(bb), :] = y[p][0]
                    z[1, q + 4 * p, chunk(bb), :] = y[p][1]
                toks.append(fence(z))
            _fft16([(z[0, a, chunk(bb), :], z[1, a, chunk(bb), :]) for a in range(16)], sign, emit)
            return toks

        ys = {}

        def fwd(g, k2, toks):
            z = zs[g]
            ur, ui = z[0, k2, 0:64, :], z[1, k2, 0:64, :]
            tr, ti = _twiddle((z[0, k2, 64:128, :], z[1, k2, 64:128, :]), k2, 32, -1)
            for hf in range(2):
                v = _ilv(ur + tr, ui + ti) if hf == 0 else _ilv(ur - tr, ui - ti)
                lhs = _with_tokens(emat[k2 + 16 * hf], toks if hf == 0 else None)
                xr, xi = _dilv(_dot(_bf(lhs), v.astype(bf16)))
                ys["x", 16 * g + k2] = xr
                wr = wf[g, pl.ds(k2 * WPITCH + hf, 64, stride=2), :]
                wi = wf[g + 3, pl.ds(k2 * WPITCH + hf, 64, stride=2), :]
                ys[g, k2, hf] = _ilv(xr * wr - xi * wi, xr * wi + xi * wr).astype(bf16)

        def inv(g, k2, toks):
            z = zs[g]
            t0 = _dot(_bf(_with_tokens(emat[32 + k2], toks)), ys.pop((g, k2, 0)))
            t1 = _dot(_bf(emat[48 + k2]), ys.pop((g, k2, 1)))
            z[0, k2, 0:64, :], z[1, k2, 0:64, :] = _dilv(t0 + t1)
            z[0, k2, 64:128, :], z[1, k2, 64:128, :] = _twiddle(_dilv(t0 - t1), k2, 32, 1)

        units = [(g, k2) for g in range(3) for k2 in range(16)]
        toks = None
        lag = CFG["inv_lag"]
        for i in range(len(units) + lag):
            if i < len(units):
                fwd(*units[i], toks)
            if i >= lag:
                inv(*units[i - lag], toks if i >= len(units) else None)
            toks = []
            if i in CFG["fwd_at"]:
                toks += radix(2, CFG["fwd_at"].index(i), -1)
            for n, at in enumerate(CFG["inv_at"]):
                if at == i:
                    if not toks:
                        back, r = CFG["rel"]
                        zs[n // 16][1, zero, 128:ZPITCH, :] = ys["x", min(i - back, 47)][8 * r:8 * r + 8]
                    toks += radix(n // 16, n % 16, 1)
            pos = CFG["tok_pos"] if len(toks) <= 4 else range(8)
            toks = {j: pltpu.bitcast(t, u32) for j, t in zip(pos, toks)}

    def dinv_thunks(bb, finish):
        st = {}

        def part(g):
            def run():
                z = zs[g]
                ys = [(z[0, a, chunk(bb), :], z[1, a, chunk(bb), :]) for a in range(16)]
                if g >= CFG["inv_groups"]:
                    ys = _fft16(ys, 1)
                tr = jnp.concatenate([y[0] for y in ys], axis=0)
                ti = jnp.concatenate([y[1] for y in ys], axis=0)
                if g == 0 and CFG["pack_i"]:
                    lane = lax.broadcasted_iota(jnp.int32, (128, 128), 1)
                    v = jnp.where(lane <= 64, tr, pltpu.roll(ti, 64, 1))
                    st[0] = _dot(v.astype(bf16), _bf(small[8]))
                elif g == 0:
                    st[0] = _dot(tr.astype(bf16), _bf(small[8])) + _dot(ti.astype(bf16), _bf(small[9]))
                else:
                    k, ki, kr = [_dot(v.astype(bf16), _bf(small[7 + 3 * g + i]))
                                 for i, v in enumerate((tr + _mu() * ti, ti, tr))]
                    st[2 * g - 1], st[2 * g] = k + ki, k + kr
            return run

        def fin():
            p0, p1, q1, p2, q2 = [st[j] for j in range(5)]
            t = p1 + p2
            m, n = p0 - 0.25 * t, R5_D * (p1 - p2)
            e1, e2 = m + n, m - n
            o1, o2 = q1 + R5_R * q2, R5_R * q1 - q2
            y = jnp.concatenate([p0 + t, e1 - o1, e2 - o2, e2 + o2, e1 + o1], axis=1)
            finish(xb[:, chunk(bb), :].reshape(128, DM) + y)
        return [part(0), part(1), part(2), fin]

    def out_copy(bb):
        return pltpu.make_async_copy(xin.at[:, bb], out_hbm.at[:, bb], osem.at[bb])

    def layer(li, carry0):
        if full or CFG["only"] == "group":
            _loop("step", 0, 16, group, mem_ref[...].astype(f32))
        if full or CFG["only"] == "spec":
            _loop("post", 0, 4, post, 0, unroll=CFG["post_unroll"])

            with jax.named_scope("spectral"):
                spectral((li >> 1))
        if not full and CFG["only"] != "out":
            return carry0

        def run_chunks(th, order, lag):
            seq = [t[g] for t in th for g in order]
            for i in range(len(seq) + lag):
                if i < len(seq):
                    seq[i]()
                if i >= lag and (i - lag) % 3 == 2:
                    th[(i - lag) // 3][3]()

        @pl.when(li == 0)
        def _():
            with jax.named_scope("dinv_tails"):
                run_chunks([dinv_thunks(4 * u + 3, functools.partial(
                    lambda u, x: set_input(4 * u + 3, _round_bf16(x), u), u)) for u in range(4)],
                    *CFG["tails_order"])

            def batch(it, carry):
                bb = body_chunk(it)
                side = dinv_thunks(bb, lambda x: set_input(bb, _round_bf16(x), None))
                for k, f in enumerate(batch_thunks(it)):
                    f()
                    if k in CFG["dinv_at"]:
                        side.pop(0)()
                return carry
            _loop("batch", 0, 12, batch, 0, unroll=CFG["batch_unroll"])

        @pl.when(li == 1)
        def _():
            with jax.named_scope("dinv_out"):
                def store_out(bb, x):
                    xin[:, bb] = x.reshape(16, 8, DM).astype(bf16)
                    out_copy(bb).start()
                run_chunks([dinv_thunks(bb, functools.partial(store_out, bb)) for bb in range(16)],
                           *CFG["out_order"])
                for bb in range(16):
                    out_copy(bb).wait()
        return carry0

    if CFG["only"] != "pro":
        lax.fori_loop(0, 2, layer, 0)
    else:
        zero = zero_ref[0]
        xin[0, 0, :, 0:128] = (qb[zero, 0, 0] + wf[zero, 0:8, :] + xa[zero, 0:8, 0:128]).astype(bf16)
        out_copy(0).start()
        out_copy(0).wait()


@functools.partial(jax.jit, static_argnames=("A_seg_len",))
def pallas_interleave_layers__memory_aug_recurrent_mem_tr__spectral_gfnet__prompt_kernel(
    A_x, A_mem0, A_Wq, A_Wk, A_Wv, A_Wo, A_seg_len, B_x, B_w_r, B_w_i,
):
    assert A_seg_len == SEG and A_x.shape == (1, S, DM)
    small, emat = _tables()
    hbm = pl.BlockSpec(memory_space=pltpu.HBM)
    out = pl.pallas_call(
        _kernel,
        out_shape=jax.ShapeDtypeStruct((16, 16, 8, DM), bf16),
        in_specs=[hbm] * 10,
        out_specs=hbm,
        scratch_shapes=[
            pltpu.VMEM((16, 16, 8, DM), bf16),
            pltpu.VMEM((33, 128, DM), f32),
            pltpu.VMEM((16, 128, DM), f32),
            pltpu.VMEM((16, 8, DM), f32),
            pltpu.VMEM((12, 2, 320, 8, DH), bf16),
            pltpu.VMEM((13, 8 * HPITCH, 128), u32),
            pltpu.VMEM((13, 8 * HPITCH, 128), u32),
            pltpu.VMEM((5, H * DH, 128), bf16),
            pltpu.VMEM((16, 4, 96, 8, 128), f32),
            pltpu.VMEM((4, 5, 64, 128), u32),
            pltpu.VMEM((2, 16, ZPITCH, 128), f32),
            pltpu.VMEM((2, 16, ZPITCH, 128), f32),
            pltpu.VMEM((2, 16, ZPITCH, 128), f32),
            pltpu.VMEM((6, 16 * WPITCH + 32, 128), f32),
            pltpu.VMEM((9, DF, 512), bf16),
            pltpu.VMEM((4, 328, 128), f32),
            pltpu.VMEM((SMALL_TILES, 64, 128), u32),
            pltpu.VMEM((64, 64, 128), u32),
            pltpu.VMEM((80, 80), f32),
            pltpu.VMEM((MEM, DM), bf16),
            pltpu.SMEM((1,), jnp.int32),
            pltpu.SemaphoreType.DMA((46,)),
            pltpu.SemaphoreType.DMA((16,)),
        ],
        compiler_params=pltpu.CompilerParams(vmem_limit_bytes=120 * 1024 * 1024,
                                             disable_semaphore_checks=True),
    )(
        A_x.reshape(16, 16, 8, DM), A_mem0.reshape(MEM, DM),
        *[w.reshape(2, 320, H, DH) for w in (A_Wq, A_Wk, A_Wv)], A_Wo.reshape(H * DH, DM), B_w_r.T, B_w_i.T,
        jnp.asarray(small), jnp.asarray(emat),
    )
    return out.reshape(1, S, DM)
```

```python
import functools
import math

import jax
import jax.numpy as jnp
import numpy as np
from jax import lax
import jax.experimental.pallas as pl
import jax.experimental.pallas.tpu as pltpu

f32, bf16, u32 = jnp.float32, jnp.bfloat16, jnp.uint32

S, DM, H, DH, MEM, SEG = 2048, 640, 32, 128, 8, 32
NSEG = S // SEG
NPAIR = H // 2
DF = DM // 2 + 1
EPS = 1e-5
WPITCH = 132

HPITCH = 164
ZPITCH = 136

S1 = math.sin(2 * math.pi / 5)
R5_D = (math.cos(2 * math.pi / 5) - math.cos(4 * math.pi / 5)) / 2
R5_R = math.sin(4 * math.pi / 5) / S1


def _to_bf16_bits(a):
    u = np.ascontiguousarray(a, dtype=np.float32).view(np.uint32).astype(np.uint64)
    return ((u + 0x7FFF + ((u >> 16) & 1)) >> 16).astype(np.uint32)


def _pack_rows(a):
    b = _to_bf16_bits(a)
    return b[..., 0::2, :] | (b[..., 1::2, :] << 16)


@functools.lru_cache(maxsize=None)
def _tables():
    b = np.arange(128)
    l0 = np.arange(0, DF, 5)
    l1 = np.concatenate([np.arange(1, 320, 5), np.arange(4, 320, 5)])
    l2 = np.concatenate([np.arange(2, 320, 5), np.arange(3, 320, 5)])
    sg = np.concatenate([np.ones(64), -np.ones(64)])

    def th(l):
        return 2 * np.pi * ((b[:, None] * l[None, :]) % DM) / DM

    sc = 1.0 / (S * DM)
    fw = np.zeros((8, 128, 128))
    iw = np.zeros((8, 128, 128))
    t = th(l0)
    cl = np.full((65, 1), 2.0)
    cl[0] = cl[-1] = 1.0
    fw[0, :, :65], fw[1, :, :65] = np.cos(t), -np.sin(t)
    iw[0, :65], iw[1, :65] = cl * np.cos(t.T) * sc, -cl * np.sin(t.T) * sc
    if CFG["pack_f"]:
        fw[0, :, 65:] = fw[1, :, 1:64]
    if CFG["pack_i"]:
        iw[0, 65:] = iw[1, 1:64]
    mu = S1 * sg
    for g, l in ((1, l1), (2, l2)):
        t = th(l)
        c, s = np.cos(t), np.sin(t)
        fw[3 * g - 1:3 * g + 2] = c, -mu * s - c, mu * c - s
        iw[3 * g - 1:3 * g + 2] = [2 * sc * m.T for m in (c, -s - mu * c, mu * s - c)]
    n = np.arange(64)
    order = np.concatenate([np.concatenate([np.arange(8) + 8 * j, np.arange(8) + 8 * j + 64])
                            for j in range(8)])
    e = np.zeros((2, 32, 128, 128))
    for k2 in range(32):
        t = 2 * np.pi * (((32 * n[:, None] + k2) * n[None, :]) % S) / S
        er, ei = np.cos(t), -np.sin(t)
        m = np.block([[er, -ei], [ei, er]])[order][:, order]
        e[0, k2], e[1, k2] = m, m.T
    small = np.concatenate([_pack_rows(fw), _pack_rows(iw)], axis=0)
    return small, _pack_rows(e).reshape(64, 64, 128)


SMALL_TILES = 16


def _loop(name, lo, hi, body, init, **kw):
    with jax.named_scope(name):
        return lax.fori_loop(lo, hi, body, init, **kw)


def _bf(x):
    return pltpu.bitcast(x, bf16)


def _dot(a, b):
    return jnp.dot(a, b, preferred_element_type=f32)


def _round_bf16(x):
    return x.astype(bf16).astype(f32)


def _layernorm(x):
    m = jnp.mean(x, axis=-1, keepdims=True)
    xc = x - m
    v = jnp.mean(xc * xc, axis=-1, keepdims=True)
    return xc * lax.rsqrt(v + EPS)


def _fft4(x, sign):
    (ar, ai), (br, bi), (cr, ci), (dr, di) = x
    t0r, t0i, t1r, t1i = ar + cr, ai + ci, ar - cr, ai - ci
    t2r, t2i, t3r, t3i = br + dr, bi + di, br - dr, bi - di
    y0, y2 = (t0r + t2r, t0i + t2i), (t0r - t2r, t0i - t2i)
    p, q = (t1r + t3i, t1i - t3r), (t1r - t3i, t1i + t3r)
    return [y0, p, y2, q] if sign < 0 else [y0, q, y2, p]


def _twiddle(z, n, period, sign):
    zr, zi = z
    n = n % period
    if n == 0:
        return z
    if 4 * n == period:
        return (-zi, zr) if sign > 0 else (zi, -zr)
    c, s = math.cos(2 * math.pi * n / period), sign * math.sin(2 * math.pi * n / period)
    if (8 * n) % period == 0:
        a, d = zr + zi, zr - zi
        if c * s > 0:
            return (d * c, a * c)
        return (a * c, d * s)
    return (zr * c - zi * s, zr * s + zi * c)


def _mu():
    lane = lax.broadcasted_iota(jnp.int32, (1, 128), 1)
    return jnp.where(lane < 64, S1, -S1).astype(f32)


def _ilv(r, i):
    n = r.shape[0] // 8
    return jnp.concatenate([r.reshape(n, 8, 128), i.reshape(n, 8, 128)], axis=1).reshape(16 * n, 128)


def _dilv(x):
    n = x.shape[0] // 16
    x = x.reshape(n, 16, 128)
    return x[:, :8].reshape(8 * n, 128), x[:, 8:].reshape(8 * n, 128)


def _with_tokens(x, toks):
    if not toks:
        return x
    return jnp.concatenate(
        [x[8 * j:8 * j + 8] | toks[j] if j in toks else x[8 * j:8 * j + 8]
         for j in range(x.shape[0] // 8)], axis=0)


def _fft16(x, sign, emit=None):
    cols = [_fft4([x[4 * j + r] for j in range(4)], sign) for r in range(4)]
    out = [None] * 16
    for q in range(4):
        y = _fft4([_twiddle(cols[r][q], r * q, 16, sign) for r in range(4)], sign)
        for p in range(4):
            out[q + 4 * p] = y[p]
        if emit is not None:
            emit(q, y)
    return out


CFG = dict(steps=((4.5, 16.5, 6, 4, 0, 8), (5, 16.5, 5, 7, 8, 12), (5, 16.5, 6, 6, 8, 12), (5, 16.5, 8, 7, 8, 0)),
           post_js=((0, 1, 2), (3, 4)),
           post_order=(0, 1, 6, 3, 4, 5, 8, 2, 7, 9, 10, 11), post_at=(32, 46, 76, 108),
           tails_order=((1, 2, 0), 5), out_order=((1, 2, 0), 5), pack_f=True, pack_i=True,
           inv_at=tuple(range(28, 44)), inv_groups=1, inv_lag=4, tok_pos=(4, 5, 6, 7),
           fwd_at=(7, 8, 9, 10, 12, 13, 14, 16, 17, 18, 20, 21, 22, 24, 25, 26), rel=(0, 1), dinv_at=(8, 9, 10, 11), batch_unroll=2, post_unroll=1,
           pro_nre=14, re_pos=(3, 5, 7), ln_at=(22, 29, 31, 31), ln_at2=(4, 7, 10, 13),
           perm_at=tuple(range(12, 24)), only=None)


def _interleave(main, side):
    n, k = len(main), 0
    for i, f in enumerate(main):
        f()
        while k < len(side) and (k + 1) * n <= (i + 1) * len(side):
            side[k]()
            k += 1
    for f in side[k:]:
        f()


def _kernel(x_hbm, mem_hbm, wq_hbm, wk_hbm, wv_hbm, wo_hbm, wr_hbm, wi_hbm,
            small_hbm, e_hbm, out_hbm,
            xin, xa, xb, to, raw, wa, wb, wo_t, qb, hl, z0, z1, z2, wf,
            wri, wtmp, small, emat, fill_ref, mem_ref, zero_ref, sem, osem):
    zs = (z0, z1, z2)
    w_hbm = (wq_hbm, wk_hbm, wv_hbm)

    def body_chunk(i):
        return 4 * (i & 3) + (i >> 2)

    def cp_w(i):
        src = w_hbm[i >> 2].at[:, :, pl.ds(8 * (i & 3), 8), :] if isinstance(i, int) else raw.at[i]
        return pltpu.make_async_copy(src, raw.at[i], sem.at[i])

    def cp_x(bb):
        return pltpu.make_async_copy(x_hbm.at[:, bb], xin.at[:, bb], sem.at[12 + bb])

    def cp_f(i):
        src = ((wr_hbm, wi_hbm)[i >> 2].at[:, pl.ds(512 * (i & 3), 512)]
               if isinstance(i, int) else wri.at[i])
        return pltpu.make_async_copy(src, wri.at[i], sem.at[36 + i])

    cp_rest = [pltpu.make_async_copy(wo_hbm.at[:, pl.ds(128 * j, 128)], wo_t.at[j], sem.at[28 + j])
               for j in range(5)]
    cp_rest += [pltpu.make_async_copy(mem_hbm, mem_ref, sem.at[33]),
                pltpu.make_async_copy(small_hbm, small, sem.at[44]),
               pltpu.make_async_copy(e_hbm, emat, sem.at[45])]

    full = CFG["only"] in (None, "pro")
    for u in range(4 if full else 0):
        cp_x(4 * u + 3).start()
    if full:
        cp_w(0).start()
    for i in range(12 if full else 0):
        if i < 11:
            cp_w(i + 1).start()
        cp_x(body_chunk(i)).start()
        if 3 <= i < 11:
            cp_f(i - 3).start()
    for cp in cp_rest if full else ():
        cp.start()

    zero_ref[0] = 0

    r = lax.broadcasted_iota(jnp.int32, (80, 80), 0)
    c = lax.broadcasted_iota(jnp.int32, (80, 80), 1)

    def head(i):
        return jnp.where(i < 64, i // 32, (i - 64) // 8)

    def pos(i):
        return jnp.where(i < 64, i % 32, 32 + (i - 64) % 8)

    ok = (pos(r) < MEM) | (pos(r) >= pos(c))
    fill_ref[...] = jnp.where(head(r) == head(c), jnp.where(ok, 0.0, -1e9), -jnp.inf).astype(f32)
    wtmp[:, 320:328, :] = jnp.zeros((4, 8, 128), f32)
    xa[32, 0:8, 0:128] = jnp.zeros((8, 128), f32)
    wa[12, 0:8, :] = jnp.zeros((8, 128), u32)
    wb[12, 0:8, :] = jnp.zeros((8, 128), u32)
    wf[5, 16 * WPITCH:16 * WPITCH + 8, :] = jnp.zeros((8, 128), f32)
    for z in zs:
        z[0, 0, 128:ZPITCH, :] = jnp.zeros((8, 128), f32)

    def chunk(bb):
        if isinstance(bb, int):
            return slice(8 * bb, 8 * bb + 8)
        return pl.ds(pl.multiple_of(8 * bb, 8), 8)

    def set_input(bb, x, tail_u, a0=0):
        n = x.shape[0] // 8
        xa[a0:a0 + n, chunk(bb), :] = x.reshape(n, 8, DM)
        y = _layernorm(x)
        if tail_u is None:
            xa[16 + a0:16 + a0 + n, chunk(bb), :] = y.reshape(n, 8, DM)
        else:
            blk = [[y[64 * r:64 * r + 64, 128 * kt:128 * kt + 128] for kt in range(5)] for r in range(2)]
            ops = []
            for kp in range(2):
                (a11, a12), (a21, a22) = [blk[r][2 * kp:2 * kp + 2] for r in range(2)]
                ops += [a11 + a22, a21 + a22, a11, a22, a11 + a12, a21 - a11, a12 - a22]
            for i, v in enumerate(ops + [blk[0][4], blk[1][4]]):
                hl[tail_u >> 1, i, 32 * (tail_u & 1):32 * (tail_u & 1) + 32, :] = (
                    pltpu.bitcast(v.astype(bf16), u32))

    def load_x(bb, a0=0, n=16):
        return xin[a0:a0 + n, bb].astype(f32).reshape(8 * n, DM)

    def wtile(cid, j, e):
        w = (wa, wb)[e]
        return jnp.concatenate([w[cid, (4 * hf + j) * HPITCH:(4 * hf + j) * HPITCH + 160, :]
                                for hf in range(2)], axis=0)

    def relayout(i, cid, e):
        for r in range(4 * i, 4 * i + 4):
            a, b = [pltpu.bitcast(raw[cid, :, d].reshape(16, 128), u32) for d in (2 * r, 2 * r + 1)]
            v = (a & 0xFFFF) | (b << 16) if e == 0 else (a >> 16) | (b & jnp.uint32(0xFFFF0000))
            (wa, wb)[e][cid, pl.ds(r, 8, stride=HPITCH), :] = v

    def batch_thunks(cid):
        def unit(e, jp, s):
            c = {}

            def w(n, kt):
                return _bf(wtile(cid, 2 * jp + n, e)[64 * kt:64 * kt + 64])

            def wsum(x, y, sign):
                x, y = x.astype(f32), y.astype(f32)
                return (x + y if sign > 0 else x - y).astype(bf16)

            def rhs(i, kp):
                k0, k1 = 2 * kp, 2 * kp + 1
                return (lambda: wsum(w(0, k0), w(1, k1), 1), lambda: w(0, k0),
                        lambda: wsum(w(1, k0), w(1, k1), -1), lambda: wsum(w(0, k1), w(0, k0), -1),
                        lambda: w(1, k1), lambda: wsum(w(0, k0), w(1, k0), 1),
                        lambda: wsum(w(0, k1), w(1, k1), 1))[i]()

            def prod(i, toks=None):
                l0, l1 = _bf(_with_tokens(hl[s, i], toks)), _bf(hl[s, 7 + i])
                return _dot(l0, rhs(i, 0)) + _dot(l1, rhs(i, 1))

            def last(r, n, toks=None):
                return _dot(_bf(_with_tokens(hl[s, 14 + r], toks)), w(n, 4))

            def store(r, n):
                y = c.pop((r, n)).reshape(2, 8, 8, 128)
                for k in range(2):
                    qb[8 * r:8 * r + 8, 2 * s + k, 8 * cid + 2 * (2 * jp + n) + e] = y[k]

            def t0(toks=None):
                c[1, 1] = last(1, 1, toks) + prod(5)
                m1 = prod(0)
                c[1, 1], c[0, 0] = c[1, 1] + m1, m1

            def t1(toks=None):
                c[0, 0] = c[0, 0] + last(0, 0, toks) + prod(6)
                m2 = prod(1)
                c[1, 1], c[1, 0] = c[1, 1] - m2, m2

            def t2(toks=None):
                m3 = prod(2, toks)
                c[1, 1] = c[1, 1] + m3
                store(1, 1)
                m5 = prod(4)
                c[0, 1], c[0, 0] = m3 + m5, c[0, 0] - m5

            def t3(toks=None):
                c[0, 1] = c[0, 1] + last(0, 1, toks)
                store(0, 1)
                m4 = prod(3)
                c[0, 0] = c[0, 0] + m4
                store(0, 0)
                c[1, 0] = c[1, 0] + m4 + last(1, 0)
                store(1, 0)
            return [t0, t1, t2, t3]
        return [f for e in range(2) for jp in range(2) for s in range(2) for f in unit(e, jp, s)]

    def wperm_thunks(piece, j):
        m = (piece >> 2) & 1
        wt = wtmp.at[j]

        def load():
            wt[0:DF, :] = wri[piece, :, 128 * j:128 * j + 128].astype(f32)

        def one(g):
            def run():
                if g == 0:
                    t = jnp.concatenate([wt[pl.ds(0, 64, stride=5), :], wt[320:328, :],
                                         jnp.zeros((56, 128), f32)], axis=0)
                else:
                    t = jnp.concatenate([wt[pl.ds(g, 64, stride=5), :],
                                         wt[pl.ds(5 - g, 64, stride=5), :]], axis=0)
                y = t.T
                sub = wf.at[3 * m + g, pl.ds(pl.multiple_of((piece & 3) * 32, 32), 16 * WPITCH - 96)]
                for k in range(8):
                    for hf in range(2):
                        sub[pl.ds(8 * j + k + 8 * hf * WPITCH, 8, stride=WPITCH), :] = (
                            y[16 * k + 8 * hf:16 * k + 8 * hf + 8])
            return run
        return [load] + [one(g) for g in range(3)]

    def half_pass(cid, half, fill, zero, timed=()):
        nre = CFG["pro_nre"]
        toks = None
        for k, f in enumerate(batch_thunks(cid)[16 * half:16 * half + 16]):
            f(toks)
            toks = {}
            for pos, f in zip((0, 4, 1, 6), [f for at, f in timed if at == k]):
                toks[pos] = f()
            if fill is not None:
                for n, r in enumerate(r for r in range(40) if r * nre // 40 == k):
                    relayout(r, fill, 1 - half)
                    toks[CFG["re_pos"][n]] = (wb, wa)[half][12 + zero, 0:8, :]

    def ln_parts(bb, zero):
        def part(j):
            set_input(bb, load_x(bb, 4 * j, 4), None, 4 * j)
            return pltpu.bitcast(xa[32 + zero, 0:8, 0:128], u32)
        return [functools.partial(part, j) for j in range(4)]

    def perm_parts(piece, zero):
        def part(fs):
            for f in fs:
                f()
            return pltpu.bitcast(wf[5 + zero, 16 * WPITCH:16 * WPITCH + 8, :], u32)
        out = []
        for j in range(4):
            th = wperm_thunks(piece, j)
            out += [functools.partial(part, th[0:2]), functools.partial(part, th[2:3]),
                    functools.partial(part, th[3:4])]
        return out

    def pro0():
        for u in range(4):
            cp_x(4 * u + 3).wait()
        for u in range(4):
            set_input(4 * u + 3, load_x(4 * u + 3), u)
        cp_w(0).wait()
        zero = zero_ref[0]
        for i in range(40):
            relayout(i, 0, 0)
        half_pass(0, 0, zero, zero)

    def pro1(it, carry):
        bb = body_chunk(it)
        with jax.named_scope("pro1_wait"):
            cp_w(it + 1).wait()

            @pl.when(it >= 3)
            def _():
                cp_f(it - 3).wait()
            cp_x(bb).wait()
        piece = jnp.where(it >= 3, it - 3, 8)
        zero = it >> 4
        timed = sorted(list(zip(CFG["ln_at"], ln_parts(bb, zero)))
                       + list(zip(CFG["perm_at"], perm_parts(piece, zero))), key=lambda x: x[0])
        half_pass(it, 1, it + 1, zero, [x for x in timed if x[0] < 16])
        half_pass(it + 1, 0, it + 1, zero, [(k - 16, f) for k, f in timed if k >= 16])
        return carry

    def pro2():
        cp_x(body_chunk(11)).wait()
        for cp in cp_rest:
            cp.wait()
        zero = zero_ref[0]
        half_pass(11, 1, None, zero, list(zip(CFG["ln_at2"], ln_parts(body_chunk(11), zero))))

    if full:
        with jax.named_scope("pro0"):
            pro0()
        _loop("pro1", 0, 11, pro1, 0)
        with jax.named_scope("pro2"):
            pro2()

    scale = DH ** -0.5

    def wo_dot(hh, oo):
        return [_dot(oo, wo_t[j, 128 * hh:128 * hh + 128, :]) for j in range(5)]

    def addl(acc, res):
        return res if acc is None else [a + b for a, b in zip(acc, res)]

    def group(g, mem):
        for ph in range(4):
            h = jnp.concatenate([mem, xa[16 + g, 32 * ph:32 * ph + 24, :]], axis=0).astype(bf16)
            pr, sm, oos = {}, {}, {}
            lat_s, lat_pv, lat_wo, v_delay, n_first, n_last = CFG["steps"][ph]

            def stacked(p, m):
                tails = [qb[g, ph, 32 * m + 2 * p + e] for e in range(2)]
                return jnp.concatenate([pr[p, m, 0], pr[p, m, 1]] + tails, axis=0).astype(bf16)

            def scores(p):
                sc = lax.dot_general(stacked(p, 0), stacked(p, 1), (((1,), (1,)), ((), ())),
                                     preferred_element_type=f32)
                fill = fill_ref[...]
                sc = jnp.where(fill == 0.0, sc * scale, fill)
                mx = jnp.max(sc, axis=-1, keepdims=True)
                e = jnp.exp(sc - mx)
                rl = pl.reciprocal(jnp.sum(e, axis=-1, keepdims=True), approx=True)
                sm[p] = (e * rl).astype(bf16)

            def pv(p):
                o = _dot(sm[p], stacked(p, 2))
                for e in range(2):
                    qb[g, ph, 2 * p + e] = o[64 + 8 * e:72 + 8 * e]
                    oos[2 * p + e] = o[32 * e:32 * e + 32].astype(bf16)

            keyed = []
            for p in range(NPAIR):
                keyed += [(4 * p + 2 * m + e, (p, m, e)) for m in range(2) for e in range(2)]
                keyed += [(4 * p + 3.5 + v_delay, (p, 2, e)) for e in range(2)]
            bulk = [x for _, x in sorted(keyed, key=lambda kv: kv[0])]
            acc, t, nwo, pend, ready = None, 0.0, 0, [], []
            if n_first:
                first, bulk = bulk[:n_first], bulk[n_first:]
                for kt in range(5):
                    for p, m, e in first:
                        w = wtile(4 * m + (p >> 2), p & 3, e)[64 * kt:64 * kt + 64]
                        y = _dot(h[:, 128 * kt:128 * kt + 128], _bf(w))
                        pr[p, m, e] = y if kt == 0 else pr[p, m, e] + y
                t = float(len(first))
                pend = [(t + lat_s, "S", p) for p, m, e in first if m == 1 and e == 1]
            while nwo < H - n_last or pend:
                pend.sort()
                if pend and pend[0][0] <= t:
                    _, kind, p = pend.pop(0)
                    if kind == "S":
                        scores(p)
                        pend.append((t + lat_pv, "V", p))
                    else:
                        pv(p)
                        ready += [(t + lat_wo, 2 * p + e) for e in range(2)]
                    t += 0.5
                elif bulk:
                    p, m, e = bulk.pop(0)
                    pr[p, m, e] = _dot(h, _bf(wtile(4 * m + (p >> 2), p & 3, e)))
                    t += 1
                    if m == 1 and e == 1:
                        pend.append((t + lat_s, "S", p))
                elif ready and ready[0][0] <= t and nwo < H - n_last:
                    _, hh = ready.pop(0)
                    acc = addl(acc, wo_dot(hh, oos[hh]))
                    t += 1
                    nwo += 1
                else:
                    t += 0.5
            for j in range(5):
                for _, hh in ready:
                    acc[j] = acc[j] + _dot(oos[hh], wo_t[j, 128 * hh:128 * hh + 128, :])
            out = jnp.concatenate(acc, axis=1)
            xa[16 + g, 32 * ph:32 * ph + 24, :] = out[8:32]
            mem = _round_bf16(out[0:8])
        return mem

    def dfwd_thunks(rows, tail):
        st = {}

        def pre():
            o = to[...] if tail else xa[16:32, rows, :]
            x = _round_bf16(xa[0:16, rows, :] + o)
            xb[:, rows, :] = x
            y = _layernorm(x.reshape(128, DM))
            x0, x1, x2, x3, x4 = [y[:, 128 * a:128 * a + 128] for a in range(5)]
            t1, t2, t3, t4 = x1 + x4, x2 + x3, x1 - x4, x2 - x3
            t = t1 + t2
            m, n = x0 - 0.25 * t, R5_D * (t1 - t2)
            st["u"] = [x0 + t, (m + n, t3 + R5_R * t4), (m - n, R5_R * t3 - t4)]

        def part(g):
            def run():
                if g == 0:
                    pre()
                    u0 = st["u"][0].astype(bf16)
                    zr = _dot(u0, _bf(small[0]))
                    if CFG["pack_f"]:
                        lane = lax.broadcasted_iota(jnp.int32, (128, 128), 1)
                        zi = jnp.where((lane & 63) == 0, 0.0, pltpu.roll(zr, 64, 1))
                    else:
                        zi = _dot(u0, _bf(small[1]))
                else:
                    a, b = st["u"][g]
                    k, kb, ka = [_dot(v.astype(bf16), _bf(small[3 * g - 1 + i]))
                                 for i, v in enumerate((a + b, b, a))]
                    zr, zi = k + kb, ka - _mu() * k
                ys = [(zr[8 * a:8 * a + 8], zi[8 * a:8 * a + 8]) for a in range(16)]
                if g < 2:
                    ys = _fft16(ys, -1)
                for a in range(16):
                    zs[g][0, a, rows, :] = ys[a][0]
                    zs[g][1, a, rows, :] = ys[a][1]
            return run
        return [part(g) for g in range(3)]

    def post(u, carry):
        base = pl.multiple_of(32 * u, 32)
        side = []
        for q in range(4):
            side += dfwd_thunks(pl.ds(base + 8 * q, 8), q == 3)
        side = [side[i] for i in CFG["post_order"]]
        k = 0
        at = list(CFG["post_at"])
        for js in CFG["post_js"]:
            acc = None
            for hh in range(H):
                oo = qb[:, u, hh].reshape(128, 128).astype(bf16)
                acc = addl(acc, [_dot(oo, wo_t[j, 128 * hh:128 * hh + 128, :]) for j in js])
                k += len(js)
                while at and at[0] <= k:
                    at.pop(0)
                    side.pop(0)()
            for j, y in zip(js, acc):
                to[:, :, 128 * j:128 * j + 128] = y.reshape(16, 8, 128)
        for f in side:
            f()
        return carry

    def spectral(zero):
        def fence(z):
            return z[0, zero, 128:ZPITCH, :]

        def radix(g, bb, sign):
            z = zs[g]
            toks = []

            def emit(q, y):
                for p in range(4):
                    z[0, q + 4 * p, chunk(bb), :] = y[p][0]
                    z[1, q + 4 * p, chunk(bb), :] = y[p][1]
                toks.append(fence(z))
            _fft16([(z[0, a, chunk(bb), :], z[1, a, chunk(bb), :]) for a in range(16)], sign, emit)
            return toks

        ys = {}

        def fwd(g, k2, toks):
            z = zs[g]
            ur, ui = z[0, k2, 0:64, :], z[1, k2, 0:64, :]
            tr, ti = _twiddle((z[0, k2, 64:128, :], z[1, k2, 64:128, :]), k2, 32, -1)
            for hf in range(2):
                v = _ilv(ur + tr, ui + ti) if hf == 0 else _ilv(ur - tr, ui - ti)
                lhs = _with_tokens(emat[k2 + 16 * hf], toks if hf == 0 else None)
                xr, xi = _dilv(_dot(_bf(lhs), v.astype(bf16)))
                ys["x", 16 * g + k2] = xr
                wr = wf[g, pl.ds(k2 * WPITCH + hf, 64, stride=2), :]
                wi = wf[g + 3, pl.ds(k2 * WPITCH + hf, 64, stride=2), :]
                ys[g, k2, hf] = _ilv(xr * wr - xi * wi, xr * wi + xi * wr).astype(bf16)

        def inv(g, k2, toks):
            z = zs[g]
            t0 = _dot(_bf(_with_tokens(emat[32 + k2], toks)), ys.pop((g, k2, 0)))
            t1 = _dot(_bf(emat[48 + k2]), ys.pop((g, k2, 1)))
            z[0, k2, 0:64, :], z[1, k2, 0:64, :] = _dilv(t0 + t1)
            z[0, k2, 64:128, :], z[1, k2, 64:128, :] = _twiddle(_dilv(t0 - t1), k2, 32, 1)

        units = [(g, k2) for g in range(3) for k2 in range(16)]
        toks = None
        lag = CFG["inv_lag"]
        for i in range(len(units) + lag):
            if i < len(units):
                fwd(*units[i], toks)
            if i >= lag:
                inv(*units[i - lag], toks if i >= len(units) else None)
            toks = []
            if i in CFG["fwd_at"]:
                toks += radix(2, CFG["fwd_at"].index(i), -1)
            for n, at in enumerate(CFG["inv_at"]):
                if at == i:
                    if not toks:
                        back, r = CFG["rel"]
                        zs[n // 16][1, zero, 128:ZPITCH, :] = ys["x", min(i - back, 47)][8 * r:8 * r + 8]
                    toks += radix(n // 16, n % 16, 1)
            pos = CFG["tok_pos"] if len(toks) <= 4 else range(8)
            toks = {j: pltpu.bitcast(t, u32) for j, t in zip(pos, toks)}

    def dinv_thunks(bb, finish):
        st = {}

        def part(g):
            def run():
                z = zs[g]
                ys = [(z[0, a, chunk(bb), :], z[1, a, chunk(bb), :]) for a in range(16)]
                if g >= CFG["inv_groups"]:
                    ys = _fft16(ys, 1)
                tr = jnp.concatenate([y[0] for y in ys], axis=0)
                ti = jnp.concatenate([y[1] for y in ys], axis=0)
                if g == 0 and CFG["pack_i"]:
                    lane = lax.broadcasted_iota(jnp.int32, (128, 128), 1)
                    v = jnp.where(lane <= 64, tr, pltpu.roll(ti, 64, 1))
                    st[0] = _dot(v.astype(bf16), _bf(small[8]))
                elif g == 0:
                    st[0] = _dot(tr.astype(bf16), _bf(small[8])) + _dot(ti.astype(bf16), _bf(small[9]))
                else:
                    k, ki, kr = [_dot(v.astype(bf16), _bf(small[7 + 3 * g + i]))
                                 for i, v in enumerate((tr + _mu() * ti, ti, tr))]
                    st[2 * g - 1], st[2 * g] = k + ki, k + kr
            return run

        def fin():
            p0, p1, q1, p2, q2 = [st[j] for j in range(5)]
            t = p1 + p2
            m, n = p0 - 0.25 * t, R5_D * (p1 - p2)
            e1, e2 = m + n, m - n
            o1, o2 = q1 + R5_R * q2, R5_R * q1 - q2
            y = jnp.concatenate([p0 + t, e1 - o1, e2 - o2, e2 + o2, e1 + o1], axis=1)
            finish(xb[:, chunk(bb), :].reshape(128, DM) + y)
        return [part(0), part(1), part(2), fin]

    def out_copy(bb):
        return pltpu.make_async_copy(xin.at[:, bb], out_hbm.at[:, bb], osem.at[bb])

    def layer(li, carry0):
        if full or CFG["only"] == "group":
            _loop("step", 0, 16, group, mem_ref[...].astype(f32))
        if full or CFG["only"] == "spec":
            _loop("post", 0, 4, post, 0, unroll=CFG["post_unroll"])

            with jax.named_scope("spectral"):
                spectral((li >> 1))
        if not full and CFG["only"] != "out":
            return carry0

        def run_chunks(th, order, lag):
            seq = [t[g] for t in th for g in order]
            for i in range(len(seq) + lag):
                if i < len(seq):
                    seq[i]()
                if i >= lag and (i - lag) % 3 == 2:
                    th[(i - lag) // 3][3]()

        @pl.when(li == 0)
        def _():
            with jax.named_scope("dinv_tails"):
                run_chunks([dinv_thunks(4 * u + 3, functools.partial(
                    lambda u, x: set_input(4 * u + 3, _round_bf16(x), u), u)) for u in range(4)],
                    *CFG["tails_order"])

            def batch(it, carry):
                bb = body_chunk(it)
                side = dinv_thunks(bb, lambda x: set_input(bb, _round_bf16(x), None))
                for k, f in enumerate(batch_thunks(it)):
                    f()
                    if k in CFG["dinv_at"]:
                        side.pop(0)()
                return carry
            _loop("batch", 0, 12, batch, 0, unroll=CFG["batch_unroll"])

        @pl.when(li == 1)
        def _():
            with jax.named_scope("dinv_out"):
                def store_out(bb, x):
                    xin[:, bb] = x.reshape(16, 8, DM).astype(bf16)
                    out_copy(bb).start()
                run_chunks([dinv_thunks(bb, functools.partial(store_out, bb)) for bb in range(16)],
                           *CFG["out_order"])
                for bb in range(16):
                    out_copy(bb).wait()
        return carry0

    if CFG["only"] != "pro":
        lax.fori_loop(0, 2, layer, 0)
    else:
        zero = zero_ref[0]
        xin[0, 0, :, 0:128] = (qb[zero, 0, 0] + wf[zero, 0:8, :] + xa[zero, 0:8, 0:128]).astype(bf16)
        out_copy(0).start()
        out_copy(0).wait()


@functools.partial(jax.jit, static_argnames=("A_seg_len",))
def pallas_interleave_layers__memory_aug_recurrent_mem_tr__spectral_gfnet__prompt_kernel(
    A_x, A_mem0, A_Wq, A_Wk, A_Wv, A_Wo, A_seg_len, B_x, B_w_r, B_w_i,
):
    assert A_seg_len == SEG and A_x.shape == (1, S, DM)
    small, emat = _tables()
    hbm = pl.BlockSpec(memory_space=pltpu.HBM)
    out = pl.pallas_call(
        _kernel,
        out_shape=jax.ShapeDtypeStruct((16, 16, 8, DM), bf16),
        in_specs=[hbm] * 10,
        out_specs=hbm,
        scratch_shapes=[
            pltpu.VMEM((16, 16, 8, DM), bf16),
            pltpu.VMEM((33, 128, DM), f32),
            pltpu.VMEM((16, 128, DM), f32),
            pltpu.VMEM((16, 8, DM), f32),
            pltpu.VMEM((12, 2, 320, 8, DH), bf16),
            pltpu.VMEM((13, 8 * HPITCH, 128), u32),
            pltpu.VMEM((13, 8 * HPITCH, 128), u32),
            pltpu.VMEM((5, H * DH, 128), bf16),
            pltpu.VMEM((16, 4, 96, 8, 128), f32),
            pltpu.VMEM((2, 16, 64, 128), u32),
            pltpu.VMEM((2, 16, ZPITCH, 128), f32),
            pltpu.VMEM((2, 16, ZPITCH, 128), f32),
            pltpu.VMEM((2, 16, ZPITCH, 128), f32),
            pltpu.VMEM((6, 16 * WPITCH + 32, 128), f32),
            pltpu.VMEM((9, DF, 512), bf16),
            pltpu.VMEM((4, 328, 128), f32),
            pltpu.VMEM((SMALL_TILES, 64, 128), u32),
            pltpu.VMEM((64, 64, 128), u32),
            pltpu.VMEM((80, 80), f32),
            pltpu.VMEM((MEM, DM), bf16),
            pltpu.SMEM((1,), jnp.int32),
            pltpu.SemaphoreType.DMA((46,)),
            pltpu.SemaphoreType.DMA((16,)),
        ],
        compiler_params=pltpu.CompilerParams(vmem_limit_bytes=120 * 1024 * 1024,
                                             disable_semaphore_checks=True),
    )(
        A_x.reshape(16, 16, 8, DM), A_mem0.reshape(MEM, DM),
        *[w.reshape(2, 320, H, DH) for w in (A_Wq, A_Wk, A_Wv)], A_Wo.reshape(H * DH, DM), B_w_r.T, B_w_i.T,
        jnp.asarray(small), jnp.asarray(emat),
    )
    return out.reshape(1, S, DM)
```

```python
import functools
import math

import jax
import jax.numpy as jnp
import numpy as np
from jax import lax
import jax.experimental.pallas as pl
import jax.experimental.pallas.tpu as pltpu

f32, bf16, u32 = jnp.float32, jnp.bfloat16, jnp.uint32

S, DM, H, DH, MEM, SEG = 2048, 640, 32, 128, 8, 32
NSEG = S // SEG
NPAIR = H // 2
DF = DM // 2 + 1
EPS = 1e-5
WPITCH = 132

HPITCH = 164
ZPITCH = 136

S1 = math.sin(2 * math.pi / 5)
R5_D = (math.cos(2 * math.pi / 5) - math.cos(4 * math.pi / 5)) / 2
R5_R = math.sin(4 * math.pi / 5) / S1


def _to_bf16_bits(a):
    u = np.ascontiguousarray(a, dtype=np.float32).view(np.uint32).astype(np.uint64)
    return ((u + 0x7FFF + ((u >> 16) & 1)) >> 16).astype(np.uint32)


def _pack_rows(a):
    b = _to_bf16_bits(a)
    return b[..., 0::2, :] | (b[..., 1::2, :] << 16)


@functools.lru_cache(maxsize=None)
def _tables():
    b = np.arange(128)
    l0 = np.arange(0, DF, 5)
    l1 = np.concatenate([np.arange(1, 320, 5), np.arange(4, 320, 5)])
    l2 = np.concatenate([np.arange(2, 320, 5), np.arange(3, 320, 5)])
    sg = np.concatenate([np.ones(64), -np.ones(64)])

    def th(l):
        return 2 * np.pi * ((b[:, None] * l[None, :]) % DM) / DM

    sc = 1.0 / (S * DM)
    fw = np.zeros((8, 128, 128))
    iw = np.zeros((8, 128, 128))
    t = th(l0)
    cl = np.full((65, 1), 2.0)
    cl[0] = cl[-1] = 1.0
    fw[0, :, :65], fw[1, :, :65] = np.cos(t), -np.sin(t)
    iw[0, :65], iw[1, :65] = cl * np.cos(t.T) * sc, -cl * np.sin(t.T) * sc
    if CFG["pack_f"]:
        fw[0, :, 65:] = fw[1, :, 1:64]
    if CFG["pack_i"]:
        iw[0, 65:] = iw[1, 1:64]
    mu = S1 * sg
    for g, l in ((1, l1), (2, l2)):
        t = th(l)
        c, s = np.cos(t), np.sin(t)
        fw[3 * g - 1:3 * g + 2] = c, -mu * s - c, mu * c - s
        iw[3 * g - 1:3 * g + 2] = [2 * sc * m.T for m in (c, -s - mu * c, mu * s - c)]
    n = np.arange(64)
    order = np.concatenate([np.concatenate([np.arange(8) + 8 * j, np.arange(8) + 8 * j + 64])
                            for j in range(8)])
    e = np.zeros((2, 32, 128, 128))
    for k2 in range(32):
        t = 2 * np.pi * (((32 * n[:, None] + k2) * n[None, :]) % S) / S
        er, ei = np.cos(t), -np.sin(t)
        m = np.block([[er, -ei], [ei, er]])[order][:, order]
        e[0, k2], e[1, k2] = m, m.T
    small = np.concatenate([_pack_rows(fw), _pack_rows(iw)], axis=0)
    return small, _pack_rows(e).reshape(64, 64, 128)


SMALL_TILES = 16


def _loop(name, lo, hi, body, init, **kw):
    with jax.named_scope(name):
        return lax.fori_loop(lo, hi, body, init, **kw)


def _bf(x):
    return pltpu.bitcast(x, bf16)


def _dot(a, b):
    return jnp.dot(a, b, preferred_element_type=f32)


def _round_bf16(x):
    return x.astype(bf16).astype(f32)


def _layernorm(x):
    m = jnp.mean(x, axis=-1, keepdims=True)
    xc = x - m
    v = jnp.mean(xc * xc, axis=-1, keepdims=True)
    return xc * lax.rsqrt(v + EPS)


def _fft4(x, sign):
    (ar, ai), (br, bi), (cr, ci), (dr, di) = x
    t0r, t0i, t1r, t1i = ar + cr, ai + ci, ar - cr, ai - ci
    t2r, t2i, t3r, t3i = br + dr, bi + di, br - dr, bi - di
    y0, y2 = (t0r + t2r, t0i + t2i), (t0r - t2r, t0i - t2i)
    p, q = (t1r + t3i, t1i - t3r), (t1r - t3i, t1i + t3r)
    return [y0, p, y2, q] if sign < 0 else [y0, q, y2, p]


def _twiddle(z, n, period, sign):
    zr, zi = z
    n = n % period
    if n == 0:
        return z
    if 4 * n == period:
        return (-zi, zr) if sign > 0 else (zi, -zr)
    c, s = math.cos(2 * math.pi * n / period), sign * math.sin(2 * math.pi * n / period)
    if (8 * n) % period == 0:
        a, d = zr + zi, zr - zi
        if c * s > 0:
            return (d * c, a * c)
        return (a * c, d * s)
    return (zr * c - zi * s, zr * s + zi * c)


def _bsum(x, y, sign):
    x, y = x.astype(f32), y.astype(f32)
    return (x + y if sign > 0 else x - y).astype(bf16)


def _strassen_lhs(a11, a12, a21, a22):
    return [lambda: a11() + a22(), lambda: a21() + a22(), a11, a22,
            lambda: a11() + a12(), lambda: a21() - a11(), lambda: a12() - a22()]


def _strassen_rhs(b11, b12, b21, b22):
    return [lambda: _bsum(b11(), b22(), 1), b11, lambda: _bsum(b12(), b22(), -1),
            lambda: _bsum(b21(), b11(), -1), b22, lambda: _bsum(b11(), b12(), 1),
            lambda: _bsum(b21(), b22(), 1)]


WS_SLOT = {0: 0, 2: 1, 3: 2, 5: 3, 6: 4}


def _mu():
    lane = lax.broadcasted_iota(jnp.int32, (1, 128), 1)
    return jnp.where(lane < 64, S1, -S1).astype(f32)


def _ilv(r, i):
    n = r.shape[0] // 8
    return jnp.concatenate([r.reshape(n, 8, 128), i.reshape(n, 8, 128)], axis=1).reshape(16 * n, 128)


def _dilv(x):
    n = x.shape[0] // 16
    x = x.reshape(n, 16, 128)
    return x[:, :8].reshape(8 * n, 128), x[:, 8:].reshape(8 * n, 128)


def _with_tokens(x, toks):
    if not toks:
        return x
    return jnp.concatenate(
        [x[8 * j:8 * j + 8] | toks[j] if j in toks else x[8 * j:8 * j + 8]
         for j in range(x.shape[0] // 8)], axis=0)


def _fft16(x, sign, emit=None):
    cols = [_fft4([x[4 * j + r] for j in range(4)], sign) for r in range(4)]
    out = [None] * 16
    for q in range(4):
        y = _fft4([_twiddle(cols[r][q], r * q, 16, sign) for r in range(4)], sign)
        for p in range(4):
            out[q + 4 * p] = y[p]
        if emit is not None:
            emit(q, y)
    return out


CFG = dict(steps=((4.5, 16.5, 6, 4, 0, 8), (5, 16.5, 5, 7, 8, 12), (5, 16.5, 6, 6, 8, 12), (5, 16.5, 8, 7, 8, 0)),
           post_passes=((0, 1), (2, 3), (4, 5), (6, 7)),
           post_order=(0, 1, 6, 3, 4, 2, 8, 5, 7, 9, 10, 11), post_at=(26, 42, 68, 96),
           tails_order=((1, 2, 0), 5), out_order=((1, 2, 0), 5), pack_f=True, pack_i=True,
           inv_at=tuple(range(28, 44)), inv_groups=1, inv_lag=4, tok_pos=(4, 5, 6, 7),
           fwd_at=(7, 8, 9, 10, 12, 13, 14, 16, 17, 18, 20, 21, 22, 24, 25, 26), rel=(0, 1), dinv_at=(8, 9, 10, 11), batch_unroll=2, post_unroll=1,
           ws_split=8, ws_at=tuple(range(32)), pro_nre=14, re_pos=(3, 5, 7), ln_at=(22, 29, 31, 31), ln_at2=(4, 7, 10, 13),
           perm_at=tuple(range(12, 24)), only=None)


def _interleave(main, side):
    n, k = len(main), 0
    for i, f in enumerate(main):
        f()
        while k < len(side) and (k + 1) * n <= (i + 1) * len(side):
            side[k]()
            k += 1
    for f in side[k:]:
        f()


def _kernel(x_hbm, mem_hbm, wq_hbm, wk_hbm, wv_hbm, wo_hbm, wr_hbm, wi_hbm,
            small_hbm, e_hbm, out_hbm,
            xin, xa, xb, to, raw, wa, wb, wo_t, ws, qb, hl, z0, z1, z2, wf,
            wri, wtmp, small, emat, fill_ref, mem_ref, zero_ref, sem, osem):
    zs = (z0, z1, z2)
    w_hbm = (wq_hbm, wk_hbm, wv_hbm)

    def body_chunk(i):
        return 4 * (i & 3) + (i >> 2)

    def cp_w(i):
        src = w_hbm[i >> 2].at[:, :, pl.ds(8 * (i & 3), 8), :] if isinstance(i, int) else raw.at[i]
        return pltpu.make_async_copy(src, raw.at[i], sem.at[i])

    def cp_x(bb):
        return pltpu.make_async_copy(x_hbm.at[:, bb], xin.at[:, bb], sem.at[12 + bb])

    def cp_f(i):
        src = ((wr_hbm, wi_hbm)[i >> 2].at[:, pl.ds(512 * (i & 3), 512)]
               if isinstance(i, int) else wri.at[i])
        return pltpu.make_async_copy(src, wri.at[i], sem.at[36 + i])

    def cp_wo(i):
        rows = pl.ds(pl.multiple_of(512 * i, 512), 512)
        return [pltpu.make_async_copy(wo_hbm.at[rows, pl.ds(128 * j, 128)], wo_t.at[j, rows], sem.at[28 + i])
                for j in range(5)]

    cp_rest = [pltpu.make_async_copy(mem_hbm, mem_ref, sem.at[46]),
                pltpu.make_async_copy(small_hbm, small, sem.at[44]),
               pltpu.make_async_copy(e_hbm, emat, sem.at[45])]

    full = CFG["only"] in (None, "pro")
    for u in range(4 if full else 0):
        cp_x(4 * u + 3).start()
    if full:
        cp_w(0).start()
    for i in range(12 if full else 0):
        if i < 11:
            cp_w(i + 1).start()
        cp_x(body_chunk(i)).start()
        if 3 <= i < 11:
            cp_f(i - 3).start()
            for cp in cp_wo(i - 3):
                cp.start()
    for cp in cp_rest if full else ():
        cp.start()

    zero_ref[0] = 0

    r = lax.broadcasted_iota(jnp.int32, (80, 80), 0)
    c = lax.broadcasted_iota(jnp.int32, (80, 80), 1)

    def head(i):
        return jnp.where(i < 64, i // 32, (i - 64) // 8)

    def pos(i):
        return jnp.where(i < 64, i % 32, 32 + (i - 64) % 8)

    ok = (pos(r) < MEM) | (pos(r) >= pos(c))
    fill_ref[...] = jnp.where(head(r) == head(c), jnp.where(ok, 0.0, -1e9), -jnp.inf).astype(f32)
    wtmp[:, 320:328, :] = jnp.zeros((4, 8, 128), f32)
    xa[32, 0:8, 0:128] = jnp.zeros((8, 128), f32)
    ws[18, 0, 0:16, :] = jnp.zeros((16, 128), bf16)
    wa[12, 0:8, :] = jnp.zeros((8, 128), u32)
    wb[12, 0:8, :] = jnp.zeros((8, 128), u32)
    wf[5, 16 * WPITCH:16 * WPITCH + 8, :] = jnp.zeros((8, 128), f32)
    for z in zs:
        z[0, 0, 128:ZPITCH, :] = jnp.zeros((8, 128), f32)

    def chunk(bb):
        if isinstance(bb, int):
            return slice(8 * bb, 8 * bb + 8)
        return pl.ds(pl.multiple_of(8 * bb, 8), 8)

    def set_input(bb, x, tail_u, a0=0):
        n = x.shape[0] // 8
        xa[a0:a0 + n, chunk(bb), :] = x.reshape(n, 8, DM)
        y = _layernorm(x)
        if tail_u is None:
            xa[16 + a0:16 + a0 + n, chunk(bb), :] = y.reshape(n, 8, DM)
        else:
            blk = [[y[64 * r:64 * r + 64, 128 * kt:128 * kt + 128] for kt in range(5)] for r in range(2)]
            ops = []
            for kp in range(2):
                (a11, a12), (a21, a22) = [blk[r][2 * kp:2 * kp + 2] for r in range(2)]
                ops += [a11 + a22, a21 + a22, a11, a22, a11 + a12, a21 - a11, a12 - a22]
            for i, v in enumerate(ops + [blk[0][4], blk[1][4]]):
                hl[tail_u >> 1, i, 32 * (tail_u & 1):32 * (tail_u & 1) + 32, :] = (
                    pltpu.bitcast(v.astype(bf16), u32))

    def load_x(bb, a0=0, n=16):
        return xin[a0:a0 + n, bb].astype(f32).reshape(8 * n, DM)

    def wtile(cid, j, e):
        w = (wa, wb)[e]
        return jnp.concatenate([w[cid, (4 * hf + j) * HPITCH:(4 * hf + j) * HPITCH + 160, :]
                                for hf in range(2)], axis=0)

    def relayout(i, cid, e):
        for r in range(4 * i, 4 * i + 4):
            a, b = [pltpu.bitcast(raw[cid, :, d].reshape(16, 128), u32) for d in (2 * r, 2 * r + 1)]
            v = (a & 0xFFFF) | (b << 16) if e == 0 else (a >> 16) | (b & jnp.uint32(0xFFFF0000))
            (wa, wb)[e][cid, pl.ds(r, 8, stride=HPITCH), :] = v

    def batch_thunks(cid):
        def unit(e, jp, s):
            c = {}

            def w(n, kt):
                return _bf(wtile(cid, 2 * jp + n, e)[64 * kt:64 * kt + 64])

            def rhs(i, kp):
                return _strassen_rhs(*[functools.partial(w, n, 2 * kp + k)
                                       for k in range(2) for n in range(2)])[i]()

            def prod(i, toks=None):
                l0, l1 = _bf(_with_tokens(hl[s, i], toks)), _bf(hl[s, 7 + i])
                return _dot(l0, rhs(i, 0)) + _dot(l1, rhs(i, 1))

            def last(r, n, toks=None):
                return _dot(_bf(_with_tokens(hl[s, 14 + r], toks)), w(n, 4))

            def store(r, n):
                y = c.pop((r, n)).reshape(2, 8, 8, 128)
                for k in range(2):
                    qb[8 * r:8 * r + 8, 2 * s + k, 8 * cid + 2 * (2 * jp + n) + e] = y[k]

            def t0(toks=None):
                c[1, 1] = last(1, 1, toks) + prod(5)
                m1 = prod(0)
                c[1, 1], c[0, 0] = c[1, 1] + m1, m1

            def t1(toks=None):
                c[0, 0] = c[0, 0] + last(0, 0, toks) + prod(6)
                m2 = prod(1)
                c[1, 1], c[1, 0] = c[1, 1] - m2, m2

            def t2(toks=None):
                m3 = prod(2, toks)
                c[1, 1] = c[1, 1] + m3
                store(1, 1)
                m5 = prod(4)
                c[0, 1], c[0, 0] = m3 + m5, c[0, 0] - m5

            def t3(toks=None):
                c[0, 1] = c[0, 1] + last(0, 1, toks)
                store(0, 1)
                m4 = prod(3)
                c[0, 0] = c[0, 0] + m4
                store(0, 0)
                c[1, 0] = c[1, 0] + m4 + last(1, 0)
                store(1, 0)
            return [t0, t1, t2, t3]
        return [f for e in range(2) for jp in range(2) for s in range(2) for f in unit(e, jp, s)]

    def wperm_thunks(piece, j):
        m = (piece >> 2) & 1
        wt = wtmp.at[j]

        def load():
            wt[0:DF, :] = wri[piece, :, 128 * j:128 * j + 128].astype(f32)

        def one(g):
            def run():
                if g == 0:
                    t = jnp.concatenate([wt[pl.ds(0, 64, stride=5), :], wt[320:328, :],
                                         jnp.zeros((56, 128), f32)], axis=0)
                else:
                    t = jnp.concatenate([wt[pl.ds(g, 64, stride=5), :],
                                         wt[pl.ds(5 - g, 64, stride=5), :]], axis=0)
                y = t.T
                sub = wf.at[3 * m + g, pl.ds(pl.multiple_of((piece & 3) * 32, 32), 16 * WPITCH - 96)]
                for k in range(8):
                    for hf in range(2):
                        sub[pl.ds(8 * j + k + 8 * hf * WPITCH, 8, stride=WPITCH), :] = (
                            y[16 * k + 8 * hf:16 * k + 8 * hf + 8])
            return run
        return [load] + [one(g) for g in range(3)]

    def half_pass(cid, half, fill, zero, timed=()):
        nre = CFG["pro_nre"]
        toks = None
        for k, f in enumerate(batch_thunks(cid)[16 * half:16 * half + 16]):
            f(toks)
            toks = {}
            for pos, f in zip((0, 4, 1, 6), [f for at, f in timed if at == k]):
                toks[pos] = f()
            if fill is not None:
                for n, r in enumerate(r for r in range(40) if r * nre // 40 == k):
                    relayout(r, fill, 1 - half)
                    toks[CFG["re_pos"][n]] = (wb, wa)[half][12 + zero, 0:8, :]

    def ln_parts(bb, zero):
        def part(j):
            set_input(bb, load_x(bb, 4 * j, 4), None, 4 * j)
            return pltpu.bitcast(xa[32 + zero, 0:8, 0:128], u32)
        return [functools.partial(part, j) for j in range(4)]

    def perm_parts(piece, zero):
        def part(fs):
            for f in fs:
                f()
            return pltpu.bitcast(wf[5 + zero, 16 * WPITCH:16 * WPITCH + 8, :], u32)
        out = []
        for j in range(4):
            th = wperm_thunks(piece, j)
            out += [functools.partial(part, th[0:2]), functools.partial(part, th[2:3]),
                    functools.partial(part, th[3:4])]
        return out

    def ws_parts(piece, zero):
        nr = 128 // CFG["ws_split"]

        def part(pp, np_, r0):
            base = pl.multiple_of(512 * piece, 512) + 256 * pp + r0

            def tile(k, n):
                return wo_t[2 * np_ + n, pl.ds(base + 128 * k, nr), :]
            rhs = _strassen_rhs(*[functools.partial(tile, k, n) for k in range(2) for n in range(2)])
            for i, slot in WS_SLOT.items():
                ws[2 * piece + pp, 5 * np_ + slot, r0:r0 + nr, :] = rhs[i]()
            return pltpu.bitcast(ws[18 + zero, 0, 0:16, :], u32)
        return [functools.partial(part, pp, np_, r0)
                for pp in range(2) for np_ in range(2) for r0 in range(0, 128, nr)]

    def pro0():
        for u in range(4):
            cp_x(4 * u + 3).wait()
        for u in range(4):
            set_input(4 * u + 3, load_x(4 * u + 3), u)
        cp_w(0).wait()
        zero = zero_ref[0]
        for i in range(40):
            relayout(i, 0, 0)
        half_pass(0, 0, zero, zero)

    def pro1(it, carry):
        bb = body_chunk(it)
        with jax.named_scope("pro1_wait"):
            cp_w(it + 1).wait()

            @pl.when(it >= 3)
            def _():
                cp_f(it - 3).wait()
                for cp in cp_wo(it - 3):
                    cp.wait()
            cp_x(bb).wait()
        piece = jnp.where(it >= 3, it - 3, 8)
        zero = it >> 4
        timed = sorted(list(zip(CFG["ln_at"], ln_parts(bb, zero)))
                       + list(zip(CFG["ws_at"], ws_parts(piece, zero)))
                       + list(zip(CFG["perm_at"], perm_parts(piece, zero))), key=lambda x: x[0])
        half_pass(it, 1, it + 1, zero, [x for x in timed if x[0] < 16])
        half_pass(it + 1, 0, it + 1, zero, [(k - 16, f) for k, f in timed if k >= 16])
        return carry

    def pro2():
        cp_x(body_chunk(11)).wait()
        for cp in cp_rest:
            cp.wait()
        zero = zero_ref[0]
        half_pass(11, 1, None, zero, list(zip(CFG["ln_at2"], ln_parts(body_chunk(11), zero))))

    if full:
        with jax.named_scope("pro0"):
            pro0()
        _loop("pro1", 0, 11, pro1, 0)
        with jax.named_scope("pro2"):
            pro2()

    scale = DH ** -0.5

    def wo_dot(hh, oo):
        return [_dot(oo, wo_t[j, 128 * hh:128 * hh + 128, :]) for j in range(5)]

    def addl(acc, res):
        return res if acc is None else [a + b for a, b in zip(acc, res)]

    def group(g, mem):
        for ph in range(4):
            h = jnp.concatenate([mem, xa[16 + g, 32 * ph:32 * ph + 24, :]], axis=0).astype(bf16)
            pr, sm, oos = {}, {}, {}
            lat_s, lat_pv, lat_wo, v_delay, n_first, n_last = CFG["steps"][ph]

            def stacked(p, m):
                tails = [qb[g, ph, 32 * m + 2 * p + e] for e in range(2)]
                return jnp.concatenate([pr[p, m, 0], pr[p, m, 1]] + tails, axis=0).astype(bf16)

            def scores(p):
                sc = lax.dot_general(stacked(p, 0), stacked(p, 1), (((1,), (1,)), ((), ())),
                                     preferred_element_type=f32)
                fill = fill_ref[...]
                sc = jnp.where(fill == 0.0, sc * scale, fill)
                mx = jnp.max(sc, axis=-1, keepdims=True)
                e = jnp.exp(sc - mx)
                rl = pl.reciprocal(jnp.sum(e, axis=-1, keepdims=True), approx=True)
                sm[p] = (e * rl).astype(bf16)

            def pv(p):
                o = _dot(sm[p], stacked(p, 2))
                for e in range(2):
                    qb[g, ph, 2 * p + e] = o[64 + 8 * e:72 + 8 * e]
                    oos[2 * p + e] = o[32 * e:32 * e + 32].astype(bf16)

            keyed = []
            for p in range(NPAIR):
                keyed += [(4 * p + 2 * m + e, (p, m, e)) for m in range(2) for e in range(2)]
                keyed += [(4 * p + 3.5 + v_delay, (p, 2, e)) for e in range(2)]
            bulk = [x for _, x in sorted(keyed, key=lambda kv: kv[0])]
            acc, t, nwo, pend, ready = None, 0.0, 0, [], []
            if n_first:
                first, bulk = bulk[:n_first], bulk[n_first:]
                for kt in range(5):
                    for p, m, e in first:
                        w = wtile(4 * m + (p >> 2), p & 3, e)[64 * kt:64 * kt + 64]
                        y = _dot(h[:, 128 * kt:128 * kt + 128], _bf(w))
                        pr[p, m, e] = y if kt == 0 else pr[p, m, e] + y
                t = float(len(first))
                pend = [(t + lat_s, "S", p) for p, m, e in first if m == 1 and e == 1]
            while nwo < H - n_last or pend:
                pend.sort()
                if pend and pend[0][0] <= t:
                    _, kind, p = pend.pop(0)
                    if kind == "S":
                        scores(p)
                        pend.append((t + lat_pv, "V", p))
                    else:
                        pv(p)
                        ready += [(t + lat_wo, 2 * p + e) for e in range(2)]
                    t += 0.5
                elif bulk:
                    p, m, e = bulk.pop(0)
                    pr[p, m, e] = _dot(h, _bf(wtile(4 * m + (p >> 2), p & 3, e)))
                    t += 1
                    if m == 1 and e == 1:
                        pend.append((t + lat_s, "S", p))
                elif ready and ready[0][0] <= t and nwo < H - n_last:
                    _, hh = ready.pop(0)
                    acc = addl(acc, wo_dot(hh, oos[hh]))
                    t += 1
                    nwo += 1
                else:
                    t += 0.5
            for j in range(5):
                for _, hh in ready:
                    acc[j] = acc[j] + _dot(oos[hh], wo_t[j, 128 * hh:128 * hh + 128, :])
            out = jnp.concatenate(acc, axis=1)
            xa[16 + g, 32 * ph:32 * ph + 24, :] = out[8:32]
            mem = _round_bf16(out[0:8])
        return mem

    def dfwd_thunks(rows, tail):
        st = {}

        def pre():
            o = to[...] if tail else xa[16:32, rows, :]
            x = _round_bf16(xa[0:16, rows, :] + o)
            xb[:, rows, :] = x
            y = _layernorm(x.reshape(128, DM))
            x0, x1, x2, x3, x4 = [y[:, 128 * a:128 * a + 128] for a in range(5)]
            t1, t2, t3, t4 = x1 + x4, x2 + x3, x1 - x4, x2 - x3
            t = t1 + t2
            m, n = x0 - 0.25 * t, R5_D * (t1 - t2)
            st["u"] = [x0 + t, (m + n, t3 + R5_R * t4), (m - n, R5_R * t3 - t4)]

        def part(g):
            def run():
                if g == 0:
                    pre()
                    u0 = st["u"][0].astype(bf16)
                    zr = _dot(u0, _bf(small[0]))
                    if CFG["pack_f"]:
                        lane = lax.broadcasted_iota(jnp.int32, (128, 128), 1)
                        zi = jnp.where((lane & 63) == 0, 0.0, pltpu.roll(zr, 64, 1))
                    else:
                        zi = _dot(u0, _bf(small[1]))
                else:
                    a, b = st["u"][g]
                    k, kb, ka = [_dot(v.astype(bf16), _bf(small[3 * g - 1 + i]))
                                 for i, v in enumerate((a + b, b, a))]
                    zr, zi = k + kb, ka - _mu() * k
                ys = [(zr[8 * a:8 * a + 8], zi[8 * a:8 * a + 8]) for a in range(16)]
                if g < 2:
                    ys = _fft16(ys, -1)
                for a in range(16):
                    zs[g][0, a, rows, :] = ys[a][0]
                    zs[g][1, a, rows, :] = ys[a][1]
            return run
        return [part(g) for g in range(3)]

    def post(u, carry):
        base = pl.multiple_of(32 * u, 32)
        side = []
        for q in range(4):
            side += dfwd_thunks(pl.ds(base + 8 * q, 8), q == 3)
        side = [side[i] for i in CFG["post_order"]]
        k = 0
        at = list(CFG["post_at"])
        m = {}
        for prods in CFG["post_passes"]:
            acc = None
            for p in range(NPAIR):
                lhs = _strassen_lhs(*[
                    functools.partial(lambda r, e: qb[8 * r:8 * r + 8, u, 2 * p + e].reshape(64, 128), r, e)
                    for r in range(2) for e in range(2)])
                res = []
                for i in prods:
                    if i == 7:
                        oo = jnp.concatenate([qb[:, u, 2 * p + e].reshape(128, 128) for e in range(2)], axis=1)
                        res.append(_dot(oo.astype(bf16), wo_t[4, 256 * p:256 * p + 256, :]))
                        k += 2
                        continue
                    a = lhs[i]().astype(bf16)
                    for np_ in range(2):
                        if i in WS_SLOT:
                            w = ws[p, 5 * np_ + WS_SLOT[i]]
                        else:
                            kk = 0 if i == 1 else 1
                            w = wo_t[2 * np_ + kk, 256 * p + 128 * kk:256 * p + 128 * kk + 128, :]
                        res.append(_dot(a, w))
                    k += 1
                acc = addl(acc, res)
                while at and at[0] <= k:
                    at.pop(0)
                    side.pop(0)()
            for i in prods:
                m[i] = [acc.pop(0)] if i == 7 else [acc.pop(0), acc.pop(0)]
        cols = []
        for np_ in range(2):
            m1, m2, m3, m4, m5, m6, m7 = [m[i][np_] for i in range(7)]
            cols.append(jnp.concatenate([m1 + m4 - m5 + m7, m2 + m4], axis=0))
            cols.append(jnp.concatenate([m3 + m5, m1 - m2 + m3 + m6], axis=0))
        to[...] = jnp.concatenate(cols + m[7], axis=1).reshape(16, 8, DM)
        for f in side:
            f()
        return carry

    def spectral(zero):
        def fence(z):
            return z[0, zero, 128:ZPITCH, :]

        def radix(g, bb, sign):
            z = zs[g]
            toks = []

            def emit(q, y):
                for p in range(4):
                    z[0, q + 4 * p, chunk(bb), :] = y[p][0]
                    z[1, q + 4 * p, chunk(bb), :] = y[p][1]
                toks.append(fence(z))
            _fft16([(z[0, a, chunk(bb), :], z[1, a, chunk(bb), :]) for a in range(16)], sign, emit)
            return toks

        ys = {}

        def fwd(g, k2, toks):
            z = zs[g]
            ur, ui = z[0, k2, 0:64, :], z[1, k2, 0:64, :]
            tr, ti = _twiddle((z[0, k2, 64:128, :], z[1, k2, 64:128, :]), k2, 32, -1)
            for hf in range(2):
                v = _ilv(ur + tr, ui + ti) if hf == 0 else _ilv(ur - tr, ui - ti)
                lhs = _with_tokens(emat[k2 + 16 * hf], toks if hf == 0 else None)
                xr, xi = _dilv(_dot(_bf(lhs), v.astype(bf16)))
                ys["x", 16 * g + k2] = xr
                wr = wf[g, pl.ds(k2 * WPITCH + hf, 64, stride=2), :]
                wi = wf[g + 3, pl.ds(k2 * WPITCH + hf, 64, stride=2), :]
                ys[g, k2, hf] = _ilv(xr * wr - xi * wi, xr * wi + xi * wr).astype(bf16)

        def inv(g, k2, toks):
            z = zs[g]
            t0 = _dot(_bf(_with_tokens(emat[32 + k2], toks)), ys.pop((g, k2, 0)))
            t1 = _dot(_bf(emat[48 + k2]), ys.pop((g, k2, 1)))
            z[0, k2, 0:64, :], z[1, k2, 0:64, :] = _dilv(t0 + t1)
            z[0, k2, 64:128, :], z[1, k2, 64:128, :] = _twiddle(_dilv(t0 - t1), k2, 32, 1)

        units = [(g, k2) for g in range(3) for k2 in range(16)]
        toks = None
        lag = CFG["inv_lag"]
        for i in range(len(units) + lag):
            if i < len(units):
                fwd(*units[i], toks)
            if i >= lag:
                inv(*units[i - lag], toks if i >= len(units) else None)
            toks = []
            if i in CFG["fwd_at"]:
                toks += radix(2, CFG["fwd_at"].index(i), -1)
            for n, at in enumerate(CFG["inv_at"]):
                if at == i:
                    if not toks:
                        back, r = CFG["rel"]
                        zs[n // 16][1, zero, 128:ZPITCH, :] = ys["x", min(i - back, 47)][8 * r:8 * r + 8]
                    toks += radix(n // 16, n % 16, 1)
            pos = CFG["tok_pos"] if len(toks) <= 4 else range(8)
            toks = {j: pltpu.bitcast(t, u32) for j, t in zip(pos, toks)}

    def dinv_thunks(bb, finish):
        st = {}

        def part(g):
            def run():
                z = zs[g]
                ys = [(z[0, a, chunk(bb), :], z[1, a, chunk(bb), :]) for a in range(16)]
                if g >= CFG["inv_groups"]:
                    ys = _fft16(ys, 1)
                tr = jnp.concatenate([y[0] for y in ys], axis=0)
                ti = jnp.concatenate([y[1] for y in ys], axis=0)
                if g == 0 and CFG["pack_i"]:
                    lane = lax.broadcasted_iota(jnp.int32, (128, 128), 1)
                    v = jnp.where(lane <= 64, tr, pltpu.roll(ti, 64, 1))
                    st[0] = _dot(v.astype(bf16), _bf(small[8]))
                elif g == 0:
                    st[0] = _dot(tr.astype(bf16), _bf(small[8])) + _dot(ti.astype(bf16), _bf(small[9]))
                else:
                    k, ki, kr = [_dot(v.astype(bf16), _bf(small[7 + 3 * g + i]))
                                 for i, v in enumerate((tr + _mu() * ti, ti, tr))]
                    st[2 * g - 1], st[2 * g] = k + ki, k + kr
            return run

        def fin():
            p0, p1, q1, p2, q2 = [st[j] for j in range(5)]
            t = p1 + p2
            m, n = p0 - 0.25 * t, R5_D * (p1 - p2)
            e1, e2 = m + n, m - n
            o1, o2 = q1 + R5_R * q2, R5_R * q1 - q2
            y = jnp.concatenate([p0 + t, e1 - o1, e2 - o2, e2 + o2, e1 + o1], axis=1)
            finish(xb[:, chunk(bb), :].reshape(128, DM) + y)
        return [part(0), part(1), part(2), fin]

    def out_copy(bb):
        return pltpu.make_async_copy(xin.at[:, bb], out_hbm.at[:, bb], osem.at[bb])

    def layer(li, carry0):
        if full or CFG["only"] == "group":
            _loop("step", 0, 16, group, mem_ref[...].astype(f32))
        if full or CFG["only"] == "spec":
            _loop("post", 0, 4, post, 0, unroll=CFG["post_unroll"])

            with jax.named_scope("spectral"):
                spectral((li >> 1))
        if not full and CFG["only"] != "out":
            return carry0

        def run_chunks(th, order, lag):
            seq = [t[g] for t in th for g in order]
            for i in range(len(seq) + lag):
                if i < len(seq):
                    seq[i]()
                if i >= lag and (i - lag) % 3 == 2:
                    th[(i - lag) // 3][3]()

        @pl.when(li == 0)
        def _():
            with jax.named_scope("dinv_tails"):
                run_chunks([dinv_thunks(4 * u + 3, functools.partial(
                    lambda u, x: set_input(4 * u + 3, _round_bf16(x), u), u)) for u in range(4)],
                    *CFG["tails_order"])

            def batch(it, carry):
                bb = body_chunk(it)
                side = dinv_thunks(bb, lambda x: set_input(bb, _round_bf16(x), None))
                for k, f in enumerate(batch_thunks(it)):
                    f()
                    if k in CFG["dinv_at"]:
                        side.pop(0)()
                return carry
            _loop("batch", 0, 12, batch, 0, unroll=CFG["batch_unroll"])

        @pl.when(li == 1)
        def _():
            with jax.named_scope("dinv_out"):
                def store_out(bb, x):
                    xin[:, bb] = x.reshape(16, 8, DM).astype(bf16)
                    out_copy(bb).start()
                run_chunks([dinv_thunks(bb, functools.partial(store_out, bb)) for bb in range(16)],
                           *CFG["out_order"])
                for bb in range(16):
                    out_copy(bb).wait()
        return carry0

    if CFG["only"] != "pro":
        lax.fori_loop(0, 2, layer, 0)
    else:
        zero = zero_ref[0]
        xin[0, 0, :, 0:128] = (qb[zero, 0, 0] + wf[zero, 0:8, :] + xa[zero, 0:8, 0:128]).astype(bf16) + ws[zero, 0, 0:8, :]
        out_copy(0).start()
        out_copy(0).wait()


@functools.partial(jax.jit, static_argnames=("A_seg_len",))
def pallas_interleave_layers__memory_aug_recurrent_mem_tr__spectral_gfnet__prompt_kernel(
    A_x, A_mem0, A_Wq, A_Wk, A_Wv, A_Wo, A_seg_len, B_x, B_w_r, B_w_i,
):
    assert A_seg_len == SEG and A_x.shape == (1, S, DM)
    small, emat = _tables()
    hbm = pl.BlockSpec(memory_space=pltpu.HBM)
    out = pl.pallas_call(
        _kernel,
        out_shape=jax.ShapeDtypeStruct((16, 16, 8, DM), bf16),
        in_specs=[hbm] * 10,
        out_specs=hbm,
        scratch_shapes=[
            pltpu.VMEM((16, 16, 8, DM), bf16),
            pltpu.VMEM((33, 128, DM), f32),
            pltpu.VMEM((16, 128, DM), f32),
            pltpu.VMEM((16, 8, DM), f32),
            pltpu.VMEM((12, 2, 320, 8, DH), bf16),
            pltpu.VMEM((13, 8 * HPITCH, 128), u32),
            pltpu.VMEM((13, 8 * HPITCH, 128), u32),
            pltpu.VMEM((5, H * DH + 512, 128), bf16),
            pltpu.VMEM((19, 10, 128, 128), bf16),
            pltpu.VMEM((16, 4, 96, 8, 128), f32),
            pltpu.VMEM((2, 16, 64, 128), u32),
            pltpu.VMEM((2, 16, ZPITCH, 128), f32),
            pltpu.VMEM((2, 16, ZPITCH, 128), f32),
            pltpu.VMEM((2, 16, ZPITCH, 128), f32),
            pltpu.VMEM((6, 16 * WPITCH + 32, 128), f32),
            pltpu.VMEM((9, DF, 512), bf16),
            pltpu.VMEM((4, 328, 128), f32),
            pltpu.VMEM((SMALL_TILES, 64, 128), u32),
            pltpu.VMEM((64, 64, 128), u32),
            pltpu.VMEM((80, 80), f32),
            pltpu.VMEM((MEM, DM), bf16),
            pltpu.SMEM((1,), jnp.int32),
            pltpu.SemaphoreType.DMA((47,)),
            pltpu.SemaphoreType.DMA((16,)),
        ],
        compiler_params=pltpu.CompilerParams(vmem_limit_bytes=120 * 1024 * 1024,
                                             disable_semaphore_checks=True),
    )(
        A_x.reshape(16, 16, 8, DM), A_mem0.reshape(MEM, DM),
        *[w.reshape(2, 320, H, DH) for w in (A_Wq, A_Wk, A_Wv)], A_Wo.reshape(H * DH, DM), B_w_r.T, B_w_i.T,
        jnp.asarray(small), jnp.asarray(emat),
    )
    return out.reshape(1, S, DM)
```

```python
import functools
import math

import jax
import jax.numpy as jnp
import numpy as np
from jax import lax
import jax.experimental.pallas as pl
import jax.experimental.pallas.tpu as pltpu

f32, bf16, u32 = jnp.float32, jnp.bfloat16, jnp.uint32

S, DM, H, DH, MEM, SEG = 2048, 640, 32, 128, 8, 32
NSEG = S // SEG
NPAIR = H // 2
DF = DM // 2 + 1
EPS = 1e-5
WPITCH = 132

HPITCH = 164
ZPITCH = 136

S1 = math.sin(2 * math.pi / 5)
R5_D = (math.cos(2 * math.pi / 5) - math.cos(4 * math.pi / 5)) / 2
R5_R = math.sin(4 * math.pi / 5) / S1


def _to_bf16_bits(a):
    u = np.ascontiguousarray(a, dtype=np.float32).view(np.uint32).astype(np.uint64)
    return ((u + 0x7FFF + ((u >> 16) & 1)) >> 16).astype(np.uint32)


def _pack_rows(a):
    b = _to_bf16_bits(a)
    return b[..., 0::2, :] | (b[..., 1::2, :] << 16)


@functools.lru_cache(maxsize=None)
def _tables():
    b = np.arange(128)
    l0 = np.arange(0, DF, 5)
    l1 = np.concatenate([np.arange(1, 320, 5), np.arange(4, 320, 5)])
    l2 = np.concatenate([np.arange(2, 320, 5), np.arange(3, 320, 5)])
    sg = np.concatenate([np.ones(64), -np.ones(64)])

    def th(l):
        return 2 * np.pi * ((b[:, None] * l[None, :]) % DM) / DM

    sc = 1.0 / (S * DM)
    fw = np.zeros((8, 128, 128))
    iw = np.zeros((8, 128, 128))
    t = th(l0)
    cl = np.full((65, 1), 2.0)
    cl[0] = cl[-1] = 1.0
    fw[0, :, :65], fw[1, :, :65] = np.cos(t), -np.sin(t)
    iw[0, :65], iw[1, :65] = cl * np.cos(t.T) * sc, -cl * np.sin(t.T) * sc
    if CFG["pack_f"]:
        fw[0, :, 65:] = fw[1, :, 1:64]
    if CFG["pack_i"]:
        iw[0, 65:] = iw[1, 1:64]
    mu = S1 * sg
    for g, l in ((1, l1), (2, l2)):
        t = th(l)
        c, s = np.cos(t), np.sin(t)
        fw[3 * g - 1:3 * g + 2] = c, -mu * s - c, mu * c - s
        iw[3 * g - 1:3 * g + 2] = [2 * sc * m.T for m in (c, -s - mu * c, mu * s - c)]
    n = np.arange(64)
    order = np.concatenate([np.concatenate([np.arange(8) + 8 * j, np.arange(8) + 8 * j + 64])
                            for j in range(8)])
    e = np.zeros((2, 32, 128, 128))
    for k2 in range(32):
        t = 2 * np.pi * (((32 * n[:, None] + k2) * n[None, :]) % S) / S
        er, ei = np.cos(t), -np.sin(t)
        m = np.block([[er, -ei], [ei, er]])[order][:, order]
        e[0, k2], e[1, k2] = m, m.T
    small = np.concatenate([_pack_rows(fw), _pack_rows(iw)], axis=0)
    return small, _pack_rows(e).reshape(64, 64, 128)


SMALL_TILES = 16


def _loop(name, lo, hi, body, init, **kw):
    with jax.named_scope(name):
        return lax.fori_loop(lo, hi, body, init, **kw)


def _bf(x):
    return pltpu.bitcast(x, bf16)


def _dot(a, b):
    return jnp.dot(a, b, preferred_element_type=f32)


def _round_bf16(x):
    return x.astype(bf16).astype(f32)


def _layernorm(x):
    m = jnp.mean(x, axis=-1, keepdims=True)
    xc = x - m
    v = jnp.mean(xc * xc, axis=-1, keepdims=True)
    return xc * lax.rsqrt(v + EPS)


def _fft4(x, sign):
    (ar, ai), (br, bi), (cr, ci), (dr, di) = x
    t0r, t0i, t1r, t1i = ar + cr, ai + ci, ar - cr, ai - ci
    t2r, t2i, t3r, t3i = br + dr, bi + di, br - dr, bi - di
    y0, y2 = (t0r + t2r, t0i + t2i), (t0r - t2r, t0i - t2i)
    p, q = (t1r + t3i, t1i - t3r), (t1r - t3i, t1i + t3r)
    return [y0, p, y2, q] if sign < 0 else [y0, q, y2, p]


def _twiddle(z, n, period, sign):
    zr, zi = z
    n = n % period
    if n == 0:
        return z
    if 4 * n == period:
        return (-zi, zr) if sign > 0 else (zi, -zr)
    c, s = math.cos(2 * math.pi * n / period), sign * math.sin(2 * math.pi * n / period)
    if (8 * n) % period == 0:
        a, d = zr + zi, zr - zi
        if c * s > 0:
            return (d * c, a * c)
        return (a * c, d * s)
    return (zr * c - zi * s, zr * s + zi * c)


def _bsum(x, y, sign):
    x, y = x.astype(f32), y.astype(f32)
    return (x + y if sign > 0 else x - y).astype(bf16)


def _strassen_lhs(a11, a12, a21, a22):
    return [lambda: a11() + a22(), lambda: a21() + a22(), a11, a22,
            lambda: a11() + a12(), lambda: a21() - a11(), lambda: a12() - a22()]


def _strassen_rhs(b11, b12, b21, b22):
    return [lambda: _bsum(b11(), b22(), 1), b11, lambda: _bsum(b12(), b22(), -1),
            lambda: _bsum(b21(), b11(), -1), b22, lambda: _bsum(b11(), b12(), 1),
            lambda: _bsum(b21(), b22(), 1)]


WS_SLOT = {0: 0, 2: 1, 3: 2, 5: 3, 6: 4}


def _mu():
    lane = lax.broadcasted_iota(jnp.int32, (1, 128), 1)
    return jnp.where(lane < 64, S1, -S1).astype(f32)


def _ilv(r, i):
    n = r.shape[0] // 8
    return jnp.concatenate([r.reshape(n, 8, 128), i.reshape(n, 8, 128)], axis=1).reshape(16 * n, 128)


def _dilv(x):
    n = x.shape[0] // 16
    x = x.reshape(n, 16, 128)
    return x[:, :8].reshape(8 * n, 128), x[:, 8:].reshape(8 * n, 128)


def _with_tokens(x, toks):
    if not toks:
        return x
    return jnp.concatenate(
        [x[8 * j:8 * j + 8] | toks[j] if j in toks else x[8 * j:8 * j + 8]
         for j in range(x.shape[0] // 8)], axis=0)


def _fft16(x, sign, emit=None):
    cols = [_fft4([x[4 * j + r] for j in range(4)], sign) for r in range(4)]
    out = [None] * 16
    for q in range(4):
        y = _fft4([_twiddle(cols[r][q], r * q, 16, sign) for r in range(4)], sign)
        for p in range(4):
            out[q + 4 * p] = y[p]
        if emit is not None:
            emit(q, y)
    return out


CFG = dict(steps=((4.5, 16.5, 6, 4, 0, 8), (5, 16.5, 5, 7, 8, 12), (5, 16.5, 6, 6, 8, 12), (5, 16.5, 8, 7, 8, 0)),
           post_dl=20, post_passes=((0, 1), (2, 3), (4, 5), (6, 7)),
           post_order=(0, 1, 6, 3, 4, 2, 8, 5, 7, 9, 10, 11), post_at=(22, 26, 68, 96),
           tails_order=((1, 2, 0), 5), out_order=((1, 2, 0), 5), pack_f=True, pack_i=True,
           inv_at=tuple(range(28, 44)), inv_groups=1, inv_lag=4, tok_pos=(4, 5, 6, 7),
           fwd_at=(7, 8, 9, 10, 12, 13, 14, 16, 17, 18, 20, 21, 22, 24, 25, 26), rel=(0, 1), dinv_at=(8, 9, 10, 11), batch_unroll=2, post_unroll=1,
           ws_split=8, ws_at=tuple(range(32)), pro_nre=14, re_pos=(3, 5, 7), ln_at=(22, 29, 31, 31), ln_at2=(4, 7, 10, 13),
           perm_at=tuple(range(12, 24)), only=None)


def _interleave(main, side):
    n, k = len(main), 0
    for i, f in enumerate(main):
        f()
        while k < len(side) and (k + 1) * n <= (i + 1) * len(side):
            side[k]()
            k += 1
    for f in side[k:]:
        f()


def _kernel(x_hbm, mem_hbm, wq_hbm, wk_hbm, wv_hbm, wo_hbm, wr_hbm, wi_hbm,
            small_hbm, e_hbm, out_hbm,
            xin, xa, xb, to, raw, wa, wb, wo_t, ws, qb, hl, z0, z1, z2, wf,
            wri, wtmp, small, emat, fill_ref, mem_ref, zero_ref, sem, osem):
    zs = (z0, z1, z2)
    w_hbm = (wq_hbm, wk_hbm, wv_hbm)

    def body_chunk(i):
        return 4 * (i & 3) + (i >> 2)

    def cp_w(i):
        src = w_hbm[i >> 2].at[:, :, pl.ds(8 * (i & 3), 8), :] if isinstance(i, int) else raw.at[i]
        return pltpu.make_async_copy(src, raw.at[i], sem.at[i])

    def cp_x(bb):
        return pltpu.make_async_copy(x_hbm.at[:, bb], xin.at[:, bb], sem.at[12 + bb])

    def cp_f(i):
        src = ((wr_hbm, wi_hbm)[i >> 2].at[:, pl.ds(512 * (i & 3), 512)]
               if isinstance(i, int) else wri.at[i])
        return pltpu.make_async_copy(src, wri.at[i], sem.at[36 + i])

    def cp_wo(i):
        rows = pl.ds(pl.multiple_of(512 * i, 512), 512)
        return [pltpu.make_async_copy(wo_hbm.at[rows, pl.ds(128 * j, 128)], wo_t.at[j, rows], sem.at[28 + i])
                for j in range(5)]

    cp_rest = [pltpu.make_async_copy(mem_hbm, mem_ref, sem.at[46]),
                pltpu.make_async_copy(small_hbm, small, sem.at[44]),
               pltpu.make_async_copy(e_hbm, emat, sem.at[45])]

    full = CFG["only"] in (None, "pro")
    for u in range(4 if full else 0):
        cp_x(4 * u + 3).start()
    if full:
        cp_w(0).start()
    for i in range(12 if full else 0):
        if i < 11:
            cp_w(i + 1).start()
        cp_x(body_chunk(i)).start()
        if 3 <= i < 11:
            cp_f(i - 3).start()
            for cp in cp_wo(i - 3):
                cp.start()
    for cp in cp_rest if full else ():
        cp.start()

    zero_ref[0] = 0

    r = lax.broadcasted_iota(jnp.int32, (80, 80), 0)
    c = lax.broadcasted_iota(jnp.int32, (80, 80), 1)

    def head(i):
        return jnp.where(i < 64, i // 32, (i - 64) // 8)

    def pos(i):
        return jnp.where(i < 64, i % 32, 32 + (i - 64) % 8)

    ok = (pos(r) < MEM) | (pos(r) >= pos(c))
    fill_ref[...] = jnp.where(head(r) == head(c), jnp.where(ok, 0.0, -1e9), -jnp.inf).astype(f32)
    wtmp[:, 320:328, :] = jnp.zeros((4, 8, 128), f32)
    xa[32, 0:8, 0:128] = jnp.zeros((8, 128), f32)
    ws[18, 0, 0:16, :] = jnp.zeros((16, 128), bf16)
    wa[12, 0:8, :] = jnp.zeros((8, 128), u32)
    wb[12, 0:8, :] = jnp.zeros((8, 128), u32)
    wf[5, 16 * WPITCH:16 * WPITCH + 8, :] = jnp.zeros((8, 128), f32)
    for z in zs:
        z[0, 0, 128:ZPITCH, :] = jnp.zeros((8, 128), f32)

    def chunk(bb):
        if isinstance(bb, int):
            return slice(8 * bb, 8 * bb + 8)
        return pl.ds(pl.multiple_of(8 * bb, 8), 8)

    def set_input(bb, x, tail_u, a0=0):
        n = x.shape[0] // 8
        xa[a0:a0 + n, chunk(bb), :] = x.reshape(n, 8, DM)
        y = _layernorm(x)
        if tail_u is None:
            xa[16 + a0:16 + a0 + n, chunk(bb), :] = y.reshape(n, 8, DM)
        else:
            blk = [[y[64 * r:64 * r + 64, 128 * kt:128 * kt + 128] for kt in range(5)] for r in range(2)]
            ops = []
            for kp in range(2):
                (a11, a12), (a21, a22) = [blk[r][2 * kp:2 * kp + 2] for r in range(2)]
                ops += [a11 + a22, a21 + a22, a11, a22, a11 + a12, a21 - a11, a12 - a22]
            for i, v in enumerate(ops + [blk[0][4], blk[1][4]]):
                hl[tail_u >> 1, i, 32 * (tail_u & 1):32 * (tail_u & 1) + 32, :] = (
                    pltpu.bitcast(v.astype(bf16), u32))

    def load_x(bb, a0=0, n=16):
        return xin[a0:a0 + n, bb].astype(f32).reshape(8 * n, DM)

    def wtile(cid, j, e):
        w = (wa, wb)[e]
        return jnp.concatenate([w[cid, (4 * hf + j) * HPITCH:(4 * hf + j) * HPITCH + 160, :]
                                for hf in range(2)], axis=0)

    def relayout(i, cid, e):
        for r in range(4 * i, 4 * i + 4):
            a, b = [pltpu.bitcast(raw[cid, :, d].reshape(16, 128), u32) for d in (2 * r, 2 * r + 1)]
            v = (a & 0xFFFF) | (b << 16) if e == 0 else (a >> 16) | (b & jnp.uint32(0xFFFF0000))
            (wa, wb)[e][cid, pl.ds(r, 8, stride=HPITCH), :] = v

    def batch_thunks(cid):
        def unit(e, jp, s):
            c = {}

            def w(n, kt):
                return _bf(wtile(cid, 2 * jp + n, e)[64 * kt:64 * kt + 64])

            def rhs(i, kp):
                return _strassen_rhs(*[functools.partial(w, n, 2 * kp + k)
                                       for k in range(2) for n in range(2)])[i]()

            def prod(i, toks=None):
                l0, l1 = _bf(_with_tokens(hl[s, i], toks)), _bf(hl[s, 7 + i])
                return _dot(l0, rhs(i, 0)) + _dot(l1, rhs(i, 1))

            def last(r, n, toks=None):
                return _dot(_bf(_with_tokens(hl[s, 14 + r], toks)), w(n, 4))

            def store(r, n):
                y = c.pop((r, n)).reshape(2, 8, 8, 128)
                for k in range(2):
                    qb[8 * r:8 * r + 8, 2 * s + k, 8 * cid + 2 * (2 * jp + n) + e] = y[k]

            def t0(toks=None):
                c[1, 1] = last(1, 1, toks) + prod(5)
                m1 = prod(0)
                c[1, 1], c[0, 0] = c[1, 1] + m1, m1

            def t1(toks=None):
                c[0, 0] = c[0, 0] + last(0, 0, toks) + prod(6)
                m2 = prod(1)
                c[1, 1], c[1, 0] = c[1, 1] - m2, m2

            def t2(toks=None):
                m3 = prod(2, toks)
                c[1, 1] = c[1, 1] + m3
                store(1, 1)
                m5 = prod(4)
                c[0, 1], c[0, 0] = m3 + m5, c[0, 0] - m5

            def t3(toks=None):
                c[0, 1] = c[0, 1] + last(0, 1, toks)
                store(0, 1)
                m4 = prod(3)
                c[0, 0] = c[0, 0] + m4
                store(0, 0)
                c[1, 0] = c[1, 0] + m4 + last(1, 0)
                store(1, 0)
            return [t0, t1, t2, t3]
        return [f for e in range(2) for jp in range(2) for s in range(2) for f in unit(e, jp, s)]

    def wperm_thunks(piece, j):
        m = (piece >> 2) & 1
        wt = wtmp.at[j]

        def load():
            wt[0:DF, :] = wri[piece, :, 128 * j:128 * j + 128].astype(f32)

        def one(g):
            def run():
                if g == 0:
                    t = jnp.concatenate([wt[pl.ds(0, 64, stride=5), :], wt[320:328, :],
                                         jnp.zeros((56, 128), f32)], axis=0)
                else:
                    t = jnp.concatenate([wt[pl.ds(g, 64, stride=5), :],
                                         wt[pl.ds(5 - g, 64, stride=5), :]], axis=0)
                y = t.T
                sub = wf.at[3 * m + g, pl.ds(pl.multiple_of((piece & 3) * 32, 32), 16 * WPITCH - 96)]
                for k in range(8):
                    for hf in range(2):
                        sub[pl.ds(8 * j + k + 8 * hf * WPITCH, 8, stride=WPITCH), :] = (
                            y[16 * k + 8 * hf:16 * k + 8 * hf + 8])
            return run
        return [load] + [one(g) for g in range(3)]

    def half_pass(cid, half, fill, zero, timed=()):
        nre = CFG["pro_nre"]
        toks = None
        for k, f in enumerate(batch_thunks(cid)[16 * half:16 * half + 16]):
            f(toks)
            toks = {}
            for n, f in enumerate(f for at, f in timed if at == k):
                toks[(0, 4, 1, 6)[n]] = f()
            if fill is not None:
                for n, r in enumerate(r for r in range(40) if r * nre // 40 == k):
                    relayout(r, fill, 1 - half)
                    toks[CFG["re_pos"][n]] = (wb, wa)[half][12 + zero, 0:8, :]

    def ln_parts(bb, zero):
        def part(j):
            set_input(bb, load_x(bb, 4 * j, 4), None, 4 * j)
            return pltpu.bitcast(xa[32 + zero, 0:8, 0:128], u32)
        return [functools.partial(part, j) for j in range(4)]

    def perm_parts(piece, zero):
        def part(fs):
            for f in fs:
                f()
            return pltpu.bitcast(wf[5 + zero, 16 * WPITCH:16 * WPITCH + 8, :], u32)
        out = []
        for j in range(4):
            th = wperm_thunks(piece, j)
            out += [functools.partial(part, th[0:2]), functools.partial(part, th[2:3]),
                    functools.partial(part, th[3:4])]
        return out

    def ws_parts(piece, zero):
        nr = 128 // CFG["ws_split"]

        def part(pp, np_, r0):
            base = pl.multiple_of(512 * piece, 512) + 256 * pp + r0

            def tile(k, n):
                return wo_t[2 * np_ + n, pl.ds(base + 128 * k, nr), :]
            rhs = _strassen_rhs(*[functools.partial(tile, k, n) for k in range(2) for n in range(2)])
            for i, slot in WS_SLOT.items():
                ws[2 * piece + pp, 5 * np_ + slot, r0:r0 + nr, :] = rhs[i]()
            return pltpu.bitcast(ws[18 + zero, 0, 0:16, :], u32)
        return [functools.partial(part, pp, np_, r0)
                for pp in range(2) for np_ in range(2) for r0 in range(0, 128, nr)]

    def pro0():
        for u in range(4):
            cp_x(4 * u + 3).wait()
        for u in range(4):
            set_input(4 * u + 3, load_x(4 * u + 3), u)
        cp_w(0).wait()
        zero = zero_ref[0]
        for i in range(40):
            relayout(i, 0, 0)
        half_pass(0, 0, zero, zero)

    def pro1(it, carry):
        bb = body_chunk(it)
        with jax.named_scope("pro1_wait"):
            cp_w(it + 1).wait()

            @pl.when(it >= 3)
            def _():
                cp_f(it - 3).wait()
                for cp in cp_wo(it - 3):
                    cp.wait()
            cp_x(bb).wait()
        piece = jnp.where(it >= 3, it - 3, 8)
        zero = it >> 4
        timed = sorted(list(zip(CFG["ln_at"], ln_parts(bb, zero)))
                       + list(zip(CFG["ws_at"], ws_parts(piece, zero)))
                       + list(zip(CFG["perm_at"], perm_parts(piece, zero))), key=lambda x: x[0])
        half_pass(it, 1, it + 1, zero, [x for x in timed if x[0] < 16])
        half_pass(it + 1, 0, it + 1, zero, [(k - 16, f) for k, f in timed if k >= 16])
        return carry

    def pro2():
        cp_x(body_chunk(11)).wait()
        for cp in cp_rest:
            cp.wait()
        zero = zero_ref[0]
        half_pass(11, 1, None, zero, list(zip(CFG["ln_at2"], ln_parts(body_chunk(11), zero))))

    if full:
        with jax.named_scope("pro0"):
            pro0()
        _loop("pro1", 0, 11, pro1, 0)
        with jax.named_scope("pro2"):
            pro2()

    scale = DH ** -0.5

    def wo_dot(hh, oo):
        return [_dot(oo, wo_t[j, 128 * hh:128 * hh + 128, :]) for j in range(5)]

    def addl(acc, res):
        return res if acc is None else [a + b for a, b in zip(acc, res)]

    def group(g, mem):
        for ph in range(4):
            h = jnp.concatenate([mem, xa[16 + g, 32 * ph:32 * ph + 24, :]], axis=0).astype(bf16)
            pr, sm, oos = {}, {}, {}
            lat_s, lat_pv, lat_wo, v_delay, n_first, n_last = CFG["steps"][ph]

            def stacked(p, m):
                tails = [qb[g, ph, 32 * m + 2 * p + e] for e in range(2)]
                return jnp.concatenate([pr[p, m, 0], pr[p, m, 1]] + tails, axis=0).astype(bf16)

            def scores(p):
                sc = lax.dot_general(stacked(p, 0), stacked(p, 1), (((1,), (1,)), ((), ())),
                                     preferred_element_type=f32)
                fill = fill_ref[...]
                sc = jnp.where(fill == 0.0, sc * scale, fill)
                mx = jnp.max(sc, axis=-1, keepdims=True)
                e = jnp.exp(sc - mx)
                rl = pl.reciprocal(jnp.sum(e, axis=-1, keepdims=True), approx=True)
                sm[p] = (e * rl).astype(bf16)

            def pv(p):
                o = _dot(sm[p], stacked(p, 2))
                for e in range(2):
                    qb[g, ph, 2 * p + e] = o[64 + 8 * e:72 + 8 * e]
                    oos[2 * p + e] = o[32 * e:32 * e + 32].astype(bf16)

            keyed = []
            for p in range(NPAIR):
                keyed += [(4 * p + 2 * m + e, (p, m, e)) for m in range(2) for e in range(2)]
                keyed += [(4 * p + 3.5 + v_delay, (p, 2, e)) for e in range(2)]
            bulk = [x for _, x in sorted(keyed, key=lambda kv: kv[0])]
            acc, t, nwo, pend, ready = None, 0.0, 0, [], []
            if n_first:
                first, bulk = bulk[:n_first], bulk[n_first:]
                for kt in range(5):
                    for p, m, e in first:
                        w = wtile(4 * m + (p >> 2), p & 3, e)[64 * kt:64 * kt + 64]
                        y = _dot(h[:, 128 * kt:128 * kt + 128], _bf(w))
                        pr[p, m, e] = y if kt == 0 else pr[p, m, e] + y
                t = float(len(first))
                pend = [(t + lat_s, "S", p) for p, m, e in first if m == 1 and e == 1]
            while nwo < H - n_last or pend:
                pend.sort()
                if pend and pend[0][0] <= t:
                    _, kind, p = pend.pop(0)
                    if kind == "S":
                        scores(p)
                        pend.append((t + lat_pv, "V", p))
                    else:
                        pv(p)
                        ready += [(t + lat_wo, 2 * p + e) for e in range(2)]
                    t += 0.5
                elif bulk:
                    p, m, e = bulk.pop(0)
                    pr[p, m, e] = _dot(h, _bf(wtile(4 * m + (p >> 2), p & 3, e)))
                    t += 1
                    if m == 1 and e == 1:
                        pend.append((t + lat_s, "S", p))
                elif ready and ready[0][0] <= t and nwo < H - n_last:
                    _, hh = ready.pop(0)
                    acc = addl(acc, wo_dot(hh, oos[hh]))
                    t += 1
                    nwo += 1
                else:
                    t += 0.5
            for j in range(5):
                for _, hh in ready:
                    acc[j] = acc[j] + _dot(oos[hh], wo_t[j, 128 * hh:128 * hh + 128, :])
            out = jnp.concatenate(acc, axis=1)
            xa[16 + g, 32 * ph:32 * ph + 24, :] = out[8:32]
            mem = _round_bf16(out[0:8])
        return mem

    def dfwd_thunks(rows, tail):
        st = {}

        def pre():
            o = to[...] if tail else xa[16:32, rows, :]
            x = _round_bf16(xa[0:16, rows, :] + o)
            xb[:, rows, :] = x
            y = _layernorm(x.reshape(128, DM))
            x0, x1, x2, x3, x4 = [y[:, 128 * a:128 * a + 128] for a in range(5)]
            t1, t2, t3, t4 = x1 + x4, x2 + x3, x1 - x4, x2 - x3
            t = t1 + t2
            m, n = x0 - 0.25 * t, R5_D * (t1 - t2)
            st["u"] = [x0 + t, (m + n, t3 + R5_R * t4), (m - n, R5_R * t3 - t4)]

        def part(g):
            def run():
                if g == 0:
                    pre()
                    u0 = st["u"][0].astype(bf16)
                    zr = _dot(u0, _bf(small[0]))
                    if CFG["pack_f"]:
                        lane = lax.broadcasted_iota(jnp.int32, (128, 128), 1)
                        zi = jnp.where((lane & 63) == 0, 0.0, pltpu.roll(zr, 64, 1))
                    else:
                        zi = _dot(u0, _bf(small[1]))
                else:
                    a, b = st["u"][g]
                    k, kb, ka = [_dot(v.astype(bf16), _bf(small[3 * g - 1 + i]))
                                 for i, v in enumerate((a + b, b, a))]
                    zr, zi = k + kb, ka - _mu() * k
                ys = [(zr[8 * a:8 * a + 8], zi[8 * a:8 * a + 8]) for a in range(16)]
                if g < 2:
                    ys = _fft16(ys, -1)
                for a in range(16):
                    zs[g][0, a, rows, :] = ys[a][0]
                    zs[g][1, a, rows, :] = ys[a][1]
            return run
        return [part(g) for g in range(3)]

    def post(u, carry):
        base = pl.multiple_of(32 * u, 32)
        side = []
        for q in range(4):
            side += dfwd_thunks(pl.ds(base + 8 * q, 8), q == 3)
        side = [side[i] for i in CFG["post_order"]]
        k = 0
        at = list(CFG["post_at"])
        m, due = {}, []
        for prods in CFG["post_passes"]:
            acc = None
            for p in range(NPAIR):
                lhs = _strassen_lhs(*[
                    functools.partial(lambda r, e: qb[8 * r:8 * r + 8, u, 2 * p + e].reshape(64, 128), r, e)
                    for r in range(2) for e in range(2)])
                res = []
                for i in prods:
                    if i == 7:
                        oo = jnp.concatenate([qb[:, u, 2 * p + e].reshape(128, 128) for e in range(2)], axis=1)
                        res.append(_dot(oo.astype(bf16), wo_t[4, 256 * p:256 * p + 256, :]))
                        k += 2
                        continue
                    a = lhs[i]().astype(bf16)
                    for np_ in range(2):
                        if i in WS_SLOT:
                            w = ws[p, 5 * np_ + WS_SLOT[i]]
                        else:
                            kk = 0 if i == 1 else 1
                            w = wo_t[2 * np_ + kk, 256 * p + 128 * kk:256 * p + 128 * kk + 128, :]
                        if due and due[0][0] <= k:
                            w = _bf(_with_tokens(pltpu.bitcast(w, u32), {0: due.pop(0)[1]}))
                        res.append(_dot(a, w))
                    k += 1
                acc = addl(acc, res)
                while at and at[0] <= k:
                    g = CFG["post_order"][len(CFG["post_at"]) - len(at)] % 3
                    at.pop(0)
                    side.pop(0)()
                    if g == 0 and CFG["post_dl"]:
                        due.append((k + CFG["post_dl"],
                                    pltpu.bitcast(z0[0, u >> 2, 128:ZPITCH, :], u32)))
            for i in prods:
                m[i] = [acc.pop(0)] if i == 7 else [acc.pop(0), acc.pop(0)]
        cols = []
        for np_ in range(2):
            m1, m2, m3, m4, m5, m6, m7 = [m[i][np_] for i in range(7)]
            cols.append(jnp.concatenate([m1 + m4 - m5 + m7, m2 + m4], axis=0))
            cols.append(jnp.concatenate([m3 + m5, m1 - m2 + m3 + m6], axis=0))
        to[...] = jnp.concatenate(cols + m[7], axis=1).reshape(16, 8, DM)
        for f in side:
            f()
        return carry

    def spectral(zero):
        def fence(z):
            return z[0, zero, 128:ZPITCH, :]

        def radix(g, bb, sign):
            z = zs[g]
            toks = []

            def emit(q, y):
                for p in range(4):
                    z[0, q + 4 * p, chunk(bb), :] = y[p][0]
                    z[1, q + 4 * p, chunk(bb), :] = y[p][1]
                toks.append(fence(z))
            _fft16([(z[0, a, chunk(bb), :], z[1, a, chunk(bb), :]) for a in range(16)], sign, emit)
            return toks

        ys = {}

        def fwd(g, k2, toks):
            z = zs[g]
            ur, ui = z[0, k2, 0:64, :], z[1, k2, 0:64, :]
            tr, ti = _twiddle((z[0, k2, 64:128, :], z[1, k2, 64:128, :]), k2, 32, -1)
            for hf in range(2):
                v = _ilv(ur + tr, ui + ti) if hf == 0 else _ilv(ur - tr, ui - ti)
                lhs = _with_tokens(emat[k2 + 16 * hf], toks if hf == 0 else None)
                xr, xi = _dilv(_dot(_bf(lhs), v.astype(bf16)))
                ys["x", 16 * g + k2] = xr
                wr = wf[g, pl.ds(k2 * WPITCH + hf, 64, stride=2), :]
                wi = wf[g + 3, pl.ds(k2 * WPITCH + hf, 64, stride=2), :]
                ys[g, k2, hf] = _ilv(xr * wr - xi * wi, xr * wi + xi * wr).astype(bf16)

        def inv(g, k2, toks):
            z = zs[g]
            t0 = _dot(_bf(_with_tokens(emat[32 + k2], toks)), ys.pop((g, k2, 0)))
            t1 = _dot(_bf(emat[48 + k2]), ys.pop((g, k2, 1)))
            z[0, k2, 0:64, :], z[1, k2, 0:64, :] = _dilv(t0 + t1)
            z[0, k2, 64:128, :], z[1, k2, 64:128, :] = _twiddle(_dilv(t0 - t1), k2, 32, 1)

        units = [(g, k2) for g in range(3) for k2 in range(16)]
        toks = None
        lag = CFG["inv_lag"]
        for i in range(len(units) + lag):
            if i < len(units):
                fwd(*units[i], toks)
            if i >= lag:
                inv(*units[i - lag], toks if i >= len(units) else None)
            toks = []
            if i in CFG["fwd_at"]:
                toks += radix(2, CFG["fwd_at"].index(i), -1)
            for n, at in enumerate(CFG["inv_at"]):
                if at == i:
                    if not toks:
                        back, r = CFG["rel"]
                        zs[n // 16][1, zero, 128:ZPITCH, :] = ys["x", min(i - back, 47)][8 * r:8 * r + 8]
                    toks += radix(n // 16, n % 16, 1)
            pos = CFG["tok_pos"] if len(toks) <= 4 else range(8)
            toks = {j: pltpu.bitcast(t, u32) for j, t in zip(pos, toks)}

    def dinv_thunks(bb, finish):
        st = {}

        def part(g):
            def run():
                z = zs[g]
                ys = [(z[0, a, chunk(bb), :], z[1, a, chunk(bb), :]) for a in range(16)]
                if g >= CFG["inv_groups"]:
                    ys = _fft16(ys, 1)
                tr = jnp.concatenate([y[0] for y in ys], axis=0)
                ti = jnp.concatenate([y[1] for y in ys], axis=0)
                if g == 0 and CFG["pack_i"]:
                    lane = lax.broadcasted_iota(jnp.int32, (128, 128), 1)
                    v = jnp.where(lane <= 64, tr, pltpu.roll(ti, 64, 1))
                    st[0] = _dot(v.astype(bf16), _bf(small[8]))
                elif g == 0:
                    st[0] = _dot(tr.astype(bf16), _bf(small[8])) + _dot(ti.astype(bf16), _bf(small[9]))
                else:
                    k, ki, kr = [_dot(v.astype(bf16), _bf(small[7 + 3 * g + i]))
                                 for i, v in enumerate((tr + _mu() * ti, ti, tr))]
                    st[2 * g - 1], st[2 * g] = k + ki, k + kr
            return run

        def fin():
            p0, p1, q1, p2, q2 = [st[j] for j in range(5)]
            t = p1 + p2
            m, n = p0 - 0.25 * t, R5_D * (p1 - p2)
            e1, e2 = m + n, m - n
            o1, o2 = q1 + R5_R * q2, R5_R * q1 - q2
            y = jnp.concatenate([p0 + t, e1 - o1, e2 - o2, e2 + o2, e1 + o1], axis=1)
            finish(xb[:, chunk(bb), :].reshape(128, DM) + y)
        return [part(0), part(1), part(2), fin]

    def out_copy(bb):
        return pltpu.make_async_copy(xin.at[:, bb], out_hbm.at[:, bb], osem.at[bb])

    def layer(li, carry0):
        if full or CFG["only"] == "group":
            _loop("step", 0, 16, group, mem_ref[...].astype(f32))
        if full or CFG["only"] == "spec":
            _loop("post", 0, 4, post, 0, unroll=CFG["post_unroll"])

            with jax.named_scope("spectral"):
                spectral((li >> 1))
        if not full and CFG["only"] != "out":
            return carry0

        def run_chunks(th, order, lag):
            seq = [t[g] for t in th for g in order]
            for i in range(len(seq) + lag):
                if i < len(seq):
                    seq[i]()
                if i >= lag and (i - lag) % 3 == 2:
                    th[(i - lag) // 3][3]()

        @pl.when(li == 0)
        def _():
            with jax.named_scope("dinv_tails"):
                run_chunks([dinv_thunks(4 * u + 3, functools.partial(
                    lambda u, x: set_input(4 * u + 3, _round_bf16(x), u), u)) for u in range(4)],
                    *CFG["tails_order"])

            def batch(it, carry):
                bb = body_chunk(it)
                side = dinv_thunks(bb, lambda x: set_input(bb, _round_bf16(x), None))
                for k, f in enumerate(batch_thunks(it)):
                    f()
                    if k in CFG["dinv_at"]:
                        side.pop(0)()
                return carry
            _loop("batch", 0, 12, batch, 0, unroll=CFG["batch_unroll"])

        @pl.when(li == 1)
        def _():
            with jax.named_scope("dinv_out"):
                def store_out(bb, x):
                    xin[:, bb] = x.reshape(16, 8, DM).astype(bf16)
                    out_copy(bb).start()
                run_chunks([dinv_thunks(bb, functools.partial(store_out, bb)) for bb in range(16)],
                           *CFG["out_order"])
                for bb in range(16):
                    out_copy(bb).wait()
        return carry0

    if CFG["only"] != "pro":
        lax.fori_loop(0, 2, layer, 0)
    else:
        zero = zero_ref[0]
        xin[0, 0, :, 0:128] = (qb[zero, 0, 0] + wf[zero, 0:8, :] + xa[zero, 0:8, 0:128]).astype(bf16) + ws[zero, 0, 0:8, :]
        out_copy(0).start()
        out_copy(0).wait()


@jax.jit
def pallas_interleave_layers__memory_aug_recurrent_mem_tr__spectral_gfnet__prompt_kernel(
    A_x, A_mem0, A_Wq, A_Wk, A_Wv, A_Wo, A_seg_len, B_x, B_w_r, B_w_i,
):
    assert A_x.shape == (1, S, DM) and A_mem0.shape == (1, MEM, DM)
    small, emat = _tables()
    hbm = pl.BlockSpec(memory_space=pltpu.HBM)
    out = pl.pallas_call(
        _kernel,
        out_shape=jax.ShapeDtypeStruct((16, 16, 8, DM), bf16),
        in_specs=[hbm] * 10,
        out_specs=hbm,
        scratch_shapes=[
            pltpu.VMEM((16, 16, 8, DM), bf16),
            pltpu.VMEM((33, 128, DM), f32),
            pltpu.VMEM((16, 128, DM), f32),
            pltpu.VMEM((16, 8, DM), f32),
            pltpu.VMEM((12, 2, 320, 8, DH), bf16),
            pltpu.VMEM((13, 8 * HPITCH, 128), u32),
            pltpu.VMEM((13, 8 * HPITCH, 128), u32),
            pltpu.VMEM((5, H * DH + 512, 128), bf16),
            pltpu.VMEM((19, 10, 128, 128), bf16),
            pltpu.VMEM((16, 4, 96, 8, 128), f32),
            pltpu.VMEM((2, 16, 64, 128), u32),
            pltpu.VMEM((2, 16, ZPITCH, 128), f32),
            pltpu.VMEM((2, 16, ZPITCH, 128), f32),
            pltpu.VMEM((2, 16, ZPITCH, 128), f32),
            pltpu.VMEM((6, 16 * WPITCH + 32, 128), f32),
            pltpu.VMEM((9, DF, 512), bf16),
            pltpu.VMEM((4, 328, 128), f32),
            pltpu.VMEM((SMALL_TILES, 64, 128), u32),
            pltpu.VMEM((64, 64, 128), u32),
            pltpu.VMEM((80, 80), f32),
            pltpu.VMEM((MEM, DM), bf16),
            pltpu.SMEM((1,), jnp.int32),
            pltpu.SemaphoreType.DMA((47,)),
            pltpu.SemaphoreType.DMA((16,)),
        ],
        compiler_params=pltpu.CompilerParams(vmem_limit_bytes=120 * 1024 * 1024,
                                             disable_semaphore_checks=True),
    )(
        A_x.reshape(16, 16, 8, DM), A_mem0.reshape(MEM, DM),
        *[w.reshape(2, 320, H, DH) for w in (A_Wq, A_Wk, A_Wv)], A_Wo.reshape(H * DH, DM), B_w_r.T, B_w_i.T,
        jnp.asarray(small), jnp.asarray(emat),
    )
    return out.reshape(1, S, DM)
```

```python
import functools
import math

import jax
import jax.numpy as jnp
import numpy as np
from jax import lax
import jax.experimental.pallas as pl
import jax.experimental.pallas.tpu as pltpu

f32, bf16, u32 = jnp.float32, jnp.bfloat16, jnp.uint32

S, DM, H, DH, MEM, SEG = 2048, 640, 32, 128, 8, 32
NSEG = S // SEG
NPAIR = H // 2
DF = DM // 2 + 1
EPS = 1e-5
WPITCH = 132

HPITCH = 164
ZPITCH = 136

S1 = math.sin(2 * math.pi / 5)
R5_D = (math.cos(2 * math.pi / 5) - math.cos(4 * math.pi / 5)) / 2
R5_R = math.sin(4 * math.pi / 5) / S1


def _to_bf16_bits(a):
    u = np.ascontiguousarray(a, dtype=np.float32).view(np.uint32).astype(np.uint64)
    return ((u + 0x7FFF + ((u >> 16) & 1)) >> 16).astype(np.uint32)


def _pack_rows(a):
    b = _to_bf16_bits(a)
    return b[..., 0::2, :] | (b[..., 1::2, :] << 16)


@functools.lru_cache(maxsize=None)
def _tables():
    b = np.arange(128)
    l0 = np.arange(0, DF, 5)
    l1 = np.concatenate([np.arange(1, 320, 5), np.arange(4, 320, 5)])
    l2 = np.concatenate([np.arange(2, 320, 5), np.arange(3, 320, 5)])
    sg = np.concatenate([np.ones(64), -np.ones(64)])

    def th(l):
        return 2 * np.pi * ((b[:, None] * l[None, :]) % DM) / DM

    sc = 1.0 / (S * DM)
    fw = np.zeros((8, 128, 128))
    iw = np.zeros((8, 128, 128))
    t = th(l0)
    cl = np.full((65, 1), 2.0)
    cl[0] = cl[-1] = 1.0
    fw[0, :, :65], fw[1, :, :65] = np.cos(t), -np.sin(t)
    iw[0, :65], iw[1, :65] = cl * np.cos(t.T) * sc, -cl * np.sin(t.T) * sc
    if CFG["pack_f"]:
        fw[0, :, 65:] = fw[1, :, 1:64]
    if CFG["pack_i"]:
        iw[0, 65:] = iw[1, 1:64]
    mu = S1 * sg
    for g, l in ((1, l1), (2, l2)):
        t = th(l)
        c, s = np.cos(t), np.sin(t)
        fw[3 * g - 1:3 * g + 2] = c, -mu * s - c, mu * c - s
        iw[3 * g - 1:3 * g + 2] = [2 * sc * m.T for m in (c, -s - mu * c, mu * s - c)]
    n = np.arange(64)
    order = np.concatenate([np.concatenate([np.arange(8) + 8 * j, np.arange(8) + 8 * j + 64])
                            for j in range(8)])
    e = np.zeros((2, 32, 128, 128))
    for k2 in range(32):
        t = 2 * np.pi * (((32 * n[:, None] + k2) * n[None, :]) % S) / S
        er, ei = np.cos(t), -np.sin(t)
        m = np.block([[er, -ei], [ei, er]])[order][:, order]
        e[0, k2], e[1, k2] = m, m.T
    small = np.concatenate([_pack_rows(fw), _pack_rows(iw)], axis=0)
    return small, _pack_rows(e).reshape(64, 64, 128)


SMALL_TILES = 16


def _loop(name, lo, hi, body, init, **kw):
    with jax.named_scope(name):
        return lax.fori_loop(lo, hi, body, init, **kw)


def _bf(x):
    return pltpu.bitcast(x, bf16)


def _dot(a, b):
    return jnp.dot(a, b, preferred_element_type=f32)


def _round_bf16(x):
    return x.astype(bf16).astype(f32)


def _layernorm(x):
    m = jnp.mean(x, axis=-1, keepdims=True)
    xc = x - m
    v = jnp.mean(xc * xc, axis=-1, keepdims=True)
    return xc * lax.rsqrt(v + EPS)


def _fft4(x, sign):
    (ar, ai), (br, bi), (cr, ci), (dr, di) = x
    t0r, t0i, t1r, t1i = ar + cr, ai + ci, ar - cr, ai - ci
    t2r, t2i, t3r, t3i = br + dr, bi + di, br - dr, bi - di
    y0, y2 = (t0r + t2r, t0i + t2i), (t0r - t2r, t0i - t2i)
    p, q = (t1r + t3i, t1i - t3r), (t1r - t3i, t1i + t3r)
    return [y0, p, y2, q] if sign < 0 else [y0, q, y2, p]


def _twiddle(z, n, period, sign):
    zr, zi = z
    n = n % period
    if n == 0:
        return z
    if 4 * n == period:
        return (-zi, zr) if sign > 0 else (zi, -zr)
    c, s = math.cos(2 * math.pi * n / period), sign * math.sin(2 * math.pi * n / period)
    if (8 * n) % period == 0:
        a, d = zr + zi, zr - zi
        if c * s > 0:
            return (d * c, a * c)
        return (a * c, d * s)
    return (zr * c - zi * s, zr * s + zi * c)


def _bsum(x, y, sign):
    x, y = x.astype(f32), y.astype(f32)
    return (x + y if sign > 0 else x - y).astype(bf16)


def _strassen_lhs(a11, a12, a21, a22):
    return [lambda: a11() + a22(), lambda: a21() + a22(), a11, a22,
            lambda: a11() + a12(), lambda: a21() - a11(), lambda: a12() - a22()]


def _strassen_rhs(b11, b12, b21, b22):
    return [lambda: _bsum(b11(), b22(), 1), b11, lambda: _bsum(b12(), b22(), -1),
            lambda: _bsum(b21(), b11(), -1), b22, lambda: _bsum(b11(), b12(), 1),
            lambda: _bsum(b21(), b22(), 1)]


WS_SLOT = {0: 0, 2: 1, 3: 2, 5: 3, 6: 4}


def _mu():
    lane = lax.broadcasted_iota(jnp.int32, (1, 128), 1)
    return jnp.where(lane < 64, S1, -S1).astype(f32)


def _ilv(r, i):
    n = r.shape[0] // 8
    return jnp.concatenate([r.reshape(n, 8, 128), i.reshape(n, 8, 128)], axis=1).reshape(16 * n, 128)


def _dilv(x):
    n = x.shape[0] // 16
    x = x.reshape(n, 16, 128)
    return x[:, :8].reshape(8 * n, 128), x[:, 8:].reshape(8 * n, 128)


def _with_tokens(x, toks):
    if not toks:
        return x
    return jnp.concatenate(
        [x[8 * j:8 * j + 8] | toks[j] if j in toks else x[8 * j:8 * j + 8]
         for j in range(x.shape[0] // 8)], axis=0)


def _fft16(x, sign, emit=None):
    cols = [_fft4([x[4 * j + r] for j in range(4)], sign) for r in range(4)]
    out = [None] * 16
    for q in range(4):
        y = _fft4([_twiddle(cols[r][q], r * q, 16, sign) for r in range(4)], sign)
        for p in range(4):
            out[q + 4 * p] = y[p]
        if emit is not None:
            emit(q, y)
    return out


CFG = dict(steps=((4.5, 16.5, 6, 4, 0, 8), (5, 16.5, 5, 7, 8, 12), (5, 16.5, 6, 6, 8, 12), (5, 16.5, 8, 7, 8, 0)),
           post_dl=20, post_passes=((0, 1), (2, 3), (4, 5), (6, 7)),
           post_order=(0, 1, 6, 3, 4, 2, 8, 5, 7, 9, 10, 11), post_at=(22, 26, 68, 96),
           tails_order=((1, 2, 0), 5), out_order=((1, 2, 0), 5), pack_f=True, pack_i=True,
           inv_at=tuple(range(28, 44)), inv_groups=1, inv_lag=4, tok_pos=(4, 5, 6, 7),
           fwd_at=(7, 8, 9, 10, 12, 13, 14, 16, 17, 18, 20, 21, 22, 24, 25, 26), rel=(0, 1), dinv_at=(8, 9, 10, 11), batch_unroll=2, post_unroll=1,
           ws_split=8, ws_at=tuple(range(32)), pro_nre=14, re_pos=(3, 5, 7), ln_at=(22, 29, 31, 31), ln_at2=(4, 7, 10, 13),
           perm_at=tuple(range(12, 24)), only=None)


def _interleave(main, side):
    n, k = len(main), 0
    for i, f in enumerate(main):
        f()
        while k < len(side) and (k + 1) * n <= (i + 1) * len(side):
            side[k]()
            k += 1
    for f in side[k:]:
        f()


def _kernel(x_hbm, mem_hbm, wq_hbm, wk_hbm, wv_hbm, wo_hbm, wr_hbm, wi_hbm,
            small_hbm, e_hbm, out_hbm,
            xin, xa, xb, to, raw, wa, wb, wo_t, ws, qb, hl, z0, z1, z2, wf,
            wri, wtmp, small, emat, fill_ref, mem_ref, zero_ref, sem, osem):
    zs = (z0, z1, z2)
    w_hbm = (wq_hbm, wk_hbm, wv_hbm)

    def body_chunk(i):
        return 4 * (i & 3) + (i >> 2)

    def cp_w(i):
        src = w_hbm[i >> 2].at[:, :, pl.ds(8 * (i & 3), 8), :] if isinstance(i, int) else raw.at[i]
        return pltpu.make_async_copy(src, raw.at[i], sem.at[i])

    def cp_x(bb):
        return pltpu.make_async_copy(x_hbm.at[:, bb], xin.at[:, bb], sem.at[12 + bb])

    def cp_f(i):
        src = ((wr_hbm, wi_hbm)[i >> 2].at[:, pl.ds(512 * (i & 3), 512)]
               if isinstance(i, int) else wri.at[i])
        return pltpu.make_async_copy(src, wri.at[i], sem.at[36 + i])

    def cp_wo(i):
        rows = pl.ds(pl.multiple_of(512 * i, 512), 512)
        return [pltpu.make_async_copy(wo_hbm.at[rows, pl.ds(128 * j, 128)], wo_t.at[j, rows], sem.at[28 + i])
                for j in range(5)]

    cp_rest = [pltpu.make_async_copy(mem_hbm, mem_ref, sem.at[46]),
                pltpu.make_async_copy(small_hbm, small, sem.at[44]),
               pltpu.make_async_copy(e_hbm, emat, sem.at[45])]

    full = CFG["only"] in (None, "pro")
    for u in range(4 if full else 0):
        cp_x(4 * u + 3).start()
    if full:
        cp_w(0).start()
    for i in range(12 if full else 0):
        if i < 11:
            cp_w(i + 1).start()
        cp_x(body_chunk(i)).start()
        if 3 <= i < 11:
            cp_f(i - 3).start()
            for cp in cp_wo(i - 3):
                cp.start()
    for cp in cp_rest if full else ():
        cp.start()

    zero_ref[0] = 0

    r = lax.broadcasted_iota(jnp.int32, (80, 80), 0)
    c = lax.broadcasted_iota(jnp.int32, (80, 80), 1)

    def head(i):
        return jnp.where(i < 64, i // 32, (i - 64) // 8)

    def pos(i):
        return jnp.where(i < 64, i % 32, 32 + (i - 64) % 8)

    ok = (pos(r) < MEM) | (pos(r) >= pos(c))
    fill_ref[...] = jnp.where(head(r) == head(c), jnp.where(ok, 0.0, -1e9), -jnp.inf).astype(f32)
    wtmp[:, 320:328, :] = jnp.zeros((4, 8, 128), f32)
    xa[32, 0:8, 0:128] = jnp.zeros((8, 128), f32)
    ws[18, 0, 0:16, :] = jnp.zeros((16, 128), bf16)
    wa[12, 0:8, :] = jnp.zeros((8, 128), u32)
    wb[12, 0:8, :] = jnp.zeros((8, 128), u32)
    wf[5, 16 * WPITCH:16 * WPITCH + 8, :] = jnp.zeros((8, 128), f32)
    for z in zs:
        z[0, 0, 128:ZPITCH, :] = jnp.zeros((8, 128), f32)

    def chunk(bb):
        if isinstance(bb, int):
            return slice(8 * bb, 8 * bb + 8)
        return pl.ds(pl.multiple_of(8 * bb, 8), 8)

    def set_input(bb, x, tail_u, a0=0):
        n = x.shape[0] // 8
        xa[a0:a0 + n, chunk(bb), :] = x.reshape(n, 8, DM)
        y = _layernorm(x)
        if tail_u is None:
            xa[16 + a0:16 + a0 + n, chunk(bb), :] = y.reshape(n, 8, DM)
        else:
            blk = [[y[64 * r:64 * r + 64, 128 * kt:128 * kt + 128] for kt in range(5)] for r in range(2)]
            ops = []
            for kp in range(2):
                (a11, a12), (a21, a22) = [blk[r][2 * kp:2 * kp + 2] for r in range(2)]
                ops += [a11 + a22, a21 + a22, a11, a22, a11 + a12, a21 - a11, a12 - a22]
            for i, v in enumerate(ops + [blk[0][4], blk[1][4]]):
                hl[tail_u >> 1, i, 32 * (tail_u & 1):32 * (tail_u & 1) + 32, :] = (
                    pltpu.bitcast(v.astype(bf16), u32))

    def load_x(bb, a0=0, n=16):
        return xin[a0:a0 + n, bb].astype(f32).reshape(8 * n, DM)

    def wtile(cid, j, e):
        w = (wa, wb)[e]
        return jnp.concatenate([w[cid, (4 * hf + j) * HPITCH:(4 * hf + j) * HPITCH + 160, :]
                                for hf in range(2)], axis=0)

    def relayout(i, cid, e):
        for r in range(4 * i, 4 * i + 4):
            a, b = [pltpu.bitcast(raw[cid, :, d].reshape(16, 128), u32) for d in (2 * r, 2 * r + 1)]
            v = (a & 0xFFFF) | (b << 16) if e == 0 else (a >> 16) | (b & jnp.uint32(0xFFFF0000))
            (wa, wb)[e][cid, pl.ds(r, 8, stride=HPITCH), :] = v

    def batch_thunks(cid):
        def unit(e, jp, s):
            c = {}

            def w(n, kt):
                return _bf(wtile(cid, 2 * jp + n, e)[64 * kt:64 * kt + 64])

            def rhs(i, kp):
                return _strassen_rhs(*[functools.partial(w, n, 2 * kp + k)
                                       for k in range(2) for n in range(2)])[i]()

            def prod(i, toks=None):
                l0, l1 = _bf(_with_tokens(hl[s, i], toks)), _bf(hl[s, 7 + i])
                return _dot(l0, rhs(i, 0)) + _dot(l1, rhs(i, 1))

            def last(r, n, toks=None):
                return _dot(_bf(_with_tokens(hl[s, 14 + r], toks)), w(n, 4))

            def store(r, n):
                y = c.pop((r, n)).reshape(2, 8, 8, 128)
                for k in range(2):
                    qb[8 * r:8 * r + 8, 2 * s + k, 8 * cid + 2 * (2 * jp + n) + e] = y[k]

            def t0(toks=None):
                c[1, 1] = last(1, 1, toks) + prod(5)
                m1 = prod(0)
                c[1, 1], c[0, 0] = c[1, 1] + m1, m1

            def t1(toks=None):
                c[0, 0] = c[0, 0] + last(0, 0, toks) + prod(6)
                m2 = prod(1)
                c[1, 1], c[1, 0] = c[1, 1] - m2, m2

            def t2(toks=None):
                m3 = prod(2, toks)
                c[1, 1] = c[1, 1] + m3
                store(1, 1)
                m5 = prod(4)
                c[0, 1], c[0, 0] = m3 + m5, c[0, 0] - m5

            def t3(toks=None):
                c[0, 1] = c[0, 1] + last(0, 1, toks)
                store(0, 1)
                m4 = prod(3)
                c[0, 0] = c[0, 0] + m4
                store(0, 0)
                c[1, 0] = c[1, 0] + m4 + last(1, 0)
                store(1, 0)
            return [t0, t1, t2, t3]
        return [f for e in range(2) for jp in range(2) for s in range(2) for f in unit(e, jp, s)]

    def wperm_thunks(piece, j):
        m = (piece >> 2) & 1
        wt = wtmp.at[j]

        def load():
            wt[0:DF, :] = wri[piece, :, 128 * j:128 * j + 128].astype(f32)

        def one(g):
            def run():
                if g == 0:
                    t = jnp.concatenate([wt[pl.ds(0, 64, stride=5), :], wt[320:328, :],
                                         jnp.zeros((56, 128), f32)], axis=0)
                else:
                    t = jnp.concatenate([wt[pl.ds(g, 64, stride=5), :],
                                         wt[pl.ds(5 - g, 64, stride=5), :]], axis=0)
                y = t.T
                sub = wf.at[3 * m + g, pl.ds(pl.multiple_of((piece & 3) * 32, 32), 16 * WPITCH - 96)]
                for k in range(8):
                    for hf in range(2):
                        sub[pl.ds(8 * j + k + 8 * hf * WPITCH, 8, stride=WPITCH), :] = (
                            y[16 * k + 8 * hf:16 * k + 8 * hf + 8])
            return run
        return [load] + [one(g) for g in range(3)]

    def half_pass(cid, half, fill, zero, timed=()):
        nre = CFG["pro_nre"]
        toks = None
        for k, f in enumerate(batch_thunks(cid)[16 * half:16 * half + 16]):
            f(toks)
            toks = {}
            for n, f in enumerate(f for at, f in timed if at == k):
                toks[(0, 4, 1, 6)[n]] = f()
            if fill is not None:
                for n, r in enumerate(r for r in range(40) if r * nre // 40 == k):
                    relayout(r, fill, 1 - half)
                    toks[CFG["re_pos"][n]] = (wb, wa)[half][12 + zero, 0:8, :]

    def ln_parts(bb, zero):
        def part(j):
            set_input(bb, load_x(bb, 4 * j, 4), None, 4 * j)
            return pltpu.bitcast(xa[32 + zero, 0:8, 0:128], u32)
        return [functools.partial(part, j) for j in range(4)]

    def perm_parts(piece, zero):
        def part(fs):
            for f in fs:
                f()
            return pltpu.bitcast(wf[5 + zero, 16 * WPITCH:16 * WPITCH + 8, :], u32)
        out = []
        for j in range(4):
            th = wperm_thunks(piece, j)
            out += [functools.partial(part, th[0:2]), functools.partial(part, th[2:3]),
                    functools.partial(part, th[3:4])]
        return out

    def ws_parts(piece, zero):
        nr = 128 // CFG["ws_split"]

        def part(pp, np_, r0):
            base = pl.multiple_of(512 * piece, 512) + 256 * pp + r0

            def tile(k, n):
                return wo_t[2 * np_ + n, pl.ds(base + 128 * k, nr), :]
            rhs = _strassen_rhs(*[functools.partial(tile, k, n) for k in range(2) for n in range(2)])
            for i, slot in WS_SLOT.items():
                ws[2 * piece + pp, 5 * np_ + slot, r0:r0 + nr, :] = rhs[i]()
            return pltpu.bitcast(ws[18 + zero, 0, 0:16, :], u32)
        return [functools.partial(part, pp, np_, r0)
                for pp in range(2) for np_ in range(2) for r0 in range(0, 128, nr)]

    def pro0():
        for u in range(4):
            cp_x(4 * u + 3).wait()
        for u in range(4):
            set_input(4 * u + 3, load_x(4 * u + 3), u)
        cp_w(0).wait()
        zero = zero_ref[0]
        for i in range(40):
            relayout(i, 0, 0)
        half_pass(0, 0, zero, zero)

    def pro1(it, carry):
        bb = body_chunk(it)
        with jax.named_scope("pro1_wait"):
            cp_w(it + 1).wait()

            @pl.when(it >= 3)
            def _():
                cp_f(it - 3).wait()
                for cp in cp_wo(it - 3):
                    cp.wait()
            cp_x(bb).wait()
        piece = jnp.where(it >= 3, it - 3, 8)
        zero = it >> 4
        timed = sorted(list(zip(CFG["ln_at"], ln_parts(bb, zero)))
                       + list(zip(CFG["ws_at"], ws_parts(piece, zero)))
                       + list(zip(CFG["perm_at"], perm_parts(piece, zero))), key=lambda x: x[0])
        half_pass(it, 1, it + 1, zero, [x for x in timed if x[0] < 16])
        half_pass(it + 1, 0, it + 1, zero, [(k - 16, f) for k, f in timed if k >= 16])
        return carry

    def pro2():
        cp_x(body_chunk(11)).wait()
        for cp in cp_rest:
            cp.wait()
        zero = zero_ref[0]
        half_pass(11, 1, None, zero, list(zip(CFG["ln_at2"], ln_parts(body_chunk(11), zero))))

    if full:
        with jax.named_scope("pro0"):
            pro0()
        _loop("pro1", 0, 11, pro1, 0)
        with jax.named_scope("pro2"):
            pro2()

    scale = DH ** -0.5

    def wo_dot(hh, oo):
        return [_dot(oo, wo_t[j, 128 * hh:128 * hh + 128, :]) for j in range(5)]

    def addl(acc, res):
        return res if acc is None else [a + b for a, b in zip(acc, res)]

    def group(g, mem):
        for ph in range(4):
            h = jnp.concatenate([mem, xa[16 + g, 32 * ph:32 * ph + 24, :]], axis=0).astype(bf16)
            pr, sm, oos = {}, {}, {}
            lat_s, lat_pv, lat_wo, v_delay, n_first, n_last = CFG["steps"][ph]

            def stacked(p, m):
                tails = [qb[g, ph, 32 * m + 2 * p + e] for e in range(2)]
                return jnp.concatenate([pr[p, m, 0], pr[p, m, 1]] + tails, axis=0).astype(bf16)

            def scores(p):
                sc = lax.dot_general(stacked(p, 0), stacked(p, 1), (((1,), (1,)), ((), ())),
                                     preferred_element_type=f32)
                fill = fill_ref[...]
                sc = jnp.where(fill == 0.0, sc * scale, fill)
                mx = jnp.max(sc, axis=-1, keepdims=True)
                e = jnp.exp(sc - mx)
                rl = pl.reciprocal(jnp.sum(e, axis=-1, keepdims=True), approx=True)
                sm[p] = (e * rl).astype(bf16)

            def pv(p):
                o = _dot(sm[p], stacked(p, 2))
                for e in range(2):
                    qb[g, ph, 2 * p + e] = o[64 + 8 * e:72 + 8 * e]
                    oos[2 * p + e] = o[32 * e:32 * e + 32].astype(bf16)

            keyed = []
            for p in range(NPAIR):
                keyed += [(4 * p + 2 * m + e, (p, m, e)) for m in range(2) for e in range(2)]
                keyed += [(4 * p + 3.5 + v_delay, (p, 2, e)) for e in range(2)]
            bulk = [x for _, x in sorted(keyed, key=lambda kv: kv[0])]
            acc, t, nwo, pend, ready = None, 0.0, 0, [], []
            if n_first:
                first, bulk = bulk[:n_first], bulk[n_first:]
                for kt in range(5):
                    for p, m, e in first:
                        w = wtile(4 * m + (p >> 2), p & 3, e)[64 * kt:64 * kt + 64]
                        y = _dot(h[:, 128 * kt:128 * kt + 128], _bf(w))
                        pr[p, m, e] = y if kt == 0 else pr[p, m, e] + y
                t = float(len(first))
                pend = [(t + lat_s, "S", p) for p, m, e in first if m == 1 and e == 1]
            while nwo < H - n_last or pend:
                pend.sort()
                if pend and pend[0][0] <= t:
                    _, kind, p = pend.pop(0)
                    if kind == "S":
                        scores(p)
                        pend.append((t + lat_pv, "V", p))
                    else:
                        pv(p)
                        ready += [(t + lat_wo, 2 * p + e) for e in range(2)]
                    t += 0.5
                elif bulk:
                    p, m, e = bulk.pop(0)
                    pr[p, m, e] = _dot(h, _bf(wtile(4 * m + (p >> 2), p & 3, e)))
                    t += 1
                    if m == 1 and e == 1:
                        pend.append((t + lat_s, "S", p))
                elif ready and ready[0][0] <= t and nwo < H - n_last:
                    _, hh = ready.pop(0)
                    acc = addl(acc, wo_dot(hh, oos[hh]))
                    t += 1
                    nwo += 1
                else:
                    t += 0.5
            for j in range(5):
                for _, hh in ready:
                    acc[j] = acc[j] + _dot(oos[hh], wo_t[j, 128 * hh:128 * hh + 128, :])
            out = jnp.concatenate(acc, axis=1)
            xa[16 + g, 32 * ph:32 * ph + 24, :] = out[8:32]
            mem = _round_bf16(out[0:8])
        return mem

    def dfwd_thunks(seg, q):
        st = {}
        rows = chunk(q)
        xav, xbv, zv = xa.at[:, seg], xb.at[:, seg], [z.at[:, :, seg] for z in zs]

        def pre():
            o = to[...] if q == 3 else xav[16:32, rows, :]
            x = _round_bf16(xav[0:16, rows, :] + o)
            xbv[:, rows, :] = x
            y = _layernorm(x.reshape(128, DM))
            x0, x1, x2, x3, x4 = [y[:, 128 * a:128 * a + 128] for a in range(5)]
            t1, t2, t3, t4 = x1 + x4, x2 + x3, x1 - x4, x2 - x3
            t = t1 + t2
            m, n = x0 - 0.25 * t, R5_D * (t1 - t2)
            st["u"] = [x0 + t, (m + n, t3 + R5_R * t4), (m - n, R5_R * t3 - t4)]

        def part(g):
            def run():
                if g == 0:
                    pre()
                    u0 = st["u"][0].astype(bf16)
                    zr = _dot(u0, _bf(small[0]))
                    if CFG["pack_f"]:
                        lane = lax.broadcasted_iota(jnp.int32, (128, 128), 1)
                        zi = jnp.where((lane & 63) == 0, 0.0, pltpu.roll(zr, 64, 1))
                    else:
                        zi = _dot(u0, _bf(small[1]))
                else:
                    a, b = st["u"][g]
                    k, kb, ka = [_dot(v.astype(bf16), _bf(small[3 * g - 1 + i]))
                                 for i, v in enumerate((a + b, b, a))]
                    zr, zi = k + kb, ka - _mu() * k
                ys = [(zr[8 * a:8 * a + 8], zi[8 * a:8 * a + 8]) for a in range(16)]
                if g < 2:
                    ys = _fft16(ys, -1)
                for a in range(16):
                    zv[g][0, a, rows, :] = ys[a][0]
                    zv[g][1, a, rows, :] = ys[a][1]
            return run
        return [part(g) for g in range(3)]

    def post(u, carry):
        base = pl.multiple_of(32 * u, 32)
        side = []
        for q in range(4):
            side += dfwd_thunks(pl.ds(base, 32), q)
        side = [side[i] for i in CFG["post_order"]]
        k = 0
        at = list(CFG["post_at"])
        m, due = {}, []
        for prods in CFG["post_passes"]:
            acc = None
            for p in range(NPAIR):
                lhs = _strassen_lhs(*[
                    functools.partial(lambda r, e: qb[8 * r:8 * r + 8, u, 2 * p + e].reshape(64, 128), r, e)
                    for r in range(2) for e in range(2)])
                res = []
                for i in prods:
                    if i == 7:
                        oo = jnp.concatenate([qb[:, u, 2 * p + e].reshape(128, 128) for e in range(2)], axis=1)
                        res.append(_dot(oo.astype(bf16), wo_t[4, 256 * p:256 * p + 256, :]))
                        k += 2
                        continue
                    a = lhs[i]().astype(bf16)
                    for np_ in range(2):
                        if i in WS_SLOT:
                            w = ws[p, 5 * np_ + WS_SLOT[i]]
                        else:
                            kk = 0 if i == 1 else 1
                            w = wo_t[2 * np_ + kk, 256 * p + 128 * kk:256 * p + 128 * kk + 128, :]
                        if due and due[0][0] <= k:
                            w = _bf(_with_tokens(pltpu.bitcast(w, u32), {0: due.pop(0)[1]}))
                        res.append(_dot(a, w))
                    k += 1
                acc = addl(acc, res)
                while at and at[0] <= k:
                    g = CFG["post_order"][len(CFG["post_at"]) - len(at)] % 3
                    at.pop(0)
                    side.pop(0)()
                    if g == 0 and CFG["post_dl"]:
                        due.append((k + CFG["post_dl"],
                                    pltpu.bitcast(z0[0, u >> 2, 128:ZPITCH, :], u32)))
            for i in prods:
                m[i] = [acc.pop(0)] if i == 7 else [acc.pop(0), acc.pop(0)]
        cols = []
        for np_ in range(2):
            m1, m2, m3, m4, m5, m6, m7 = [m[i][np_] for i in range(7)]
            cols.append(jnp.concatenate([m1 + m4 - m5 + m7, m2 + m4], axis=0))
            cols.append(jnp.concatenate([m3 + m5, m1 - m2 + m3 + m6], axis=0))
        to[...] = jnp.concatenate(cols + m[7], axis=1).reshape(16, 8, DM)
        for f in side:
            f()
        return carry

    def spectral(zero):
        def fence(z):
            return z[0, zero, 128:ZPITCH, :]

        def radix(g, bb, sign):
            z = zs[g]
            toks = []

            def emit(q, y):
                for p in range(4):
                    z[0, q + 4 * p, chunk(bb), :] = y[p][0]
                    z[1, q + 4 * p, chunk(bb), :] = y[p][1]
                toks.append(fence(z))
            _fft16([(z[0, a, chunk(bb), :], z[1, a, chunk(bb), :]) for a in range(16)], sign, emit)
            return toks

        ys = {}

        def fwd(g, k2, toks):
            z = zs[g]
            ur, ui = z[0, k2, 0:64, :], z[1, k2, 0:64, :]
            tr, ti = _twiddle((z[0, k2, 64:128, :], z[1, k2, 64:128, :]), k2, 32, -1)
            for hf in range(2):
                v = _ilv(ur + tr, ui + ti) if hf == 0 else _ilv(ur - tr, ui - ti)
                lhs = _with_tokens(emat[k2 + 16 * hf], toks if hf == 0 else None)
                xr, xi = _dilv(_dot(_bf(lhs), v.astype(bf16)))
                ys["x", 16 * g + k2] = xr
                wr = wf[g, pl.ds(k2 * WPITCH + hf, 64, stride=2), :]
                wi = wf[g + 3, pl.ds(k2 * WPITCH + hf, 64, stride=2), :]
                ys[g, k2, hf] = _ilv(xr * wr - xi * wi, xr * wi + xi * wr).astype(bf16)

        def inv(g, k2, toks):
            z = zs[g]
            t0 = _dot(_bf(_with_tokens(emat[32 + k2], toks)), ys.pop((g, k2, 0)))
            t1 = _dot(_bf(emat[48 + k2]), ys.pop((g, k2, 1)))
            z[0, k2, 0:64, :], z[1, k2, 0:64, :] = _dilv(t0 + t1)
            z[0, k2, 64:128, :], z[1, k2, 64:128, :] = _twiddle(_dilv(t0 - t1), k2, 32, 1)

        units = [(g, k2) for g in range(3) for k2 in range(16)]
        toks = None
        lag = CFG["inv_lag"]
        for i in range(len(units) + lag):
            if i < len(units):
                fwd(*units[i], toks)
            if i >= lag:
                inv(*units[i - lag], toks if i >= len(units) else None)
            toks = []
            if i in CFG["fwd_at"]:
                toks += radix(2, CFG["fwd_at"].index(i), -1)
            for n, at in enumerate(CFG["inv_at"]):
                if at == i:
                    if not toks:
                        back, r = CFG["rel"]
                        zs[n // 16][1, zero, 128:ZPITCH, :] = ys["x", min(i - back, 47)][8 * r:8 * r + 8]
                    toks += radix(n // 16, n % 16, 1)
            pos = CFG["tok_pos"] if len(toks) <= 4 else range(8)
            toks = {j: pltpu.bitcast(t, u32) for j, t in zip(pos, toks)}

    def dinv_thunks(bb, finish):
        st = {}

        def part(g):
            def run():
                z = zs[g]
                ys = [(z[0, a, chunk(bb), :], z[1, a, chunk(bb), :]) for a in range(16)]
                if g >= CFG["inv_groups"]:
                    ys = _fft16(ys, 1)
                tr = jnp.concatenate([y[0] for y in ys], axis=0)
                ti = jnp.concatenate([y[1] for y in ys], axis=0)
                if g == 0 and CFG["pack_i"]:
                    lane = lax.broadcasted_iota(jnp.int32, (128, 128), 1)
                    v = jnp.where(lane <= 64, tr, pltpu.roll(ti, 64, 1))
                    st[0] = _dot(v.astype(bf16), _bf(small[8]))
                elif g == 0:
                    st[0] = _dot(tr.astype(bf16), _bf(small[8])) + _dot(ti.astype(bf16), _bf(small[9]))
                else:
                    k, ki, kr = [_dot(v.astype(bf16), _bf(small[7 + 3 * g + i]))
                                 for i, v in enumerate((tr + _mu() * ti, ti, tr))]
                    st[2 * g - 1], st[2 * g] = k + ki, k + kr
            return run

        def fin():
            p0, p1, q1, p2, q2 = [st[j] for j in range(5)]
            t = p1 + p2
            m, n = p0 - 0.25 * t, R5_D * (p1 - p2)
            e1, e2 = m + n, m - n
            o1, o2 = q1 + R5_R * q2, R5_R * q1 - q2
            y = jnp.concatenate([p0 + t, e1 - o1, e2 - o2, e2 + o2, e1 + o1], axis=1)
            finish(xb[:, chunk(bb), :].reshape(128, DM) + y)
        return [part(0), part(1), part(2), fin]

    def out_copy(bb):
        return pltpu.make_async_copy(xin.at[:, bb], out_hbm.at[:, bb], osem.at[bb])

    def layer(li, carry0):
        if full or CFG["only"] == "group":
            _loop("step", 0, 16, group, mem_ref[...].astype(f32))
        if full or CFG["only"] == "spec":
            _loop("post", 0, 4, post, 0, unroll=CFG["post_unroll"])

            with jax.named_scope("spectral"):
                spectral((li >> 1))
        if not full and CFG["only"] != "out":
            return carry0

        def run_chunks(th, order, lag):
            seq = [t[g] for t in th for g in order]
            for i in range(len(seq) + lag):
                if i < len(seq):
                    seq[i]()
                if i >= lag and (i - lag) % 3 == 2:
                    th[(i - lag) // 3][3]()

        @pl.when(li == 0)
        def _():
            with jax.named_scope("dinv_tails"):
                run_chunks([dinv_thunks(4 * u + 3, functools.partial(
                    lambda u, x: set_input(4 * u + 3, _round_bf16(x), u), u)) for u in range(4)],
                    *CFG["tails_order"])

            def batch(it, carry):
                bb = body_chunk(it)
                side = dinv_thunks(bb, lambda x: set_input(bb, _round_bf16(x), None))
                for k, f in enumerate(batch_thunks(it)):
                    f()
                    if k in CFG["dinv_at"]:
                        side.pop(0)()
                return carry
            _loop("batch", 0, 12, batch, 0, unroll=CFG["batch_unroll"])

        @pl.when(li == 1)
        def _():
            with jax.named_scope("dinv_out"):
                def store_out(bb, x):
                    xin[:, bb] = x.reshape(16, 8, DM).astype(bf16)
                    out_copy(bb).start()
                run_chunks([dinv_thunks(bb, functools.partial(store_out, bb)) for bb in range(16)],
                           *CFG["out_order"])
                for bb in range(16):
                    out_copy(bb).wait()
        return carry0

    if CFG["only"] != "pro":
        lax.fori_loop(0, 2, layer, 0)
    else:
        zero = zero_ref[0]
        xin[0, 0, :, 0:128] = (qb[zero, 0, 0] + wf[zero, 0:8, :] + xa[zero, 0:8, 0:128]).astype(bf16) + ws[zero, 0, 0:8, :]
        out_copy(0).start()
        out_copy(0).wait()


@jax.jit
def pallas_interleave_layers__memory_aug_recurrent_mem_tr__spectral_gfnet__prompt_kernel(
    A_x, A_mem0, A_Wq, A_Wk, A_Wv, A_Wo, A_seg_len, B_x, B_w_r, B_w_i,
):
    assert A_x.shape == (1, S, DM) and A_mem0.shape == (1, MEM, DM)
    small, emat = _tables()
    hbm = pl.BlockSpec(memory_space=pltpu.HBM)
    out = pl.pallas_call(
        _kernel,
        out_shape=jax.ShapeDtypeStruct((16, 16, 8, DM), bf16),
        in_specs=[hbm] * 10,
        out_specs=hbm,
        scratch_shapes=[
            pltpu.VMEM((16, 16, 8, DM), bf16),
            pltpu.VMEM((33, 128, DM), f32),
            pltpu.VMEM((16, 128, DM), f32),
            pltpu.VMEM((16, 8, DM), f32),
            pltpu.VMEM((12, 2, 320, 8, DH), bf16),
            pltpu.VMEM((13, 8 * HPITCH, 128), u32),
            pltpu.VMEM((13, 8 * HPITCH, 128), u32),
            pltpu.VMEM((5, H * DH + 512, 128), bf16),
            pltpu.VMEM((19, 10, 128, 128), bf16),
            pltpu.VMEM((16, 4, 96, 8, 128), f32),
            pltpu.VMEM((2, 16, 64, 128), u32),
            pltpu.VMEM((2, 16, ZPITCH, 128), f32),
            pltpu.VMEM((2, 16, ZPITCH, 128), f32),
            pltpu.VMEM((2, 16, ZPITCH, 128), f32),
            pltpu.VMEM((6, 16 * WPITCH + 32, 128), f32),
            pltpu.VMEM((9, DF, 512), bf16),
            pltpu.VMEM((4, 328, 128), f32),
            pltpu.VMEM((SMALL_TILES, 64, 128), u32),
            pltpu.VMEM((64, 64, 128), u32),
            pltpu.VMEM((80, 80), f32),
            pltpu.VMEM((MEM, DM), bf16),
            pltpu.SMEM((1,), jnp.int32),
            pltpu.SemaphoreType.DMA((47,)),
            pltpu.SemaphoreType.DMA((16,)),
        ],
        compiler_params=pltpu.CompilerParams(vmem_limit_bytes=120 * 1024 * 1024,
                                             disable_semaphore_checks=True),
    )(
        A_x.reshape(16, 16, 8, DM), A_mem0.reshape(MEM, DM),
        *[w.reshape(2, 320, H, DH) for w in (A_Wq, A_Wk, A_Wv)], A_Wo.reshape(H * DH, DM), B_w_r.T, B_w_i.T,
        jnp.asarray(small), jnp.asarray(emat),
    )
    return out.reshape(1, S, DM)
```

```python
import functools
import math

import jax
import jax.numpy as jnp
import numpy as np
from jax import lax
import jax.experimental.pallas as pl
import jax.experimental.pallas.tpu as pltpu

f32, bf16, u32 = jnp.float32, jnp.bfloat16, jnp.uint32

S, DM, H, DH, MEM, SEG = 2048, 640, 32, 128, 8, 32
NSEG = S // SEG
NPAIR = H // 2
DF = DM // 2 + 1
EPS = 1e-5
WPITCH = 132

HPITCH = 164
ZPITCH = 136

S1 = math.sin(2 * math.pi / 5)
R5_D = (math.cos(2 * math.pi / 5) - math.cos(4 * math.pi / 5)) / 2
R5_R = math.sin(4 * math.pi / 5) / S1


def _to_bf16_bits(a):
    u = np.ascontiguousarray(a, dtype=np.float32).view(np.uint32).astype(np.uint64)
    return ((u + 0x7FFF + ((u >> 16) & 1)) >> 16).astype(np.uint32)


def _pack_rows(a):
    b = _to_bf16_bits(a)
    return b[..., 0::2, :] | (b[..., 1::2, :] << 16)


@functools.lru_cache(maxsize=None)
def _tables():
    b = np.arange(128)
    l0 = np.arange(0, DF, 5)
    l1 = np.concatenate([np.arange(1, 320, 5), np.arange(4, 320, 5)])
    l2 = np.concatenate([np.arange(2, 320, 5), np.arange(3, 320, 5)])
    sg = np.concatenate([np.ones(64), -np.ones(64)])

    def th(l):
        return 2 * np.pi * ((b[:, None] * l[None, :]) % DM) / DM

    sc = 1.0 / (S * DM)
    fw = np.zeros((8, 128, 128))
    iw = np.zeros((8, 128, 128))
    t = th(l0)
    cl = np.full((65, 1), 2.0)
    cl[0] = cl[-1] = 1.0
    fw[0, :, :65], fw[1, :, :65] = np.cos(t), -np.sin(t)
    iw[0, :65], iw[1, :65] = cl * np.cos(t.T) * sc, -cl * np.sin(t.T) * sc
    if CFG["pack_f"]:
        fw[0, :, 65:] = fw[1, :, 1:64]
    if CFG["pack_i"]:
        iw[0, 65:] = iw[1, 1:64]
    mu = S1 * sg
    for g, l in ((1, l1), (2, l2)):
        t = th(l)
        c, s = np.cos(t), np.sin(t)
        fw[3 * g - 1:3 * g + 2] = c, -mu * s - c, mu * c - s
        iw[3 * g - 1:3 * g + 2] = [2 * sc * m.T for m in (c, -s - mu * c, mu * s - c)]
    n = np.arange(64)
    order = np.concatenate([np.concatenate([np.arange(8) + 8 * j, np.arange(8) + 8 * j + 64])
                            for j in range(8)])
    e = np.zeros((2, 32, 128, 128))
    for k2 in range(32):
        t = 2 * np.pi * (((32 * n[:, None] + k2) * n[None, :]) % S) / S
        er, ei = np.cos(t), -np.sin(t)
        m = np.block([[er, -ei], [ei, er]])[order][:, order]
        e[0, k2], e[1, k2] = m, m.T
    small = np.concatenate([_pack_rows(fw), _pack_rows(iw)], axis=0)
    return small, _pack_rows(e).reshape(64, 64, 128)


SMALL_TILES = 16


def _loop(name, lo, hi, body, init, **kw):
    with jax.named_scope(name):
        return lax.fori_loop(lo, hi, body, init, **kw)


def _bf(x):
    return pltpu.bitcast(x, bf16)


def _dot(a, b):
    return jnp.dot(a, b, preferred_element_type=f32)


def _round_bf16(x):
    return x.astype(bf16).astype(f32)


def _layernorm(x):
    m = jnp.mean(x, axis=-1, keepdims=True)
    xc = x - m
    v = jnp.mean(xc * xc, axis=-1, keepdims=True)
    return xc * lax.rsqrt(v + EPS)


def _fft4(x, sign):
    (ar, ai), (br, bi), (cr, ci), (dr, di) = x
    t0r, t0i, t1r, t1i = ar + cr, ai + ci, ar - cr, ai - ci
    t2r, t2i, t3r, t3i = br + dr, bi + di, br - dr, bi - di
    y0, y2 = (t0r + t2r, t0i + t2i), (t0r - t2r, t0i - t2i)
    p, q = (t1r + t3i, t1i - t3r), (t1r - t3i, t1i + t3r)
    return [y0, p, y2, q] if sign < 0 else [y0, q, y2, p]


def _twiddle(z, n, period, sign):
    zr, zi = z
    n = n % period
    if n == 0:
        return z
    if 4 * n == period:
        return (-zi, zr) if sign > 0 else (zi, -zr)
    c, s = math.cos(2 * math.pi * n / period), sign * math.sin(2 * math.pi * n / period)
    if (8 * n) % period == 0:
        a, d = zr + zi, zr - zi
        if c * s > 0:
            return (d * c, a * c)
        return (a * c, d * s)
    return (zr * c - zi * s, zr * s + zi * c)


def _bsum(x, y, sign):
    x, y = x.astype(f32), y.astype(f32)
    return (x + y if sign > 0 else x - y).astype(bf16)


def _strassen_lhs(a11, a12, a21, a22):
    return [lambda: a11() + a22(), lambda: a21() + a22(), a11, a22,
            lambda: a11() + a12(), lambda: a21() - a11(), lambda: a12() - a22()]


def _strassen_rhs(b11, b12, b21, b22):
    return [lambda: _bsum(b11(), b22(), 1), b11, lambda: _bsum(b12(), b22(), -1),
            lambda: _bsum(b21(), b11(), -1), b22, lambda: _bsum(b11(), b12(), 1),
            lambda: _bsum(b21(), b22(), 1)]


WS_SLOT = {0: 0, 2: 1, 3: 2, 5: 3, 6: 4}


def _mu():
    lane = lax.broadcasted_iota(jnp.int32, (1, 128), 1)
    return jnp.where(lane < 64, S1, -S1).astype(f32)


def _ilv(r, i):
    n = r.shape[0] // 8
    return jnp.concatenate([r.reshape(n, 8, 128), i.reshape(n, 8, 128)], axis=1).reshape(16 * n, 128)


def _dilv(x):
    n = x.shape[0] // 16
    x = x.reshape(n, 16, 128)
    return x[:, :8].reshape(8 * n, 128), x[:, 8:].reshape(8 * n, 128)


def _with_tokens(x, toks):
    if not toks:
        return x
    return jnp.concatenate(
        [x[8 * j:8 * j + 8] | toks[j] if j in toks else x[8 * j:8 * j + 8]
         for j in range(x.shape[0] // 8)], axis=0)


def _fft16(x, sign, emit=None):
    cols = [_fft4([x[4 * j + r] for j in range(4)], sign) for r in range(4)]
    out = [None] * 16
    for q in range(4):
        y = _fft4([_twiddle(cols[r][q], r * q, 16, sign) for r in range(4)], sign)
        for p in range(4):
            out[q + 4 * p] = y[p]
        if emit is not None:
            emit(q, y)
    return out


CFG = dict(steps=((4.5, 16.5, 6, 4, 0, 8), (5, 16.5, 5, 7, 8, 12), (5, 16.5, 6, 6, 8, 12), (5, 16.5, 8, 7, 8, 0)),
           post_dl=20, post_passes=((0, 1), (2, 3), (4, 5), (6, 7)),
           post_order=(0, 1, 6, 3, 4, 2, 8, 5, 7, 9, 10, 11), post_at=(22, 26, 68, 96),
           tails_order=((1, 2, 0), 5), out_order=((1, 2, 0), 5), pack_f=True, pack_i=True,
           inv_at=tuple(range(28, 44)), inv_groups=1, inv_lag=4, tok_pos=(4, 5, 6, 7),
           fwd_at=(7, 8, 9, 10, 12, 13, 14, 16, 17, 18, 20, 21, 22, 24, 25, 26), rel=(0, 1), dinv_at=(8, 9, 10, 11), batch_unroll=2, post_unroll=1,
           ws_split=4, ws_at=(9, 9, 10, 11, 12, 13, 14, 15, 16, 16, 17, 18, 19, 20, 21, 22),
           pro_nre=15, re_pos=(2, 3, 7), ln_at=(13, 20, 27, 31), ln_at2=(4, 7, 10, 13),
           perm_at=(11, 13, 15, 18, 20, 23, 25, 27, 30, 31, 31, 31), only=None)


def _interleave(main, side):
    n, k = len(main), 0
    for i, f in enumerate(main):
        f()
        while k < len(side) and (k + 1) * n <= (i + 1) * len(side):
            side[k]()
            k += 1
    for f in side[k:]:
        f()


def _kernel(x_hbm, mem_hbm, wq_hbm, wk_hbm, wv_hbm, wo_hbm, wr_hbm, wi_hbm,
            small_hbm, e_hbm, out_hbm,
            xin, xa, xb, to, raw, wa, wb, wo_t, ws, qb, hl, z0, z1, z2, wf,
            wri, wtmp, small, emat, fill_ref, mem_ref, zero_ref, sem, osem):
    zs = (z0, z1, z2)
    w_hbm = (wq_hbm, wk_hbm, wv_hbm)

    def body_chunk(i):
        return 4 * (i & 3) + (i >> 2)

    def cp_w(i):
        src = w_hbm[i >> 2].at[:, :, pl.ds(8 * (i & 3), 8), :] if isinstance(i, int) else raw.at[i]
        return pltpu.make_async_copy(src, raw.at[i], sem.at[i])

    def cp_x(bb):
        return pltpu.make_async_copy(x_hbm.at[:, bb], xin.at[:, bb], sem.at[12 + bb])

    def cp_f(i):
        src = ((wr_hbm, wi_hbm)[i >> 2].at[:, pl.ds(512 * (i & 3), 512)]
               if isinstance(i, int) else wri.at[i])
        return pltpu.make_async_copy(src, wri.at[i], sem.at[36 + i])

    def cp_wo(i):
        rows = pl.ds(pl.multiple_of(512 * i, 512), 512)
        return [pltpu.make_async_copy(wo_hbm.at[rows, pl.ds(128 * j, 128)], wo_t.at[j, rows], sem.at[28 + i])
                for j in range(5)]

    cp_rest = [pltpu.make_async_copy(mem_hbm, mem_ref, sem.at[46]),
                pltpu.make_async_copy(small_hbm, small, sem.at[44]),
               pltpu.make_async_copy(e_hbm, emat, sem.at[45])]

    full = CFG["only"] in (None, "pro")
    for u in range(4 if full else 0):
        cp_x(4 * u + 3).start()
    if full:
        cp_w(0).start()
    for i in range(12 if full else 0):
        if i < 11:
            cp_w(i + 1).start()
        cp_x(body_chunk(i)).start()
        if 3 <= i < 11:
            cp_f(i - 3).start()
            for cp in cp_wo(i - 3):
                cp.start()
    for cp in cp_rest if full else ():
        cp.start()

    zero_ref[0] = 0

    r = lax.broadcasted_iota(jnp.int32, (80, 80), 0)
    c = lax.broadcasted_iota(jnp.int32, (80, 80), 1)

    def head(i):
        return jnp.where(i < 64, i // 32, (i - 64) // 8)

    def pos(i):
        return jnp.where(i < 64, i % 32, 32 + (i - 64) % 8)

    ok = (pos(r) < MEM) | (pos(r) >= pos(c))
    fill_ref[...] = jnp.where(head(r) == head(c), jnp.where(ok, 0.0, -1e9), -jnp.inf).astype(f32)
    wtmp[:, 320:328, :] = jnp.zeros((4, 8, 128), f32)
    xa[32, 0:8, 0:128] = jnp.zeros((8, 128), f32)
    ws[18, 0, 0:16, :] = jnp.zeros((16, 128), bf16)
    wa[12, 0:8, :] = jnp.zeros((8, 128), u32)
    wb[12, 0:8, :] = jnp.zeros((8, 128), u32)
    wf[5, 16 * WPITCH:16 * WPITCH + 8, :] = jnp.zeros((8, 128), f32)
    for z in zs:
        z[0, 0, 128:ZPITCH, :] = jnp.zeros((8, 128), f32)

    def chunk(bb):
        if isinstance(bb, int):
            return slice(8 * bb, 8 * bb + 8)
        return pl.ds(pl.multiple_of(8 * bb, 8), 8)

    def set_input(bb, x, tail_u, a0=0):
        n = x.shape[0] // 8
        xa[a0:a0 + n, chunk(bb), :] = x.reshape(n, 8, DM)
        y = _layernorm(x)
        if tail_u is None:
            xa[16 + a0:16 + a0 + n, chunk(bb), :] = y.reshape(n, 8, DM)
        else:
            blk = [[y[64 * r:64 * r + 64, 128 * kt:128 * kt + 128] for kt in range(5)] for r in range(2)]
            ops = []
            for kp in range(2):
                (a11, a12), (a21, a22) = [blk[r][2 * kp:2 * kp + 2] for r in range(2)]
                ops += [a11 + a22, a21 + a22, a11, a22, a11 + a12, a21 - a11, a12 - a22]
            for i, v in enumerate(ops + [blk[0][4], blk[1][4]]):
                hl[tail_u >> 1, i, 32 * (tail_u & 1):32 * (tail_u & 1) + 32, :] = (
                    pltpu.bitcast(v.astype(bf16), u32))

    def load_x(bb, a0=0, n=16):
        return xin[a0:a0 + n, bb].astype(f32).reshape(8 * n, DM)

    def wtile(cid, j, e):
        w = (wa, wb)[e]
        return jnp.concatenate([w[cid, (4 * hf + j) * HPITCH:(4 * hf + j) * HPITCH + 160, :]
                                for hf in range(2)], axis=0)

    def relayout(i, cid, e):
        for r in range(4 * i, 4 * i + 4):
            a, b = [pltpu.bitcast(raw[cid, :, d].reshape(16, 128), u32) for d in (2 * r, 2 * r + 1)]
            v = (a & 0xFFFF) | (b << 16) if e == 0 else (a >> 16) | (b & jnp.uint32(0xFFFF0000))
            (wa, wb)[e][cid, pl.ds(r, 8, stride=HPITCH), :] = v

    def batch_thunks(cid):
        qv = qb.at[:, :, pl.ds(8 * cid, 8)]

        def unit(e, jp, s):
            c = {}

            def w(n, kt):
                return _bf(wtile(cid, 2 * jp + n, e)[64 * kt:64 * kt + 64])

            def rhs(i, kp):
                return _strassen_rhs(*[functools.partial(w, n, 2 * kp + k)
                                       for k in range(2) for n in range(2)])[i]()

            def prod(i, toks=None):
                l0, l1 = _bf(_with_tokens(hl[s, i], toks)), _bf(hl[s, 7 + i])
                return _dot(l0, rhs(i, 0)) + _dot(l1, rhs(i, 1))

            def last(r, n, toks=None):
                return _dot(_bf(_with_tokens(hl[s, 14 + r], toks)), w(n, 4))

            def store(r, n):
                y = c.pop((r, n)).reshape(2, 8, 8, 128)
                for k in range(2):
                    qv[8 * r:8 * r + 8, 2 * s + k, 2 * (2 * jp + n) + e] = y[k]

            def t0(toks=None):
                c[1, 1] = last(1, 1, toks) + prod(5)
                m1 = prod(0)
                c[1, 1], c[0, 0] = c[1, 1] + m1, m1

            def t1(toks=None):
                c[0, 0] = c[0, 0] + last(0, 0, toks) + prod(6)
                m2 = prod(1)
                c[1, 1], c[1, 0] = c[1, 1] - m2, m2

            def t2(toks=None):
                m3 = prod(2, toks)
                c[1, 1] = c[1, 1] + m3
                store(1, 1)
                m5 = prod(4)
                c[0, 1], c[0, 0] = m3 + m5, c[0, 0] - m5

            def t3(toks=None):
                c[0, 1] = c[0, 1] + last(0, 1, toks)
                store(0, 1)
                m4 = prod(3)
                c[0, 0] = c[0, 0] + m4
                store(0, 0)
                c[1, 0] = c[1, 0] + m4 + last(1, 0)
                store(1, 0)
            return [t0, t1, t2, t3]
        return [f for e in range(2) for jp in range(2) for s in range(2) for f in unit(e, jp, s)]

    def wperm_thunks(piece, j):
        m = (piece >> 2) & 1
        wt = wtmp.at[j]

        def load():
            wt[0:DF, :] = wri[piece, :, 128 * j:128 * j + 128].astype(f32)

        def one(g):
            def run():
                if g == 0:
                    t = jnp.concatenate([wt[pl.ds(0, 64, stride=5), :], wt[320:328, :],
                                         jnp.zeros((56, 128), f32)], axis=0)
                else:
                    t = jnp.concatenate([wt[pl.ds(g, 64, stride=5), :],
                                         wt[pl.ds(5 - g, 64, stride=5), :]], axis=0)
                y = t.T
                sub = wf.at[3 * m + g, pl.ds(pl.multiple_of((piece & 3) * 32, 32), 16 * WPITCH - 96)]
                for k in range(8):
                    for hf in range(2):
                        sub[pl.ds(8 * j + k + 8 * hf * WPITCH, 8, stride=WPITCH), :] = (
                            y[16 * k + 8 * hf:16 * k + 8 * hf + 8])
            return run
        return [load] + [one(g) for g in range(3)]

    def half_pass(cid, half, fill, zero, timed=()):
        nre = CFG["pro_nre"]
        toks = None
        for k, f in enumerate(batch_thunks(cid)[16 * half:16 * half + 16]):
            f(toks)
            toks = {}
            for n, f in enumerate(f for at, f in timed if at == k):
                toks[(0, 4, 1, 6)[n]] = f()
            if fill is not None:
                for n, r in enumerate(r for r in range(40) if r * nre // 40 == k):
                    relayout(r, fill, 1 - half)
                    toks[CFG["re_pos"][n]] = (wb, wa)[half][12 + zero, 0:8, :]

    def ln_parts(bb, zero):
        def part(j):
            set_input(bb, load_x(bb, 4 * j, 4), None, 4 * j)
            return pltpu.bitcast(xa[32 + zero, 0:8, 0:128], u32)
        return [functools.partial(part, j) for j in range(4)]

    def perm_parts(piece, zero):
        def part(fs):
            for f in fs:
                f()
            return pltpu.bitcast(wf[5 + zero, 16 * WPITCH:16 * WPITCH + 8, :], u32)
        out = []
        for j in range(4):
            th = wperm_thunks(piece, j)
            out += [functools.partial(part, th[0:2]), functools.partial(part, th[2:3]),
                    functools.partial(part, th[3:4])]
        return out

    def ws_parts(piece, zero):
        nr = 128 // CFG["ws_split"]

        src = wo_t.at[:, pl.ds(pl.multiple_of(512 * piece, 512), 512)]
        dst = ws.at[pl.ds(2 * piece, 2)]

        def part(pp, np_, r0):
            def tile(k, n):
                lo = 256 * pp + 128 * k + r0
                return src[2 * np_ + n, lo:lo + nr, :]
            rhs = _strassen_rhs(*[functools.partial(tile, k, n) for k in range(2) for n in range(2)])
            for i, slot in WS_SLOT.items():
                dst[pp, 5 * np_ + slot, r0:r0 + nr, :] = rhs[i]()
            return pltpu.bitcast(ws[18 + zero, 0, 0:16, :], u32)
        return [functools.partial(part, pp, np_, r0)
                for pp in range(2) for np_ in range(2) for r0 in range(0, 128, nr)]

    def pro0():
        for u in range(4):
            cp_x(4 * u + 3).wait()
        for u in range(4):
            set_input(4 * u + 3, load_x(4 * u + 3), u)
        cp_w(0).wait()
        zero = zero_ref[0]
        for i in range(40):
            relayout(i, 0, 0)
        half_pass(0, 0, zero, zero)

    def pro1(it, carry):
        bb = body_chunk(it)
        with jax.named_scope("pro1_wait"):
            cp_w(it + 1).wait()

            @pl.when(it >= 3)
            def _():
                cp_f(it - 3).wait()
                for cp in cp_wo(it - 3):
                    cp.wait()
            cp_x(bb).wait()
        piece = jnp.where(it >= 3, it - 3, 8)
        zero = it >> 4
        timed = sorted(list(zip(CFG["ln_at"], ln_parts(bb, zero)))
                       + list(zip(CFG["ws_at"], ws_parts(piece, zero)))
                       + list(zip(CFG["perm_at"], perm_parts(piece, zero))), key=lambda x: x[0])
        half_pass(it, 1, it + 1, zero, [x for x in timed if x[0] < 16])
        half_pass(it + 1, 0, it + 1, zero, [(k - 16, f) for k, f in timed if k >= 16])
        return carry

    def pro2():
        cp_x(body_chunk(11)).wait()
        for cp in cp_rest:
            cp.wait()
        zero = zero_ref[0]
        half_pass(11, 1, None, zero, list(zip(CFG["ln_at2"], ln_parts(body_chunk(11), zero))))

    if full:
        with jax.named_scope("pro0"):
            pro0()
        _loop("pro1", 0, 11, pro1, 0)
        with jax.named_scope("pro2"):
            pro2()

    scale = DH ** -0.5

    def wo_dot(hh, oo):
        return [_dot(oo, wo_t[j, 128 * hh:128 * hh + 128, :]) for j in range(5)]

    def addl(acc, res):
        return res if acc is None else [a + b for a, b in zip(acc, res)]

    def group(g, mem):
        for ph in range(4):
            h = jnp.concatenate([mem, xa[16 + g, 32 * ph:32 * ph + 24, :]], axis=0).astype(bf16)
            pr, sm, oos = {}, {}, {}
            lat_s, lat_pv, lat_wo, v_delay, n_first, n_last = CFG["steps"][ph]

            def stacked(p, m):
                tails = [qb[g, ph, 32 * m + 2 * p + e] for e in range(2)]
                return jnp.concatenate([pr[p, m, 0], pr[p, m, 1]] + tails, axis=0).astype(bf16)

            def scores(p):
                sc = lax.dot_general(stacked(p, 0), stacked(p, 1), (((1,), (1,)), ((), ())),
                                     preferred_element_type=f32)
                fill = fill_ref[...]
                sc = jnp.where(fill == 0.0, sc * scale, fill)
                mx = jnp.max(sc, axis=-1, keepdims=True)
                e = jnp.exp(sc - mx)
                rl = pl.reciprocal(jnp.sum(e, axis=-1, keepdims=True), approx=True)
                sm[p] = (e * rl).astype(bf16)

            def pv(p):
                o = _dot(sm[p], stacked(p, 2))
                for e in range(2):
                    qb[g, ph, 2 * p + e] = o[64 + 8 * e:72 + 8 * e]
                    oos[2 * p + e] = o[32 * e:32 * e + 32].astype(bf16)

            keyed = []
            for p in range(NPAIR):
                keyed += [(4 * p + 2 * m + e, (p, m, e)) for m in range(2) for e in range(2)]
                keyed += [(4 * p + 3.5 + v_delay, (p, 2, e)) for e in range(2)]
            bulk = [x for _, x in sorted(keyed, key=lambda kv: kv[0])]
            acc, t, nwo, pend, ready = None, 0.0, 0, [], []
            if n_first:
                first, bulk = bulk[:n_first], bulk[n_first:]
                for kt in range(5):
                    for p, m, e in first:
                        w = wtile(4 * m + (p >> 2), p & 3, e)[64 * kt:64 * kt + 64]
                        y = _dot(h[:, 128 * kt:128 * kt + 128], _bf(w))
                        pr[p, m, e] = y if kt == 0 else pr[p, m, e] + y
                t = float(len(first))
                pend = [(t + lat_s, "S", p) for p, m, e in first if m == 1 and e == 1]
            while nwo < H - n_last or pend:
                pend.sort()
                if pend and pend[0][0] <= t:
                    _, kind, p = pend.pop(0)
                    if kind == "S":
                        scores(p)
                        pend.append((t + lat_pv, "V", p))
                    else:
                        pv(p)
                        ready += [(t + lat_wo, 2 * p + e) for e in range(2)]
                    t += 0.5
                elif bulk:
                    p, m, e = bulk.pop(0)
                    pr[p, m, e] = _dot(h, _bf(wtile(4 * m + (p >> 2), p & 3, e)))
                    t += 1
                    if m == 1 and e == 1:
                        pend.append((t + lat_s, "S", p))
                elif ready and ready[0][0] <= t and nwo < H - n_last:
                    _, hh = ready.pop(0)
                    acc = addl(acc, wo_dot(hh, oos[hh]))
                    t += 1
                    nwo += 1
                else:
                    t += 0.5
            for j in range(5):
                for _, hh in ready:
                    acc[j] = acc[j] + _dot(oos[hh], wo_t[j, 128 * hh:128 * hh + 128, :])
            out = jnp.concatenate(acc, axis=1)
            xa[16 + g, 32 * ph:32 * ph + 24, :] = out[8:32]
            mem = _round_bf16(out[0:8])
        return mem

    def dfwd_thunks(seg, q):
        st = {}
        rows = chunk(q)
        xav, xbv, zv = xa.at[:, seg], xb.at[:, seg], [z.at[:, :, seg] for z in zs]

        def pre():
            o = to[...] if q == 3 else xav[16:32, rows, :]
            x = _round_bf16(xav[0:16, rows, :] + o)
            xbv[:, rows, :] = x
            y = _layernorm(x.reshape(128, DM))
            x0, x1, x2, x3, x4 = [y[:, 128 * a:128 * a + 128] for a in range(5)]
            t1, t2, t3, t4 = x1 + x4, x2 + x3, x1 - x4, x2 - x3
            t = t1 + t2
            m, n = x0 - 0.25 * t, R5_D * (t1 - t2)
            st["u"] = [x0 + t, (m + n, t3 + R5_R * t4), (m - n, R5_R * t3 - t4)]

        def part(g):
            def run():
                if g == 0:
                    pre()
                    u0 = st["u"][0].astype(bf16)
                    zr = _dot(u0, _bf(small[0]))
                    if CFG["pack_f"]:
                        lane = lax.broadcasted_iota(jnp.int32, (128, 128), 1)
                        zi = jnp.where((lane & 63) == 0, 0.0, pltpu.roll(zr, 64, 1))
                    else:
                        zi = _dot(u0, _bf(small[1]))
                else:
                    a, b = st["u"][g]
                    k, kb, ka = [_dot(v.astype(bf16), _bf(small[3 * g - 1 + i]))
                                 for i, v in enumerate((a + b, b, a))]
                    zr, zi = k + kb, ka - _mu() * k
                ys = [(zr[8 * a:8 * a + 8], zi[8 * a:8 * a + 8]) for a in range(16)]
                if g < 2:
                    ys = _fft16(ys, -1)
                for a in range(16):
                    zv[g][0, a, rows, :] = ys[a][0]
                    zv[g][1, a, rows, :] = ys[a][1]
            return run
        return [part(g) for g in range(3)]

    def post(u, carry):
        base = pl.multiple_of(32 * u, 32)
        side = []
        for q in range(4):
            side += dfwd_thunks(pl.ds(base, 32), q)
        side = [side[i] for i in CFG["post_order"]]
        k = 0
        at = list(CFG["post_at"])
        m, due = {}, []
        for prods in CFG["post_passes"]:
            acc = None
            for p in range(NPAIR):
                lhs = _strassen_lhs(*[
                    functools.partial(lambda r, e: qb[8 * r:8 * r + 8, u, 2 * p + e].reshape(64, 128), r, e)
                    for r in range(2) for e in range(2)])
                res = []
                for i in prods:
                    if i == 7:
                        oo = jnp.concatenate([qb[:, u, 2 * p + e].reshape(128, 128) for e in range(2)], axis=1)
                        res.append(_dot(oo.astype(bf16), wo_t[4, 256 * p:256 * p + 256, :]))
                        k += 2
                        continue
                    a = lhs[i]().astype(bf16)
                    for np_ in range(2):
                        if i in WS_SLOT:
                            w = ws[p, 5 * np_ + WS_SLOT[i]]
                        else:
                            kk = 0 if i == 1 else 1
                            w = wo_t[2 * np_ + kk, 256 * p + 128 * kk:256 * p + 128 * kk + 128, :]
                        if due and due[0][0] <= k:
                            w = _bf(_with_tokens(pltpu.bitcast(w, u32), {0: due.pop(0)[1]}))
                        res.append(_dot(a, w))
                    k += 1
                acc = addl(acc, res)
                while at and at[0] <= k:
                    g = CFG["post_order"][len(CFG["post_at"]) - len(at)] % 3
                    at.pop(0)
                    side.pop(0)()
                    if g == 0 and CFG["post_dl"]:
                        due.append((k + CFG["post_dl"],
                                    pltpu.bitcast(z0[0, u >> 2, 128:ZPITCH, :], u32)))
            for i in prods:
                m[i] = [acc.pop(0)] if i == 7 else [acc.pop(0), acc.pop(0)]
        cols = []
        for np_ in range(2):
            m1, m2, m3, m4, m5, m6, m7 = [m[i][np_] for i in range(7)]
            cols.append(jnp.concatenate([m1 + m4 - m5 + m7, m2 + m4], axis=0))
            cols.append(jnp.concatenate([m3 + m5, m1 - m2 + m3 + m6], axis=0))
        to[...] = jnp.concatenate(cols + m[7], axis=1).reshape(16, 8, DM)
        for f in side:
            f()
        return carry

    def spectral(zero):
        def fence(z):
            return z[0, zero, 128:ZPITCH, :]

        def radix(g, bb, sign):
            z = zs[g]
            toks = []

            def emit(q, y):
                for p in range(4):
                    z[0, q + 4 * p, chunk(bb), :] = y[p][0]
                    z[1, q + 4 * p, chunk(bb), :] = y[p][1]
                toks.append(fence(z))
            _fft16([(z[0, a, chunk(bb), :], z[1, a, chunk(bb), :]) for a in range(16)], sign, emit)
            return toks

        ys = {}

        def fwd(g, k2, toks):
            z = zs[g]
            ur, ui = z[0, k2, 0:64, :], z[1, k2, 0:64, :]
            tr, ti = _twiddle((z[0, k2, 64:128, :], z[1, k2, 64:128, :]), k2, 32, -1)
            for hf in range(2):
                v = _ilv(ur + tr, ui + ti) if hf == 0 else _ilv(ur - tr, ui - ti)
                lhs = _with_tokens(emat[k2 + 16 * hf], toks if hf == 0 else None)
                xr, xi = _dilv(_dot(_bf(lhs), v.astype(bf16)))
                ys["x", 16 * g + k2] = xr
                wr = wf[g, pl.ds(k2 * WPITCH + hf, 64, stride=2), :]
                wi = wf[g + 3, pl.ds(k2 * WPITCH + hf, 64, stride=2), :]
                ys[g, k2, hf] = _ilv(xr * wr - xi * wi, xr * wi + xi * wr).astype(bf16)

        def inv(g, k2, toks):
            z = zs[g]
            t0 = _dot(_bf(_with_tokens(emat[32 + k2], toks)), ys.pop((g, k2, 0)))
            t1 = _dot(_bf(emat[48 + k2]), ys.pop((g, k2, 1)))
            z[0, k2, 0:64, :], z[1, k2, 0:64, :] = _dilv(t0 + t1)
            z[0, k2, 64:128, :], z[1, k2, 64:128, :] = _twiddle(_dilv(t0 - t1), k2, 32, 1)

        units = [(g, k2) for g in range(3) for k2 in range(16)]
        toks = None
        lag = CFG["inv_lag"]
        for i in range(len(units) + lag):
            if i < len(units):
                fwd(*units[i], toks)
            if i >= lag:
                inv(*units[i - lag], toks if i >= len(units) else None)
            toks = []
            if i in CFG["fwd_at"]:
                toks += radix(2, CFG["fwd_at"].index(i), -1)
            for n, at in enumerate(CFG["inv_at"]):
                if at == i:
                    if not toks:
                        back, r = CFG["rel"]
                        zs[n // 16][1, zero, 128:ZPITCH, :] = ys["x", min(i - back, 47)][8 * r:8 * r + 8]
                    toks += radix(n // 16, n % 16, 1)
            pos = CFG["tok_pos"] if len(toks) <= 4 else range(8)
            toks = {j: pltpu.bitcast(t, u32) for j, t in zip(pos, toks)}

    def dinv_thunks(bb, finish):
        st = {}

        def part(g):
            def run():
                z = zs[g]
                ys = [(z[0, a, chunk(bb), :], z[1, a, chunk(bb), :]) for a in range(16)]
                if g >= CFG["inv_groups"]:
                    ys = _fft16(ys, 1)
                tr = jnp.concatenate([y[0] for y in ys], axis=0)
                ti = jnp.concatenate([y[1] for y in ys], axis=0)
                if g == 0 and CFG["pack_i"]:
                    lane = lax.broadcasted_iota(jnp.int32, (128, 128), 1)
                    v = jnp.where(lane <= 64, tr, pltpu.roll(ti, 64, 1))
                    st[0] = _dot(v.astype(bf16), _bf(small[8]))
                elif g == 0:
                    st[0] = _dot(tr.astype(bf16), _bf(small[8])) + _dot(ti.astype(bf16), _bf(small[9]))
                else:
                    k, ki, kr = [_dot(v.astype(bf16), _bf(small[7 + 3 * g + i]))
                                 for i, v in enumerate((tr + _mu() * ti, ti, tr))]
                    st[2 * g - 1], st[2 * g] = k + ki, k + kr
            return run

        def fin():
            p0, p1, q1, p2, q2 = [st[j] for j in range(5)]
            t = p1 + p2
            m, n = p0 - 0.25 * t, R5_D * (p1 - p2)
            e1, e2 = m + n, m - n
            o1, o2 = q1 + R5_R * q2, R5_R * q1 - q2
            y = jnp.concatenate([p0 + t, e1 - o1, e2 - o2, e2 + o2, e1 + o1], axis=1)
            finish(xb[:, chunk(bb), :].reshape(128, DM) + y)
        return [part(0), part(1), part(2), fin]

    def out_copy(bb):
        return pltpu.make_async_copy(xin.at[:, bb], out_hbm.at[:, bb], osem.at[bb])

    def layer(li, carry0):
        if full or CFG["only"] == "group":
            _loop("step", 0, 16, group, mem_ref[...].astype(f32))
        if full or CFG["only"] == "spec":
            _loop("post", 0, 4, post, 0, unroll=CFG["post_unroll"])

            with jax.named_scope("spectral"):
                spectral((li >> 1))
        if not full and CFG["only"] != "out":
            return carry0

        def run_chunks(th, order, lag):
            seq = [t[g] for t in th for g in order]
            for i in range(len(seq) + lag):
                if i < len(seq):
                    seq[i]()
                if i >= lag and (i - lag) % 3 == 2:
                    th[(i - lag) // 3][3]()

        @pl.when(li == 0)
        def _():
            with jax.named_scope("dinv_tails"):
                run_chunks([dinv_thunks(4 * u + 3, functools.partial(
                    lambda u, x: set_input(4 * u + 3, _round_bf16(x), u), u)) for u in range(4)],
                    *CFG["tails_order"])

            def batch(it, carry):
                bb = body_chunk(it)
                side = dinv_thunks(bb, lambda x: set_input(bb, _round_bf16(x), None))
                for k, f in enumerate(batch_thunks(it)):
                    f()
                    if k in CFG["dinv_at"]:
                        side.pop(0)()
                return carry
            _loop("batch", 0, 12, batch, 0, unroll=CFG["batch_unroll"])

        @pl.when(li == 1)
        def _():
            with jax.named_scope("dinv_out"):
                def store_out(bb, x):
                    xin[:, bb] = x.reshape(16, 8, DM).astype(bf16)
                    out_copy(bb).start()
                run_chunks([dinv_thunks(bb, functools.partial(store_out, bb)) for bb in range(16)],
                           *CFG["out_order"])
                for bb in range(16):
                    out_copy(bb).wait()
        return carry0

    if CFG["only"] != "pro":
        lax.fori_loop(0, 2, layer, 0)
    else:
        zero = zero_ref[0]
        xin[0, 0, :, 0:128] = (qb[zero, 0, 0] + wf[zero, 0:8, :] + xa[zero, 0:8, 0:128]).astype(bf16) + ws[zero, 0, 0:8, :]
        out_copy(0).start()
        out_copy(0).wait()


@jax.jit
def pallas_interleave_layers__memory_aug_recurrent_mem_tr__spectral_gfnet__prompt_kernel(
    A_x, A_mem0, A_Wq, A_Wk, A_Wv, A_Wo, A_seg_len, B_x, B_w_r, B_w_i,
):
    assert A_x.shape == (1, S, DM) and A_mem0.shape == (1, MEM, DM)
    small, emat = _tables()
    hbm = pl.BlockSpec(memory_space=pltpu.HBM)
    out = pl.pallas_call(
        _kernel,
        out_shape=jax.ShapeDtypeStruct((16, 16, 8, DM), bf16),
        in_specs=[hbm] * 10,
        out_specs=hbm,
        scratch_shapes=[
            pltpu.VMEM((16, 16, 8, DM), bf16),
            pltpu.VMEM((33, 128, DM), f32),
            pltpu.VMEM((16, 128, DM), f32),
            pltpu.VMEM((16, 8, DM), f32),
            pltpu.VMEM((12, 2, 320, 8, DH), bf16),
            pltpu.VMEM((13, 8 * HPITCH, 128), u32),
            pltpu.VMEM((13, 8 * HPITCH, 128), u32),
            pltpu.VMEM((5, H * DH + 512, 128), bf16),
            pltpu.VMEM((19, 10, 128, 128), bf16),
            pltpu.VMEM((16, 4, 96, 8, 128), f32),
            pltpu.VMEM((2, 16, 64, 128), u32),
            pltpu.VMEM((2, 16, ZPITCH, 128), f32),
            pltpu.VMEM((2, 16, ZPITCH, 128), f32),
            pltpu.VMEM((2, 16, ZPITCH, 128), f32),
            pltpu.VMEM((6, 16 * WPITCH + 32, 128), f32),
            pltpu.VMEM((9, DF, 512), bf16),
            pltpu.VMEM((4, 328, 128), f32),
            pltpu.VMEM((SMALL_TILES, 64, 128), u32),
            pltpu.VMEM((64, 64, 128), u32),
            pltpu.VMEM((80, 80), f32),
            pltpu.VMEM((MEM, DM), bf16),
            pltpu.SMEM((1,), jnp.int32),
            pltpu.SemaphoreType.DMA((47,)),
            pltpu.SemaphoreType.DMA((16,)),
        ],
        compiler_params=pltpu.CompilerParams(vmem_limit_bytes=120 * 1024 * 1024,
                                             disable_semaphore_checks=True),
    )(
        A_x.reshape(16, 16, 8, DM), A_mem0.reshape(MEM, DM),
        *[w.reshape(2, 320, H, DH) for w in (A_Wq, A_Wk, A_Wv)], A_Wo.reshape(H * DH, DM), B_w_r.T, B_w_i.T,
        jnp.asarray(small), jnp.asarray(emat),
    )
    return out.reshape(1, S, DM)
```

```python
import functools
import math

import jax
import jax.numpy as jnp
import numpy as np
from jax import lax
import jax.experimental.pallas as pl
import jax.experimental.pallas.tpu as pltpu

f32, bf16, u32 = jnp.float32, jnp.bfloat16, jnp.uint32

S, DM, H, DH, MEM, SEG = 2048, 640, 32, 128, 8, 32
NSEG = S // SEG
NPAIR = H // 2
DF = DM // 2 + 1
EPS = 1e-5
WPITCH = 132

HPITCH = 164
ZPITCH = 136

S1 = math.sin(2 * math.pi / 5)
R5_D = (math.cos(2 * math.pi / 5) - math.cos(4 * math.pi / 5)) / 2
R5_R = math.sin(4 * math.pi / 5) / S1


def _to_bf16_bits(a):
    u = np.ascontiguousarray(a, dtype=np.float32).view(np.uint32).astype(np.uint64)
    return ((u + 0x7FFF + ((u >> 16) & 1)) >> 16).astype(np.uint32)


def _pack_rows(a):
    b = _to_bf16_bits(a)
    return b[..., 0::2, :] | (b[..., 1::2, :] << 16)


@functools.lru_cache(maxsize=None)
def _tables():
    b = np.arange(128)
    l0 = np.arange(0, DF, 5)
    l1 = np.concatenate([np.arange(1, 320, 5), np.arange(4, 320, 5)])
    l2 = np.concatenate([np.arange(2, 320, 5), np.arange(3, 320, 5)])
    sg = np.concatenate([np.ones(64), -np.ones(64)])

    def th(l):
        return 2 * np.pi * ((b[:, None] * l[None, :]) % DM) / DM

    sc = 1.0 / (S * DM)
    fw = np.zeros((8, 128, 128))
    iw = np.zeros((8, 128, 128))
    t = th(l0)
    cl = np.full((65, 1), 2.0)
    cl[0] = cl[-1] = 1.0
    fw[0, :, :65], fw[1, :, :65] = np.cos(t), -np.sin(t)
    iw[0, :65], iw[1, :65] = cl * np.cos(t.T) * sc, -cl * np.sin(t.T) * sc
    if CFG["pack_f"]:
        fw[0, :, 65:] = fw[1, :, 1:64]
    if CFG["pack_i"]:
        iw[0, 65:] = iw[1, 1:64]
    mu = S1 * sg
    for g, l in ((1, l1), (2, l2)):
        t = th(l)
        c, s = np.cos(t), np.sin(t)
        fw[3 * g - 1:3 * g + 2] = c, -mu * s - c, mu * c - s
        iw[3 * g - 1:3 * g + 2] = [2 * sc * m.T for m in (c, -s - mu * c, mu * s - c)]
    n = np.arange(64)
    order = np.concatenate([np.concatenate([np.arange(8) + 8 * j, np.arange(8) + 8 * j + 64])
                            for j in range(8)])
    e = np.zeros((2, 32, 128, 128))
    for k2 in range(32):
        t = 2 * np.pi * (((32 * n[:, None] + k2) * n[None, :]) % S) / S
        er, ei = np.cos(t), -np.sin(t)
        m = np.block([[er, -ei], [ei, er]])[order][:, order]
        e[0, k2], e[1, k2] = m, m.T
    small = np.concatenate([_pack_rows(fw), _pack_rows(iw)], axis=0)
    return small, _pack_rows(e).reshape(64, 64, 128)


SMALL_TILES = 16


def _loop(name, lo, hi, body, init, **kw):
    with jax.named_scope(name):
        return lax.fori_loop(lo, hi, body, init, **kw)


def _bf(x):
    return pltpu.bitcast(x, bf16)


def _dot(a, b):
    return jnp.dot(a, b, preferred_element_type=f32)


def _round_bf16(x):
    return x.astype(bf16).astype(f32)


def _layernorm(x):
    m = jnp.mean(x, axis=-1, keepdims=True)
    xc = x - m
    v = jnp.mean(xc * xc, axis=-1, keepdims=True)
    return xc * lax.rsqrt(v + EPS)


def _fft4(x, sign):
    (ar, ai), (br, bi), (cr, ci), (dr, di) = x
    t0r, t0i, t1r, t1i = ar + cr, ai + ci, ar - cr, ai - ci
    t2r, t2i, t3r, t3i = br + dr, bi + di, br - dr, bi - di
    y0, y2 = (t0r + t2r, t0i + t2i), (t0r - t2r, t0i - t2i)
    p, q = (t1r + t3i, t1i - t3r), (t1r - t3i, t1i + t3r)
    return [y0, p, y2, q] if sign < 0 else [y0, q, y2, p]


def _twiddle(z, n, period, sign):
    zr, zi = z
    n = n % period
    if n == 0:
        return z
    if 4 * n == period:
        return (-zi, zr) if sign > 0 else (zi, -zr)
    c, s = math.cos(2 * math.pi * n / period), sign * math.sin(2 * math.pi * n / period)
    if (8 * n) % period == 0:
        a, d = zr + zi, zr - zi
        if c * s > 0:
            return (d * c, a * c)
        return (a * c, d * s)
    return (zr * c - zi * s, zr * s + zi * c)


def _bsum(x, y, sign):
    x, y = x.astype(f32), y.astype(f32)
    return (x + y if sign > 0 else x - y).astype(bf16)


def _strassen_lhs(a11, a12, a21, a22):
    return [lambda: a11() + a22(), lambda: a21() + a22(), a11, a22,
            lambda: a11() + a12(), lambda: a21() - a11(), lambda: a12() - a22()]


def _strassen_rhs(b11, b12, b21, b22):
    return [lambda: _bsum(b11(), b22(), 1), b11, lambda: _bsum(b12(), b22(), -1),
            lambda: _bsum(b21(), b11(), -1), b22, lambda: _bsum(b11(), b12(), 1),
            lambda: _bsum(b21(), b22(), 1)]


STRASSEN_OUT = [(((0, 0), 1), ((1, 1), 1)), (((1, 0), 1), ((1, 1), -1)), (((0, 1), 1), ((1, 1), 1)),
                (((0, 0), 1), ((1, 0), 1)), (((0, 0), -1), ((0, 1), 1)), (((1, 1), 1),), (((0, 0), 1),),
                (((0, 0), 1),), (((0, 1), 1),), (((1, 0), 1),), (((1, 1), 1),)]
WS_SLOT = {0: 0, 2: 1, 3: 2, 5: 3, 6: 4}


def _mu():
    lane = lax.broadcasted_iota(jnp.int32, (1, 128), 1)
    return jnp.where(lane < 64, S1, -S1).astype(f32)


def _ilv(r, i):
    n = r.shape[0] // 8
    return jnp.concatenate([r.reshape(n, 8, 128), i.reshape(n, 8, 128)], axis=1).reshape(16 * n, 128)


def _dilv(x):
    n = x.shape[0] // 16
    x = x.reshape(n, 16, 128)
    return x[:, :8].reshape(8 * n, 128), x[:, 8:].reshape(8 * n, 128)


def _with_tokens(x, toks):
    if not toks:
        return x
    return jnp.concatenate(
        [x[8 * j:8 * j + 8] | toks[j] if j in toks else x[8 * j:8 * j + 8]
         for j in range(x.shape[0] // 8)], axis=0)


def _fft16(x, sign, emit=None):
    cols = [_fft4([x[4 * j + r] for j in range(4)], sign) for r in range(4)]
    out = [None] * 16
    for q in range(4):
        y = _fft4([_twiddle(cols[r][q], r * q, 16, sign) for r in range(4)], sign)
        for p in range(4):
            out[q + 4 * p] = y[p]
        if emit is not None:
            emit(q, y)
    return out


CFG = dict(steps=((4.5, 16.5, 6, 4, 0, 8), (5, 16.5, 5, 7, 8, 12), (5, 16.5, 6, 6, 8, 12), (5, 16.5, 8, 7, 8, 0)),
           post_dl=20, post_passes=((0, 1), (2, 3), (4, 5), (6, 7)),
           post_order=(0, 1, 6, 3, 4, 2, 8, 5, 7, 9, 10, 11), post_at=(22, 26, 68, 96),
           tails_order=((1, 2, 0), 5), out_order=((1, 2, 0), 5), pack_f=True, pack_i=True,
           inv_at=tuple(range(28, 44)), inv_groups=1, inv_lag=4, tok_pos=(4, 5, 6, 7),
           fwd_at=(7, 8, 9, 10, 12, 13, 14, 16, 17, 18, 20, 21, 22, 24, 25, 26), rel=(0, 1), dinv_at=(17, 18, 19, 19), dinv_order=(2, 1, 0),
           unit_order=((10, 5, 0), (7, 6, 1), (2, 4), (8, 3, 9)), two=False, batch_unroll=2, post_unroll=1,
           ws_split=4, ws_at=(9, 9, 10, 11, 12, 13, 14, 15, 16, 16, 17, 18, 19, 20, 21, 22),
           pro_nre=15, re_pos=(2, 3, 7), ln_at=(13, 20, 27, 31), ln_at2=(4, 7, 10, 13),
           perm_at=(11, 13, 15, 18, 20, 23, 25, 27, 30, 31, 31, 31), only=None)


def _interleave(main, side):
    n, k = len(main), 0
    for i, f in enumerate(main):
        f()
        while k < len(side) and (k + 1) * n <= (i + 1) * len(side):
            side[k]()
            k += 1
    for f in side[k:]:
        f()


def _kernel(x_hbm, mem_hbm, wq_hbm, wk_hbm, wv_hbm, wo_hbm, wr_hbm, wi_hbm,
            small_hbm, e_hbm, out_hbm,
            xin, xa, xb, to, raw, wa, wb, wo_t, ws, qb, hl, z0, z1, z2, wf,
            wri, wtmp, small, emat, fill_ref, mem_ref, zero_ref, sem, osem):
    zs = (z0, z1, z2)
    w_hbm = (wq_hbm, wk_hbm, wv_hbm)

    def body_chunk(i):
        return 4 * (i & 3) + (i >> 2)

    def cp_w(i):
        src = w_hbm[i >> 2].at[:, :, pl.ds(8 * (i & 3), 8), :] if isinstance(i, int) else raw.at[i]
        return pltpu.make_async_copy(src, raw.at[i], sem.at[i])

    def cp_x(bb):
        return pltpu.make_async_copy(x_hbm.at[:, bb], xin.at[:, bb], sem.at[12 + bb])

    def cp_f(i):
        src = ((wr_hbm, wi_hbm)[i >> 2].at[:, pl.ds(512 * (i & 3), 512)]
               if isinstance(i, int) else wri.at[i])
        return pltpu.make_async_copy(src, wri.at[i], sem.at[36 + i])

    def cp_wo(i):
        rows = pl.ds(pl.multiple_of(512 * i, 512), 512)
        return [pltpu.make_async_copy(wo_hbm.at[rows, pl.ds(128 * j, 128)], wo_t.at[j, rows], sem.at[28 + i])
                for j in range(5)]

    cp_rest = [pltpu.make_async_copy(mem_hbm, mem_ref, sem.at[46]),
                pltpu.make_async_copy(small_hbm, small, sem.at[44]),
               pltpu.make_async_copy(e_hbm, emat, sem.at[45])]

    full = CFG["only"] in (None, "pro")
    for u in range(4 if full else 0):
        cp_x(4 * u + 3).start()
    if full:
        cp_w(0).start()
    for i in range(12 if full else 0):
        if i < 11:
            cp_w(i + 1).start()
        cp_x(body_chunk(i)).start()
        if 3 <= i < 11:
            cp_f(i - 3).start()
            for cp in cp_wo(i - 3):
                cp.start()
    for cp in cp_rest if full else ():
        cp.start()

    zero_ref[0] = 0

    r = lax.broadcasted_iota(jnp.int32, (80, 80), 0)
    c = lax.broadcasted_iota(jnp.int32, (80, 80), 1)

    def head(i):
        return jnp.where(i < 64, i // 32, (i - 64) // 8)

    def pos(i):
        return jnp.where(i < 64, i % 32, 32 + (i - 64) % 8)

    ok = (pos(r) < MEM) | (pos(r) >= pos(c))
    fill_ref[...] = jnp.where(head(r) == head(c), jnp.where(ok, 0.0, -1e9), -jnp.inf).astype(f32)
    wtmp[:, 320:328, :] = jnp.zeros((4, 8, 128), f32)
    xa[32, 0:8, 0:128] = jnp.zeros((8, 128), f32)
    ws[18, 0, 0:16, :] = jnp.zeros((16, 128), bf16)
    wa[12, 0:8, :] = jnp.zeros((8, 128), u32)
    wb[12, 0:8, :] = jnp.zeros((8, 128), u32)
    wf[5, 16 * WPITCH:16 * WPITCH + 8, :] = jnp.zeros((8, 128), f32)
    for z in zs:
        z[0, 0, 128:ZPITCH, :] = jnp.zeros((8, 128), f32)

    def chunk(bb):
        if isinstance(bb, int):
            return slice(8 * bb, 8 * bb + 8)
        return pl.ds(pl.multiple_of(8 * bb, 8), 8)

    def set_input(bb, x, tail_u, a0=0):
        n = x.shape[0] // 8
        xa[a0:a0 + n, chunk(bb), :] = x.reshape(n, 8, DM)
        y = _layernorm(x)
        if tail_u is None:
            xa[16 + a0:16 + a0 + n, chunk(bb), :] = y.reshape(n, 8, DM)
        else:
            blk = [[y[64 * r:64 * r + 64, 128 * kt:128 * kt + 128] for kt in range(5)] for r in range(2)]
            ops = []
            for kp in range(2):
                (a11, a12), (a21, a22) = [blk[r][2 * kp:2 * kp + 2] for r in range(2)]
                ops += [a11 + a22, a21 + a22, a11, a22, a11 + a12, a21 - a11, a12 - a22]
            for i, v in enumerate(ops + [blk[0][4], blk[1][4]]):
                hl[tail_u >> 1, i, 32 * (tail_u & 1):32 * (tail_u & 1) + 32, :] = (
                    pltpu.bitcast(v.astype(bf16), u32))

    def load_x(bb, a0=0, n=16):
        return xin[a0:a0 + n, bb].astype(f32).reshape(8 * n, DM)

    def wtile(cid, j, e):
        w = (wa, wb)[e]
        return jnp.concatenate([w[cid, (4 * hf + j) * HPITCH:(4 * hf + j) * HPITCH + 160, :]
                                for hf in range(2)], axis=0)

    def relayout(i, cid, e):
        for r in range(4 * i, 4 * i + 4):
            a, b = [pltpu.bitcast(raw[cid, :, d].reshape(16, 128), u32) for d in (2 * r, 2 * r + 1)]
            v = (a & 0xFFFF) | (b << 16) if e == 0 else (a >> 16) | (b & jnp.uint32(0xFFFF0000))
            (wa, wb)[e][cid, pl.ds(r, 8, stride=HPITCH), :] = v

    def batch_thunks(cid):
        qv = qb.at[:, :, pl.ds(8 * cid, 8)]

        def unit(e, jp, s):
            c = {}

            def w(n, kt):
                return _bf(wtile(cid, 2 * jp + n, e)[64 * kt:64 * kt + 64])

            def rhs(i, kp):
                return _strassen_rhs(*[functools.partial(w, n, 2 * kp + k)
                                       for k in range(2) for n in range(2)])[i]()

            def prod(i, toks=None):
                l0, l1 = _bf(_with_tokens(hl[s, i], toks)), _bf(hl[s, 7 + i])
                return _dot(l0, rhs(i, 0)) + _dot(l1, rhs(i, 1))

            def last(r, n, toks=None):
                return _dot(_bf(_with_tokens(hl[s, 14 + r], toks)), w(n, 4))

            def store(r, n):
                y = c.pop((r, n)).reshape(2, 8, 8, 128)
                for k in range(2):
                    qv[8 * r:8 * r + 8, 2 * s + k, 2 * (2 * jp + n) + e] = y[k]

            left = {(0, 0): 5, (0, 1): 3, (1, 0): 3, (1, 1): 5}

            def thunk(items):
                def run(toks=None):
                    for i in items:
                        y = prod(i, toks) if i < 7 else last((i - 7) >> 1, (i - 7) & 1, toks)
                        toks = None
                        for blk, sign in STRASSEN_OUT[i]:
                            if blk not in c:
                                c[blk] = y if sign > 0 else -y
                            else:
                                c[blk] = c[blk] + y if sign > 0 else c[blk] - y
                            left[blk] -= 1
                            if left[blk] == 0:
                                store(*blk)
                return run
            return [thunk(items) for items in CFG["unit_order"]]
        return [f for e in range(2) for jp in range(2) for s in range(2) for f in unit(e, jp, s)]

    def wperm_thunks(piece, j):
        m = (piece >> 2) & 1
        wt = wtmp.at[j]

        def load():
            wt[0:DF, :] = wri[piece, :, 128 * j:128 * j + 128].astype(f32)

        def one(g):
            def run():
                if g == 0:
                    t = jnp.concatenate([wt[pl.ds(0, 64, stride=5), :], wt[320:328, :],
                                         jnp.zeros((56, 128), f32)], axis=0)
                else:
                    t = jnp.concatenate([wt[pl.ds(g, 64, stride=5), :],
                                         wt[pl.ds(5 - g, 64, stride=5), :]], axis=0)
                y = t.T
                sub = wf.at[3 * m + g, pl.ds(pl.multiple_of((piece & 3) * 32, 32), 16 * WPITCH - 96)]
                for k in range(8):
                    for hf in range(2):
                        sub[pl.ds(8 * j + k + 8 * hf * WPITCH, 8, stride=WPITCH), :] = (
                            y[16 * k + 8 * hf:16 * k + 8 * hf + 8])
            return run
        return [load] + [one(g) for g in range(3)]

    def half_pass(cid, half, fill, zero, timed=()):
        nre = CFG["pro_nre"]
        toks = None
        for k, f in enumerate(batch_thunks(cid)[16 * half:16 * half + 16]):
            f(toks)
            toks = {}
            for n, f in enumerate(f for at, f in timed if at == k):
                toks[(0, 4, 1, 6)[n]] = f()
            if fill is not None:
                for n, r in enumerate(r for r in range(40) if r * nre // 40 == k):
                    relayout(r, fill, 1 - half)
                    toks[CFG["re_pos"][n]] = (wb, wa)[half][12 + zero, 0:8, :]

    def ln_parts(bb, zero):
        def part(j):
            set_input(bb, load_x(bb, 4 * j, 4), None, 4 * j)
            return pltpu.bitcast(xa[32 + zero, 0:8, 0:128], u32)
        return [functools.partial(part, j) for j in range(4)]

    def perm_parts(piece, zero):
        def part(fs):
            for f in fs:
                f()
            return pltpu.bitcast(wf[5 + zero, 16 * WPITCH:16 * WPITCH + 8, :], u32)
        out = []
        for j in range(4):
            th = wperm_thunks(piece, j)
            out += [functools.partial(part, th[0:2]), functools.partial(part, th[2:3]),
                    functools.partial(part, th[3:4])]
        return out

    def ws_parts(piece, zero):
        nr = 128 // CFG["ws_split"]

        src = wo_t.at[:, pl.ds(pl.multiple_of(512 * piece, 512), 512)]
        dst = ws.at[pl.ds(2 * piece, 2)]

        def part(pp, np_, r0):
            def tile(k, n):
                lo = 256 * pp + 128 * k + r0
                return src[2 * np_ + n, lo:lo + nr, :]
            rhs = _strassen_rhs(*[functools.partial(tile, k, n) for k in range(2) for n in range(2)])
            for i, slot in WS_SLOT.items():
                dst[pp, 5 * np_ + slot, r0:r0 + nr, :] = rhs[i]()
            return pltpu.bitcast(ws[18 + zero, 0, 0:16, :], u32)
        return [functools.partial(part, pp, np_, r0)
                for pp in range(2) for np_ in range(2) for r0 in range(0, 128, nr)]

    def pro0():
        for u in range(4):
            cp_x(4 * u + 3).wait()
        for u in range(4):
            set_input(4 * u + 3, load_x(4 * u + 3), u)
        cp_w(0).wait()
        zero = zero_ref[0]
        for i in range(40):
            relayout(i, 0, 0)
        half_pass(0, 0, zero, zero)

    def pro1(it, carry):
        bb = body_chunk(it)
        with jax.named_scope("pro1_wait"):
            cp_w(it + 1).wait()

            @pl.when(it >= 3)
            def _():
                cp_f(it - 3).wait()
                for cp in cp_wo(it - 3):
                    cp.wait()
            cp_x(bb).wait()
        piece = jnp.where(it >= 3, it - 3, 8)
        zero = it >> 4
        timed = sorted(list(zip(CFG["ln_at"], ln_parts(bb, zero)))
                       + list(zip(CFG["ws_at"], ws_parts(piece, zero)))
                       + list(zip(CFG["perm_at"], perm_parts(piece, zero))), key=lambda x: x[0])
        half_pass(it, 1, it + 1, zero, [x for x in timed if x[0] < 16])
        half_pass(it + 1, 0, it + 1, zero, [(k - 16, f) for k, f in timed if k >= 16])
        return carry

    def pro2():
        cp_x(body_chunk(11)).wait()
        for cp in cp_rest:
            cp.wait()
        zero = zero_ref[0]
        half_pass(11, 1, None, zero, list(zip(CFG["ln_at2"], ln_parts(body_chunk(11), zero))))

    if full:
        with jax.named_scope("pro0"):
            pro0()
        _loop("pro1", 0, 11, pro1, 0)
        with jax.named_scope("pro2"):
            pro2()

    scale = DH ** -0.5

    def wo_dot(hh, oo):
        return [_dot(oo, wo_t[j, 128 * hh:128 * hh + 128, :]) for j in range(5)]

    def addl(acc, res):
        return res if acc is None else [a + b for a, b in zip(acc, res)]

    def group(g, mem):
        for ph in range(4):
            h = jnp.concatenate([mem, xa[16 + g, 32 * ph:32 * ph + 24, :]], axis=0).astype(bf16)
            pr, sm, oos = {}, {}, {}
            lat_s, lat_pv, lat_wo, v_delay, n_first, n_last = CFG["steps"][ph]

            def stacked(p, m):
                tails = [qb[g, ph, 32 * m + 2 * p + e] for e in range(2)]
                return jnp.concatenate([pr[p, m, 0], pr[p, m, 1]] + tails, axis=0).astype(bf16)

            def scores(p):
                sc = lax.dot_general(stacked(p, 0), stacked(p, 1), (((1,), (1,)), ((), ())),
                                     preferred_element_type=f32)
                fill = fill_ref[...]
                sc = jnp.where(fill == 0.0, sc * scale, fill)
                mx = jnp.max(sc, axis=-1, keepdims=True)
                e = jnp.exp(sc - mx)
                rl = pl.reciprocal(jnp.sum(e, axis=-1, keepdims=True), approx=True)
                sm[p] = (e * rl).astype(bf16)

            def pv(p):
                o = _dot(sm[p], stacked(p, 2))
                for e in range(2):
                    qb[g, ph, 2 * p + e] = o[64 + 8 * e:72 + 8 * e]
                    oos[2 * p + e] = o[32 * e:32 * e + 32].astype(bf16)

            keyed = []
            for p in range(NPAIR):
                keyed += [(4 * p + 2 * m + e, (p, m, e)) for m in range(2) for e in range(2)]
                keyed += [(4 * p + 3.5 + v_delay, (p, 2, e)) for e in range(2)]
            bulk = [x for _, x in sorted(keyed, key=lambda kv: kv[0])]
            acc, t, nwo, pend, ready = None, 0.0, 0, [], []
            if n_first:
                first, bulk = bulk[:n_first], bulk[n_first:]
                for kt in range(5):
                    for p, m, e in first:
                        w = wtile(4 * m + (p >> 2), p & 3, e)[64 * kt:64 * kt + 64]
                        y = _dot(h[:, 128 * kt:128 * kt + 128], _bf(w))
                        pr[p, m, e] = y if kt == 0 else pr[p, m, e] + y
                t = float(len(first))
                pend = [(t + lat_s, "S", p) for p, m, e in first if m == 1 and e == 1]
            while nwo < H - n_last or pend:
                pend.sort()
                if pend and pend[0][0] <= t:
                    _, kind, p = pend.pop(0)
                    if kind == "S":
                        scores(p)
                        pend.append((t + lat_pv, "V", p))
                    else:
                        pv(p)
                        ready += [(t + lat_wo, 2 * p + e) for e in range(2)]
                    t += 0.5
                elif bulk:
                    p, m, e = bulk.pop(0)
                    pr[p, m, e] = _dot(h, _bf(wtile(4 * m + (p >> 2), p & 3, e)))
                    t += 1
                    if m == 1 and e == 1:
                        pend.append((t + lat_s, "S", p))
                elif ready and ready[0][0] <= t and nwo < H - n_last:
                    _, hh = ready.pop(0)
                    acc = addl(acc, wo_dot(hh, oos[hh]))
                    t += 1
                    nwo += 1
                else:
                    t += 0.5
            for j in range(5):
                for _, hh in ready:
                    acc[j] = acc[j] + _dot(oos[hh], wo_t[j, 128 * hh:128 * hh + 128, :])
            out = jnp.concatenate(acc, axis=1)
            xa[16 + g, 32 * ph:32 * ph + 24, :] = out[8:32]
            mem = _round_bf16(out[0:8])
        return mem

    def dfwd_thunks(seg, q):
        st = {}
        rows = chunk(q)
        xav, xbv, zv = xa.at[:, seg], xb.at[:, seg], [z.at[:, :, seg] for z in zs]

        def pre():
            o = to[...] if q == 3 else xav[16:32, rows, :]
            x = _round_bf16(xav[0:16, rows, :] + o)
            xbv[:, rows, :] = x
            y = _layernorm(x.reshape(128, DM))
            x0, x1, x2, x3, x4 = [y[:, 128 * a:128 * a + 128] for a in range(5)]
            t1, t2, t3, t4 = x1 + x4, x2 + x3, x1 - x4, x2 - x3
            t = t1 + t2
            m, n = x0 - 0.25 * t, R5_D * (t1 - t2)
            st["u"] = [x0 + t, (m + n, t3 + R5_R * t4), (m - n, R5_R * t3 - t4)]

        def part(g):
            def run():
                if g == 0:
                    pre()
                    u0 = st["u"][0].astype(bf16)
                    zr = _dot(u0, _bf(small[0]))
                    if CFG["pack_f"]:
                        lane = lax.broadcasted_iota(jnp.int32, (128, 128), 1)
                        zi = jnp.where((lane & 63) == 0, 0.0, pltpu.roll(zr, 64, 1))
                    else:
                        zi = _dot(u0, _bf(small[1]))
                else:
                    a, b = st["u"][g]
                    k, kb, ka = [_dot(v.astype(bf16), _bf(small[3 * g - 1 + i]))
                                 for i, v in enumerate((a + b, b, a))]
                    zr, zi = k + kb, ka - _mu() * k
                ys = [(zr[8 * a:8 * a + 8], zi[8 * a:8 * a + 8]) for a in range(16)]
                if g < 2:
                    ys = _fft16(ys, -1)
                for a in range(16):
                    zv[g][0, a, rows, :] = ys[a][0]
                    zv[g][1, a, rows, :] = ys[a][1]
            return run
        return [part(g) for g in range(3)]

    def post(u, carry):
        base = pl.multiple_of(32 * u, 32)
        side = []
        for q in range(4):
            side += dfwd_thunks(pl.ds(base, 32), q)
        side = [side[i] for i in CFG["post_order"]]
        k = 0
        at = list(CFG["post_at"])
        m, due = {}, []
        for prods in CFG["post_passes"]:
            acc = None
            for p in range(NPAIR):
                lhs = _strassen_lhs(*[
                    functools.partial(lambda r, e: qb[8 * r:8 * r + 8, u, 2 * p + e].reshape(64, 128), r, e)
                    for r in range(2) for e in range(2)])
                res = []
                for i in prods:
                    if i == 7:
                        oo = jnp.concatenate([qb[:, u, 2 * p + e].reshape(128, 128) for e in range(2)], axis=1)
                        res.append(_dot(oo.astype(bf16), wo_t[4, 256 * p:256 * p + 256, :]))
                        k += 2
                        continue
                    a = lhs[i]().astype(bf16)
                    for np_ in range(2):
                        if i in WS_SLOT:
                            w = ws[p, 5 * np_ + WS_SLOT[i]]
                        else:
                            kk = 0 if i == 1 else 1
                            w = wo_t[2 * np_ + kk, 256 * p + 128 * kk:256 * p + 128 * kk + 128, :]
                        if due and due[0][0] <= k:
                            w = _bf(_with_tokens(pltpu.bitcast(w, u32), {0: due.pop(0)[1]}))
                        res.append(_dot(a, w))
                    k += 1
                acc = addl(acc, res)
                while at and at[0] <= k:
                    g = CFG["post_order"][len(CFG["post_at"]) - len(at)] % 3
                    at.pop(0)
                    side.pop(0)()
                    if g == 0 and CFG["post_dl"]:
                        due.append((k + CFG["post_dl"],
                                    pltpu.bitcast(z0[0, u >> 2, 128:ZPITCH, :], u32)))
            for i in prods:
                m[i] = [acc.pop(0)] if i == 7 else [acc.pop(0), acc.pop(0)]
        cols = []
        for np_ in range(2):
            m1, m2, m3, m4, m5, m6, m7 = [m[i][np_] for i in range(7)]
            cols.append(jnp.concatenate([m1 + m4 - m5 + m7, m2 + m4], axis=0))
            cols.append(jnp.concatenate([m3 + m5, m1 - m2 + m3 + m6], axis=0))
        to[...] = jnp.concatenate(cols + m[7], axis=1).reshape(16, 8, DM)
        for f in side:
            f()
        return carry

    def spectral(zero):
        def fence(z):
            return z[0, zero, 128:ZPITCH, :]

        def radix(g, bb, sign):
            z = zs[g]
            toks = []

            def emit(q, y):
                for p in range(4):
                    z[0, q + 4 * p, chunk(bb), :] = y[p][0]
                    z[1, q + 4 * p, chunk(bb), :] = y[p][1]
                toks.append(fence(z))
            _fft16([(z[0, a, chunk(bb), :], z[1, a, chunk(bb), :]) for a in range(16)], sign, emit)
            return toks

        ys = {}

        def fwd(g, k2, toks):
            z = zs[g]
            ur, ui = z[0, k2, 0:64, :], z[1, k2, 0:64, :]
            tr, ti = _twiddle((z[0, k2, 64:128, :], z[1, k2, 64:128, :]), k2, 32, -1)
            for hf in range(2):
                v = _ilv(ur + tr, ui + ti) if hf == 0 else _ilv(ur - tr, ui - ti)
                lhs = _with_tokens(emat[k2 + 16 * hf], toks if hf == 0 else None)
                xr, xi = _dilv(_dot(_bf(lhs), v.astype(bf16)))
                ys["x", 16 * g + k2] = xr
                wr = wf[g, pl.ds(k2 * WPITCH + hf, 64, stride=2), :]
                wi = wf[g + 3, pl.ds(k2 * WPITCH + hf, 64, stride=2), :]
                ys[g, k2, hf] = _ilv(xr * wr - xi * wi, xr * wi + xi * wr).astype(bf16)

        def inv(g, k2, toks):
            z = zs[g]
            t0 = _dot(_bf(_with_tokens(emat[32 + k2], toks)), ys.pop((g, k2, 0)))
            t1 = _dot(_bf(emat[48 + k2]), ys.pop((g, k2, 1)))
            z[0, k2, 0:64, :], z[1, k2, 0:64, :] = _dilv(t0 + t1)
            z[0, k2, 64:128, :], z[1, k2, 64:128, :] = _twiddle(_dilv(t0 - t1), k2, 32, 1)

        units = [(g, k2) for g in range(3) for k2 in range(16)]
        toks = None
        lag = CFG["inv_lag"]
        for i in range(len(units) + lag):
            if i < len(units):
                fwd(*units[i], toks)
            if i >= lag:
                inv(*units[i - lag], toks if i >= len(units) else None)
            toks = []
            if i in CFG["fwd_at"]:
                toks += radix(2, CFG["fwd_at"].index(i), -1)
            for n, at in enumerate(CFG["inv_at"]):
                if at == i:
                    if not toks:
                        back, r = CFG["rel"]
                        zs[n // 16][1, zero, 128:ZPITCH, :] = ys["x", min(i - back, 47)][8 * r:8 * r + 8]
                    toks += radix(n // 16, n % 16, 1)
            pos = CFG["tok_pos"] if len(toks) <= 4 else range(8)
            toks = {j: pltpu.bitcast(t, u32) for j, t in zip(pos, toks)}

    def dinv_thunks(bb, finish):
        st = {}

        def part(g):
            def run():
                z = zs[g]
                ys = [(z[0, a, chunk(bb), :], z[1, a, chunk(bb), :]) for a in range(16)]
                if g >= CFG["inv_groups"]:
                    ys = _fft16(ys, 1)
                tr = jnp.concatenate([y[0] for y in ys], axis=0)
                ti = jnp.concatenate([y[1] for y in ys], axis=0)
                if g == 0 and CFG["pack_i"]:
                    lane = lax.broadcasted_iota(jnp.int32, (128, 128), 1)
                    v = jnp.where(lane <= 64, tr, pltpu.roll(ti, 64, 1))
                    st[0] = _dot(v.astype(bf16), _bf(small[8]))
                elif g == 0:
                    st[0] = _dot(tr.astype(bf16), _bf(small[8])) + _dot(ti.astype(bf16), _bf(small[9]))
                else:
                    k, ki, kr = [_dot(v.astype(bf16), _bf(small[7 + 3 * g + i]))
                                 for i, v in enumerate((tr + _mu() * ti, ti, tr))]
                    st[2 * g - 1], st[2 * g] = k + ki, k + kr
            return run

        def fin():
            p0, p1, q1, p2, q2 = [st[j] for j in range(5)]
            t = p1 + p2
            m, n = p0 - 0.25 * t, R5_D * (p1 - p2)
            e1, e2 = m + n, m - n
            o1, o2 = q1 + R5_R * q2, R5_R * q1 - q2
            y = jnp.concatenate([p0 + t, e1 - o1, e2 - o2, e2 + o2, e1 + o1], axis=1)
            finish(xb[:, chunk(bb), :].reshape(128, DM) + y)
        return [part(0), part(1), part(2), fin]

    def out_copy(bb):
        return pltpu.make_async_copy(xin.at[:, bb], out_hbm.at[:, bb], osem.at[bb])

    def layer(li, carry0):
        if full or CFG["only"] == "group":
            _loop("step", 0, 16, group, mem_ref[...].astype(f32))
        if full or CFG["only"] == "spec":
            _loop("post", 0, 4, post, 0, unroll=CFG["post_unroll"])

            with jax.named_scope("spectral"):
                spectral((li >> 1))
        if not full and CFG["only"] != "out":
            return carry0

        def run_chunks(th, order, lag):
            seq = [t[g] for t in th for g in order]
            for i in range(len(seq) + lag):
                if i < len(seq):
                    seq[i]()
                if i >= lag and (i - lag) % 3 == 2:
                    th[(i - lag) // 3][3]()

        @pl.when(li == 0)
        def _():
            with jax.named_scope("dinv_tails"):
                run_chunks([dinv_thunks(4 * u + 3, functools.partial(
                    lambda u, x: set_input(4 * u + 3, _round_bf16(x), u), u)) for u in range(4)],
                    *CFG["tails_order"])

            def batch(it, carry):
                bb = body_chunk(it)
                side = dinv_thunks(bb, lambda x: set_input(bb, _round_bf16(x), None))
                for k, f in enumerate(batch_thunks(it)):
                    f()
                    for at, g in zip(CFG["dinv_at"], CFG["dinv_order"] + (3,)):
                        if at == k:
                            side[g]()
                return carry
            _loop("batch", 0, 12, batch, 0, unroll=CFG["batch_unroll"])

        @pl.when(li == 1)
        def _():
            with jax.named_scope("dinv_out"):
                def store_out(bb, x):
                    xin[:, bb] = x.reshape(16, 8, DM).astype(bf16)
                    out_copy(bb).start()
                run_chunks([dinv_thunks(bb, functools.partial(store_out, bb)) for bb in range(16)],
                           *CFG["out_order"])
                for bb in range(16):
                    out_copy(bb).wait()
        return carry0

    if CFG["only"] != "pro":
        lax.fori_loop(0, 2, layer, 0)
    if CFG["only"] in ("pro", "out"):
        zero = zero_ref[0]
        xin[0, 0, :, 0:128] = (qb[zero, 0, 0] + wf[zero, 0:8, :] + xa[zero, 0:8, 0:128]).astype(bf16) + ws[zero, 0, 0:8, :]
        out_copy(0).start()
        out_copy(0).wait()


@jax.jit
def pallas_interleave_layers__memory_aug_recurrent_mem_tr__spectral_gfnet__prompt_kernel(
    A_x, A_mem0, A_Wq, A_Wk, A_Wv, A_Wo, A_seg_len, B_x, B_w_r, B_w_i,
):
    assert A_x.shape == (1, S, DM) and A_mem0.shape == (1, MEM, DM)
    small, emat = _tables()
    hbm = pl.BlockSpec(memory_space=pltpu.HBM)
    out = pl.pallas_call(
        _kernel,
        out_shape=jax.ShapeDtypeStruct((16, 16, 8, DM), bf16),
        in_specs=[hbm] * 10,
        out_specs=hbm,
        scratch_shapes=[
            pltpu.VMEM((16, 16, 8, DM), bf16),
            pltpu.VMEM((33, 128, DM), f32),
            pltpu.VMEM((16, 128, DM), f32),
            pltpu.VMEM((16, 8, DM), f32),
            pltpu.VMEM((12, 2, 320, 8, DH), bf16),
            pltpu.VMEM((13, 8 * HPITCH, 128), u32),
            pltpu.VMEM((13, 8 * HPITCH, 128), u32),
            pltpu.VMEM((5, H * DH + 512, 128), bf16),
            pltpu.VMEM((19, 10, 128, 128), bf16),
            pltpu.VMEM((16, 4, 96, 8, 128), f32),
            pltpu.VMEM((2, 16, 64, 128), u32),
            pltpu.VMEM((2, 16, ZPITCH, 128), f32),
            pltpu.VMEM((2, 16, ZPITCH, 128), f32),
            pltpu.VMEM((2, 16, ZPITCH, 128), f32),
            pltpu.VMEM((6, 16 * WPITCH + 32, 128), f32),
            pltpu.VMEM((9, DF, 512), bf16),
            pltpu.VMEM((4, 328, 128), f32),
            pltpu.VMEM((SMALL_TILES, 64, 128), u32),
            pltpu.VMEM((64, 64, 128), u32),
            pltpu.VMEM((80, 80), f32),
            pltpu.VMEM((MEM, DM), bf16),
            pltpu.SMEM((1,), jnp.int32),
            pltpu.SemaphoreType.DMA((47,)),
            pltpu.SemaphoreType.DMA((16,)),
        ],
        compiler_params=pltpu.CompilerParams(vmem_limit_bytes=120 * 1024 * 1024,
                                             disable_semaphore_checks=True),
    )(
        A_x.reshape(16, 16, 8, DM), A_mem0.reshape(MEM, DM),
        *[w.reshape(2, 320, H, DH) for w in (A_Wq, A_Wk, A_Wv)], A_Wo.reshape(H * DH, DM), B_w_r.T, B_w_i.T,
        jnp.asarray(small), jnp.asarray(emat),
    )
    return out.reshape(1, S, DM)
```

```python
import functools
import math

import jax
import jax.numpy as jnp
import numpy as np
from jax import lax
import jax.experimental.pallas as pl
import jax.experimental.pallas.tpu as pltpu

f32, bf16, u32 = jnp.float32, jnp.bfloat16, jnp.uint32

S, DM, H, DH, MEM, SEG = 2048, 640, 32, 128, 8, 32
NSEG = S // SEG
NPAIR = H // 2
DF = DM // 2 + 1
EPS = 1e-5
WPITCH = 132

HPITCH = 164
ZPITCH = 136

S1 = math.sin(2 * math.pi / 5)
R5_D = (math.cos(2 * math.pi / 5) - math.cos(4 * math.pi / 5)) / 2
R5_R = math.sin(4 * math.pi / 5) / S1


def _to_bf16_bits(a):
    u = np.ascontiguousarray(a, dtype=np.float32).view(np.uint32).astype(np.uint64)
    return ((u + 0x7FFF + ((u >> 16) & 1)) >> 16).astype(np.uint32)


def _pack_rows(a):
    b = _to_bf16_bits(a)
    return b[..., 0::2, :] | (b[..., 1::2, :] << 16)


@functools.lru_cache(maxsize=None)
def _tables():
    b = np.arange(128)
    l0 = np.arange(0, DF, 5)
    l1 = np.concatenate([np.arange(1, 320, 5), np.arange(4, 320, 5)])
    l2 = np.concatenate([np.arange(2, 320, 5), np.arange(3, 320, 5)])
    sg = np.concatenate([np.ones(64), -np.ones(64)])

    def th(l):
        return 2 * np.pi * ((b[:, None] * l[None, :]) % DM) / DM

    sc = 1.0 / (S * DM)
    fw = np.zeros((8, 128, 128))
    iw = np.zeros((8, 128, 128))
    t = th(l0)
    cl = np.full((65, 1), 2.0)
    cl[0] = cl[-1] = 1.0
    fw[0, :, :65], fw[1, :, :65] = np.cos(t), -np.sin(t)
    iw[0, :65], iw[1, :65] = cl * np.cos(t.T) * sc, -cl * np.sin(t.T) * sc
    if CFG["pack_f"]:
        fw[0, :, 65:] = fw[1, :, 1:64]
    if CFG["pack_i"]:
        iw[0, 65:] = iw[1, 1:64]
    mu = S1 * sg
    for g, l in ((1, l1), (2, l2)):
        t = th(l)
        c, s = np.cos(t), np.sin(t)
        fw[3 * g - 1:3 * g + 2] = c, -mu * s - c, mu * c - s
        iw[3 * g - 1:3 * g + 2] = [2 * sc * m.T for m in (c, -s - mu * c, mu * s - c)]
    n = np.arange(64)
    order = np.concatenate([np.concatenate([np.arange(8) + 8 * j, np.arange(8) + 8 * j + 64])
                            for j in range(8)])
    e = np.zeros((2, 32, 128, 128))
    for k2 in range(32):
        t = 2 * np.pi * (((32 * n[:, None] + k2) * n[None, :]) % S) / S
        er, ei = np.cos(t), -np.sin(t)
        m = np.block([[er, -ei], [ei, er]])[order][:, order]
        e[0, k2], e[1, k2] = m, m.T
    small = np.concatenate([_pack_rows(fw), _pack_rows(iw)], axis=0)
    return small, _pack_rows(e).reshape(64, 64, 128)


SMALL_TILES = 16


def _loop(name, lo, hi, body, init, **kw):
    with jax.named_scope(name):
        return lax.fori_loop(lo, hi, body, init, **kw)


def _bf(x):
    return pltpu.bitcast(x, bf16)


def _dot(a, b):
    return jnp.dot(a, b, preferred_element_type=f32)


def _round_bf16(x):
    return x.astype(bf16).astype(f32)


def _layernorm(x):
    m = jnp.mean(x, axis=-1, keepdims=True)
    xc = x - m
    v = jnp.mean(xc * xc, axis=-1, keepdims=True)
    return xc * lax.rsqrt(v + EPS)


def _fft4(x, sign):
    (ar, ai), (br, bi), (cr, ci), (dr, di) = x
    t0r, t0i, t1r, t1i = ar + cr, ai + ci, ar - cr, ai - ci
    t2r, t2i, t3r, t3i = br + dr, bi + di, br - dr, bi - di
    y0, y2 = (t0r + t2r, t0i + t2i), (t0r - t2r, t0i - t2i)
    p, q = (t1r + t3i, t1i - t3r), (t1r - t3i, t1i + t3r)
    return [y0, p, y2, q] if sign < 0 else [y0, q, y2, p]


def _twiddle(z, n, period, sign):
    zr, zi = z
    n = n % period
    if n == 0:
        return z
    if 4 * n == period:
        return (-zi, zr) if sign > 0 else (zi, -zr)
    c, s = math.cos(2 * math.pi * n / period), sign * math.sin(2 * math.pi * n / period)
    if (8 * n) % period == 0:
        a, d = zr + zi, zr - zi
        if c * s > 0:
            return (d * c, a * c)
        return (a * c, d * s)
    return (zr * c - zi * s, zr * s + zi * c)


def _bsum(x, y, sign):
    x, y = x.astype(f32), y.astype(f32)
    return (x + y if sign > 0 else x - y).astype(bf16)


def _strassen_lhs(a11, a12, a21, a22):
    return [lambda: a11() + a22(), lambda: a21() + a22(), a11, a22,
            lambda: a11() + a12(), lambda: a21() - a11(), lambda: a12() - a22()]


def _strassen_rhs(b11, b12, b21, b22):
    return [lambda: _bsum(b11(), b22(), 1), b11, lambda: _bsum(b12(), b22(), -1),
            lambda: _bsum(b21(), b11(), -1), b22, lambda: _bsum(b11(), b12(), 1),
            lambda: _bsum(b21(), b22(), 1)]


STRASSEN_OUT = [(((0, 0), 1), ((1, 1), 1)), (((1, 0), 1), ((1, 1), -1)), (((0, 1), 1), ((1, 1), 1)),
                (((0, 0), 1), ((1, 0), 1)), (((0, 0), -1), ((0, 1), 1)), (((1, 1), 1),), (((0, 0), 1),),
                (((0, 0), 1),), (((0, 1), 1),), (((1, 0), 1),), (((1, 1), 1),)]
WS_SLOT = {0: 0, 2: 1, 3: 2, 5: 3, 6: 4}


def _mu():
    lane = lax.broadcasted_iota(jnp.int32, (1, 128), 1)
    return jnp.where(lane < 64, S1, -S1).astype(f32)


def _ilv(r, i):
    n = r.shape[0] // 8
    return jnp.concatenate([r.reshape(n, 8, 128), i.reshape(n, 8, 128)], axis=1).reshape(16 * n, 128)


def _dilv(x):
    n = x.shape[0] // 16
    x = x.reshape(n, 16, 128)
    return x[:, :8].reshape(8 * n, 128), x[:, 8:].reshape(8 * n, 128)


def _with_tokens(x, toks):
    if not toks:
        return x
    return jnp.concatenate(
        [x[8 * j:8 * j + 8] | toks[j] if j in toks else x[8 * j:8 * j + 8]
         for j in range(x.shape[0] // 8)], axis=0)


def _fft16(x, sign, emit=None):
    cols = [_fft4([x[4 * j + r] for j in range(4)], sign) for r in range(4)]
    out = [None] * 16
    for q in range(4):
        y = _fft4([_twiddle(cols[r][q], r * q, 16, sign) for r in range(4)], sign)
        for p in range(4):
            out[q + 4 * p] = y[p]
        if emit is not None:
            emit(q, y)
    return out


CFG = dict(steps=((4.5, 16.5, 6, 4, 0, 8), (5, 16.5, 5, 7, 8, 12), (5, 16.5, 6, 6, 8, 12), (5, 16.5, 8, 7, 8, 0)),
           post_dl=20, post_passes=((0, 1), (2, 3), (4, 5), (6, 7)),
           post_order=(0, 1, 6, 3, 4, 2, 8, 5, 7, 9, 10, 11), post_at=(22, 26, 68, 96),
           tails_order=((1, 2, 0), 5), out_order=((1, 2, 0), 5), pack_f=True, pack_i=True,
           inv_at=tuple(range(28, 44)), inv_groups=1, inv_lag=4, tok_pos=(4, 5, 6, 7),
           fwd_at=(7, 8, 9, 10, 12, 13, 14, 16, 17, 18, 20, 21, 22, 24, 25, 26), rel=(0, 1), dinv_at=(0, 0, 1, 1), dinv_order=(2, 1, 0),
           unit_order=((10, 5, 0), (7, 6, 1), (2, 4), (8, 3, 9)), two='f32',
           two_inner=(5, 4, 2, 8, 0, 3, 6, 7, 10, 1, 9),
           two_outer=((2, 2), (5, 3), (1, None), (0, None), (4, 0), (3, None), (6, 1)),
           batch_unroll=2, post_unroll=1,
           ws_split=4, ws_at=(9, 9, 10, 11, 12, 13, 14, 15, 16, 16, 17, 18, 19, 20, 21, 22),
           pro_nre=15, re_pos=(2, 3, 7), ln_at=(13, 20, 27, 31), ln_at2=(4, 7, 10, 13),
           perm_at=(11, 13, 15, 18, 20, 23, 25, 27, 30, 31, 31, 31), only=None)


def _interleave(main, side):
    n, k = len(main), 0
    for i, f in enumerate(main):
        f()
        while k < len(side) and (k + 1) * n <= (i + 1) * len(side):
            side[k]()
            k += 1
    for f in side[k:]:
        f()


def _kernel(x_hbm, mem_hbm, wq_hbm, wk_hbm, wv_hbm, wo_hbm, wr_hbm, wi_hbm,
            small_hbm, e_hbm, out_hbm,
            xin, xa, xb, to, raw, wa, wb, wo_t, ws, qb, hl, hl2, z0, z1, z2, wf,
            wri, wtmp, small, emat, fill_ref, mem_ref, zero_ref, sem, osem):
    zs = (z0, z1, z2)
    w_hbm = (wq_hbm, wk_hbm, wv_hbm)

    def body_chunk(i):
        return 4 * (i & 3) + (i >> 2)

    def cp_w(i):
        src = w_hbm[i >> 2].at[:, :, pl.ds(8 * (i & 3), 8), :] if isinstance(i, int) else raw.at[i]
        return pltpu.make_async_copy(src, raw.at[i], sem.at[i])

    def cp_x(bb):
        return pltpu.make_async_copy(x_hbm.at[:, bb], xin.at[:, bb], sem.at[12 + bb])

    def cp_f(i):
        src = ((wr_hbm, wi_hbm)[i >> 2].at[:, pl.ds(512 * (i & 3), 512)]
               if isinstance(i, int) else wri.at[i])
        return pltpu.make_async_copy(src, wri.at[i], sem.at[36 + i])

    def cp_wo(i):
        rows = pl.ds(pl.multiple_of(512 * i, 512), 512)
        return [pltpu.make_async_copy(wo_hbm.at[rows, pl.ds(128 * j, 128)], wo_t.at[j, rows], sem.at[28 + i])
                for j in range(5)]

    cp_rest = [pltpu.make_async_copy(mem_hbm, mem_ref, sem.at[46]),
                pltpu.make_async_copy(small_hbm, small, sem.at[44]),
               pltpu.make_async_copy(e_hbm, emat, sem.at[45])]

    full = CFG["only"] in (None, "pro")
    for u in range(4 if full else 0):
        cp_x(4 * u + 3).start()
    if full:
        cp_w(0).start()
    for i in range(12 if full else 0):
        if i < 11:
            cp_w(i + 1).start()
        cp_x(body_chunk(i)).start()
        if 3 <= i < 11:
            cp_f(i - 3).start()
            for cp in cp_wo(i - 3):
                cp.start()
    for cp in cp_rest if full else ():
        cp.start()

    zero_ref[0] = 0

    r = lax.broadcasted_iota(jnp.int32, (80, 80), 0)
    c = lax.broadcasted_iota(jnp.int32, (80, 80), 1)

    def head(i):
        return jnp.where(i < 64, i // 32, (i - 64) // 8)

    def pos(i):
        return jnp.where(i < 64, i % 32, 32 + (i - 64) % 8)

    ok = (pos(r) < MEM) | (pos(r) >= pos(c))
    fill_ref[...] = jnp.where(head(r) == head(c), jnp.where(ok, 0.0, -1e9), -jnp.inf).astype(f32)
    wtmp[:, 320:328, :] = jnp.zeros((4, 8, 128), f32)
    xa[32, 0:8, 0:128] = jnp.zeros((8, 128), f32)
    ws[18, 0, 0:16, :] = jnp.zeros((16, 128), bf16)
    wa[12, 0:8, :] = jnp.zeros((8, 128), u32)
    wb[12, 0:8, :] = jnp.zeros((8, 128), u32)
    wf[5, 16 * WPITCH:16 * WPITCH + 8, :] = jnp.zeros((8, 128), f32)
    for z in zs:
        z[0, 0, 128:ZPITCH, :] = jnp.zeros((8, 128), f32)

    def chunk(bb):
        if isinstance(bb, int):
            return slice(8 * bb, 8 * bb + 8)
        return pl.ds(pl.multiple_of(8 * bb, 8), 8)

    def set_input(bb, x, tail_u, a0=0, two=False):
        n = x.shape[0] // 8
        xa[a0:a0 + n, chunk(bb), :] = x.reshape(n, 8, DM)
        y = _layernorm(x)
        if tail_u is None:
            xa[16 + a0:16 + a0 + n, chunk(bb), :] = y.reshape(n, 8, DM)
        elif two:
            blk = [[y[32 * r:32 * r + 32, 128 * kt:128 * kt + 128] for kt in range(5)] for r in range(4)]
            lv1 = [_strassen_lhs(*[functools.partial(lambda v: v, blk[2 * rr + r][2 * kk + k])
                                   for rr in range(2) for kk in range(2)])
                   for r in range(2) for k in range(2)]
            ops = []
            for i in range(7):
                sub = [f[i]() for f in lv1]
                ops += [f() for f in _strassen_lhs(*[functools.partial(lambda v: v, v) for v in sub])]
            for i, v in enumerate(ops + [blk[r][4] for r in range(4)]):
                hl2[i, 16 * tail_u:16 * tail_u + 16, :] = pltpu.bitcast(v.astype(bf16), u32)
        else:
            blk = [[y[64 * r:64 * r + 64, 128 * kt:128 * kt + 128] for kt in range(5)] for r in range(2)]
            ops = []
            for kp in range(2):
                (a11, a12), (a21, a22) = [blk[r][2 * kp:2 * kp + 2] for r in range(2)]
                ops += [a11 + a22, a21 + a22, a11, a22, a11 + a12, a21 - a11, a12 - a22]
            for i, v in enumerate(ops + [blk[0][4], blk[1][4]]):
                hl[tail_u >> 1, i, 32 * (tail_u & 1):32 * (tail_u & 1) + 32, :] = (
                    pltpu.bitcast(v.astype(bf16), u32))

    def load_x(bb, a0=0, n=16):
        return xin[a0:a0 + n, bb].astype(f32).reshape(8 * n, DM)

    def wtile(cid, j, e):
        w = (wa, wb)[e]
        return jnp.concatenate([w[cid, (4 * hf + j) * HPITCH:(4 * hf + j) * HPITCH + 160, :]
                                for hf in range(2)], axis=0)

    def relayout(i, cid, e):
        for r in range(4 * i, 4 * i + 4):
            a, b = [pltpu.bitcast(raw[cid, :, d].reshape(16, 128), u32) for d in (2 * r, 2 * r + 1)]
            v = (a & 0xFFFF) | (b << 16) if e == 0 else (a >> 16) | (b & jnp.uint32(0xFFFF0000))
            (wa, wb)[e][cid, pl.ds(r, 8, stride=HPITCH), :] = v

    def batch_thunks(cid):
        qv = qb.at[:, :, pl.ds(8 * cid, 8)]

        def unit(e, jp, s):
            c = {}

            def w(n, kt):
                return _bf(wtile(cid, 2 * jp + n, e)[64 * kt:64 * kt + 64])

            def rhs(i, kp):
                return _strassen_rhs(*[functools.partial(w, n, 2 * kp + k)
                                       for k in range(2) for n in range(2)])[i]()

            def prod(i, toks=None):
                l0, l1 = _bf(_with_tokens(hl[s, i], toks)), _bf(hl[s, 7 + i])
                return _dot(l0, rhs(i, 0)) + _dot(l1, rhs(i, 1))

            def last(r, n, toks=None):
                return _dot(_bf(_with_tokens(hl[s, 14 + r], toks)), w(n, 4))

            def store(r, n):
                y = c.pop((r, n)).reshape(2, 8, 8, 128)
                for k in range(2):
                    qv[8 * r:8 * r + 8, 2 * s + k, 2 * (2 * jp + n) + e] = y[k]

            left = {(0, 0): 5, (0, 1): 3, (1, 0): 3, (1, 1): 5}

            def thunk(items):
                def run(toks=None):
                    for i in items:
                        y = prod(i, toks) if i < 7 else last((i - 7) >> 1, (i - 7) & 1, toks)
                        toks = None
                        for blk, sign in STRASSEN_OUT[i]:
                            if blk not in c:
                                c[blk] = y if sign > 0 else -y
                            else:
                                c[blk] = c[blk] + y if sign > 0 else c[blk] - y
                            left[blk] -= 1
                            if left[blk] == 0:
                                store(*blk)
                return run
            return [thunk(items) for items in CFG["unit_order"]]
        return [f for e in range(2) for jp in range(2) for s in range(2) for f in unit(e, jp, s)]

    def batch2_thunks(cid):
        qv = qb.at[:, :, pl.ds(8 * cid, 8)]
        RH = [((0, 0, 1), (1, 1, 1)), ((0, 0, 1),), ((0, 1, 1), (1, 1, -1)), ((1, 0, 1), (0, 0, -1)),
              ((1, 1, 1),), ((0, 0, 1), (0, 1, 1)), ((1, 0, 1), (1, 1, 1))]

        def unit(e):
            c = {}
            left = {(r, n): (5, 3, 3, 5)[2 * (r >> 1) + (n >> 1)] for r in range(4) for n in range(4)}

            def w(n, kt):
                return _bf(wtile(cid, n, e)[64 * kt:64 * kt + 64])

            def acc(blk, y, sign):
                if blk not in c:
                    c[blk] = y if sign > 0 else -y
                else:
                    c[blk] = c[blk] + y if sign > 0 else c[blk] - y
                left[blk] -= 1
                if left[blk] == 0:
                    r, n = blk
                    y = c.pop(blk).reshape(4, 4, 8, 128)
                    for u in range(4):
                        qv[4 * r:4 * r + 4, u, 2 * n + e] = y[u]

            def outer(I, k4):
                st = {}

                def lvl1(k, n):
                    if (k, n) not in st:
                        t = [(w(2 * nn + n, 2 * kk + k), sg) for kk, nn, sg in RH[I]]
                        if len(t) == 1:
                            st[k, n] = t[0][0]
                        elif CFG["two"] == "pack":
                            st[k, n] = _bsum(t[0][0], t[1][0], t[1][1])
                        else:
                            x, y = t[0][0].astype(f32), t[1][0].astype(f32)
                            st[k, n] = x + y if t[1][1] > 0 else x - y
                    return st[k, n]
                p = {}
                pl_ = {(0, 0): 4, (0, 1): 2, (1, 0): 2, (1, 1): 4}

                def half(items):
                    def run(toks=None):
                        for i in items:
                            if i >= 7:
                                r, n = k4[i - 7]
                                acc((r, n), _dot(_bf(hl2[49 + r]), w(n, 4)), 1)
                                continue
                            t = [(lvl1(k, n), sg) for k, n, sg in RH[i]]
                            rhs = t[0][0].astype(bf16) if len(t) == 1 else _bsum(t[0][0], t[1][0], t[1][1])
                            y = _dot(_bf(_with_tokens(hl2[7 * I + i], toks)), rhs)
                            toks = None
                            for blk, sign in STRASSEN_OUT[i]:
                                if blk not in p:
                                    p[blk] = y if sign > 0 else -y
                                else:
                                    p[blk] = p[blk] + y if sign > 0 else p[blk] - y
                                pl_[blk] -= 1
                                if pl_[blk] == 0:
                                    for (R, N), sg in STRASSEN_OUT[I]:
                                        acc((2 * R + blk[0], 2 * N + blk[1]), p[blk], sg)
                    return run
                items = [i for i in CFG["two_inner"] if i < 7 + len(k4)]
                return [half(items[:len(items) // 2]), half(items[len(items) // 2:])]
            out = []
            for I, q in CFG["two_outer"]:
                k4 = [] if q is None else [(2 * (q >> 1) + (j >> 1), 2 * (q & 1) + (j & 1)) for j in range(4)]
                out += outer(I, k4)
            return out
        return unit(0) + unit(1)

    def wperm_thunks(piece, j):
        m = (piece >> 2) & 1
        wt = wtmp.at[j]

        def load():
            wt[0:DF, :] = wri[piece, :, 128 * j:128 * j + 128].astype(f32)

        def one(g):
            def run():
                if g == 0:
                    t = jnp.concatenate([wt[pl.ds(0, 64, stride=5), :], wt[320:328, :],
                                         jnp.zeros((56, 128), f32)], axis=0)
                else:
                    t = jnp.concatenate([wt[pl.ds(g, 64, stride=5), :],
                                         wt[pl.ds(5 - g, 64, stride=5), :]], axis=0)
                y = t.T
                sub = wf.at[3 * m + g, pl.ds(pl.multiple_of((piece & 3) * 32, 32), 16 * WPITCH - 96)]
                for k in range(8):
                    for hf in range(2):
                        sub[pl.ds(8 * j + k + 8 * hf * WPITCH, 8, stride=WPITCH), :] = (
                            y[16 * k + 8 * hf:16 * k + 8 * hf + 8])
            return run
        return [load] + [one(g) for g in range(3)]

    def half_pass(cid, half, fill, zero, timed=()):
        nre = CFG["pro_nre"]
        toks = None
        for k, f in enumerate(batch_thunks(cid)[16 * half:16 * half + 16]):
            f(toks)
            toks = {}
            for n, f in enumerate(f for at, f in timed if at == k):
                toks[(0, 4, 1, 6)[n]] = f()
            if fill is not None:
                for n, r in enumerate(r for r in range(40) if r * nre // 40 == k):
                    relayout(r, fill, 1 - half)
                    toks[CFG["re_pos"][n]] = (wb, wa)[half][12 + zero, 0:8, :]

    def ln_parts(bb, zero):
        def part(j):
            set_input(bb, load_x(bb, 4 * j, 4), None, 4 * j)
            return pltpu.bitcast(xa[32 + zero, 0:8, 0:128], u32)
        return [functools.partial(part, j) for j in range(4)]

    def perm_parts(piece, zero):
        def part(fs):
            for f in fs:
                f()
            return pltpu.bitcast(wf[5 + zero, 16 * WPITCH:16 * WPITCH + 8, :], u32)
        out = []
        for j in range(4):
            th = wperm_thunks(piece, j)
            out += [functools.partial(part, th[0:2]), functools.partial(part, th[2:3]),
                    functools.partial(part, th[3:4])]
        return out

    def ws_parts(piece, zero):
        nr = 128 // CFG["ws_split"]

        src = wo_t.at[:, pl.ds(pl.multiple_of(512 * piece, 512), 512)]
        dst = ws.at[pl.ds(2 * piece, 2)]

        def part(pp, np_, r0):
            def tile(k, n):
                lo = 256 * pp + 128 * k + r0
                return src[2 * np_ + n, lo:lo + nr, :]
            rhs = _strassen_rhs(*[functools.partial(tile, k, n) for k in range(2) for n in range(2)])
            for i, slot in WS_SLOT.items():
                dst[pp, 5 * np_ + slot, r0:r0 + nr, :] = rhs[i]()
            return pltpu.bitcast(ws[18 + zero, 0, 0:16, :], u32)
        return [functools.partial(part, pp, np_, r0)
                for pp in range(2) for np_ in range(2) for r0 in range(0, 128, nr)]

    def pro0():
        for u in range(4):
            cp_x(4 * u + 3).wait()
        for u in range(4):
            set_input(4 * u + 3, load_x(4 * u + 3), u)
        cp_w(0).wait()
        zero = zero_ref[0]
        for i in range(40):
            relayout(i, 0, 0)
        half_pass(0, 0, zero, zero)

    def pro1(it, carry):
        bb = body_chunk(it)
        with jax.named_scope("pro1_wait"):
            cp_w(it + 1).wait()

            @pl.when(it >= 3)
            def _():
                cp_f(it - 3).wait()
                for cp in cp_wo(it - 3):
                    cp.wait()
            cp_x(bb).wait()
        piece = jnp.where(it >= 3, it - 3, 8)
        zero = it >> 4
        timed = sorted(list(zip(CFG["ln_at"], ln_parts(bb, zero)))
                       + list(zip(CFG["ws_at"], ws_parts(piece, zero)))
                       + list(zip(CFG["perm_at"], perm_parts(piece, zero))), key=lambda x: x[0])
        half_pass(it, 1, it + 1, zero, [x for x in timed if x[0] < 16])
        half_pass(it + 1, 0, it + 1, zero, [(k - 16, f) for k, f in timed if k >= 16])
        return carry

    def pro2():
        cp_x(body_chunk(11)).wait()
        for cp in cp_rest:
            cp.wait()
        zero = zero_ref[0]
        half_pass(11, 1, None, zero, list(zip(CFG["ln_at2"], ln_parts(body_chunk(11), zero))))

    if full:
        with jax.named_scope("pro0"):
            pro0()
        _loop("pro1", 0, 11, pro1, 0)
        with jax.named_scope("pro2"):
            pro2()

    scale = DH ** -0.5

    def wo_dot(hh, oo):
        return [_dot(oo, wo_t[j, 128 * hh:128 * hh + 128, :]) for j in range(5)]

    def addl(acc, res):
        return res if acc is None else [a + b for a, b in zip(acc, res)]

    def group(g, mem):
        for ph in range(4):
            h = jnp.concatenate([mem, xa[16 + g, 32 * ph:32 * ph + 24, :]], axis=0).astype(bf16)
            pr, sm, oos = {}, {}, {}
            lat_s, lat_pv, lat_wo, v_delay, n_first, n_last = CFG["steps"][ph]

            def stacked(p, m):
                tails = [qb[g, ph, 32 * m + 2 * p + e] for e in range(2)]
                return jnp.concatenate([pr[p, m, 0], pr[p, m, 1]] + tails, axis=0).astype(bf16)

            def scores(p):
                sc = lax.dot_general(stacked(p, 0), stacked(p, 1), (((1,), (1,)), ((), ())),
                                     preferred_element_type=f32)
                fill = fill_ref[...]
                sc = jnp.where(fill == 0.0, sc * scale, fill)
                mx = jnp.max(sc, axis=-1, keepdims=True)
                e = jnp.exp(sc - mx)
                rl = pl.reciprocal(jnp.sum(e, axis=-1, keepdims=True), approx=True)
                sm[p] = (e * rl).astype(bf16)

            def pv(p):
                o = _dot(sm[p], stacked(p, 2))
                for e in range(2):
                    qb[g, ph, 2 * p + e] = o[64 + 8 * e:72 + 8 * e]
                    oos[2 * p + e] = o[32 * e:32 * e + 32].astype(bf16)

            keyed = []
            for p in range(NPAIR):
                keyed += [(4 * p + 2 * m + e, (p, m, e)) for m in range(2) for e in range(2)]
                keyed += [(4 * p + 3.5 + v_delay, (p, 2, e)) for e in range(2)]
            bulk = [x for _, x in sorted(keyed, key=lambda kv: kv[0])]
            acc, t, nwo, pend, ready = None, 0.0, 0, [], []
            if n_first:
                first, bulk = bulk[:n_first], bulk[n_first:]
                for kt in range(5):
                    for p, m, e in first:
                        w = wtile(4 * m + (p >> 2), p & 3, e)[64 * kt:64 * kt + 64]
                        y = _dot(h[:, 128 * kt:128 * kt + 128], _bf(w))
                        pr[p, m, e] = y if kt == 0 else pr[p, m, e] + y
                t = float(len(first))
                pend = [(t + lat_s, "S", p) for p, m, e in first if m == 1 and e == 1]
            while nwo < H - n_last or pend:
                pend.sort()
                if pend and pend[0][0] <= t:
                    _, kind, p = pend.pop(0)
                    if kind == "S":
                        scores(p)
                        pend.append((t + lat_pv, "V", p))
                    else:
                        pv(p)
                        ready += [(t + lat_wo, 2 * p + e) for e in range(2)]
                    t += 0.5
                elif bulk:
                    p, m, e = bulk.pop(0)
                    pr[p, m, e] = _dot(h, _bf(wtile(4 * m + (p >> 2), p & 3, e)))
                    t += 1
                    if m == 1 and e == 1:
                        pend.append((t + lat_s, "S", p))
                elif ready and ready[0][0] <= t and nwo < H - n_last:
                    _, hh = ready.pop(0)
                    acc = addl(acc, wo_dot(hh, oos[hh]))
                    t += 1
                    nwo += 1
                else:
                    t += 0.5
            for j in range(5):
                for _, hh in ready:
                    acc[j] = acc[j] + _dot(oos[hh], wo_t[j, 128 * hh:128 * hh + 128, :])
            out = jnp.concatenate(acc, axis=1)
            xa[16 + g, 32 * ph:32 * ph + 24, :] = out[8:32]
            mem = _round_bf16(out[0:8])
        return mem

    def dfwd_thunks(seg, q):
        st = {}
        rows = chunk(q)
        xav, xbv, zv = xa.at[:, seg], xb.at[:, seg], [z.at[:, :, seg] for z in zs]

        def pre():
            o = to[...] if q == 3 else xav[16:32, rows, :]
            x = _round_bf16(xav[0:16, rows, :] + o)
            xbv[:, rows, :] = x
            y = _layernorm(x.reshape(128, DM))
            x0, x1, x2, x3, x4 = [y[:, 128 * a:128 * a + 128] for a in range(5)]
            t1, t2, t3, t4 = x1 + x4, x2 + x3, x1 - x4, x2 - x3
            t = t1 + t2
            m, n = x0 - 0.25 * t, R5_D * (t1 - t2)
            st["u"] = [x0 + t, (m + n, t3 + R5_R * t4), (m - n, R5_R * t3 - t4)]

        def part(g):
            def run():
                if g == 0:
                    pre()
                    u0 = st["u"][0].astype(bf16)
                    zr = _dot(u0, _bf(small[0]))
                    if CFG["pack_f"]:
                        lane = lax.broadcasted_iota(jnp.int32, (128, 128), 1)
                        zi = jnp.where((lane & 63) == 0, 0.0, pltpu.roll(zr, 64, 1))
                    else:
                        zi = _dot(u0, _bf(small[1]))
                else:
                    a, b = st["u"][g]
                    k, kb, ka = [_dot(v.astype(bf16), _bf(small[3 * g - 1 + i]))
                                 for i, v in enumerate((a + b, b, a))]
                    zr, zi = k + kb, ka - _mu() * k
                ys = [(zr[8 * a:8 * a + 8], zi[8 * a:8 * a + 8]) for a in range(16)]
                if g < 2:
                    ys = _fft16(ys, -1)
                for a in range(16):
                    zv[g][0, a, rows, :] = ys[a][0]
                    zv[g][1, a, rows, :] = ys[a][1]
            return run
        return [part(g) for g in range(3)]

    def post(u, carry):
        base = pl.multiple_of(32 * u, 32)
        side = []
        for q in range(4):
            side += dfwd_thunks(pl.ds(base, 32), q)
        side = [side[i] for i in CFG["post_order"]]
        k = 0
        at = list(CFG["post_at"])
        m, due = {}, []
        for prods in CFG["post_passes"]:
            acc = None
            for p in range(NPAIR):
                lhs = _strassen_lhs(*[
                    functools.partial(lambda r, e: qb[8 * r:8 * r + 8, u, 2 * p + e].reshape(64, 128), r, e)
                    for r in range(2) for e in range(2)])
                res = []
                for i in prods:
                    if i == 7:
                        oo = jnp.concatenate([qb[:, u, 2 * p + e].reshape(128, 128) for e in range(2)], axis=1)
                        res.append(_dot(oo.astype(bf16), wo_t[4, 256 * p:256 * p + 256, :]))
                        k += 2
                        continue
                    a = lhs[i]().astype(bf16)
                    for np_ in range(2):
                        if i in WS_SLOT:
                            w = ws[p, 5 * np_ + WS_SLOT[i]]
                        else:
                            kk = 0 if i == 1 else 1
                            w = wo_t[2 * np_ + kk, 256 * p + 128 * kk:256 * p + 128 * kk + 128, :]
                        if due and due[0][0] <= k:
                            w = _bf(_with_tokens(pltpu.bitcast(w, u32), {0: due.pop(0)[1]}))
                        res.append(_dot(a, w))
                    k += 1
                acc = addl(acc, res)
                while at and at[0] <= k:
                    g = CFG["post_order"][len(CFG["post_at"]) - len(at)] % 3
                    at.pop(0)
                    side.pop(0)()
                    if g == 0 and CFG["post_dl"]:
                        due.append((k + CFG["post_dl"],
                                    pltpu.bitcast(z0[0, u >> 2, 128:ZPITCH, :], u32)))
            for i in prods:
                m[i] = [acc.pop(0)] if i == 7 else [acc.pop(0), acc.pop(0)]
        cols = []
        for np_ in range(2):
            m1, m2, m3, m4, m5, m6, m7 = [m[i][np_] for i in range(7)]
            cols.append(jnp.concatenate([m1 + m4 - m5 + m7, m2 + m4], axis=0))
            cols.append(jnp.concatenate([m3 + m5, m1 - m2 + m3 + m6], axis=0))
        to[...] = jnp.concatenate(cols + m[7], axis=1).reshape(16, 8, DM)
        for f in side:
            f()
        return carry

    def spectral(zero):
        def fence(z):
            return z[0, zero, 128:ZPITCH, :]

        def radix(g, bb, sign):
            z = zs[g]
            toks = []

            def emit(q, y):
                for p in range(4):
                    z[0, q + 4 * p, chunk(bb), :] = y[p][0]
                    z[1, q + 4 * p, chunk(bb), :] = y[p][1]
                toks.append(fence(z))
            _fft16([(z[0, a, chunk(bb), :], z[1, a, chunk(bb), :]) for a in range(16)], sign, emit)
            return toks

        ys = {}

        def fwd(g, k2, toks):
            z = zs[g]
            ur, ui = z[0, k2, 0:64, :], z[1, k2, 0:64, :]
            tr, ti = _twiddle((z[0, k2, 64:128, :], z[1, k2, 64:128, :]), k2, 32, -1)
            for hf in range(2):
                v = _ilv(ur + tr, ui + ti) if hf == 0 else _ilv(ur - tr, ui - ti)
                lhs = _with_tokens(emat[k2 + 16 * hf], toks if hf == 0 else None)
                xr, xi = _dilv(_dot(_bf(lhs), v.astype(bf16)))
                ys["x", 16 * g + k2] = xr
                wr = wf[g, pl.ds(k2 * WPITCH + hf, 64, stride=2), :]
                wi = wf[g + 3, pl.ds(k2 * WPITCH + hf, 64, stride=2), :]
                ys[g, k2, hf] = _ilv(xr * wr - xi * wi, xr * wi + xi * wr).astype(bf16)

        def inv(g, k2, toks):
            z = zs[g]
            t0 = _dot(_bf(_with_tokens(emat[32 + k2], toks)), ys.pop((g, k2, 0)))
            t1 = _dot(_bf(emat[48 + k2]), ys.pop((g, k2, 1)))
            z[0, k2, 0:64, :], z[1, k2, 0:64, :] = _dilv(t0 + t1)
            z[0, k2, 64:128, :], z[1, k2, 64:128, :] = _twiddle(_dilv(t0 - t1), k2, 32, 1)

        units = [(g, k2) for g in range(3) for k2 in range(16)]
        toks = None
        lag = CFG["inv_lag"]
        for i in range(len(units) + lag):
            if i < len(units):
                fwd(*units[i], toks)
            if i >= lag:
                inv(*units[i - lag], toks if i >= len(units) else None)
            toks = []
            if i in CFG["fwd_at"]:
                toks += radix(2, CFG["fwd_at"].index(i), -1)
            for n, at in enumerate(CFG["inv_at"]):
                if at == i:
                    if not toks:
                        back, r = CFG["rel"]
                        zs[n // 16][1, zero, 128:ZPITCH, :] = ys["x", min(i - back, 47)][8 * r:8 * r + 8]
                    toks += radix(n // 16, n % 16, 1)
            pos = CFG["tok_pos"] if len(toks) <= 4 else range(8)
            toks = {j: pltpu.bitcast(t, u32) for j, t in zip(pos, toks)}

    def dinv_thunks(bb, finish):
        st = {}

        def part(g):
            def run():
                z = zs[g]
                ys = [(z[0, a, chunk(bb), :], z[1, a, chunk(bb), :]) for a in range(16)]
                if g >= CFG["inv_groups"]:
                    ys = _fft16(ys, 1)
                tr = jnp.concatenate([y[0] for y in ys], axis=0)
                ti = jnp.concatenate([y[1] for y in ys], axis=0)
                if g == 0 and CFG["pack_i"]:
                    lane = lax.broadcasted_iota(jnp.int32, (128, 128), 1)
                    v = jnp.where(lane <= 64, tr, pltpu.roll(ti, 64, 1))
                    st[0] = _dot(v.astype(bf16), _bf(small[8]))
                elif g == 0:
                    st[0] = _dot(tr.astype(bf16), _bf(small[8])) + _dot(ti.astype(bf16), _bf(small[9]))
                else:
                    k, ki, kr = [_dot(v.astype(bf16), _bf(small[7 + 3 * g + i]))
                                 for i, v in enumerate((tr + _mu() * ti, ti, tr))]
                    st[2 * g - 1], st[2 * g] = k + ki, k + kr
            return run

        def fin():
            p0, p1, q1, p2, q2 = [st[j] for j in range(5)]
            t = p1 + p2
            m, n = p0 - 0.25 * t, R5_D * (p1 - p2)
            e1, e2 = m + n, m - n
            o1, o2 = q1 + R5_R * q2, R5_R * q1 - q2
            y = jnp.concatenate([p0 + t, e1 - o1, e2 - o2, e2 + o2, e1 + o1], axis=1)
            finish(xb[:, chunk(bb), :].reshape(128, DM) + y)
        return [part(0), part(1), part(2), fin]

    def out_copy(bb):
        return pltpu.make_async_copy(xin.at[:, bb], out_hbm.at[:, bb], osem.at[bb])

    def layer(li, carry0):
        if full or CFG["only"] == "group":
            _loop("step", 0, 16, group, mem_ref[...].astype(f32))
        if full or CFG["only"] == "spec":
            _loop("post", 0, 4, post, 0, unroll=CFG["post_unroll"])

            with jax.named_scope("spectral"):
                spectral((li >> 1))
        if not full and CFG["only"] != "out":
            return carry0

        def run_chunks(th, order, lag):
            seq = [t[g] for t in th for g in order]
            for i in range(len(seq) + lag):
                if i < len(seq):
                    seq[i]()
                if i >= lag and (i - lag) % 3 == 2:
                    th[(i - lag) // 3][3]()

        @pl.when(li == 0)
        def _():
            with jax.named_scope("dinv_tails"):
                run_chunks([dinv_thunks(4 * u + 3, functools.partial(
                    lambda u, x: set_input(4 * u + 3, _round_bf16(x), u, two=bool(CFG["two"])), u))
                    for u in range(4)],
                    *CFG["tails_order"])

            def batch(it, carry):
                bb = body_chunk(it)
                side = dinv_thunks(bb, lambda x: set_input(bb, _round_bf16(x), None))
                for k, f in enumerate(batch2_thunks(it) if CFG["two"] else batch_thunks(it)):
                    f()
                    for at, g in zip(CFG["dinv_at"], CFG["dinv_order"] + (3,)):
                        if at == k:
                            side[g]()
                return carry
            _loop("batch", 0, 12, batch, 0, unroll=CFG["batch_unroll"])

        @pl.when(li == 1)
        def _():
            with jax.named_scope("dinv_out"):
                def store_out(bb, x):
                    xin[:, bb] = x.reshape(16, 8, DM).astype(bf16)
                    out_copy(bb).start()
                run_chunks([dinv_thunks(bb, functools.partial(store_out, bb)) for bb in range(16)],
                           *CFG["out_order"])
                for bb in range(16):
                    out_copy(bb).wait()
        return carry0

    if CFG["only"] != "pro":
        lax.fori_loop(0, 2, layer, 0)
    if CFG["only"] in ("pro", "out"):
        zero = zero_ref[0]
        xin[0, 0, :, 0:128] = (qb[zero, 0, 0] + wf[zero, 0:8, :] + xa[zero, 0:8, 0:128]).astype(bf16) + ws[zero, 0, 0:8, :]
        out_copy(0).start()
        out_copy(0).wait()


@jax.jit
def pallas_interleave_layers__memory_aug_recurrent_mem_tr__spectral_gfnet__prompt_kernel(
    A_x, A_mem0, A_Wq, A_Wk, A_Wv, A_Wo, A_seg_len, B_x, B_w_r, B_w_i,
):
    assert A_x.shape == (1, S, DM) and A_mem0.shape == (1, MEM, DM)
    small, emat = _tables()
    hbm = pl.BlockSpec(memory_space=pltpu.HBM)
    out = pl.pallas_call(
        _kernel,
        out_shape=jax.ShapeDtypeStruct((16, 16, 8, DM), bf16),
        in_specs=[hbm] * 10,
        out_specs=hbm,
        scratch_shapes=[
            pltpu.VMEM((16, 16, 8, DM), bf16),
            pltpu.VMEM((33, 128, DM), f32),
            pltpu.VMEM((16, 128, DM), f32),
            pltpu.VMEM((16, 8, DM), f32),
            pltpu.VMEM((12, 2, 320, 8, DH), bf16),
            pltpu.VMEM((13, 8 * HPITCH, 128), u32),
            pltpu.VMEM((13, 8 * HPITCH, 128), u32),
            pltpu.VMEM((5, H * DH + 512, 128), bf16),
            pltpu.VMEM((19, 10, 128, 128), bf16),
            pltpu.VMEM((16, 4, 96, 8, 128), f32),
            pltpu.VMEM((2, 16, 64, 128), u32),
            pltpu.VMEM((53, 64, 128), u32),
            pltpu.VMEM((2, 16, ZPITCH, 128), f32),
            pltpu.VMEM((2, 16, ZPITCH, 128), f32),
            pltpu.VMEM((2, 16, ZPITCH, 128), f32),
            pltpu.VMEM((6, 16 * WPITCH + 32, 128), f32),
            pltpu.VMEM((9, DF, 512), bf16),
            pltpu.VMEM((4, 328, 128), f32),
            pltpu.VMEM((SMALL_TILES, 64, 128), u32),
            pltpu.VMEM((64, 64, 128), u32),
            pltpu.VMEM((80, 80), f32),
            pltpu.VMEM((MEM, DM), bf16),
            pltpu.SMEM((1,), jnp.int32),
            pltpu.SemaphoreType.DMA((47,)),
            pltpu.SemaphoreType.DMA((16,)),
        ],
        compiler_params=pltpu.CompilerParams(vmem_limit_bytes=120 * 1024 * 1024,
                                             disable_semaphore_checks=True),
    )(
        A_x.reshape(16, 16, 8, DM), A_mem0.reshape(MEM, DM),
        *[w.reshape(2, 320, H, DH) for w in (A_Wq, A_Wk, A_Wv)], A_Wo.reshape(H * DH, DM), B_w_r.T, B_w_i.T,
        jnp.asarray(small), jnp.asarray(emat),
    )
    return out.reshape(1, S, DM)
```

```python
import functools
import math

import jax
import jax.numpy as jnp
import numpy as np
from jax import lax
import jax.experimental.pallas as pl
import jax.experimental.pallas.tpu as pltpu

f32, bf16, u32 = jnp.float32, jnp.bfloat16, jnp.uint32

S, DM, H, DH, MEM, SEG = 2048, 640, 32, 128, 8, 32
NSEG = S // SEG
NPAIR = H // 2
DF = DM // 2 + 1
EPS = 1e-5
WPITCH = 132

HPITCH = 164
ZPITCH = 136

S1 = math.sin(2 * math.pi / 5)
R5_D = (math.cos(2 * math.pi / 5) - math.cos(4 * math.pi / 5)) / 2
R5_R = math.sin(4 * math.pi / 5) / S1


def _to_bf16_bits(a):
    u = np.ascontiguousarray(a, dtype=np.float32).view(np.uint32).astype(np.uint64)
    return ((u + 0x7FFF + ((u >> 16) & 1)) >> 16).astype(np.uint32)


def _pack_rows(a):
    b = _to_bf16_bits(a)
    return b[..., 0::2, :] | (b[..., 1::2, :] << 16)


@functools.lru_cache(maxsize=None)
def _tables():
    b = np.arange(128)
    l0 = np.arange(0, DF, 5)
    l1 = np.concatenate([np.arange(1, 320, 5), np.arange(4, 320, 5)])
    l2 = np.concatenate([np.arange(2, 320, 5), np.arange(3, 320, 5)])
    sg = np.concatenate([np.ones(64), -np.ones(64)])

    def th(l):
        return 2 * np.pi * ((b[:, None] * l[None, :]) % DM) / DM

    sc = 1.0 / (S * DM)
    fw = np.zeros((8, 128, 128))
    iw = np.zeros((8, 128, 128))
    t = th(l0)
    cl = np.full((65, 1), 2.0)
    cl[0] = cl[-1] = 1.0
    fw[0, :, :65], fw[1, :, :65] = np.cos(t), -np.sin(t)
    iw[0, :65], iw[1, :65] = cl * np.cos(t.T) * sc, -cl * np.sin(t.T) * sc
    if CFG["pack_f"]:
        fw[0, :, 65:] = fw[1, :, 1:64]
    if CFG["pack_i"]:
        iw[0, 65:] = iw[1, 1:64]
    mu = S1 * sg
    for g, l in ((1, l1), (2, l2)):
        t = th(l)
        c, s = np.cos(t), np.sin(t)
        fw[3 * g - 1:3 * g + 2] = c, -mu * s - c, mu * c - s
        iw[3 * g - 1:3 * g + 2] = [2 * sc * m.T for m in (c, -s - mu * c, mu * s - c)]
    n = np.arange(64)
    order = np.concatenate([np.concatenate([np.arange(8) + 8 * j, np.arange(8) + 8 * j + 64])
                            for j in range(8)])
    e = np.zeros((2, 32, 128, 128))
    for k2 in range(32):
        t = 2 * np.pi * (((32 * n[:, None] + k2) * n[None, :]) % S) / S
        er, ei = np.cos(t), -np.sin(t)
        m = np.block([[er, -ei], [ei, er]])[order][:, order]
        e[0, k2], e[1, k2] = m, m.T
    small = np.concatenate([_pack_rows(fw), _pack_rows(iw)], axis=0)
    return small, _pack_rows(e).reshape(64, 64, 128)


SMALL_TILES = 16


def _loop(name, lo, hi, body, init, **kw):
    with jax.named_scope(name):
        return lax.fori_loop(lo, hi, body, init, **kw)


def _bf(x):
    return pltpu.bitcast(x, bf16)


def _dot(a, b):
    return jnp.dot(a, b, preferred_element_type=f32)


def _round_bf16(x):
    return x.astype(bf16).astype(f32)


def _layernorm(x):
    m = jnp.mean(x, axis=-1, keepdims=True)
    xc = x - m
    v = jnp.mean(xc * xc, axis=-1, keepdims=True)
    return xc * lax.rsqrt(v + EPS)


def _fft4(x, sign):
    (ar, ai), (br, bi), (cr, ci), (dr, di) = x
    t0r, t0i, t1r, t1i = ar + cr, ai + ci, ar - cr, ai - ci
    t2r, t2i, t3r, t3i = br + dr, bi + di, br - dr, bi - di
    y0, y2 = (t0r + t2r, t0i + t2i), (t0r - t2r, t0i - t2i)
    p, q = (t1r + t3i, t1i - t3r), (t1r - t3i, t1i + t3r)
    return [y0, p, y2, q] if sign < 0 else [y0, q, y2, p]


def _twiddle(z, n, period, sign):
    zr, zi = z
    n = n % period
    if n == 0:
        return z
    if 4 * n == period:
        return (-zi, zr) if sign > 0 else (zi, -zr)
    c, s = math.cos(2 * math.pi * n / period), sign * math.sin(2 * math.pi * n / period)
    if (8 * n) % period == 0:
        a, d = zr + zi, zr - zi
        if c * s > 0:
            return (d * c, a * c)
        return (a * c, d * s)
    return (zr * c - zi * s, zr * s + zi * c)


def _bsum(x, y, sign):
    x, y = x.astype(f32), y.astype(f32)
    return (x + y if sign > 0 else x - y).astype(bf16)


def _strassen_lhs(a11, a12, a21, a22):
    return [lambda: a11() + a22(), lambda: a21() + a22(), a11, a22,
            lambda: a11() + a12(), lambda: a21() - a11(), lambda: a12() - a22()]


def _strassen_rhs(b11, b12, b21, b22):
    return [lambda: _bsum(b11(), b22(), 1), b11, lambda: _bsum(b12(), b22(), -1),
            lambda: _bsum(b21(), b11(), -1), b22, lambda: _bsum(b11(), b12(), 1),
            lambda: _bsum(b21(), b22(), 1)]


STRASSEN_OUT = [(((0, 0), 1), ((1, 1), 1)), (((1, 0), 1), ((1, 1), -1)), (((0, 1), 1), ((1, 1), 1)),
                (((0, 0), 1), ((1, 0), 1)), (((0, 0), -1), ((0, 1), 1)), (((1, 1), 1),), (((0, 0), 1),),
                (((0, 0), 1),), (((0, 1), 1),), (((1, 0), 1),), (((1, 1), 1),)]
WS_SLOT = {0: 0, 2: 1, 3: 2, 5: 3, 6: 4}


def _mu():
    lane = lax.broadcasted_iota(jnp.int32, (1, 128), 1)
    return jnp.where(lane < 64, S1, -S1).astype(f32)


def _ilv(r, i):
    n = r.shape[0] // 8
    return jnp.concatenate([r.reshape(n, 8, 128), i.reshape(n, 8, 128)], axis=1).reshape(16 * n, 128)


def _dilv(x):
    n = x.shape[0] // 16
    x = x.reshape(n, 16, 128)
    return x[:, :8].reshape(8 * n, 128), x[:, 8:].reshape(8 * n, 128)


def _with_tokens(x, toks):
    if not toks:
        return x
    return jnp.concatenate(
        [x[8 * j:8 * j + 8] | toks[j] if j in toks else x[8 * j:8 * j + 8]
         for j in range(x.shape[0] // 8)], axis=0)


def _fft16(x, sign, emit=None):
    cols = [_fft4([x[4 * j + r] for j in range(4)], sign) for r in range(4)]
    out = [None] * 16
    for q in range(4):
        y = _fft4([_twiddle(cols[r][q], r * q, 16, sign) for r in range(4)], sign)
        for p in range(4):
            out[q + 4 * p] = y[p]
        if emit is not None:
            emit(q, y)
    return out


CFG = dict(steps=((4.5, 16.5, 6, 4, 0, 8), (5, 16.5, 5, 7, 8, 12), (5, 16.5, 6, 6, 8, 12), (5, 16.5, 8, 7, 8, 0)),
           post_dl=20, post_passes=((0, 1), (2, 3), (4, 5), (6, 7)),
           post_order=(0, 1, 6, 3, 4, 2, 8, 5, 7, 9, 10, 11), post_at=(22, 26, 68, 96),
           tails_order=((1, 2, 0), 5), out_order=((1, 2, 0), 5), pack_f=True, pack_i=True,
           inv_at=tuple(range(28, 44)), inv_groups=1, inv_lag=4, tok_pos=(4, 5, 6, 7),
           fwd_at=(7, 8, 9, 10, 12, 13, 14, 16, 17, 18, 20, 21, 22, 24, 25, 26), rel=(0, 1), dinv_at=(0, 0, 1, 1), dinv_order=(2, 1, 0),

           two_inner=(5, 4, 2, 8, 0, 3, 6, 7, 10, 1, 9),
           two_outer=((2, 2), (5, 3), (1, None), (0, None), (4, 0), (3, None), (6, 1)),
           batch_unroll=2, post_unroll=1,
           ws_split=4, ws_at=(15, 15, 16, 16, 17, 18, 18, 19, 20, 20, 21, 21, 22, 23, 23, 24),
           pro_inner=(4, 2, 5, 8, 0, 3, 6, 7, 9, 10, 1),
           pro_outer=((2, 2), (5, 3), (1, 0), (0, None), (4, None), (3, None), (6, 1)),
           pro_nre=13, re_pos=(2, 2, 5, 5), ln_at=(11, 17, 23, 27), ln_at2=(4, 7, 10, 13),
           perm_at=tuple(range(10, 22)), only=None)


def _interleave(main, side):
    n, k = len(main), 0
    for i, f in enumerate(main):
        f()
        while k < len(side) and (k + 1) * n <= (i + 1) * len(side):
            side[k]()
            k += 1
    for f in side[k:]:
        f()


def _kernel(x_hbm, mem_hbm, wq_hbm, wk_hbm, wv_hbm, wo_hbm, wr_hbm, wi_hbm,
            small_hbm, e_hbm, out_hbm,
            xin, xa, xb, to, raw, wa, wb, wo_t, ws, qb, hl, z0, z1, z2, wf,
            wri, wtmp, small, emat, fill_ref, mem_ref, zero_ref, sem, osem):
    zs = (z0, z1, z2)
    w_hbm = (wq_hbm, wk_hbm, wv_hbm)

    def body_chunk(i):
        return 4 * (i & 3) + (i >> 2)

    def cp_w(i):
        src = w_hbm[i >> 2].at[:, :, pl.ds(8 * (i & 3), 8), :] if isinstance(i, int) else raw.at[i]
        return pltpu.make_async_copy(src, raw.at[i], sem.at[i])

    def cp_x(bb):
        return pltpu.make_async_copy(x_hbm.at[:, bb], xin.at[:, bb], sem.at[12 + bb])

    def cp_f(i):
        src = ((wr_hbm, wi_hbm)[i >> 2].at[:, pl.ds(512 * (i & 3), 512)]
               if isinstance(i, int) else wri.at[i])
        return pltpu.make_async_copy(src, wri.at[i], sem.at[36 + i])

    def cp_wo(i):
        rows = pl.ds(pl.multiple_of(512 * i, 512), 512)
        return [pltpu.make_async_copy(wo_hbm.at[rows, pl.ds(128 * j, 128)], wo_t.at[j, rows], sem.at[28 + i])
                for j in range(5)]

    cp_rest = [pltpu.make_async_copy(mem_hbm, mem_ref, sem.at[46]),
                pltpu.make_async_copy(small_hbm, small, sem.at[44]),
               pltpu.make_async_copy(e_hbm, emat, sem.at[45])]

    full = CFG["only"] in (None, "pro")
    for u in range(4 if full else 0):
        cp_x(4 * u + 3).start()
    if full:
        cp_w(0).start()
    for i in range(12 if full else 0):
        if i < 11:
            cp_w(i + 1).start()
        cp_x(body_chunk(i)).start()
        if 3 <= i < 11:
            cp_f(i - 3).start()
            for cp in cp_wo(i - 3):
                cp.start()
    for cp in cp_rest if full else ():
        cp.start()

    zero_ref[0] = 0

    r = lax.broadcasted_iota(jnp.int32, (80, 80), 0)
    c = lax.broadcasted_iota(jnp.int32, (80, 80), 1)

    def head(i):
        return jnp.where(i < 64, i // 32, (i - 64) // 8)

    def pos(i):
        return jnp.where(i < 64, i % 32, 32 + (i - 64) % 8)

    ok = (pos(r) < MEM) | (pos(r) >= pos(c))
    fill_ref[...] = jnp.where(head(r) == head(c), jnp.where(ok, 0.0, -1e9), -jnp.inf).astype(f32)
    wtmp[:, 320:328, :] = jnp.zeros((4, 8, 128), f32)
    xa[32, 0:8, 0:128] = jnp.zeros((8, 128), f32)
    ws[18, 0, 0:16, :] = jnp.zeros((16, 128), bf16)
    wa[12, 0:8, :] = jnp.zeros((8, 128), u32)
    wb[12, 0:8, :] = jnp.zeros((8, 128), u32)
    wf[5, 16 * WPITCH:16 * WPITCH + 8, :] = jnp.zeros((8, 128), f32)
    for z in zs:
        z[0, 0, 128:ZPITCH, :] = jnp.zeros((8, 128), f32)

    def chunk(bb):
        if isinstance(bb, int):
            return slice(8 * bb, 8 * bb + 8)
        return pl.ds(pl.multiple_of(8 * bb, 8), 8)

    def set_input(bb, x, tail_u, a0=0):
        n = x.shape[0] // 8
        xa[a0:a0 + n, chunk(bb), :] = x.reshape(n, 8, DM)
        y = _layernorm(x)
        if tail_u is None:
            xa[16 + a0:16 + a0 + n, chunk(bb), :] = y.reshape(n, 8, DM)
        else:
            blk = [[y[32 * r:32 * r + 32, 128 * kt:128 * kt + 128] for kt in range(5)] for r in range(4)]
            lv1 = [_strassen_lhs(*[functools.partial(lambda v: v, blk[2 * rr + r][2 * kk + k])
                                   for rr in range(2) for kk in range(2)])
                   for r in range(2) for k in range(2)]
            ops = []
            for i in range(7):
                sub = [f[i]() for f in lv1]
                ops += [f() for f in _strassen_lhs(*[functools.partial(lambda v: v, v) for v in sub])]
            for i, v in enumerate(ops + [blk[r][4] for r in range(4)]):
                hl[i, 16 * tail_u:16 * tail_u + 16, :] = pltpu.bitcast(v.astype(bf16), u32)

    def load_x(bb, a0=0, n=16):
        return xin[a0:a0 + n, bb].astype(f32).reshape(8 * n, DM)

    def wtile(cid, j, e):
        w = (wa, wb)[e]
        return jnp.concatenate([w[cid, (4 * hf + j) * HPITCH:(4 * hf + j) * HPITCH + 160, :]
                                for hf in range(2)], axis=0)

    def relayout(i, cid, e):
        for r in range(4 * i, 4 * i + 4):
            a, b = [pltpu.bitcast(raw[cid, :, d].reshape(16, 128), u32) for d in (2 * r, 2 * r + 1)]
            v = (a & 0xFFFF) | (b << 16) if e == 0 else (a >> 16) | (b & jnp.uint32(0xFFFF0000))
            (wa, wb)[e][cid, pl.ds(r, 8, stride=HPITCH), :] = v

    def batch_thunks(cid, inner, outer_order):
        qv = qb.at[:, :, pl.ds(8 * cid, 8)]
        RH = [((0, 0, 1), (1, 1, 1)), ((0, 0, 1),), ((0, 1, 1), (1, 1, -1)), ((1, 0, 1), (0, 0, -1)),
              ((1, 1, 1),), ((0, 0, 1), (0, 1, 1)), ((1, 0, 1), (1, 1, 1))]

        def unit(e):
            c = {}
            left = {(r, n): (5, 3, 3, 5)[2 * (r >> 1) + (n >> 1)] for r in range(4) for n in range(4)}

            def w(n, kt):
                return _bf(wtile(cid, n, e)[64 * kt:64 * kt + 64])

            def acc(blk, y, sign):
                if blk not in c:
                    c[blk] = y if sign > 0 else -y
                else:
                    c[blk] = c[blk] + y if sign > 0 else c[blk] - y
                left[blk] -= 1
                if left[blk] == 0:
                    r, n = blk
                    y = c.pop(blk).reshape(4, 4, 8, 128)
                    for u in range(4):
                        qv[4 * r:4 * r + 4, u, 2 * n + e] = y[u]

            def outer(I, k4):
                st = {}

                def lvl1(k, n):
                    if (k, n) not in st:
                        t = [(w(2 * nn + n, 2 * kk + k), sg) for kk, nn, sg in RH[I]]
                        if len(t) == 1:
                            st[k, n] = t[0][0]
                        else:
                            x, y = t[0][0].astype(f32), t[1][0].astype(f32)
                            st[k, n] = x + y if t[1][1] > 0 else x - y
                    return st[k, n]
                p = {}
                pl_ = {(0, 0): 4, (0, 1): 2, (1, 0): 2, (1, 1): 4}

                def half(items):
                    def run(toks=None):
                        for i in items:
                            if i >= 7:
                                r, n = k4[i - 7]
                                acc((r, n), _dot(_bf(_with_tokens(hl[49 + r], toks)), w(n, 4)), 1)
                                toks = None
                                continue
                            t = [(lvl1(k, n), sg) for k, n, sg in RH[i]]
                            rhs = t[0][0].astype(bf16) if len(t) == 1 else _bsum(t[0][0], t[1][0], t[1][1])
                            y = _dot(_bf(_with_tokens(hl[7 * I + i], toks)), rhs)
                            toks = None
                            for blk, sign in STRASSEN_OUT[i]:
                                if blk not in p:
                                    p[blk] = y if sign > 0 else -y
                                else:
                                    p[blk] = p[blk] + y if sign > 0 else p[blk] - y
                                pl_[blk] -= 1
                                if pl_[blk] == 0:
                                    for (R, N), sg in STRASSEN_OUT[I]:
                                        acc((2 * R + blk[0], 2 * N + blk[1]), p[blk], sg)
                    return run
                items = [i for i in inner if i < 7 + len(k4)]
                return [half(items[:len(items) // 2]), half(items[len(items) // 2:])]
            out = []
            for I, q in outer_order:
                k4 = [] if q is None else [(2 * (q >> 1) + (j >> 1), 2 * (q & 1) + (j & 1)) for j in range(4)]
                out += outer(I, k4)
            return out
        return unit(0) + unit(1)

    def wperm_thunks(piece, j):
        m = (piece >> 2) & 1
        wt = wtmp.at[j]

        def load():
            wt[0:DF, :] = wri[piece, :, 128 * j:128 * j + 128].astype(f32)

        def one(g):
            def run():
                if g == 0:
                    t = jnp.concatenate([wt[pl.ds(0, 64, stride=5), :], wt[320:328, :],
                                         jnp.zeros((56, 128), f32)], axis=0)
                else:
                    t = jnp.concatenate([wt[pl.ds(g, 64, stride=5), :],
                                         wt[pl.ds(5 - g, 64, stride=5), :]], axis=0)
                y = t.T
                sub = wf.at[3 * m + g, pl.ds(pl.multiple_of((piece & 3) * 32, 32), 16 * WPITCH - 96)]
                for k in range(8):
                    for hf in range(2):
                        sub[pl.ds(8 * j + k + 8 * hf * WPITCH, 8, stride=WPITCH), :] = (
                            y[16 * k + 8 * hf:16 * k + 8 * hf + 8])
            return run
        return [load] + [one(g) for g in range(3)]

    def half_pass(cid, half, fill, zero, timed=()):
        nre = CFG["pro_nre"]
        toks = None
        for k, f in enumerate(batch_thunks(cid, CFG["pro_inner"], CFG["pro_outer"])[14 * half:14 * half + 14]):
            f(toks)
            toks = {}
            for n, f in enumerate(f for at, f in timed if at == k):
                toks[(0, 4, 1, 6)[n]] = f()
            if fill is not None:
                for n, r in enumerate(r for r in range(40) if r * nre // 40 == k):
                    relayout(r, fill, 1 - half)
                    toks[CFG["re_pos"][n]] = (wb, wa)[half][12 + zero, 0:8, :]

    def ln_parts(bb, zero):
        def part(j):
            set_input(bb, load_x(bb, 4 * j, 4), None, 4 * j)
            return pltpu.bitcast(xa[32 + zero, 0:8, 0:128], u32)
        return [functools.partial(part, j) for j in range(4)]

    def perm_parts(piece, zero):
        def part(fs):
            for f in fs:
                f()
            return pltpu.bitcast(wf[5 + zero, 16 * WPITCH:16 * WPITCH + 8, :], u32)
        out = []
        for j in range(4):
            th = wperm_thunks(piece, j)
            out += [functools.partial(part, th[0:2]), functools.partial(part, th[2:3]),
                    functools.partial(part, th[3:4])]
        return out

    def ws_parts(piece, zero):
        nr = 128 // CFG["ws_split"]

        src = wo_t.at[:, pl.ds(pl.multiple_of(512 * piece, 512), 512)]
        dst = ws.at[pl.ds(2 * piece, 2)]

        def part(pp, np_, r0):
            def tile(k, n):
                lo = 256 * pp + 128 * k + r0
                return src[2 * np_ + n, lo:lo + nr, :]
            rhs = _strassen_rhs(*[functools.partial(tile, k, n) for k in range(2) for n in range(2)])
            for i, slot in WS_SLOT.items():
                dst[pp, 5 * np_ + slot, r0:r0 + nr, :] = rhs[i]()
            return pltpu.bitcast(ws[18 + zero, 0, 0:16, :], u32)
        return [functools.partial(part, pp, np_, r0)
                for pp in range(2) for np_ in range(2) for r0 in range(0, 128, nr)]

    def pro0():
        for u in range(4):
            cp_x(4 * u + 3).wait()
        for u in range(4):
            set_input(4 * u + 3, load_x(4 * u + 3), u)
        cp_w(0).wait()
        zero = zero_ref[0]
        for i in range(40):
            relayout(i, 0, 0)
        half_pass(0, 0, zero, zero)

    def pro1(it, carry):
        bb = body_chunk(it)
        with jax.named_scope("pro1_wait"):
            cp_w(it + 1).wait()

            @pl.when(it >= 3)
            def _():
                cp_f(it - 3).wait()
                for cp in cp_wo(it - 3):
                    cp.wait()
            cp_x(bb).wait()
        piece = jnp.where(it >= 3, it - 3, 8)
        zero = it >> 4
        timed = sorted(list(zip(CFG["ln_at"], ln_parts(bb, zero)))
                       + list(zip(CFG["ws_at"], ws_parts(piece, zero)))
                       + list(zip(CFG["perm_at"], perm_parts(piece, zero))), key=lambda x: x[0])
        half_pass(it, 1, it + 1, zero, [x for x in timed if x[0] < 14])
        half_pass(it + 1, 0, it + 1, zero, [(k - 14, f) for k, f in timed if k >= 14])
        return carry

    def pro2():
        cp_x(body_chunk(11)).wait()
        cp_rest[0].wait()
        zero = zero_ref[0]
        half_pass(11, 1, None, zero, list(zip(CFG["ln_at2"], ln_parts(body_chunk(11), zero))))

    if full:
        with jax.named_scope("pro0"):
            pro0()
        _loop("pro1", 0, 11, pro1, 0)
        with jax.named_scope("pro2"):
            pro2()

    scale = DH ** -0.5

    def wo_dot(hh, oo):
        return [_dot(oo, wo_t[j, 128 * hh:128 * hh + 128, :]) for j in range(5)]

    def addl(acc, res):
        return res if acc is None else [a + b for a, b in zip(acc, res)]

    def group(g, mem):
        for ph in range(4):
            h = jnp.concatenate([mem, xa[16 + g, 32 * ph:32 * ph + 24, :]], axis=0).astype(bf16)
            pr, sm, oos = {}, {}, {}
            lat_s, lat_pv, lat_wo, v_delay, n_first, n_last = CFG["steps"][ph]

            def stacked(p, m):
                tails = [qb[g, ph, 32 * m + 2 * p + e] for e in range(2)]
                return jnp.concatenate([pr[p, m, 0], pr[p, m, 1]] + tails, axis=0).astype(bf16)

            def scores(p):
                sc = lax.dot_general(stacked(p, 0), stacked(p, 1), (((1,), (1,)), ((), ())),
                                     preferred_element_type=f32)
                fill = fill_ref[...]
                sc = jnp.where(fill == 0.0, sc * scale, fill)
                mx = jnp.max(sc, axis=-1, keepdims=True)
                e = jnp.exp(sc - mx)
                rl = pl.reciprocal(jnp.sum(e, axis=-1, keepdims=True), approx=True)
                sm[p] = (e * rl).astype(bf16)

            def pv(p):
                o = _dot(sm[p], stacked(p, 2))
                for e in range(2):
                    qb[g, ph, 2 * p + e] = o[64 + 8 * e:72 + 8 * e]
                    oos[2 * p + e] = o[32 * e:32 * e + 32].astype(bf16)

            keyed = []
            for p in range(NPAIR):
                keyed += [(4 * p + 2 * m + e, (p, m, e)) for m in range(2) for e in range(2)]
                keyed += [(4 * p + 3.5 + v_delay, (p, 2, e)) for e in range(2)]
            bulk = [x for _, x in sorted(keyed, key=lambda kv: kv[0])]
            acc, t, nwo, pend, ready = None, 0.0, 0, [], []
            if n_first:
                first, bulk = bulk[:n_first], bulk[n_first:]
                for kt in range(5):
                    for p, m, e in first:
                        w = wtile(4 * m + (p >> 2), p & 3, e)[64 * kt:64 * kt + 64]
                        y = _dot(h[:, 128 * kt:128 * kt + 128], _bf(w))
                        pr[p, m, e] = y if kt == 0 else pr[p, m, e] + y
                t = float(len(first))
                pend = [(t + lat_s, "S", p) for p, m, e in first if m == 1 and e == 1]
            while nwo < H - n_last or pend:
                pend.sort()
                if pend and pend[0][0] <= t:
                    _, kind, p = pend.pop(0)
                    if kind == "S":
                        scores(p)
                        pend.append((t + lat_pv, "V", p))
                    else:
                        pv(p)
                        ready += [(t + lat_wo, 2 * p + e) for e in range(2)]
                    t += 0.5
                elif bulk:
                    p, m, e = bulk.pop(0)
                    pr[p, m, e] = _dot(h, _bf(wtile(4 * m + (p >> 2), p & 3, e)))
                    t += 1
                    if m == 1 and e == 1:
                        pend.append((t + lat_s, "S", p))
                elif ready and ready[0][0] <= t and nwo < H - n_last:
                    _, hh = ready.pop(0)
                    acc = addl(acc, wo_dot(hh, oos[hh]))
                    t += 1
                    nwo += 1
                else:
                    t += 0.5
            for j in range(5):
                for _, hh in ready:
                    acc[j] = acc[j] + _dot(oos[hh], wo_t[j, 128 * hh:128 * hh + 128, :])
            out = jnp.concatenate(acc, axis=1)
            xa[16 + g, 32 * ph:32 * ph + 24, :] = out[8:32]
            mem = _round_bf16(out[0:8])
        return mem

    def dfwd_thunks(seg, q):
        st = {}
        rows = chunk(q)
        xav, xbv, zv = xa.at[:, seg], xb.at[:, seg], [z.at[:, :, seg] for z in zs]

        def pre():
            o = to[...] if q == 3 else xav[16:32, rows, :]
            x = _round_bf16(xav[0:16, rows, :] + o)
            xbv[:, rows, :] = x
            y = _layernorm(x.reshape(128, DM))
            x0, x1, x2, x3, x4 = [y[:, 128 * a:128 * a + 128] for a in range(5)]
            t1, t2, t3, t4 = x1 + x4, x2 + x3, x1 - x4, x2 - x3
            t = t1 + t2
            m, n = x0 - 0.25 * t, R5_D * (t1 - t2)
            st["u"] = [x0 + t, (m + n, t3 + R5_R * t4), (m - n, R5_R * t3 - t4)]

        def part(g):
            def run():
                if g == 0:
                    pre()
                    u0 = st["u"][0].astype(bf16)
                    zr = _dot(u0, _bf(small[0]))
                    if CFG["pack_f"]:
                        lane = lax.broadcasted_iota(jnp.int32, (128, 128), 1)
                        zi = jnp.where((lane & 63) == 0, 0.0, pltpu.roll(zr, 64, 1))
                    else:
                        zi = _dot(u0, _bf(small[1]))
                else:
                    a, b = st["u"][g]
                    k, kb, ka = [_dot(v.astype(bf16), _bf(small[3 * g - 1 + i]))
                                 for i, v in enumerate((a + b, b, a))]
                    zr, zi = k + kb, ka - _mu() * k
                ys = [(zr[8 * a:8 * a + 8], zi[8 * a:8 * a + 8]) for a in range(16)]
                if g < 2:
                    ys = _fft16(ys, -1)
                for a in range(16):
                    zv[g][0, a, rows, :] = ys[a][0]
                    zv[g][1, a, rows, :] = ys[a][1]
            return run
        return [part(g) for g in range(3)]

    def post(u, carry):
        base = pl.multiple_of(32 * u, 32)
        side = []
        for q in range(4):
            side += dfwd_thunks(pl.ds(base, 32), q)
        side = [side[i] for i in CFG["post_order"]]
        k = 0
        at = list(CFG["post_at"])
        m, due = {}, []
        for prods in CFG["post_passes"]:
            acc = None
            for p in range(NPAIR):
                lhs = _strassen_lhs(*[
                    functools.partial(lambda r, e: qb[8 * r:8 * r + 8, u, 2 * p + e].reshape(64, 128), r, e)
                    for r in range(2) for e in range(2)])
                res = []
                for i in prods:
                    if i == 7:
                        oo = jnp.concatenate([qb[:, u, 2 * p + e].reshape(128, 128) for e in range(2)], axis=1)
                        res.append(_dot(oo.astype(bf16), wo_t[4, 256 * p:256 * p + 256, :]))
                        k += 2
                        continue
                    a = lhs[i]().astype(bf16)
                    for np_ in range(2):
                        if i in WS_SLOT:
                            w = ws[p, 5 * np_ + WS_SLOT[i]]
                        else:
                            kk = 0 if i == 1 else 1
                            w = wo_t[2 * np_ + kk, 256 * p + 128 * kk:256 * p + 128 * kk + 128, :]
                        if due and due[0][0] <= k:
                            w = _bf(_with_tokens(pltpu.bitcast(w, u32), {0: due.pop(0)[1]}))
                        res.append(_dot(a, w))
                    k += 1
                acc = addl(acc, res)
                while at and at[0] <= k:
                    g = CFG["post_order"][len(CFG["post_at"]) - len(at)] % 3
                    at.pop(0)
                    side.pop(0)()
                    if g == 0 and CFG["post_dl"]:
                        due.append((k + CFG["post_dl"],
                                    pltpu.bitcast(z0[0, u >> 2, 128:ZPITCH, :], u32)))
            for i in prods:
                m[i] = [acc.pop(0)] if i == 7 else [acc.pop(0), acc.pop(0)]
        cols = []
        for np_ in range(2):
            m1, m2, m3, m4, m5, m6, m7 = [m[i][np_] for i in range(7)]
            cols.append(jnp.concatenate([m1 + m4 - m5 + m7, m2 + m4], axis=0))
            cols.append(jnp.concatenate([m3 + m5, m1 - m2 + m3 + m6], axis=0))
        to[...] = jnp.concatenate(cols + m[7], axis=1).reshape(16, 8, DM)
        for f in side:
            f()
        return carry

    def spectral(zero):
        def fence(z):
            return z[0, zero, 128:ZPITCH, :]

        def radix(g, bb, sign):
            z = zs[g]
            toks = []

            def emit(q, y):
                for p in range(4):
                    z[0, q + 4 * p, chunk(bb), :] = y[p][0]
                    z[1, q + 4 * p, chunk(bb), :] = y[p][1]
                toks.append(fence(z))
            _fft16([(z[0, a, chunk(bb), :], z[1, a, chunk(bb), :]) for a in range(16)], sign, emit)
            return toks

        ys = {}

        def fwd(g, k2, toks):
            z = zs[g]
            ur, ui = z[0, k2, 0:64, :], z[1, k2, 0:64, :]
            tr, ti = _twiddle((z[0, k2, 64:128, :], z[1, k2, 64:128, :]), k2, 32, -1)
            for hf in range(2):
                v = _ilv(ur + tr, ui + ti) if hf == 0 else _ilv(ur - tr, ui - ti)
                lhs = _with_tokens(emat[k2 + 16 * hf], toks if hf == 0 else None)
                xr, xi = _dilv(_dot(_bf(lhs), v.astype(bf16)))
                ys["x", 16 * g + k2] = xr
                wr = wf[g, pl.ds(k2 * WPITCH + hf, 64, stride=2), :]
                wi = wf[g + 3, pl.ds(k2 * WPITCH + hf, 64, stride=2), :]
                ys[g, k2, hf] = _ilv(xr * wr - xi * wi, xr * wi + xi * wr).astype(bf16)

        def inv(g, k2, toks):
            z = zs[g]
            t0 = _dot(_bf(_with_tokens(emat[32 + k2], toks)), ys.pop((g, k2, 0)))
            t1 = _dot(_bf(emat[48 + k2]), ys.pop((g, k2, 1)))
            z[0, k2, 0:64, :], z[1, k2, 0:64, :] = _dilv(t0 + t1)
            z[0, k2, 64:128, :], z[1, k2, 64:128, :] = _twiddle(_dilv(t0 - t1), k2, 32, 1)

        units = [(g, k2) for g in range(3) for k2 in range(16)]
        toks = None
        lag = CFG["inv_lag"]
        for i in range(len(units) + lag):
            if i < len(units):
                fwd(*units[i], toks)
            if i >= lag:
                inv(*units[i - lag], toks if i >= len(units) else None)
            toks = []
            if i in CFG["fwd_at"]:
                toks += radix(2, CFG["fwd_at"].index(i), -1)
            for n, at in enumerate(CFG["inv_at"]):
                if at == i:
                    if not toks:
                        back, r = CFG["rel"]
                        zs[n // 16][1, zero, 128:ZPITCH, :] = ys["x", min(i - back, 47)][8 * r:8 * r + 8]
                    toks += radix(n // 16, n % 16, 1)
            pos = CFG["tok_pos"] if len(toks) <= 4 else range(8)
            toks = {j: pltpu.bitcast(t, u32) for j, t in zip(pos, toks)}

    def dinv_thunks(bb, finish):
        st = {}

        def part(g):
            def run():
                z = zs[g]
                ys = [(z[0, a, chunk(bb), :], z[1, a, chunk(bb), :]) for a in range(16)]
                if g >= CFG["inv_groups"]:
                    ys = _fft16(ys, 1)
                tr = jnp.concatenate([y[0] for y in ys], axis=0)
                ti = jnp.concatenate([y[1] for y in ys], axis=0)
                if g == 0 and CFG["pack_i"]:
                    lane = lax.broadcasted_iota(jnp.int32, (128, 128), 1)
                    v = jnp.where(lane <= 64, tr, pltpu.roll(ti, 64, 1))
                    st[0] = _dot(v.astype(bf16), _bf(small[8]))
                elif g == 0:
                    st[0] = _dot(tr.astype(bf16), _bf(small[8])) + _dot(ti.astype(bf16), _bf(small[9]))
                else:
                    k, ki, kr = [_dot(v.astype(bf16), _bf(small[7 + 3 * g + i]))
                                 for i, v in enumerate((tr + _mu() * ti, ti, tr))]
                    st[2 * g - 1], st[2 * g] = k + ki, k + kr
            return run

        def fin():
            p0, p1, q1, p2, q2 = [st[j] for j in range(5)]
            t = p1 + p2
            m, n = p0 - 0.25 * t, R5_D * (p1 - p2)
            e1, e2 = m + n, m - n
            o1, o2 = q1 + R5_R * q2, R5_R * q1 - q2
            y = jnp.concatenate([p0 + t, e1 - o1, e2 - o2, e2 + o2, e1 + o1], axis=1)
            finish(xb[:, chunk(bb), :].reshape(128, DM) + y)
        return [part(0), part(1), part(2), fin]

    def out_copy(bb):
        return pltpu.make_async_copy(xin.at[:, bb], out_hbm.at[:, bb], osem.at[bb])

    def layer(li, carry0):
        if full or CFG["only"] == "group":
            _loop("step", 0, 16, group, mem_ref[...].astype(f32))
        if full or CFG["only"] == "spec":
            if full:
                @pl.when(li == 0)
                def _():
                    for cp in cp_rest[1:]:
                        cp.wait()
            _loop("post", 0, 4, post, 0, unroll=CFG["post_unroll"])

            with jax.named_scope("spectral"):
                spectral((li >> 1))
        if not full and CFG["only"] != "out":
            return carry0

        def run_chunks(th, order, lag):
            seq = [t[g] for t in th for g in order]
            for i in range(len(seq) + lag):
                if i < len(seq):
                    seq[i]()
                if i >= lag and (i - lag) % 3 == 2:
                    th[(i - lag) // 3][3]()

        @pl.when(li == 0)
        def _():
            with jax.named_scope("dinv_tails"):
                run_chunks([dinv_thunks(4 * u + 3, functools.partial(
                    lambda u, x: set_input(4 * u + 3, _round_bf16(x), u), u))
                    for u in range(4)],
                    *CFG["tails_order"])

            def batch(it, carry):
                bb = body_chunk(it)
                side = dinv_thunks(bb, lambda x: set_input(bb, _round_bf16(x), None))
                for k, f in enumerate(batch_thunks(it, CFG["two_inner"], CFG["two_outer"])):
                    f()
                    for at, g in zip(CFG["dinv_at"], CFG["dinv_order"] + (3,)):
                        if at == k:
                            side[g]()
                return carry
            _loop("batch", 0, 12, batch, 0, unroll=CFG["batch_unroll"])

        @pl.when(li == 1)
        def _():
            with jax.named_scope("dinv_out"):
                def store_out(bb, x):
                    xin[:, bb] = x.reshape(16, 8, DM).astype(bf16)
                    out_copy(bb).start()
                run_chunks([dinv_thunks(bb, functools.partial(store_out, bb)) for bb in range(16)],
                           *CFG["out_order"])
                for bb in range(16):
                    out_copy(bb).wait()
        return carry0

    if CFG["only"] != "pro":
        lax.fori_loop(0, 2, layer, 0)
    if CFG["only"] in ("pro", "out"):
        zero = zero_ref[0]
        xin[0, 0, :, 0:128] = (qb[zero, 0, 0] + wf[zero, 0:8, :] + xa[zero, 0:8, 0:128]).astype(bf16) + ws[zero, 0, 0:8, :]
        out_copy(0).start()
        out_copy(0).wait()
        for cp in cp_rest[1:] if full else ():
            cp.wait()


@jax.jit
def pallas_interleave_layers__memory_aug_recurrent_mem_tr__spectral_gfnet__prompt_kernel(
    A_x, A_mem0, A_Wq, A_Wk, A_Wv, A_Wo, A_seg_len, B_x, B_w_r, B_w_i,
):
    assert A_x.shape == (1, S, DM) and A_mem0.shape == (1, MEM, DM)
    small, emat = _tables()
    hbm = pl.BlockSpec(memory_space=pltpu.HBM)
    out = pl.pallas_call(
        _kernel,
        out_shape=jax.ShapeDtypeStruct((16, 16, 8, DM), bf16),
        in_specs=[hbm] * 10,
        out_specs=hbm,
        scratch_shapes=[
            pltpu.VMEM((16, 16, 8, DM), bf16),
            pltpu.VMEM((33, 128, DM), f32),
            pltpu.VMEM((16, 128, DM), f32),
            pltpu.VMEM((16, 8, DM), f32),
            pltpu.VMEM((12, 2, 320, 8, DH), bf16),
            pltpu.VMEM((13, 8 * HPITCH, 128), u32),
            pltpu.VMEM((13, 8 * HPITCH, 128), u32),
            pltpu.VMEM((5, H * DH + 512, 128), bf16),
            pltpu.VMEM((19, 10, 128, 128), bf16),
            pltpu.VMEM((16, 4, 96, 8, 128), f32),
            pltpu.VMEM((53, 64, 128), u32),
            pltpu.VMEM((2, 16, ZPITCH, 128), f32),
            pltpu.VMEM((2, 16, ZPITCH, 128), f32),
            pltpu.VMEM((2, 16, ZPITCH, 128), f32),
            pltpu.VMEM((6, 16 * WPITCH + 32, 128), f32),
            pltpu.VMEM((9, DF, 512), bf16),
            pltpu.VMEM((4, 328, 128), f32),
            pltpu.VMEM((SMALL_TILES, 64, 128), u32),
            pltpu.VMEM((64, 64, 128), u32),
            pltpu.VMEM((80, 80), f32),
            pltpu.VMEM((MEM, DM), bf16),
            pltpu.SMEM((1,), jnp.int32),
            pltpu.SemaphoreType.DMA((47,)),
            pltpu.SemaphoreType.DMA((16,)),
        ],
        compiler_params=pltpu.CompilerParams(vmem_limit_bytes=120 * 1024 * 1024,
                                             disable_semaphore_checks=True),
    )(
        A_x.reshape(16, 16, 8, DM), A_mem0.reshape(MEM, DM),
        *[w.reshape(2, 320, H, DH) for w in (A_Wq, A_Wk, A_Wv)], A_Wo.reshape(H * DH, DM), B_w_r.T, B_w_i.T,
        jnp.asarray(small), jnp.asarray(emat),
    )
    return out.reshape(1, S, DM)
```

```python
import functools
import math

import jax
import jax.numpy as jnp
import numpy as np
from jax import lax
import jax.experimental.pallas as pl
import jax.experimental.pallas.tpu as pltpu

f32, bf16, u32 = jnp.float32, jnp.bfloat16, jnp.uint32

S, DM, H, DH, MEM, SEG = 2048, 640, 32, 128, 8, 32
NSEG = S // SEG
NPAIR = H // 2
DF = DM // 2 + 1
EPS = 1e-5
WPITCH = 132

HPITCH = 164
ZPITCH = 136

S1 = math.sin(2 * math.pi / 5)
R5_D = (math.cos(2 * math.pi / 5) - math.cos(4 * math.pi / 5)) / 2
R5_R = math.sin(4 * math.pi / 5) / S1


def _to_bf16_bits(a):
    u = np.ascontiguousarray(a, dtype=np.float32).view(np.uint32).astype(np.uint64)
    return ((u + 0x7FFF + ((u >> 16) & 1)) >> 16).astype(np.uint32)


def _pack_rows(a):
    b = _to_bf16_bits(a)
    return b[..., 0::2, :] | (b[..., 1::2, :] << 16)


@functools.lru_cache(maxsize=None)
def _tables():
    b = np.arange(128)
    l0 = np.arange(0, DF, 5)
    l1 = np.concatenate([np.arange(1, 320, 5), np.arange(4, 320, 5)])
    l2 = np.concatenate([np.arange(2, 320, 5), np.arange(3, 320, 5)])
    sg = np.concatenate([np.ones(64), -np.ones(64)])

    def th(l):
        return 2 * np.pi * ((b[:, None] * l[None, :]) % DM) / DM

    sc = 1.0 / (S * DM)
    fw = np.zeros((8, 128, 128))
    iw = np.zeros((8, 128, 128))
    t = th(l0)
    cl = np.full((65, 1), 2.0)
    cl[0] = cl[-1] = 1.0
    fw[0, :, :65], fw[1, :, :65] = np.cos(t), -np.sin(t)
    iw[0, :65], iw[1, :65] = cl * np.cos(t.T) * sc, -cl * np.sin(t.T) * sc
    if CFG["pack_f"]:
        fw[0, :, 65:] = fw[1, :, 1:64]
    if CFG["pack_i"]:
        iw[0, 65:] = iw[1, 1:64]
    mu = S1 * sg
    for g, l in ((1, l1), (2, l2)):
        t = th(l)
        c, s = np.cos(t), np.sin(t)
        fw[3 * g - 1:3 * g + 2] = c, -mu * s - c, mu * c - s
        iw[3 * g - 1:3 * g + 2] = [2 * sc * m.T for m in (c, -s - mu * c, mu * s - c)]
    n = np.arange(64)
    order = np.concatenate([np.concatenate([np.arange(8) + 8 * j, np.arange(8) + 8 * j + 64])
                            for j in range(8)])
    e = np.zeros((2, 32, 128, 128))
    for k2 in range(32):
        t = 2 * np.pi * (((32 * n[:, None] + k2) * n[None, :]) % S) / S
        er, ei = np.cos(t), -np.sin(t)
        m = np.block([[er, -ei], [ei, er]])[order][:, order]
        e[0, k2], e[1, k2] = m, m.T
    small = np.concatenate([_pack_rows(fw), _pack_rows(iw)], axis=0)
    return small, _pack_rows(e).reshape(64, 64, 128)


SMALL_TILES = 16


def _loop(name, lo, hi, body, init, **kw):
    with jax.named_scope(name):
        return lax.fori_loop(lo, hi, body, init, **kw)


def _bf(x):
    return pltpu.bitcast(x, bf16)


def _dot(a, b):
    return jnp.dot(a, b, preferred_element_type=f32)


def _round_bf16(x):
    return x.astype(bf16).astype(f32)


def _layernorm(x):
    m = jnp.mean(x, axis=-1, keepdims=True)
    xc = x - m
    v = jnp.mean(xc * xc, axis=-1, keepdims=True)
    return xc * lax.rsqrt(v + EPS)


def _fft4(x, sign):
    (ar, ai), (br, bi), (cr, ci), (dr, di) = x
    t0r, t0i, t1r, t1i = ar + cr, ai + ci, ar - cr, ai - ci
    t2r, t2i, t3r, t3i = br + dr, bi + di, br - dr, bi - di
    y0, y2 = (t0r + t2r, t0i + t2i), (t0r - t2r, t0i - t2i)
    p, q = (t1r + t3i, t1i - t3r), (t1r - t3i, t1i + t3r)
    return [y0, p, y2, q] if sign < 0 else [y0, q, y2, p]


def _twiddle(z, n, period, sign):
    zr, zi = z
    n = n % period
    if n == 0:
        return z
    if 4 * n == period:
        return (-zi, zr) if sign > 0 else (zi, -zr)
    c, s = math.cos(2 * math.pi * n / period), sign * math.sin(2 * math.pi * n / period)
    if (8 * n) % period == 0:
        a, d = zr + zi, zr - zi
        if c * s > 0:
            return (d * c, a * c)
        return (a * c, d * s)
    return (zr * c - zi * s, zr * s + zi * c)


def _bsum(x, y, sign):
    x, y = x.astype(f32), y.astype(f32)
    return (x + y if sign > 0 else x - y).astype(bf16)


def _strassen_lhs(a11, a12, a21, a22):
    return [lambda: a11() + a22(), lambda: a21() + a22(), a11, a22,
            lambda: a11() + a12(), lambda: a21() - a11(), lambda: a12() - a22()]


def _strassen_rhs(b11, b12, b21, b22):
    return [lambda: _bsum(b11(), b22(), 1), b11, lambda: _bsum(b12(), b22(), -1),
            lambda: _bsum(b21(), b11(), -1), b22, lambda: _bsum(b11(), b12(), 1),
            lambda: _bsum(b21(), b22(), 1)]


STRASSEN_OUT = [(((0, 0), 1), ((1, 1), 1)), (((1, 0), 1), ((1, 1), -1)), (((0, 1), 1), ((1, 1), 1)),
                (((0, 0), 1), ((1, 0), 1)), (((0, 0), -1), ((0, 1), 1)), (((1, 1), 1),), (((0, 0), 1),),
                (((0, 0), 1),), (((0, 1), 1),), (((1, 0), 1),), (((1, 1), 1),)]
WS_SLOT = {0: 0, 2: 1, 3: 2, 5: 3, 6: 4}


def _mu():
    lane = lax.broadcasted_iota(jnp.int32, (1, 128), 1)
    return jnp.where(lane < 64, S1, -S1).astype(f32)


def _ilv(r, i):
    n = r.shape[0] // 8
    return jnp.concatenate([r.reshape(n, 8, 128), i.reshape(n, 8, 128)], axis=1).reshape(16 * n, 128)


def _dilv(x):
    n = x.shape[0] // 16
    x = x.reshape(n, 16, 128)
    return x[:, :8].reshape(8 * n, 128), x[:, 8:].reshape(8 * n, 128)


def _with_tokens(x, toks):
    if not toks:
        return x
    return jnp.concatenate(
        [x[8 * j:8 * j + 8] | toks[j] if j in toks else x[8 * j:8 * j + 8]
         for j in range(x.shape[0] // 8)], axis=0)


def _fft16(x, sign, emit=None):
    cols = [_fft4([x[4 * j + r] for j in range(4)], sign) for r in range(4)]
    out = [None] * 16
    for q in range(4):
        y = _fft4([_twiddle(cols[r][q], r * q, 16, sign) for r in range(4)], sign)
        for p in range(4):
            out[q + 4 * p] = y[p]
        if emit is not None:
            emit(q, y)
    return out


CFG = dict(steps=((4.5, 16.5, 6, 4, 0, 8), (5, 16.5, 5, 7, 8, 12), (5, 16.5, 6, 6, 8, 12), (5, 16.5, 8, 7, 8, 0)),
           post_dl=20, post_passes=((0, 1), (2, 3), (4, 5), (6, 7)),
           post_order=(0, 1, 6, 3, 4, 2, 8, 5, 7, 9, 10, 11), post_at=(22, 26, 68, 96),
           tails_order=((1, 2, 0), 5), out_order=((1, 2, 0), 5), pack_f=True, pack_i=True,
           inv_at=tuple(range(28, 44)), inv_groups=1, inv_lag=4, tok_pos=(4, 5, 6, 7),
           fwd_at=(7, 8, 9, 10, 12, 13, 14, 16, 17, 18, 20, 21, 22, 24, 25, 26), rel=(0, 1), dinv_at=(0, 0, 1, 1), dinv_order=(2, 1, 0),

           two_inner=(5, 4, 2, 8, 0, 3, 6, 7, 10, 1, 9),
           two_outer=((2, 2), (5, 3), (1, None), (0, None), (4, 0), (3, None), (6, 1)),
           batch_unroll=2, post_unroll=1,
           ws_split=4, ws_at=(15, 15, 16, 16, 17, 18, 18, 19, 20, 20, 21, 21, 22, 23, 23, 24),
           pro_inner=(4, 2, 5, 8, 0, 3, 6, 7, 9, 10, 1),
           pro_outer=((2, 2), (5, 3), (1, 0), (0, None), (4, None), (3, None), (6, 1)),
           pro_nre=13, re_pos=(2, 2, 5, 5), ln_at=(11, 17, 23, 27), ln_at2=(3, 4, 6, 7, 9, 10, 12, 13),
           perm_at=tuple(range(10, 22)), only=None)


def _interleave(main, side):
    n, k = len(main), 0
    for i, f in enumerate(main):
        f()
        while k < len(side) and (k + 1) * n <= (i + 1) * len(side):
            side[k]()
            k += 1
    for f in side[k:]:
        f()


def _kernel(x_hbm, mem_hbm, wq_hbm, wk_hbm, wv_hbm, wo_hbm, wr_hbm, wi_hbm,
            small_hbm, e_hbm, out_hbm,
            xin, xa, xb, to, raw, wa, wb, wo_t, ws, qb, hl, z0, z1, z2, wf,
            wri, wtmp, small, emat, fill_ref, mem_ref, zero_ref, sem, osem):
    zs = (z0, z1, z2)
    w_hbm = (wq_hbm, wk_hbm, wv_hbm)

    def body_chunk(i):
        return 4 * (i & 3) + (i >> 2)

    def cp_w(i):
        src = w_hbm[i >> 2].at[:, :, pl.ds(8 * (i & 3), 8), :] if isinstance(i, int) else raw.at[i]
        return pltpu.make_async_copy(src, raw.at[i], sem.at[i])

    def cp_x(bb):
        return pltpu.make_async_copy(x_hbm.at[:, bb], xin.at[:, bb], sem.at[12 + bb])

    def cp_f(i):
        src = ((wr_hbm, wi_hbm)[i >> 2].at[:, pl.ds(512 * (i & 3), 512)]
               if isinstance(i, int) else wri.at[i])
        return pltpu.make_async_copy(src, wri.at[i], sem.at[36 + i])

    def cp_wo(i):
        rows = pl.ds(pl.multiple_of(512 * i, 512), 512)
        return [pltpu.make_async_copy(wo_hbm.at[rows, pl.ds(128 * j, 128)], wo_t.at[j, rows], sem.at[28 + i])
                for j in range(5)]

    cp_rest = [pltpu.make_async_copy(mem_hbm, mem_ref, sem.at[46]),
                pltpu.make_async_copy(small_hbm, small, sem.at[44]),
               pltpu.make_async_copy(e_hbm, emat, sem.at[45])]

    full = CFG["only"] in (None, "pro")
    for u in range(4 if full else 0):
        cp_x(4 * u + 3).start()
    if full:
        cp_w(0).start()
    for i in range(12 if full else 0):
        if i < 11:
            cp_w(i + 1).start()
        cp_x(body_chunk(i)).start()
        if 3 <= i < 11:
            cp_f(i - 3).start()
            for cp in cp_wo(i - 3):
                cp.start()
    for cp in cp_rest if full else ():
        cp.start()

    zero_ref[0] = 0

    r = lax.broadcasted_iota(jnp.int32, (80, 80), 0)
    c = lax.broadcasted_iota(jnp.int32, (80, 80), 1)

    def head(i):
        return jnp.where(i < 64, i // 32, (i - 64) // 8)

    def pos(i):
        return jnp.where(i < 64, i % 32, 32 + (i - 64) % 8)

    ok = (pos(r) < MEM) | (pos(r) >= pos(c))
    fill_ref[...] = jnp.where(head(r) == head(c), jnp.where(ok, 0.0, -1e9), -jnp.inf).astype(f32)
    wtmp[:, 320:328, :] = jnp.zeros((4, 8, 128), f32)
    xa[32, 0:8, 0:128] = jnp.zeros((8, 128), f32)
    ws[18, 0, 0:16, :] = jnp.zeros((16, 128), bf16)
    wa[12, 0:8, :] = jnp.zeros((8, 128), u32)
    wb[12, 0:8, :] = jnp.zeros((8, 128), u32)
    wf[5, 16 * WPITCH:16 * WPITCH + 8, :] = jnp.zeros((8, 128), f32)
    for z in zs:
        z[0, 0, 128:ZPITCH, :] = jnp.zeros((8, 128), f32)

    def chunk(bb):
        if isinstance(bb, int):
            return slice(8 * bb, 8 * bb + 8)
        return pl.ds(pl.multiple_of(8 * bb, 8), 8)

    def set_input(bb, x, tail_u, a0=0):
        n = x.shape[0] // 8
        xa[a0:a0 + n, chunk(bb), :] = x.reshape(n, 8, DM)
        y = _layernorm(x)
        if tail_u is None:
            xa[16 + a0:16 + a0 + n, chunk(bb), :] = y.reshape(n, 8, DM)
        else:
            blk = [[y[32 * r:32 * r + 32, 128 * kt:128 * kt + 128] for kt in range(5)] for r in range(4)]
            lv1 = [_strassen_lhs(*[functools.partial(lambda v: v, blk[2 * rr + r][2 * kk + k])
                                   for rr in range(2) for kk in range(2)])
                   for r in range(2) for k in range(2)]
            ops = []
            for i in range(7):
                sub = [f[i]() for f in lv1]
                ops += [f() for f in _strassen_lhs(*[functools.partial(lambda v: v, v) for v in sub])]
            for i, v in enumerate(ops + [blk[r][4] for r in range(4)]):
                hl[i, 16 * tail_u:16 * tail_u + 16, :] = pltpu.bitcast(v.astype(bf16), u32)

    def load_x(bb, a0=0, n=16):
        return xin[a0:a0 + n, bb].astype(f32).reshape(8 * n, DM)

    def wtile(cid, j, e):
        w = (wa, wb)[e]
        return jnp.concatenate([w[cid, (4 * hf + j) * HPITCH:(4 * hf + j) * HPITCH + 160, :]
                                for hf in range(2)], axis=0)

    def relayout(i, cid, e):
        for r in range(4 * i, 4 * i + 4):
            a, b = [pltpu.bitcast(raw[cid, :, d].reshape(16, 128), u32) for d in (2 * r, 2 * r + 1)]
            v = (a & 0xFFFF) | (b << 16) if e == 0 else (a >> 16) | (b & jnp.uint32(0xFFFF0000))
            (wa, wb)[e][cid, pl.ds(r, 8, stride=HPITCH), :] = v

    def batch_thunks(cid, inner, outer_order):
        qv = qb.at[:, :, pl.ds(8 * cid, 8)]
        RH = [((0, 0, 1), (1, 1, 1)), ((0, 0, 1),), ((0, 1, 1), (1, 1, -1)), ((1, 0, 1), (0, 0, -1)),
              ((1, 1, 1),), ((0, 0, 1), (0, 1, 1)), ((1, 0, 1), (1, 1, 1))]

        def unit(e):
            c = {}
            left = {(r, n): (5, 3, 3, 5)[2 * (r >> 1) + (n >> 1)] for r in range(4) for n in range(4)}

            def w(n, kt):
                return _bf(wtile(cid, n, e)[64 * kt:64 * kt + 64])

            def acc(blk, y, sign):
                if blk not in c:
                    c[blk] = y if sign > 0 else -y
                else:
                    c[blk] = c[blk] + y if sign > 0 else c[blk] - y
                left[blk] -= 1
                if left[blk] == 0:
                    r, n = blk
                    y = c.pop(blk).reshape(4, 4, 8, 128)
                    for u in range(4):
                        qv[4 * r:4 * r + 4, u, 2 * n + e] = y[u]

            def outer(I, k4):
                st = {}

                def lvl1(k, n):
                    if (k, n) not in st:
                        t = [(w(2 * nn + n, 2 * kk + k), sg) for kk, nn, sg in RH[I]]
                        if len(t) == 1:
                            st[k, n] = t[0][0]
                        else:
                            x, y = t[0][0].astype(f32), t[1][0].astype(f32)
                            st[k, n] = x + y if t[1][1] > 0 else x - y
                    return st[k, n]
                p = {}
                pl_ = {(0, 0): 4, (0, 1): 2, (1, 0): 2, (1, 1): 4}

                def half(items):
                    def run(toks=None):
                        for i in items:
                            if i >= 7:
                                r, n = k4[i - 7]
                                acc((r, n), _dot(_bf(_with_tokens(hl[49 + r], toks)), w(n, 4)), 1)
                                toks = None
                                continue
                            t = [(lvl1(k, n), sg) for k, n, sg in RH[i]]
                            rhs = t[0][0].astype(bf16) if len(t) == 1 else _bsum(t[0][0], t[1][0], t[1][1])
                            y = _dot(_bf(_with_tokens(hl[7 * I + i], toks)), rhs)
                            toks = None
                            for blk, sign in STRASSEN_OUT[i]:
                                if blk not in p:
                                    p[blk] = y if sign > 0 else -y
                                else:
                                    p[blk] = p[blk] + y if sign > 0 else p[blk] - y
                                pl_[blk] -= 1
                                if pl_[blk] == 0:
                                    for (R, N), sg in STRASSEN_OUT[I]:
                                        acc((2 * R + blk[0], 2 * N + blk[1]), p[blk], sg)
                    return run
                items = [i for i in inner if i < 7 + len(k4)]
                return [half(items[:len(items) // 2]), half(items[len(items) // 2:])]
            out = []
            for I, q in outer_order:
                k4 = [] if q is None else [(2 * (q >> 1) + (j >> 1), 2 * (q & 1) + (j & 1)) for j in range(4)]
                out += outer(I, k4)
            return out
        return unit(0) + unit(1)

    def wperm_thunks(piece, j):
        m = (piece >> 2) & 1
        wt = wtmp.at[j]

        def load():
            wt[0:DF, :] = wri[piece, :, 128 * j:128 * j + 128].astype(f32)

        def one(g):
            def run():
                if g == 0:
                    t = jnp.concatenate([wt[pl.ds(0, 64, stride=5), :], wt[320:328, :],
                                         jnp.zeros((56, 128), f32)], axis=0)
                else:
                    t = jnp.concatenate([wt[pl.ds(g, 64, stride=5), :],
                                         wt[pl.ds(5 - g, 64, stride=5), :]], axis=0)
                y = t.T
                sub = wf.at[3 * m + g, pl.ds(pl.multiple_of((piece & 3) * 32, 32), 16 * WPITCH - 96)]
                for k in range(8):
                    for hf in range(2):
                        sub[pl.ds(8 * j + k + 8 * hf * WPITCH, 8, stride=WPITCH), :] = (
                            y[16 * k + 8 * hf:16 * k + 8 * hf + 8])
            return run
        return [load] + [one(g) for g in range(3)]

    def half_pass(cid, half, fill, zero, timed=()):
        nre = CFG["pro_nre"]
        toks = None
        for k, f in enumerate(batch_thunks(cid, CFG["pro_inner"], CFG["pro_outer"])[14 * half:14 * half + 14]):
            f(toks)
            toks = {}
            for n, f in enumerate(f for at, f in timed if at == k):
                toks[(0, 4, 1, 6)[n]] = f()
            if fill is not None:
                for n, r in enumerate(r for r in range(40) if r * nre // 40 == k):
                    relayout(r, fill, 1 - half)
                    toks[CFG["re_pos"][n]] = (wb, wa)[half][12 + zero, 0:8, :]

    def ln_parts(bb, zero):
        def part(j):
            set_input(bb, load_x(bb, 4 * j, 4), None, 4 * j)
            return pltpu.bitcast(xa[32 + zero, 0:8, 0:128], u32)
        return [functools.partial(part, j) for j in range(4)]

    def perm_parts(piece, zero):
        def part(fs):
            for f in fs:
                f()
            return pltpu.bitcast(wf[5 + zero, 16 * WPITCH:16 * WPITCH + 8, :], u32)
        out = []
        for j in range(4):
            th = wperm_thunks(piece, j)
            out += [functools.partial(part, th[0:2]), functools.partial(part, th[2:3]),
                    functools.partial(part, th[3:4])]
        return out

    def ws_parts(piece, zero):
        nr = 128 // CFG["ws_split"]

        src = wo_t.at[:, pl.ds(pl.multiple_of(512 * piece, 512), 512)]
        dst = ws.at[pl.ds(2 * piece, 2)]

        def part(pp, np_, r0):
            def tile(k, n):
                lo = 256 * pp + 128 * k + r0
                return src[2 * np_ + n, lo:lo + nr, :]
            rhs = _strassen_rhs(*[functools.partial(tile, k, n) for k in range(2) for n in range(2)])
            for i, slot in WS_SLOT.items():
                dst[pp, 5 * np_ + slot, r0:r0 + nr, :] = rhs[i]()
            return pltpu.bitcast(ws[18 + zero, 0, 0:16, :], u32)
        return [functools.partial(part, pp, np_, r0)
                for pp in range(2) for np_ in range(2) for r0 in range(0, 128, nr)]

    def pro0():
        for u in range(4):
            cp_x(4 * u + 3).wait()
        for u in range(4):
            set_input(4 * u + 3, load_x(4 * u + 3), u)
        cp_w(0).wait()
        zero = zero_ref[0]
        for i in range(40):
            relayout(i, 0, 0)
        half_pass(0, 0, zero, zero)

    def pro1(it, carry):
        bb = jnp.where(it == 0, 3, body_chunk(it - 1))
        with jax.named_scope("pro1_wait"):
            cp_w(it + 1).wait()

            @pl.when(it >= 1)
            def _():
                cp_x(bb).wait()

            @pl.when(it >= 3)
            def _():
                cp_f(it - 3).wait()
                for cp in cp_wo(it - 3):
                    cp.wait()
        piece = jnp.where(it >= 3, it - 3, 8)
        zero = it >> 4
        timed = sorted(list(zip(CFG["ln_at"], ln_parts(bb, zero)))
                       + list(zip(CFG["ws_at"], ws_parts(piece, zero)))
                       + list(zip(CFG["perm_at"], perm_parts(piece, zero))), key=lambda x: x[0])
        half_pass(it, 1, it + 1, zero, [x for x in timed if x[0] < 14])
        half_pass(it + 1, 0, it + 1, zero, [(k - 14, f) for k, f in timed if k >= 14])
        return carry

    def pro2():
        cp_x(body_chunk(10)).wait()
        cp_x(body_chunk(11)).wait()
        cp_rest[0].wait()
        zero = zero_ref[0]
        half_pass(11, 1, None, zero, list(zip(
            CFG["ln_at2"], ln_parts(body_chunk(10), zero) + ln_parts(body_chunk(11), zero))))

    if full:
        with jax.named_scope("pro0"):
            pro0()
        _loop("pro1", 0, 11, pro1, 0)
        with jax.named_scope("pro2"):
            pro2()

    scale = DH ** -0.5

    def wo_dot(hh, oo):
        return [_dot(oo, wo_t[j, 128 * hh:128 * hh + 128, :]) for j in range(5)]

    def addl(acc, res):
        return res if acc is None else [a + b for a, b in zip(acc, res)]

    def group(g, mem):
        for ph in range(4):
            h = jnp.concatenate([mem, xa[16 + g, 32 * ph:32 * ph + 24, :]], axis=0).astype(bf16)
            pr, sm, oos = {}, {}, {}
            lat_s, lat_pv, lat_wo, v_delay, n_first, n_last = CFG["steps"][ph]

            def stacked(p, m):
                tails = [qb[g, ph, 32 * m + 2 * p + e] for e in range(2)]
                return jnp.concatenate([pr[p, m, 0], pr[p, m, 1]] + tails, axis=0).astype(bf16)

            def scores(p):
                sc = lax.dot_general(stacked(p, 0), stacked(p, 1), (((1,), (1,)), ((), ())),
                                     preferred_element_type=f32)
                fill = fill_ref[...]
                sc = jnp.where(fill == 0.0, sc * scale, fill)
                mx = jnp.max(sc, axis=-1, keepdims=True)
                e = jnp.exp(sc - mx)
                rl = pl.reciprocal(jnp.sum(e, axis=-1, keepdims=True), approx=True)
                sm[p] = (e * rl).astype(bf16)

            def pv(p):
                o = _dot(sm[p], stacked(p, 2))
                for e in range(2):
                    qb[g, ph, 2 * p + e] = o[64 + 8 * e:72 + 8 * e]
                    oos[2 * p + e] = o[32 * e:32 * e + 32].astype(bf16)

            keyed = []
            for p in range(NPAIR):
                keyed += [(4 * p + 2 * m + e, (p, m, e)) for m in range(2) for e in range(2)]
                keyed += [(4 * p + 3.5 + v_delay, (p, 2, e)) for e in range(2)]
            bulk = [x for _, x in sorted(keyed, key=lambda kv: kv[0])]
            acc, t, nwo, pend, ready = None, 0.0, 0, [], []
            if n_first:
                first, bulk = bulk[:n_first], bulk[n_first:]
                for kt in range(5):
                    for p, m, e in first:
                        w = wtile(4 * m + (p >> 2), p & 3, e)[64 * kt:64 * kt + 64]
                        y = _dot(h[:, 128 * kt:128 * kt + 128], _bf(w))
                        pr[p, m, e] = y if kt == 0 else pr[p, m, e] + y
                t = float(len(first))
                pend = [(t + lat_s, "S", p) for p, m, e in first if m == 1 and e == 1]
            while nwo < H - n_last or pend:
                pend.sort()
                if pend and pend[0][0] <= t:
                    _, kind, p = pend.pop(0)
                    if kind == "S":
                        scores(p)
                        pend.append((t + lat_pv, "V", p))
                    else:
                        pv(p)
                        ready += [(t + lat_wo, 2 * p + e) for e in range(2)]
                    t += 0.5
                elif bulk:
                    p, m, e = bulk.pop(0)
                    pr[p, m, e] = _dot(h, _bf(wtile(4 * m + (p >> 2), p & 3, e)))
                    t += 1
                    if m == 1 and e == 1:
                        pend.append((t + lat_s, "S", p))
                elif ready and ready[0][0] <= t and nwo < H - n_last:
                    _, hh = ready.pop(0)
                    acc = addl(acc, wo_dot(hh, oos[hh]))
                    t += 1
                    nwo += 1
                else:
                    t += 0.5
            for j in range(5):
                for _, hh in ready:
                    acc[j] = acc[j] + _dot(oos[hh], wo_t[j, 128 * hh:128 * hh + 128, :])
            out = jnp.concatenate(acc, axis=1)
            xa[16 + g, 32 * ph:32 * ph + 24, :] = out[8:32]
            mem = _round_bf16(out[0:8])
        return mem

    def dfwd_thunks(seg, q):
        st = {}
        rows = chunk(q)
        xav, xbv, zv = xa.at[:, seg], xb.at[:, seg], [z.at[:, :, seg] for z in zs]

        def pre():
            o = to[...] if q == 3 else xav[16:32, rows, :]
            x = _round_bf16(xav[0:16, rows, :] + o)
            xbv[:, rows, :] = x
            y = _layernorm(x.reshape(128, DM))
            x0, x1, x2, x3, x4 = [y[:, 128 * a:128 * a + 128] for a in range(5)]
            t1, t2, t3, t4 = x1 + x4, x2 + x3, x1 - x4, x2 - x3
            t = t1 + t2
            m, n = x0 - 0.25 * t, R5_D * (t1 - t2)
            st["u"] = [x0 + t, (m + n, t3 + R5_R * t4), (m - n, R5_R * t3 - t4)]

        def part(g):
            def run():
                if g == 0:
                    pre()
                    u0 = st["u"][0].astype(bf16)
                    zr = _dot(u0, _bf(small[0]))
                    if CFG["pack_f"]:
                        lane = lax.broadcasted_iota(jnp.int32, (128, 128), 1)
                        zi = jnp.where((lane & 63) == 0, 0.0, pltpu.roll(zr, 64, 1))
                    else:
                        zi = _dot(u0, _bf(small[1]))
                else:
                    a, b = st["u"][g]
                    k, kb, ka = [_dot(v.astype(bf16), _bf(small[3 * g - 1 + i]))
                                 for i, v in enumerate((a + b, b, a))]
                    zr, zi = k + kb, ka - _mu() * k
                ys = [(zr[8 * a:8 * a + 8], zi[8 * a:8 * a + 8]) for a in range(16)]
                if g < 2:
                    ys = _fft16(ys, -1)
                for a in range(16):
                    zv[g][0, a, rows, :] = ys[a][0]
                    zv[g][1, a, rows, :] = ys[a][1]
            return run
        return [part(g) for g in range(3)]

    def post(u, carry):
        base = pl.multiple_of(32 * u, 32)
        side = []
        for q in range(4):
            side += dfwd_thunks(pl.ds(base, 32), q)
        side = [side[i] for i in CFG["post_order"]]
        k = 0
        at = list(CFG["post_at"])
        m, due = {}, []
        for prods in CFG["post_passes"]:
            acc = None
            for p in range(NPAIR):
                lhs = _strassen_lhs(*[
                    functools.partial(lambda r, e: qb[8 * r:8 * r + 8, u, 2 * p + e].reshape(64, 128), r, e)
                    for r in range(2) for e in range(2)])
                res = []
                for i in prods:
                    if i == 7:
                        oo = jnp.concatenate([qb[:, u, 2 * p + e].reshape(128, 128) for e in range(2)], axis=1)
                        res.append(_dot(oo.astype(bf16), wo_t[4, 256 * p:256 * p + 256, :]))
                        k += 2
                        continue
                    a = lhs[i]().astype(bf16)
                    for np_ in range(2):
                        if i in WS_SLOT:
                            w = ws[p, 5 * np_ + WS_SLOT[i]]
                        else:
                            kk = 0 if i == 1 else 1
                            w = wo_t[2 * np_ + kk, 256 * p + 128 * kk:256 * p + 128 * kk + 128, :]
                        if due and due[0][0] <= k:
                            w = _bf(_with_tokens(pltpu.bitcast(w, u32), {0: due.pop(0)[1]}))
                        res.append(_dot(a, w))
                    k += 1
                acc = addl(acc, res)
                while at and at[0] <= k:
                    g = CFG["post_order"][len(CFG["post_at"]) - len(at)] % 3
                    at.pop(0)
                    side.pop(0)()
                    if g == 0 and CFG["post_dl"]:
                        due.append((k + CFG["post_dl"],
                                    pltpu.bitcast(z0[0, u >> 2, 128:ZPITCH, :], u32)))
            for i in prods:
                m[i] = [acc.pop(0)] if i == 7 else [acc.pop(0), acc.pop(0)]
        cols = []
        for np_ in range(2):
            m1, m2, m3, m4, m5, m6, m7 = [m[i][np_] for i in range(7)]
            cols.append(jnp.concatenate([m1 + m4 - m5 + m7, m2 + m4], axis=0))
            cols.append(jnp.concatenate([m3 + m5, m1 - m2 + m3 + m6], axis=0))
        to[...] = jnp.concatenate(cols + m[7], axis=1).reshape(16, 8, DM)
        for f in side:
            f()
        return carry

    def spectral(zero):
        def fence(z):
            return z[0, zero, 128:ZPITCH, :]

        def radix(g, bb, sign):
            z = zs[g]
            toks = []

            def emit(q, y):
                for p in range(4):
                    z[0, q + 4 * p, chunk(bb), :] = y[p][0]
                    z[1, q + 4 * p, chunk(bb), :] = y[p][1]
                toks.append(fence(z))
            _fft16([(z[0, a, chunk(bb), :], z[1, a, chunk(bb), :]) for a in range(16)], sign, emit)
            return toks

        ys = {}

        def fwd(g, k2, toks):
            z = zs[g]
            ur, ui = z[0, k2, 0:64, :], z[1, k2, 0:64, :]
            tr, ti = _twiddle((z[0, k2, 64:128, :], z[1, k2, 64:128, :]), k2, 32, -1)
            for hf in range(2):
                v = _ilv(ur + tr, ui + ti) if hf == 0 else _ilv(ur - tr, ui - ti)
                lhs = _with_tokens(emat[k2 + 16 * hf], toks if hf == 0 else None)
                xr, xi = _dilv(_dot(_bf(lhs), v.astype(bf16)))
                ys["x", 16 * g + k2] = xr
                wr = wf[g, pl.ds(k2 * WPITCH + hf, 64, stride=2), :]
                wi = wf[g + 3, pl.ds(k2 * WPITCH + hf, 64, stride=2), :]
                ys[g, k2, hf] = _ilv(xr * wr - xi * wi, xr * wi + xi * wr).astype(bf16)

        def inv(g, k2, toks):
            z = zs[g]
            t0 = _dot(_bf(_with_tokens(emat[32 + k2], toks)), ys.pop((g, k2, 0)))
            t1 = _dot(_bf(emat[48 + k2]), ys.pop((g, k2, 1)))
            z[0, k2, 0:64, :], z[1, k2, 0:64, :] = _dilv(t0 + t1)
            z[0, k2, 64:128, :], z[1, k2, 64:128, :] = _twiddle(_dilv(t0 - t1), k2, 32, 1)

        units = [(g, k2) for g in range(3) for k2 in range(16)]
        toks = None
        lag = CFG["inv_lag"]
        for i in range(len(units) + lag):
            if i < len(units):
                fwd(*units[i], toks)
            if i >= lag:
                inv(*units[i - lag], toks if i >= len(units) else None)
            toks = []
            if i in CFG["fwd_at"]:
                toks += radix(2, CFG["fwd_at"].index(i), -1)
            for n, at in enumerate(CFG["inv_at"]):
                if at == i:
                    if not toks:
                        back, r = CFG["rel"]
                        zs[n // 16][1, zero, 128:ZPITCH, :] = ys["x", min(i - back, 47)][8 * r:8 * r + 8]
                    toks += radix(n // 16, n % 16, 1)
            pos = CFG["tok_pos"] if len(toks) <= 4 else range(8)
            toks = {j: pltpu.bitcast(t, u32) for j, t in zip(pos, toks)}

    def dinv_thunks(bb, finish):
        st = {}

        def part(g):
            def run():
                z = zs[g]
                ys = [(z[0, a, chunk(bb), :], z[1, a, chunk(bb), :]) for a in range(16)]
                if g >= CFG["inv_groups"]:
                    ys = _fft16(ys, 1)
                tr = jnp.concatenate([y[0] for y in ys], axis=0)
                ti = jnp.concatenate([y[1] for y in ys], axis=0)
                if g == 0 and CFG["pack_i"]:
                    lane = lax.broadcasted_iota(jnp.int32, (128, 128), 1)
                    v = jnp.where(lane <= 64, tr, pltpu.roll(ti, 64, 1))
                    st[0] = _dot(v.astype(bf16), _bf(small[8]))
                elif g == 0:
                    st[0] = _dot(tr.astype(bf16), _bf(small[8])) + _dot(ti.astype(bf16), _bf(small[9]))
                else:
                    k, ki, kr = [_dot(v.astype(bf16), _bf(small[7 + 3 * g + i]))
                                 for i, v in enumerate((tr + _mu() * ti, ti, tr))]
                    st[2 * g - 1], st[2 * g] = k + ki, k + kr
            return run

        def fin():
            p0, p1, q1, p2, q2 = [st[j] for j in range(5)]
            t = p1 + p2
            m, n = p0 - 0.25 * t, R5_D * (p1 - p2)
            e1, e2 = m + n, m - n
            o1, o2 = q1 + R5_R * q2, R5_R * q1 - q2
            y = jnp.concatenate([p0 + t, e1 - o1, e2 - o2, e2 + o2, e1 + o1], axis=1)
            finish(xb[:, chunk(bb), :].reshape(128, DM) + y)
        return [part(0), part(1), part(2), fin]

    def out_copy(bb):
        return pltpu.make_async_copy(xin.at[:, bb], out_hbm.at[:, bb], osem.at[bb])

    def layer(li, carry0):
        if full or CFG["only"] == "group":
            _loop("step", 0, 16, group, mem_ref[...].astype(f32))
        if full or CFG["only"] == "spec":
            if full:
                @pl.when(li == 0)
                def _():
                    for cp in cp_rest[1:]:
                        cp.wait()
            _loop("post", 0, 4, post, 0, unroll=CFG["post_unroll"])

            with jax.named_scope("spectral"):
                spectral((li >> 1))
        if not full and CFG["only"] != "out":
            return carry0

        def run_chunks(th, order, lag):
            seq = [t[g] for t in th for g in order]
            for i in range(len(seq) + lag):
                if i < len(seq):
                    seq[i]()
                if i >= lag and (i - lag) % 3 == 2:
                    th[(i - lag) // 3][3]()

        @pl.when(li == 0)
        def _():
            with jax.named_scope("dinv_tails"):
                run_chunks([dinv_thunks(4 * u + 3, functools.partial(
                    lambda u, x: set_input(4 * u + 3, _round_bf16(x), u), u))
                    for u in range(4)],
                    *CFG["tails_order"])

            def batch(it, carry):
                bb = body_chunk(it)
                side = dinv_thunks(bb, lambda x: set_input(bb, _round_bf16(x), None))
                for k, f in enumerate(batch_thunks(it, CFG["two_inner"], CFG["two_outer"])):
                    f()
                    for at, g in zip(CFG["dinv_at"], CFG["dinv_order"] + (3,)):
                        if at == k:
                            side[g]()
                return carry
            _loop("batch", 0, 12, batch, 0, unroll=CFG["batch_unroll"])

        @pl.when(li == 1)
        def _():
            with jax.named_scope("dinv_out"):
                def store_out(bb, x):
                    xin[:, bb] = x.reshape(16, 8, DM).astype(bf16)
                    out_copy(bb).start()
                run_chunks([dinv_thunks(bb, functools.partial(store_out, bb)) for bb in range(16)],
                           *CFG["out_order"])
                for bb in range(16):
                    out_copy(bb).wait()
        return carry0

    if CFG["only"] != "pro":
        lax.fori_loop(0, 2, layer, 0)
    if CFG["only"] in ("pro", "out"):
        zero = zero_ref[0]
        xin[0, 0, :, 0:128] = (qb[zero, 0, 0] + wf[zero, 0:8, :] + xa[zero, 0:8, 0:128]).astype(bf16) + ws[zero, 0, 0:8, :]
        out_copy(0).start()
        out_copy(0).wait()
        for cp in cp_rest[1:] if full else ():
            cp.wait()


@jax.jit
def pallas_interleave_layers__memory_aug_recurrent_mem_tr__spectral_gfnet__prompt_kernel(
    A_x, A_mem0, A_Wq, A_Wk, A_Wv, A_Wo, A_seg_len, B_x, B_w_r, B_w_i,
):
    assert A_x.shape == (1, S, DM) and A_mem0.shape == (1, MEM, DM)
    small, emat = _tables()
    hbm = pl.BlockSpec(memory_space=pltpu.HBM)
    out = pl.pallas_call(
        _kernel,
        out_shape=jax.ShapeDtypeStruct((16, 16, 8, DM), bf16),
        in_specs=[hbm] * 10,
        out_specs=hbm,
        scratch_shapes=[
            pltpu.VMEM((16, 16, 8, DM), bf16),
            pltpu.VMEM((33, 128, DM), f32),
            pltpu.VMEM((16, 128, DM), f32),
            pltpu.VMEM((16, 8, DM), f32),
            pltpu.VMEM((12, 2, 320, 8, DH), bf16),
            pltpu.VMEM((13, 8 * HPITCH, 128), u32),
            pltpu.VMEM((13, 8 * HPITCH, 128), u32),
            pltpu.VMEM((5, H * DH + 512, 128), bf16),
            pltpu.VMEM((19, 10, 128, 128), bf16),
            pltpu.VMEM((16, 4, 96, 8, 128), f32),
            pltpu.VMEM((53, 64, 128), u32),
            pltpu.VMEM((2, 16, ZPITCH, 128), f32),
            pltpu.VMEM((2, 16, ZPITCH, 128), f32),
            pltpu.VMEM((2, 16, ZPITCH, 128), f32),
            pltpu.VMEM((6, 16 * WPITCH + 32, 128), f32),
            pltpu.VMEM((9, DF, 512), bf16),
            pltpu.VMEM((4, 328, 128), f32),
            pltpu.VMEM((SMALL_TILES, 64, 128), u32),
            pltpu.VMEM((64, 64, 128), u32),
            pltpu.VMEM((80, 80), f32),
            pltpu.VMEM((MEM, DM), bf16),
            pltpu.SMEM((1,), jnp.int32),
            pltpu.SemaphoreType.DMA((47,)),
            pltpu.SemaphoreType.DMA((16,)),
        ],
        compiler_params=pltpu.CompilerParams(vmem_limit_bytes=120 * 1024 * 1024,
                                             disable_semaphore_checks=True),
    )(
        A_x.reshape(16, 16, 8, DM), A_mem0.reshape(MEM, DM),
        *[w.reshape(2, 320, H, DH) for w in (A_Wq, A_Wk, A_Wv)], A_Wo.reshape(H * DH, DM), B_w_r.T, B_w_i.T,
        jnp.asarray(small), jnp.asarray(emat),
    )
    return out.reshape(1, S, DM)
```

```python
import functools
import math

import jax
import jax.numpy as jnp
import numpy as np
from jax import lax
import jax.experimental.pallas as pl
import jax.experimental.pallas.tpu as pltpu

f32, bf16, u32 = jnp.float32, jnp.bfloat16, jnp.uint32

S, DM, H, DH, MEM, SEG = 2048, 640, 32, 128, 8, 32
NPAIR = H // 2
DF = DM // 2 + 1
EPS = 1e-5
WPITCH = 132
HPITCH = 164
ZPITCH = 136

S1 = math.sin(2 * math.pi / 5)
R5_D = (math.cos(2 * math.pi / 5) - math.cos(4 * math.pi / 5)) / 2
R5_R = math.sin(4 * math.pi / 5) / S1


def _to_bf16_bits(a):
    u = np.ascontiguousarray(a, dtype=np.float32).view(np.uint32).astype(np.uint64)
    return ((u + 0x7FFF + ((u >> 16) & 1)) >> 16).astype(np.uint32)


def _pack_rows(a):
    b = _to_bf16_bits(a)
    return b[..., 0::2, :] | (b[..., 1::2, :] << 16)


@functools.lru_cache(maxsize=None)
def _tables():
    b = np.arange(128)
    l0 = np.arange(0, DF, 5)
    l1 = np.concatenate([np.arange(1, 320, 5), np.arange(4, 320, 5)])
    l2 = np.concatenate([np.arange(2, 320, 5), np.arange(3, 320, 5)])
    sg = np.concatenate([np.ones(64), -np.ones(64)])

    def th(l):
        return 2 * np.pi * ((b[:, None] * l[None, :]) % DM) / DM

    sc = 1.0 / (S * DM)
    fw = np.zeros((7, 128, 128))
    iw = np.zeros((7, 128, 128))
    t = th(l0)
    cl = np.full((128, 1), 2.0)
    cl[0] = cl[64] = 1.0
    fw[0] = np.concatenate([np.cos(t), -np.sin(t[:, 1:64])], axis=1)
    iw[0] = cl * sc * fw[0].T
    mu = S1 * sg
    for g, l in ((1, l1), (2, l2)):
        t = th(l)
        c, s = np.cos(t), np.sin(t)
        fw[3 * g - 2:3 * g + 1] = c, -mu * s - c, mu * c - s
        iw[3 * g - 2:3 * g + 1] = [2 * sc * m.T for m in (c, -s - mu * c, mu * s - c)]
    n = np.arange(64)
    order = np.concatenate([np.concatenate([np.arange(8) + 8 * j, np.arange(8) + 8 * j + 64])
                            for j in range(8)])
    e = np.zeros((2, 32, 128, 128))
    for k2 in range(32):
        t = 2 * np.pi * (((32 * n[:, None] + k2) * n[None, :]) % S) / S
        er, ei = np.cos(t), -np.sin(t)
        m = np.block([[er, -ei], [ei, er]])[order][:, order]
        e[0, k2], e[1, k2] = m, m.T
    small = np.concatenate([_pack_rows(fw), _pack_rows(iw)], axis=0)
    return small, _pack_rows(e).reshape(64, 64, 128)


def _loop(name, lo, hi, body, init, **kw):
    with jax.named_scope(name):
        return lax.fori_loop(lo, hi, body, init, **kw)


def _bf(x):
    return pltpu.bitcast(x, bf16)


def _dot(a, b):
    return jnp.dot(a, b, preferred_element_type=f32)


def _round_bf16(x):
    return x.astype(bf16).astype(f32)


def _layernorm(x):
    m = jnp.mean(x, axis=-1, keepdims=True)
    xc = x - m
    v = jnp.mean(xc * xc, axis=-1, keepdims=True)
    return xc * lax.rsqrt(v + EPS)


def _fft4(x, sign):
    (ar, ai), (br, bi), (cr, ci), (dr, di) = x
    t0r, t0i, t1r, t1i = ar + cr, ai + ci, ar - cr, ai - ci
    t2r, t2i, t3r, t3i = br + dr, bi + di, br - dr, bi - di
    y0, y2 = (t0r + t2r, t0i + t2i), (t0r - t2r, t0i - t2i)
    p, q = (t1r + t3i, t1i - t3r), (t1r - t3i, t1i + t3r)
    return [y0, p, y2, q] if sign < 0 else [y0, q, y2, p]


def _twiddle(z, n, period, sign):
    zr, zi = z
    n = n % period
    if n == 0:
        return z
    if 4 * n == period:
        return (-zi, zr) if sign > 0 else (zi, -zr)
    c, s = math.cos(2 * math.pi * n / period), sign * math.sin(2 * math.pi * n / period)
    if (8 * n) % period == 0:
        a, d = zr + zi, zr - zi
        if c * s > 0:
            return (d * c, a * c)
        return (a * c, d * s)
    return (zr * c - zi * s, zr * s + zi * c)


STRASSEN_LHS = (((0, 0, 1), (1, 1, 1)), ((1, 0, 1), (1, 1, 1)), ((0, 0, 1),), ((1, 1, 1),),
                ((0, 0, 1), (0, 1, 1)), ((1, 0, 1), (0, 0, -1)), ((0, 1, 1), (1, 1, -1)))
STRASSEN_RHS = (((0, 0, 1), (1, 1, 1)), ((0, 0, 1),), ((0, 1, 1), (1, 1, -1)), ((1, 0, 1), (0, 0, -1)),
                ((1, 1, 1),), ((0, 0, 1), (0, 1, 1)), ((1, 0, 1), (1, 1, 1)))
STRASSEN_OUT = ((((0, 0), 1), ((1, 1), 1)), (((1, 0), 1), ((1, 1), -1)), (((0, 1), 1), ((1, 1), 1)),
                (((0, 0), 1), ((1, 0), 1)), (((0, 0), -1), ((0, 1), 1)), (((1, 1), 1),), (((0, 0), 1),))
WS_SLOT = {0: 0, 2: 1, 3: 2, 5: 3, 6: 4}


def _operand(terms, block):
    x = block(*terms[0][:2])
    if len(terms) == 1:
        return x
    x, y = x.astype(f32), block(*terms[1][:2]).astype(f32)
    return x + y if terms[1][2] > 0 else x - y


def _accumulate(acc, key, y, sign):
    if key not in acc:
        acc[key] = y if sign > 0 else -y
    else:
        acc[key] = acc[key] + y if sign > 0 else acc[key] - y


def _mu():
    lane = lax.broadcasted_iota(jnp.int32, (1, 128), 1)
    return jnp.where(lane < 64, S1, -S1).astype(f32)


def _ilv(r, i):
    n = r.shape[0] // 8
    return jnp.concatenate([r.reshape(n, 8, 128), i.reshape(n, 8, 128)], axis=1).reshape(16 * n, 128)


def _dilv(x):
    n = x.shape[0] // 16
    x = x.reshape(n, 16, 128)
    return x[:, :8].reshape(8 * n, 128), x[:, 8:].reshape(8 * n, 128)


def _with_tokens(x, toks):
    if not toks:
        return x
    return jnp.concatenate(
        [x[8 * j:8 * j + 8] | toks[j] if j in toks else x[8 * j:8 * j + 8]
         for j in range(x.shape[0] // 8)], axis=0)


def _fft16(x, sign, emit=None):
    cols = [_fft4([x[4 * j + r] for j in range(4)], sign) for r in range(4)]
    out = [None] * 16
    for q in range(4):
        y = _fft4([_twiddle(cols[r][q], r * q, 16, sign) for r in range(4)], sign)
        for p in range(4):
            out[q + 4 * p] = y[p]
        if emit is not None:
            emit(q, y)
    return out


CFG = dict(
    steps=((4.5, 16.5, 6, 4, 0, 8), (5, 16.5, 5, 7, 8, 12), (5, 16.5, 6, 6, 8, 12), (5, 16.5, 8, 7, 8, 0)),
    pro_inner=(4, 2, 5, 8, 0, 3, 6, 7, 9, 10, 1),
    pro_outer=((2, 2), (5, 3), (1, 0), (0, None), (4, None), (3, None), (6, 1)),
    pro_nre=13, re_pos=(2, 2, 5, 5), ln_at=(11, 17, 23, 27), ln_at2=(3, 4, 6, 7, 9, 10, 12, 13),
    perm_at=tuple(range(10, 22)),
    ws_split=4, ws_at=(15, 15, 16, 16, 17, 18, 18, 19, 20, 20, 21, 21, 22, 23, 23, 24),
    post_passes=((0, 1), (2, 3), (4, 5), (6, 7)), post_dl=20,
    post_order=(0, 1, 6, 3, 4, 2, 8, 5, 7, 9, 10, 11), post_at=(22, 26, 68, 96),
    fwd_at=(7, 8, 9, 10, 12, 13, 14, 16, 17, 18, 20, 21, 22, 24, 25, 26),
    inv_at=tuple(range(28, 44)), inv_lag=4, tok_pos=(4, 5, 6, 7), rel=(0, 1),
    tails_order=((1, 2, 0), 5), out_order=((1, 2, 0), 5),
    two_inner=(5, 4, 2, 8, 0, 3, 6, 7, 10, 1, 9),
    two_outer=((2, 2), (5, 3), (1, None), (0, None), (4, 0), (3, None), (6, 1)),
    dinv_at=(0, 0, 1, 1), dinv_order=(2, 1, 0),
    only=None)


def _kernel(x_hbm, mem_hbm, wq_hbm, wk_hbm, wv_hbm, wo_hbm, wr_hbm, wi_hbm,
            small_hbm, e_hbm, out_hbm,
            xin, xa, xb, to, raw, wa, wb, wo_t, ws, qb, hl, z0, z1, z2, wf,
            wri, wtmp, small, emat, fill_ref, mem_ref, zero_ref, sem, osem):
    zs = (z0, z1, z2)
    w_hbm = (wq_hbm, wk_hbm, wv_hbm)

    def body_chunk(i):
        return 4 * (i & 3) + (i >> 2)

    def cp_w(i):
        src = w_hbm[i >> 2].at[:, :, pl.ds(8 * (i & 3), 8), :] if isinstance(i, int) else raw.at[i]
        return pltpu.make_async_copy(src, raw.at[i], sem.at[i])

    def cp_x(bb):
        return pltpu.make_async_copy(x_hbm.at[:, bb], xin.at[:, bb], sem.at[12 + bb])

    def cp_f(i):
        src = ((wr_hbm, wi_hbm)[i >> 2].at[:, pl.ds(512 * (i & 3), 512)]
               if isinstance(i, int) else wri.at[i])
        return pltpu.make_async_copy(src, wri.at[i], sem.at[36 + i])

    def cp_wo(i):
        rows = pl.ds(pl.multiple_of(512 * i, 512), 512)
        return [pltpu.make_async_copy(wo_hbm.at[rows, pl.ds(128 * j, 128)], wo_t.at[j, rows], sem.at[28 + i])
                for j in range(5)]

    cp_rest = [pltpu.make_async_copy(mem_hbm, mem_ref, sem.at[46]),
               pltpu.make_async_copy(small_hbm, small, sem.at[44]),
               pltpu.make_async_copy(e_hbm, emat, sem.at[45])]

    full = CFG["only"] in (None, "pro")
    for u in range(4 if full else 0):
        cp_x(4 * u + 3).start()
    if full:
        cp_w(0).start()
    for i in range(12 if full else 0):
        if i < 11:
            cp_w(i + 1).start()
        cp_x(body_chunk(i)).start()
        if 3 <= i < 11:
            cp_f(i - 3).start()
            for cp in cp_wo(i - 3):
                cp.start()
    for cp in cp_rest if full else ():
        cp.start()

    zero_ref[0] = 0

    r = lax.broadcasted_iota(jnp.int32, (80, 80), 0)
    c = lax.broadcasted_iota(jnp.int32, (80, 80), 1)

    def head(i):
        return jnp.where(i < 64, i // 32, (i - 64) // 8)

    def pos(i):
        return jnp.where(i < 64, i % 32, 32 + (i - 64) % 8)

    ok = (pos(r) < MEM) | (pos(r) >= pos(c))
    fill_ref[...] = jnp.where(head(r) == head(c), jnp.where(ok, 0.0, -1e9), -jnp.inf).astype(f32)
    wtmp[:, 320:328, :] = jnp.zeros((4, 8, 128), f32)
    xa[32, 0:8, 0:128] = jnp.zeros((8, 128), f32)
    ws[18, 0, 0:16, :] = jnp.zeros((16, 128), bf16)
    wa[12, 0:8, :] = jnp.zeros((8, 128), u32)
    wb[12, 0:8, :] = jnp.zeros((8, 128), u32)
    wf[5, 16 * WPITCH:16 * WPITCH + 8, :] = jnp.zeros((8, 128), f32)
    for z in zs:
        z[0, 0, 128:ZPITCH, :] = jnp.zeros((8, 128), f32)

    def chunk(bb):
        if isinstance(bb, int):
            return slice(8 * bb, 8 * bb + 8)
        return pl.ds(pl.multiple_of(8 * bb, 8), 8)

    def set_input(bb, x, tail_u, a0=0):
        n = x.shape[0] // 8
        xa[a0:a0 + n, chunk(bb), :] = x.reshape(n, 8, DM)
        y = _layernorm(x)
        if tail_u is None:
            xa[16 + a0:16 + a0 + n, chunk(bb), :] = y.reshape(n, 8, DM)
        else:
            blk = [[y[32 * r:32 * r + 32, 128 * kt:128 * kt + 128] for kt in range(5)] for r in range(4)]
            ops = []
            for outer in STRASSEN_LHS:
                sub = [[_operand(outer, lambda rr, kk: blk[2 * rr + r][2 * kk + k]) for k in range(2)]
                       for r in range(2)]
                ops += [_operand(inner, lambda r, k: sub[r][k]) for inner in STRASSEN_LHS]
            for i, v in enumerate(ops + [blk[r][4] for r in range(4)]):
                hl[i, 16 * tail_u:16 * tail_u + 16, :] = pltpu.bitcast(v.astype(bf16), u32)

    def load_x(bb, a0=0, n=16):
        return xin[a0:a0 + n, bb].astype(f32).reshape(8 * n, DM)

    def wtile(cid, j, e):
        w = (wa, wb)[e]
        return jnp.concatenate([w[cid, (4 * hf + j) * HPITCH:(4 * hf + j) * HPITCH + 160, :]
                                for hf in range(2)], axis=0)

    def relayout(i, cid, e):
        for r in range(4 * i, 4 * i + 4):
            a, b = [pltpu.bitcast(raw[cid, :, d].reshape(16, 128), u32) for d in (2 * r, 2 * r + 1)]
            v = (a & 0xFFFF) | (b << 16) if e == 0 else (a >> 16) | (b & jnp.uint32(0xFFFF0000))
            (wa, wb)[e][cid, pl.ds(r, 8, stride=HPITCH), :] = v

    def batch_thunks(cid, inner_order, outer_order):
        qv = qb.at[:, :, pl.ds(8 * cid, 8)]

        def unit(e):
            c = {}
            left = {(r, n): (5, 3, 3, 5)[2 * (r >> 1) + (n >> 1)] for r in range(4) for n in range(4)}

            def w(kt, n):
                return _bf(wtile(cid, n, e)[64 * kt:64 * kt + 64])

            def add_out(blk, y, sign):
                _accumulate(c, blk, y, sign)
                left[blk] -= 1
                if left[blk] == 0:
                    r, n = blk
                    y = c.pop(blk).reshape(4, 4, 8, 128)
                    for u in range(4):
                        qv[4 * r:4 * r + 4, u, 2 * n + e] = y[u]

            def outer(io, k4):
                p = {}
                todo = {(0, 0): 4, (0, 1): 2, (1, 0): 2, (1, 1): 4}

                @functools.lru_cache(maxsize=None)
                def sub(k, n):
                    return _operand(STRASSEN_RHS[io], lambda kk, nn: w(2 * kk + k, 2 * nn + n))

                def thunk(items):
                    def run(toks=None):
                        for i in items:
                            if i >= 7:
                                r, n = k4[i - 7]
                                add_out((r, n), _dot(_bf(_with_tokens(hl[49 + r], toks)), w(4, n)), 1)
                                toks = None
                                continue
                            rhs = _operand(STRASSEN_RHS[i], sub).astype(bf16)
                            y = _dot(_bf(_with_tokens(hl[7 * io + i], toks)), rhs)
                            toks = None
                            for blk, sign in STRASSEN_OUT[i]:
                                _accumulate(p, blk, y, sign)
                                todo[blk] -= 1
                                if todo[blk] == 0:
                                    for (rr, nn), sg in STRASSEN_OUT[io]:
                                        add_out((2 * rr + blk[0], 2 * nn + blk[1]), p[blk], sg)
                    return run
                items = [i for i in inner_order if i < 7 + len(k4)]
                return [thunk(items[:len(items) // 2]), thunk(items[len(items) // 2:])]
            out = []
            for io, q in outer_order:
                out += outer(io, [] if q is None else
                             [(2 * (q >> 1) + (j >> 1), 2 * (q & 1) + (j & 1)) for j in range(4)])
            return out
        return unit(0) + unit(1)

    def wperm_thunks(piece, j):
        m = (piece >> 2) & 1
        wt = wtmp.at[j]

        def load():
            wt[0:DF, :] = wri[piece, :, 128 * j:128 * j + 128].astype(f32)

        def one(g):
            def run():
                if g == 0:
                    t = jnp.concatenate([wt[pl.ds(0, 64, stride=5), :], wt[320:328, :],
                                         jnp.zeros((56, 128), f32)], axis=0)
                else:
                    t = jnp.concatenate([wt[pl.ds(g, 64, stride=5), :],
                                         wt[pl.ds(5 - g, 64, stride=5), :]], axis=0)
                y = t.T
                sub = wf.at[3 * m + g, pl.ds(pl.multiple_of((piece & 3) * 32, 32), 16 * WPITCH - 96)]
                for k in range(8):
                    for hf in range(2):
                        sub[pl.ds(8 * j + k + 8 * hf * WPITCH, 8, stride=WPITCH), :] = (
                            y[16 * k + 8 * hf:16 * k + 8 * hf + 8])
            return run
        return [load] + [one(g) for g in range(3)]

    def half_pass(cid, half, fill, zero, timed=()):
        nre = CFG["pro_nre"]
        toks = None
        for k, f in enumerate(batch_thunks(cid, CFG["pro_inner"], CFG["pro_outer"])[14 * half:14 * half + 14]):
            f(toks)
            toks = {}
            for n, f in enumerate(f for at, f in timed if at == k):
                toks[(0, 4, 1, 6)[n]] = f()
            if fill is not None:
                for n, r in enumerate(r for r in range(40) if r * nre // 40 == k):
                    relayout(r, fill, 1 - half)
                    toks[CFG["re_pos"][n]] = (wb, wa)[half][12 + zero, 0:8, :]

    def ln_parts(bb, zero):
        def part(j):
            set_input(bb, load_x(bb, 4 * j, 4), None, 4 * j)
            return pltpu.bitcast(xa[32 + zero, 0:8, 0:128], u32)
        return [functools.partial(part, j) for j in range(4)]

    def perm_parts(piece, zero):
        def part(fs):
            for f in fs:
                f()
            return pltpu.bitcast(wf[5 + zero, 16 * WPITCH:16 * WPITCH + 8, :], u32)
        out = []
        for j in range(4):
            th = wperm_thunks(piece, j)
            out += [functools.partial(part, th[0:2]), functools.partial(part, th[2:3]),
                    functools.partial(part, th[3:4])]
        return out

    def ws_parts(piece, zero):
        nr = 128 // CFG["ws_split"]

        src = wo_t.at[:, pl.ds(pl.multiple_of(512 * piece, 512), 512)]
        dst = ws.at[pl.ds(2 * piece, 2)]

        def part(pp, np_, r0):
            def tile(k, n):
                lo = 256 * pp + 128 * k + r0
                return src[2 * np_ + n, lo:lo + nr, :]
            for i, slot in WS_SLOT.items():
                dst[pp, 5 * np_ + slot, r0:r0 + nr, :] = _operand(STRASSEN_RHS[i], tile).astype(bf16)
            return pltpu.bitcast(ws[18 + zero, 0, 0:16, :], u32)
        return [functools.partial(part, pp, np_, r0)
                for pp in range(2) for np_ in range(2) for r0 in range(0, 128, nr)]

    def pro0():
        for u in range(4):
            cp_x(4 * u + 3).wait()
        for u in range(4):
            set_input(4 * u + 3, load_x(4 * u + 3), u)
        cp_w(0).wait()
        zero = zero_ref[0]
        for i in range(40):
            relayout(i, 0, 0)
        half_pass(0, 0, zero, zero)

    def pro1(it, carry):
        bb = jnp.where(it == 0, 3, body_chunk(it - 1))
        with jax.named_scope("pro1_wait"):
            cp_w(it + 1).wait()

            @pl.when(it >= 1)
            def _():
                cp_x(bb).wait()

            @pl.when(it >= 3)
            def _():
                cp_f(it - 3).wait()
                for cp in cp_wo(it - 3):
                    cp.wait()
        piece = jnp.where(it >= 3, it - 3, 8)
        zero = it >> 4
        timed = sorted(list(zip(CFG["ln_at"], ln_parts(bb, zero)))
                       + list(zip(CFG["ws_at"], ws_parts(piece, zero)))
                       + list(zip(CFG["perm_at"], perm_parts(piece, zero))), key=lambda x: x[0])
        half_pass(it, 1, it + 1, zero, [x for x in timed if x[0] < 14])
        half_pass(it + 1, 0, it + 1, zero, [(k - 14, f) for k, f in timed if k >= 14])
        return carry

    def pro2():
        cp_x(body_chunk(10)).wait()
        cp_x(body_chunk(11)).wait()
        cp_rest[0].wait()
        zero = zero_ref[0]
        half_pass(11, 1, None, zero, list(zip(
            CFG["ln_at2"], ln_parts(body_chunk(10), zero) + ln_parts(body_chunk(11), zero))))

    if full:
        with jax.named_scope("pro0"):
            pro0()
        _loop("pro1", 0, 11, pro1, 0)
        with jax.named_scope("pro2"):
            pro2()

    scale = DH ** -0.5

    def wo_dot(hh, oo):
        return [_dot(oo, wo_t[j, 128 * hh:128 * hh + 128, :]) for j in range(5)]

    def addl(acc, res):
        return res if acc is None else [a + b for a, b in zip(acc, res)]

    def group(g, mem):
        for ph in range(4):
            h = jnp.concatenate([mem, xa[16 + g, 32 * ph:32 * ph + 24, :]], axis=0).astype(bf16)
            pr, sm, oos = {}, {}, {}
            lat_s, lat_pv, lat_wo, v_delay, n_first, n_last = CFG["steps"][ph]

            def stacked(p, m):
                tails = [qb[g, ph, 32 * m + 2 * p + e] for e in range(2)]
                return jnp.concatenate([pr[p, m, 0], pr[p, m, 1]] + tails, axis=0).astype(bf16)

            def scores(p):
                sc = lax.dot_general(stacked(p, 0), stacked(p, 1), (((1,), (1,)), ((), ())),
                                     preferred_element_type=f32)
                fill = fill_ref[...]
                sc = jnp.where(fill == 0.0, sc * scale, fill)
                mx = jnp.max(sc, axis=-1, keepdims=True)
                e = jnp.exp(sc - mx)
                rl = pl.reciprocal(jnp.sum(e, axis=-1, keepdims=True), approx=True)
                sm[p] = (e * rl).astype(bf16)

            def pv(p):
                o = _dot(sm[p], stacked(p, 2))
                for e in range(2):
                    qb[g, ph, 2 * p + e] = o[64 + 8 * e:72 + 8 * e]
                    oos[2 * p + e] = o[32 * e:32 * e + 32].astype(bf16)

            keyed = []
            for p in range(NPAIR):
                keyed += [(4 * p + 2 * m + e, (p, m, e)) for m in range(2) for e in range(2)]
                keyed += [(4 * p + 3.5 + v_delay, (p, 2, e)) for e in range(2)]
            bulk = [x for _, x in sorted(keyed, key=lambda kv: kv[0])]
            acc, t, nwo, pend, ready = None, 0.0, 0, [], []
            if n_first:
                first, bulk = bulk[:n_first], bulk[n_first:]
                for kt in range(5):
                    for p, m, e in first:
                        w = wtile(4 * m + (p >> 2), p & 3, e)[64 * kt:64 * kt + 64]
                        y = _dot(h[:, 128 * kt:128 * kt + 128], _bf(w))
                        pr[p, m, e] = y if kt == 0 else pr[p, m, e] + y
                t = float(len(first))
                pend = [(t + lat_s, "S", p) for p, m, e in first if m == 1 and e == 1]
            while nwo < H - n_last or pend:
                pend.sort()
                if pend and pend[0][0] <= t:
                    _, kind, p = pend.pop(0)
                    if kind == "S":
                        scores(p)
                        pend.append((t + lat_pv, "V", p))
                    else:
                        pv(p)
                        ready += [(t + lat_wo, 2 * p + e) for e in range(2)]
                    t += 0.5
                elif bulk:
                    p, m, e = bulk.pop(0)
                    pr[p, m, e] = _dot(h, _bf(wtile(4 * m + (p >> 2), p & 3, e)))
                    t += 1
                    if m == 1 and e == 1:
                        pend.append((t + lat_s, "S", p))
                elif ready and ready[0][0] <= t and nwo < H - n_last:
                    _, hh = ready.pop(0)
                    acc = addl(acc, wo_dot(hh, oos[hh]))
                    t += 1
                    nwo += 1
                else:
                    t += 0.5
            for j in range(5):
                for _, hh in ready:
                    acc[j] = acc[j] + _dot(oos[hh], wo_t[j, 128 * hh:128 * hh + 128, :])
            out = jnp.concatenate(acc, axis=1)
            xa[16 + g, 32 * ph:32 * ph + 24, :] = out[8:32]
            mem = _round_bf16(out[0:8])
        return mem

    def dfwd_thunks(seg, q):
        st = {}
        rows = chunk(q)
        xav, xbv, zv = xa.at[:, seg], xb.at[:, seg], [z.at[:, :, seg] for z in zs]

        def pre():
            o = to[...] if q == 3 else xav[16:32, rows, :]
            x = _round_bf16(xav[0:16, rows, :] + o)
            xbv[:, rows, :] = x
            y = _layernorm(x.reshape(128, DM))
            x0, x1, x2, x3, x4 = [y[:, 128 * a:128 * a + 128] for a in range(5)]
            t1, t2, t3, t4 = x1 + x4, x2 + x3, x1 - x4, x2 - x3
            t = t1 + t2
            m, n = x0 - 0.25 * t, R5_D * (t1 - t2)
            st["u"] = [x0 + t, (m + n, t3 + R5_R * t4), (m - n, R5_R * t3 - t4)]

        def part(g):
            def run():
                if g == 0:
                    pre()
                    u0 = st["u"][0].astype(bf16)
                    zr = _dot(u0, _bf(small[0]))
                    lane = lax.broadcasted_iota(jnp.int32, (128, 128), 1)
                    zi = jnp.where((lane & 63) == 0, 0.0, pltpu.roll(zr, 64, 1))
                else:
                    a, b = st["u"][g]
                    k, kb, ka = [_dot(v.astype(bf16), _bf(small[3 * g - 2 + i]))
                                 for i, v in enumerate((a + b, b, a))]
                    zr, zi = k + kb, ka - _mu() * k
                ys = [(zr[8 * a:8 * a + 8], zi[8 * a:8 * a + 8]) for a in range(16)]
                if g < 2:
                    ys = _fft16(ys, -1)
                for a in range(16):
                    zv[g][0, a, rows, :] = ys[a][0]
                    zv[g][1, a, rows, :] = ys[a][1]
            return run
        return [part(g) for g in range(3)]

    def post(u, carry):
        base = pl.multiple_of(32 * u, 32)
        side = []
        for q in range(4):
            side += dfwd_thunks(pl.ds(base, 32), q)
        side = [side[i] for i in CFG["post_order"]]
        k = 0
        at = list(CFG["post_at"])
        m, due = {}, []
        for prods in CFG["post_passes"]:
            acc = None
            for p in range(NPAIR):
                res = []
                for i in prods:
                    if i == 7:
                        oo = jnp.concatenate([qb[:, u, 2 * p + e].reshape(128, 128) for e in range(2)], axis=1)
                        res.append(_dot(oo.astype(bf16), wo_t[4, 256 * p:256 * p + 256, :]))
                        k += 2
                        continue
                    a = _operand(STRASSEN_LHS[i], lambda r, e: (
                        qb[8 * r:8 * r + 8, u, 2 * p + e].reshape(64, 128))).astype(bf16)
                    for np_ in range(2):
                        if i in WS_SLOT:
                            w = ws[p, 5 * np_ + WS_SLOT[i]]
                        else:
                            kk = 0 if i == 1 else 1
                            w = wo_t[2 * np_ + kk, 256 * p + 128 * kk:256 * p + 128 * kk + 128, :]
                        if due and due[0][0] <= k:
                            w = _bf(_with_tokens(pltpu.bitcast(w, u32), {0: due.pop(0)[1]}))
                        res.append(_dot(a, w))
                    k += 1
                acc = addl(acc, res)
                while at and at[0] <= k:
                    g = CFG["post_order"][len(CFG["post_at"]) - len(at)] % 3
                    at.pop(0)
                    side.pop(0)()
                    if g == 0:
                        due.append((k + CFG["post_dl"],
                                    pltpu.bitcast(z0[0, u >> 2, 128:ZPITCH, :], u32)))
            for i in prods:
                m[i] = [acc.pop(0)] if i == 7 else [acc.pop(0), acc.pop(0)]
        cols = []
        for np_ in range(2):
            m1, m2, m3, m4, m5, m6, m7 = [m[i][np_] for i in range(7)]
            cols.append(jnp.concatenate([m1 + m4 - m5 + m7, m2 + m4], axis=0))
            cols.append(jnp.concatenate([m3 + m5, m1 - m2 + m3 + m6], axis=0))
        to[...] = jnp.concatenate(cols + m[7], axis=1).reshape(16, 8, DM)
        for f in side:
            f()
        return carry

    def spectral(zero):
        def fence(z):
            return z[0, zero, 128:ZPITCH, :]

        def radix(g, bb, sign):
            z = zs[g]
            toks = []

            def emit(q, y):
                for p in range(4):
                    z[0, q + 4 * p, chunk(bb), :] = y[p][0]
                    z[1, q + 4 * p, chunk(bb), :] = y[p][1]
                toks.append(fence(z))
            _fft16([(z[0, a, chunk(bb), :], z[1, a, chunk(bb), :]) for a in range(16)], sign, emit)
            return toks

        ys = {}

        def fwd(g, k2, toks):
            z = zs[g]
            ur, ui = z[0, k2, 0:64, :], z[1, k2, 0:64, :]
            tr, ti = _twiddle((z[0, k2, 64:128, :], z[1, k2, 64:128, :]), k2, 32, -1)
            for hf in range(2):
                v = _ilv(ur + tr, ui + ti) if hf == 0 else _ilv(ur - tr, ui - ti)
                lhs = _with_tokens(emat[k2 + 16 * hf], toks if hf == 0 else None)
                xr, xi = _dilv(_dot(_bf(lhs), v.astype(bf16)))
                ys["x", 16 * g + k2] = xr
                wr = wf[g, pl.ds(k2 * WPITCH + hf, 64, stride=2), :]
                wi = wf[g + 3, pl.ds(k2 * WPITCH + hf, 64, stride=2), :]
                ys[g, k2, hf] = _ilv(xr * wr - xi * wi, xr * wi + xi * wr).astype(bf16)

        def inv(g, k2, toks):
            z = zs[g]
            t0 = _dot(_bf(_with_tokens(emat[32 + k2], toks)), ys.pop((g, k2, 0)))
            t1 = _dot(_bf(emat[48 + k2]), ys.pop((g, k2, 1)))
            z[0, k2, 0:64, :], z[1, k2, 0:64, :] = _dilv(t0 + t1)
            z[0, k2, 64:128, :], z[1, k2, 64:128, :] = _twiddle(_dilv(t0 - t1), k2, 32, 1)

        units = [(g, k2) for g in range(3) for k2 in range(16)]
        toks = None
        lag = CFG["inv_lag"]
        for i in range(len(units) + lag):
            if i < len(units):
                fwd(*units[i], toks)
            if i >= lag:
                inv(*units[i - lag], toks if i >= len(units) else None)
            toks = []
            if i in CFG["fwd_at"]:
                toks = radix(2, CFG["fwd_at"].index(i), -1)
            if i in CFG["inv_at"]:
                back, r = CFG["rel"]
                z0[1, zero, 128:ZPITCH, :] = ys["x", min(i - back, 47)][8 * r:8 * r + 8]
                toks = radix(0, CFG["inv_at"].index(i), 1)
            toks = {j: pltpu.bitcast(t, u32) for j, t in zip(CFG["tok_pos"], toks)}

    def dinv_thunks(bb, finish):
        st = {}

        def part(g):
            def run():
                z = zs[g]
                ys = [(z[0, a, chunk(bb), :], z[1, a, chunk(bb), :]) for a in range(16)]
                if g > 0:
                    ys = _fft16(ys, 1)
                tr = jnp.concatenate([y[0] for y in ys], axis=0)
                ti = jnp.concatenate([y[1] for y in ys], axis=0)
                if g == 0:
                    lane = lax.broadcasted_iota(jnp.int32, (128, 128), 1)
                    v = jnp.where(lane <= 64, tr, pltpu.roll(ti, 64, 1))
                    st[0] = _dot(v.astype(bf16), _bf(small[7]))
                else:
                    k, ki, kr = [_dot(v.astype(bf16), _bf(small[5 + 3 * g + i]))
                                 for i, v in enumerate((tr + _mu() * ti, ti, tr))]
                    st[2 * g - 1], st[2 * g] = k + ki, k + kr
            return run

        def fin():
            p0, p1, q1, p2, q2 = [st[j] for j in range(5)]
            t = p1 + p2
            m, n = p0 - 0.25 * t, R5_D * (p1 - p2)
            e1, e2 = m + n, m - n
            o1, o2 = q1 + R5_R * q2, R5_R * q1 - q2
            y = jnp.concatenate([p0 + t, e1 - o1, e2 - o2, e2 + o2, e1 + o1], axis=1)
            finish(xb[:, chunk(bb), :].reshape(128, DM) + y)
        return [part(0), part(1), part(2), fin]

    def out_copy(bb):
        return pltpu.make_async_copy(xin.at[:, bb], out_hbm.at[:, bb], osem.at[bb])

    def layer(li, carry0):
        if full or CFG["only"] == "group":
            _loop("step", 0, 16, group, mem_ref[...].astype(f32))
        if full or CFG["only"] == "spec":
            if full:
                @pl.when(li == 0)
                def _():
                    for cp in cp_rest[1:]:
                        cp.wait()
            _loop("post", 0, 4, post, 0)

            with jax.named_scope("spectral"):
                spectral(li >> 1)
        if not full and CFG["only"] != "out":
            return carry0

        def run_chunks(th, order, lag):
            seq = [t[g] for t in th for g in order]
            for i in range(len(seq) + lag):
                if i < len(seq):
                    seq[i]()
                if i >= lag and (i - lag) % 3 == 2:
                    th[(i - lag) // 3][3]()

        @pl.when(li == 0)
        def _():
            with jax.named_scope("dinv_tails"):
                run_chunks([dinv_thunks(4 * u + 3, functools.partial(
                    lambda u, x: set_input(4 * u + 3, _round_bf16(x), u), u))
                    for u in range(4)],
                    *CFG["tails_order"])

            def batch(it, carry):
                bb = body_chunk(it)
                side = dinv_thunks(bb, lambda x: set_input(bb, _round_bf16(x), None))
                for k, f in enumerate(batch_thunks(it, CFG["two_inner"], CFG["two_outer"])):
                    f()
                    for at, g in zip(CFG["dinv_at"], CFG["dinv_order"] + (3,)):
                        if at == k:
                            side[g]()
                return carry
            _loop("batch", 0, 12, batch, 0, unroll=2)

        @pl.when(li == 1)
        def _():
            with jax.named_scope("dinv_out"):
                def store_out(bb, x):
                    xin[:, bb] = x.reshape(16, 8, DM).astype(bf16)
                    out_copy(bb).start()
                run_chunks([dinv_thunks(bb, functools.partial(store_out, bb)) for bb in range(16)],
                           *CFG["out_order"])
                for bb in range(16):
                    out_copy(bb).wait()
        return carry0

    if CFG["only"] != "pro":
        lax.fori_loop(0, 2, layer, 0)
    if CFG["only"] in ("pro", "out"):
        zero = zero_ref[0]
        xin[0, 0, :, 0:128] = (qb[zero, 0, 0] + wf[zero, 0:8, :] + xa[zero, 0:8, 0:128]).astype(bf16) + ws[zero, 0, 0:8, :]
        out_copy(0).start()
        out_copy(0).wait()
        for cp in cp_rest[1:] if full else ():
            cp.wait()


@jax.jit
def pallas_interleave_layers__memory_aug_recurrent_mem_tr__spectral_gfnet__prompt_kernel(
    A_x, A_mem0, A_Wq, A_Wk, A_Wv, A_Wo, A_seg_len, B_x, B_w_r, B_w_i,
):
    assert A_x.shape == (1, S, DM) and A_mem0.shape == (1, MEM, DM)
    small, emat = _tables()
    hbm = pl.BlockSpec(memory_space=pltpu.HBM)
    out = pl.pallas_call(
        _kernel,
        out_shape=jax.ShapeDtypeStruct((16, 16, 8, DM), bf16),
        in_specs=[hbm] * 10,
        out_specs=hbm,
        scratch_shapes=[
            pltpu.VMEM((16, 16, 8, DM), bf16),
            pltpu.VMEM((33, 128, DM), f32),
            pltpu.VMEM((16, 128, DM), f32),
            pltpu.VMEM((16, 8, DM), f32),
            pltpu.VMEM((12, 2, 320, 8, DH), bf16),
            pltpu.VMEM((13, 8 * HPITCH, 128), u32),
            pltpu.VMEM((13, 8 * HPITCH, 128), u32),
            pltpu.VMEM((5, H * DH + 512, 128), bf16),
            pltpu.VMEM((19, 10, 128, 128), bf16),
            pltpu.VMEM((16, 4, 96, 8, 128), f32),
            pltpu.VMEM((53, 64, 128), u32),
            pltpu.VMEM((2, 16, ZPITCH, 128), f32),
            pltpu.VMEM((2, 16, ZPITCH, 128), f32),
            pltpu.VMEM((2, 16, ZPITCH, 128), f32),
            pltpu.VMEM((6, 16 * WPITCH + 32, 128), f32),
            pltpu.VMEM((9, DF, 512), bf16),
            pltpu.VMEM((4, 328, 128), f32),
            pltpu.VMEM((14, 64, 128), u32),
            pltpu.VMEM((64, 64, 128), u32),
            pltpu.VMEM((80, 80), f32),
            pltpu.VMEM((MEM, DM), bf16),
            pltpu.SMEM((1,), jnp.int32),
            pltpu.SemaphoreType.DMA((47,)),
            pltpu.SemaphoreType.DMA((16,)),
        ],
        compiler_params=pltpu.CompilerParams(vmem_limit_bytes=120 * 1024 * 1024,
                                             disable_semaphore_checks=True),
    )(
        A_x.reshape(16, 16, 8, DM), A_mem0.reshape(MEM, DM),
        *[w.reshape(2, 320, H, DH) for w in (A_Wq, A_Wk, A_Wv)], A_Wo.reshape(H * DH, DM), B_w_r.T, B_w_i.T,
        jnp.asarray(small), jnp.asarray(emat),
    )
    return out.reshape(1, S, DM)
```

```python
import functools
import math

import jax
import jax.numpy as jnp
import numpy as np
from jax import lax
import jax.experimental.pallas as pl
import jax.experimental.pallas.tpu as pltpu

f32, bf16, u32 = jnp.float32, jnp.bfloat16, jnp.uint32

S, DM, H, DH, MEM, SEG = 2048, 640, 32, 128, 8, 32
NPAIR = H // 2
DF = DM // 2 + 1
EPS = 1e-5
WPITCH = 132
HPITCH = 164
ZPITCH = 136

S1 = math.sin(2 * math.pi / 5)
R5_D = (math.cos(2 * math.pi / 5) - math.cos(4 * math.pi / 5)) / 2
R5_R = math.sin(4 * math.pi / 5) / S1


def _to_bf16_bits(a):
    u = np.ascontiguousarray(a, dtype=np.float32).view(np.uint32).astype(np.uint64)
    return ((u + 0x7FFF + ((u >> 16) & 1)) >> 16).astype(np.uint32)


def _pack_rows(a):
    b = _to_bf16_bits(a)
    return b[..., 0::2, :] | (b[..., 1::2, :] << 16)


@functools.lru_cache(maxsize=None)
def _tables():
    b = np.arange(128)
    l0 = np.arange(0, DF, 5)
    l1 = np.concatenate([np.arange(1, 320, 5), np.arange(4, 320, 5)])
    l2 = np.concatenate([np.arange(2, 320, 5), np.arange(3, 320, 5)])
    sg = np.concatenate([np.ones(64), -np.ones(64)])

    def th(l):
        return 2 * np.pi * ((b[:, None] * l[None, :]) % DM) / DM

    sc = 1.0 / (S * DM)
    fw = np.zeros((7, 128, 128))
    iw = np.zeros((7, 128, 128))
    t = th(l0)
    cl = np.full((128, 1), 2.0)
    cl[0] = cl[64] = 1.0
    fw[0] = np.concatenate([np.cos(t), -np.sin(t[:, 1:64])], axis=1)
    iw[0] = cl * sc * fw[0].T
    mu = S1 * sg
    for g, l in ((1, l1), (2, l2)):
        t = th(l)
        c, s = np.cos(t), np.sin(t)
        fw[3 * g - 2:3 * g + 1] = c, -mu * s - c, mu * c - s
        iw[3 * g - 2:3 * g + 1] = [2 * sc * m.T for m in (c, -s - mu * c, mu * s - c)]
    n = np.arange(64)
    order = np.concatenate([np.concatenate([np.arange(8) + 8 * j, np.arange(8) + 8 * j + 64])
                            for j in range(8)])
    e = np.zeros((2, 32, 128, 128))
    for k2 in range(32):
        t = 2 * np.pi * (((32 * n[:, None] + k2) * n[None, :]) % S) / S
        er, ei = np.cos(t), -np.sin(t)
        m = np.block([[er, -ei], [ei, er]])[order][:, order]
        e[0, k2], e[1, k2] = m, m.T
    small = np.concatenate([_pack_rows(fw), _pack_rows(iw)], axis=0)
    return small, _pack_rows(e).reshape(64, 64, 128)


def _loop(name, lo, hi, body, init, **kw):
    with jax.named_scope(name):
        return lax.fori_loop(lo, hi, body, init, **kw)


def _bf(x):
    return pltpu.bitcast(x, bf16)


def _dot(a, b):
    return jnp.dot(a, b, preferred_element_type=f32)


def _round_bf16(x):
    return x.astype(bf16).astype(f32)


def _layernorm(x):
    m = jnp.mean(x, axis=-1, keepdims=True)
    xc = x - m
    v = jnp.mean(xc * xc, axis=-1, keepdims=True)
    return xc * lax.rsqrt(v + EPS)


def _fft4(x, sign):
    (ar, ai), (br, bi), (cr, ci), (dr, di) = x
    t0r, t0i, t1r, t1i = ar + cr, ai + ci, ar - cr, ai - ci
    t2r, t2i, t3r, t3i = br + dr, bi + di, br - dr, bi - di
    y0, y2 = (t0r + t2r, t0i + t2i), (t0r - t2r, t0i - t2i)
    p, q = (t1r + t3i, t1i - t3r), (t1r - t3i, t1i + t3r)
    return [y0, p, y2, q] if sign < 0 else [y0, q, y2, p]


def _twiddle(z, n, period, sign):
    zr, zi = z
    n = n % period
    if n == 0:
        return z
    if 4 * n == period:
        return (-zi, zr) if sign > 0 else (zi, -zr)
    c, s = math.cos(2 * math.pi * n / period), sign * math.sin(2 * math.pi * n / period)
    if (8 * n) % period == 0:
        a, d = zr + zi, zr - zi
        if c * s > 0:
            return (d * c, a * c)
        return (a * c, d * s)
    return (zr * c - zi * s, zr * s + zi * c)


STRASSEN_LHS = (((0, 0, 1), (1, 1, 1)), ((1, 0, 1), (1, 1, 1)), ((0, 0, 1),), ((1, 1, 1),),
                ((0, 0, 1), (0, 1, 1)), ((1, 0, 1), (0, 0, -1)), ((0, 1, 1), (1, 1, -1)))
STRASSEN_RHS = (((0, 0, 1), (1, 1, 1)), ((0, 0, 1),), ((0, 1, 1), (1, 1, -1)), ((1, 0, 1), (0, 0, -1)),
                ((1, 1, 1),), ((0, 0, 1), (0, 1, 1)), ((1, 0, 1), (1, 1, 1)))
STRASSEN_OUT = ((((0, 0), 1), ((1, 1), 1)), (((1, 0), 1), ((1, 1), -1)), (((0, 1), 1), ((1, 1), 1)),
                (((0, 0), 1), ((1, 0), 1)), (((0, 0), -1), ((0, 1), 1)), (((1, 1), 1),), (((0, 0), 1),))
WS_SLOT = {0: 0, 2: 1, 3: 2, 5: 3, 6: 4}


def _operand(terms, block):
    x = block(*terms[0][:2])
    if len(terms) == 1:
        return x
    x, y = x.astype(f32), block(*terms[1][:2]).astype(f32)
    return x + y if terms[1][2] > 0 else x - y


def _accumulate(acc, key, y, sign):
    if key not in acc:
        acc[key] = y if sign > 0 else -y
    else:
        acc[key] = acc[key] + y if sign > 0 else acc[key] - y


def _mu():
    lane = lax.broadcasted_iota(jnp.int32, (1, 128), 1)
    return jnp.where(lane < 64, S1, -S1).astype(f32)


def _ilv(r, i):
    n = r.shape[0] // 8
    return jnp.concatenate([r.reshape(n, 8, 128), i.reshape(n, 8, 128)], axis=1).reshape(16 * n, 128)


def _dilv(x):
    n = x.shape[0] // 16
    x = x.reshape(n, 16, 128)
    return x[:, :8].reshape(8 * n, 128), x[:, 8:].reshape(8 * n, 128)


def _with_tokens(x, toks):
    if not toks:
        return x
    return jnp.concatenate(
        [x[8 * j:8 * j + 8] | toks[j] if j in toks else x[8 * j:8 * j + 8]
         for j in range(x.shape[0] // 8)], axis=0)


def _fft16(x, sign, emit=None):
    cols = [_fft4([x[4 * j + r] for j in range(4)], sign) for r in range(4)]
    out = [None] * 16
    for q in range(4):
        y = _fft4([_twiddle(cols[r][q], r * q, 16, sign) for r in range(4)], sign)
        for p in range(4):
            out[q + 4 * p] = y[p]
        if emit is not None:
            emit(q, y)
    return out


CFG = dict(
    steps=((4.5, 16.5, 6, 4, 0, 8), (5, 16.5, 5, 7, 8, 12), (5, 16.5, 6, 6, 8, 12), (5, 16.5, 8, 7, 8, 0)),
    moves=(((125, 127), (15, 14), (34, 35), (91, 89), (11, 14), (20, 18), (1, 0), (107, 106)),
           ((9, 11), (134, 133), (129, 126), (83, 85)), ((96, 94), (6, 5)), ((33, 34),)),
    pro_inner=(4, 2, 5, 8, 0, 3, 6, 7, 9, 10, 1),
    pro_outer=((2, 2), (5, 3), (1, 0), (0, None), (4, None), (3, None), (6, 1)),
    pro_nre=13, re_pos=(2, 2, 5, 5), ln_at=(11, 17, 23, 27), ln_at2=(3, 4, 6, 7, 9, 10, 12, 13),
    perm_at=tuple(range(10, 22)),
    ws_split=4, ws_at=(15, 15, 16, 16, 17, 18, 18, 19, 20, 20, 21, 21, 22, 23, 23, 24),
    post_passes=((0, 1), (2, 3), (4, 5), (6, 7)), post_dl=20,
    post_order=(0, 1, 6, 3, 4, 2, 8, 5, 7, 9, 10, 11), post_at=(26, 38, 58, 96),
    fwd_at=(7, 8, 9, 10, 12, 13, 14, 16, 17, 18, 20, 21, 22, 24, 25, 26),
    inv_at=tuple(range(28, 44)), inv_lag=4, tok_pos=(4, 5, 6, 7), rel=(0, 1),
    tails_order=((1, 2, 0), 5), out_order=((1, 2, 0), 5),
    two_inner=(5, 4, 2, 8, 0, 3, 6, 7, 9, 10, 1),
    two_outer=((2, 2), (5, 3), (1, None), (0, None), (4, 0), (3, None), (6, 1)),
    dinv_at=(0, 0, 1, 1), dinv_order=(2, 1, 0),
    only=None)


def _step_order(params, moves):
    lat_s, lat_pv, lat_wo, v_delay, n_first, n_last = params
    keyed = []
    for p in range(NPAIR):
        keyed += [(4 * p + 2 * m + e, ("proj", p, m, e)) for m in range(2) for e in range(2)]
        keyed += [(4 * p + 3.5 + v_delay, ("proj", p, 2, e)) for e in range(2)]
    bulk = [x for _, x in sorted(keyed, key=lambda kv: kv[0])]
    first, bulk = bulk[:n_first], bulk[n_first:]
    t, nwo, seq, ready = float(n_first), 0, [], []
    pend = [(t + lat_s, "scores", p) for _, p, m, e in first if m == 1 and e == 1]
    while nwo < H - n_last or pend:
        pend.sort(key=lambda x: (x[0], x[1] == "pv", x[2]))
        if pend and pend[0][0] <= t:
            _, kind, p = pend.pop(0)
            seq.append((kind, p, 0, 0))
            if kind == "scores":
                pend.append((t + lat_pv, "pv", p))
            else:
                ready += [(t + lat_wo, p, e) for e in range(2)]
            t += 0.5
        elif bulk:
            seq.append(bulk.pop(0))
            t += 1
            if seq[-1][2:] == (1, 1):
                pend.append((t + lat_s, "scores", seq[-1][1]))
        elif ready and ready[0][0] <= t and nwo < H - n_last:
            _, p, e = ready.pop(0)
            seq.append(("wo", p, 0, e))
            t += 1
            nwo += 1
        else:
            t += 0.5
    for i, j in moves:
        seq.insert(j, seq.pop(i))
    return first, seq, [2 * p + e for _, p, e in ready]


def _kernel(x_hbm, mem_hbm, wq_hbm, wk_hbm, wv_hbm, wo_hbm, wr_hbm, wi_hbm,
            small_hbm, e_hbm, out_hbm,
            xin, xa, xb, to, raw, wa, wb, wo_t, ws, qb, hl, z0, z1, z2, wf,
            wri, wtmp, small, emat, fill_ref, mem_ref, zero_ref, sem, osem):
    zs = (z0, z1, z2)
    w_hbm = (wq_hbm, wk_hbm, wv_hbm)

    def body_chunk(i):
        return 4 * (i & 3) + (i >> 2)

    def cp_w(i):
        src = w_hbm[i >> 2].at[:, :, pl.ds(8 * (i & 3), 8), :] if isinstance(i, int) else raw.at[i]
        return pltpu.make_async_copy(src, raw.at[i], sem.at[i])

    def cp_x(bb):
        return pltpu.make_async_copy(x_hbm.at[:, bb], xin.at[:, bb], sem.at[12 + bb])

    def cp_f(i):
        src = ((wr_hbm, wi_hbm)[i >> 2].at[:, pl.ds(512 * (i & 3), 512)]
               if isinstance(i, int) else wri.at[i])
        return pltpu.make_async_copy(src, wri.at[i], sem.at[36 + i])

    def cp_wo(i):
        rows = pl.ds(pl.multiple_of(512 * i, 512), 512)
        return [pltpu.make_async_copy(wo_hbm.at[rows, pl.ds(128 * j, 128)], wo_t.at[j, rows], sem.at[28 + i])
                for j in range(5)]

    cp_rest = [pltpu.make_async_copy(mem_hbm, mem_ref, sem.at[46]),
               pltpu.make_async_copy(small_hbm, small, sem.at[44]),
               pltpu.make_async_copy(e_hbm, emat, sem.at[45])]

    full = CFG["only"] in (None, "pro")
    for u in range(4 if full else 0):
        cp_x(4 * u + 3).start()
    if full:
        cp_w(0).start()
    for i in range(12 if full else 0):
        if i < 11:
            cp_w(i + 1).start()
        cp_x(body_chunk(i)).start()
        if 3 <= i < 11:
            cp_f(i - 3).start()
            for cp in cp_wo(i - 3):
                cp.start()
    for cp in cp_rest if full else ():
        cp.start()

    zero_ref[0] = 0

    r = lax.broadcasted_iota(jnp.int32, (80, 80), 0)
    c = lax.broadcasted_iota(jnp.int32, (80, 80), 1)

    def head(i):
        return jnp.where(i < 64, i // 32, (i - 64) // 8)

    def pos(i):
        return jnp.where(i < 64, i % 32, 32 + (i - 64) % 8)

    ok = (pos(r) < MEM) | (pos(r) >= pos(c))
    fill_ref[...] = jnp.where(head(r) == head(c), jnp.where(ok, 0.0, -1e9), -jnp.inf).astype(f32)
    wtmp[:, 320:328, :] = jnp.zeros((4, 8, 128), f32)
    xa[32, 0:8, 0:128] = jnp.zeros((8, 128), f32)
    ws[18, 0, 0:16, :] = jnp.zeros((16, 128), bf16)
    wa[12, 0:8, :] = jnp.zeros((8, 128), u32)
    wb[12, 0:8, :] = jnp.zeros((8, 128), u32)
    wf[5, 16 * WPITCH:16 * WPITCH + 8, :] = jnp.zeros((8, 128), f32)
    for z in zs:
        z[0, 0, 128:ZPITCH, :] = jnp.zeros((8, 128), f32)

    def chunk(bb):
        if isinstance(bb, int):
            return slice(8 * bb, 8 * bb + 8)
        return pl.ds(pl.multiple_of(8 * bb, 8), 8)

    def set_input(bb, x, tail_u, a0=0):
        n = x.shape[0] // 8
        xa[a0:a0 + n, chunk(bb), :] = x.reshape(n, 8, DM)
        y = _layernorm(x)
        if tail_u is None:
            xa[16 + a0:16 + a0 + n, chunk(bb), :] = y.reshape(n, 8, DM)
        else:
            blk = [[y[32 * r:32 * r + 32, 128 * kt:128 * kt + 128] for kt in range(5)] for r in range(4)]
            ops = []
            for outer in STRASSEN_LHS:
                sub = [[_operand(outer, lambda rr, kk: blk[2 * rr + r][2 * kk + k]) for k in range(2)]
                       for r in range(2)]
                ops += [_operand(inner, lambda r, k: sub[r][k]) for inner in STRASSEN_LHS]
            for i, v in enumerate(ops + [blk[r][4] for r in range(4)]):
                hl[i, 16 * tail_u:16 * tail_u + 16, :] = pltpu.bitcast(v.astype(bf16), u32)

    def load_x(bb, a0=0, n=16):
        return xin[a0:a0 + n, bb].astype(f32).reshape(8 * n, DM)

    def wtile(cid, j, e):
        w = (wa, wb)[e]
        return jnp.concatenate([w[cid, (4 * hf + j) * HPITCH:(4 * hf + j) * HPITCH + 160, :]
                                for hf in range(2)], axis=0)

    def relayout(i, cid, e):
        for r in range(4 * i, 4 * i + 4):
            a, b = [pltpu.bitcast(raw[cid, :, d].reshape(16, 128), u32) for d in (2 * r, 2 * r + 1)]
            v = (a & 0xFFFF) | (b << 16) if e == 0 else (a >> 16) | (b & jnp.uint32(0xFFFF0000))
            (wa, wb)[e][cid, pl.ds(r, 8, stride=HPITCH), :] = v

    def batch_thunks(cid, inner_order, outer_order):
        qv = qb.at[:, :, pl.ds(8 * cid, 8)]

        def unit(e):
            c = {}
            left = {(r, n): (5, 3, 3, 5)[2 * (r >> 1) + (n >> 1)] for r in range(4) for n in range(4)}

            def w(kt, n):
                return _bf(wtile(cid, n, e)[64 * kt:64 * kt + 64])

            def add_out(blk, y, sign):
                _accumulate(c, blk, y, sign)
                left[blk] -= 1
                if left[blk] == 0:
                    r, n = blk
                    y = c.pop(blk).reshape(4, 4, 8, 128)
                    for u in range(4):
                        qv[4 * r:4 * r + 4, u, 2 * n + e] = y[u]

            def outer(io, k4):
                p = {}
                todo = {(0, 0): 4, (0, 1): 2, (1, 0): 2, (1, 1): 4}

                @functools.lru_cache(maxsize=None)
                def sub(k, n):
                    return _operand(STRASSEN_RHS[io], lambda kk, nn: w(2 * kk + k, 2 * nn + n))

                def thunk(items):
                    def run(toks=None):
                        for i in items:
                            if i >= 7:
                                r, n = k4[i - 7]
                                add_out((r, n), _dot(_bf(_with_tokens(hl[49 + r], toks)), w(4, n)), 1)
                                toks = None
                                continue
                            rhs = _operand(STRASSEN_RHS[i], sub).astype(bf16)
                            y = _dot(_bf(_with_tokens(hl[7 * io + i], toks)), rhs)
                            toks = None
                            for blk, sign in STRASSEN_OUT[i]:
                                _accumulate(p, blk, y, sign)
                                todo[blk] -= 1
                                if todo[blk] == 0:
                                    for (rr, nn), sg in STRASSEN_OUT[io]:
                                        add_out((2 * rr + blk[0], 2 * nn + blk[1]), p[blk], sg)
                    return run
                items = [i for i in inner_order if i < 7 + len(k4)]
                return [thunk(items[:len(items) // 2]), thunk(items[len(items) // 2:])]
            out = []
            for io, q in outer_order:
                out += outer(io, [] if q is None else
                             [(2 * (q >> 1) + (j >> 1), 2 * (q & 1) + (j & 1)) for j in range(4)])
            return out
        return unit(0) + unit(1)

    def wperm_thunks(piece, j):
        m = (piece >> 2) & 1
        wt = wtmp.at[j]

        def load():
            wt[0:DF, :] = wri[piece, :, 128 * j:128 * j + 128].astype(f32)

        def one(g):
            def run():
                if g == 0:
                    t = jnp.concatenate([wt[pl.ds(0, 64, stride=5), :], wt[320:328, :],
                                         jnp.zeros((56, 128), f32)], axis=0)
                else:
                    t = jnp.concatenate([wt[pl.ds(g, 64, stride=5), :],
                                         wt[pl.ds(5 - g, 64, stride=5), :]], axis=0)
                y = t.T
                sub = wf.at[3 * m + g, pl.ds(pl.multiple_of((piece & 3) * 32, 32), 16 * WPITCH - 96)]
                for k in range(8):
                    for hf in range(2):
                        sub[pl.ds(8 * j + k + 8 * hf * WPITCH, 8, stride=WPITCH), :] = (
                            y[16 * k + 8 * hf:16 * k + 8 * hf + 8])
            return run
        return [load] + [one(g) for g in range(3)]

    def half_pass(cid, half, fill, zero, timed=()):
        nre = CFG["pro_nre"]
        toks = None
        for k, f in enumerate(batch_thunks(cid, CFG["pro_inner"], CFG["pro_outer"])[14 * half:14 * half + 14]):
            f(toks)
            toks = {}
            for n, f in enumerate(f for at, f in timed if at == k):
                toks[(0, 4, 1, 6)[n]] = f()
            if fill is not None:
                for n, r in enumerate(r for r in range(40) if r * nre // 40 == k):
                    relayout(r, fill, 1 - half)
                    toks[CFG["re_pos"][n]] = (wb, wa)[half][12 + zero, 0:8, :]

    def ln_parts(bb, zero):
        def part(j):
            set_input(bb, load_x(bb, 4 * j, 4), None, 4 * j)
            return pltpu.bitcast(xa[32 + zero, 0:8, 0:128], u32)
        return [functools.partial(part, j) for j in range(4)]

    def perm_parts(piece, zero):
        def part(fs):
            for f in fs:
                f()
            return pltpu.bitcast(wf[5 + zero, 16 * WPITCH:16 * WPITCH + 8, :], u32)
        out = []
        for j in range(4):
            th = wperm_thunks(piece, j)
            out += [functools.partial(part, th[0:2]), functools.partial(part, th[2:3]),
                    functools.partial(part, th[3:4])]
        return out

    def ws_parts(piece, zero):
        nr = 128 // CFG["ws_split"]

        src = wo_t.at[:, pl.ds(pl.multiple_of(512 * piece, 512), 512)]
        dst = ws.at[pl.ds(2 * piece, 2)]

        def part(pp, np_, r0):
            def tile(k, n):
                lo = 256 * pp + 128 * k + r0
                return src[2 * np_ + n, lo:lo + nr, :]
            for i, slot in WS_SLOT.items():
                dst[pp, 5 * np_ + slot, r0:r0 + nr, :] = _operand(STRASSEN_RHS[i], tile).astype(bf16)
            return pltpu.bitcast(ws[18 + zero, 0, 0:16, :], u32)
        return [functools.partial(part, pp, np_, r0)
                for pp in range(2) for np_ in range(2) for r0 in range(0, 128, nr)]

    def pro0():
        for u in range(4):
            cp_x(4 * u + 3).wait()
        for u in range(4):
            set_input(4 * u + 3, load_x(4 * u + 3), u)
        cp_w(0).wait()
        zero = zero_ref[0]
        for i in range(40):
            relayout(i, 0, 0)
        half_pass(0, 0, zero, zero)

    def pro1(it, carry):
        bb = jnp.where(it == 0, 3, body_chunk(it - 1))
        with jax.named_scope("pro1_wait"):
            cp_w(it + 1).wait()

            @pl.when(it >= 1)
            def _():
                cp_x(bb).wait()

            @pl.when(it >= 3)
            def _():
                cp_f(it - 3).wait()
                for cp in cp_wo(it - 3):
                    cp.wait()
        piece = jnp.where(it >= 3, it - 3, 8)
        zero = it >> 4
        timed = sorted(list(zip(CFG["ln_at"], ln_parts(bb, zero)))
                       + list(zip(CFG["ws_at"], ws_parts(piece, zero)))
                       + list(zip(CFG["perm_at"], perm_parts(piece, zero))), key=lambda x: x[0])
        half_pass(it, 1, it + 1, zero, [x for x in timed if x[0] < 14])
        half_pass(it + 1, 0, it + 1, zero, [(k - 14, f) for k, f in timed if k >= 14])
        return carry

    def pro2():
        cp_x(body_chunk(10)).wait()
        cp_x(body_chunk(11)).wait()
        cp_rest[0].wait()
        zero = zero_ref[0]
        half_pass(11, 1, None, zero, list(zip(
            CFG["ln_at2"], ln_parts(body_chunk(10), zero) + ln_parts(body_chunk(11), zero))))

    if full:
        with jax.named_scope("pro0"):
            pro0()
        _loop("pro1", 0, 11, pro1, 0)
        with jax.named_scope("pro2"):
            pro2()

    scale = DH ** -0.5

    def wo_dot(hh, oo):
        return [_dot(oo, wo_t[j, 128 * hh:128 * hh + 128, :]) for j in range(5)]

    def addl(acc, res):
        return res if acc is None else [a + b for a, b in zip(acc, res)]

    def group(g, mem):
        for ph in range(4):
            h = jnp.concatenate([mem, xa[16 + g, 32 * ph:32 * ph + 24, :]], axis=0).astype(bf16)
            pr, sm, oos = {}, {}, {}

            def stacked(p, m):
                tails = [qb[g, ph, 32 * m + 2 * p + e] for e in range(2)]
                return jnp.concatenate([pr[p, m, 0], pr[p, m, 1]] + tails, axis=0).astype(bf16)

            def scores(p):
                sc = lax.dot_general(stacked(p, 0), stacked(p, 1), (((1,), (1,)), ((), ())),
                                     preferred_element_type=f32)
                fill = fill_ref[...]
                sc = jnp.where(fill == 0.0, sc * scale, fill)
                mx = jnp.max(sc, axis=-1, keepdims=True)
                e = jnp.exp(sc - mx)
                rl = pl.reciprocal(jnp.sum(e, axis=-1, keepdims=True), approx=True)
                sm[p] = (e * rl).astype(bf16)

            def pv(p):
                o = _dot(sm[p], stacked(p, 2))
                for e in range(2):
                    qb[g, ph, 2 * p + e] = o[64 + 8 * e:72 + 8 * e]
                    oos[2 * p + e] = o[32 * e:32 * e + 32].astype(bf16)

            first, seq, last = _step_order(CFG["steps"][ph], CFG["moves"][ph])
            for kt in range(5):
                for _, p, m, e in first:
                    w = wtile(4 * m + (p >> 2), p & 3, e)[64 * kt:64 * kt + 64]
                    y = _dot(h[:, 128 * kt:128 * kt + 128], _bf(w))
                    pr[p, m, e] = y if kt == 0 else pr[p, m, e] + y
            acc = None
            for kind, p, m, e in seq:
                if kind == "proj":
                    pr[p, m, e] = _dot(h, _bf(wtile(4 * m + (p >> 2), p & 3, e)))
                elif kind == "scores":
                    scores(p)
                elif kind == "pv":
                    pv(p)
                else:
                    acc = addl(acc, wo_dot(2 * p + e, oos[2 * p + e]))
            for j in range(5):
                for hh in last:
                    acc[j] = acc[j] + _dot(oos[hh], wo_t[j, 128 * hh:128 * hh + 128, :])
            out = jnp.concatenate(acc, axis=1)
            xa[16 + g, 32 * ph:32 * ph + 24, :] = out[8:32]
            mem = _round_bf16(out[0:8])
        return mem

    def dfwd_thunks(seg, q):
        st = {}
        rows = chunk(q)
        xav, xbv, zv = xa.at[:, seg], xb.at[:, seg], [z.at[:, :, seg] for z in zs]

        def pre():
            o = to[...] if q == 3 else xav[16:32, rows, :]
            x = _round_bf16(xav[0:16, rows, :] + o)
            xbv[:, rows, :] = x
            y = _layernorm(x.reshape(128, DM))
            x0, x1, x2, x3, x4 = [y[:, 128 * a:128 * a + 128] for a in range(5)]
            t1, t2, t3, t4 = x1 + x4, x2 + x3, x1 - x4, x2 - x3
            t = t1 + t2
            m, n = x0 - 0.25 * t, R5_D * (t1 - t2)
            st["u"] = [x0 + t, (m + n, t3 + R5_R * t4), (m - n, R5_R * t3 - t4)]

        def part(g):
            def run():
                if g == 0:
                    pre()
                    u0 = st["u"][0].astype(bf16)
                    zr = _dot(u0, _bf(small[0]))
                    lane = lax.broadcasted_iota(jnp.int32, (128, 128), 1)
                    zi = jnp.where((lane & 63) == 0, 0.0, pltpu.roll(zr, 64, 1))
                else:
                    a, b = st["u"][g]
                    k, kb, ka = [_dot(v.astype(bf16), _bf(small[3 * g - 2 + i]))
                                 for i, v in enumerate((a + b, b, a))]
                    zr, zi = k + kb, ka - _mu() * k
                ys = [(zr[8 * a:8 * a + 8], zi[8 * a:8 * a + 8]) for a in range(16)]
                if g < 2:
                    ys = _fft16(ys, -1)
                for a in range(16):
                    zv[g][0, a, rows, :] = ys[a][0]
                    zv[g][1, a, rows, :] = ys[a][1]
            return run
        return [part(g) for g in range(3)]

    def post(u, carry):
        base = pl.multiple_of(32 * u, 32)
        side = []
        for q in range(4):
            side += dfwd_thunks(pl.ds(base, 32), q)
        side = [side[i] for i in CFG["post_order"]]
        k = 0
        at = list(CFG["post_at"])
        m, due = {}, []
        for prods in CFG["post_passes"]:
            acc = None
            for p in range(NPAIR):
                res = []
                for i in prods:
                    if i == 7:
                        oo = jnp.concatenate([qb[:, u, 2 * p + e].reshape(128, 128) for e in range(2)], axis=1)
                        res.append(_dot(oo.astype(bf16), wo_t[4, 256 * p:256 * p + 256, :]))
                        k += 2
                        continue
                    a = _operand(STRASSEN_LHS[i], lambda r, e: (
                        qb[8 * r:8 * r + 8, u, 2 * p + e].reshape(64, 128))).astype(bf16)
                    for np_ in range(2):
                        if i in WS_SLOT:
                            w = ws[p, 5 * np_ + WS_SLOT[i]]
                        else:
                            kk = 0 if i == 1 else 1
                            w = wo_t[2 * np_ + kk, 256 * p + 128 * kk:256 * p + 128 * kk + 128, :]
                        if due and due[0][0] <= k:
                            w = _bf(_with_tokens(pltpu.bitcast(w, u32), {0: due.pop(0)[1]}))
                        res.append(_dot(a, w))
                    k += 1
                acc = addl(acc, res)
                while at and at[0] <= k:
                    g = CFG["post_order"][len(CFG["post_at"]) - len(at)] % 3
                    at.pop(0)
                    side.pop(0)()
                    if g == 0:
                        due.append((k + CFG["post_dl"],
                                    pltpu.bitcast(z0[0, u >> 2, 128:ZPITCH, :], u32)))
            for i in prods:
                m[i] = [acc.pop(0)] if i == 7 else [acc.pop(0), acc.pop(0)]
        cols = []
        for np_ in range(2):
            m1, m2, m3, m4, m5, m6, m7 = [m[i][np_] for i in range(7)]
            cols.append(jnp.concatenate([m1 + m4 - m5 + m7, m2 + m4], axis=0))
            cols.append(jnp.concatenate([m3 + m5, m1 - m2 + m3 + m6], axis=0))
        to[...] = jnp.concatenate(cols + m[7], axis=1).reshape(16, 8, DM)
        for f in side:
            f()
        return carry

    def spectral(zero):
        def fence(z):
            return z[0, zero, 128:ZPITCH, :]

        def radix(g, bb, sign):
            z = zs[g]
            toks = []

            def emit(q, y):
                for p in range(4):
                    z[0, q + 4 * p, chunk(bb), :] = y[p][0]
                    z[1, q + 4 * p, chunk(bb), :] = y[p][1]
                toks.append(fence(z))
            _fft16([(z[0, a, chunk(bb), :], z[1, a, chunk(bb), :]) for a in range(16)], sign, emit)
            return toks

        ys = {}

        def fwd(g, k2, toks):
            z = zs[g]
            ur, ui = z[0, k2, 0:64, :], z[1, k2, 0:64, :]
            tr, ti = _twiddle((z[0, k2, 64:128, :], z[1, k2, 64:128, :]), k2, 32, -1)
            for hf in range(2):
                v = _ilv(ur + tr, ui + ti) if hf == 0 else _ilv(ur - tr, ui - ti)
                lhs = _with_tokens(emat[k2 + 16 * hf], toks if hf == 0 else None)
                xr, xi = _dilv(_dot(_bf(lhs), v.astype(bf16)))
                ys["x", 16 * g + k2] = xr
                wr = wf[g, pl.ds(k2 * WPITCH + hf, 64, stride=2), :]
                wi = wf[g + 3, pl.ds(k2 * WPITCH + hf, 64, stride=2), :]
                ys[g, k2, hf] = _ilv(xr * wr - xi * wi, xr * wi + xi * wr).astype(bf16)

        def inv(g, k2, toks):
            z = zs[g]
            t0 = _dot(_bf(_with_tokens(emat[32 + k2], toks)), ys.pop((g, k2, 0)))
            t1 = _dot(_bf(emat[48 + k2]), ys.pop((g, k2, 1)))
            z[0, k2, 0:64, :], z[1, k2, 0:64, :] = _dilv(t0 + t1)
            z[0, k2, 64:128, :], z[1, k2, 64:128, :] = _twiddle(_dilv(t0 - t1), k2, 32, 1)

        units = [(g, k2) for g in range(3) for k2 in range(16)]
        toks = None
        lag = CFG["inv_lag"]
        for i in range(len(units) + lag):
            if i < len(units):
                fwd(*units[i], toks)
            if i >= lag:
                inv(*units[i - lag], toks if i >= len(units) else None)
            toks = []
            if i in CFG["fwd_at"]:
                toks = radix(2, CFG["fwd_at"].index(i), -1)
            if i in CFG["inv_at"]:
                back, r = CFG["rel"]
                z0[1, zero, 128:ZPITCH, :] = ys["x", min(i - back, 47)][8 * r:8 * r + 8]
                toks = radix(0, CFG["inv_at"].index(i), 1)
            toks = {j: pltpu.bitcast(t, u32) for j, t in zip(CFG["tok_pos"], toks)}

    def dinv_thunks(bb, finish):
        st = {}

        def part(g):
            def run():
                z = zs[g]
                ys = [(z[0, a, chunk(bb), :], z[1, a, chunk(bb), :]) for a in range(16)]
                if g > 0:
                    ys = _fft16(ys, 1)
                tr = jnp.concatenate([y[0] for y in ys], axis=0)
                ti = jnp.concatenate([y[1] for y in ys], axis=0)
                if g == 0:
                    lane = lax.broadcasted_iota(jnp.int32, (128, 128), 1)
                    v = jnp.where(lane <= 64, tr, pltpu.roll(ti, 64, 1))
                    st[0] = _dot(v.astype(bf16), _bf(small[7]))
                else:
                    k, ki, kr = [_dot(v.astype(bf16), _bf(small[5 + 3 * g + i]))
                                 for i, v in enumerate((tr + _mu() * ti, ti, tr))]
                    st[2 * g - 1], st[2 * g] = k + ki, k + kr
            return run

        def fin():
            p0, p1, q1, p2, q2 = [st[j] for j in range(5)]
            t = p1 + p2
            m, n = p0 - 0.25 * t, R5_D * (p1 - p2)
            e1, e2 = m + n, m - n
            o1, o2 = q1 + R5_R * q2, R5_R * q1 - q2
            y = jnp.concatenate([p0 + t, e1 - o1, e2 - o2, e2 + o2, e1 + o1], axis=1)
            finish(xb[:, chunk(bb), :].reshape(128, DM) + y)
        return [part(0), part(1), part(2), fin]

    def out_copy(bb):
        return pltpu.make_async_copy(xin.at[:, bb], out_hbm.at[:, bb], osem.at[bb])

    def layer(li, carry0):
        if full or CFG["only"] == "group":
            _loop("step", 0, 16, group, mem_ref[...].astype(f32))
        if full or CFG["only"] == "spec":
            if full:
                @pl.when(li == 0)
                def _():
                    for cp in cp_rest[1:]:
                        cp.wait()
            _loop("post", 0, 4, post, 0)

            with jax.named_scope("spectral"):
                spectral(li >> 1)
        if not full and CFG["only"] != "out":
            return carry0

        def run_chunks(th, order, lag):
            seq = [t[g] for t in th for g in order]
            for i in range(len(seq) + lag):
                if i < len(seq):
                    seq[i]()
                if i >= lag and (i - lag) % 3 == 2:
                    th[(i - lag) // 3][3]()

        @pl.when(li == 0)
        def _():
            with jax.named_scope("dinv_tails"):
                run_chunks([dinv_thunks(4 * u + 3, functools.partial(
                    lambda u, x: set_input(4 * u + 3, _round_bf16(x), u), u))
                    for u in range(4)],
                    *CFG["tails_order"])

            def batch(it, carry):
                bb = body_chunk(it)
                side = dinv_thunks(bb, lambda x: set_input(bb, _round_bf16(x), None))
                for k, f in enumerate(batch_thunks(it, CFG["two_inner"], CFG["two_outer"])):
                    f()
                    for at, g in zip(CFG["dinv_at"], CFG["dinv_order"] + (3,)):
                        if at == k:
                            side[g]()
                return carry
            _loop("batch", 0, 12, batch, 0, unroll=2)

        @pl.when(li == 1)
        def _():
            with jax.named_scope("dinv_out"):
                def store_out(bb, x):
                    xin[:, bb] = x.reshape(16, 8, DM).astype(bf16)
                    out_copy(bb).start()
                run_chunks([dinv_thunks(bb, functools.partial(store_out, bb)) for bb in range(16)],
                           *CFG["out_order"])
                for bb in range(16):
                    out_copy(bb).wait()
        return carry0

    if CFG["only"] != "pro":
        lax.fori_loop(0, 2, layer, 0)
    if CFG["only"] in ("pro", "out"):
        zero = zero_ref[0]
        xin[0, 0, :, 0:128] = (qb[zero, 0, 0] + wf[zero, 0:8, :] + xa[zero, 0:8, 0:128]).astype(bf16) + ws[zero, 0, 0:8, :]
        out_copy(0).start()
        out_copy(0).wait()
        for cp in cp_rest[1:] if full else ():
            cp.wait()


@jax.jit
def pallas_interleave_layers__memory_aug_recurrent_mem_tr__spectral_gfnet__prompt_kernel(
    A_x, A_mem0, A_Wq, A_Wk, A_Wv, A_Wo, A_seg_len, B_x, B_w_r, B_w_i,
):
    assert A_x.shape == (1, S, DM) and A_mem0.shape == (1, MEM, DM)
    small, emat = _tables()
    hbm = pl.BlockSpec(memory_space=pltpu.HBM)
    out = pl.pallas_call(
        _kernel,
        out_shape=jax.ShapeDtypeStruct((16, 16, 8, DM), bf16),
        in_specs=[hbm] * 10,
        out_specs=hbm,
        scratch_shapes=[
            pltpu.VMEM((16, 16, 8, DM), bf16),
            pltpu.VMEM((33, 128, DM), f32),
            pltpu.VMEM((16, 128, DM), f32),
            pltpu.VMEM((16, 8, DM), f32),
            pltpu.VMEM((12, 2, 320, 8, DH), bf16),
            pltpu.VMEM((13, 8 * HPITCH, 128), u32),
            pltpu.VMEM((13, 8 * HPITCH, 128), u32),
            pltpu.VMEM((5, H * DH + 512, 128), bf16),
            pltpu.VMEM((19, 10, 128, 128), bf16),
            pltpu.VMEM((16, 4, 96, 8, 128), f32),
            pltpu.VMEM((53, 64, 128), u32),
            pltpu.VMEM((2, 16, ZPITCH, 128), f32),
            pltpu.VMEM((2, 16, ZPITCH, 128), f32),
            pltpu.VMEM((2, 16, ZPITCH, 128), f32),
            pltpu.VMEM((6, 16 * WPITCH + 32, 128), f32),
            pltpu.VMEM((9, DF, 512), bf16),
            pltpu.VMEM((4, 328, 128), f32),
            pltpu.VMEM((14, 64, 128), u32),
            pltpu.VMEM((64, 64, 128), u32),
            pltpu.VMEM((80, 80), f32),
            pltpu.VMEM((MEM, DM), bf16),
            pltpu.SMEM((1,), jnp.int32),
            pltpu.SemaphoreType.DMA((47,)),
            pltpu.SemaphoreType.DMA((16,)),
        ],
        compiler_params=pltpu.CompilerParams(vmem_limit_bytes=120 * 1024 * 1024,
                                             disable_semaphore_checks=True),
    )(
        A_x.reshape(16, 16, 8, DM), A_mem0.reshape(MEM, DM),
        *[w.reshape(2, 320, H, DH) for w in (A_Wq, A_Wk, A_Wv)], A_Wo.reshape(H * DH, DM), B_w_r.T, B_w_i.T,
        jnp.asarray(small), jnp.asarray(emat),
    )
    return out.reshape(1, S, DM)
```

```python
import functools
import math

import jax
import jax.numpy as jnp
import numpy as np
from jax import lax
import jax.experimental.pallas as pl
import jax.experimental.pallas.tpu as pltpu

f32, bf16, u32 = jnp.float32, jnp.bfloat16, jnp.uint32

S, DM, H, DH, MEM, SEG = 2048, 640, 32, 128, 8, 32
NPAIR = H // 2
DF = DM // 2 + 1
EPS = 1e-5
WPITCH = 132
HPITCH = 164
ZPITCH = 136

S1 = math.sin(2 * math.pi / 5)
R5_D = (math.cos(2 * math.pi / 5) - math.cos(4 * math.pi / 5)) / 2
R5_R = math.sin(4 * math.pi / 5) / S1


def _to_bf16_bits(a):
    u = np.ascontiguousarray(a, dtype=np.float32).view(np.uint32).astype(np.uint64)
    return ((u + 0x7FFF + ((u >> 16) & 1)) >> 16).astype(np.uint32)


def _pack_rows(a):
    b = _to_bf16_bits(a)
    return b[..., 0::2, :] | (b[..., 1::2, :] << 16)


@functools.lru_cache(maxsize=None)
def _tables():
    b = np.arange(128)
    l0 = np.arange(0, DF, 5)
    l1 = np.concatenate([np.arange(1, 320, 5), np.arange(4, 320, 5)])
    l2 = np.concatenate([np.arange(2, 320, 5), np.arange(3, 320, 5)])
    sg = np.concatenate([np.ones(64), -np.ones(64)])

    def th(l):
        return 2 * np.pi * ((b[:, None] * l[None, :]) % DM) / DM

    sc = 1.0 / (S * DM)
    fw = np.zeros((7, 128, 128))
    iw = np.zeros((7, 128, 128))
    t = th(l0)
    cl = np.full((128, 1), 2.0)
    cl[0] = cl[64] = 1.0
    fw[0] = np.concatenate([np.cos(t), -np.sin(t[:, 1:64])], axis=1)
    iw[0] = cl * sc * fw[0].T
    mu = S1 * sg
    for g, l in ((1, l1), (2, l2)):
        t = th(l)
        c, s = np.cos(t), np.sin(t)
        fw[3 * g - 2:3 * g + 1] = c, -mu * s - c, mu * c - s
        iw[3 * g - 2:3 * g + 1] = [2 * sc * m.T for m in (c, -s - mu * c, mu * s - c)]
    n = np.arange(64)
    order = np.concatenate([np.concatenate([np.arange(8) + 8 * j, np.arange(8) + 8 * j + 64])
                            for j in range(8)])
    e = np.zeros((2, 32, 128, 128))
    for k2 in range(32):
        t = 2 * np.pi * (((32 * n[:, None] + k2) * n[None, :]) % S) / S
        er, ei = np.cos(t), -np.sin(t)
        m = np.block([[er, -ei], [ei, er]])[order][:, order]
        e[0, k2], e[1, k2] = m, m.T
    small = np.concatenate([_pack_rows(fw), _pack_rows(iw)], axis=0)
    return small, _pack_rows(e).reshape(64, 64, 128)


def _loop(name, lo, hi, body, init, **kw):
    with jax.named_scope(name):
        return lax.fori_loop(lo, hi, body, init, **kw)


def _bf(x):
    return pltpu.bitcast(x, bf16)


def _dot(a, b):
    return jnp.dot(a, b, preferred_element_type=f32)


def _round_bf16(x):
    return x.astype(bf16).astype(f32)


def _layernorm(x):
    m = jnp.mean(x, axis=-1, keepdims=True)
    xc = x - m
    v = jnp.mean(xc * xc, axis=-1, keepdims=True)
    return xc * lax.rsqrt(v + EPS)


def _fft4(x, sign):
    (ar, ai), (br, bi), (cr, ci), (dr, di) = x
    t0r, t0i, t1r, t1i = ar + cr, ai + ci, ar - cr, ai - ci
    t2r, t2i, t3r, t3i = br + dr, bi + di, br - dr, bi - di
    y0, y2 = (t0r + t2r, t0i + t2i), (t0r - t2r, t0i - t2i)
    p, q = (t1r + t3i, t1i - t3r), (t1r - t3i, t1i + t3r)
    return [y0, p, y2, q] if sign < 0 else [y0, q, y2, p]


def _twiddle(z, n, period, sign):
    zr, zi = z
    n = n % period
    if n == 0:
        return z
    if 4 * n == period:
        return (-zi, zr) if sign > 0 else (zi, -zr)
    c, s = math.cos(2 * math.pi * n / period), sign * math.sin(2 * math.pi * n / period)
    if (8 * n) % period == 0:
        a, d = zr + zi, zr - zi
        if c * s > 0:
            return (d * c, a * c)
        return (a * c, d * s)
    return (zr * c - zi * s, zr * s + zi * c)


STRASSEN_LHS = (((0, 0, 1), (1, 1, 1)), ((1, 0, 1), (1, 1, 1)), ((0, 0, 1),), ((1, 1, 1),),
                ((0, 0, 1), (0, 1, 1)), ((1, 0, 1), (0, 0, -1)), ((0, 1, 1), (1, 1, -1)))
STRASSEN_RHS = (((0, 0, 1), (1, 1, 1)), ((0, 0, 1),), ((0, 1, 1), (1, 1, -1)), ((1, 0, 1), (0, 0, -1)),
                ((1, 1, 1),), ((0, 0, 1), (0, 1, 1)), ((1, 0, 1), (1, 1, 1)))
STRASSEN_OUT = ((((0, 0), 1), ((1, 1), 1)), (((1, 0), 1), ((1, 1), -1)), (((0, 1), 1), ((1, 1), 1)),
                (((0, 0), 1), ((1, 0), 1)), (((0, 0), -1), ((0, 1), 1)), (((1, 1), 1),), (((0, 0), 1),))
WS_SLOT = {0: 0, 2: 1, 3: 2, 5: 3, 6: 4}


def _operand(terms, block):
    x = block(*terms[0][:2])
    if len(terms) == 1:
        return x
    x, y = x.astype(f32), block(*terms[1][:2]).astype(f32)
    return x + y if terms[1][2] > 0 else x - y


def _accumulate(acc, key, y, sign):
    if key not in acc:
        acc[key] = y if sign > 0 else -y
    else:
        acc[key] = acc[key] + y if sign > 0 else acc[key] - y


def _mu():
    lane = lax.broadcasted_iota(jnp.int32, (1, 128), 1)
    return jnp.where(lane < 64, S1, -S1).astype(f32)


def _ilv(r, i):
    n = r.shape[0] // 8
    return jnp.concatenate([r.reshape(n, 8, 128), i.reshape(n, 8, 128)], axis=1).reshape(16 * n, 128)


def _dilv(x):
    n = x.shape[0] // 16
    x = x.reshape(n, 16, 128)
    return x[:, :8].reshape(8 * n, 128), x[:, 8:].reshape(8 * n, 128)


def _with_tokens(x, toks):
    if not toks:
        return x
    return jnp.concatenate(
        [x[8 * j:8 * j + 8] | toks[j] if j in toks else x[8 * j:8 * j + 8]
         for j in range(x.shape[0] // 8)], axis=0)


def _fft16(x, sign, emit=None):
    cols = [_fft4([x[4 * j + r] for j in range(4)], sign) for r in range(4)]
    out = [None] * 16
    for q in range(4):
        y = _fft4([_twiddle(cols[r][q], r * q, 16, sign) for r in range(4)], sign)
        for p in range(4):
            out[q + 4 * p] = y[p]
        if emit is not None:
            emit(q, y)
    return out


CFG = dict(
    steps=((4.5, 16.5, 6, 4, 0, 8), (5, 16.5, 5, 7, 8, 12), (5, 16.5, 6, 6, 8, 12), (5, 16.5, 8, 7, 8, 0)),
    moves=(((125, 127), (15, 14), (34, 35), (91, 89), (11, 14), (20, 18), (1, 0), (107, 106)),
           ((9, 11), (134, 133), (129, 126), (83, 85)), ((96, 94), (6, 5)), ((33, 34),)),
    pro_inner=(4, 2, 5, 8, 0, 3, 6, 7, 9, 10, 1),
    pro_outer=((2, 2), (5, 3), (1, 0), (0, None), (4, None), (3, None), (6, 1)),
    pro_nre=13, re_pos=(2, 2, 5, 5), ln_at=(11, 17, 23, 27), ln_at2=(3, 4, 6, 7, 9, 10, 12, 13),
    perm_at=tuple(range(10, 22)),
    ws_split=4, ws_at=(15, 15, 16, 16, 17, 18, 18, 19, 20, 20, 21, 21, 22, 23, 23, 24),
    post_passes=((0, 1), (2, 3), (4, 5), (6, 7)), post_dl=20,
    post_order=(0, 1, 6, 3, 4, 2, 8, 5, 7, 9, 10, 11), post_at=(26, 38, 58, 96),
    fwd_at=(7, 8, 9, 10, 12, 13, 14, 16, 17, 18, 20, 21, 22, 24, 25, 26),
    inv_at=tuple(range(28, 44)), inv_lag=4, tok_pos=(4, 5, 6, 7), rel=(0, 1),
    tails_order=((1, 2, 0), 5), out_order=((1, 2, 0), 5),
    two_inner=(2, 8, 5, 4, 0, 6, 3, 7, 9, 10, 1),
    two_outer=((2, 2), (5, 3), (1, None), (0, None), (4, 0), (3, None), (6, 1)),
    dinv_at=(0, 0, 1, 1), dinv_order=(2, 1, 0),
    only=None)


def _step_order(params, moves):
    lat_s, lat_pv, lat_wo, v_delay, n_first, n_last = params
    keyed = []
    for p in range(NPAIR):
        keyed += [(4 * p + 2 * m + e, ("proj", p, m, e)) for m in range(2) for e in range(2)]
        keyed += [(4 * p + 3.5 + v_delay, ("proj", p, 2, e)) for e in range(2)]
    bulk = [x for _, x in sorted(keyed, key=lambda kv: kv[0])]
    first, bulk = bulk[:n_first], bulk[n_first:]
    t, nwo, seq, ready = float(n_first), 0, [], []
    pend = [(t + lat_s, "scores", p) for _, p, m, e in first if m == 1 and e == 1]
    while nwo < H - n_last or pend:
        pend.sort(key=lambda x: (x[0], x[1] == "pv", x[2]))
        if pend and pend[0][0] <= t:
            _, kind, p = pend.pop(0)
            seq.append((kind, p, 0, 0))
            if kind == "scores":
                pend.append((t + lat_pv, "pv", p))
            else:
                ready += [(t + lat_wo, p, e) for e in range(2)]
            t += 0.5
        elif bulk:
            seq.append(bulk.pop(0))
            t += 1
            if seq[-1][2:] == (1, 1):
                pend.append((t + lat_s, "scores", seq[-1][1]))
        elif ready and ready[0][0] <= t and nwo < H - n_last:
            _, p, e = ready.pop(0)
            seq.append(("wo", p, 0, e))
            t += 1
            nwo += 1
        else:
            t += 0.5
    for i, j in moves:
        seq.insert(j, seq.pop(i))
    return first, seq, [2 * p + e for _, p, e in ready]


def _kernel(x_hbm, mem_hbm, wq_hbm, wk_hbm, wv_hbm, wo_hbm, wr_hbm, wi_hbm,
            small_hbm, e_hbm, out_hbm,
            xin, xa, xb, to, raw, wa, wb, wo_t, ws, qb, hl, z0, z1, z2, wf,
            wri, wtmp, small, emat, fill_ref, mem_ref, zero_ref, sem, osem):
    zs = (z0, z1, z2)
    w_hbm = (wq_hbm, wk_hbm, wv_hbm)

    def body_chunk(i):
        return 4 * (i & 3) + (i >> 2)

    def cp_w(i):
        src = w_hbm[i >> 2].at[:, :, pl.ds(8 * (i & 3), 8), :] if isinstance(i, int) else raw.at[i]
        return pltpu.make_async_copy(src, raw.at[i], sem.at[i])

    def cp_x(bb):
        return pltpu.make_async_copy(x_hbm.at[:, bb], xin.at[:, bb], sem.at[12 + bb])

    def cp_f(i):
        src = ((wr_hbm, wi_hbm)[i >> 2].at[:, pl.ds(512 * (i & 3), 512)]
               if isinstance(i, int) else wri.at[i])
        return pltpu.make_async_copy(src, wri.at[i], sem.at[36 + i])

    def cp_wo(i):
        rows = pl.ds(pl.multiple_of(512 * i, 512), 512)
        return [pltpu.make_async_copy(wo_hbm.at[rows, pl.ds(128 * j, 128)], wo_t.at[j, rows], sem.at[28 + i])
                for j in range(5)]

    cp_rest = [pltpu.make_async_copy(mem_hbm, mem_ref, sem.at[46]),
               pltpu.make_async_copy(small_hbm, small, sem.at[44]),
               pltpu.make_async_copy(e_hbm, emat, sem.at[45])]

    full = CFG["only"] in (None, "pro")
    for u in range(4 if full else 0):
        cp_x(4 * u + 3).start()
    if full:
        cp_w(0).start()
    for i in range(12 if full else 0):
        if i < 11:
            cp_w(i + 1).start()
        cp_x(body_chunk(i)).start()
        if 3 <= i < 11:
            cp_f(i - 3).start()
            for cp in cp_wo(i - 3):
                cp.start()
    for cp in cp_rest if full else ():
        cp.start()

    zero_ref[0] = 0

    r = lax.broadcasted_iota(jnp.int32, (80, 80), 0)
    c = lax.broadcasted_iota(jnp.int32, (80, 80), 1)

    def head(i):
        return jnp.where(i < 64, i // 32, (i - 64) // 8)

    def pos(i):
        return jnp.where(i < 64, i % 32, 32 + (i - 64) % 8)

    ok = (pos(r) < MEM) | (pos(r) >= pos(c))
    fill_ref[...] = jnp.where(head(r) == head(c), jnp.where(ok, 0.0, -1e9), -jnp.inf).astype(f32)
    wtmp[:, 320:328, :] = jnp.zeros((4, 8, 128), f32)
    xa[32, 0:8, 0:128] = jnp.zeros((8, 128), f32)
    ws[18, 0, 0:16, :] = jnp.zeros((16, 128), bf16)
    wa[12, 0:8, :] = jnp.zeros((8, 128), u32)
    wb[12, 0:8, :] = jnp.zeros((8, 128), u32)
    wf[5, 16 * WPITCH:16 * WPITCH + 8, :] = jnp.zeros((8, 128), f32)
    for z in zs:
        z[0, 0, 128:ZPITCH, :] = jnp.zeros((8, 128), f32)

    def chunk(bb):
        if isinstance(bb, int):
            return slice(8 * bb, 8 * bb + 8)
        return pl.ds(pl.multiple_of(8 * bb, 8), 8)

    def set_input(bb, x, tail_u, a0=0, win=None):
        n = x.shape[0] // 8
        xav = xa if win is None else xa.at[:, win]
        xav[a0:a0 + n, chunk(bb), :] = x.reshape(n, 8, DM)
        y = _layernorm(x)
        if tail_u is None:
            xav[16 + a0:16 + a0 + n, chunk(bb), :] = y.reshape(n, 8, DM)
        else:
            blk = [[y[32 * r:32 * r + 32, 128 * kt:128 * kt + 128] for kt in range(5)] for r in range(4)]
            rows = (slice(16 * tail_u, 16 * tail_u + 16) if isinstance(tail_u, int)
                    else pl.ds(pl.multiple_of(16 * tail_u, 16), 16))
            ops = []
            for outer in STRASSEN_LHS:
                sub = [[_operand(outer, lambda rr, kk: blk[2 * rr + r][2 * kk + k]) for k in range(2)]
                       for r in range(2)]
                ops += [_operand(inner, lambda r, k: sub[r][k]) for inner in STRASSEN_LHS]
            for i, v in enumerate(ops + [blk[r][4] for r in range(4)]):
                hl[i, rows, :] = pltpu.bitcast(v.astype(bf16), u32)

    def load_x(bb, a0=0, n=16):
        return xin[a0:a0 + n, bb].astype(f32).reshape(8 * n, DM)

    def wtile(cid, j, e):
        w = (wa, wb)[e]
        return jnp.concatenate([w[cid, (4 * hf + j) * HPITCH:(4 * hf + j) * HPITCH + 160, :]
                                for hf in range(2)], axis=0)

    def relayout(i, cid, e):
        for r in range(4 * i, 4 * i + 4):
            a, b = [pltpu.bitcast(raw[cid, :, d].reshape(16, 128), u32) for d in (2 * r, 2 * r + 1)]
            v = (a & 0xFFFF) | (b << 16) if e == 0 else (a >> 16) | (b & jnp.uint32(0xFFFF0000))
            (wa, wb)[e][cid, pl.ds(r, 8, stride=HPITCH), :] = v

    def batch_thunks(cid, inner_order, outer_order):
        qv = qb.at[:, :, pl.ds(8 * cid, 8)]

        def unit(e):
            c = {}
            left = {(r, n): (5, 3, 3, 5)[2 * (r >> 1) + (n >> 1)] for r in range(4) for n in range(4)}

            def w(kt, n):
                return _bf(wtile(cid, n, e)[64 * kt:64 * kt + 64])

            def add_out(blk, y, sign):
                _accumulate(c, blk, y, sign)
                left[blk] -= 1
                if left[blk] == 0:
                    r, n = blk
                    y = c.pop(blk).reshape(4, 4, 8, 128)
                    for u in range(4):
                        qv[4 * r:4 * r + 4, u, 2 * n + e] = y[u]

            def outer(io, k4):
                p = {}
                todo = {(0, 0): 4, (0, 1): 2, (1, 0): 2, (1, 1): 4}

                @functools.lru_cache(maxsize=None)
                def sub(k, n):
                    return _operand(STRASSEN_RHS[io], lambda kk, nn: w(2 * kk + k, 2 * nn + n))

                def thunk(items):
                    def run(toks=None):
                        for i in items:
                            if i >= 7:
                                r, n = k4[i - 7]
                                add_out((r, n), _dot(_bf(_with_tokens(hl[49 + r], toks)), w(4, n)), 1)
                                toks = None
                                continue
                            rhs = _operand(STRASSEN_RHS[i], sub).astype(bf16)
                            y = _dot(_bf(_with_tokens(hl[7 * io + i], toks)), rhs)
                            toks = None
                            for blk, sign in STRASSEN_OUT[i]:
                                _accumulate(p, blk, y, sign)
                                todo[blk] -= 1
                                if todo[blk] == 0:
                                    for (rr, nn), sg in STRASSEN_OUT[io]:
                                        add_out((2 * rr + blk[0], 2 * nn + blk[1]), p[blk], sg)
                    return run
                items = [i for i in inner_order if i < 7 + len(k4)]
                return [thunk(items[:len(items) // 2]), thunk(items[len(items) // 2:])]
            out = []
            for io, q in outer_order:
                out += outer(io, [] if q is None else
                             [(2 * (q >> 1) + (j >> 1), 2 * (q & 1) + (j & 1)) for j in range(4)])
            return out
        return unit(0) + unit(1)

    def wperm_thunks(piece, j):
        m = (piece >> 2) & 1
        wt = wtmp.at[j]

        def load():
            wt[0:DF, :] = wri[piece, :, 128 * j:128 * j + 128].astype(f32)

        def one(g):
            def run():
                if g == 0:
                    t = jnp.concatenate([wt[pl.ds(0, 64, stride=5), :], wt[320:328, :],
                                         jnp.zeros((56, 128), f32)], axis=0)
                else:
                    t = jnp.concatenate([wt[pl.ds(g, 64, stride=5), :],
                                         wt[pl.ds(5 - g, 64, stride=5), :]], axis=0)
                y = t.T
                sub = wf.at[3 * m + g, pl.ds(pl.multiple_of((piece & 3) * 32, 32), 16 * WPITCH - 96)]
                for k in range(8):
                    for hf in range(2):
                        sub[pl.ds(8 * j + k + 8 * hf * WPITCH, 8, stride=WPITCH), :] = (
                            y[16 * k + 8 * hf:16 * k + 8 * hf + 8])
            return run
        return [load] + [one(g) for g in range(3)]

    def half_pass(cid, half, fill, zero, timed=()):
        nre = CFG["pro_nre"]
        toks = None
        for k, f in enumerate(batch_thunks(cid, CFG["pro_inner"], CFG["pro_outer"])[14 * half:14 * half + 14]):
            f(toks)
            toks = {}
            for n, f in enumerate(f for at, f in timed if at == k):
                toks[(0, 4, 1, 6)[n]] = f()
            if fill is not None:
                for n, r in enumerate(r for r in range(40) if r * nre // 40 == k):
                    relayout(r, fill, 1 - half)
                    toks[CFG["re_pos"][n]] = (wb, wa)[half][12 + zero, 0:8, :]

    def ln_parts(bb, zero):
        def part(j):
            set_input(bb, load_x(bb, 4 * j, 4), None, 4 * j)
            return pltpu.bitcast(xa[32 + zero, 0:8, 0:128], u32)
        return [functools.partial(part, j) for j in range(4)]

    def perm_parts(piece, zero):
        def part(fs):
            for f in fs:
                f()
            return pltpu.bitcast(wf[5 + zero, 16 * WPITCH:16 * WPITCH + 8, :], u32)
        out = []
        for j in range(4):
            th = wperm_thunks(piece, j)
            out += [functools.partial(part, th[0:2]), functools.partial(part, th[2:3]),
                    functools.partial(part, th[3:4])]
        return out

    def ws_parts(piece, zero):
        nr = 128 // CFG["ws_split"]

        src = wo_t.at[:, pl.ds(pl.multiple_of(512 * piece, 512), 512)]
        dst = ws.at[pl.ds(2 * piece, 2)]

        def part(pp, np_, r0):
            def tile(k, n):
                lo = 256 * pp + 128 * k + r0
                return src[2 * np_ + n, lo:lo + nr, :]
            for i, slot in WS_SLOT.items():
                dst[pp, 5 * np_ + slot, r0:r0 + nr, :] = _operand(STRASSEN_RHS[i], tile).astype(bf16)
            return pltpu.bitcast(ws[18 + zero, 0, 0:16, :], u32)
        return [functools.partial(part, pp, np_, r0)
                for pp in range(2) for np_ in range(2) for r0 in range(0, 128, nr)]

    def pro0():
        def tails(i, carry):
            for u in (2 * i, 2 * i + 1):
                cp_x(4 * u + 3).wait()
            for u in (2 * i, 2 * i + 1):
                set_input(4 * u + 3, load_x(4 * u + 3), u)
            return carry
        lax.fori_loop(0, 2, tails, 0)
        cp_w(0).wait()
        zero = zero_ref[0]
        for i in range(40):
            relayout(i, 0, 0)
        half_pass(0, 0, zero, zero)

    def pro1(it, carry):
        bb = jnp.where(it == 0, 3, body_chunk(it - 1))
        with jax.named_scope("pro1_wait"):
            cp_w(it + 1).wait()

            @pl.when(it >= 1)
            def _():
                cp_x(bb).wait()

            @pl.when(it >= 3)
            def _():
                cp_f(it - 3).wait()
                for cp in cp_wo(it - 3):
                    cp.wait()
        piece = jnp.where(it >= 3, it - 3, 8)
        zero = it >> 4
        timed = sorted(list(zip(CFG["ln_at"], ln_parts(bb, zero)))
                       + list(zip(CFG["ws_at"], ws_parts(piece, zero)))
                       + list(zip(CFG["perm_at"], perm_parts(piece, zero))), key=lambda x: x[0])
        half_pass(it, 1, it + 1, zero, [x for x in timed if x[0] < 14])
        half_pass(it + 1, 0, it + 1, zero, [(k - 14, f) for k, f in timed if k >= 14])
        return carry

    def pro2():
        cp_x(body_chunk(10)).wait()
        cp_x(body_chunk(11)).wait()
        cp_rest[0].wait()
        zero = zero_ref[0]
        half_pass(11, 1, None, zero, list(zip(
            CFG["ln_at2"], ln_parts(body_chunk(10), zero) + ln_parts(body_chunk(11), zero))))

    if full:
        with jax.named_scope("pro0"):
            pro0()
        _loop("pro1", 0, 11, pro1, 0)
        with jax.named_scope("pro2"):
            pro2()

    scale = DH ** -0.5

    def wo_dot(hh, oo):
        return [_dot(oo, wo_t[j, 128 * hh:128 * hh + 128, :]) for j in range(5)]

    def addl(acc, res):
        return res if acc is None else [a + b for a, b in zip(acc, res)]

    def group(g, mem):
        for ph in range(4):
            h = jnp.concatenate([mem, xa[16 + g, 32 * ph:32 * ph + 24, :]], axis=0).astype(bf16)
            pr, sm, oos = {}, {}, {}

            def stacked(p, m):
                tails = [qb[g, ph, 32 * m + 2 * p + e] for e in range(2)]
                return jnp.concatenate([pr[p, m, 0], pr[p, m, 1]] + tails, axis=0).astype(bf16)

            def scores(p):
                sc = lax.dot_general(stacked(p, 0), stacked(p, 1), (((1,), (1,)), ((), ())),
                                     preferred_element_type=f32)
                fill = fill_ref[...]
                sc = jnp.where(fill == 0.0, sc * scale, fill)
                mx = jnp.max(sc, axis=-1, keepdims=True)
                e = jnp.exp(sc - mx)
                rl = pl.reciprocal(jnp.sum(e, axis=-1, keepdims=True), approx=True)
                sm[p] = (e * rl).astype(bf16)

            def pv(p):
                o = _dot(sm[p], stacked(p, 2))
                for e in range(2):
                    qb[g, ph, 2 * p + e] = o[64 + 8 * e:72 + 8 * e]
                    oos[2 * p + e] = o[32 * e:32 * e + 32].astype(bf16)

            first, seq, last = _step_order(CFG["steps"][ph], CFG["moves"][ph])
            for kt in range(5):
                for _, p, m, e in first:
                    w = wtile(4 * m + (p >> 2), p & 3, e)[64 * kt:64 * kt + 64]
                    y = _dot(h[:, 128 * kt:128 * kt + 128], _bf(w))
                    pr[p, m, e] = y if kt == 0 else pr[p, m, e] + y
            acc = None
            for kind, p, m, e in seq:
                if kind == "proj":
                    pr[p, m, e] = _dot(h, _bf(wtile(4 * m + (p >> 2), p & 3, e)))
                elif kind == "scores":
                    scores(p)
                elif kind == "pv":
                    pv(p)
                else:
                    acc = addl(acc, wo_dot(2 * p + e, oos[2 * p + e]))
            for j in range(5):
                for hh in last:
                    acc[j] = acc[j] + _dot(oos[hh], wo_t[j, 128 * hh:128 * hh + 128, :])
            out = jnp.concatenate(acc, axis=1)
            xa[16 + g, 32 * ph:32 * ph + 24, :] = out[8:32]
            mem = _round_bf16(out[0:8])
        return mem

    def dfwd_thunks(seg, q):
        st = {}
        rows = chunk(q)
        xav, xbv, zv = xa.at[:, seg], xb.at[:, seg], [z.at[:, :, seg] for z in zs]

        def pre():
            o = to[...] if q == 3 else xav[16:32, rows, :]
            x = _round_bf16(xav[0:16, rows, :] + o)
            xbv[:, rows, :] = x
            y = _layernorm(x.reshape(128, DM))
            x0, x1, x2, x3, x4 = [y[:, 128 * a:128 * a + 128] for a in range(5)]
            t1, t2, t3, t4 = x1 + x4, x2 + x3, x1 - x4, x2 - x3
            t = t1 + t2
            m, n = x0 - 0.25 * t, R5_D * (t1 - t2)
            st["u"] = [x0 + t, (m + n, t3 + R5_R * t4), (m - n, R5_R * t3 - t4)]

        def part(g):
            def run():
                if g == 0:
                    pre()
                    u0 = st["u"][0].astype(bf16)
                    zr = _dot(u0, _bf(small[0]))
                    lane = lax.broadcasted_iota(jnp.int32, (128, 128), 1)
                    zi = jnp.where((lane & 63) == 0, 0.0, pltpu.roll(zr, 64, 1))
                else:
                    a, b = st["u"][g]
                    k, kb, ka = [_dot(v.astype(bf16), _bf(small[3 * g - 2 + i]))
                                 for i, v in enumerate((a + b, b, a))]
                    zr, zi = k + kb, ka - _mu() * k
                ys = [(zr[8 * a:8 * a + 8], zi[8 * a:8 * a + 8]) for a in range(16)]
                if g < 2:
                    ys = _fft16(ys, -1)
                for a in range(16):
                    zv[g][0, a, rows, :] = ys[a][0]
                    zv[g][1, a, rows, :] = ys[a][1]
            return run
        return [part(g) for g in range(3)]

    def post(u, carry):
        base = pl.multiple_of(32 * u, 32)
        side = []
        for q in range(4):
            side += dfwd_thunks(pl.ds(base, 32), q)
        side = [side[i] for i in CFG["post_order"]]
        k = 0
        at = list(CFG["post_at"])
        m, due = {}, []
        for prods in CFG["post_passes"]:
            acc = None
            for p in range(NPAIR):
                res = []
                for i in prods:
                    if i == 7:
                        oo = jnp.concatenate([qb[:, u, 2 * p + e].reshape(128, 128) for e in range(2)], axis=1)
                        res.append(_dot(oo.astype(bf16), wo_t[4, 256 * p:256 * p + 256, :]))
                        k += 2
                        continue
                    a = _operand(STRASSEN_LHS[i], lambda r, e: (
                        qb[8 * r:8 * r + 8, u, 2 * p + e].reshape(64, 128))).astype(bf16)
                    for np_ in range(2):
                        if i in WS_SLOT:
                            w = ws[p, 5 * np_ + WS_SLOT[i]]
                        else:
                            kk = 0 if i == 1 else 1
                            w = wo_t[2 * np_ + kk, 256 * p + 128 * kk:256 * p + 128 * kk + 128, :]
                        if due and due[0][0] <= k:
                            w = _bf(_with_tokens(pltpu.bitcast(w, u32), {0: due.pop(0)[1]}))
                        res.append(_dot(a, w))
                    k += 1
                acc = addl(acc, res)
                while at and at[0] <= k:
                    g = CFG["post_order"][len(CFG["post_at"]) - len(at)] % 3
                    at.pop(0)
                    side.pop(0)()
                    if g == 0:
                        due.append((k + CFG["post_dl"],
                                    pltpu.bitcast(z0[0, u >> 2, 128:ZPITCH, :], u32)))
            for i in prods:
                m[i] = [acc.pop(0)] if i == 7 else [acc.pop(0), acc.pop(0)]
        cols = []
        for np_ in range(2):
            m1, m2, m3, m4, m5, m6, m7 = [m[i][np_] for i in range(7)]
            cols.append(jnp.concatenate([m1 + m4 - m5 + m7, m2 + m4], axis=0))
            cols.append(jnp.concatenate([m3 + m5, m1 - m2 + m3 + m6], axis=0))
        to[...] = jnp.concatenate(cols + m[7], axis=1).reshape(16, 8, DM)
        for f in side:
            f()
        return carry

    def spectral(zero):
        def fence(z):
            return z[0, zero, 128:ZPITCH, :]

        def radix(g, bb, sign):
            z = zs[g]
            toks = []

            def emit(q, y):
                for p in range(4):
                    z[0, q + 4 * p, chunk(bb), :] = y[p][0]
                    z[1, q + 4 * p, chunk(bb), :] = y[p][1]
                toks.append(fence(z))
            _fft16([(z[0, a, chunk(bb), :], z[1, a, chunk(bb), :]) for a in range(16)], sign, emit)
            return toks

        ys = {}

        def fwd(g, k2, toks):
            z = zs[g]
            ur, ui = z[0, k2, 0:64, :], z[1, k2, 0:64, :]
            tr, ti = _twiddle((z[0, k2, 64:128, :], z[1, k2, 64:128, :]), k2, 32, -1)
            for hf in range(2):
                v = _ilv(ur + tr, ui + ti) if hf == 0 else _ilv(ur - tr, ui - ti)
                lhs = _with_tokens(emat[k2 + 16 * hf], toks if hf == 0 else None)
                xr, xi = _dilv(_dot(_bf(lhs), v.astype(bf16)))
                ys["x", 16 * g + k2] = xr
                wr = wf[g, pl.ds(k2 * WPITCH + hf, 64, stride=2), :]
                wi = wf[g + 3, pl.ds(k2 * WPITCH + hf, 64, stride=2), :]
                ys[g, k2, hf] = _ilv(xr * wr - xi * wi, xr * wi + xi * wr).astype(bf16)

        def inv(g, k2, toks):
            z = zs[g]
            t0 = _dot(_bf(_with_tokens(emat[32 + k2], toks)), ys.pop((g, k2, 0)))
            t1 = _dot(_bf(emat[48 + k2]), ys.pop((g, k2, 1)))
            z[0, k2, 0:64, :], z[1, k2, 0:64, :] = _dilv(t0 + t1)
            z[0, k2, 64:128, :], z[1, k2, 64:128, :] = _twiddle(_dilv(t0 - t1), k2, 32, 1)

        units = [(g, k2) for g in range(3) for k2 in range(16)]
        toks = None
        lag = CFG["inv_lag"]
        for i in range(len(units) + lag):
            if i < len(units):
                fwd(*units[i], toks)
            if i >= lag:
                inv(*units[i - lag], toks if i >= len(units) else None)
            toks = []
            if i in CFG["fwd_at"]:
                toks = radix(2, CFG["fwd_at"].index(i), -1)
            if i in CFG["inv_at"]:
                back, r = CFG["rel"]
                z0[1, zero, 128:ZPITCH, :] = ys["x", min(i - back, 47)][8 * r:8 * r + 8]
                toks = radix(0, CFG["inv_at"].index(i), 1)
            toks = {j: pltpu.bitcast(t, u32) for j, t in zip(CFG["tok_pos"], toks)}

    def dinv_thunks(bb, finish, win=None):
        st = {}
        xbv = xb if win is None else xb.at[:, win]

        def part(g):
            def run():
                z = zs[g] if win is None else zs[g].at[:, :, win]
                ys = [(z[0, a, chunk(bb), :], z[1, a, chunk(bb), :]) for a in range(16)]
                if g > 0:
                    ys = _fft16(ys, 1)
                tr = jnp.concatenate([y[0] for y in ys], axis=0)
                ti = jnp.concatenate([y[1] for y in ys], axis=0)
                if g == 0:
                    lane = lax.broadcasted_iota(jnp.int32, (128, 128), 1)
                    v = jnp.where(lane <= 64, tr, pltpu.roll(ti, 64, 1))
                    st[0] = _dot(v.astype(bf16), _bf(small[7]))
                else:
                    k, ki, kr = [_dot(v.astype(bf16), _bf(small[5 + 3 * g + i]))
                                 for i, v in enumerate((tr + _mu() * ti, ti, tr))]
                    st[2 * g - 1], st[2 * g] = k + ki, k + kr
            return run

        def fin():
            p0, p1, q1, p2, q2 = [st[j] for j in range(5)]
            t = p1 + p2
            m, n = p0 - 0.25 * t, R5_D * (p1 - p2)
            e1, e2 = m + n, m - n
            o1, o2 = q1 + R5_R * q2, R5_R * q1 - q2
            y = jnp.concatenate([p0 + t, e1 - o1, e2 - o2, e2 + o2, e1 + o1], axis=1)
            finish(xbv[:, chunk(bb), :].reshape(128, DM) + y)
        return [part(0), part(1), part(2), fin]

    def out_copy(bb):
        return pltpu.make_async_copy(xin.at[:, bb], out_hbm.at[:, bb], osem.at[bb])

    def layer(li, carry0):
        if full or CFG["only"] == "group":
            _loop("step", 0, 16, group, mem_ref[...].astype(f32))
        if full or CFG["only"] == "spec":
            if full:
                @pl.when(li == 0)
                def _():
                    for cp in cp_rest[1:]:
                        cp.wait()
            _loop("post", 0, 4, post, 0)

            with jax.named_scope("spectral"):
                spectral(li >> 1)
        if not full and CFG["only"] != "out":
            return carry0

        def run_chunks(th, order, lag):
            seq = [t[g] for t in th for g in order]
            for i in range(len(seq) + lag):
                if i < len(seq):
                    seq[i]()
                if i >= lag and (i - lag) % 3 == 2:
                    th[(i - lag) // 3][3]()

        @pl.when(li == 0)
        def _():
            with jax.named_scope("dinv_tails"):
                run_chunks([dinv_thunks(4 * u + 3, functools.partial(
                    lambda u, x: set_input(4 * u + 3, _round_bf16(x), u), u))
                    for u in range(4)],
                    *CFG["tails_order"])

            def batch(u, carry):
                win = pl.ds(pl.multiple_of(32 * u, 32), 32)
                for q in range(3):
                    side = dinv_thunks(q, functools.partial(
                        lambda q, x: set_input(q, _round_bf16(x), None, win=win), q), win)
                    for k, f in enumerate(batch_thunks(3 * u + q, CFG["two_inner"], CFG["two_outer"])):
                        f()
                        for at, g in zip(CFG["dinv_at"], CFG["dinv_order"] + (3,)):
                            if at == k:
                                side[g]()
                return carry
            _loop("batch", 0, 4, batch, 0)

        @pl.when(li == 1)
        def _():
            def out_half(hf, carry):
                xv = xin.at[:, pl.ds(8 * hf, 8)]

                def store_out(q, x):
                    xv[:, q] = x.reshape(16, 8, DM).astype(bf16)
                    out_copy(8 * hf + q).start()
                win = pl.ds(pl.multiple_of(64 * hf, 64), 64)
                run_chunks([dinv_thunks(q, functools.partial(store_out, q), win) for q in range(8)],
                           *CFG["out_order"])
                return carry
            with jax.named_scope("dinv_out"):
                lax.fori_loop(0, 2, out_half, 0)
                for bb in range(16):
                    out_copy(bb).wait()
        return carry0

    if CFG["only"] != "pro":
        lax.fori_loop(0, 2, layer, 0)
    if CFG["only"] in ("pro", "out"):
        zero = zero_ref[0]
        xin[0, 0, :, 0:128] = (qb[zero, 0, 0] + wf[zero, 0:8, :] + xa[zero, 0:8, 0:128]).astype(bf16) + ws[zero, 0, 0:8, :]
        out_copy(0).start()
        out_copy(0).wait()
        for cp in cp_rest[1:] if full else ():
            cp.wait()


@jax.jit
def pallas_interleave_layers__memory_aug_recurrent_mem_tr__spectral_gfnet__prompt_kernel(
    A_x, A_mem0, A_Wq, A_Wk, A_Wv, A_Wo, A_seg_len, B_x, B_w_r, B_w_i,
):
    assert A_x.shape == (1, S, DM) and A_mem0.shape == (1, MEM, DM)
    small, emat = _tables()
    hbm = pl.BlockSpec(memory_space=pltpu.HBM)
    out = pl.pallas_call(
        _kernel,
        out_shape=jax.ShapeDtypeStruct((16, 16, 8, DM), bf16),
        in_specs=[hbm] * 10,
        out_specs=hbm,
        scratch_shapes=[
            pltpu.VMEM((16, 16, 8, DM), bf16),
            pltpu.VMEM((33, 128, DM), f32),
            pltpu.VMEM((16, 128, DM), f32),
            pltpu.VMEM((16, 8, DM), f32),
            pltpu.VMEM((12, 2, 320, 8, DH), bf16),
            pltpu.VMEM((13, 8 * HPITCH, 128), u32),
            pltpu.VMEM((13, 8 * HPITCH, 128), u32),
            pltpu.VMEM((5, H * DH + 512, 128), bf16),
            pltpu.VMEM((19, 10, 128, 128), bf16),
            pltpu.VMEM((16, 4, 96, 8, 128), f32),
            pltpu.VMEM((53, 64, 128), u32),
            pltpu.VMEM((2, 16, ZPITCH, 128), f32),
            pltpu.VMEM((2, 16, ZPITCH, 128), f32),
            pltpu.VMEM((2, 16, ZPITCH, 128), f32),
            pltpu.VMEM((6, 16 * WPITCH + 32, 128), f32),
            pltpu.VMEM((9, DF, 512), bf16),
            pltpu.VMEM((4, 328, 128), f32),
            pltpu.VMEM((14, 64, 128), u32),
            pltpu.VMEM((64, 64, 128), u32),
            pltpu.VMEM((80, 80), f32),
            pltpu.VMEM((MEM, DM), bf16),
            pltpu.SMEM((1,), jnp.int32),
            pltpu.SemaphoreType.DMA((47,)),
            pltpu.SemaphoreType.DMA((16,)),
        ],
        compiler_params=pltpu.CompilerParams(vmem_limit_bytes=120 * 1024 * 1024,
                                             disable_semaphore_checks=True),
    )(
        A_x.reshape(16, 16, 8, DM), A_mem0.reshape(MEM, DM),
        *[w.reshape(2, 320, H, DH) for w in (A_Wq, A_Wk, A_Wv)], A_Wo.reshape(H * DH, DM), B_w_r.T, B_w_i.T,
        jnp.asarray(small), jnp.asarray(emat),
    )
    return out.reshape(1, S, DM)
```

```python
import functools
import math

import jax
import jax.numpy as jnp
import numpy as np
from jax import lax
import jax.experimental.pallas as pl
import jax.experimental.pallas.tpu as pltpu

f32, bf16, u32 = jnp.float32, jnp.bfloat16, jnp.uint32

S, DM, H, DH, MEM, SEG = 2048, 640, 32, 128, 8, 32
NPAIR = H // 2
DF = DM // 2 + 1
EPS = 1e-5
WPITCH = 132
HPITCH = 164
ZPITCH = 136

S1 = math.sin(2 * math.pi / 5)
R5_D = (math.cos(2 * math.pi / 5) - math.cos(4 * math.pi / 5)) / 2
R5_R = math.sin(4 * math.pi / 5) / S1


def _to_bf16_bits(a):
    u = np.ascontiguousarray(a, dtype=np.float32).view(np.uint32).astype(np.uint64)
    return ((u + 0x7FFF + ((u >> 16) & 1)) >> 16).astype(np.uint32)


def _pack_rows(a):
    b = _to_bf16_bits(a)
    return b[..., 0::2, :] | (b[..., 1::2, :] << 16)


@functools.lru_cache(maxsize=None)
def _tables():
    b = np.arange(128)
    l0 = np.arange(0, DF, 5)
    l1 = np.concatenate([np.arange(1, 320, 5), np.arange(4, 320, 5)])
    l2 = np.concatenate([np.arange(2, 320, 5), np.arange(3, 320, 5)])
    sg = np.concatenate([np.ones(64), -np.ones(64)])

    def th(l):
        return 2 * np.pi * ((b[:, None] * l[None, :]) % DM) / DM

    sc = 1.0 / (S * DM)
    fw = np.zeros((7, 128, 128))
    iw = np.zeros((7, 128, 128))
    t = th(l0)
    cl = np.full((128, 1), 2.0)
    cl[0] = cl[64] = 1.0
    fw[0] = np.concatenate([np.cos(t), -np.sin(t[:, 1:64])], axis=1)
    iw[0] = cl * sc * fw[0].T
    mu = S1 * sg
    for g, l in ((1, l1), (2, l2)):
        t = th(l)
        c, s = np.cos(t), np.sin(t)
        fw[3 * g - 2:3 * g + 1] = c, -mu * s - c, mu * c - s
        iw[3 * g - 2:3 * g + 1] = [2 * sc * m.T for m in (c, -s - mu * c, mu * s - c)]
    n = np.arange(64)
    order = np.concatenate([np.concatenate([np.arange(8) + 8 * j, np.arange(8) + 8 * j + 64])
                            for j in range(8)])
    e = np.zeros((2, 32, 128, 128))
    for k2 in range(32):
        t = 2 * np.pi * (((32 * n[:, None] + k2) * n[None, :]) % S) / S
        er, ei = np.cos(t), -np.sin(t)
        m = np.block([[er, -ei], [ei, er]])[order][:, order]
        e[0, k2], e[1, k2] = m, m.T
    small = np.concatenate([_pack_rows(fw), _pack_rows(iw)], axis=0)
    return small, _pack_rows(e).reshape(64, 64, 128)


def _loop(name, lo, hi, body, init, **kw):
    with jax.named_scope(name):
        return lax.fori_loop(lo, hi, body, init, **kw)


def _bf(x):
    return pltpu.bitcast(x, bf16)


def _dot(a, b):
    return jnp.dot(a, b, preferred_element_type=f32)


def _round_bf16(x):
    return x.astype(bf16).astype(f32)


def _layernorm(x):
    m = jnp.mean(x, axis=-1, keepdims=True)
    xc = x - m
    v = jnp.mean(xc * xc, axis=-1, keepdims=True)
    return xc * lax.rsqrt(v + EPS)


def _fft4(x, sign):
    (ar, ai), (br, bi), (cr, ci), (dr, di) = x
    t0r, t0i, t1r, t1i = ar + cr, ai + ci, ar - cr, ai - ci
    t2r, t2i, t3r, t3i = br + dr, bi + di, br - dr, bi - di
    y0, y2 = (t0r + t2r, t0i + t2i), (t0r - t2r, t0i - t2i)
    p, q = (t1r + t3i, t1i - t3r), (t1r - t3i, t1i + t3r)
    return [y0, p, y2, q] if sign < 0 else [y0, q, y2, p]


def _twiddle(z, n, period, sign):
    zr, zi = z
    n = n % period
    if n == 0:
        return z
    if 4 * n == period:
        return (-zi, zr) if sign > 0 else (zi, -zr)
    c, s = math.cos(2 * math.pi * n / period), sign * math.sin(2 * math.pi * n / period)
    if (8 * n) % period == 0:
        a, d = zr + zi, zr - zi
        if c * s > 0:
            return (d * c, a * c)
        return (a * c, d * s)
    return (zr * c - zi * s, zr * s + zi * c)


STRASSEN_LHS = (((0, 0, 1), (1, 1, 1)), ((1, 0, 1), (1, 1, 1)), ((0, 0, 1),), ((1, 1, 1),),
                ((0, 0, 1), (0, 1, 1)), ((1, 0, 1), (0, 0, -1)), ((0, 1, 1), (1, 1, -1)))
STRASSEN_RHS = (((0, 0, 1), (1, 1, 1)), ((0, 0, 1),), ((0, 1, 1), (1, 1, -1)), ((1, 0, 1), (0, 0, -1)),
                ((1, 1, 1),), ((0, 0, 1), (0, 1, 1)), ((1, 0, 1), (1, 1, 1)))
STRASSEN_OUT = ((((0, 0), 1), ((1, 1), 1)), (((1, 0), 1), ((1, 1), -1)), (((0, 1), 1), ((1, 1), 1)),
                (((0, 0), 1), ((1, 0), 1)), (((0, 0), -1), ((0, 1), 1)), (((1, 1), 1),), (((0, 0), 1),))
WS_SLOT = {0: 0, 2: 1, 3: 2, 5: 3, 6: 4}


def _operand(terms, block):
    x = block(*terms[0][:2])
    if len(terms) == 1:
        return x
    x, y = x.astype(f32), block(*terms[1][:2]).astype(f32)
    return x + y if terms[1][2] > 0 else x - y


def _accumulate(acc, key, y, sign):
    if key not in acc:
        acc[key] = y if sign > 0 else -y
    else:
        acc[key] = acc[key] + y if sign > 0 else acc[key] - y


def _mu():
    lane = lax.broadcasted_iota(jnp.int32, (1, 128), 1)
    return jnp.where(lane < 64, S1, -S1).astype(f32)


def _ilv(r, i):
    n = r.shape[0] // 8
    return jnp.concatenate([r.reshape(n, 8, 128), i.reshape(n, 8, 128)], axis=1).reshape(16 * n, 128)


def _dilv(x):
    n = x.shape[0] // 16
    x = x.reshape(n, 16, 128)
    return x[:, :8].reshape(8 * n, 128), x[:, 8:].reshape(8 * n, 128)


def _with_tokens(x, toks):
    if not toks:
        return x
    return jnp.concatenate(
        [x[8 * j:8 * j + 8] | toks[j] if j in toks else x[8 * j:8 * j + 8]
         for j in range(x.shape[0] // 8)], axis=0)


def _fft16(x, sign, emit=None):
    cols = [_fft4([x[4 * j + r] for j in range(4)], sign) for r in range(4)]
    out = [None] * 16
    for q in range(4):
        y = _fft4([_twiddle(cols[r][q], r * q, 16, sign) for r in range(4)], sign)
        for p in range(4):
            out[q + 4 * p] = y[p]
        if emit is not None:
            emit(q, y)
    return out


CFG = dict(
    steps=((4.5, 16.5, 6, 4, 0, 8), (5, 16.5, 5, 7, 8, 12), (5, 16.5, 6, 6, 8, 12), (5, 16.5, 8, 7, 8, 0)),
    moves=(((125, 127), (15, 14), (34, 35), (91, 89), (11, 14), (20, 18), (1, 0), (107, 106)),
           ((9, 11), (134, 133), (129, 126), (83, 85)), ((96, 94), (6, 5)), ((33, 34),)),
    pro_inner=(4, 2, 5, 0, 8, 6, 3, 7, 10, 9, 1),
    pro_outer=((2, 0), (1, 2), (0, None), (5, 3), (4, None), (3, 1), (6, None)),
    pro_nre=11, re_pos=(2, 3, 5, 7), ln_at=(23, 27, 27, 27), ln_at2=(3, 4, 6, 8, 8, 13, 13, 13),
    perm_at=tuple(range(4, 28, 2)),
    ws_split=4, ws_at=(15, 15, 16, 16, 17, 18, 18, 19, 20, 20, 21, 21, 22, 23, 23, 24),
    post_passes=((0, 1), (2, 3), (4, 5), (6, 7)), post_dl=20,
    post_order=(0, 1, 6, 3, 4, 2, 8, 5, 7, 9, 10, 11), post_at=(24, 38, 58, 114),
    fwd_at=(7, 8, 9, 10, 12, 13, 14, 16, 17, 18, 20, 21, 22, 24, 25, 26),
    inv_at=tuple(range(28, 44)), inv_lag=4, tok_pos=(4, 5, 6, 7), rel=(0, 1),
    tails_order=((1, 2, 0), 5), out_order=((1, 2, 0), 5),
    two_inner=(2, 5, 8, 4, 0, 1, 3, 6, 7, 9, 10),
    two_outer=((2, 2), (5, 3), (1, None), (0, None), (4, 0), (3, None), (6, 1)),
    dinv_at=(0, 0, 1, 1), dinv_order=(2, 1, 0),
    only=None)


def _step_order(params, moves):
    lat_s, lat_pv, lat_wo, v_delay, n_first, n_last = params
    keyed = []
    for p in range(NPAIR):
        keyed += [(4 * p + 2 * m + e, ("proj", p, m, e)) for m in range(2) for e in range(2)]
        keyed += [(4 * p + 3.5 + v_delay, ("proj", p, 2, e)) for e in range(2)]
    bulk = [x for _, x in sorted(keyed, key=lambda kv: kv[0])]
    first, bulk = bulk[:n_first], bulk[n_first:]
    t, nwo, seq, ready = float(n_first), 0, [], []
    pend = [(t + lat_s, "scores", p) for _, p, m, e in first if m == 1 and e == 1]
    while nwo < H - n_last or pend:
        pend.sort(key=lambda x: (x[0], x[1] == "pv", x[2]))
        if pend and pend[0][0] <= t:
            _, kind, p = pend.pop(0)
            seq.append((kind, p, 0, 0))
            if kind == "scores":
                pend.append((t + lat_pv, "pv", p))
            else:
                ready += [(t + lat_wo, p, e) for e in range(2)]
            t += 0.5
        elif bulk:
            seq.append(bulk.pop(0))
            t += 1
            if seq[-1][2:] == (1, 1):
                pend.append((t + lat_s, "scores", seq[-1][1]))
        elif ready and ready[0][0] <= t and nwo < H - n_last:
            _, p, e = ready.pop(0)
            seq.append(("wo", p, 0, e))
            t += 1
            nwo += 1
        else:
            t += 0.5
    for i, j in moves:
        seq.insert(j, seq.pop(i))
    return first, seq, [2 * p + e for _, p, e in ready]


def _kernel(x_hbm, mem_hbm, wq_hbm, wk_hbm, wv_hbm, wo_hbm, wr_hbm, wi_hbm,
            small_hbm, e_hbm, out_hbm,
            xin, xa, xb, to, raw, wa, wb, wo_t, ws, qb, hl, z0, z1, z2, wf,
            wri, wtmp, small, emat, fill_ref, mem_ref, zero_ref, sem, osem):
    zs = (z0, z1, z2)
    w_hbm = (wq_hbm, wk_hbm, wv_hbm)

    def body_chunk(i):
        return 4 * (i & 3) + (i >> 2)

    def cp_w(i):
        src = w_hbm[i >> 2].at[:, :, pl.ds(8 * (i & 3), 8), :] if isinstance(i, int) else raw.at[i]
        return pltpu.make_async_copy(src, raw.at[i], sem.at[i])

    def cp_x(bb):
        return pltpu.make_async_copy(x_hbm.at[:, bb], xin.at[:, bb], sem.at[12 + bb])

    def cp_f(i):
        src = ((wr_hbm, wi_hbm)[i >> 2].at[:, pl.ds(512 * (i & 3), 512)]
               if isinstance(i, int) else wri.at[i])
        return pltpu.make_async_copy(src, wri.at[i], sem.at[36 + i])

    def cp_wo(i):
        rows = pl.ds(pl.multiple_of(512 * i, 512), 512)
        return [pltpu.make_async_copy(wo_hbm.at[rows, pl.ds(128 * j, 128)], wo_t.at[j, rows], sem.at[28 + i])
                for j in range(4)]

    cp_rest = [pltpu.make_async_copy(mem_hbm, mem_ref, sem.at[46]),
               pltpu.make_async_copy(wo_hbm.at[:, pl.ds(512, 128)], wo_t.at[4, pl.ds(0, H * DH)], sem.at[47]),
               pltpu.make_async_copy(small_hbm, small, sem.at[44]),
               pltpu.make_async_copy(e_hbm, emat, sem.at[45])]

    full = CFG["only"] in (None, "pro")
    for u in range(4 if full else 0):
        cp_x(4 * u + 3).start()
    if full:
        cp_w(0).start()
    for i in range(12 if full else 0):
        if i < 11:
            cp_w(i + 1).start()
        if i >= 1:
            cp_x(body_chunk(i - 1)).start()
        if i == 11:
            cp_x(body_chunk(11)).start()
        if 2 <= i < 10:
            cp_f(i - 2).start()
        if 3 <= i < 11:
            for cp in cp_wo(i - 3):
                cp.start()
    for cp in cp_rest if full else ():
        cp.start()

    zero_ref[0] = 0

    r = lax.broadcasted_iota(jnp.int32, (80, 80), 0)
    c = lax.broadcasted_iota(jnp.int32, (80, 80), 1)

    def head(i):
        return jnp.where(i < 64, i // 32, (i - 64) // 8)

    def pos(i):
        return jnp.where(i < 64, i % 32, 32 + (i - 64) % 8)

    ok = (pos(r) < MEM) | (pos(r) >= pos(c))
    fill_ref[...] = jnp.where(head(r) == head(c), jnp.where(ok, 0.0, -1e9), -jnp.inf).astype(f32)
    wtmp[:, 320:328, :] = jnp.zeros((4, 8, 128), f32)
    xa[32, 0:8, 0:128] = jnp.zeros((8, 128), f32)
    ws[18, 0, 0:16, :] = jnp.zeros((16, 128), bf16)
    wa[12, 0:8, :] = jnp.zeros((8, 128), u32)
    wb[12, 0:8, :] = jnp.zeros((8, 128), u32)
    wf[5, 16 * WPITCH:16 * WPITCH + 8, :] = jnp.zeros((8, 128), f32)
    for z in zs:
        z[0, 0, 128:ZPITCH, :] = jnp.zeros((8, 128), f32)

    def chunk(bb):
        if isinstance(bb, int):
            return slice(8 * bb, 8 * bb + 8)
        return pl.ds(pl.multiple_of(8 * bb, 8), 8)

    def set_input(bb, x, tail_u, a0=0, win=None):
        n = x.shape[0] // 8
        xav = xa if win is None else xa.at[:, win]
        xav[a0:a0 + n, chunk(bb), :] = x.reshape(n, 8, DM)
        y = _layernorm(x)
        if tail_u is None:
            xav[16 + a0:16 + a0 + n, chunk(bb), :] = y.reshape(n, 8, DM)
        else:
            blk = [[y[32 * r:32 * r + 32, 128 * kt:128 * kt + 128] for kt in range(5)] for r in range(4)]
            rows = (slice(16 * tail_u, 16 * tail_u + 16) if isinstance(tail_u, int)
                    else pl.ds(pl.multiple_of(16 * tail_u, 16), 16))
            ops = []
            for outer in STRASSEN_LHS:
                sub = [[_operand(outer, lambda rr, kk: blk[2 * rr + r][2 * kk + k]) for k in range(2)]
                       for r in range(2)]
                ops += [_operand(inner, lambda r, k: sub[r][k]) for inner in STRASSEN_LHS]
            for i, v in enumerate(ops + [blk[r][4] for r in range(4)]):
                hl[i, rows, :] = pltpu.bitcast(v.astype(bf16), u32)

    def load_x(bb, a0=0, n=16):
        return xin[a0:a0 + n, bb].astype(f32).reshape(8 * n, DM)

    def wtile(cid, j, e):
        w = (wa, wb)[e]
        return jnp.concatenate([w[cid, (4 * hf + j) * HPITCH:(4 * hf + j) * HPITCH + 160, :]
                                for hf in range(2)], axis=0)

    def relayout(i, cid, e):
        for r in range(4 * i, 4 * i + 4):
            a, b = [pltpu.bitcast(raw[cid, :, d].reshape(16, 128), u32) for d in (2 * r, 2 * r + 1)]
            v = (a & 0xFFFF) | (b << 16) if e == 0 else (a >> 16) | (b & jnp.uint32(0xFFFF0000))
            (wa, wb)[e][cid, pl.ds(r, 8, stride=HPITCH), :] = v

    def batch_thunks(cid, inner_order, outer_order):
        qv = qb.at[:, :, pl.ds(8 * cid, 8)]

        def unit(e):
            c = {}
            left = {(r, n): (5, 3, 3, 5)[2 * (r >> 1) + (n >> 1)] for r in range(4) for n in range(4)}

            def w(kt, n):
                return _bf(wtile(cid, n, e)[64 * kt:64 * kt + 64])

            def add_out(blk, y, sign):
                _accumulate(c, blk, y, sign)
                left[blk] -= 1
                if left[blk] == 0:
                    r, n = blk
                    y = c.pop(blk).reshape(4, 4, 8, 128)
                    for u in range(4):
                        qv[4 * r:4 * r + 4, u, 2 * n + e] = y[u]

            def outer(io, k4):
                p = {}
                todo = {(0, 0): 4, (0, 1): 2, (1, 0): 2, (1, 1): 4}

                @functools.lru_cache(maxsize=None)
                def sub(k, n):
                    return _operand(STRASSEN_RHS[io], lambda kk, nn: w(2 * kk + k, 2 * nn + n))

                def thunk(items):
                    def run(toks=None):
                        for i in items:
                            if i >= 7:
                                r, n = k4[i - 7]
                                add_out((r, n), _dot(_bf(_with_tokens(hl[49 + r], toks)), w(4, n)), 1)
                                toks = None
                                continue
                            rhs = _operand(STRASSEN_RHS[i], sub).astype(bf16)
                            y = _dot(_bf(_with_tokens(hl[7 * io + i], toks)), rhs)
                            toks = None
                            for blk, sign in STRASSEN_OUT[i]:
                                _accumulate(p, blk, y, sign)
                                todo[blk] -= 1
                                if todo[blk] == 0:
                                    for (rr, nn), sg in STRASSEN_OUT[io]:
                                        add_out((2 * rr + blk[0], 2 * nn + blk[1]), p[blk], sg)
                    return run
                items = [i for i in inner_order if i < 7 + len(k4)]
                return [thunk(items[:len(items) // 2]), thunk(items[len(items) // 2:])]
            out = []
            for io, q in outer_order:
                out += outer(io, [] if q is None else
                             [(2 * (q >> 1) + (j >> 1), 2 * (q & 1) + (j & 1)) for j in range(4)])
            return out
        return unit(0) + unit(1)

    def wperm_thunks(piece, j):
        m = (piece >> 2) & 1
        wt = wtmp.at[j]
        sub = wf.at[pl.ds(3 * m, 3), pl.ds(pl.multiple_of((piece & 3) * 32, 32), 16 * WPITCH - 96)]

        def load():
            wt[0:DF, :] = wri[piece, :, 128 * j:128 * j + 128].astype(f32)

        def one(g):
            def run():
                if g == 0:
                    t = jnp.concatenate([wt[pl.ds(0, 64, stride=5), :], wt[320:328, :],
                                         jnp.zeros((56, 128), f32)], axis=0)
                else:
                    t = jnp.concatenate([wt[pl.ds(g, 64, stride=5), :],
                                         wt[pl.ds(5 - g, 64, stride=5), :]], axis=0)
                y = t.T
                for k in range(8):
                    for hf in range(2):
                        sub[g, pl.ds(8 * j + k + 8 * hf * WPITCH, 8, stride=WPITCH), :] = (
                            y[16 * k + 8 * hf:16 * k + 8 * hf + 8])
            return run
        return [load] + [one(g) for g in range(3)]

    def half_pass(cid, half, fill, zero, timed=()):
        nre = CFG["pro_nre"]
        toks = None
        for k, f in enumerate(batch_thunks(cid, CFG["pro_inner"], CFG["pro_outer"])[14 * half:14 * half + 14]):
            f(toks)
            toks = {}
            for n, f in enumerate(f for at, f in timed if at == k):
                toks[(0, 4, 1, 6)[n]] = f()
            if fill is not None:
                for n, r in enumerate(r for r in range(40) if r * nre // 40 == k):
                    relayout(r, fill, 1 - half)
                    toks[CFG["re_pos"][n]] = (wb, wa)[half][12 + zero, 0:8, :]

    def ln_parts(bb, zero):
        def part(j):
            set_input(bb, load_x(bb, 4 * j, 4), None, 4 * j)
            return pltpu.bitcast(xa[32 + zero, 0:8, 0:128], u32)
        return [functools.partial(part, j) for j in range(4)]

    def perm_parts(piece, nxt, zero):
        def part(fs):
            for f in fs:
                f()
            return pltpu.bitcast(wf[5 + zero, 16 * WPITCH:16 * WPITCH + 8, :], u32)
        out = []
        for j in range(4):
            th = wperm_thunks(piece, j)
            out += [functools.partial(part, th[1:2]), functools.partial(part, th[2:3]),
                    functools.partial(part, th[3:4] + wperm_thunks(nxt, j)[0:1])]
        return out

    def ws_parts(piece, zero):
        nr = 128 // CFG["ws_split"]

        src = wo_t.at[:, pl.ds(pl.multiple_of(512 * piece, 512), 512)]
        dst = ws.at[pl.ds(2 * piece, 2)]

        def part(pp, np_, r0):
            def tile(k, n):
                lo = 256 * pp + 128 * k + r0
                return src[2 * np_ + n, lo:lo + nr, :]
            for i, slot in WS_SLOT.items():
                dst[pp, 5 * np_ + slot, r0:r0 + nr, :] = _operand(STRASSEN_RHS[i], tile).astype(bf16)
            return pltpu.bitcast(ws[18 + zero, 0, 0:16, :], u32)
        return [functools.partial(part, pp, np_, r0)
                for pp in range(2) for np_ in range(2) for r0 in range(0, 128, nr)]

    def pro0():
        def tails(i, carry):
            for u in (2 * i, 2 * i + 1):
                cp_x(4 * u + 3).wait()
            for u in (2 * i, 2 * i + 1):
                set_input(4 * u + 3, load_x(4 * u + 3), u)
            return carry
        lax.fori_loop(0, 2, tails, 0)
        cp_w(0).wait()
        zero = zero_ref[0]
        for i in range(40):
            relayout(i, 0, 0)
        half_pass(0, 0, zero, zero)

    def pro1(it, carry):
        bb = jnp.where(it == 0, 3, body_chunk(it - 1))
        nxt = jnp.where(it >= 2, it - 2, 8)
        with jax.named_scope("pro1_wait"):
            cp_w(it + 1).wait()

            @pl.when(it >= 1)
            def _():
                cp_x(bb).wait()

            @pl.when(nxt < 8)
            def _():
                cp_f(nxt).wait()

            @pl.when(it >= 3)
            def _():
                for cp in cp_wo(it - 3):
                    cp.wait()
        piece = jnp.where(it >= 3, it - 3, 8)
        zero = it >> 4
        timed = sorted(list(zip(CFG["ln_at"], ln_parts(bb, zero)))
                       + list(zip(CFG["ws_at"], ws_parts(piece, zero)))
                       + list(zip(CFG["perm_at"], perm_parts(piece, nxt, zero))), key=lambda x: x[0])
        half_pass(it, 1, it + 1, zero, [x for x in timed if x[0] < 14])
        half_pass(it + 1, 0, it + 1, zero, [(k - 14, f) for k, f in timed if k >= 14])
        return carry

    def pro2():
        cp_x(body_chunk(10)).wait()
        cp_x(body_chunk(11)).wait()
        zero = zero_ref[0]
        half_pass(11, 1, None, zero, list(zip(
            CFG["ln_at2"], ln_parts(body_chunk(10), zero) + ln_parts(body_chunk(11), zero))))

    if full:
        with jax.named_scope("pro0"):
            pro0()
        _loop("pro1", 0, 11, pro1, 0)
        with jax.named_scope("pro2"):
            pro2()
        for cp in cp_rest[:2]:
            cp.wait()

    scale = DH ** -0.5

    def wo_dot(hh, oo):
        return [_dot(oo, wo_t[j, 128 * hh:128 * hh + 128, :]) for j in range(5)]

    def addl(acc, res):
        return res if acc is None else [a + b for a, b in zip(acc, res)]

    def group(g, mem):
        for ph in range(4):
            h = jnp.concatenate([mem, xa[16 + g, 32 * ph:32 * ph + 24, :]], axis=0).astype(bf16)
            pr, sm, oos = {}, {}, {}

            def stacked(p, m):
                tails = [qb[g, ph, 32 * m + 2 * p + e] for e in range(2)]
                return jnp.concatenate([pr[p, m, 0], pr[p, m, 1]] + tails, axis=0).astype(bf16)

            def scores(p):
                sc = lax.dot_general(stacked(p, 0), stacked(p, 1), (((1,), (1,)), ((), ())),
                                     preferred_element_type=f32)
                fill = fill_ref[...]
                sc = jnp.where(fill == 0.0, sc * scale, fill)
                mx = jnp.max(sc, axis=-1, keepdims=True)
                e = jnp.exp(sc - mx)
                rl = pl.reciprocal(jnp.sum(e, axis=-1, keepdims=True), approx=True)
                sm[p] = (e * rl).astype(bf16)

            def pv(p):
                o = _dot(sm[p], stacked(p, 2))
                for e in range(2):
                    qb[g, ph, 2 * p + e] = o[64 + 8 * e:72 + 8 * e]
                    oos[2 * p + e] = o[32 * e:32 * e + 32].astype(bf16)

            first, seq, last = _step_order(CFG["steps"][ph], CFG["moves"][ph])
            for kt in range(5):
                for _, p, m, e in first:
                    w = wtile(4 * m + (p >> 2), p & 3, e)[64 * kt:64 * kt + 64]
                    y = _dot(h[:, 128 * kt:128 * kt + 128], _bf(w))
                    pr[p, m, e] = y if kt == 0 else pr[p, m, e] + y
            acc = None
            for kind, p, m, e in seq:
                if kind == "proj":
                    pr[p, m, e] = _dot(h, _bf(wtile(4 * m + (p >> 2), p & 3, e)))
                elif kind == "scores":
                    scores(p)
                elif kind == "pv":
                    pv(p)
                else:
                    acc = addl(acc, wo_dot(2 * p + e, oos[2 * p + e]))
            for j in range(5):
                for hh in last:
                    acc[j] = acc[j] + _dot(oos[hh], wo_t[j, 128 * hh:128 * hh + 128, :])
            out = jnp.concatenate(acc, axis=1)
            xa[16 + g, 32 * ph:32 * ph + 24, :] = out[8:32]
            mem = _round_bf16(out[0:8])
        return mem

    def dfwd_thunks(seg, q):
        st = {}
        rows = chunk(q)
        xav, xbv, zv = xa.at[:, seg], xb.at[:, seg], [z.at[:, :, seg] for z in zs]

        def pre():
            o = to[...] if q == 3 else xav[16:32, rows, :]
            x = _round_bf16(xav[0:16, rows, :] + o)
            xbv[:, rows, :] = x
            y = _layernorm(x.reshape(128, DM))
            x0, x1, x2, x3, x4 = [y[:, 128 * a:128 * a + 128] for a in range(5)]
            t1, t2, t3, t4 = x1 + x4, x2 + x3, x1 - x4, x2 - x3
            t = t1 + t2
            m, n = x0 - 0.25 * t, R5_D * (t1 - t2)
            st["u"] = [x0 + t, (m + n, t3 + R5_R * t4), (m - n, R5_R * t3 - t4)]

        def part(g):
            def run():
                if g == 0:
                    pre()
                    u0 = st["u"][0].astype(bf16)
                    zr = _dot(u0, _bf(small[0]))
                    lane = lax.broadcasted_iota(jnp.int32, (128, 128), 1)
                    zi = jnp.where((lane & 63) == 0, 0.0, pltpu.roll(zr, 64, 1))
                else:
                    a, b = st["u"][g]
                    k, kb, ka = [_dot(v.astype(bf16), _bf(small[3 * g - 2 + i]))
                                 for i, v in enumerate((a + b, b, a))]
                    zr, zi = k + kb, ka - _mu() * k
                ys = [(zr[8 * a:8 * a + 8], zi[8 * a:8 * a + 8]) for a in range(16)]
                if g < 2:
                    ys = _fft16(ys, -1)
                for a in range(16):
                    zv[g][0, a, rows, :] = ys[a][0]
                    zv[g][1, a, rows, :] = ys[a][1]
            return run
        return [part(g) for g in range(3)]

    def post(u, carry):
        base = pl.multiple_of(32 * u, 32)
        side = []
        for q in range(4):
            side += dfwd_thunks(pl.ds(base, 32), q)
        side = [side[i] for i in CFG["post_order"]]
        k = 0
        at = list(CFG["post_at"])
        m, due = {}, []
        for prods in CFG["post_passes"]:
            acc = None
            for p in range(NPAIR):
                res = []
                for i in prods:
                    if i == 7:
                        oo = jnp.concatenate([qb[:, u, 2 * p + e].reshape(128, 128) for e in range(2)], axis=1)
                        res.append(_dot(oo.astype(bf16), wo_t[4, 256 * p:256 * p + 256, :]))
                        k += 2
                        continue
                    a = _operand(STRASSEN_LHS[i], lambda r, e: (
                        qb[8 * r:8 * r + 8, u, 2 * p + e].reshape(64, 128))).astype(bf16)
                    for np_ in range(2):
                        if i in WS_SLOT:
                            w = ws[p, 5 * np_ + WS_SLOT[i]]
                        else:
                            kk = 0 if i == 1 else 1
                            w = wo_t[2 * np_ + kk, 256 * p + 128 * kk:256 * p + 128 * kk + 128, :]
                        if due and due[0][0] <= k:
                            w = _bf(_with_tokens(pltpu.bitcast(w, u32), {0: due.pop(0)[1]}))
                        res.append(_dot(a, w))
                    k += 1
                acc = addl(acc, res)
                while at and at[0] <= k:
                    g = CFG["post_order"][len(CFG["post_at"]) - len(at)] % 3
                    at.pop(0)
                    side.pop(0)()
                    if g == 0:
                        due.append((k + CFG["post_dl"],
                                    pltpu.bitcast(z0[0, u >> 2, 128:ZPITCH, :], u32)))
            for i in prods:
                m[i] = [acc.pop(0)] if i == 7 else [acc.pop(0), acc.pop(0)]
        cols = []
        for np_ in range(2):
            m1, m2, m3, m4, m5, m6, m7 = [m[i][np_] for i in range(7)]
            cols.append(jnp.concatenate([m1 + m4 - m5 + m7, m2 + m4], axis=0))
            cols.append(jnp.concatenate([m3 + m5, m1 - m2 + m3 + m6], axis=0))
        to[...] = jnp.concatenate(cols + m[7], axis=1).reshape(16, 8, DM)
        for f in side:
            f()
        return carry

    def spectral(zero):
        def fence(z):
            return z[0, zero, 128:ZPITCH, :]

        def radix(g, bb, sign):
            z = zs[g]
            toks = []

            def emit(q, y):
                for p in range(4):
                    z[0, q + 4 * p, chunk(bb), :] = y[p][0]
                    z[1, q + 4 * p, chunk(bb), :] = y[p][1]
                toks.append(fence(z))
            _fft16([(z[0, a, chunk(bb), :], z[1, a, chunk(bb), :]) for a in range(16)], sign, emit)
            return toks

        ys = {}

        def fwd(g, k2, toks):
            z = zs[g]
            ur, ui = z[0, k2, 0:64, :], z[1, k2, 0:64, :]
            tr, ti = _twiddle((z[0, k2, 64:128, :], z[1, k2, 64:128, :]), k2, 32, -1)
            for hf in range(2):
                v = _ilv(ur + tr, ui + ti) if hf == 0 else _ilv(ur - tr, ui - ti)
                lhs = _with_tokens(emat[k2 + 16 * hf], toks if hf == 0 else None)
                xr, xi = _dilv(_dot(_bf(lhs), v.astype(bf16)))
                ys["x", 16 * g + k2] = xr
                wr = wf[g, pl.ds(k2 * WPITCH + hf, 64, stride=2), :]
                wi = wf[g + 3, pl.ds(k2 * WPITCH + hf, 64, stride=2), :]
                ys[g, k2, hf] = _ilv(xr * wr - xi * wi, xr * wi + xi * wr).astype(bf16)

        def inv(g, k2, toks):
            z = zs[g]
            t0 = _dot(_bf(_with_tokens(emat[32 + k2], toks)), ys.pop((g, k2, 0)))
            t1 = _dot(_bf(emat[48 + k2]), ys.pop((g, k2, 1)))
            z[0, k2, 0:64, :], z[1, k2, 0:64, :] = _dilv(t0 + t1)
            z[0, k2, 64:128, :], z[1, k2, 64:128, :] = _twiddle(_dilv(t0 - t1), k2, 32, 1)

        units = [(g, k2) for g in range(3) for k2 in range(16)]
        toks = None
        lag = CFG["inv_lag"]
        for i in range(len(units) + lag):
            if i < len(units):
                fwd(*units[i], toks)
            if i >= lag:
                inv(*units[i - lag], toks if i >= len(units) else None)
            toks = []
            if i in CFG["fwd_at"]:
                toks = radix(2, CFG["fwd_at"].index(i), -1)
            if i in CFG["inv_at"]:
                back, r = CFG["rel"]
                z0[1, zero, 128:ZPITCH, :] = ys["x", min(i - back, 47)][8 * r:8 * r + 8]
                toks = radix(0, CFG["inv_at"].index(i), 1)
            toks = {j: pltpu.bitcast(t, u32) for j, t in zip(CFG["tok_pos"], toks)}

    def dinv_thunks(bb, finish, win=None):
        st = {}
        xbv = xb if win is None else xb.at[:, win]

        def part(g):
            def run():
                z = zs[g] if win is None else zs[g].at[:, :, win]
                ys = [(z[0, a, chunk(bb), :], z[1, a, chunk(bb), :]) for a in range(16)]
                if g > 0:
                    ys = _fft16(ys, 1)
                tr = jnp.concatenate([y[0] for y in ys], axis=0)
                ti = jnp.concatenate([y[1] for y in ys], axis=0)
                if g == 0:
                    lane = lax.broadcasted_iota(jnp.int32, (128, 128), 1)
                    v = jnp.where(lane <= 64, tr, pltpu.roll(ti, 64, 1))
                    st[0] = _dot(v.astype(bf16), _bf(small[7]))
                else:
                    k, ki, kr = [_dot(v.astype(bf16), _bf(small[5 + 3 * g + i]))
                                 for i, v in enumerate((tr + _mu() * ti, ti, tr))]
                    st[2 * g - 1], st[2 * g] = k + ki, k + kr
            return run

        def fin():
            p0, p1, q1, p2, q2 = [st[j] for j in range(5)]
            t = p1 + p2
            m, n = p0 - 0.25 * t, R5_D * (p1 - p2)
            e1, e2 = m + n, m - n
            o1, o2 = q1 + R5_R * q2, R5_R * q1 - q2
            y = jnp.concatenate([p0 + t, e1 - o1, e2 - o2, e2 + o2, e1 + o1], axis=1)
            finish(xbv[:, chunk(bb), :].reshape(128, DM) + y)
        return [part(0), part(1), part(2), fin]

    def out_copy(bb):
        return pltpu.make_async_copy(xin.at[:, bb], out_hbm.at[:, bb], osem.at[bb])

    def layer(li, carry0):
        if full or CFG["only"] == "group":
            _loop("step", 0, 16, group, mem_ref[...].astype(f32))
        if full or CFG["only"] == "spec":
            if full:
                @pl.when(li == 0)
                def _():
                    for cp in cp_rest[2:]:
                        cp.wait()
            _loop("post", 0, 4, post, 0)

            with jax.named_scope("spectral"):
                spectral(li >> 1)
        if not full and CFG["only"] != "out":
            return carry0

        def run_chunks(th, order, lag):
            seq = [t[g] for t in th for g in order]
            for i in range(len(seq) + lag):
                if i < len(seq):
                    seq[i]()
                if i >= lag and (i - lag) % 3 == 2:
                    th[(i - lag) // 3][3]()

        @pl.when(li == 0)
        def _():
            with jax.named_scope("dinv_tails"):
                run_chunks([dinv_thunks(4 * u + 3, functools.partial(
                    lambda u, x: set_input(4 * u + 3, _round_bf16(x), u), u))
                    for u in range(4)],
                    *CFG["tails_order"])

            def batch(u, carry):
                win = pl.ds(pl.multiple_of(32 * u, 32), 32)
                for q in range(3):
                    side = dinv_thunks(q, functools.partial(
                        lambda q, x: set_input(q, _round_bf16(x), None, win=win), q), win)
                    for k, f in enumerate(batch_thunks(3 * u + q, CFG["two_inner"], CFG["two_outer"])):
                        f()
                        for at, g in zip(CFG["dinv_at"], CFG["dinv_order"] + (3,)):
                            if at == k:
                                side[g]()
                return carry
            _loop("batch", 0, 4, batch, 0)

        @pl.when(li == 1)
        def _():
            def out_half(hf, carry):
                xv = xin.at[:, pl.ds(8 * hf, 8)]

                def store_out(q, x):
                    xv[:, q] = x.reshape(16, 8, DM).astype(bf16)
                    out_copy(8 * hf + q).start()
                win = pl.ds(pl.multiple_of(64 * hf, 64), 64)
                run_chunks([dinv_thunks(q, functools.partial(store_out, q), win) for q in range(8)],
                           *CFG["out_order"])
                return carry
            with jax.named_scope("dinv_out"):
                lax.fori_loop(0, 2, out_half, 0)
                for bb in range(16):
                    out_copy(bb).wait()
        return carry0

    if CFG["only"] != "pro":
        lax.fori_loop(0, 2, layer, 0)
    if CFG["only"] in ("pro", "out"):
        zero = zero_ref[0]
        xin[0, 0, :, 0:128] = (qb[zero, 0, 0] + wf[zero, 0:8, :] + xa[zero, 0:8, 0:128]).astype(bf16) + ws[zero, 0, 0:8, :]
        out_copy(0).start()
        out_copy(0).wait()
        for cp in cp_rest[2:] if full else ():
            cp.wait()


@jax.jit
def pallas_interleave_layers__memory_aug_recurrent_mem_tr__spectral_gfnet__prompt_kernel(
    A_x, A_mem0, A_Wq, A_Wk, A_Wv, A_Wo, A_seg_len, B_x, B_w_r, B_w_i,
):
    assert A_x.shape == (1, S, DM) and A_mem0.shape == (1, MEM, DM)
    small, emat = _tables()
    hbm = pl.BlockSpec(memory_space=pltpu.HBM)
    out = pl.pallas_call(
        _kernel,
        out_shape=jax.ShapeDtypeStruct((16, 16, 8, DM), bf16),
        in_specs=[hbm] * 10,
        out_specs=hbm,
        scratch_shapes=[
            pltpu.VMEM((16, 16, 8, DM), bf16),
            pltpu.VMEM((33, 128, DM), f32),
            pltpu.VMEM((16, 128, DM), f32),
            pltpu.VMEM((16, 8, DM), f32),
            pltpu.VMEM((12, 2, 320, 8, DH), bf16),
            pltpu.VMEM((13, 8 * HPITCH, 128), u32),
            pltpu.VMEM((13, 8 * HPITCH, 128), u32),
            pltpu.VMEM((5, H * DH + 512, 128), bf16),
            pltpu.VMEM((19, 10, 128, 128), bf16),
            pltpu.VMEM((16, 4, 96, 8, 128), f32),
            pltpu.VMEM((53, 64, 128), u32),
            pltpu.VMEM((2, 16, ZPITCH, 128), f32),
            pltpu.VMEM((2, 16, ZPITCH, 128), f32),
            pltpu.VMEM((2, 16, ZPITCH, 128), f32),
            pltpu.VMEM((6, 16 * WPITCH + 32, 128), f32),
            pltpu.VMEM((9, DF, 512), bf16),
            pltpu.VMEM((4, 328, 128), f32),
            pltpu.VMEM((14, 64, 128), u32),
            pltpu.VMEM((64, 64, 128), u32),
            pltpu.VMEM((80, 80), f32),
            pltpu.VMEM((MEM, DM), bf16),
            pltpu.SMEM((1,), jnp.int32),
            pltpu.SemaphoreType.DMA((48,)),
            pltpu.SemaphoreType.DMA((16,)),
        ],
        compiler_params=pltpu.CompilerParams(vmem_limit_bytes=120 * 1024 * 1024,
                                             disable_semaphore_checks=True),
    )(
        A_x.reshape(16, 16, 8, DM), A_mem0.reshape(MEM, DM),
        *[w.reshape(2, 320, H, DH) for w in (A_Wq, A_Wk, A_Wv)], A_Wo.reshape(H * DH, DM), B_w_r.T, B_w_i.T,
        jnp.asarray(small), jnp.asarray(emat),
    )
    return out.reshape(1, S, DM)
```
